```python
import jax
import jax.numpy as jnp

def _softmax(x, axis=-1):
    return jax.nn.softmax(x, axis=axis)

def _gelu(x):
    return jax.nn.gelu(x, approximate=True)

def _silu(x):
    return jax.nn.silu(x)

def _sigmoid(x):
    return jax.nn.sigmoid(x)

def _layernorm(x, axis=-1, eps=1e-05):
    m = jnp.mean(x, axis=axis, keepdims=True)
    v = jnp.var(x, axis=axis, keepdims=True)
    return (x - m) / jnp.sqrt(v + eps)

def _scatter_add(tgt, idx, src, axis=0):
    return tgt.at[idx].add(src)

def _segment_sum(src, seg, n):
    return jax.ops.segment_sum(src, seg, n)

class _Rng:

    def __init__(self, key):
        self._k = key

    def _next(self):
        self._k, sub = jax.random.split(self._k)
        return sub

    def normal(self, shape):
        return jax.random.normal(self._next(), shape, dtype=jnp.bfloat16)

    def randint(self, lo, hi, shape):
        return jax.random.randint(self._next(), shape, lo, hi, dtype=jnp.int32)

    def uniform(self, shape, lo=0.0, hi=1.0):
        return jax.random.uniform(self._next(), shape, jnp.bfloat16, lo, hi)

    def permutation(self, n):
        return jax.random.permutation(self._next(), n)
kernel_name = 'adaLN_cond__ssm_conv_h3__mixer_s_mlp__prompt'

def setup_inputs():
    _rng = _Rng(jax.random.key(int.from_bytes(__import__("os").urandom(4), "little")))
    _w = lambda a: (lambda t: t.astype(jnp.bfloat16) if jnp.issubdtype(t.dtype, jnp.floating) else t)(jnp.asarray(a))

    def _A_setup():
        B, S, D = (1, 2048, 640)
        ks = 4
        return {'q': _w((lambda *s: _rng.normal(s) * 0.05)(B, S, D)), 'k': _w((lambda *s: _rng.normal(s) * 0.05)(B, S, D)), 'v': _w((lambda *s: _rng.normal(s) * 0.05)(B, S, D)), 'shift_k': _w((lambda *s: _rng.normal(s) * 0.05)(D, ks) * 0.5), 'ssm_k': _w((lambda *s: _rng.normal(s) * 0.05)(D, S) * (1.0 / S ** 0.5)), 'ssm_D': _w((lambda *s: _rng.normal(s) * 0.05)(D))}
    _A_in = _A_setup()

    def _B_setup():
        B, S, D, F = (1, 2048, 640, 1728)
        return {'x': _w((lambda *s: _rng.normal(s) * 0.05)(B, S, D)), 'w1': _w((lambda *s: _rng.normal(s) * 0.05)(D, D) * D ** (-0.5)), 'w2': _w((lambda *s: _rng.normal(s) * 0.05)(D, D) * D ** (-0.5)), 'w3': _w((lambda *s: _rng.normal(s) * 0.05)(D, F) * D ** (-0.5)), 'w4': _w((lambda *s: _rng.normal(s) * 0.05)(F, D) * F ** (-0.5))}
    _B_in = _B_setup()
    return {'A_q': _A_in['q'], 'A_k': _A_in['k'], 'A_v': _A_in['v'], 'A_shift_k': _A_in['shift_k'], 'A_ssm_k': _A_in['ssm_k'], 'A_ssm_D': _A_in['ssm_D'], 'B_x': _B_in['x'], 'B_w1': _B_in['w1'], 'B_w2': _B_in['w2'], 'B_w3': _B_in['w3'], 'B_w4': _B_in['w4'], 'c': _w((lambda *s: _rng.normal(s) * 0.05)(1, 640)), 'w_mod': _w((lambda *s: _rng.normal(s) * 0.05)(640, 6 * 640) * 640 ** (-0.5))}

def reference(A_q, A_k, A_v, A_shift_k, A_ssm_k, A_ssm_D, B_x, B_w1, B_w2, B_w3, B_w4, c, w_mod):

    def _A_ref(q, k, v, shift_k, ssm_k, ssm_D):
        B, S, D = q.shape
        ks = shift_k.shape[-1]
        k_pad = jnp.pad(k, ((0, 0), (ks - 1, 0), (0, 0)))
        k_shift = jnp.zeros_like(k)
        for t in range(ks):
            k_shift = k_shift + k_pad[:, t:t + S, :] * shift_k[:, ks - 1 - t][None, None, :]
        kv = k_shift * v
        L = 2 * S
        kv_pad = jnp.pad(kv, ((0, 0), (0, S), (0, 0)))
        kf_pad = jnp.pad(ssm_k, ((0, 0), (0, S)))
        kv_f = (lambda x, axes=(-2, -1): jnp.fft.rfft2(x.astype(jnp.float32), axes=axes))(kv_pad[:, None, :, :], axes=(1, 2))
        kf_f = (lambda x, axes=(-2, -1): jnp.fft.rfft2(x.astype(jnp.float32), axes=axes))(kf_pad[:, None, :], axes=(1, 2))
        kf_f = (lambda x, *d: x.transpose(*d))(kf_f, 1, 2, 0)
        y_f = kv_f * kf_f[None, :, :, :]
        y = (lambda x, s, axes=(-2, -1): jnp.fft.irfft2(x, s=s, axes=axes).astype(jnp.bfloat16))(y_f, (1, L), axes=(1, 2))[:, 0, :S, :]
        y = y + kv * ssm_D[None, None, :]
        return q * y

    def _B_ref(x, w1, w2, w3, w4):
        B, S, D = x.shape
        h = _gelu(_layernorm(x, axis=-1) @ w1)
        c = D // 4
        g0 = jnp.pad(h[:, :, 0 * c:1 * c], ((0, 0), (1, 0), (0, 0)))[:, :S, :]
        g1 = jnp.pad(h[:, :, 1 * c:2 * c], ((0, 0), (0, 1), (0, 0)))[:, 1:, :]
        g2 = jnp.pad(h[:, :, 2 * c:3 * c], ((0, 0), (2, 0), (0, 0)))[:, :S, :]
        g3 = jnp.pad(h[:, :, 3 * c:], ((0, 0), (0, 2), (0, 0)))[:, 2:, :]
        hs = jnp.concatenate([g0, g1, g2, g3], axis=-1) @ w2
        x1 = x + hs
        h2 = _gelu(_layernorm(x1, axis=-1) @ w3) @ w4
        return x1 + h2
    x = A_q
    mod = (_silu(c) @ w_mod).reshape(c.shape[0], 6, 1, -1)
    sa, ca, ga, sb, cb, gb = (mod[:, 0].copy(), mod[:, 1].copy(), mod[:, 2].copy(), mod[:, 3].copy(), mod[:, 4].copy(), mod[:, 5].copy())
    h = _layernorm(x, axis=-1) * (1 + ca) + sa
    x = x + ga * _A_ref(h, A_k, A_v, A_shift_k, A_ssm_k, A_ssm_D)
    h = _layernorm(x, axis=-1) * (1 + cb) + sb
    x = x + gb * _B_ref(h, B_w1, B_w2, B_w3, B_w4)
    return x
```

```python
import functools
import math

import numpy as np
import jax
import jax.numpy as jnp
from jax import lax
import jax.experimental.pallas as pl
import jax.experimental.pallas.tpu as pltpu

F32 = jnp.float32
BF16 = jnp.bfloat16

LANES = 128
BLK = 128
EPS = 1e-05


def _dft_tables():
    p = np.arange(BLK)[:, None]
    n = np.arange(BLK)[None, :]
    ang = 2.0 * np.pi * (((4 * p + 1) * n) % (4 * BLK)) / (4 * BLK)
    re = np.cos(ang).reshape(BLK // 8, 8, BLK)
    im = (-np.sin(ang)).reshape(BLK // 8, 8, BLK)
    fwd = np.concatenate([re, im], axis=1).reshape(2 * BLK, BLK)
    inv = fwd.T / BLK
    return fwd.astype(np.float32), np.ascontiguousarray(inv).astype(np.float32)


def _ln(x):
    m = jnp.mean(x, axis=-1, keepdims=True)
    d = x - m
    v = jnp.mean(d * d, axis=-1, keepdims=True)
    return d * lax.rsqrt(v + EPS)


def _gelu(x):
    c0 = math.sqrt(2.0 / math.pi)
    t = jnp.tanh(x * (c0 + (c0 * 0.044715) * (x * x)))
    hx = 0.5 * x
    return hx + hx * t


def _dot(a, b):
    return jnp.dot(a, b, preferred_element_type=F32)


def _dot_nt(a, b):
    return lax.dot_general(a, b, (((1,), (1,)), ((), ())), preferred_element_type=F32)


def _kernel(q_hbm, k_hbm, v_hbm, sh_hbm, sk_hbm, sd_hbm, w1_hbm, w2_hbm, w3_hbm, w4_hbm,
            c_hbm, wm_hbm, fw_hbm, iv_hbm,
            o_hbm,
            q_v, k_v, v_v, sh_v, sk_v, sd_v, w1_v, w2_v, w3_v, w4_v, c_v, wm_v, fw_v, iv_v,
            o_v, kf_s, u_s, kk_s, yy_s, y_s, mod_s, par_s, h1_s, x_s, h_s, z_s,
            sem_small, sem_conv, sem_wm, sem_w, sem_q, sem_o,
            *, S, D, FF, TA, TB):
    NC = D // LANES
    NB = S // BLK
    NG = BLK // 8
    HALO = 16

    small = [
        pltpu.make_async_copy(fw_hbm, fw_v, sem_small.at[0]),
        pltpu.make_async_copy(sh_hbm, sh_v, sem_small.at[1]),
        pltpu.make_async_copy(sd_hbm, sd_v, sem_small.at[2]),
        pltpu.make_async_copy(iv_hbm, iv_v, sem_small.at[3]),
        pltpu.make_async_copy(c_hbm, c_v, sem_small.at[4]),
    ]

    def conv_copies(c):
        col = pl.ds(pl.multiple_of(c * LANES, LANES), LANES)
        return [
            pltpu.make_async_copy(sk_hbm.at[col, :], sk_v.at[c], sem_conv.at[0, c]),
            pltpu.make_async_copy(k_hbm.at[:, col], k_v.at[c], sem_conv.at[1, c]),
            pltpu.make_async_copy(v_hbm.at[:, col], v_v.at[c], sem_conv.at[2, c]),
        ]

    def wm_copy(j):
        col = pl.ds(pl.multiple_of(j * D, LANES), D)
        return pltpu.make_async_copy(wm_hbm.at[:, col], wm_v.at[j], sem_wm.at[j])

    w_copies = [
        pltpu.make_async_copy(w1_hbm, w1_v, sem_w.at[0]),
        pltpu.make_async_copy(w2_hbm, w2_v, sem_w.at[1]),
        pltpu.make_async_copy(w3_hbm, w3_v, sem_w.at[2]),
        pltpu.make_async_copy(w4_hbm, w4_v, sem_w.at[3]),
    ]
    q_copy = pltpu.make_async_copy(q_hbm, q_v, sem_q.at[0])

    for cp in small:
        cp.start()
    for cp in conv_copies(0):
        cp.start()

    kf_s[0:8, :] = jnp.zeros((8, LANES), F32)
    for c in range(NC):
        h1_s[c, 0:8, :] = jnp.zeros((8, LANES), F32)
        h1_s[c, S + 8:S + 16, :] = jnp.zeros((8, LANES), F32)

    for cp in small:
        cp.wait()
    shf = sh_v[...].astype(F32)
    sdf = sd_v[...].astype(F32).reshape(1, D)
    for c in range(NC):
        par_s[c, 0:4, :] = shf[:, c * LANES:(c + 1) * LANES]
        par_s[c, 4:5, :] = sdf[:, c * LANES:(c + 1) * LANES]
    cf = c_v[...].astype(F32)
    sc = (cf * jax.nn.sigmoid(cf)).astype(BF16)
    sc16 = jnp.broadcast_to(sc, (16, D))

    def mod_chunk(j):
        wm_copy(j).wait()
        mod_s[j] = _dot(sc16, wm_v[j])[0:8, :]

    def conv_tile(c, carry):
        @pl.when(c + 1 < NC)
        def _():
            for cp in conv_copies(c + 1):
                cp.start()
        wm_copy(c).start()

        @pl.when(c == NC - 1)
        def _():
            q_copy.start()
            w_copies[0].start()
            w_copies[1].start()

        @pl.when(c > 0)
        def _():
            mod_chunk(c - 1)

        for cp in conv_copies(c):
            cp.wait()

        fw = fw_v[...]
        par = par_s[c]
        w = [par[t:t + 1, :] for t in range(4)]
        dd = par[4:5, :]
        for j in range(NB):
            kk_s[j] = _dot_nt(fw, sk_v[c, :, j * BLK:(j + 1) * BLK])
        for i in range(NB):
            kf_s[8 + i * BLK:8 + (i + 1) * BLK, :] = k_v[c, i * BLK:(i + 1) * BLK, :].astype(F32)
        for i in range(NB):
            base = 8 + i * BLK
            ks = kf_s[base:base + BLK, :] * w[0]
            for t in range(1, 4):
                ks = ks + kf_s[base - t:base - t + BLK, :] * w[t]
            kv = ks * v_v[c, i * BLK:(i + 1) * BLK, :].astype(F32)
            u_s[i] = _dot(fw, kv.astype(BF16))

        def group(g, carry2):
            r0 = pl.multiple_of(g * 16, 16)
            rre = pl.ds(r0, 8)
            rim = pl.ds(r0 + 8, 8)
            a = [u_s[i, rre, :] for i in range(NB)]
            b = [u_s[i, rim, :] for i in range(NB)]
            kr = [kk_s[j, rre, :] for j in range(NB)]
            ki = [kk_s[j, rim, :] for j in range(NB)]
            cc = [kr[0] + dd] + [kr[j] - ki[j - 1] for j in range(1, NB)]
            dm = [ki[0]] + [ki[j] + kr[j - 1] for j in range(1, NB)]
            gg = [dm[j] - cc[j] for j in range(NB)]
            ee = [dm[j] + cc[j] for j in range(NB)]
            ss = [a[i] + b[i] for i in range(NB)]
            for o in range(NB):
                p1 = cc[o] * ss[0]
                for i in range(1, o + 1):
                    p1 = p1 + cc[o - i] * ss[i]
                re = p1
                im = p1
                for i in range(o + 1):
                    re = re - ee[o - i] * b[i]
                    im = im + gg[o - i] * a[i]
                yy_s[o, pl.ds(r0, 16), :] = jnp.concatenate([re, im], axis=0).astype(BF16)
            return carry2

        lax.fori_loop(0, NG, group, 0, unroll=True)

        iv = iv_v[...]
        for o in range(NB):
            y_s[c, o * BLK:(o + 1) * BLK, :] = _dot(iv, yy_s[o])
        return carry

    lax.fori_loop(0, NC, conv_tile, 0)
    w_copies[2].start()
    w_copies[3].start()
    wm_copy(NC).start()
    mod_chunk(NC - 1)

    sa = mod_s[0, 0:1, :]
    ca = mod_s[1, 0:1, :]
    ga = mod_s[2, 0:1, :]
    sb = mod_s[3, 0:1, :]
    cb = mod_s[4, 0:1, :]
    a_mul = ga * (1.0 + ca)
    a_add = ga * sa
    b_mul = 1.0 + cb

    def stage_a(r0, n):
        rows = pl.ds(r0, n)
        q = q_v[rows, :].astype(F32)
        y = jnp.concatenate([y_s[c, rows, :] for c in range(NC)], axis=1)
        x = q + (_ln(q) * a_mul + a_add) * y
        h = _ln(x) * b_mul + sb
        g1 = _gelu(_dot(_ln(h).astype(BF16), w1_v[...]))
        x_s[rows, :] = x
        h_s[rows, :] = h
        for c in range(NC):
            h1_s[c, pl.ds(r0 + 8, n), :] = g1[:, c * LANES:(c + 1) * LANES]

    grp = D // 4
    shifts = (-1, 1, -2, 2)

    def stage_w2(r0, n):
        lane = lax.broadcasted_iota(jnp.int32, (n, LANES), 1)
        parts = []
        for c in range(NC):
            lo, hi = c * LANES, (c + 1) * LANES
            g_lo, g_hi = lo // grp, (hi - 1) // grp
            val = h1_s[c, pl.ds(r0 + 8 + shifts[g_lo], n), :]
            if g_hi != g_lo:
                other = h1_s[c, pl.ds(r0 + 8 + shifts[g_hi], n), :]
                val = jnp.where(lane < (g_hi * grp - lo), val, other)
            parts.append(val.astype(BF16))
        hs = _dot(jnp.concatenate(parts, axis=1), w2_v[...])
        rows = pl.ds(r0, n)
        x1 = h_s[rows, :] + hs
        z_s[rows, :] = _ln(x1).astype(BF16)
        h_s[rows, :] = x1

    q_copy.wait()
    w_copies[0].wait()
    stage_a(0, TA + HALO)
    w_copies[1].wait()

    def loop_a(t, carry):
        stage_w2(pl.multiple_of(t * TA, TA), TA)
        stage_a(pl.multiple_of((t + 1) * TA + HALO, HALO), TA)
        return carry

    NA = S // TA
    lax.fori_loop(0, NA - 2, loop_a, 0)
    stage_w2((NA - 2) * TA, TA)
    stage_a((NA - 1) * TA + HALO, TA - HALO)
    stage_w2((NA - 1) * TA, TA)

    mod_chunk(NC)
    gb = mod_s[NC, 0:1, :]
    w_copies[2].wait()
    w_copies[3].wait()

    def out_copy(t):
        rows = pl.ds(pl.multiple_of(t * TB, TB), TB)
        return pltpu.make_async_copy(o_v.at[rows, :], o_hbm.at[rows, :], sem_o.at[t])

    def loop_b(t, carry):
        rows = pl.ds(pl.multiple_of(t * TB, TB), TB)
        g3 = _gelu(_dot_nt(z_s[rows, :], w3_v[...])).astype(BF16)
        h2 = _dot(g3, w4_v[...])
        o_v[rows, :] = (x_s[rows, :] + gb * (h_s[rows, :] + h2)).astype(BF16)
        out_copy(t).start()
        return carry

    NT = S // TB
    lax.fori_loop(0, NT, loop_b, 0)
    for t in range(NT):
        out_copy(t).wait()


@jax.jit
def pallas_adaLN_cond__ssm_conv_h3__mixer_s_mlp__prompt_kernel(
    A_q: jax.Array,
    A_k: jax.Array,
    A_v: jax.Array,
    A_shift_k: jax.Array,
    A_ssm_k: jax.Array,
    A_ssm_D: jax.Array,
    B_x: jax.Array,
    B_w1: jax.Array,
    B_w2: jax.Array,
    B_w3: jax.Array,
    B_w4: jax.Array,
    c: jax.Array,
    w_mod: jax.Array,
):
    B, S, D = A_q.shape
    assert B == 1
    FF = B_w3.shape[1]
    NC = D // LANES
    NB = S // BLK
    TA = 256
    TB = 256
    fwd, inv = _dft_tables()
    fwd = jnp.asarray(fwd, BF16)
    inv = jnp.asarray(inv, BF16)

    args = (A_q.reshape(S, D), A_k.reshape(S, D), A_v.reshape(S, D), A_shift_k.T, A_ssm_k,
            A_ssm_D, B_w1, B_w2, B_w3.T, B_w4, c, w_mod, fwd, inv)
    scratch = [
        pltpu.VMEM((S, D), BF16),
        pltpu.VMEM((NC, S, LANES), BF16),
        pltpu.VMEM((NC, S, LANES), BF16),
        pltpu.VMEM((4, D), BF16),
        pltpu.VMEM((NC, LANES, S), BF16),
        pltpu.VMEM((D,), BF16),
        pltpu.VMEM((D, D), BF16),
        pltpu.VMEM((D, D), BF16),
        pltpu.VMEM((FF, D), BF16),
        pltpu.VMEM((FF, D), BF16),
        pltpu.VMEM((1, D), BF16),
        pltpu.VMEM((6, D, D), BF16),
        pltpu.VMEM((2 * BLK, BLK), BF16),
        pltpu.VMEM((BLK, 2 * BLK), BF16),
        pltpu.VMEM((S, D), BF16),
        pltpu.VMEM((S + 8, LANES), F32),
        pltpu.VMEM((NB, 2 * BLK, LANES), F32),
        pltpu.VMEM((NB, 2 * BLK, LANES), F32),
        pltpu.VMEM((NB, 2 * BLK, LANES), BF16),
        pltpu.VMEM((NC, S, LANES), F32),
        pltpu.VMEM((6, 8, D), F32),
        pltpu.VMEM((NC, 8, LANES), F32),
        pltpu.VMEM((NC, S + 16, LANES), F32),
        pltpu.VMEM((S, D), F32),
        pltpu.VMEM((S, D), F32),
        pltpu.VMEM((S, D), BF16),
        pltpu.SemaphoreType.DMA((5,)),
        pltpu.SemaphoreType.DMA((3, NC)),
        pltpu.SemaphoreType.DMA((6,)),
        pltpu.SemaphoreType.DMA((4,)),
        pltpu.SemaphoreType.DMA((1,)),
        pltpu.SemaphoreType.DMA((S // TB,)),
    ]
    out = pl.pallas_call(
        functools.partial(_kernel, S=S, D=D, FF=FF, TA=TA, TB=TB),
        in_specs=[pl.BlockSpec(memory_space=pl.ANY)] * len(args),
        out_specs=pl.BlockSpec(memory_space=pl.ANY),
        out_shape=jax.ShapeDtypeStruct((S, D), BF16),
        scratch_shapes=scratch,
        compiler_params=pltpu.CompilerParams(vmem_limit_bytes=100 * 1024 * 1024),
    )(*args)
    return out.reshape(B, S, D)
```

```python
import functools
import math

import jax
import jax.numpy as jnp
from jax import lax
import jax.experimental.pallas as pl
import jax.experimental.pallas.tpu as pltpu

F32 = jnp.float32
BF16 = jnp.bfloat16
U32 = jnp.uint32

LANES = 128
BLK = 128
PH = 4
EPS = 1e-05
TRIM = 100
SPLIT = 2
FREE = 30
PINLN = 0


def _as_bf16(x):
    return pltpu.bitcast(x, BF16)


def _lo(x):
    return pltpu.bitcast(x << 16, F32)


def _hi(x):
    return pltpu.bitcast(x & jnp.uint32(0xFFFF0000), F32)


def _dft4(re, im, sign):
    ar, ai = re[0] + re[2], im[0] + im[2]
    br, bi = re[0] - re[2], im[0] - im[2]
    cr, ci = re[1] + re[3], im[1] + im[3]
    dr, di = re[1] - re[3], im[1] - im[3]
    o0 = (ar + cr, ai + ci)
    o2 = (ar - cr, ai - ci)
    m = (br + di, bi - dr)
    p = (br - di, bi + dr)
    o1, o3 = (m, p) if sign < 0 else (p, m)
    return [o0[0], o1[0], o2[0], o3[0]], [o0[1], o1[1], o2[1], o3[1]]


def _ln(x):
    m = jnp.mean(x, axis=-1, keepdims=True)
    d = x - m
    v = jnp.mean(d * d, axis=-1, keepdims=True)
    return d * lax.rsqrt(v + EPS)


def _gelu(x):
    c0 = math.sqrt(2.0 / math.pi)
    t = jnp.tanh(x * (c0 + (c0 * 0.044715) * (x * x)))
    hx = 0.5 * x
    return hx + hx * t


def _dot(a, b):
    return jnp.dot(a, b, preferred_element_type=F32)


def _dot_nt(a, b):
    return lax.dot_general(a, b, (((1,), (1,)), ((), ())), preferred_element_type=F32)


def _kernel(q_hbm, k_hbm, v_hbm, sh_hbm, sk_hbm, sd_hbm, w1_hbm, w2_hbm, w3_hbm, w4_hbm, c_hbm, wm_hbm,
            o_hbm,
            q_v, k_v, v_v, sh_v, sk_v, sd_v, w1_v, w2_v, w3_v, w4_v, c_v, wm_v,
            fw_s, iv_s, o_v, u_s, kk_s, vv_s, wu_s, y_s, mod_s, h1_s, x_s, h_s, z_s, s3_s, s4_s,
            sem, sem_o,
            *, S, D, FF, TILES, TB):
    NC = D // LANES
    NG = BLK // 8
    LB = PH * BLK
    NBL = S // LB
    R = BLK // PH
    HALO = 16
    FP = w3_v.shape[1]
    FH = FP // 2
    NH = FH // LANES

    small = [
        pltpu.make_async_copy(sh_hbm, sh_v, sem.at[0]),
        pltpu.make_async_copy(sd_hbm, sd_v, sem.at[0]),
        pltpu.make_async_copy(c_hbm, c_v, sem.at[0]),
    ]

    def conv_copies(c):
        col = pl.ds(c * LANES, LANES)
        return [
            pltpu.make_async_copy(sk_hbm.at[col, :], sk_v.at[c], sem.at[1 + c]),
            pltpu.make_async_copy(k_hbm.at[:, col], k_v.at[c, pl.ds(16, S), :], sem.at[1 + c]),
            pltpu.make_async_copy(v_hbm.at[:, col], v_v.at[c], sem.at[1 + c]),
        ]

    def col_copies(src, dst, c0, s):
        rows = pl.ds(0, src.shape[0])
        return [pltpu.make_async_copy(src.at[:, pl.ds((c0 + c) * LANES, LANES)], dst.at[c0 + c, rows, :], sem.at[s])
                for c in range(NC)]

    wm_copies = [col_copies(wm_hbm, wm_v, j * NC, 6 + j) for j in range(6)]
    w_copies = [col_copies(src, dst, 0, 12 + j)
                for j, (src, dst) in enumerate(((w1_hbm, w1_v), (w2_hbm, w2_v), (w3_hbm, w3_v), (w4_hbm, w4_v)))]

    B0 = [0]
    for n in TILES:
        B0.append(B0[-1] + n)
    NA = len(TILES)
    A0 = [0] + [r + HALO for r in B0[1:-1]] + [S]
    q_copies = [
        [pltpu.make_async_copy(q_hbm.at[pl.ds(A0[t], A0[t + 1] - A0[t])], q_v.at[pl.ds(A0[t], A0[t + 1] - A0[t])],
                               sem.at[16 + t])]
        for t in range(NA)
    ]

    def start_all(cps, priority=0):
        for cp in cps:
            cp.start(priority=priority)

    def wait_all(cps):
        for cp in cps:
            cp.wait()

    def packed(ref, c0=0):
        ru = ref.bitcast(U32)
        return _as_bf16(jnp.concatenate([ru[c0 + c] for c in range(NC)], axis=1))

    first = conv_copies(0)
    start_all(first[:1] + small + first[1:] + conv_copies(1))

    for c in range(NC):
        k_v[c, 0:16, :] = jnp.zeros((16, LANES), BF16)
        h1_s[c, 0:8, :] = jnp.zeros((8, LANES), F32)
        h1_s[c, S + 8:S + 16, :] = jnp.zeros((8, LANES), F32)
        w3_v[c, FF:FP, :] = jnp.zeros((FP - FF, LANES), BF16)
        w4_v[c, FF:FP, :] = jnp.zeros((FP - FF, LANES), BF16)

    prow = lax.broadcasted_iota(jnp.int32, (BLK, BLK), 0)
    pcol = lax.broadcasted_iota(jnp.int32, (BLK, BLK), 1)
    ang = (((4 * prow + 1) * pcol) & (4 * BLK - 1)).astype(F32) * (2.0 * math.pi / (4 * BLK))
    tw = (4 * prow + 1).astype(F32) * (2.0 * math.pi / (4 * LB))
    mr, mi = jnp.cos(ang), -jnp.sin(ang)
    zr_, zi_ = jnp.cos(tw), -jnp.sin(tw)
    eye = jnp.where(prow == pcol, 1.0 / LB, 0.0).astype(BF16)
    for i in range(PH):
        both = jnp.stack([mr.reshape(NG, 8, BLK), mi.reshape(NG, 8, BLK)], axis=1).reshape(2 * BLK, BLK)
        fw_s[i] = both.astype(BF16)
        for h in range(2):
            iv_s[i, h] = _dot_nt(eye, both[h * BLK:(h + 1) * BLK, :].astype(BF16)).astype(BF16)
        if i + 1 < PH:
            mr, mi = mr * zr_ - mi * zi_, mr * zi_ + mi * zr_
    perm = jnp.where(pcol == (prow % R) * PH + prow // R, 1.0, 0.0).astype(BF16)
    fw_u = fw_s.bitcast(U32)
    iv_u = iv_s.bitcast(U32)

    wait_all(small)
    shf = sh_v[...].astype(F32)
    sdf = sd_v[...].astype(F32).reshape(1, D)
    cf = c_v[...].astype(F32)
    sc = (cf * jax.nn.sigmoid(cf)).astype(BF16)
    sc16 = jnp.broadcast_to(sc, (16, D))

    def mod_chunk(j):
        mod_s[j] = _dot(sc16, packed(wm_v, j * NC))[0:8, :]

    k_u = k_v.bitcast(U32)
    v_u = v_v.bitcast(U32)
    wu_u = wu_s.bitcast(U32)
    z_u = z_s.bitcast(U32)

    never = zr_[0:8, :] > 2.0

    def after(token, x):
        if token.dtype != x.dtype:
            token = pltpu.bitcast(token, x.dtype)
        return jnp.where(jnp.broadcast_to(never, x.shape), token, x)

    def split(t):
        t4 = t.reshape(NG, 2, 8, LANES)
        return t4[:, 0], t4[:, 1]

    def perm_k(c, b, toks):
        kt = [_dot_nt(perm, sk_v[c, :, b * LB + t * BLK:b * LB + (t + 1) * BLK]) for t in range(PH)]
        for r in range(BLK // 16):
            toks.append(kt[0][16 * r:16 * r + 8, :])
        return [jnp.concatenate([kt[t][i * R:(i + 1) * R, :] for t in range(PH)], axis=0).astype(BF16)
                for i in range(PH)]

    def spectrum(wts, dst, b, toks, dc=None, pins=None):
        tr, ti = [], []
        for i in range(PH):
            lhs = fw_u[i]
            if pins is not None and i < len(pins):
                lhs = after(pins[i], lhs.reshape(NG, 8, LANES)).reshape(BLK, LANES)
            r_, i_ = split(_dot(_as_bf16(lhs), wts[i]))
            tr.append(r_)
            ti.append(i_)
        for g in range(NG):
            toks.append(ti[PH - 1][g])
        if dc is not None:
            tr[0] = tr[0] + dc
        sr, si = _dft4(tr, ti, -1)
        for qq in range(PH):
            dst[:, b, qq, 0] = sr[qq]
            dst[:, b, qq, 1] = si[qq]

    def gated(c, b):
        w = [shf[t:t + 1, c * LANES:(c + 1) * LANES] for t in range(4)]
        kc = {}
        for o in range(-2, 2):
            words = k_u[c, pl.ds(8 + b * (LB // 2) + o, BLK, stride=2), :]
            if o > -2:
                kc[2 * o] = _lo(words)
            kc[2 * o + 1] = _hi(words)
        vc = {}
        for o in range(2):
            words = v_u[c, pl.ds(b * (LB // 2) + o, BLK, stride=2), :]
            vc[2 * o] = _lo(words)
            vc[2 * o + 1] = _hi(words)
        for i in range(PH):
            ks = kc[i] * w[0]
            for t in range(1, 4):
                ks = ks + kc[i - t] * w[t]
            wu_s[b, i] = (ks * vc[i]).astype(BF16)
        return [wu_u[b, i] for i in range(PH)]

    def kv_pins(kvb):
        return [jnp.stack([kvb[2 * m + (r % 2)][8 * (r // 2):8 * (r // 2) + 8, :] for r in range(NG)])
                for m in range(2)]

    def mac(c, toks):
        us, ks = u_s[c % 2], kk_s[c % 2]
        zp = None
        for o in range(NBL):
            zr, zi = [], []
            for qq in range(PH):
                accr = acci = None
                for b in range(o + 1):
                    a_, b_ = us[:, b, qq, 0], us[:, b, qq, 1]
                    c_, d_ = ks[:, o - b, qq, 0], ks[:, o - b, qq, 1]
                    if qq == 0 and b == o:
                        a_ = after(toks[o], a_)
                    tr_ = a_ * c_ - b_ * d_
                    ti_ = a_ * d_ + b_ * c_
                    accr = tr_ if accr is None else accr + tr_
                    acci = ti_ if acci is None else acci + ti_
                zr.append(accr)
                zi.append(acci)
            if zp is None:
                yr, yi = zr, zi
            else:
                yr = [zr[qq] - zp[1][qq] for qq in range(PH)]
                yi = [zi[qq] + zp[0][qq] for qq in range(PH)]
            zp = (zr, zi)
            vr, vi = _dft4(yr, yi, +1)
            for i in range(PH):
                vv_s[c % 2][o, i] = jnp.stack([vr[i], vi[i]], axis=1).reshape(2 * BLK, LANES).astype(BF16)

    def inverse(c, toks, pins=None, between=None):
        vv_u = vv_s[c % 2].bitcast(U32)
        HB = BLK // 2
        for o in range(NBL):
            for i in range(PH):
                yv = None
                for h in range(2):
                    lhs = iv_u[i, h]
                    if pins is not None and h == 0:
                        pin = pins[o][i % 2][8 * (i // 2):8 * (i // 2) + 8]
                        lhs = after(pin, lhs.reshape(8, 8, LANES)).reshape(HB, LANES)
                    t = _dot(_as_bf16(lhs), _as_bf16(vv_u[o, i, h * HB:(h + 1) * HB, :]))
                    yv = t if yv is None else yv + t
                if i % 2 == 0:
                    for r in range(BLK // 16):
                        toks.append(yv[16 * r:16 * r + 8, :])
                y_s[c, pl.ds(o * LB + i, BLK, stride=PH), :] = yv
            if between is not None:
                between(o)

    def mac_tokens(toks):
        n = len(toks) - 3
        cum = (44, 128, 244, 392)
        return [jnp.stack([toks[max(0, ((g * 392 + cum[o]) * n) // (392 * NG) - 1)] for g in range(NG)])
                for o in range(NBL)]

    def conv_round(c, between=None):
        toks = []
        kv = pins = None
        if c < NC:
            kv = [gated(c, b) for b in range(NBL)]
            pins = [kv_pins(kv[b]) for b in range(NBL)]
        if c >= 2:
            inverse(c - 2, toks, pins, between)
            if c < NC:
                toks = []
        if c < NC:
            wts = [perm_k(c, b, toks) for b in range(NBL)]
            dc = sdf[:, c * LANES:(c + 1) * LANES]
            if c >= 2:
                for b in range(NBL):
                    spectrum(wts[b], kk_s[c % 2], b, toks, dc if b == 0 else None)
                    spectrum([_as_bf16(x) for x in kv[b]], u_s[c % 2], b, toks)
            else:
                order = ('k0', 'k1', 'k2', 'u0', 'k3', 'u1', 'u2', 'u3')
                pin_at = {'k0': 0, 'k1': 1, 'u0': 2, 'k3': 3}
                for name in order:
                    b = int(name[1])
                    pin = pins[pin_at[name]] if name in pin_at else None
                    if name[0] == 'k':
                        spectrum(wts[b], kk_s[c % 2], b, toks, dc if b == 0 else None, pin)
                    else:
                        spectrum([_as_bf16(x) for x in kv[b]], u_s[c % 2], b, toks, None, pin)
        if 1 <= c <= NC:
            mac(c - 1, mac_tokens(toks))

    def pace(x, toks):
        if toks is None:
            return x
        n = x.shape[0] // 8
        m = len(toks)
        idx = [(r * (m + FREE)) // n - FREE for r in range(n)]
        f = len([i for i in idx if i < 0])
        tk = jnp.stack([toks[i] for i in idx[f:]])
        first = after(tk, x[8 * f:, 0:LANES].reshape(n - f, 8, LANES)).reshape(8 * (n - f), LANES)
        if f:
            first = jnp.concatenate([x[:8 * f, 0:LANES], first], axis=0)
        return jnp.concatenate([first, x[:, LANES:]], axis=1)

    def tokens_of(x):
        return [x[8 * r:8 * r + 8, c * LANES:(c + 1) * LANES] for c in range(NC) for r in range(x.shape[0] // 8)]

    def store_bf16(ref, r0, x):
        for c in range(NC):
            ref[c, r0:r0 + x.shape[0], :] = x[:, c * LANES:(c + 1) * LANES].astype(BF16)

    def load_bf16(ref_u, r0, n):
        return _as_bf16(jnp.concatenate([ref_u[c, pl.ds(r0 // 2, n // 2), :] for c in range(NC)], axis=1))

    def stage_p1(t, toks):
        r0, r1 = A0[t], A0[t + 1]
        ga = mod_s[2, 0:1, :]
        a_mul = ga * (1.0 + mod_s[1, 0:1, :])
        a_add = ga * mod_s[0, 0:1, :]
        q = pace(q_v[r0:r1, :].astype(F32), toks)
        y = jnp.concatenate([y_s[c, r0:r1, :] for c in range(NC)], axis=1)
        x = q + (_ln(q) * a_mul + a_add) * y
        x_s[r0:r1, :] = x
        return _ln(x)

    def stage_p2(t, nx):
        r0, r1 = A0[t], A0[t + 1]
        h = nx * (1.0 + mod_s[4, 0:1, :]) + mod_s[3, 0:1, :]
        h_s[r0:r1, :] = h
        store_bf16(z_s, S + r0, _ln(h))
        words = [z_u[c, (S + r0) // 2:(S + r1) // 2, :] for c in range(NC)]
        return [words[c][8 * j:8 * j + 8, :] for j in range((r1 - r0) // 16) for c in range(NC)]

    def chunks(r0, r1, k):
        n = (r1 - r0) // 16
        cuts = [r0 + 16 * ((n * j) // k) for j in range(k + 1)]
        return list(zip(cuts[:-1], cuts[1:]))

    def stage_m1(t, k):
        toks = []
        for r0, r1 in chunks(A0[t], A0[t + 1], k):
            g1 = _gelu(_dot(load_bf16(z_u, S + r0, r1 - r0), packed(w1_v)))
            for c in range(NC):
                h1_s[c, r0 + 8:r1 + 8, :] = g1[:, c * LANES:(c + 1) * LANES]
            toks += tokens_of(g1)
        return toks

    grp = D // 4
    shifts = (-1, 1, -2, 2)

    def stage_m2(t, k):
        out = []
        for r0, r1 in chunks(B0[t], B0[t + 1], k):
            n = r1 - r0
            lane = lax.broadcasted_iota(jnp.int32, (n, LANES), 1)
            parts = []
            for c in range(NC):
                lo, hi = c * LANES, (c + 1) * LANES
                g_lo, g_hi = lo // grp, (hi - 1) // grp
                val = h1_s[c, pl.ds(r0 + 8 + shifts[g_lo], n), :]
                if g_hi != g_lo:
                    other = h1_s[c, pl.ds(r0 + 8 + shifts[g_hi], n), :]
                    val = jnp.where(lane < (g_hi * grp - lo), val, other)
                parts.append(val)
            x1 = h_s[r0:r1, :] + _dot(jnp.concatenate(parts, axis=1).astype(BF16), packed(w2_v))
            out.append((r0, r1, x1))
        return out

    def store_x1(parts, pins, first=0.0):
        total = sum((r1 - r0) // 8 * NC for r0, r1, _ in parts)
        where = {}
        if pins and PINLN:
            lo = int(total * first)
            for j, p in enumerate(pins):
                where[lo + ((j + 1) * (total - lo)) // len(pins) - 1] = p
        pos = 0
        for r0, r1, x1 in parts:
            n = (r1 - r0) // 8
            for c in range(NC):
                col = x1[:, c * LANES:(c + 1) * LANES]
                hit = [r for r in range(n) if pos + r in where]
                if hit:
                    col3 = col.reshape(n, 8, LANES)
                    pinned = after(jnp.stack([where[pos + r] for r in hit]), jnp.stack([col3[r] for r in hit]))
                    rows = [col3[r] for r in range(n)]
                    for j, r in enumerate(hit):
                        rows[r] = pinned[j]
                    col = jnp.concatenate(rows, axis=0)
                h_s[r0:r1, c * LANES:(c + 1) * LANES] = col
                pos += n

    def stage_l(t, toks):
        r0, r1 = B0[t], B0[t + 1]
        store_bf16(z_s, r0, _ln(pace(h_s[r0:r1, :], toks)))

    def weight_sums(src, dst, transposed, toks):
        n = FH // 16

        def block(c, lo, tk):
            x = src[c, lo:lo + FH, :].astype(F32)
            if tk is None:
                return x
            x4 = x.reshape(n, 2, 8, LANES)
            return jnp.stack([after(tk, x4[:, 0]), x4[:, 1]], axis=1).reshape(FH, LANES)

        for j in range(2):
            tk = jnp.stack([toks[((j * n + r) * len(toks)) // (2 * n)] for r in range(n)])
            b11 = block(j, 0, tk)
            b22 = block(2 + j, FH, tk)
            e1, e2 = block(j, FH, None), block(2 + j, 0, None)
            b12, b21 = (e1, e2) if transposed else (e2, e1)
            dst[0, j] = (b11 + b22).astype(BF16)
            dst[1, j] = (b12 - b22).astype(BF16)
            dst[2, j] = (b21 - b11).astype(BF16)
            dst[3, j] = (b11 + b12).astype(BF16)
            dst[4, j] = (b21 + b22).astype(BF16)

    later = {
        0: (conv_copies(2) + conv_copies(3), 0),
        1: (conv_copies(4) + wm_copies[0] + wm_copies[1], 0),
        2: (wm_copies[2] + q_copies[0] + wm_copies[4], 0),
        3: (wm_copies[3] + w_copies[0], 0),
        4: (q_copies[1] + w_copies[1] + sum(q_copies[2:], []), 1),
        5: (w_copies[2] + w_copies[3] + wm_copies[5], 1),
    }
    for c in range(NC + 1):
        with jax.named_scope("r%d_wait" % c):
            if c < NC:
                wait_all(conv_copies(c))
            else:
                wait_all(wm_copies[0] + wm_copies[1] + wm_copies[2])
        with jax.named_scope("r%d" % c):
            start_all(*later[c])
            conv_round(c, (lambda o: mod_chunk(o) if o < 3 else None) if c == NC else None)
    with jax.named_scope("r6_wait"):
        wait_all(q_copies[0])
    with jax.named_scope("r6"):
        conv_round(NC + 1)
        nx0 = stage_p1(0, None)
    with jax.named_scope("p2_wait"):
        wait_all(wm_copies[4] + wm_copies[3])
    with jax.named_scope("p2"):
        mod_chunk(4)
        mod_chunk(3)
        stage_p2(0, nx0)
    with jax.named_scope("w1_wait"):
        wait_all(w_copies[0])
    with jax.named_scope("m1_0"):
        stage_m1(0, 4)
    with jax.named_scope("w2_wait"):
        wait_all(q_copies[1] + w_copies[1])
    with jax.named_scope("m2_0"):
        x1 = stage_m2(0, 4)
        toks = sum((tokens_of(p[2]) for p in x1), [])
        pins = stage_p2(1, stage_p1(1, toks[:len(toks) - TRIM]))
        store_x1(x1, pins, 0.4)
    for t in range(1, NA):
        with jax.named_scope("a%d" % t):
            if t + 1 < NA:
                wait_all(q_copies[t + 1])
            else:
                wait_all(w_copies[2] + w_copies[3] + wm_copies[5])
            toks = stage_m1(t, SPLIT)
            x1 = stage_m2(t, SPLIT)
            toks = toks + sum((tokens_of(p[2]) for p in x1), [])
            toks = toks[:len(toks) - TRIM]
            stage_l(t - 1, toks)
            if t + 1 < NA:
                store_x1(x1, stage_p2(t + 1, stage_p1(t + 1, toks)))
            else:
                store_x1(x1, None)
                weight_sums(w3_v, s3_s, True, toks[:len(toks) // 2])
                weight_sums(w4_v, s4_s, False, toks[len(toks) // 2:])
                mod_chunk(NC)
                stage_l(t, None)

    gb = mod_s[NC, 0:1, :]
    w3_u, w4_u, s3_u, s4_u = (r.bitcast(U32) for r in (w3_v, w4_v, s3_s, s4_s))
    TH = TB // 2
    HL = LANES // 2

    def lhs_sums(a11, a12, a21, a22):
        return [a11 + a22, a21 + a22, a11, a22, a11 + a12, a21 - a11, a12 - a22]

    def combine(m):
        return m[0] + m[3] - m[4] + m[6], m[2] + m[4], m[1] + m[3], m[0] - m[1] + m[2] + m[5]

    def out_copy(t):
        rows = pl.ds(pl.multiple_of(t * TB, TB), TB)
        return pltpu.make_async_copy(o_v.at[rows, :], o_hbm.at[rows, :], sem_o.at[0])

    ORDER = (2, 3, 1, 4, 0, 5, 6)

    def loop_b(t, carry):
        r0 = pl.multiple_of(t * TB, TB)

        def zf(half, cs):
            rows = pl.ds(pl.multiple_of(r0 + half * TH, TH), TH)
            return jnp.concatenate([z_s[c, rows, :].astype(F32) for c in cs], axis=1)

        def zb(half, cs):
            rows = pl.ds(pl.multiple_of(t * TH + half * (TH // 2), TH // 2), TH // 2)
            return _as_bf16(jnp.concatenate([z_u[c, rows, :] for c in cs], axis=1))

        la = [x.astype(BF16) for x in lhs_sums(zf(0, (0, 1)), zf(0, (2, 3)), zf(1, (0, 1)), zf(1, (2, 3)))]
        la[2] = zb(0, (0, 1))
        la[3] = zb(1, (2, 3))
        zr = [zb(0, (4,)), zb(1, (4,))]

        lb = [[] for _ in range(7)]
        g12, g21 = [], []
        for n in range(NH):
            lo = slice(n * HL, (n + 1) * HL)
            hi = slice(FH // 2 + n * HL, FH // 2 + (n + 1) * HL)
            ssum = lambda i: _as_bf16(jnp.concatenate([s3_u[i, 0, lo], s3_u[i, 1, lo]], axis=1))
            rhs = [ssum(0), _as_bf16(jnp.concatenate([w3_u[0, lo], w3_u[1, lo]], axis=1)), ssum(1), ssum(2),
                   _as_bf16(jnp.concatenate([w3_u[2, hi], w3_u[3, hi]], axis=1)), ssum(3), ssum(4)]
            rem = [[_dot_nt(zr[h], _as_bf16(w3_u[4, sl])) for sl in (lo, hi)] for h in range(2)]
            m = [None] * 7
            for i in ORDER:
                m[i] = _dot_nt(la[i], rhs[i])
            c11, c12, c21, c22 = combine(m)
            g = [_gelu(c11 + rem[0][0]), _gelu(c12 + rem[0][1]), _gelu(c21 + rem[1][0]), _gelu(c22 + rem[1][1])]
            for i, x in enumerate(lhs_sums(*g)):
                lb[i].append(x)
            g12.append(g[1])
            g21.append(g[2])
        top = jnp.concatenate(lb[2] + g12, axis=1).astype(BF16)
        bot = jnp.concatenate(g21 + lb[3], axis=1).astype(BF16)
        lb = [jnp.concatenate(x, axis=1).astype(BF16) for x in lb]
        w4r = _as_bf16(w4_u[4])
        res = [[None] * NC for _ in range(2)]
        res[0][4] = _dot(top, w4r)
        res[1][4] = _dot(bot, w4r)
        for j in range(2):
            rhs = [s4_u[0, j], w4_u[j, 0:FH // 2], s4_u[1, j], s4_u[2, j], w4_u[2 + j, FH // 2:FH],
                   s4_u[3, j], s4_u[4, j]]
            m = [None] * 7
            for i in ORDER:
                m[i] = _dot(lb[i], _as_bf16(rhs[i]))
            res[0][j], res[0][2 + j], res[1][j], res[1][2 + j] = combine(m)
        h2 = jnp.concatenate([jnp.concatenate(res[0], axis=1), jnp.concatenate(res[1], axis=1)], axis=0)
        rows = pl.ds(r0, TB)
        o_v[rows, :] = (x_s[rows, :] + gb * (h_s[rows, :] + h2)).astype(BF16)
        out_copy(t).start()
        return carry

    NT = S // TB
    with jax.named_scope("ph2b"):
        lax.fori_loop(0, NT, loop_b, 0)
    with jax.named_scope("tail"):
        for t in range(NT):
            out_copy(t).wait()


@jax.jit
def pallas_adaLN_cond__ssm_conv_h3__mixer_s_mlp__prompt_kernel(
    A_q: jax.Array,
    A_k: jax.Array,
    A_v: jax.Array,
    A_shift_k: jax.Array,
    A_ssm_k: jax.Array,
    A_ssm_D: jax.Array,
    B_x: jax.Array,
    B_w1: jax.Array,
    B_w2: jax.Array,
    B_w3: jax.Array,
    B_w4: jax.Array,
    c: jax.Array,
    w_mod: jax.Array,
):
    B, S, D = A_q.shape
    assert B == 1
    FF = B_w3.shape[1]
    NC = D // LANES
    NG = BLK // 8
    NBL = S // (PH * BLK)
    FP = -(-FF // (2 * LANES)) * 2 * LANES
    TILES = (384, 320, 448, 448, 448)
    assert sum(TILES) == S
    TB = 256

    args = (A_q.reshape(S, D), A_k.reshape(S, D), A_v.reshape(S, D), A_shift_k.T, A_ssm_k,
            A_ssm_D, B_w1, B_w2, B_w3.T, B_w4, c, w_mod)
    scratch = [
        pltpu.VMEM((S, D), BF16),
        pltpu.VMEM((NC, S + 16, LANES), BF16),
        pltpu.VMEM((NC, S, LANES), BF16),
        pltpu.VMEM((4, D), BF16),
        pltpu.VMEM((NC, LANES, S), BF16),
        pltpu.VMEM((D,), BF16),
        pltpu.VMEM((NC, D, LANES), BF16),
        pltpu.VMEM((NC, D, LANES), BF16),
        pltpu.VMEM((NC, FP, LANES), BF16),
        pltpu.VMEM((NC, FP, LANES), BF16),
        pltpu.VMEM((1, D), BF16),
        pltpu.VMEM((6 * NC, D, LANES), BF16),
        pltpu.VMEM((PH, 2 * BLK, BLK), BF16),
        pltpu.VMEM((PH, 2, BLK, BLK), BF16),
        pltpu.VMEM((S, D), BF16),
        [pltpu.VMEM((NG, NBL, PH, 2, 8, LANES), F32)] * 2,
        [pltpu.VMEM((NG, NBL, PH, 2, 8, LANES), F32)] * 2,
        [pltpu.VMEM((NBL, PH, 2 * BLK, LANES), BF16)] * 2,
        pltpu.VMEM((NBL, PH, BLK, LANES), BF16),
        pltpu.VMEM((NC, S, LANES), F32),
        pltpu.VMEM((6, 8, D), F32),
        pltpu.VMEM((NC, S + 16, LANES), F32),
        pltpu.VMEM((S, D), F32),
        pltpu.VMEM((S, D), F32),
        pltpu.VMEM((NC, 2 * S, LANES), BF16),
        pltpu.VMEM((5, 2, FP // 2, LANES), BF16),
        pltpu.VMEM((5, 2, FP // 2, LANES), BF16),
        pltpu.SemaphoreType.DMA((16 + len(TILES),)),
        pltpu.SemaphoreType.DMA((1,)),
    ]
    out = pl.pallas_call(
        functools.partial(_kernel, S=S, D=D, FF=FF, TILES=TILES, TB=TB),
        in_specs=[pl.BlockSpec(memory_space=pl.ANY)] * len(args),
        out_specs=pl.BlockSpec(memory_space=pl.ANY),
        out_shape=jax.ShapeDtypeStruct((S, D), BF16),
        scratch_shapes=scratch,
        compiler_params=pltpu.CompilerParams(
            vmem_limit_bytes=100 * 1024 * 1024,
            disable_bounds_checks=True,
            disable_semaphore_checks=True,
        ),
    )(*args)
    return out.reshape(B, S, D)
```

```python
import functools
import math

import jax
import jax.numpy as jnp
from jax import lax
import jax.experimental.pallas as pl
import jax.experimental.pallas.tpu as pltpu

F32 = jnp.float32
BF16 = jnp.bfloat16
U32 = jnp.uint32

LANES = 128
BLK = 128
PH = 4
EPS = 1e-05
TRIM = 100
SPLIT = 2
FREE = 30
LAT = 4
TRIMB = 350
ATOK = 1
LAG = 3
NEWSLOT = (0, 1, 2, 3, 4, 5, 6)
SH2 = 0
RSQ = 0
PINLN = 0


def _as_bf16(x):
    return pltpu.bitcast(x, BF16)


def _lo(x):
    return pltpu.bitcast(x << 16, F32)


def _hi(x):
    return pltpu.bitcast(x & jnp.uint32(0xFFFF0000), F32)


def _dft4(re, im, sign):
    ar, ai = re[0] + re[2], im[0] + im[2]
    br, bi = re[0] - re[2], im[0] - im[2]
    cr, ci = re[1] + re[3], im[1] + im[3]
    dr, di = re[1] - re[3], im[1] - im[3]
    o0 = (ar + cr, ai + ci)
    o2 = (ar - cr, ai - ci)
    m = (br + di, bi - dr)
    p = (br - di, bi + dr)
    o1, o3 = (m, p) if sign < 0 else (p, m)
    return [o0[0], o1[0], o2[0], o3[0]], [o0[1], o1[1], o2[1], o3[1]]


def _ln(x):
    m = jnp.mean(x, axis=-1, keepdims=True)
    d = x - m
    v = jnp.mean(d * d, axis=-1, keepdims=True)
    if RSQ:
        return d * jnp.exp(-0.5 * jnp.log(v + EPS))
    return d * lax.rsqrt(v + EPS)


def _gelu(x):
    c0 = math.sqrt(2.0 / math.pi)
    t = jnp.tanh(x * (c0 + (c0 * 0.044715) * (x * x)))
    hx = 0.5 * x
    return hx + hx * t


def _dot(a, b):
    return jnp.dot(a, b, preferred_element_type=F32)


def _dot_nt(a, b):
    return lax.dot_general(a, b, (((1,), (1,)), ((), ())), preferred_element_type=F32)


def _lhs_ops(a11, a12, a21, a22):
    return [a11 + a22, a21 + a22, a11, a22, a11 + a12, a21 - a11, a12 - a22]


def _rhs_ops(b11, b12, b21, b22):
    return [b11 + b22, b11, b12 - b22, b21 - b11, b22, b11 + b12, b21 + b22]


def _combine(m):
    return (m[3] - m[4]) + m[0] + m[6], m[2] + m[4], m[1] + m[3], (m[2] - m[1]) + m[0] + m[5]


_ORDER = (2, 4, 1, 3, 0, 6, 5)


def _kernel(q_hbm, k_hbm, v_hbm, sh_hbm, sk_hbm, sd_hbm, w1_hbm, w2_hbm, w3_hbm, w4_hbm, c_hbm, wm_hbm,
            o_hbm,
            q_v, k_v, v_v, sh_v, sk_v, sd_v, w1_v, w2_v, w3_v, w4_v, c_v, wm_v,
            fw_s, iv_s, o_v, u_s, kk_s, vv_s, wu_s, y_s, mod_s, par_s, h1_s, x_s, h_s, z_s, s3_s, s4_s, e3_s, e4_s, g_s, zf_s, zero_s,
            sem, sem_o,
            *, S, D, FF, TILES, TB):
    NC = D // LANES
    NG = BLK // 8
    LB = PH * BLK
    NBL = S // LB
    R = BLK // PH
    HALO = 16
    FP = w3_v.shape[1]
    FH = FP // 2
    NH = FH // LANES

    small = [
        pltpu.make_async_copy(sh_hbm, sh_v, sem.at[0]),
        pltpu.make_async_copy(sd_hbm, sd_v, sem.at[0]),
        pltpu.make_async_copy(c_hbm, c_v, sem.at[0]),
    ]

    def conv_copies(c):
        col = pl.ds(c * LANES if isinstance(c, int) else pl.multiple_of(c * LANES, LANES), LANES)
        return [
            pltpu.make_async_copy(sk_hbm.at[col, :], sk_v.at[c], sem.at[1 + c]),
            pltpu.make_async_copy(k_hbm.at[:, col], k_v.at[c, pl.ds(16, S), :], sem.at[1 + c]),
            pltpu.make_async_copy(v_hbm.at[:, col], v_v.at[c], sem.at[1 + c]),
        ]

    def col_copies(src, dst, c0, s):
        rows = pl.ds(0, src.shape[0])
        return [pltpu.make_async_copy(src.at[:, pl.ds((c0 + c) * LANES, LANES)], dst.at[c0 + c, rows, :], sem.at[s])
                for c in range(NC)]

    WM = (0, 3 * D, 5 * D, 6 * D)
    wm_copies = [[pltpu.make_async_copy(wm_hbm.at[:, pl.ds(WM[j], WM[j + 1] - WM[j])],
                                        wm_v.at[:, pl.ds(WM[j], WM[j + 1] - WM[j])], sem.at[6 + j])]
                 for j in range(3)]
    w_copies = [col_copies(src, dst, 0, 12 + j)
                for j, (src, dst) in enumerate(((w1_hbm, w1_v), (w2_hbm, w2_v), (w3_hbm, w3_v), (w4_hbm, w4_v)))]

    B0 = [0]
    for n in TILES:
        B0.append(B0[-1] + n)
    NA = len(TILES)
    A0 = [0] + [r + HALO for r in B0[1:-1]] + [S]
    q_copies = [
        [pltpu.make_async_copy(q_hbm.at[pl.ds(A0[t], A0[t + 1] - A0[t])], q_v.at[pl.ds(A0[t], A0[t + 1] - A0[t])],
                               sem.at[16 + t])]
        for t in range(NA)
    ]

    def start_all(cps, priority=0):
        for cp in cps:
            cp.start(priority=priority)

    def wait_all(cps):
        for cp in cps:
            cp.wait()

    def packed(ref, c0=0):
        ru = ref.bitcast(U32)
        return _as_bf16(jnp.concatenate([ru[c0 + c] for c in range(NC)], axis=1))

    first = conv_copies(0)
    start_all(first[:1] + small + first[1:] + conv_copies(1))

    zero_s[0] = 0
    for c in range(NC):
        k_v[c, 0:16, :] = jnp.zeros((16, LANES), BF16)
        h1_s[c, 0:8, :] = jnp.zeros((8, LANES), F32)
        h1_s[c, S + 8:S + 16, :] = jnp.zeros((8, LANES), F32)
        w3_v[c, FF:FP, :] = jnp.zeros((FP - FF, LANES), BF16)
        w4_v[c, FF:FP, :] = jnp.zeros((FP - FF, LANES), BF16)

    prow = lax.broadcasted_iota(jnp.int32, (BLK, BLK), 0)
    pcol = lax.broadcasted_iota(jnp.int32, (BLK, BLK), 1)
    ang = (((4 * prow + 1) * pcol) & (4 * BLK - 1)).astype(F32) * (2.0 * math.pi / (4 * BLK))
    tw = (4 * prow + 1).astype(F32) * (2.0 * math.pi / (4 * LB))
    mr, mi = jnp.cos(ang), -jnp.sin(ang)
    zr_, zi_ = jnp.cos(tw), -jnp.sin(tw)
    eye = jnp.where(prow == pcol, 1.0 / LB, 0.0).astype(BF16)
    for i in range(PH):
        both = jnp.stack([mr.reshape(NG, 8, BLK), mi.reshape(NG, 8, BLK)], axis=1).reshape(2 * BLK, BLK)
        fw_s[i] = both.astype(BF16)
        for h in range(2):
            iv_s[i, h] = _dot_nt(eye, both[h * BLK:(h + 1) * BLK, :].astype(BF16)).astype(BF16)
        if i + 1 < PH:
            mr, mi = mr * zr_ - mi * zi_, mr * zi_ + mi * zr_
    perm = jnp.where(pcol == (prow % R) * PH + prow // R, 1.0, 0.0).astype(BF16)
    fw_u = fw_s.bitcast(U32)
    iv_u = iv_s.bitcast(U32)

    wait_all(small)
    shf = sh_v[...].astype(F32)
    sdf = sd_v[...].astype(F32).reshape(1, D)
    for c in range(NC):
        par_s[c, 0:4, :] = shf[:, c * LANES:(c + 1) * LANES]
        par_s[c, 4:5, :] = sdf[:, c * LANES:(c + 1) * LANES]
    cf = c_v[...].astype(F32)
    sc = (cf * jax.nn.sigmoid(cf)).astype(BF16)
    sc16 = jnp.broadcast_to(sc, (16, D))

    def mod_chunk(j):
        mod_s[j] = _dot(sc16, wm_v[:, j * D:(j + 1) * D])[0:8, :]

    k_u = k_v.bitcast(U32)
    v_u = v_v.bitcast(U32)
    wu_u = wu_s.bitcast(U32)
    z_u = z_s.bitcast(U32)
    vv_u = vv_s.bitcast(U32)

    never = zr_[0:8, :] > 2.0

    def after(token, x):
        if token.dtype != x.dtype:
            token = pltpu.bitcast(token, x.dtype)
        return jnp.where(jnp.broadcast_to(never, x.shape), token, x)

    def split(t):
        t4 = t.reshape(NG, 2, 8, LANES)
        return t4[:, 0], t4[:, 1]

    def perm_k(c, b, toks):
        kt = [_dot_nt(perm, sk_v[c, :, b * LB + t * BLK:b * LB + (t + 1) * BLK]) for t in range(PH)]
        for r in range(BLK // 16):
            toks.append(kt[0][16 * r:16 * r + 8, :])
        return [jnp.concatenate([kt[t][i * R:(i + 1) * R, :] for t in range(PH)], axis=0).astype(BF16)
                for i in range(PH)]

    def spectrum(wts, dst, c, b, toks, dc=None, pins=None):
        tr, ti = [], []
        for i in range(PH):
            lhs = fw_u[i]
            if pins is not None and i < len(pins):
                lhs = after(pins[i], lhs.reshape(NG, 8, LANES)).reshape(BLK, LANES)
            r_, i_ = split(_dot(_as_bf16(lhs), wts[i]))
            tr.append(r_)
            ti.append(i_)
        for g in range(NG):
            toks.append(ti[PH - 1][g])
        if dc is not None:
            tr[0] = tr[0] + dc
        sr, si = _dft4(tr, ti, -1)
        for qq in range(PH):
            dst[c, :, b, qq, 0] = sr[qq]
            dst[c, :, b, qq, 1] = si[qq]

    def gated(c, b):
        w = [par_s[c, t:t + 1, :] for t in range(4)]
        kc = {}
        for o in range(-2, 2):
            words = k_u[c, pl.ds(8 + b * (LB // 2) + o, BLK, stride=2), :]
            if o > -2:
                kc[2 * o] = _lo(words)
            kc[2 * o + 1] = _hi(words)
        vc = {}
        for o in range(2):
            words = v_u[c, pl.ds(b * (LB // 2) + o, BLK, stride=2), :]
            vc[2 * o] = _lo(words)
            vc[2 * o + 1] = _hi(words)
        for i in range(PH):
            ks = kc[i] * w[0]
            for t in range(1, 4):
                ks = ks + kc[i - t] * w[t]
            wu_s[b, i] = (ks * vc[i]).astype(BF16)
        return [wu_u[b, i] for i in range(PH)]

    def kv_pins(kvb):
        return [jnp.stack([kvb[2 * m + (r % 2)][8 * (r // 2):8 * (r // 2) + 8, :] for r in range(NG)])
                for m in range(2)]

    def mac(c, us, ks, toks):
        zp = None
        for o in range(NBL):
            zr, zi = [], []
            for qq in range(PH):
                accr = acci = None
                for b in range(o + 1):
                    a_, b_ = us[0, :, b, qq, 0], us[0, :, b, qq, 1]
                    c_, d_ = ks[0, :, o - b, qq, 0], ks[0, :, o - b, qq, 1]
                    if qq == 0 and b == o:
                        a_ = after(toks[o], a_)
                    tr_ = a_ * c_ - b_ * d_
                    ti_ = a_ * d_ + b_ * c_
                    accr = tr_ if accr is None else accr + tr_
                    acci = ti_ if acci is None else acci + ti_
                zr.append(accr)
                zi.append(acci)
            if zp is None:
                yr, yi = zr, zi
            else:
                yr = [zr[qq] - zp[1][qq] for qq in range(PH)]
                yi = [zi[qq] + zp[0][qq] for qq in range(PH)]
            zp = (zr, zi)
            vr, vi = _dft4(yr, yi, +1)
            for i in range(PH):
                vv_s[c, o, i] = jnp.stack([vr[i], vi[i]], axis=1).reshape(2 * BLK, LANES).astype(BF16)

    def inverse(c, toks, pins=None, between=None):
        HB = BLK // 2
        for o in range(NBL):
            for i in range(PH):
                yv = None
                for h in range(2):
                    lhs = iv_u[i, h]
                    if pins is not None and h == 0:
                        pin = pins[o][i % 2][8 * (i // 2):8 * (i // 2) + 8]
                        lhs = after(pin, lhs.reshape(8, 8, LANES)).reshape(HB, LANES)
                    t = _dot(_as_bf16(lhs), _as_bf16(vv_u[c, o, i, h * HB:(h + 1) * HB, :]))
                    yv = t if yv is None else yv + t
                if i % 2 == 0:
                    for r in range(BLK // 16):
                        toks.append(yv[16 * r:16 * r + 8, :])
                y_s[c, pl.ds(o * LB + i, BLK, stride=PH), :] = yv
            if between is not None:
                between(o)

    def mac_tokens(toks):
        n = len(toks) - 3
        cum = (44, 128, 244, 392)
        return [jnp.stack([toks[max(0, ((g * 392 + cum[o]) * n) // (392 * NG) - 1)] for g in range(NG)])
                for o in range(NBL)]

    def conv_round(c, fwd, mul, inv, between=None):
        toks = []
        kv = pins = None
        cur = 1 if mul else 0
        if fwd or mul:
            win = pl.ds(c - cur, 2 if fwd and mul else 1)
            us, ks = u_s.at[win], kk_s.at[win]
        if fwd:
            kv = [gated(c, b) for b in range(NBL)]
            pins = [kv_pins(kv[b]) for b in range(NBL)]
        if inv:
            inverse(c - 2, toks, pins, between)
            if fwd:
                toks = []
        if fwd:
            wts = [perm_k(c, b, toks) for b in range(NBL)]
            dc = par_s[c, 4:5, :]
            if inv:
                order = ('k0', 'u0', 'k1', 'u1', 'k2', 'u2', 'k3', 'u3')
                pin_at = {}
            else:
                order = ('k0', 'k1', 'k2', 'u0', 'k3', 'u1', 'u2', 'u3')
                pin_at = {'k0': 0, 'k1': 1, 'u0': 2, 'k3': 3}
            for name in order:
                b = int(name[1])
                pin = pins[pin_at[name]] if name in pin_at else None
                tk = [] if (pin is not None and mul) else toks
                if name[0] == 'k':
                    spectrum(wts[b], ks, cur, b, tk, dc if b == 0 else None, pin)
                else:
                    spectrum([_as_bf16(x) for x in kv[b]], us, cur, b, tk, None, pin)
                if tk is not toks:
                    toks += tk[::4]
        if mul:
            mac(c - 1, us, ks, mac_tokens(toks))

    def pace(x, toks, free=FREE):
        if toks is None:
            return x
        n = x.shape[0] // 8
        m = len(toks)
        idx = [(r * (m + free)) // n - free for r in range(n)]
        f = len([i for i in idx if i < 0])
        tk = jnp.stack([toks[i] for i in idx[f:]])
        first = after(tk, x[8 * f:, 0:LANES].reshape(n - f, 8, LANES)).reshape(8 * (n - f), LANES)
        if f:
            first = jnp.concatenate([x[:8 * f, 0:LANES], first], axis=0)
        return jnp.concatenate([first, x[:, LANES:]], axis=1)

    def tokens_of(x):
        return [x[8 * r:8 * r + 8, c * LANES:(c + 1) * LANES] for c in range(NC) for r in range(x.shape[0] // 8)]

    def store_bf16(ref, r0, x):
        for c in range(NC):
            ref[c, r0:r0 + x.shape[0], :] = x[:, c * LANES:(c + 1) * LANES].astype(BF16)

    def load_bf16(ref_u, r0, n):
        return _as_bf16(jnp.concatenate([ref_u[c, pl.ds(r0 // 2, n // 2), :] for c in range(NC)], axis=1))

    def stage_p1(t, toks):
        r0, r1 = A0[t], A0[t + 1]
        ga = mod_s[2, 0:1, :]
        a_mul = ga * (1.0 + mod_s[1, 0:1, :])
        a_add = ga * mod_s[0, 0:1, :]
        q = pace(q_v[r0:r1, :].astype(F32), toks)
        y = jnp.concatenate([y_s[c, r0:r1, :] for c in range(NC)], axis=1)
        x = q + (_ln(q) * a_mul + a_add) * y
        x_s[r0:r1, :] = x
        return _ln(x)

    def stage_p2(t, nx, toks=None):
        r0, r1 = A0[t], A0[t + 1]
        h = nx * (1.0 + mod_s[4, 0:1, :]) + mod_s[3, 0:1, :]
        h_s[r0:r1, :] = h
        store_bf16(z_s, S + r0, _ln(pace(h, toks, 0)))

    def stage_p(t, toks):
        n = len(toks) - TRIM
        stage_p2(t, stage_p1(t, toks[:n]), toks[SH2 - FREE:n + SH2] if SH2 else None)

    def chunks(r0, r1, k):
        n = (r1 - r0) // 16
        cuts = [r0 + 16 * ((n * j) // k) for j in range(k + 1)]
        return list(zip(cuts[:-1], cuts[1:]))

    def stage_m1(t, k):
        toks = []
        for r0, r1 in chunks(A0[t], A0[t + 1], k):
            g1 = _gelu(_dot(load_bf16(z_u, S + r0, r1 - r0), packed(w1_v)))
            for c in range(NC):
                h1_s[c, r0 + 8:r1 + 8, :] = g1[:, c * LANES:(c + 1) * LANES]
            toks += tokens_of(g1)
        return toks

    grp = D // 4
    shifts = (-1, 1, -2, 2)

    def stage_m2(t, k):
        out = []
        for r0, r1 in chunks(B0[t], B0[t + 1], k):
            n = r1 - r0
            lane = lax.broadcasted_iota(jnp.int32, (n, LANES), 1)
            parts = []
            for c in range(NC):
                lo, hi = c * LANES, (c + 1) * LANES
                g_lo, g_hi = lo // grp, (hi - 1) // grp
                val = h1_s[c, pl.ds(r0 + 8 + shifts[g_lo], n), :]
                if g_hi != g_lo:
                    other = h1_s[c, pl.ds(r0 + 8 + shifts[g_hi], n), :]
                    val = jnp.where(lane < (g_hi * grp - lo), val, other)
                parts.append(val)
            x1 = h_s[r0:r1, :] + _dot(jnp.concatenate(parts, axis=1).astype(BF16), packed(w2_v))
            out.append((r0, r1, x1))
        return out

    def store_x1(parts, pins, first=0.0):
        total = sum((r1 - r0) // 8 * NC for r0, r1, _ in parts)
        where = {}
        if pins and PINLN:
            lo = int(total * first)
            for j, p in enumerate(pins):
                where[lo + ((j + 1) * (total - lo)) // len(pins) - 1] = p
        pos = 0
        for r0, r1, x1 in parts:
            n = (r1 - r0) // 8
            for c in range(NC):
                col = x1[:, c * LANES:(c + 1) * LANES]
                hit = [r for r in range(n) if pos + r in where]
                if hit:
                    col3 = col.reshape(n, 8, LANES)
                    pinned = after(jnp.stack([where[pos + r] for r in hit]), jnp.stack([col3[r] for r in hit]))
                    rows = [col3[r] for r in range(n)]
                    for j, r in enumerate(hit):
                        rows[r] = pinned[j]
                    col = jnp.concatenate(rows, axis=0)
                h_s[r0:r1, c * LANES:(c + 1) * LANES] = col
                pos += n

    TQ = TB // 4
    NT = S // TB

    def store_z(r0, slot, toks, free):
        zn = _ln(pace(h_s[pl.ds(r0, TB), :], toks, free))
        for rq in range(4):
            for c in range(NC - 1):
                zf_s[slot, rq, c, 0:TQ, :] = zn[rq * TQ:(rq + 1) * TQ, c * LANES:(c + 1) * LANES]
        z_s[NC - 1, pl.ds(r0, TB), :] = zn[:, (NC - 1) * LANES:].astype(BF16)

    NS = NH // 2

    RAW = (1, 4)

    def weight_ops(src, dst, ext, transposed, toks):
        ng = LANES // 16
        total = (NS * 7 + 2) * ng

        def tile(c, n):
            return src[c, n * LANES:(n + 1) * LANES, :].astype(F32)

        def held(x, pos, step):
            tk = jnp.stack([toks[((pos + r * step) * len(toks)) // total] for r in range(ng)])
            x4 = x.reshape(ng, 2, 8, LANES)
            return jnp.stack([after(tk, x4[:, 0]), x4[:, 1]], axis=1).reshape(LANES, LANES)

        def outer(c2, n, pos=None):
            b11, b22 = tile(c2, n), tile(2 + c2, NH + n)
            if pos is not None:
                b11, b22 = held(b11, pos, 1), held(b22, pos, 1)
            e1, e2 = tile(c2, NH + n), tile(2 + c2, n)
            return _rhs_ops(b11, e1, e2, b22) if transposed else _rhs_ops(b11, e2, e1, b22)

        for c2 in range(2):
            for i, x in enumerate(outer(c2, NH - 1, c2 * ng)):
                if i not in RAW:
                    ext[i, c2] = x.astype(BF16)
        for st in range(NS):
            t00, t11 = outer(0, 2 * st), outer(1, 2 * st + 1)
            t01, t10 = outer(0, 2 * st + 1), outer(1, 2 * st)
            for k, i in enumerate((1, 5, 2, 4, 0, 3, 6)):
                pos = (2 + st * 7) * ng + k
                a, d = held(t00[i], pos, 7), held(t11[i], pos, 7)
                ops = _rhs_ops(a, t01[i], t10[i], d) if transposed else _rhs_ops(a, t10[i], t01[i], d)
                for j, x in enumerate(ops):
                    if i not in RAW or j not in RAW:
                        dst[i, j, st * LANES:(st + 1) * LANES, :] = x.astype(BF16)

    with jax.named_scope("r0_wait"):
        wait_all(conv_copies(0))
    with jax.named_scope("r0"):
        start_all(conv_copies(2) + conv_copies(3) + conv_copies(4))
        conv_round(0, True, False, False)
    with jax.named_scope("r1_wait"):
        wait_all(conv_copies(1))
    with jax.named_scope("r1"):
        start_all(wm_copies[0] + q_copies[0] + wm_copies[1] + w_copies[0])
        conv_round(1, True, True, False)

    def full_round(c, carry):
        wait_all(conv_copies(c))
        conv_round(c, True, True, True)
        return carry

    with jax.named_scope("r234"):
        lax.fori_loop(2, NC, full_round, 0)
    with jax.named_scope("r5"):
        start_all(q_copies[1] + w_copies[1] + sum(q_copies[2:], []) + w_copies[2] + w_copies[3] + wm_copies[2], 1)
        conv_round(NC, False, True, True)
    with jax.named_scope("r6_wait"):
        wait_all(wm_copies[0] + q_copies[0])
    with jax.named_scope("r6"):
        for j in range(3):
            mod_chunk(j)
        conv_round(NC + 1, False, False, True)
        nx0 = stage_p1(0, None)
    with jax.named_scope("p2_wait"):
        wait_all(wm_copies[1])
    with jax.named_scope("p2"):
        mod_chunk(4)
        mod_chunk(3)
        stage_p2(0, nx0)
    with jax.named_scope("w1_wait"):
        wait_all(w_copies[0])
    with jax.named_scope("m1_0"):
        stage_m1(0, 4)
    with jax.named_scope("w2_wait"):
        wait_all(q_copies[1] + w_copies[1])
    with jax.named_scope("m2_0"):
        x1 = stage_m2(0, 4)
        toks = sum((tokens_of(p[2]) for p in x1), [])
        store_x1(x1, None)
        stage_p(1, toks)
    for t in range(1, NA):
        with jax.named_scope("a%d" % t):
            if t + 1 < NA:
                wait_all(q_copies[t + 1])
            else:
                wait_all(w_copies[2] + w_copies[3] + wm_copies[2])
            toks = stage_m1(t, SPLIT)
            x1 = stage_m2(t, SPLIT)
            toks = toks + sum((tokens_of(p[2]) for p in x1), [])
            store_x1(x1, None)
            if t + 1 < NA:
                stage_p(t + 1, toks)
            else:
                mod_chunk(NC)
                short = toks[:len(toks) - 20]
                cut = (len(short) * 11) // 20
                weight_ops(w3_v, s3_s, e3_s, True, short[:cut])
                weight_ops(w4_v, s4_s, e4_s, False, short[cut:])
            if t == LAT:
                store_z(0, 0, toks[:len(toks) - TRIM // 2], FREE)

    gb = mod_s[NC, 0:1, :]
    w3_u, w4_u, s3_u, s4_u, e3_u, e4_u = (r.bitcast(U32) for r in (w3_v, w4_v, s3_s, s4_s, e3_s, e4_s))
    HL = LANES // 2

    def out_copy(r0, n, c):
        rows = pl.ds(r0, n)
        return pltpu.make_async_copy(o_v.at[c, rows, :], o_hbm.at[rows, pl.ds(c * LANES, LANES)], sem_o.at[0])

    def outer_lhs(i, blk):
        terms = ((0, 0, 1, 1, 1), (1, 0, 1, 1, 1), (0, 0), (1, 1), (0, 0, 1, 0, 1), (1, 0, -1, 0, 0), (0, 1, -1, 1, 1))[i]
        x = blk(terms[0], terms[1])
        if len(terms) > 2:
            y = blk(terms[3], terms[4])
            x = x + y if terms[2] > 0 else x - y
        return x

    def one_level(w_u, e_u, i, c2):
        if i not in RAW:
            return e_u[i, c2]
        d = RAW.index(i)
        n = d * NH + NH - 1
        return w_u[2 * d + c2, n * HL:(n + 1) * HL, :]

    def two_level(w_u, s_u, i, j, st):
        if i not in RAW or j not in RAW:
            return s_u[i, j, st * HL:(st + 1) * HL, :]
        d, e = RAW.index(i), RAW.index(j)
        n = d * NH + 2 * st + e
        return w_u[2 * d + e, n * HL:(n + 1) * HL, :]

    def loop_b(t, carry):
        r0 = pl.multiple_of(t * TB, TB)
        ws = t & 1
        rs = lax.rem(t + 2, 2)
        zero = zero_s[0]

        fresh = [1]

        def later(x):
            fresh[0] += 1
            return lax.rem(t + 2 * fresh[0], 2)

        zr = [_as_bf16(z_u[NC - 1, pl.ds(pl.multiple_of(t * (TB // 2) + rq * (TQ // 2), TQ // 2), TQ // 2), :])
              for rq in range(4)]

        def z_outer(i, slot):
            return [[outer_lhs(i, lambda r1, k1: zf_s[slot, 2 * r1 + r2, 2 * k1 + k2, 0:TQ, :]) for k2 in range(2)]
                    for r2 in range(2)]

        def rem3(rq, n):
            return _dot_nt(zr[rq], _as_bf16(w3_u[NC - 1, n * HL:(n + 1) * HL, :]))

        def put_g(rq, n, pre):
            g_s[ws, rq, n, 0:TQ, :] = _gelu(pre)

        rem = {}
        for rq in range(4):
            for h in range(2):
                rem[rq, h * NH + NH - 1] = rem3(rq, h * NH + NH - 1)
        for st in range(NS):
            rem[3, NH + 2 * st + 1] = rem3(3, NH + 2 * st + 1)
        m = [None] * 7
        for i in _ORDER:
            rhs = _as_bf16(jnp.concatenate([one_level(w3_u, e3_u, i, c2) for c2 in range(2)], axis=1))
            so = z_outer(i, later(None))
            m[i] = [_dot_nt(jnp.concatenate(so[r2], axis=1).astype(BF16), rhs) for r2 in range(2)]
        for r2 in range(2):
            for blk, cval in enumerate(_combine([m[i][r2] for i in range(7)])):
                rq, n = 2 * (blk // 2) + r2, (blk % 2) * NH + NH - 1
                put_g(rq, n, cval + rem[rq, n])
        def z_inner(i, j):
            slot = later(None)
            return outer_lhs(j, lambda r2, k2: outer_lhs(
                i, lambda r1, k1: zf_s[slot, 2 * r1 + r2, 2 * k1 + k2, 0:TQ, :])).astype(BF16)

        si = [[z_inner(i, j) for j in range(7)] for i in range(7)]
        for st in range(NS):
            todo = [(2 * r1 + r2, h * NH + 2 * st + p) for r1, h in ((0, 1), (1, 0), (0, 0), (1, 1))
                    for r2 in range(2) for p in range(2)]
            todo = [x for x in todo if x not in rem]
            for key in todo[:8]:
                rem[key] = rem3(*key)
            todo = todo[8:]
            pin = [None] * 7
            for i in _ORDER:
                m = [None] * 7
                for j in _ORDER:
                    m[j] = _dot_nt(si[i][j], _as_bf16(two_level(w3_u, s3_u, i, j, st)))
                key = todo.pop(0)
                rem[key] = rem3(*key)
                pin[i] = _combine(m)
            for inner in range(4):
                for blk, cval in enumerate(_combine([pin[i][inner] for i in range(7)])):
                    rq, n = 2 * (blk // 2) + inner // 2, (blk % 2) * NH + 2 * st + inner % 2
                    put_g(rq, n, cval + rem[rq, n])

        toks = []

        def timed(x):
            toks.extend(x[8 * r:8 * r + 8, 0:LANES] for r in range(x.shape[0] // 8))
            return x

        def finish(rq, c, h2):
            rows = pl.ds(pl.multiple_of(r0 + rq * TQ, TQ), TQ)
            cols = slice(c * LANES, (c + 1) * LANES)
            o_v[c, rows, :] = (x_s[rows, cols] + gb[:, cols] * (h_s[rows, cols] + h2)).astype(BF16)

        w4r = _as_bf16(w4_u[NC - 1])

        def rem4(rq, slot):
            lhs = jnp.concatenate([g_s[slot, rq, n, 0:TQ, :] for n in range(2 * NH)], axis=1).astype(BF16)
            r = timed(_dot(lhs, w4r))
            finish(rq, NC - 1, r)
            return r

        marks = [rem4(0, rs)]
        marks = marks * LAG
        rem4(1, rs)
        pin = [None] * 7
        done = {_ORDER[1]: 1, _ORDER[3]: 2, _ORDER[5]: 0, _ORDER[6]: 3}
        for i in _ORDER:
            slot = later(marks[-LAG])
            rhs = _as_bf16(jnp.concatenate([one_level(w4_u, e4_u, i, c2) for c2 in range(2)], axis=1))
            ex = [_dot(outer_lhs(i, lambda r1, h: g_s[slot, 2 * r1 + r2, h * NH + NH - 1, 0:TQ, :]).astype(BF16), rhs)
                  for r2 in range(2)]
            marks.append(ex[0])
            m = [None] * 7
            for jn, j in enumerate(_ORDER):
                if jn in NEWSLOT:
                    slot = later(marks[-LAG])
                lhs = jnp.concatenate(
                    [outer_lhs(j, lambda r2, p: outer_lhs(
                        i, lambda r1, h: g_s[slot, 2 * r1 + r2, h * NH + 2 * st + p, 0:TQ, :]))
                     for st in range(NS)], axis=1).astype(BF16)
                m[j] = timed(_dot(lhs, _as_bf16(jnp.concatenate([two_level(w4_u, s4_u, i, j, st) for st in range(NS)], axis=0))))
                marks.append(m[j])
            pin[i] = [x + ex[inner // 2][:, (inner % 2) * LANES:(inner % 2 + 1) * LANES]
                      for inner, x in enumerate(_combine(m))]
            if i in done:
                blk = done[i]
                for inner in (1, 2, 0, 3):
                    p = [pin[k][inner] if pin[k] is not None else None for k in range(7)]
                    cval = (lambda: (p[3] - p[4]) + p[0] + p[6], lambda: p[2] + p[4], lambda: p[1] + p[3],
                            lambda: (p[2] - p[1]) + p[0] + p[5])[blk]()
                    finish(2 * (blk // 2) + inner // 2, 2 * (blk % 2) + inner % 2, cval)
                rb = pl.multiple_of(r0 + (blk // 2) * 2 * TQ, 2 * TQ)
                for e in range(2):
                    out_copy(rb, 2 * TQ, 2 * (blk % 2) + e).start()
                if blk == 0:
                    out_copy(r0, TB, NC - 1).start()
            if i in (_ORDER[1], _ORDER[3]):
                rem4(2 if i == _ORDER[1] else 3, later(marks[-LAG]))
                marks += [marks[-1]] * LAG

        nxt = jnp.minimum(t + 1, NT - 1)
        store_z(pl.multiple_of(nxt * TB, TB), 1 - ws, toks[:len(toks) - TRIMB], 0)
        return carry

    with jax.named_scope("ph2b"):
        lax.fori_loop(0, NT, loop_b, 0)
    with jax.named_scope("tail"):
        for c in range(NC):
            out_copy(0, S, c).wait()


@jax.jit
def pallas_adaLN_cond__ssm_conv_h3__mixer_s_mlp__prompt_kernel(
    A_q: jax.Array,
    A_k: jax.Array,
    A_v: jax.Array,
    A_shift_k: jax.Array,
    A_ssm_k: jax.Array,
    A_ssm_D: jax.Array,
    B_x: jax.Array,
    B_w1: jax.Array,
    B_w2: jax.Array,
    B_w3: jax.Array,
    B_w4: jax.Array,
    c: jax.Array,
    w_mod: jax.Array,
):
    B, S, D = A_q.shape
    assert B == 1
    FF = B_w3.shape[1]
    NC = D // LANES
    NG = BLK // 8
    NBL = S // (PH * BLK)
    FP = -(-FF // (2 * LANES)) * 2 * LANES
    TILES = (384, 288, 352, 448, 576)
    assert sum(TILES) == S
    TB = 512

    args = (A_q.reshape(S, D), A_k.reshape(S, D), A_v.reshape(S, D), A_shift_k.T, A_ssm_k,
            A_ssm_D, B_w1, B_w2, B_w3.T, B_w4, c, w_mod)
    scratch = [
        pltpu.VMEM((S, D), BF16),
        pltpu.VMEM((NC, S + 16, LANES), BF16),
        pltpu.VMEM((NC, S, LANES), BF16),
        pltpu.VMEM((4, D), BF16),
        pltpu.VMEM((NC, LANES, S), BF16),
        pltpu.VMEM((D,), BF16),
        pltpu.VMEM((NC, D, LANES), BF16),
        pltpu.VMEM((NC, D, LANES), BF16),
        pltpu.VMEM((NC, FP, LANES), BF16),
        pltpu.VMEM((NC, FP, LANES), BF16),
        pltpu.VMEM((1, D), BF16),
        pltpu.VMEM((D, 6 * D), BF16),
        pltpu.VMEM((PH, 2 * BLK, BLK), BF16),
        pltpu.VMEM((PH, 2, BLK, BLK), BF16),
        pltpu.VMEM((NC, S, LANES), BF16),
        pltpu.VMEM((NC, NG, NBL, PH, 2, 8, LANES), F32),
        pltpu.VMEM((NC, NG, NBL, PH, 2, 8, LANES), F32),
        pltpu.VMEM((NC, NBL, PH, 2 * BLK, LANES), BF16),
        pltpu.VMEM((NBL, PH, BLK, LANES), BF16),
        pltpu.VMEM((NC, S, LANES), F32),
        pltpu.VMEM((6, 8, D), F32),
        pltpu.VMEM((NC, 8, LANES), F32),
        pltpu.VMEM((NC, S + 16, LANES), F32),
        pltpu.VMEM((S, D), F32),
        pltpu.VMEM((S, D), F32),
        pltpu.VMEM((NC, 2 * S, LANES), BF16),
        pltpu.VMEM((7, 7, FP // 512 * LANES, LANES), BF16),
        pltpu.VMEM((7, 7, FP // 512 * LANES, LANES), BF16),
        pltpu.VMEM((7, 2, LANES, LANES), BF16),
        pltpu.VMEM((7, 2, LANES, LANES), BF16),
        pltpu.VMEM((2, 4, FP // LANES + 1, TB // 4 + 8, LANES), F32),
        pltpu.VMEM((2, 4, NC, TB // 4 + 8, LANES), F32),
        pltpu.SMEM((1,), jnp.int32),
        pltpu.SemaphoreType.DMA((16 + len(TILES),)),
        pltpu.SemaphoreType.DMA((1,)),
    ]
    out = pl.pallas_call(
        functools.partial(_kernel, S=S, D=D, FF=FF, TILES=TILES, TB=TB),
        in_specs=[pl.BlockSpec(memory_space=pl.ANY)] * len(args),
        out_specs=pl.BlockSpec(memory_space=pl.ANY),
        out_shape=jax.ShapeDtypeStruct((S, D), BF16),
        scratch_shapes=scratch,
        compiler_params=pltpu.CompilerParams(
            vmem_limit_bytes=120 * 1024 * 1024,
            disable_bounds_checks=True,
            disable_semaphore_checks=True,
        ),
    )(*args)
    return out.reshape(B, S, D)
```

```python
import functools
import math

import jax
import jax.numpy as jnp
from jax import lax
import jax.experimental.pallas as pl
import jax.experimental.pallas.tpu as pltpu

F32 = jnp.float32
BF16 = jnp.bfloat16
U32 = jnp.uint32

LANES = 128
BLK = 128
PH = 4
EPS = 1e-05
TRIM = 60
SPLIT = 2
FREE = 30
DUM = 96
RSQ = 1
ONEP = 1
W1N = 2
W2N = 3
LAT = 1
LSETS = 0
LSTEP = 4
LB1 = 100
ZB0 = 250
ZB1 = 520
REM2 = 1
ZORD = (2, 3, 0, 1, 4, 5, 6)


def _as_bf16(x):
    return pltpu.bitcast(x, BF16)


def _lo(x):
    return pltpu.bitcast(x << 16, F32)


def _hi(x):
    return pltpu.bitcast(x & jnp.uint32(0xFFFF0000), F32)


def _dft4(re, im, sign):
    ar, ai = re[0] + re[2], im[0] + im[2]
    br, bi = re[0] - re[2], im[0] - im[2]
    cr, ci = re[1] + re[3], im[1] + im[3]
    dr, di = re[1] - re[3], im[1] - im[3]
    o0 = (ar + cr, ai + ci)
    o2 = (ar - cr, ai - ci)
    m = (br + di, bi - dr)
    p = (br - di, bi + dr)
    o1, o3 = (m, p) if sign < 0 else (p, m)
    return [o0[0], o1[0], o2[0], o3[0]], [o0[1], o1[1], o2[1], o3[1]]


def _ln(x):
    inv = 1.0 / x.shape[-1]
    m = jnp.sum(x, axis=-1, keepdims=True) * inv
    if ONEP:
        v = jnp.maximum(jnp.sum(x * x, axis=-1, keepdims=True) * inv + (EPS - m * m), EPS)
        d = x - m
    else:
        d = x - m
        v = jnp.sum(d * d, axis=-1, keepdims=True) * inv + EPS
    if RSQ:
        return d * jnp.exp2(jnp.log(v) * (-0.5 / math.log(2.0)))
    return d * lax.rsqrt(v)


def _gelu(x):
    c0 = math.sqrt(2.0 / math.pi)
    t = jnp.tanh(x * (c0 + (c0 * 0.044715) * (x * x)))
    hx = 0.5 * x
    return hx + hx * t


def _dot(a, b):
    return jnp.dot(a, b, preferred_element_type=F32)


def _dot_nt(a, b):
    return lax.dot_general(a, b, (((1,), (1,)), ((), ())), preferred_element_type=F32)


def _lhs_ops(a11, a12, a21, a22):
    return [a11 + a22, a21 + a22, a11, a22, a11 + a12, a21 - a11, a12 - a22]


def _rhs_ops(b11, b12, b21, b22):
    return [b11 + b22, b11, b12 - b22, b21 - b11, b22, b11 + b12, b21 + b22]


def _combine(m):
    return (m[3] - m[4]) + m[0] + m[6], m[2] + m[4], m[1] + m[3], (m[2] - m[1]) + m[0] + m[5]


_ORDER = (2, 4, 1, 3, 0, 6, 5)


def _kernel(q_hbm, k_hbm, v_hbm, sh_hbm, sk_hbm, sd_hbm, w1_hbm, w2_hbm, w3_hbm, w4_hbm, c_hbm, wm_hbm,
            o_hbm,
            q_v, k_v, v_v, sh_v, sk_v, sd_v, w1_v, w2_v, w3_v, w4_v, c_v, wm_v,
            fw_s, iv_s, o_v, u_s, kk_s, vv_s, wu_s, y_s, mod_s, par_s, h1_s, x_s, h_s, z_s, s3_s, s4_s, e3_s, e4_s, g_s, zf_s, zr_s, la_s,
            sem, sem_o,
            *, S, D, FF, TILES, TB):
    NC = D // LANES
    NG = BLK // 8
    LB = PH * BLK
    NBL = S // LB
    R = BLK // PH
    HALO = 16
    FP = w3_v.shape[1]
    FH = FP // 2
    NH = FH // LANES

    small = [
        pltpu.make_async_copy(sh_hbm, sh_v, sem.at[0]),
        pltpu.make_async_copy(sd_hbm, sd_v, sem.at[0]),
        pltpu.make_async_copy(c_hbm, c_v, sem.at[0]),
    ]

    def conv_copies(c):
        col = pl.ds(c * LANES if isinstance(c, int) else pl.multiple_of(c * LANES, LANES), LANES)
        return [
            pltpu.make_async_copy(sk_hbm.at[col, :], sk_v.at[c], sem.at[1 + c]),
            pltpu.make_async_copy(k_hbm.at[:, col], k_v.at[c, pl.ds(16, S), :], sem.at[1 + c]),
            pltpu.make_async_copy(v_hbm.at[:, col], v_v.at[c], sem.at[1 + c]),
        ]

    def col_copies(src, dst, c0, s):
        rows = pl.ds(0, src.shape[0])
        return [pltpu.make_async_copy(src.at[:, pl.ds((c0 + c) * LANES, LANES)], dst.at[c0 + c, rows, :], sem.at[s])
                for c in range(NC)]

    WM = (0, 3 * D, 5 * D, 6 * D)
    wm_copies = [[pltpu.make_async_copy(wm_hbm.at[:, pl.ds(WM[j], WM[j + 1] - WM[j])],
                                        wm_v.at[:, pl.ds(WM[j], WM[j + 1] - WM[j])], sem.at[6 + j])]
                 for j in range(3)]
    w_copies = [col_copies(src, dst, 0, 12 + j)
                for j, (src, dst) in enumerate(((w1_hbm, w1_v), (w2_hbm, w2_v), (w3_hbm, w3_v), (w4_hbm, w4_v)))]

    B0 = [0]
    for n in TILES:
        B0.append(B0[-1] + n)
    NA = len(TILES)
    A0 = [0] + [r + HALO for r in B0[1:-1]] + [S]
    q_copies = [
        [pltpu.make_async_copy(q_hbm.at[pl.ds(A0[t], A0[t + 1] - A0[t])], q_v.at[pl.ds(A0[t], A0[t + 1] - A0[t])],
                               sem.at[16 + t])]
        for t in range(NA)
    ]

    def start_all(cps, priority=0):
        for cp in cps:
            cp.start(priority=priority)

    def wait_all(cps):
        for cp in cps:
            cp.wait()

    def packed(ref, c0=0):
        ru = ref.bitcast(U32)
        return _as_bf16(jnp.concatenate([ru[c0 + c] for c in range(NC)], axis=1))

    first = conv_copies(0)
    start_all(first[:1] + small + first[1:] + conv_copies(1))

    for c in range(NC):
        k_v[c, 0:16, :] = jnp.zeros((16, LANES), BF16)
        h1_s[c, 0:8, :] = jnp.zeros((8, LANES), F32)
        h1_s[c, S + 8:S + 16, :] = jnp.zeros((8, LANES), F32)
        w3_v[c, FF:FP, :] = jnp.zeros((FP - FF, LANES), BF16)
        w4_v[c, FF:FP, :] = jnp.zeros((FP - FF, LANES), BF16)

    prow = lax.broadcasted_iota(jnp.int32, (BLK, BLK), 0)
    pcol = lax.broadcasted_iota(jnp.int32, (BLK, BLK), 1)
    ang = (((4 * prow + 1) * pcol) & (4 * BLK - 1)).astype(F32) * (2.0 * math.pi / (4 * BLK))
    tw = (4 * prow + 1).astype(F32) * (2.0 * math.pi / (4 * LB))
    mr, mi = jnp.cos(ang), -jnp.sin(ang)
    zr_, zi_ = jnp.cos(tw), -jnp.sin(tw)
    eye = jnp.where(prow == pcol, 1.0 / LB, 0.0).astype(BF16)
    for i in range(PH):
        both = jnp.stack([mr.reshape(NG, 8, BLK), mi.reshape(NG, 8, BLK)], axis=1).reshape(2 * BLK, BLK)
        fw_s[i] = both.astype(BF16)
        for h in range(2):
            iv_s[i, h] = _dot_nt(eye, both[h * BLK:(h + 1) * BLK, :].astype(BF16)).astype(BF16)
        if i + 1 < PH:
            mr, mi = mr * zr_ - mi * zi_, mr * zi_ + mi * zr_
    perm = jnp.where(pcol == (prow % R) * PH + prow // R, 1.0, 0.0).astype(BF16)
    fw_u = fw_s.bitcast(U32)
    iv_u = iv_s.bitcast(U32)

    wait_all(small)
    shf = sh_v[...].astype(F32)
    sdf = sd_v[...].astype(F32).reshape(1, D)
    for c in range(NC):
        par_s[c, 0:4, :] = shf[:, c * LANES:(c + 1) * LANES]
        par_s[c, 4:5, :] = sdf[:, c * LANES:(c + 1) * LANES]
    cf = c_v[...].astype(F32)
    sc = (cf * jax.nn.sigmoid(cf)).astype(BF16)
    sc16 = jnp.broadcast_to(sc, (16, D))

    def mod_chunk(j):
        mod_s[j] = _dot(sc16, wm_v[:, j * D:(j + 1) * D])[0:8, :]

    k_u = k_v.bitcast(U32)
    v_u = v_v.bitcast(U32)
    wu_u = wu_s.bitcast(U32)
    z_u = z_s.bitcast(U32)
    vv_u = vv_s.bitcast(U32)

    never = zr_[0:8, :] > 2.0

    def after(token, x):
        if token.dtype != x.dtype:
            token = pltpu.bitcast(token, x.dtype)
        return jnp.where(jnp.broadcast_to(never, x.shape), token, x)

    def split(t):
        t4 = t.reshape(NG, 2, 8, LANES)
        return t4[:, 0], t4[:, 1]

    def perm_k(c, b, toks):
        kt = [_dot_nt(perm, sk_v[c, :, b * LB + t * BLK:b * LB + (t + 1) * BLK]) for t in range(PH)]
        for r in range(BLK // 16):
            toks.append(kt[0][16 * r:16 * r + 8, :])
        return [jnp.concatenate([kt[t][i * R:(i + 1) * R, :] for t in range(PH)], axis=0).astype(BF16)
                for i in range(PH)]

    def spectrum(wts, dst, c, b, toks, dc=None, pins=None):
        tr, ti = [], []
        for i in range(PH):
            lhs = fw_u[i]
            if pins is not None and i < len(pins):
                lhs = after(pins[i], lhs.reshape(NG, 8, LANES)).reshape(BLK, LANES)
            r_, i_ = split(_dot(_as_bf16(lhs), wts[i]))
            tr.append(r_)
            ti.append(i_)
        for g in range(NG):
            toks.append(ti[PH - 1][g])
        if dc is not None:
            tr[0] = tr[0] + dc
        sr, si = _dft4(tr, ti, -1)
        for qq in range(PH):
            dst[c, :, b, qq, 0] = sr[qq]
            dst[c, :, b, qq, 1] = si[qq]

    def gated(c, b):
        w = [par_s[c, t:t + 1, :] for t in range(4)]
        kc = {}
        for o in range(-2, 2):
            words = k_u[c, pl.ds(8 + b * (LB // 2) + o, BLK, stride=2), :]
            if o > -2:
                kc[2 * o] = _lo(words)
            kc[2 * o + 1] = _hi(words)
        vc = {}
        for o in range(2):
            words = v_u[c, pl.ds(b * (LB // 2) + o, BLK, stride=2), :]
            vc[2 * o] = _lo(words)
            vc[2 * o + 1] = _hi(words)
        for i in range(PH):
            ks = kc[i] * w[0]
            for t in range(1, 4):
                ks = ks + kc[i - t] * w[t]
            wu_s[b, i] = (ks * vc[i]).astype(BF16)
        return [wu_u[b, i] for i in range(PH)]

    def kv_pins(kvb):
        return [jnp.stack([kvb[2 * m + (r % 2)][8 * (r // 2):8 * (r // 2) + 8, :] for r in range(NG)])
                for m in range(2)]

    def mac(c, us, ks, toks):
        zp = None
        for o in range(NBL):
            zr, zi = [], []
            for qq in range(PH):
                accr = acci = None
                for b in range(o + 1):
                    a_, b_ = us[0, :, b, qq, 0], us[0, :, b, qq, 1]
                    c_, d_ = ks[0, :, o - b, qq, 0], ks[0, :, o - b, qq, 1]
                    if qq == 0 and b == o:
                        a_ = after(toks[o], a_)
                    tr_ = a_ * c_ - b_ * d_
                    ti_ = a_ * d_ + b_ * c_
                    accr = tr_ if accr is None else accr + tr_
                    acci = ti_ if acci is None else acci + ti_
                zr.append(accr)
                zi.append(acci)
            if zp is None:
                yr, yi = zr, zi
            else:
                yr = [zr[qq] - zp[1][qq] for qq in range(PH)]
                yi = [zi[qq] + zp[0][qq] for qq in range(PH)]
            zp = (zr, zi)
            vr, vi = _dft4(yr, yi, +1)
            for i in range(PH):
                vv_s[c, o, i] = jnp.stack([vr[i], vi[i]], axis=1).reshape(2 * BLK, LANES).astype(BF16)

    def inverse(c, toks, pins=None, between=None):
        HB = BLK // 2
        for o in range(NBL):
            for i in range(PH):
                yv = None
                for h in range(2):
                    lhs = iv_u[i, h]
                    if pins is not None and h == 0:
                        pin = pins[o][i % 2][8 * (i // 2):8 * (i // 2) + 8]
                        lhs = after(pin, lhs.reshape(8, 8, LANES)).reshape(HB, LANES)
                    t = _dot(_as_bf16(lhs), _as_bf16(vv_u[c, o, i, h * HB:(h + 1) * HB, :]))
                    yv = t if yv is None else yv + t
                if i % 2 == 0:
                    for r in range(BLK // 16):
                        toks.append(yv[16 * r:16 * r + 8, :])
                y_s[c, pl.ds(o * LB + i, BLK, stride=PH), :] = yv
            if between is not None:
                between(o)

    def mac_tokens(toks):
        n = len(toks) - 3
        cum = (44, 128, 244, 392)
        return [jnp.stack([toks[max(0, ((g * 392 + cum[o]) * n) // (392 * NG) - 1)] for g in range(NG)])
                for o in range(NBL)]

    def conv_round(c, fwd, mul, inv, between=None):
        toks = []
        kv = pins = None
        cur = 1 if mul else 0
        if fwd or mul:
            win = pl.ds(c - cur, 2 if fwd and mul else 1)
            us, ks = u_s.at[win], kk_s.at[win]
        if fwd:
            kv = [gated(c, b) for b in range(NBL)]
            pins = [kv_pins(kv[b]) for b in range(NBL)]
        if inv:
            inverse(c - 2, toks, pins, between)
            if fwd:
                toks = []
        if fwd:
            wts = [perm_k(c, b, toks) for b in range(NBL)]
            dc = par_s[c, 4:5, :]
            if inv:
                order = ('k0', 'u0', 'k1', 'u1', 'k2', 'u2', 'k3', 'u3')
                pin_at = {}
            else:
                order = ('k0', 'k1', 'k2', 'u0', 'k3', 'u1', 'u2', 'u3')
                pin_at = {'k0': 0, 'k1': 1, 'u0': 2, 'k3': 3}
            for name in order:
                b = int(name[1])
                pin = pins[pin_at[name]] if name in pin_at else None
                tk = [] if (pin is not None and mul) else toks
                if name[0] == 'k':
                    spectrum(wts[b], ks, cur, b, tk, dc if b == 0 else None, pin)
                else:
                    spectrum([_as_bf16(x) for x in kv[b]], us, cur, b, tk, None, pin)
                if tk is not toks:
                    toks += tk[::4]
        if mul:
            mac(c - 1, us, ks, mac_tokens(toks))

    def tokens_of(x):
        return [x[8 * r:8 * r + 8, c * LANES:(c + 1) * LANES] for c in range(NC) for r in range(x.shape[0] // 8)]

    def store_bf16(ref, r0, x):
        for c in range(NC):
            ref[c, r0:r0 + x.shape[0], :] = x[:, c * LANES:(c + 1) * LANES].astype(BF16)

    def load_bf16(ref_u, r0, n):
        return _as_bf16(jnp.concatenate([ref_u[c, pl.ds(r0 // 2, n // 2), :] for c in range(NC)], axis=1))

    def pick(toks, n, free):
        if toks is None:
            return [None] * n
        idx = [(r * (len(toks) + free)) // n - free for r in range(n)]
        return [toks[i] if i >= 0 else None for i in idx]

    def hold(x, tks):
        f = len([k for k in tks if k is None])
        n = len(tks)
        if f == n:
            return x
        first = after(jnp.stack(tks[f:]), x[8 * f:, 0:LANES].reshape(n - f, 8, LANES)).reshape(8 * (n - f), LANES)
        if f:
            first = jnp.concatenate([x[:8 * f, 0:LANES], first], axis=0)
        return jnp.concatenate([first, x[:, LANES:]], axis=1)

    def mods_a():
        ga = mod_s[2, 0:1, :]
        return ga * (1.0 + mod_s[1, 0:1, :]), ga * mod_s[0, 0:1, :]

    def mods_b():
        return 1.0 + mod_s[4, 0:1, :], mod_s[3, 0:1, :]

    def stage_p1(r0, r1, tks, ma):
        q = hold(q_v[r0:r1, :].astype(F32), tks)
        y = jnp.concatenate([y_s[c, r0:r1, :] for c in range(NC)], axis=1)
        x = q + (_ln(q) * ma[0] + ma[1]) * y
        x_s[r0:r1, :] = x
        return _ln(x)

    def stage_p2(r0, r1, nx, mb):
        h = nx * mb[0] + mb[1]
        h_s[r0:r1, :] = h
        store_bf16(z_s, r0, _ln(h))

    def stage_p(t, toks, free):
        lo, hi = A0[t], A0[t + 1]
        stage_p2(lo, hi, stage_p1(lo, hi, pick(toks, (hi - lo) // 8, free), mods_a()), mods_b())

    def filler(t):
        if DUM:
            red = jnp.sum(y_s[t, 0:8 * DUM, :], axis=-1, keepdims=True).reshape(DUM, 8, 1)
            g_s[t // 4, t % 4, 2 * NH, 0:8, :] = jnp.broadcast_to(jnp.sum(red, axis=0), (8, LANES))

    def chunks(r0, r1, k):
        n = (r1 - r0) // 16
        cuts = [r0 + 16 * ((n * j) // k) for j in range(k + 1)]
        return list(zip(cuts[:-1], cuts[1:]))

    def stage_m1(t, k):
        toks = []
        for r0, r1 in chunks(A0[t], A0[t + 1], k):
            g1 = _gelu(_dot(load_bf16(z_u, r0, r1 - r0), packed(w1_v)))
            for c in range(NC):
                h1_s[c, r0 + 8:r1 + 8, :] = g1[:, c * LANES:(c + 1) * LANES]
            toks += tokens_of(g1)
        return toks

    grp = D // 4
    shifts = (-1, 1, -2, 2)

    def stage_m2(t, k):
        out = []
        for r0, r1 in chunks(B0[t], B0[t + 1], k):
            n = r1 - r0
            lane = lax.broadcasted_iota(jnp.int32, (n, LANES), 1)
            parts = []
            for c in range(NC):
                lo, hi = c * LANES, (c + 1) * LANES
                g_lo, g_hi = lo // grp, (hi - 1) // grp
                val = h1_s[c, pl.ds(r0 + 8 + shifts[g_lo], n), :]
                if g_hi != g_lo:
                    other = h1_s[c, pl.ds(r0 + 8 + shifts[g_hi], n), :]
                    val = jnp.where(lane < (g_hi * grp - lo), val, other)
                parts.append(val)
            x1 = h_s[r0:r1, :] + _dot(jnp.concatenate(parts, axis=1).astype(BF16), packed(w2_v))
            h_s[r0:r1, :] = x1
            out += tokens_of(x1)
        return out

    TQ = TB // 4
    NT = S // TB

    def store_z(r0, slot, toks, free):
        zn = _ln(hold(h_s[pl.ds(r0, TB), :], pick(toks, TB // 8, free)))
        for rq in range(4):
            for c in range(NC - 1):
                zf_s[slot, rq, c, 0:TQ, :] = zn[rq * TQ:(rq + 1) * TQ, c * LANES:(c + 1) * LANES]
        zr_s[slot] = zn[:, (NC - 1) * LANES:].astype(BF16)

    def outer_lhs(i, blk):
        terms = ((0, 0, 1, 1, 1), (1, 0, 1, 1, 1), (0, 0), (1, 1), (0, 0, 1, 0, 1), (1, 0, -1, 0, 0), (0, 1, -1, 1, 1))[i]
        x = blk(terms[0], terms[1])
        if len(terms) > 2:
            y = blk(terms[3], terms[4])
            x = x + y if terms[2] > 0 else x - y
        return x

    def z_ops(slot_of, toks):
        ng = TQ // 16

        def held(x, k):
            tk = jnp.stack([toks[((k * ng + r) * len(toks)) // (7 * ng)] for r in range(ng)])
            x4 = x.reshape(ng, 2, 8, LANES)
            return jnp.stack([after(tk, x4[:, 0]), x4[:, 1]], axis=1).reshape(TQ, LANES)

        for k, i in enumerate(ZORD):
            slot = slot_of()
            so = [outer_lhs(i, lambda r1, k1: zf_s[slot, 2 * r1 + r2, 2 * k1 + k2, 0:TQ, :])
                  for r2 in range(2) for k2 in range(2)]
            for j, x in enumerate(_lhs_ops(held(so[0], k), so[1], so[2], held(so[3], k))):
                la_s[i, j] = x.astype(BF16)

    NS = NH // 2

    RAW = (1, 4)

    def weight_ops(src, dst, ext, transposed, toks):
        ng = LANES // 16
        total = (NS * 7 + 2) * ng

        def tile(c, n):
            return src[c, n * LANES:(n + 1) * LANES, :].astype(F32)

        def held(x, pos, step):
            tk = jnp.stack([toks[((pos + r * step) * len(toks)) // total] for r in range(ng)])
            x4 = x.reshape(ng, 2, 8, LANES)
            return jnp.stack([after(tk, x4[:, 0]), x4[:, 1]], axis=1).reshape(LANES, LANES)

        def outer(c2, n, pos=None):
            b11, b22 = tile(c2, n), tile(2 + c2, NH + n)
            if pos is not None:
                b11, b22 = held(b11, pos, 1), held(b22, pos, 1)
            e1, e2 = tile(c2, NH + n), tile(2 + c2, n)
            return _rhs_ops(b11, e1, e2, b22) if transposed else _rhs_ops(b11, e2, e1, b22)

        for c2 in range(2):
            for i, x in enumerate(outer(c2, NH - 1, c2 * ng)):
                if i not in RAW:
                    ext[i, c2] = x.astype(BF16)
        for st in range(NS):
            t00, t11 = outer(0, 2 * st), outer(1, 2 * st + 1)
            t01, t10 = outer(0, 2 * st + 1), outer(1, 2 * st)
            for k, i in enumerate((1, 5, 2, 4, 0, 3, 6)):
                pos = (2 + st * 7) * ng + k
                a, d = held(t00[i], pos, 7), held(t11[i], pos, 7)
                ops = _rhs_ops(a, t01[i], t10[i], d) if transposed else _rhs_ops(a, t10[i], t01[i], d)
                for j, x in enumerate(ops):
                    if i not in RAW or j not in RAW:
                        dst[i, j, st * LANES:(st + 1) * LANES, :] = x.astype(BF16)

    with jax.named_scope("r0_wait"):
        wait_all(conv_copies(0))
    with jax.named_scope("r0"):
        start_all(conv_copies(2) + conv_copies(3) + conv_copies(4))
        conv_round(0, True, False, False)
    with jax.named_scope("r1_wait"):
        wait_all(conv_copies(1))
    with jax.named_scope("r1"):
        start_all(wm_copies[0] + q_copies[0] + wm_copies[1] + w_copies[0])
        conv_round(1, True, True, False)

    def full_round(c, carry):
        wait_all(conv_copies(c))
        conv_round(c, True, True, True)
        return carry

    with jax.named_scope("r234"):
        lax.fori_loop(2, NC, full_round, 0)
    with jax.named_scope("r5"):
        start_all(q_copies[1] + w_copies[1] + sum(q_copies[2:], []) + w_copies[2] + w_copies[3] + wm_copies[2], 1)
        conv_round(NC, False, True, True)
    with jax.named_scope("r6_wait"):
        wait_all(wm_copies[0] + q_copies[0])
    with jax.named_scope("r6"):
        for j in range(3):
            mod_chunk(j)
        conv_round(NC + 1, False, False, True)
        nx0 = stage_p1(0, A0[1], [None], mods_a())
    with jax.named_scope("p2_wait"):
        wait_all(wm_copies[1])
    with jax.named_scope("p2"):
        mod_chunk(4)
        mod_chunk(3)
        stage_p2(0, A0[1], nx0, mods_b())
    with jax.named_scope("w1_wait"):
        wait_all(w_copies[0])
    with jax.named_scope("m1_0"):
        stage_m1(0, 4)
    with jax.named_scope("w2_wait"):
        wait_all(q_copies[1] + w_copies[1])
    with jax.named_scope("m2_0"):
        toks = stage_m2(0, 4)
        stage_p(1, toks[:len(toks) - TRIM], FREE)
        filler(0)
    for t in range(1, NA):
        with jax.named_scope("a%d" % t):
            if t + 1 < NA:
                wait_all(q_copies[t + 1])
            else:
                wait_all(w_copies[2] + w_copies[3] + wm_copies[2])
            t1 = stage_m1(t, SPLIT)
            t2 = stage_m2(t, SPLIT)

            def weighted(trim):
                return [x for x in t1 for _ in range(W1N)] + [x for x in t2[:len(t2) - trim] for _ in range(W2N)]

            if t + 1 < NA:
                stage_p(t + 1, weighted(TRIM), FREE * W2N)
            if t == NA - 1 - LAT:
                toks = weighted(TRIM // 2)
                store_z(0, 0, toks if LAT else toks[:len(toks) // 2], FREE * W2N)
            if t == NA - 1:
                mod_chunk(NC)
                toks = weighted(20)
                cut = len(toks) // 2
                weight_ops(w3_v, s3_s, e3_s, True, toks[:cut])
                weight_ops(w4_v, s4_s, e4_s, False, toks[cut:])
                z_ops(lambda: 0, toks if LAT else toks[(len(toks) * 5) // 8:])
            if t + 1 < NA or not LAT:
                filler(t)

    gb = mod_s[NC, 0:1, :]
    w3_u, w4_u, s3_u, s4_u, e3_u, e4_u = (r.bitcast(U32) for r in (w3_v, w4_v, s3_s, s4_s, e3_s, e4_s))
    HL = LANES // 2
    la_u = la_s.bitcast(U32)
    zr_u = zr_s.bitcast(U32)

    def out_copy(r0, n, c):
        rows = pl.ds(r0, n)
        return pltpu.make_async_copy(o_v.at[c, rows, :], o_hbm.at[rows, pl.ds(c * LANES, LANES)], sem_o.at[0])

    def one_level(w_u, e_u, i, c2):
        if i not in RAW:
            return e_u[i, c2]
        d = RAW.index(i)
        n = d * NH + NH - 1
        return w_u[2 * d + c2, n * HL:(n + 1) * HL, :]

    def two_level(w_u, s_u, i, j, st):
        if i not in RAW or j not in RAW:
            return s_u[i, j, st * HL:(st + 1) * HL, :]
        d, e = RAW.index(i), RAW.index(j)
        n = d * NH + 2 * st + e
        return w_u[2 * d + e, n * HL:(n + 1) * HL, :]

    def loop_b(t, carry):
        r0 = pl.multiple_of(t * TB, TB)
        ws = t & 1

        count = [0]

        def fresh():
            count[0] += 1
            return lax.rem(t + 2 * count[0], 2)

        zr = [_as_bf16(zr_u[ws, rq * (TQ // 2):(rq + 1) * (TQ // 2), :]) for rq in range(4)]
        ltoks = []

        def light(x):
            ltoks.extend(x[8 * r:8 * r + 8, 0:LANES] for r in range(x.shape[0] // 8))

        def z_outer(i, slot):
            return [[outer_lhs(i, lambda r1, k1: zf_s[slot, 2 * r1 + r2, 2 * k1 + k2, 0:TQ, :]) for k2 in range(2)]
                    for r2 in range(2)]

        def rem3(rq, n):
            return _dot_nt(zr[rq], _as_bf16(w3_u[NC - 1, n * HL:(n + 1) * HL, :]))

        def put_g(rq, n, pre):
            g_s[ws, rq, n, 0:TQ, :] = _gelu(pre)

        rem = {}
        for rq in range(4):
            for h in range(2):
                rem[rq, h * NH + NH - 1] = rem3(rq, h * NH + NH - 1)
        for st in range(NS):
            rem[3, NH + 2 * st + 1] = rem3(3, NH + 2 * st + 1)
        m = [None] * 7
        for i in _ORDER:
            rhs = _as_bf16(jnp.concatenate([one_level(w3_u, e3_u, i, c2) for c2 in range(2)], axis=1))
            so = z_outer(i, fresh())
            m[i] = [_dot_nt(jnp.concatenate(so[r2], axis=1).astype(BF16), rhs) for r2 in range(2)]
        for r2 in range(2):
            for blk, cval in enumerate(_combine([m[i][r2] for i in range(7)])):
                rq, n = 2 * (blk // 2) + r2, (blk % 2) * NH + NH - 1
                put_g(rq, n, cval + rem[rq, n])
        for st in range(NS):
            todo = [(2 * r1 + r2, h * NH + 2 * st + p) for r1, h in ((0, 1), (1, 0), (0, 0), (1, 1))
                    for r2 in range(2) for p in range(2)]
            todo = [x for x in todo if x not in rem]
            for key in todo[:8]:
                rem[key] = rem3(*key)
            if st >= LSETS:
                light(rem[todo[1]])
                light(rem[todo[5]])
            todo = todo[8:]
            pin = [None] * 7
            for i in _ORDER:
                m = [None] * 7
                for j in _ORDER:
                    m[j] = _dot_nt(_as_bf16(la_u[i, j]), _as_bf16(two_level(w3_u, s3_u, i, j, st)))
                if st >= LSETS and i in (2, 1, 0):
                    light(m[_ORDER[1]])
                    light(m[_ORDER[5]])
                key = todo.pop(0)
                rem[key] = rem3(*key)
                pin[i] = _combine(m)
            for inner in range(4):
                for blk, cval in enumerate(_combine([pin[i][inner] for i in range(7)])):
                    rq, n = 2 * (blk // 2) + inner // 2, (blk % 2) * NH + 2 * st + inner % 2
                    put_g(rq, n, cval + rem[rq, n])

        toks = []

        def timed(x):
            toks.extend(x[8 * r:8 * r + 8, 0:LANES] for r in range(x.shape[0] // 8))
            return x

        def finish(rq, c, h2):
            rows = pl.ds(pl.multiple_of(r0 + rq * TQ, TQ), TQ)
            cols = slice(c * LANES, (c + 1) * LANES)
            o_v[c, rows, :] = (x_s[rows, cols] + gb[:, cols] * (h_s[rows, cols] + h2)).astype(BF16)

        kord = [NH - 1, 2 * NH - 1] + [h * NH + n for st in range(NS) for h in (1, 0) for n in (2 * st + 1, 2 * st)]
        w4r = _as_bf16(jnp.concatenate([w4_u[NC - 1, n * HL:(n + 1) * HL, :] for n in kord], axis=0))

        def rem4(rq, slot):
            lhs = jnp.concatenate([g_s[slot, rq, n, 0:TQ, :] for n in kord], axis=1).astype(BF16)
            r = timed(_dot(lhs, w4r))
            finish(rq, NC - 1, r)

        rem4(0, fresh())
        rem4(1, fresh())
        pin = [None] * 7
        done = {_ORDER[1]: 1, _ORDER[3]: 2, _ORDER[5]: 0, _ORDER[6]: 3}
        for i in _ORDER:
            slot = fresh()
            rhs = _as_bf16(jnp.concatenate([one_level(w4_u, e4_u, i, c2) for c2 in range(2)], axis=1))
            ex = [_dot(outer_lhs(i, lambda r1, h: g_s[slot, 2 * r1 + r2, h * NH + NH - 1, 0:TQ, :]).astype(BF16), rhs)
                  for r2 in range(2)]
            m = [None] * 7
            for j in _ORDER:
                slot = fresh()
                lhs = jnp.concatenate(
                    [outer_lhs(j, lambda r2, p: outer_lhs(
                        i, lambda r1, h: g_s[slot, 2 * r1 + r2, h * NH + 2 * st + p, 0:TQ, :]))
                     for st in range(NS)], axis=1).astype(BF16)
                m[j] = timed(_dot(lhs, _as_bf16(jnp.concatenate([two_level(w4_u, s4_u, i, j, st) for st in range(NS)], axis=0))))
            pin[i] = [x + ex[inner // 2][:, (inner % 2) * LANES:(inner % 2 + 1) * LANES]
                      for inner, x in enumerate(_combine(m))]
            if i in done:
                blk = done[i]
                for inner in (1, 2, 0, 3):
                    p = [pin[k][inner] if pin[k] is not None else None for k in range(7)]
                    cval = (lambda: (p[3] - p[4]) + p[0] + p[6], lambda: p[2] + p[4], lambda: p[1] + p[3],
                            lambda: (p[2] - p[1]) + p[0] + p[5])[blk]()
                    finish(2 * (blk // 2) + inner // 2, 2 * (blk % 2) + inner % 2, cval)
                rb = pl.multiple_of(r0 + (blk // 2) * 2 * TQ, 2 * TQ)
                for e in range(2):
                    out_copy(rb, 2 * TQ, 2 * (blk % 2) + e).start()
                if blk == 0:
                    out_copy(r0, 3 * TQ, NC - 1).start()
            if i == _ORDER[REM2]:
                rem4(2, fresh())
        rem4(3, fresh())
        out_copy(pl.multiple_of(r0 + 3 * TQ, TQ), TQ, NC - 1).start()

        nxt = jnp.minimum(t + 1, NT - 1)
        store_z(pl.multiple_of(nxt * TB, TB), 1 - ws, ltoks[::LSTEP] + toks[:LB1], 0)
        z_ops(lambda: 1 - fresh(), toks[ZB0:ZB1])
        return carry

    with jax.named_scope("ph2b"):
        lax.fori_loop(0, NT, loop_b, 0)
    with jax.named_scope("tail"):
        for c in range(NC):
            out_copy(0, S, c).wait()


@jax.jit
def pallas_adaLN_cond__ssm_conv_h3__mixer_s_mlp__prompt_kernel(
    A_q: jax.Array,
    A_k: jax.Array,
    A_v: jax.Array,
    A_shift_k: jax.Array,
    A_ssm_k: jax.Array,
    A_ssm_D: jax.Array,
    B_x: jax.Array,
    B_w1: jax.Array,
    B_w2: jax.Array,
    B_w3: jax.Array,
    B_w4: jax.Array,
    c: jax.Array,
    w_mod: jax.Array,
):
    B, S, D = A_q.shape
    assert B == 1
    FF = B_w3.shape[1]
    NC = D // LANES
    NG = BLK // 8
    NBL = S // (PH * BLK)
    FP = -(-FF // (2 * LANES)) * 2 * LANES
    TILES = (400, 400, 608, 640)
    assert sum(TILES) == S
    TB = 512

    args = (A_q.reshape(S, D), A_k.reshape(S, D), A_v.reshape(S, D), A_shift_k.T, A_ssm_k,
            A_ssm_D, B_w1, B_w2, B_w3.T, B_w4, c, w_mod)
    scratch = [
        pltpu.VMEM((S, D), BF16),
        pltpu.VMEM((NC, S + 16, LANES), BF16),
        pltpu.VMEM((NC, S, LANES), BF16),
        pltpu.VMEM((4, D), BF16),
        pltpu.VMEM((NC, LANES, S), BF16),
        pltpu.VMEM((D,), BF16),
        pltpu.VMEM((NC, D, LANES), BF16),
        pltpu.VMEM((NC, D, LANES), BF16),
        pltpu.VMEM((NC, FP, LANES), BF16),
        pltpu.VMEM((NC, FP, LANES), BF16),
        pltpu.VMEM((1, D), BF16),
        pltpu.VMEM((D, 6 * D), BF16),
        pltpu.VMEM((PH, 2 * BLK, BLK), BF16),
        pltpu.VMEM((PH, 2, BLK, BLK), BF16),
        pltpu.VMEM((NC, S, LANES), BF16),
        pltpu.VMEM((NC, NG, NBL, PH, 2, 8, LANES), F32),
        pltpu.VMEM((NC, NG, NBL, PH, 2, 8, LANES), F32),
        pltpu.VMEM((NC, NBL, PH, 2 * BLK, LANES), BF16),
        pltpu.VMEM((NBL, PH, BLK, LANES), BF16),
        pltpu.VMEM((NC, S, LANES), F32),
        pltpu.VMEM((6, 8, D), F32),
        pltpu.VMEM((NC, 8, LANES), F32),
        pltpu.VMEM((NC, S + 16, LANES), F32),
        pltpu.VMEM((S, D), F32),
        pltpu.VMEM((S, D), F32),
        pltpu.VMEM((NC, S, LANES), BF16),
        pltpu.VMEM((7, 7, FP // 512 * LANES, LANES), BF16),
        pltpu.VMEM((7, 7, FP // 512 * LANES, LANES), BF16),
        pltpu.VMEM((7, 2, LANES, LANES), BF16),
        pltpu.VMEM((7, 2, LANES, LANES), BF16),
        pltpu.VMEM((2, 4, FP // LANES + 1, TB // 4 + 8, LANES), F32),
        pltpu.VMEM((2, 4, NC, TB // 4 + 8, LANES), F32),
        pltpu.VMEM((2, TB, LANES), BF16),
        pltpu.VMEM((7, 7, TB // 4, LANES), BF16),
        pltpu.SemaphoreType.DMA((16 + len(TILES),)),
        pltpu.SemaphoreType.DMA((1,)),
    ]
    out = pl.pallas_call(
        functools.partial(_kernel, S=S, D=D, FF=FF, TILES=TILES, TB=TB),
        in_specs=[pl.BlockSpec(memory_space=pl.ANY)] * len(args),
        out_specs=pl.BlockSpec(memory_space=pl.ANY),
        out_shape=jax.ShapeDtypeStruct((S, D), BF16),
        scratch_shapes=scratch,
        compiler_params=pltpu.CompilerParams(
            vmem_limit_bytes=120 * 1024 * 1024,
            disable_bounds_checks=True,
            disable_semaphore_checks=True,
        ),
    )(*args)
    return out.reshape(B, S, D)
```

```python
import functools
import math

import jax
import jax.numpy as jnp
from jax import lax
import jax.experimental.pallas as pl
import jax.experimental.pallas.tpu as pltpu

F32 = jnp.float32
BF16 = jnp.bfloat16
U32 = jnp.uint32

LANES = 128
BLK = 128
PH = 4
EPS = 1e-05
TRIM = 60
SPLIT = 2
FREE = 30
DUM = 96
RSQ = 1
ONEP = 1
LN1 = 999
KP = 16
VP = 0
YP = 0
GR = 8160
ZR = 2720
FT = 0
DUMB = 1
W1N = 2
W2N = 3
LAT = 1
LSETS = 0
LSTEP = 4
LB1 = 0
ZB0 = 0
ZB1 = 140
REM2 = 1
ZORD = (2, 3, 0, 1, 4, 5, 6)


def _as_bf16(x):
    return pltpu.bitcast(x, BF16)


def _lo(x):
    return pltpu.bitcast(x << 16, F32)


def _hi(x):
    return pltpu.bitcast(x & jnp.uint32(0xFFFF0000), F32)


def _dft4(re, im, sign):
    ar, ai = re[0] + re[2], im[0] + im[2]
    br, bi = re[0] - re[2], im[0] - im[2]
    cr, ci = re[1] + re[3], im[1] + im[3]
    dr, di = re[1] - re[3], im[1] - im[3]
    o0 = (ar + cr, ai + ci)
    o2 = (ar - cr, ai - ci)
    m = (br + di, bi - dr)
    p = (br - di, bi + dr)
    o1, o3 = (m, p) if sign < 0 else (p, m)
    return [o0[0], o1[0], o2[0], o3[0]], [o0[1], o1[1], o2[1], o3[1]]


def _ln(x):
    inv = 1.0 / x.shape[-1]
    m = jnp.sum(x, axis=-1, keepdims=True) * inv
    if ONEP:
        v = jnp.maximum(jnp.sum(x * x, axis=-1, keepdims=True) * inv + (EPS - m * m), EPS)
        d = x - m
    else:
        d = x - m
        v = jnp.sum(d * d, axis=-1, keepdims=True) * inv + EPS
    if RSQ:
        return d * jnp.exp2(jnp.log(v) * (-0.5 / math.log(2.0)))
    return d * lax.rsqrt(v)


def _gelu(x):
    c0 = math.sqrt(2.0 / math.pi)
    t = jnp.tanh(x * (c0 + (c0 * 0.044715) * (x * x)))
    hx = 0.5 * x
    return hx + hx * t


def _dot(a, b):
    return jnp.dot(a, b, preferred_element_type=F32)


def _dot_nt(a, b):
    return lax.dot_general(a, b, (((1,), (1,)), ((), ())), preferred_element_type=F32)


def _lhs_ops(a11, a12, a21, a22):
    return [a11 + a22, a21 + a22, a11, a22, a11 + a12, a21 - a11, a12 - a22]


def _rhs_ops(b11, b12, b21, b22):
    return [b11 + b22, b11, b12 - b22, b21 - b11, b22, b11 + b12, b21 + b22]


def _combine(m):
    return (m[3] - m[4]) + m[0] + m[6], m[2] + m[4], m[1] + m[3], (m[2] - m[1]) + m[0] + m[5]


_ORDER = (2, 4, 1, 3, 0, 6, 5)


def _kernel(q_hbm, k_hbm, v_hbm, sh_hbm, sk_hbm, sd_hbm, w1_hbm, w2_hbm, w3_hbm, w4_hbm, c_hbm, wm_hbm,
            o_hbm,
            q_v, k_v, v_v, sh_v, sk_v, sd_v, w1_v, w2_v, w3_v, w4_v, c_v, wm_v,
            fw_s, iv_s, o_v, u_s, kk_s, vv_s, wu_s, y_s, mod_s, par_s, h1_s, x_s, h_s, z_s, s3_s, s4_s, e4_s, g_s, zf_s, zr_s, la_s,
            sem, sem_o,
            *, S, D, FF, TILES, TB):
    NC = D // LANES
    NG = BLK // 8
    LB = PH * BLK
    NBL = S // LB
    R = BLK // PH
    HALO = 16
    FP = w4_v.shape[1]
    FH = FP // 2
    NH = FH // LANES

    small = [
        pltpu.make_async_copy(sh_hbm, sh_v, sem.at[0]),
        pltpu.make_async_copy(sd_hbm, sd_v, sem.at[0]),
        pltpu.make_async_copy(c_hbm, c_v, sem.at[0]),
    ]

    def conv_copies(c):
        col = pl.ds(c * LANES if isinstance(c, int) else pl.multiple_of(c * LANES, LANES), LANES)
        return [
            pltpu.make_async_copy(sk_hbm.at[col, :], sk_v.at[c], sem.at[1 + c]),
            pltpu.make_async_copy(k_hbm.at[:, col], k_v.at[c, pl.ds(16, S), :], sem.at[1 + c]),
            pltpu.make_async_copy(v_hbm.at[:, col], v_v.at[c, pl.ds(0, S), :], sem.at[1 + c]),
        ]

    def col_copies(src, dst, c0, s):
        rows = pl.ds(0, src.shape[0])
        return [pltpu.make_async_copy(src.at[:, pl.ds((c0 + c) * LANES, LANES)], dst.at[c0 + c, rows, :], sem.at[s])
                for c in range(NC)]

    WM = (0, 3 * D, 5 * D, 6 * D)
    wm_copies = [[pltpu.make_async_copy(wm_hbm.at[:, pl.ds(WM[j], WM[j + 1] - WM[j])],
                                        wm_v.at[:, pl.ds(WM[j], WM[j + 1] - WM[j])], sem.at[6 + j])]
                 for j in range(3)]
    w_copies = [col_copies(src, dst, 0, 12 + j)
                for j, (src, dst) in enumerate(((w1_hbm, w1_v), (w2_hbm, w2_v), (w3_hbm, w3_v), (w4_hbm, w4_v)))]

    B0 = [0]
    for n in TILES:
        B0.append(B0[-1] + n)
    NA = len(TILES)
    A0 = [0] + [r + HALO for r in B0[1:-1]] + [S]
    q_copies = [
        [pltpu.make_async_copy(q_hbm.at[pl.ds(A0[t], A0[t + 1] - A0[t])], q_v.at[pl.ds(A0[t], A0[t + 1] - A0[t])],
                               sem.at[16 + t])]
        for t in range(NA)
    ]

    def start_all(cps, priority=0):
        for cp in cps:
            cp.start(priority=priority)

    def wait_all(cps):
        for cp in cps:
            cp.wait()

    def packed(ref, c0=0):
        ru = ref.bitcast(U32)
        return _as_bf16(jnp.concatenate([ru[c0 + c] for c in range(NC)], axis=1))

    first = conv_copies(0)
    start_all(first[:1] + small + first[1:] + conv_copies(1))

    for c in range(NC):
        k_v[c, 0:16, :] = jnp.zeros((16, LANES), BF16)
        h1_s[c, 0:8, :] = jnp.zeros((8, LANES), F32)
        h1_s[c, S + 8:S + 16, :] = jnp.zeros((8, LANES), F32)
        w4_v[c, FF:FP, :] = jnp.zeros((FP - FF, LANES), BF16)

    prow = lax.broadcasted_iota(jnp.int32, (BLK, BLK), 0)
    pcol = lax.broadcasted_iota(jnp.int32, (BLK, BLK), 1)
    ang = (((4 * prow + 1) * pcol) & (4 * BLK - 1)).astype(F32) * (2.0 * math.pi / (4 * BLK))
    tw = (4 * prow + 1).astype(F32) * (2.0 * math.pi / (4 * LB))
    mr, mi = jnp.cos(ang), -jnp.sin(ang)
    zr_, zi_ = jnp.cos(tw), -jnp.sin(tw)
    eye = jnp.where(prow == pcol, 1.0 / LB, 0.0).astype(BF16)
    for i in range(PH):
        both = jnp.stack([mr.reshape(NG, 8, BLK), mi.reshape(NG, 8, BLK)], axis=1).reshape(2 * BLK, BLK)
        fw_s[i] = both.astype(BF16)
        for h in range(2):
            iv_s[i, h] = _dot_nt(eye, both[h * BLK:(h + 1) * BLK, :].astype(BF16)).astype(BF16)
        if i + 1 < PH:
            mr, mi = mr * zr_ - mi * zi_, mr * zi_ + mi * zr_
    perm = jnp.where(pcol == (prow % R) * PH + prow // R, 1.0, 0.0).astype(BF16)
    fw_u = fw_s.bitcast(U32)
    iv_u = iv_s.bitcast(U32)

    wait_all(small)
    shf = sh_v[...].astype(F32)
    sdf = sd_v[...].astype(F32).reshape(1, D)
    for c in range(NC):
        par_s[c, 0:4, :] = shf[:, c * LANES:(c + 1) * LANES]
        par_s[c, 4:5, :] = sdf[:, c * LANES:(c + 1) * LANES]
    cf = c_v[...].astype(F32)
    sc = (cf * jax.nn.sigmoid(cf)).astype(BF16)
    sc16 = jnp.broadcast_to(sc, (16, D))

    def mod_chunk(j):
        mod_s[j] = _dot(sc16, wm_v[:, j * D:(j + 1) * D])[0:8, :]

    k_u = k_v.bitcast(U32)
    v_u = v_v.bitcast(U32)
    wu_u = wu_s.bitcast(U32)
    z_u = z_s.bitcast(U32)
    vv_u = vv_s.bitcast(U32)

    never = zr_[0:8, :] > 2.0

    def after(token, x):
        if token.dtype != x.dtype:
            token = pltpu.bitcast(token, x.dtype)
        return jnp.where(jnp.broadcast_to(never, x.shape), token, x)

    def split(t):
        t4 = t.reshape(NG, 2, 8, LANES)
        return t4[:, 0], t4[:, 1]

    def perm_k(c, b, toks):
        kt = [_dot_nt(perm, sk_v[c, :, b * LB + t * BLK:b * LB + (t + 1) * BLK]) for t in range(PH)]
        for r in range(BLK // 16):
            toks.append(kt[0][16 * r:16 * r + 8, :])
        return [jnp.concatenate([kt[t][i * R:(i + 1) * R, :] for t in range(PH)], axis=0).astype(BF16)
                for i in range(PH)]

    def spectrum(wts, dst, c, b, toks, dc=None, pins=None):
        tr, ti = [], []
        for i in range(PH):
            lhs = fw_u[i]
            if pins is not None and i < len(pins):
                lhs = after(pins[i], lhs.reshape(NG, 8, LANES)).reshape(BLK, LANES)
            r_, i_ = split(_dot(_as_bf16(lhs), wts[i]))
            tr.append(r_)
            ti.append(i_)
        for g in range(NG):
            toks.append(ti[PH - 1][g])
        if dc is not None:
            tr[0] = tr[0] + dc
        sr, si = _dft4(tr, ti, -1)
        for qq in range(PH):
            dst[c, :, b, qq, 0] = sr[qq]
            dst[c, :, b, qq, 1] = si[qq]

    def gated(c, b):
        w = [par_s[c, t:t + 1, :] for t in range(4)]
        kc = {}
        for o in range(-2, 2):
            words = k_u[c, pl.ds(8 + b * (LB // 2) + o, BLK, stride=2), :]
            if o > -2:
                kc[2 * o] = _lo(words)
            kc[2 * o + 1] = _hi(words)
        vc = {}
        for o in range(2):
            words = v_u[c, pl.ds(b * (LB // 2) + o, BLK, stride=2), :]
            vc[2 * o] = _lo(words)
            vc[2 * o + 1] = _hi(words)
        for i in range(PH):
            ks = kc[i] * w[0]
            for t in range(1, 4):
                ks = ks + kc[i - t] * w[t]
            wu_s[b, i] = (ks * vc[i]).astype(BF16)
        return [wu_u[b, i] for i in range(PH)]

    def kv_pins(kvb):
        return [jnp.stack([kvb[2 * m + (r % 2)][8 * (r // 2):8 * (r // 2) + 8, :] for r in range(NG)])
                for m in range(2)]

    def mac(c, us, ks, toks):
        zp = None
        for o in range(NBL):
            zr, zi = [], []
            for qq in range(PH):
                accr = acci = None
                for b in range(o + 1):
                    a_, b_ = us[0, :, b, qq, 0], us[0, :, b, qq, 1]
                    c_, d_ = ks[0, :, o - b, qq, 0], ks[0, :, o - b, qq, 1]
                    if qq == 0 and b == o:
                        a_ = after(toks[o], a_)
                    tr_ = a_ * c_ - b_ * d_
                    ti_ = a_ * d_ + b_ * c_
                    accr = tr_ if accr is None else accr + tr_
                    acci = ti_ if acci is None else acci + ti_
                zr.append(accr)
                zi.append(acci)
            if zp is None:
                yr, yi = zr, zi
            else:
                yr = [zr[qq] - zp[1][qq] for qq in range(PH)]
                yi = [zi[qq] + zp[0][qq] for qq in range(PH)]
            zp = (zr, zi)
            vr, vi = _dft4(yr, yi, +1)
            for i in range(PH):
                vv_s[c, o, i] = jnp.stack([vr[i], vi[i]], axis=1).reshape(2 * BLK, LANES).astype(BF16)

    def inverse(c, toks, pins=None, between=None):
        HB = BLK // 2
        for o in range(NBL):
            for i in range(PH):
                yv = None
                for h in range(2):
                    lhs = iv_u[i, h]
                    if pins is not None and h == 0:
                        pin = pins[o][i % 2][8 * (i // 2):8 * (i // 2) + 8]
                        lhs = after(pin, lhs.reshape(8, 8, LANES)).reshape(HB, LANES)
                    t = _dot(_as_bf16(lhs), _as_bf16(vv_u[c, o, i, h * HB:(h + 1) * HB, :]))
                    yv = t if yv is None else yv + t
                if i % 2 == 0:
                    for r in range(BLK // 16):
                        toks.append(yv[16 * r:16 * r + 8, :])
                y_s[c, pl.ds(o * LB + i, BLK, stride=PH), :] = yv
            if between is not None:
                between(o)

    def mac_tokens(toks):
        n = len(toks) - 3
        cum = (44, 128, 244, 392)
        return [jnp.stack([toks[max(0, ((g * 392 + cum[o]) * n) // (392 * NG) - 1)] for g in range(NG)])
                for o in range(NBL)]

    def conv_round(c, fwd, mul, inv, between=None):
        toks = []
        kv = pins = None
        cur = 1 if mul else 0
        if fwd or mul:
            win = pl.ds(c - cur, 2 if fwd and mul else 1)
            us, ks = u_s.at[win], kk_s.at[win]
        if fwd:
            kv = [gated(c, b) for b in range(NBL)]
            pins = [kv_pins(kv[b]) for b in range(NBL)]
        if inv:
            inverse(c - 2, toks, pins, between)
            if fwd:
                toks = []
        if fwd:
            wts = [perm_k(c, b, toks) for b in range(NBL)]
            dc = par_s[c, 4:5, :]
            if inv:
                order = ('k0', 'u0', 'k1', 'u1', 'k2', 'u2', 'k3', 'u3')
                pin_at = {}
            else:
                order = ('k0', 'k1', 'k2', 'u0', 'k3', 'u1', 'u2', 'u3')
                pin_at = {'k0': 0, 'k1': 1, 'u0': 2, 'k3': 3}
            for name in order:
                b = int(name[1])
                pin = pins[pin_at[name]] if name in pin_at else None
                tk = [] if (pin is not None and mul) else toks
                if name[0] == 'k':
                    spectrum(wts[b], ks, cur, b, tk, dc if b == 0 else None, pin)
                else:
                    spectrum([_as_bf16(x) for x in kv[b]], us, cur, b, tk, None, pin)
                if tk is not toks:
                    toks += tk[::4]
        if mul:
            mac(c - 1, us, ks, mac_tokens(toks))

    def tokens_of(x):
        return [x[8 * r:8 * r + 8, c * LANES:(c + 1) * LANES] for c in range(NC) for r in range(x.shape[0] // 8)]

    def store_bf16(ref, r0, x):
        for c in range(NC):
            ref[c, r0:r0 + x.shape[0], :] = x[:, c * LANES:(c + 1) * LANES].astype(BF16)

    def load_bf16(ref_u, r0, n):
        return _as_bf16(jnp.concatenate([ref_u[c, pl.ds(r0 // 2, n // 2), :] for c in range(NC)], axis=1))

    def pick(toks, n, free):
        if toks is None:
            return [None] * n
        idx = [(r * (len(toks) + free)) // n - free for r in range(n)]
        return [toks[i] if i >= 0 else None for i in idx]

    def hold(x, tks):
        f = len([k for k in tks if k is None])
        n = len(tks)
        if f == n:
            return x
        first = after(jnp.stack(tks[f:]), x[8 * f:, 0:LANES].reshape(n - f, 8, LANES)).reshape(8 * (n - f), LANES)
        if f:
            first = jnp.concatenate([x[:8 * f, 0:LANES], first], axis=0)
        return jnp.concatenate([first, x[:, LANES:]], axis=1)

    def mods_a():
        ga = mod_s[2, 0:1, :]
        return ga * (1.0 + mod_s[1, 0:1, :]), ga * mod_s[0, 0:1, :]

    def mods_b():
        return 1.0 + mod_s[4, 0:1, :], mod_s[3, 0:1, :]

    def stage_p1(r0, r1, tks, ma):
        q = hold(q_v[r0:r1, :].astype(F32), tks)
        y = jnp.concatenate([y_s[c, r0:r1, :] for c in range(NC)], axis=1)
        x = q + (_ln(q) * ma[0] + ma[1]) * y
        x_s[r0:r1, :] = x
        return _ln(x)

    def stage_p2(r0, r1, nx, mb):
        h = nx * mb[0] + mb[1]
        h_s[r0:r1, :] = h
        store_bf16(z_s, r0, _ln(h))

    def stage_p(t, toks, free):
        lo, hi = A0[t], A0[t + 1]
        stage_p2(lo, hi, stage_p1(lo, hi, pick(toks, (hi - lo) // 8, free), mods_a()), mods_b())

    def filler(t):
        if DUM:
            red = jnp.sum(y_s[t, 0:8 * DUM, :], axis=-1, keepdims=True).reshape(DUM, 8, 1)
            zf_s[1, (NC - 1) * (TQ + 8) + 8 * t:(NC - 1) * (TQ + 8) + 8 * t + 8, :] = jnp.broadcast_to(jnp.sum(red, axis=0), (8, LANES))

    def chunks(r0, r1, k):
        n = (r1 - r0) // 16
        cuts = [r0 + 16 * ((n * j) // k) for j in range(k + 1)]
        return list(zip(cuts[:-1], cuts[1:]))

    def stage_m1(t, k):
        toks = []
        for r0, r1 in chunks(A0[t], A0[t + 1], k):
            g1 = _gelu(_dot(load_bf16(z_u, r0, r1 - r0), packed(w1_v)))
            for c in range(NC):
                h1_s[c, r0 + 8:r1 + 8, :] = g1[:, c * LANES:(c + 1) * LANES]
            toks += tokens_of(g1)
        return toks

    grp = D // 4
    shifts = (-1, 1, -2, 2)

    def stage_m2(t, k):
        out = []
        for r0, r1 in chunks(B0[t], B0[t + 1], k):
            n = r1 - r0
            lane = lax.broadcasted_iota(jnp.int32, (n, LANES), 1)
            parts = []
            for c in range(NC):
                lo, hi = c * LANES, (c + 1) * LANES
                g_lo, g_hi = lo // grp, (hi - 1) // grp
                val = h1_s[c, pl.ds(r0 + 8 + shifts[g_lo], n), :]
                if g_hi != g_lo:
                    other = h1_s[c, pl.ds(r0 + 8 + shifts[g_hi], n), :]
                    val = jnp.where(lane < (g_hi * grp - lo), val, other)
                parts.append(val)
            x1 = h_s[r0:r1, :] + _dot(jnp.concatenate(parts, axis=1).astype(BF16), packed(w2_v))
            h_s[r0:r1, :] = x1
            out += tokens_of(x1)
        return out

    TQ = TB // 4
    NT = S // TB
    GB = 2 * NH + 1

    def blk_rows(b):
        return slice(b * (TQ + 8), b * (TQ + 8) + TQ)

    def store_z(r0, slot, toks, free):
        zn = _ln(hold(h_s[pl.ds(r0, TB), :], pick(toks, TB // 8, free)))
        for rq in range(4):
            for c in range(NC - 1):
                zf_s[slot, blk_rows(NC * rq + c), :] = zn[rq * TQ:(rq + 1) * TQ, c * LANES:(c + 1) * LANES]
        for c in range(NC):
            zr_s[c] = zn[:, c * LANES:(c + 1) * LANES].astype(BF16)

    def outer_lhs(i, blk):
        terms = ((0, 0, 1, 1, 1), (1, 0, 1, 1, 1), (0, 0), (1, 1), (0, 0, 1, 0, 1), (1, 0, -1, 0, 0), (0, 1, -1, 1, 1))[i]
        x = blk(terms[0], terms[1])
        if len(terms) > 2:
            y = blk(terms[3], terms[4])
            x = x + y if terms[2] > 0 else x - y
        return x

    def z_ops(slot_of, toks):
        ng = TQ // 16

        def held(x, k):
            tk = jnp.stack([toks[((k * ng + r) * len(toks)) // (7 * ng)] for r in range(ng)])
            x4 = x.reshape(ng, 2, 8, LANES)
            return jnp.stack([after(tk, x4[:, 0]), x4[:, 1]], axis=1).reshape(TQ, LANES)

        for k, i in enumerate(ZORD):
            slot = slot_of()
            so = [outer_lhs(i, lambda r1, k1: zf_s[slot, blk_rows(NC * (2 * r1 + r2) + 2 * k1 + k2), :])
                  for r2 in range(2) for k2 in range(2)]
            for j, x in enumerate(_lhs_ops(held(so[0], k), so[1], so[2], held(so[3], k))):
                la_s[i, j] = x.astype(BF16)

    NS = NH // 2

    RAW = (1, 4)

    def weight_ops(src, dst, ext, transposed, toks):
        ng = LANES // 16
        total = (NS * 7 + 2) * ng

        def tile(c, n):
            return src[c, n * LANES:(n + 1) * LANES, :].astype(F32)

        def held(x, pos, step):
            tk = jnp.stack([toks[((pos + r * step) * len(toks)) // total] for r in range(ng)])
            x4 = x.reshape(ng, 2, 8, LANES)
            return jnp.stack([after(tk, x4[:, 0]), x4[:, 1]], axis=1).reshape(LANES, LANES)

        def outer(c2, n, pos=None):
            b11, b22 = tile(c2, n), tile(2 + c2, NH + n)
            if pos is not None:
                b11, b22 = held(b11, pos, 1), held(b22, pos, 1)
            e1, e2 = tile(c2, NH + n), tile(2 + c2, n)
            return _rhs_ops(b11, e1, e2, b22) if transposed else _rhs_ops(b11, e2, e1, b22)

        for c2 in range(2 if ext is not None else 0):
            for i, x in enumerate(outer(c2, NH - 1, c2 * ng)):
                if i not in RAW:
                    ext[i, c2] = x.astype(BF16)
        for st in range(NS):
            t00, t11 = outer(0, 2 * st), outer(1, 2 * st + 1)
            t01, t10 = outer(0, 2 * st + 1), outer(1, 2 * st)
            for k, i in enumerate((1, 5, 2, 4, 0, 3, 6)):
                pos = (2 + st * 7) * ng + k
                a, d = held(t00[i], pos, 7), held(t11[i], pos, 7)
                ops = _rhs_ops(a, t01[i], t10[i], d) if transposed else _rhs_ops(a, t10[i], t01[i], d)
                for j, x in enumerate(ops):
                    if i not in RAW or j not in RAW:
                        dst[i, j, st * LANES:(st + 1) * LANES, :] = x.astype(BF16)

    with jax.named_scope("r0_wait"):
        wait_all(conv_copies(0))
    with jax.named_scope("r0"):
        start_all(conv_copies(2) + conv_copies(3) + conv_copies(4))
        conv_round(0, True, False, False)
    with jax.named_scope("r1_wait"):
        wait_all(conv_copies(1))
    with jax.named_scope("r1"):
        start_all(wm_copies[0] + q_copies[0] + wm_copies[1] + w_copies[0])
        conv_round(1, True, True, False)

    def full_round(c, carry):
        wait_all(conv_copies(c))
        conv_round(c, True, True, True)
        return carry

    with jax.named_scope("r234"):
        lax.fori_loop(2, NC, full_round, 0)
    with jax.named_scope("r5"):
        start_all(q_copies[1] + w_copies[1] + sum(q_copies[2:], []) + w_copies[2] + w_copies[3] + wm_copies[2], 1)
        conv_round(NC, False, True, True)
    with jax.named_scope("r6_wait"):
        wait_all(wm_copies[0] + q_copies[0])
    with jax.named_scope("r6"):
        for j in range(3):
            mod_chunk(j)
        conv_round(NC + 1, False, False, True)
        nx0 = stage_p1(0, A0[1], [None], mods_a())
    with jax.named_scope("p2_wait"):
        wait_all(wm_copies[1])
    with jax.named_scope("p2"):
        mod_chunk(4)
        mod_chunk(3)
        stage_p2(0, A0[1], nx0, mods_b())
    with jax.named_scope("w1_wait"):
        wait_all(w_copies[0])
    with jax.named_scope("m1_0"):
        stage_m1(0, 4)
    with jax.named_scope("w2_wait"):
        wait_all(q_copies[1] + w_copies[1])
    with jax.named_scope("m2_0"):
        toks = stage_m2(0, 4)
        stage_p(1, toks[:len(toks) - TRIM], FREE)
        filler(0)
    for t in range(1, NA):
        with jax.named_scope("a%d" % t):
            if t + 1 < NA:
                wait_all(q_copies[t + 1])
            else:
                wait_all(w_copies[2] + w_copies[3] + wm_copies[2])
            t1 = stage_m1(t, SPLIT)
            t2 = stage_m2(t, SPLIT)

            def weighted(trim):
                return [x for x in t1 for _ in range(W1N)] + [x for x in t2[:len(t2) - trim] for _ in range(W2N)]

            if t + 1 < NA:
                stage_p(t + 1, weighted(TRIM), FREE * W2N)
            if t == NA - 1 - LAT:
                toks = weighted(TRIM // 2)
                store_z(0, 0, toks if LAT else toks[:len(toks) // 2], FREE * W2N)
            if t == NA - 1:
                mod_chunk(NC)
                toks = weighted(20)
                cut = len(toks) // 2
                weight_ops(w3_v, s3_s, None, True, toks[:cut])
                weight_ops(w4_v, s4_s, e4_s, False, toks[cut:])
                z_ops(lambda: 0, toks if LAT else toks[(len(toks) * 5) // 8:])
            if t + 1 < NA or not LAT:
                filler(t)

    gb = mod_s[NC, 0:1, :]
    w3_u, w4_u, s3_u, s4_u, e4_u = (r.bitcast(U32) for r in (w3_v, w4_v, s3_s, s4_s, e4_s))
    HL = LANES // 2
    la_u = la_s.bitcast(U32)
    zr_u = zr_s.bitcast(U32)

    def out_copy(r0, n, c):
        rows = pl.ds(r0, n)
        return pltpu.make_async_copy(o_v.at[c, rows, :], o_hbm.at[rows, pl.ds(c * LANES, LANES)], sem_o.at[0])

    def one_level(w_u, e_u, i, c2):
        if i not in RAW:
            return e_u[i, c2]
        d = RAW.index(i)
        n = d * NH + NH - 1
        return w_u[2 * d + c2, n * HL:(n + 1) * HL, :]

    def two_level(w_u, s_u, i, j, st):
        if i not in RAW or j not in RAW:
            return s_u[i, j, st * HL:(st + 1) * HL, :]
        d, e = RAW.index(i), RAW.index(j)
        n = d * NH + 2 * st + e
        return w_u[2 * d + e, n * HL:(n + 1) * HL, :]

    def loop_b(t, carry):
        r0 = pl.multiple_of(t * TB, TB)
        ws = t & 1

        count = [0]

        def fresh():
            count[0] += 1
            return lax.rem(t + 2 * count[0], 2)

        zr = [_as_bf16(zr_u[NC - 1, rq * (TQ // 2):(rq + 1) * (TQ // 2), :]) for rq in range(4)]
        ltoks, ftoks = [], []

        def light(x):
            ltoks.extend(x[8 * r:8 * r + 8, 0:LANES] for r in range(x.shape[0] // 8))

        def rem3(rq, n):
            return _dot_nt(zr[rq], _as_bf16(w3_u[NC - 1, n * HL:(n + 1) * HL, :]))

        def put_g(rq, n, pre):
            g_s[ws, blk_rows(GB * rq + n), :] = _gelu(pre)

        rem = {}
        for st in range(NS):
            rem[3, NH + 2 * st + 1] = rem3(3, NH + 2 * st + 1)
        n0 = NH - 1
        w_mid = _as_bf16(jnp.concatenate([w3_u[c, n0 * HL:(n0 + 1) * HL, :] for c in range(NC)], axis=1))
        lo = (2 * NH - 1) * HL
        w_end = _as_bf16(jnp.concatenate([w3_u[c, lo:FF // 2, :] for c in range(NC)], axis=1))
        for rq in range(4):
            zq = _as_bf16(jnp.concatenate([zr_u[c, rq * (TQ // 2):(rq + 1) * (TQ // 2), :] for c in range(NC)], axis=1))
            mid = _dot_nt(zq, w_mid)
            ftoks.extend(mid[8 * r:8 * r + 8, :] for r in range(TQ // 8))
            put_g(rq, n0, mid)
            gt = _gelu(_dot_nt(w_end, zq))
            g_s[ws, blk_rows(GB * rq + 2 * NH - 1), :] = jnp.concatenate([gt, jnp.zeros((FP - FF, TQ), F32)], axis=0).T
        for st in range(NS):
            todo = [(2 * r1 + r2, h * NH + 2 * st + p) for r1, h in ((0, 1), (1, 0), (0, 0), (1, 1))
                    for r2 in range(2) for p in range(2)]
            todo = [x for x in todo if x not in rem]
            for key in todo[:8]:
                rem[key] = rem3(*key)
            if st >= LSETS:
                light(rem[todo[1]])
                light(rem[todo[5]])
            todo = todo[8:]
            pin = [None] * 7
            for i in _ORDER:
                m = [None] * 7
                for j in _ORDER:
                    m[j] = _dot_nt(_as_bf16(la_u[i, j]), _as_bf16(two_level(w3_u, s3_u, i, j, st)))
                if st >= LSETS and i in (2, 1, 0):
                    light(m[_ORDER[1]])
                    light(m[_ORDER[5]])
                key = todo.pop(0)
                rem[key] = rem3(*key)
                pin[i] = _combine(m)
            for inner in range(4):
                for blk, cval in enumerate(_combine([pin[i][inner] for i in range(7)])):
                    rq, n = 2 * (blk // 2) + inner // 2, (blk % 2) * NH + 2 * st + inner % 2
                    put_g(rq, n, cval + rem[rq, n])

        toks = []

        def timed(x):
            toks.extend(x[8 * r:8 * r + 8, 0:LANES] for r in range(x.shape[0] // 8))
            return x

        def finish(rq, c, h2):
            rows = pl.ds(pl.multiple_of(r0 + rq * TQ, TQ), TQ)
            cols = slice(c * LANES, (c + 1) * LANES)
            o_v[c, rows, :] = (x_s[rows, cols] + gb[:, cols] * (h_s[rows, cols] + h2)).astype(BF16)

        kord = [NH - 1, 2 * NH - 1] + [h * NH + n for st in range(NS) for h in (1, 0) for n in (2 * st + 1, 2 * st)]
        w4r = _as_bf16(jnp.concatenate([w4_u[NC - 1, n * HL:(n + 1) * HL, :] for n in kord], axis=0))

        def rem4(rq, slot):
            lhs = jnp.concatenate([g_s[slot, blk_rows(GB * rq + n), :] for n in kord], axis=1).astype(BF16)
            r = timed(_dot(lhs, w4r))
            finish(rq, NC - 1, r)

        rem4(0, fresh())
        rem4(1, fresh())
        pin = [None] * 7
        done = {_ORDER[1]: 1, _ORDER[3]: 2, _ORDER[5]: 0, _ORDER[6]: 3}
        for i in _ORDER:
            slot = fresh()
            rhs = _as_bf16(jnp.concatenate([one_level(w4_u, e4_u, i, c2) for c2 in range(2)], axis=1))
            ex = [_dot(outer_lhs(i, lambda r1, h: g_s[slot, blk_rows(GB * (2 * r1 + r2) + h * NH + NH - 1), :]).astype(BF16), rhs)
                  for r2 in range(2)]
            m = [None] * 7
            for j in _ORDER:
                slot = fresh()
                lhs = jnp.concatenate(
                    [outer_lhs(j, lambda r2, p: outer_lhs(
                        i, lambda r1, h: g_s[slot, blk_rows(GB * (2 * r1 + r2) + h * NH + 2 * st + p), :]))
                     for st in range(NS)], axis=1).astype(BF16)
                m[j] = timed(_dot(lhs, _as_bf16(jnp.concatenate([two_level(w4_u, s4_u, i, j, st) for st in range(NS)], axis=0))))
            pin[i] = [x + ex[inner // 2][:, (inner % 2) * LANES:(inner % 2 + 1) * LANES]
                      for inner, x in enumerate(_combine(m))]
            if i in done:
                blk = done[i]
                for inner in (1, 2, 0, 3):
                    p = [pin[k][inner] if pin[k] is not None else None for k in range(7)]
                    cval = (lambda: (p[3] - p[4]) + p[0] + p[6], lambda: p[2] + p[4], lambda: p[1] + p[3],
                            lambda: (p[2] - p[1]) + p[0] + p[5])[blk]()
                    finish(2 * (blk // 2) + inner // 2, 2 * (blk % 2) + inner % 2, cval)
                rb = pl.multiple_of(r0 + (blk // 2) * 2 * TQ, 2 * TQ)
                for e in range(2):
                    out_copy(rb, 2 * TQ, 2 * (blk % 2) + e).start()
                if blk == 0:
                    out_copy(r0, 3 * TQ, NC - 1).start()
            if i == _ORDER[REM2]:
                rem4(2, fresh())
        rem4(3, fresh())
        out_copy(pl.multiple_of(r0 + 3 * TQ, TQ), TQ, NC - 1).start()

        nxt = jnp.minimum(t + 1, NT - 1)
        store_z(pl.multiple_of(nxt * TB, TB), ws, ftoks[len(ftoks) - FT:] + ltoks[:LN1:LSTEP] + toks[:LB1], 0)
        z_ops(fresh, toks[ZB0:ZB1])
        if DUMB:
            filler(4)
        return carry

    with jax.named_scope("ph2b"):
        lax.fori_loop(0, NT, loop_b, 0)
    with jax.named_scope("tail"):
        pltpu.make_async_copy(o_v, o_v, sem_o.at[0]).wait()


@jax.jit
def pallas_adaLN_cond__ssm_conv_h3__mixer_s_mlp__prompt_kernel(
    A_q: jax.Array,
    A_k: jax.Array,
    A_v: jax.Array,
    A_shift_k: jax.Array,
    A_ssm_k: jax.Array,
    A_ssm_D: jax.Array,
    B_x: jax.Array,
    B_w1: jax.Array,
    B_w2: jax.Array,
    B_w3: jax.Array,
    B_w4: jax.Array,
    c: jax.Array,
    w_mod: jax.Array,
):
    B, S, D = A_q.shape
    assert B == 1
    FF = B_w3.shape[1]
    NC = D // LANES
    NG = BLK // 8
    NBL = S // (PH * BLK)
    FP = -(-FF // (2 * LANES)) * 2 * LANES
    TILES = (400, 400, 608, 640)
    assert sum(TILES) == S
    TB = 512

    args = (A_q.reshape(S, D), A_k.reshape(S, D), A_v.reshape(S, D), A_shift_k.T, A_ssm_k,
            A_ssm_D, B_w1, B_w2, B_w3.T, B_w4, c, w_mod)
    scratch = [
        pltpu.VMEM((S, D), BF16),
        pltpu.VMEM((NC, S + KP, LANES), BF16),
        pltpu.VMEM((NC, S + VP, LANES), BF16),
        pltpu.VMEM((4, D), BF16),
        pltpu.VMEM((NC, LANES, S), BF16),
        pltpu.VMEM((D,), BF16),
        pltpu.VMEM((NC, D, LANES), BF16),
        pltpu.VMEM((NC, D, LANES), BF16),
        pltpu.VMEM((NC, FF, LANES), BF16),
        pltpu.VMEM((NC, FP, LANES), BF16),
        pltpu.VMEM((1, D), BF16),
        pltpu.VMEM((D, 6 * D), BF16),
        pltpu.VMEM((PH, 2 * BLK, BLK), BF16),
        pltpu.VMEM((PH, 2, BLK, BLK), BF16),
        pltpu.VMEM((NC, S, LANES), BF16),
        pltpu.VMEM((NC, NG, NBL, PH, 2, 8, LANES), F32),
        pltpu.VMEM((NC, NG, NBL, PH, 2, 8, LANES), F32),
        pltpu.VMEM((NC, NBL, PH, 2 * BLK, LANES), BF16),
        pltpu.VMEM((NBL, PH, BLK, LANES), BF16),
        pltpu.VMEM((NC, S + YP, LANES), F32),
        pltpu.VMEM((6, 8, D), F32),
        pltpu.VMEM((NC, 8, LANES), F32),
        pltpu.VMEM((NC, S + 16, LANES), F32),
        pltpu.VMEM((S, D), F32),
        pltpu.VMEM((S, D), F32),
        pltpu.VMEM((NC, S, LANES), BF16),
        pltpu.VMEM((7, 7, FP // 512 * LANES, LANES), BF16),
        pltpu.VMEM((7, 7, FP // 512 * LANES, LANES), BF16),
        pltpu.VMEM((7, 2, LANES, LANES), BF16),
        pltpu.VMEM((2, GR, LANES), F32),
        pltpu.VMEM((2, ZR, LANES), F32),
        pltpu.VMEM((NC, TB, LANES), BF16),
        pltpu.VMEM((7, 7, TB // 4, LANES), BF16),
        pltpu.SemaphoreType.DMA((16 + len(TILES),)),
        pltpu.SemaphoreType.DMA((1,)),
    ]
    out = pl.pallas_call(
        functools.partial(_kernel, S=S, D=D, FF=FF, TILES=TILES, TB=TB),
        in_specs=[pl.BlockSpec(memory_space=pl.ANY)] * len(args),
        out_specs=pl.BlockSpec(memory_space=pl.ANY),
        out_shape=jax.ShapeDtypeStruct((S, D), BF16),
        scratch_shapes=scratch,
        compiler_params=pltpu.CompilerParams(
            vmem_limit_bytes=120 * 1024 * 1024,
            disable_bounds_checks=True,
            disable_semaphore_checks=True,
        ),
    )(*args)
    return out.reshape(B, S, D)
```

```python
import functools
import math

import jax
import jax.numpy as jnp
from jax import lax
import jax.experimental.pallas as pl
import jax.experimental.pallas.tpu as pltpu

F32 = jnp.float32
BF16 = jnp.bfloat16
U32 = jnp.uint32

LANES = 128
BLK = 128
PH = 4
EPS = 1e-05
TRIM = 60
SPLIT = 2
FREE = 30
DUM = 96
RSQ = 1
ONEP = 1
LN1 = 999
KP = 16
VP = 0
YP = 0
GR = 8160
ZR = 2720
FT = 0
DUMB = 1
STR1 = (3, )
STR2 = (3, )
WL = 3
WH = 2
ZE = 1
PRE = 0
WM2 = 2
W2P = 1
UL = 2
W1N = 2
W2N = 3
LAT = 1
LSETS = 0
LSTEP = 4
LB1 = 0
ZB0 = 0
ZB1 = 140
REM2 = 1
ZORD = (2, 3, 0, 1, 4, 5, 6)


def _as_bf16(x):
    return pltpu.bitcast(x, BF16)


def _lo(x):
    return pltpu.bitcast(x << 16, F32)


def _hi(x):
    return pltpu.bitcast(x & jnp.uint32(0xFFFF0000), F32)


def _dft4(re, im, sign):
    ar, ai = re[0] + re[2], im[0] + im[2]
    br, bi = re[0] - re[2], im[0] - im[2]
    cr, ci = re[1] + re[3], im[1] + im[3]
    dr, di = re[1] - re[3], im[1] - im[3]
    o0 = (ar + cr, ai + ci)
    o2 = (ar - cr, ai - ci)
    m = (br + di, bi - dr)
    p = (br - di, bi + dr)
    o1, o3 = (m, p) if sign < 0 else (p, m)
    return [o0[0], o1[0], o2[0], o3[0]], [o0[1], o1[1], o2[1], o3[1]]


def _ln(x):
    inv = 1.0 / x.shape[-1]
    m = jnp.sum(x, axis=-1, keepdims=True) * inv
    if ONEP:
        v = jnp.maximum(jnp.sum(x * x, axis=-1, keepdims=True) * inv + (EPS - m * m), EPS)
        d = x - m
    else:
        d = x - m
        v = jnp.sum(d * d, axis=-1, keepdims=True) * inv + EPS
    if RSQ:
        return d * jnp.exp2(jnp.log(v) * (-0.5 / math.log(2.0)))
    return d * lax.rsqrt(v)


def _gelu(x):
    c0 = math.sqrt(2.0 / math.pi)
    t = jnp.tanh(x * (c0 + (c0 * 0.044715) * (x * x)))
    hx = 0.5 * x
    return hx + hx * t


def _dot(a, b):
    return jnp.dot(a, b, preferred_element_type=F32)


def _dot_nt(a, b):
    return lax.dot_general(a, b, (((1,), (1,)), ((), ())), preferred_element_type=F32)


def _lhs_ops(a11, a12, a21, a22):
    return [a11 + a22, a21 + a22, a11, a22, a11 + a12, a21 - a11, a12 - a22]


def _rhs_ops(b11, b12, b21, b22):
    return [b11 + b22, b11, b12 - b22, b21 - b11, b22, b11 + b12, b21 + b22]


def _combine(m):
    return (m[3] - m[4]) + m[0] + m[6], m[2] + m[4], m[1] + m[3], (m[2] - m[1]) + m[0] + m[5]


_ORDER = (2, 4, 1, 3, 0, 6, 5)


def _kernel(q_hbm, k_hbm, v_hbm, sh_hbm, sk_hbm, sd_hbm, w1_hbm, w2_hbm, w3_hbm, w4_hbm, c_hbm, wm_hbm,
            o_hbm,
            q_v, k_v, v_v, sh_v, sk_v, sd_v, w1_v, w2_v, w3_v, w4_v, c_v, wm_v,
            fw_s, iv_s, o_v, u_s, kk_s, vv_s, wu_s, y_s, mod_s, par_s, h1_s, x_s, h_s, z_s, s3_s, s4_s, e4_s, g_s, zf_s, zr_s, la_s, lo_s, l2_s, s1_s, s2_s,
            sem, sem_o,
            *, S, D, FF, TILES, TB):
    NC = D // LANES
    NG = BLK // 8
    LB = PH * BLK
    NBL = S // LB
    R = BLK // PH
    HALO = 32
    FP = w4_v.shape[1]
    FH = FP // 2
    NH = FH // LANES

    small = [
        pltpu.make_async_copy(sh_hbm, sh_v, sem.at[0]),
        pltpu.make_async_copy(sd_hbm, sd_v, sem.at[0]),
        pltpu.make_async_copy(c_hbm, c_v, sem.at[0]),
    ]

    def conv_copies(c):
        col = pl.ds(c * LANES if isinstance(c, int) else pl.multiple_of(c * LANES, LANES), LANES)
        return [
            pltpu.make_async_copy(sk_hbm.at[col, :], sk_v.at[c], sem.at[9 + c if isinstance(c, int) and c < 2 else 1 + c]),
            pltpu.make_async_copy(k_hbm.at[:, col], k_v.at[c, pl.ds(16, S), :], sem.at[1 + c]),
            pltpu.make_async_copy(v_hbm.at[:, col], v_v.at[c, pl.ds(0, S), :], sem.at[1 + c]),
        ]

    def col_copies(src, dst, c0, s):
        rows = pl.ds(0, src.shape[0])
        return [pltpu.make_async_copy(src.at[:, pl.ds((c0 + c) * LANES, LANES)], dst.at[c0 + c, rows, :], sem.at[s])
                for c in range(NC)]

    WM = (0, 3 * D, 5 * D, 6 * D)
    wm_copies = [[pltpu.make_async_copy(wm_hbm.at[:, pl.ds(WM[j], WM[j + 1] - WM[j])],
                                        wm_v.at[:, pl.ds(WM[j], WM[j + 1] - WM[j])], sem.at[6 + j])]
                 for j in range(3)]
    w_copies = [col_copies(src, dst, 0, 12 + j)
                for j, (src, dst) in enumerate(((w1_hbm, w1_v), (w2_hbm, w2_v), (w3_hbm, w3_v), (w4_hbm, w4_v)))]

    B0 = [0]
    for n in TILES:
        B0.append(B0[-1] + n)
    NA = len(TILES)
    A0 = [0] + [r + HALO for r in B0[1:-1]] + [S]
    q_copies = [
        [pltpu.make_async_copy(q_hbm.at[pl.ds(A0[t], A0[t + 1] - A0[t])], q_v.at[pl.ds(A0[t], A0[t + 1] - A0[t])],
                               sem.at[16 + t])]
        for t in range(NA)
    ]

    def start_all(cps, priority=0):
        for cp in cps:
            cp.start(priority=priority)

    def wait_all(cps):
        for cp in cps:
            cp.wait()

    def packed(ref, c0=0):
        ru = ref.bitcast(U32)
        return _as_bf16(jnp.concatenate([ru[c0 + c] for c in range(NC)], axis=1))

    first, second = conv_copies(0), conv_copies(1)
    start_all(first[:1] + small + first[1:] + second)

    for c in range(NC):
        k_v[c, 0:16, :] = jnp.zeros((16, LANES), BF16)
        h1_s[c, 0:8, :] = jnp.zeros((8, LANES), F32)
        h1_s[c, S + 8:S + 16, :] = jnp.zeros((8, LANES), F32)
        w4_v[c, FF:FP, :] = jnp.zeros((FP - FF, LANES), BF16)

    prow = lax.broadcasted_iota(jnp.int32, (BLK, BLK), 0)
    pcol = lax.broadcasted_iota(jnp.int32, (BLK, BLK), 1)
    ang = (((4 * prow + 1) * pcol) & (4 * BLK - 1)).astype(F32) * (2.0 * math.pi / (4 * BLK))
    tw = (4 * prow + 1).astype(F32) * (2.0 * math.pi / (4 * LB))
    mr, mi = jnp.cos(ang), -jnp.sin(ang)
    zr_, zi_ = jnp.cos(tw), -jnp.sin(tw)
    eye = jnp.where(prow == pcol, 1.0 / LB, 0.0).astype(BF16)
    for i in range(PH):
        both = jnp.stack([mr.reshape(NG, 8, BLK), mi.reshape(NG, 8, BLK)], axis=1).reshape(2 * BLK, BLK)
        fw_s[i] = both.astype(BF16)
        for h in range(2):
            iv_s[i, h] = _dot_nt(eye, both[h * BLK:(h + 1) * BLK, :].astype(BF16)).astype(BF16)
        if i + 1 < PH:
            mr, mi = mr * zr_ - mi * zi_, mr * zi_ + mi * zr_
    perm = jnp.where(pcol == (prow % R) * PH + prow // R, 1.0, 0.0).astype(BF16)
    fw_u = fw_s.bitcast(U32)
    iv_u = iv_s.bitcast(U32)

    wait_all(small)
    shf = sh_v[...].astype(F32)
    sdf = sd_v[...].astype(F32).reshape(1, D)
    for c in range(NC):
        par_s[c, 0:4, :] = shf[:, c * LANES:(c + 1) * LANES]
        par_s[c, 4:5, :] = sdf[:, c * LANES:(c + 1) * LANES]
    cf = c_v[...].astype(F32)
    sc = (cf * jax.nn.sigmoid(cf)).astype(BF16)
    sc16 = jnp.broadcast_to(sc, (16, D))

    def mod_chunk(j):
        mod_s[j] = _dot(sc16, wm_v[:, j * D:(j + 1) * D])[0:8, :]

    k_u = k_v.bitcast(U32)
    v_u = v_v.bitcast(U32)
    wu_u = wu_s.bitcast(U32)
    z_u = z_s.bitcast(U32)
    vv_u = vv_s.bitcast(U32)
    lo_u = lo_s.bitcast(U32)
    l2_u = l2_s.bitcast(U32)

    never = zr_[0:8, :] > 2.0

    def after(token, x):
        if token.dtype != x.dtype:
            token = pltpu.bitcast(token, x.dtype)
        return jnp.where(jnp.broadcast_to(never, x.shape), token, x)

    def split(t):
        t4 = t.reshape(NG, 2, 8, LANES)
        return t4[:, 0], t4[:, 1]

    def perm_k(c, b, toks):
        kt = [_dot_nt(perm, sk_v[c, :, b * LB + t * BLK:b * LB + (t + 1) * BLK]) for t in range(PH)]
        for r in range(BLK // 16):
            toks.append(kt[0][16 * r:16 * r + 8, :])
        return [jnp.concatenate([kt[t][i * R:(i + 1) * R, :] for t in range(PH)], axis=0).astype(BF16)
                for i in range(PH)]

    def spectrum(wts, dst, c, b, toks, dc=None, pins=None):
        tr, ti = [], []
        for i in range(PH):
            lhs = fw_u[i]
            if pins is not None and i < len(pins):
                lhs = after(pins[i], lhs.reshape(NG, 8, LANES)).reshape(BLK, LANES)
            r_, i_ = split(_dot(_as_bf16(lhs), wts[i]))
            tr.append(r_)
            ti.append(i_)
        for g in range(NG):
            toks.append(ti[PH - 1][g])
        if dc is not None:
            tr[0] = tr[0] + dc
        sr, si = _dft4(tr, ti, -1)
        for qq in range(PH):
            dst[c, :, b, qq, 0] = sr[qq]
            dst[c, :, b, qq, 1] = si[qq]

    def gated(c, b):
        w = [par_s[c, t:t + 1, :] for t in range(4)]
        kc = {}
        for o in range(-2, 2):
            words = k_u[c, pl.ds(8 + b * (LB // 2) + o, BLK, stride=2), :]
            if o > -2:
                kc[2 * o] = _lo(words)
            kc[2 * o + 1] = _hi(words)
        vc = {}
        for o in range(2):
            words = v_u[c, pl.ds(b * (LB // 2) + o, BLK, stride=2), :]
            vc[2 * o] = _lo(words)
            vc[2 * o + 1] = _hi(words)
        for i in range(PH):
            ks = kc[i] * w[0]
            for t in range(1, 4):
                ks = ks + kc[i - t] * w[t]
            wu_s[b, i] = (ks * vc[i]).astype(BF16)
        return [wu_u[b, i] for i in range(PH)]

    def kv_pins(kvb):
        return [jnp.stack([kvb[2 * m + (r % 2)][8 * (r // 2):8 * (r // 2) + 8, :] for r in range(NG)])
                for m in range(2)]

    def mac(c, us, ks, toks):
        zp = None
        for o in range(NBL):
            zr, zi = [], []
            for qq in range(PH):
                accr = acci = None
                for b in range(o + 1):
                    a_, b_ = us[0, :, b, qq, 0], us[0, :, b, qq, 1]
                    c_, d_ = ks[0, :, o - b, qq, 0], ks[0, :, o - b, qq, 1]
                    if qq == 0 and b == o:
                        a_ = after(toks[o], a_)
                    tr_ = a_ * c_ - b_ * d_
                    ti_ = a_ * d_ + b_ * c_
                    accr = tr_ if accr is None else accr + tr_
                    acci = ti_ if acci is None else acci + ti_
                zr.append(accr)
                zi.append(acci)
            if zp is None:
                yr, yi = zr, zi
            else:
                yr = [zr[qq] - zp[1][qq] for qq in range(PH)]
                yi = [zi[qq] + zp[0][qq] for qq in range(PH)]
            zp = (zr, zi)
            vr, vi = _dft4(yr, yi, +1)
            for i in range(PH):
                vv_s[c, o, i] = jnp.stack([vr[i], vi[i]], axis=1).reshape(2 * BLK, LANES).astype(BF16)

    def inverse(c, toks, pins=None):
        HB = BLK // 2
        for o in range(NBL):
            for i in range(PH):
                yv = None
                for h in range(2):
                    lhs = iv_u[i, h]
                    if pins is not None and h == 0:
                        pin = pins[o][i % 2][8 * (i // 2):8 * (i // 2) + 8]
                        lhs = after(pin, lhs.reshape(8, 8, LANES)).reshape(HB, LANES)
                    t = _dot(_as_bf16(lhs), _as_bf16(vv_u[c, o, i, h * HB:(h + 1) * HB, :]))
                    yv = t if yv is None else yv + t
                if i % 2 == 0:
                    for r in range(BLK // 16):
                        toks.append(yv[16 * r:16 * r + 8, :])
                y_s[c, pl.ds(o * LB + i, BLK, stride=PH), :] = yv

    def mac_tokens(toks):
        n = len(toks) - 3
        cum = (44, 128, 244, 392)
        return [jnp.stack([toks[max(0, ((g * 392 + cum[o]) * n) // (392 * NG) - 1)] for g in range(NG)])
                for o in range(NBL)]

    def conv_round(c, fwd, mul, inv):
        toks = []
        kv = pins = None
        cur = 1 if mul else 0
        if fwd or mul:
            win = pl.ds(c - cur, 2 if fwd and mul else 1)
            us, ks = u_s.at[win], kk_s.at[win]
        if 'u' in fwd:
            kv = [gated(c, b) for b in range(NBL)]
            pins = [kv_pins(kv[b]) for b in range(NBL)]
        if inv:
            inverse(c - 2, toks, pins)
            if fwd:
                toks = []
        if 'k' in fwd:
            wts = [perm_k(c, b, toks) for b in range(NBL)]
        for b in range(NBL):
            if 'k' in fwd:
                spectrum(wts[b], ks, cur, b, toks, par_s[c, 4:5, :] if b == 0 else None)
            if 'u' in fwd:
                pin = pins[b + UL] if not inv and b + UL < NBL else None
                spectrum([_as_bf16(x) for x in kv[b]], us, cur, b, toks, None, pin)
        if mul:
            mac(c - 1, us, ks, mac_tokens(toks))

    def tokens_of(x):
        return [x[8 * r:8 * r + 8, c * LANES:(c + 1) * LANES] for c in range(NC) for r in range(x.shape[0] // 8)]

    def store_bf16(ref, r0, x):
        for c in range(NC):
            ref[c, r0:r0 + x.shape[0], :] = x[:, c * LANES:(c + 1) * LANES].astype(BF16)

    def load_bf16(ref_u, r0, n):
        return _as_bf16(jnp.concatenate([ref_u[c, pl.ds(r0 // 2, n // 2), :] for c in range(NC)], axis=1))

    def pick(toks, n, free):
        if toks is None:
            return [None] * n
        idx = [(r * (len(toks) + free)) // n - free for r in range(n)]
        return [toks[i] if i >= 0 else None for i in idx]

    def hold(x, tks):
        f = len([k for k in tks if k is None])
        n = len(tks)
        if f == n:
            return x
        first = after(jnp.stack(tks[f:]), x[8 * f:, 0:LANES].reshape(n - f, 8, LANES)).reshape(8 * (n - f), LANES)
        if f:
            first = jnp.concatenate([x[:8 * f, 0:LANES], first], axis=0)
        return jnp.concatenate([first, x[:, LANES:]], axis=1)

    def mods_a():
        ga = mod_s[2, 0:1, :]
        return ga * (1.0 + mod_s[1, 0:1, :]), ga * mod_s[0, 0:1, :]

    def mods_b():
        return 1.0 + mod_s[4, 0:1, :], mod_s[3, 0:1, :]

    def stage_p1(r0, r1, tks, ma):
        q = hold(q_v[r0:r1, :].astype(F32), tks)
        y = jnp.concatenate([y_s[c, r0:r1, :] for c in range(NC)], axis=1)
        x = q + (_ln(q) * ma[0] + ma[1]) * y
        x_s[r0:r1, :] = x
        return _ln(x)

    def halves(x):
        x4 = x.reshape(x.shape[0] // 32, 2, 16, LANES)
        return [x4[:, e].reshape(x.shape[0] // 2, LANES) for e in range(2)]

    def weave(top, bot):
        n = top.shape[0] // 16
        return jnp.stack([top.reshape(n, 16, LANES), bot.reshape(n, 16, LANES)], axis=1).reshape(32 * n, LANES)

    def row_ops(cols, tks=None):
        hv = [halves(x) for x in cols]
        if tks is not None:
            tk = jnp.stack(tks)

            def held(x):
                x4 = x.reshape(len(tks), 2, 8, LANES)
                return jnp.stack([after(tk, x4[:, 0]), x4[:, 1]], axis=1).reshape(x.shape)

            for k2 in range(2):
                hv[k2][0] = held(hv[k2][0])
                hv[2 + k2][1] = held(hv[2 + k2][1])
        per = [_lhs_ops(hv[k2][0], hv[2 + k2][0], hv[k2][1], hv[2 + k2][1]) + [hv[2 + k2][0], hv[k2][1]]
               for k2 in range(2)]
        return [[per[0][o], per[1][o]] for o in range(9)] + [hv[NC - 1]]

    def stage_p2(r0, r1, nx, mb, blockwise=False):
        h = nx * mb[0] + mb[1]
        h_s[r0:r1, :] = h
        zn = _ln(h)
        if not blockwise:
            store_bf16(z_s, r0, zn)
            return
        ops = row_ops([zn[:, c * LANES:(c + 1) * LANES] for c in range(NC)])
        for o in range(10):
            for e in range(2):
                lo_s[o, e, r0 // 2:r1 // 2, :] = ops[o][e].astype(BF16)

    def stage_p(t, toks, free):
        lo, hi = A0[t], A0[t + 1]
        stage_p2(lo, hi, stage_p1(lo, hi, pick(toks, (hi - lo) // 8, free), mods_a()), mods_b(), t in STR1)

    def square_ops(src, dst, toks):
        HK = 2 * LANES
        ng = HK // 16
        for n2 in range(2):
            tk = jnp.stack([toks[((n2 * ng + r) * len(toks)) // (2 * ng)] for r in range(ng)])

            def blk(c, k, hold_it):
                x = src[c, k * HK:(k + 1) * HK, :].astype(F32)
                if not hold_it:
                    return x
                x4 = x.reshape(ng, 2, 8, LANES)
                return jnp.stack([after(tk, x4[:, 0]), x4[:, 1]], axis=1).reshape(HK, LANES)

            for o, x in enumerate(_rhs_ops(blk(n2, 0, True), blk(2 + n2, 0, False), blk(n2, 1, False), blk(2 + n2, 1, True))):
                if o not in (1, 4):
                    dst[o, n2] = x.astype(BF16)

    def block_dots(lhs_of, w_ref, s_ref, parts, emit, WL, WH):
        w_u, s_u = w_ref.bitcast(U32), s_ref.bitcast(U32)
        toks = []

        def timed(x, weight):
            toks.extend(x[8 * r:8 * r + 8, 0:LANES] for r in range(x.shape[0] // 8) for _ in range(weight))
            return x

        def main(get):
            m = [None] * 7
            rem = [None, None]
            for o in ('t', 2, 4, 'b', 1, 3, 0, 6, 5):
                if o in ('t', 'b'):
                    e = 0 if o == 't' else 1
                    rhs = jnp.concatenate([w_u[c, 2 * LANES:D // 2, :] for c in range(NC - 1)], axis=1)
                    rem[e] = timed(_dot(get([(9, e)]), _as_bf16(rhs)), WL)
                    continue
                if o in (1, 4):
                    d = (1, 4).index(o)
                    rhs = jnp.concatenate([w_u[2 * d + n2, d * LANES:(d + 1) * LANES, :] for n2 in range(2)], axis=1)
                else:
                    rhs = jnp.concatenate([s_u[o, n2] for n2 in range(2)], axis=1)
                m[o] = timed(_dot(get([(o, 0), (o, 1)]), _as_bf16(rhs)), WH if o in (4, 3, 6, 5) else WL)
            c11, c12, c21, c22 = _combine(m)
            top = jnp.concatenate([c11, c12], axis=1) + rem[0]
            bot = jnp.concatenate([c21, c22], axis=1) + rem[1]
            return [weave(top[:, c * LANES:(c + 1) * LANES], bot[:, c * LANES:(c + 1) * LANES]) for c in range(NC - 1)]

        def last(get):
            w4c = _as_bf16(w_u[NC - 1])
            return weave(timed(_dot(get([(2, 0), (2, 1), (7, 0), (7, 1), (9, 0)]), w4c), WL),
                         timed(_dot(get([(8, 0), (8, 1), (3, 0), (3, 1), (9, 1)]), w4c), WL))

        marks = []
        for j, part in enumerate(parts):
            get = lhs_of(part, toks[marks[-1]:] if marks else None)
            marks.append(len(toks))
            if j % 2:
                tail = last(get)
                cols = main(get) + [tail]
            else:
                cols = main(get) + [last(get)]
            emit(part, cols)
        return toks

    def filler(t):
        if DUM:
            red = jnp.sum(y_s[t, 0:8 * DUM, :], axis=-1, keepdims=True).reshape(DUM, 8, 1)
            zf_s[1, (NC - 1) * (TQ + 8) + 8 * t:(NC - 1) * (TQ + 8) + 8 * t + 8, :] = jnp.broadcast_to(jnp.sum(red, axis=0), (8, LANES))

    def chunks(r0, r1, k, unit=16):
        n = (r1 - r0) // unit
        cuts = [r0 + unit * ((n * j) // k) for j in range(k + 1)]
        return list(zip(cuts[:-1], cuts[1:]))

    def stage_m1(t, k):
        def emit(part, cols):
            out = [_gelu(x) for x in cols]
            for c in range(NC):
                h1_s[c, part[0] + 8:part[1] + 8, :] = out[c]
            return out

        if t in STR1:
            def lhs_of(part, _):
                return lambda keys: _as_bf16(jnp.concatenate(
                    [lo_u[o, e, part[0] // 4:part[1] // 4, :] for o, e in keys], axis=1))
            return block_dots(lhs_of, w1_v, s1_s, chunks(A0[t], A0[t + 1], k, 32), emit, WL, WH)
        toks = []
        for r0, r1 in chunks(A0[t], A0[t + 1], k):
            pre = _dot(load_bf16(z_u, r0, r1 - r0), packed(w1_v))
            out = emit((r0, r1), [pre[:, c * LANES:(c + 1) * LANES] for c in range(NC)])
            toks += [x for x in tokens_of(jnp.concatenate(out, axis=1)) for _ in range(W1N)]
        return toks

    grp = D // 4
    shifts = (-1, 1, -2, 2)

    def shifted(r0, r1):
        n = r1 - r0
        lane = lax.broadcasted_iota(jnp.int32, (n, LANES), 1)
        cols = []
        for c in range(NC):
            lo, hi = c * LANES, (c + 1) * LANES
            g_lo, g_hi = lo // grp, (hi - 1) // grp
            val = h1_s[c, pl.ds(r0 + 8 + shifts[g_lo], n), :]
            if g_hi != g_lo:
                other = h1_s[c, pl.ds(r0 + 8 + shifts[g_hi], n), :]
                val = jnp.where(lane < (g_hi * grp - lo), val, other)
            cols.append(val)
        return cols

    def stage_m2(t, k, before=None):
        def emit(part, cols):
            x1 = h_s[part[0]:part[1], :] + jnp.concatenate(cols, axis=1)
            h_s[part[0]:part[1], :] = x1
            return x1

        if t in STR2:
            def lhs_of(part, prev):
                prev = before if prev is None else prev
                prev = prev[len(prev) // 8:(len(prev) * 7) // 8]
                ops = row_ops(shifted(*part), pick(prev, (part[1] - part[0]) // 32, 0))
                for o in range(10):
                    for e in range(2):
                        l2_s[o, e, part[0] // 2:part[1] // 2, :] = ops[o][e].astype(BF16)
                return lambda keys: _as_bf16(jnp.concatenate(
                    [l2_u[o, e, part[0] // 4:part[1] // 4, :] for o, e in keys], axis=1))
            return block_dots(lhs_of, w2_v, s2_s, chunks(B0[t], B0[t + 1], k, 32), emit, WM2, WM2)
        toks = []
        for r0, r1 in chunks(B0[t], B0[t + 1], k):
            hs = _dot(jnp.concatenate(shifted(r0, r1), axis=1).astype(BF16), packed(w2_v))
            toks += [x for x in tokens_of(emit((r0, r1), [hs])) for _ in range(W2N)]
        return toks

    TQ = TB // 4
    NT = S // TB
    GB = 2 * NH + 1

    def blk_rows(b):
        return slice(b * (TQ + 8), b * (TQ + 8) + TQ)

    def store_z(r0, slot, toks, free):
        zn = _ln(hold(h_s[pl.ds(r0, TB), :], pick(toks, TB // 8, free)))
        for rq in range(4):
            for c in range(NC - 1):
                zf_s[slot, blk_rows(NC * rq + c), :] = zn[rq * TQ:(rq + 1) * TQ, c * LANES:(c + 1) * LANES]
        for c in range(NC):
            zr_s[c] = zn[:, c * LANES:(c + 1) * LANES].astype(BF16)

    def outer_lhs(i, blk):
        terms = ((0, 0, 1, 1, 1), (1, 0, 1, 1, 1), (0, 0), (1, 1), (0, 0, 1, 0, 1), (1, 0, -1, 0, 0), (0, 1, -1, 1, 1))[i]
        x = blk(terms[0], terms[1])
        if len(terms) > 2:
            y = blk(terms[3], terms[4])
            x = x + y if terms[2] > 0 else x - y
        return x

    def z_ops(slot_of, toks):
        ng = TQ // 16

        def held(x, k):
            tk = jnp.stack([toks[((k * ng + r) * len(toks)) // (7 * ng)] for r in range(ng)])
            x4 = x.reshape(ng, 2, 8, LANES)
            return jnp.stack([after(tk, x4[:, 0]), x4[:, 1]], axis=1).reshape(TQ, LANES)

        for k, i in enumerate(ZORD):
            slot = slot_of()
            so = [outer_lhs(i, lambda r1, k1: zf_s[slot, blk_rows(NC * (2 * r1 + r2) + 2 * k1 + k2), :])
                  for r2 in range(2) for k2 in range(2)]
            for j, x in enumerate(_lhs_ops(held(so[0], k), so[1], so[2], held(so[3], k))):
                la_s[i, j] = x.astype(BF16)

    NS = NH // 2

    RAW = (1, 4)

    def weight_ops(src, dst, ext, transposed, toks):
        ng = LANES // 16
        lead = 2 if ext is not None else 0
        total = (NS * 7 + lead) * ng

        def tile(c, n):
            return src[c, n * LANES:(n + 1) * LANES, :].astype(F32)

        def held(x, pos, step):
            tk = jnp.stack([toks[((pos + r * step) * len(toks)) // total] for r in range(ng)])
            x4 = x.reshape(ng, 2, 8, LANES)
            return jnp.stack([after(tk, x4[:, 0]), x4[:, 1]], axis=1).reshape(LANES, LANES)

        def outer(c2, n, pos=None):
            b11, b22 = tile(c2, n), tile(2 + c2, NH + n)
            if pos is not None:
                b11, b22 = held(b11, pos, 1), held(b22, pos, 1)
            e1, e2 = tile(c2, NH + n), tile(2 + c2, n)
            return _rhs_ops(b11, e1, e2, b22) if transposed else _rhs_ops(b11, e2, e1, b22)

        for c2 in range(2 if ext is not None else 0):
            for i, x in enumerate(outer(c2, NH - 1, c2 * ng)):
                if i not in RAW:
                    ext[i, c2] = x.astype(BF16)
        for st in range(NS):
            t00, t11 = outer(0, 2 * st), outer(1, 2 * st + 1)
            t01, t10 = outer(0, 2 * st + 1), outer(1, 2 * st)
            for k, i in enumerate((1, 5, 2, 4, 0, 3, 6)):
                pos = (lead + st * 7) * ng + k
                a, d = held(t00[i], pos, 7), held(t11[i], pos, 7)
                ops = _rhs_ops(a, t01[i], t10[i], d) if transposed else _rhs_ops(a, t10[i], t01[i], d)
                for j, x in enumerate(ops):
                    if i not in RAW or j not in RAW:
                        dst[i, j, st * LANES:(st + 1) * LANES, :] = x.astype(BF16)

    with jax.named_scope("r0a"):
        wait_all(first[:1])
        conv_round(0, 'k', False, False)
    with jax.named_scope("r0_wait"):
        wait_all(first[1:])
    with jax.named_scope("r0b"):
        start_all(conv_copies(2) + conv_copies(3) + conv_copies(4))
        conv_round(0, 'u', False, False)
    with jax.named_scope("r1a"):
        wait_all(second[:1])
        conv_round(1, 'k', True, False)
    with jax.named_scope("r1_wait"):
        wait_all(second[1:])
    with jax.named_scope("r1b"):
        start_all(wm_copies[0] + q_copies[0] + wm_copies[1] + w_copies[0])
        conv_round(1, 'u', False, False)

    def full_round(c, carry):
        wait_all(conv_copies(c))
        conv_round(c, 'ku', True, True)
        return carry

    with jax.named_scope("r234"):
        lax.fori_loop(2, NC, full_round, 0)
    with jax.named_scope("r5"):
        start_all(q_copies[1] + w_copies[1] + sum(q_copies[2:], []) + w_copies[2] + w_copies[3] + wm_copies[2], 1)
        conv_round(NC, '', True, True)
    with jax.named_scope("r6_wait"):
        wait_all(wm_copies[0] + q_copies[0])
    with jax.named_scope("r6"):
        for j in range(3):
            mod_chunk(j)
        conv_round(NC + 1, '', False, True)
        nx0 = stage_p1(0, A0[1], [None], mods_a())
    with jax.named_scope("p2_wait"):
        wait_all(wm_copies[1])
    with jax.named_scope("p2"):
        mod_chunk(4)
        mod_chunk(3)
        stage_p2(0, A0[1], nx0, mods_b())
    with jax.named_scope("w1_wait"):
        wait_all(w_copies[0])
    with jax.named_scope("m1_0"):
        toks = stage_m1(0, 4)
        if STR1:
            square_ops(w1_v, s1_s, toks[:len(toks) - 20 * W1N])
    with jax.named_scope("w2_wait"):
        wait_all(q_copies[1] + w_copies[1])
    with jax.named_scope("m2_0"):
        toks = stage_m2(0, 4)
        stage_p(1, toks[:len(toks) - TRIM * W2N], FREE * W2N)
        if STR2 and min(STR2) == 1:
            square_ops(w2_v, s2_s, toks[len(toks) // 2:len(toks) - 10 * W2N])
        filler(0)
    for t in range(1, NA):
        with jax.named_scope("a%d" % t):
            if t + 1 < NA:
                wait_all(q_copies[t + 1])
            else:
                wait_all(w_copies[2] + w_copies[3] + wm_copies[2])
            t1 = stage_m1(t, SPLIT)
            t2 = stage_m2(t, SPLIT, t1[len(t1) - len(t1) // SPLIT:])

            def weighted(trim):
                return t1 + t2[:len(t2) - trim * W2N]

            if t + 1 < NA:
                stage_p(t + 1, weighted(TRIM), FREE * W2N)
            if STR2 and t == W2P:
                square_ops(w2_v, s2_s, weighted(10))
            if t == NA - 1 - LAT:
                toks = weighted(TRIM // 2)
                store_z(0, 0, toks if LAT and not ZE else toks[:len(toks) // 2], FREE * W2N)
                if ZE:
                    toks = weighted(10)
                    z_ops(lambda: 0, toks[(len(toks) * 5) // 8:])
            if t == NA - 1:
                mod_chunk(NC)
                toks = weighted(20)
                toks = toks[:1] * PRE + toks
                cut = (len(toks) * 21) // 44
                weight_ops(w3_v, s3_s, None, True, toks[:cut])
                weight_ops(w4_v, s4_s, e4_s, False, toks[cut:])
                if not ZE:
                    z_ops(lambda: 0, toks if LAT else toks[(len(toks) * 5) // 8:])
            if t + 1 < NA or not LAT:
                filler(t)

    gb = mod_s[NC, 0:1, :]
    w3_u, w4_u, s3_u, s4_u, e4_u = (r.bitcast(U32) for r in (w3_v, w4_v, s3_s, s4_s, e4_s))
    HL = LANES // 2
    la_u = la_s.bitcast(U32)
    zr_u = zr_s.bitcast(U32)

    def out_copy(r0, n, c):
        rows = pl.ds(r0, n)
        return pltpu.make_async_copy(o_v.at[c, rows, :], o_hbm.at[rows, pl.ds(c * LANES, LANES)], sem_o.at[0])

    def one_level(w_u, e_u, i, c2):
        if i not in RAW:
            return e_u[i, c2]
        d = RAW.index(i)
        n = d * NH + NH - 1
        return w_u[2 * d + c2, n * HL:(n + 1) * HL, :]

    def two_level(w_u, s_u, i, j, st):
        if i not in RAW or j not in RAW:
            return s_u[i, j, st * HL:(st + 1) * HL, :]
        d, e = RAW.index(i), RAW.index(j)
        n = d * NH + 2 * st + e
        return w_u[2 * d + e, n * HL:(n + 1) * HL, :]

    def loop_b(t, carry):
        r0 = pl.multiple_of(t * TB, TB)
        ws = t & 1

        count = [0]

        def fresh():
            count[0] += 1
            return lax.rem(t + 2 * count[0], 2)

        zr = [_as_bf16(zr_u[NC - 1, rq * (TQ // 2):(rq + 1) * (TQ // 2), :]) for rq in range(4)]
        ltoks, ftoks = [], []

        def light(x):
            ltoks.extend(x[8 * r:8 * r + 8, 0:LANES] for r in range(x.shape[0] // 8))

        def rem3(rq, n):
            return _dot_nt(zr[rq], _as_bf16(w3_u[NC - 1, n * HL:(n + 1) * HL, :]))

        def put_g(rq, n, pre):
            g_s[ws, blk_rows(GB * rq + n), :] = _gelu(pre)

        rem = {}
        for st in range(NS):
            rem[3, NH + 2 * st + 1] = rem3(3, NH + 2 * st + 1)
        n0 = NH - 1
        w_mid = _as_bf16(jnp.concatenate([w3_u[c, n0 * HL:(n0 + 1) * HL, :] for c in range(NC)], axis=1))
        lo = (2 * NH - 1) * HL
        w_end = _as_bf16(jnp.concatenate([w3_u[c, lo:FF // 2, :] for c in range(NC)], axis=1))
        for rq in range(4):
            zq = _as_bf16(jnp.concatenate([zr_u[c, rq * (TQ // 2):(rq + 1) * (TQ // 2), :] for c in range(NC)], axis=1))
            mid = _dot_nt(zq, w_mid)
            ftoks.extend(mid[8 * r:8 * r + 8, :] for r in range(TQ // 8))
            put_g(rq, n0, mid)
            gt = _gelu(_dot_nt(w_end, zq))
            g_s[ws, blk_rows(GB * rq + 2 * NH - 1), :] = jnp.concatenate([gt, jnp.zeros((FP - FF, TQ), F32)], axis=0).T
        for st in range(NS):
            todo = [(2 * r1 + r2, h * NH + 2 * st + p) for r1, h in ((0, 1), (1, 0), (0, 0), (1, 1))
                    for r2 in range(2) for p in range(2)]
            todo = [x for x in todo if x not in rem]
            for key in todo[:8]:
                rem[key] = rem3(*key)
            if st >= LSETS:
                light(rem[todo[1]])
                light(rem[todo[5]])
            todo = todo[8:]
            pin = [None] * 7
            for i in _ORDER:
                m = [None] * 7
                for j in _ORDER:
                    m[j] = _dot_nt(_as_bf16(la_u[i, j]), _as_bf16(two_level(w3_u, s3_u, i, j, st)))
                if st >= LSETS and i in (2, 1, 0):
                    light(m[_ORDER[1]])
                    light(m[_ORDER[5]])
                key = todo.pop(0)
                rem[key] = rem3(*key)
                pin[i] = _combine(m)
            for inner in range(4):
                for blk, cval in enumerate(_combine([pin[i][inner] for i in range(7)])):
                    rq, n = 2 * (blk // 2) + inner // 2, (blk % 2) * NH + 2 * st + inner % 2
                    put_g(rq, n, cval + rem[rq, n])

        toks = []

        def timed(x):
            toks.extend(x[8 * r:8 * r + 8, 0:LANES] for r in range(x.shape[0] // 8))
            return x

        def finish(rq, c, h2):
            rows = pl.ds(pl.multiple_of(r0 + rq * TQ, TQ), TQ)
            cols = slice(c * LANES, (c + 1) * LANES)
            o_v[c, rows, :] = (x_s[rows, cols] + gb[:, cols] * (h_s[rows, cols] + h2)).astype(BF16)

        kord = [NH - 1, 2 * NH - 1] + [h * NH + n for st in range(NS) for h in (1, 0) for n in (2 * st + 1, 2 * st)]
        w4r = _as_bf16(jnp.concatenate([w4_u[NC - 1, n * HL:(n + 1) * HL, :] for n in kord], axis=0))

        def rem4(rq, slot):
            lhs = jnp.concatenate([g_s[slot, blk_rows(GB * rq + n), :] for n in kord], axis=1).astype(BF16)
            r = timed(_dot(lhs, w4r))
            finish(rq, NC - 1, r)

        rem4(0, fresh())
        rem4(1, fresh())
        pin = [None] * 7
        done = {_ORDER[1]: 1, _ORDER[3]: 2, _ORDER[5]: 0, _ORDER[6]: 3}
        for i in _ORDER:
            slot = fresh()
            rhs = _as_bf16(jnp.concatenate([one_level(w4_u, e4_u, i, c2) for c2 in range(2)], axis=1))
            ex = [_dot(outer_lhs(i, lambda r1, h: g_s[slot, blk_rows(GB * (2 * r1 + r2) + h * NH + NH - 1), :]).astype(BF16), rhs)
                  for r2 in range(2)]
            m = [None] * 7
            for j in _ORDER:
                slot = fresh()
                lhs = jnp.concatenate(
                    [outer_lhs(j, lambda r2, p: outer_lhs(
                        i, lambda r1, h: g_s[slot, blk_rows(GB * (2 * r1 + r2) + h * NH + 2 * st + p), :]))
                     for st in range(NS)], axis=1).astype(BF16)
                m[j] = timed(_dot(lhs, _as_bf16(jnp.concatenate([two_level(w4_u, s4_u, i, j, st) for st in range(NS)], axis=0))))
            pin[i] = [x + ex[inner // 2][:, (inner % 2) * LANES:(inner % 2 + 1) * LANES]
                      for inner, x in enumerate(_combine(m))]
            if i in done:
                blk = done[i]
                for inner in (1, 2, 0, 3):
                    p = [pin[k][inner] if pin[k] is not None else None for k in range(7)]
                    cval = (lambda: (p[3] - p[4]) + p[0] + p[6], lambda: p[2] + p[4], lambda: p[1] + p[3],
                            lambda: (p[2] - p[1]) + p[0] + p[5])[blk]()
                    finish(2 * (blk // 2) + inner // 2, 2 * (blk % 2) + inner % 2, cval)
                rb = pl.multiple_of(r0 + (blk // 2) * 2 * TQ, 2 * TQ)
                for e in range(2):
                    out_copy(rb, 2 * TQ, 2 * (blk % 2) + e).start()
                if blk == 0:
                    out_copy(r0, 3 * TQ, NC - 1).start()
            if i == _ORDER[REM2]:
                rem4(2, fresh())
        rem4(3, fresh())
        out_copy(pl.multiple_of(r0 + 3 * TQ, TQ), TQ, NC - 1).start()

        nxt = jnp.minimum(t + 1, NT - 1)
        store_z(pl.multiple_of(nxt * TB, TB), ws, ftoks[len(ftoks) - FT:] + ltoks[:LN1:LSTEP] + toks[:LB1], 0)
        z_ops(fresh, toks[ZB0:ZB1])
        if DUMB:
            filler(4)
        return carry

    with jax.named_scope("ph2b"):
        lax.fori_loop(0, NT, loop_b, 0)
    with jax.named_scope("tail"):
        pltpu.make_async_copy(o_v, o_v, sem_o.at[0]).wait()


@jax.jit
def pallas_adaLN_cond__ssm_conv_h3__mixer_s_mlp__prompt_kernel(
    A_q: jax.Array,
    A_k: jax.Array,
    A_v: jax.Array,
    A_shift_k: jax.Array,
    A_ssm_k: jax.Array,
    A_ssm_D: jax.Array,
    B_x: jax.Array,
    B_w1: jax.Array,
    B_w2: jax.Array,
    B_w3: jax.Array,
    B_w4: jax.Array,
    c: jax.Array,
    w_mod: jax.Array,
):
    B, S, D = A_q.shape
    assert B == 1
    FF = B_w3.shape[1]
    NC = D // LANES
    NG = BLK // 8
    NBL = S // (PH * BLK)
    FP = -(-FF // (2 * LANES)) * 2 * LANES
    TILES = (384, 384, 576, 704)
    assert sum(TILES) == S
    TB = 512

    args = (A_q.reshape(S, D), A_k.reshape(S, D), A_v.reshape(S, D), A_shift_k.T, A_ssm_k,
            A_ssm_D, B_w1, B_w2, B_w3.T, B_w4, c, w_mod)
    scratch = [
        pltpu.VMEM((S, D), BF16),
        pltpu.VMEM((NC, S + KP, LANES), BF16),
        pltpu.VMEM((NC, S + VP, LANES), BF16),
        pltpu.VMEM((4, D), BF16),
        pltpu.VMEM((NC, LANES, S), BF16),
        pltpu.VMEM((D,), BF16),
        pltpu.VMEM((NC, D, LANES), BF16),
        pltpu.VMEM((NC, D, LANES), BF16),
        pltpu.VMEM((NC, FF, LANES), BF16),
        pltpu.VMEM((NC, FP, LANES), BF16),
        pltpu.VMEM((1, D), BF16),
        pltpu.VMEM((D, 6 * D), BF16),
        pltpu.VMEM((PH, 2 * BLK, BLK), BF16),
        pltpu.VMEM((PH, 2, BLK, BLK), BF16),
        pltpu.VMEM((NC, S, LANES), BF16),
        pltpu.VMEM((NC, NG, NBL, PH, 2, 8, LANES), F32),
        pltpu.VMEM((NC, NG, NBL, PH, 2, 8, LANES), F32),
        pltpu.VMEM((NC, NBL, PH, 2 * BLK, LANES), BF16),
        pltpu.VMEM((NBL, PH, BLK, LANES), BF16),
        pltpu.VMEM((NC, S + YP, LANES), F32),
        pltpu.VMEM((6, 8, D), F32),
        pltpu.VMEM((NC, 8, LANES), F32),
        pltpu.VMEM((NC, S + 16, LANES), F32),
        pltpu.VMEM((S, D), F32),
        pltpu.VMEM((S, D), F32),
        pltpu.VMEM((NC, S, LANES), BF16),
        pltpu.VMEM((7, 7, FP // 512 * LANES, LANES), BF16),
        pltpu.VMEM((7, 7, FP // 512 * LANES, LANES), BF16),
        pltpu.VMEM((7, 2, LANES, LANES), BF16),
        pltpu.VMEM((2, GR, LANES), F32),
        pltpu.VMEM((2, ZR, LANES), F32),
        pltpu.VMEM((NC, TB, LANES), BF16),
        pltpu.VMEM((7, 7, TB // 4, LANES), BF16),
        pltpu.VMEM((10, 2, S // 2, LANES), BF16),
        pltpu.VMEM((10, 2, S // 2, LANES), BF16),
        pltpu.VMEM((7, 2, 2 * LANES, LANES), BF16),
        pltpu.VMEM((7, 2, 2 * LANES, LANES), BF16),
        pltpu.SemaphoreType.DMA((16 + len(TILES),)),
        pltpu.SemaphoreType.DMA((1,)),
    ]
    out = pl.pallas_call(
        functools.partial(_kernel, S=S, D=D, FF=FF, TILES=TILES, TB=TB),
        in_specs=[pl.BlockSpec(memory_space=pl.ANY)] * len(args),
        out_specs=pl.BlockSpec(memory_space=pl.ANY),
        out_shape=jax.ShapeDtypeStruct((S, D), BF16),
        scratch_shapes=scratch,
        compiler_params=pltpu.CompilerParams(
            vmem_limit_bytes=126 * 1024 * 1024,
            disable_bounds_checks=True,
            disable_semaphore_checks=True,
        ),
    )(*args)
    return out.reshape(B, S, D)
```

```python
import functools
import math

import jax
import jax.numpy as jnp
from jax import lax
import jax.experimental.pallas as pl
import jax.experimental.pallas.tpu as pltpu

F32 = jnp.float32
BF16 = jnp.bfloat16
U32 = jnp.uint32

LANES = 128
BLK = 128
PH = 4
EPS = 1e-05
TRIM = 60
SPLIT = 2
FREE = 30
DUM = 96
LN1 = 999
KP = 16
VP = 0
YP = 0
GR = 8160
ZR = 2720
FT = 0
DUMB = 1
STR1 = (3, )
STR2 = (2, 3, )
WL = 3
WH = 2
ZE = 1
PRE = 0
WM2 = 2
W2P = 1
UL = 2
W1N = 2
W2N = 3
LAT = 1
LSETS = 0
LSTEP = 4
LB1 = 0
ZB0 = 0
ZB1 = 140
REM2 = 1
ZORD = (2, 3, 0, 1, 4, 5, 6)


def _as_bf16(x):
    return pltpu.bitcast(x, BF16)


def _lo(x):
    return pltpu.bitcast(x << 16, F32)


def _hi(x):
    return pltpu.bitcast(x & jnp.uint32(0xFFFF0000), F32)


def _dft4(re, im, sign):
    ar, ai = re[0] + re[2], im[0] + im[2]
    br, bi = re[0] - re[2], im[0] - im[2]
    cr, ci = re[1] + re[3], im[1] + im[3]
    dr, di = re[1] - re[3], im[1] - im[3]
    o0 = (ar + cr, ai + ci)
    o2 = (ar - cr, ai - ci)
    m = (br + di, bi - dr)
    p = (br - di, bi + dr)
    o1, o3 = (m, p) if sign < 0 else (p, m)
    return [o0[0], o1[0], o2[0], o3[0]], [o0[1], o1[1], o2[1], o3[1]]


def _ln(x, eps=EPS, unit=True):
    n = x.shape[-1]
    s1 = jnp.sum(x, axis=-1, keepdims=True)
    m = s1 * (1.0 / n)
    v = jnp.maximum(jnp.sum(x * x, axis=-1, keepdims=True) + (n * eps - s1 * m), n * eps)
    e = jnp.log(v) * (-0.5 / math.log(2.0))
    return (x - m) * jnp.exp2(e + 0.5 * math.log2(n) if unit else e)


def _gelu2(x):
    c0 = math.sqrt(2.0 / math.pi)
    return x + x * jnp.tanh(x * (c0 + (c0 * 0.044715) * (x * x)))


def _dot(a, b):
    return jnp.dot(a, b, preferred_element_type=F32)


def _dot_nt(a, b):
    return lax.dot_general(a, b, (((1,), (1,)), ((), ())), preferred_element_type=F32)


def _lhs_ops(a11, a12, a21, a22):
    return [a11 + a22, a21 + a22, a11, a22, a11 + a12, a21 - a11, a12 - a22]


def _rhs_ops(b11, b12, b21, b22):
    return [b11 + b22, b11, b12 - b22, b21 - b11, b22, b11 + b12, b21 + b22]


def _combine(m):
    return (m[3] - m[4]) + m[0] + m[6], m[2] + m[4], m[1] + m[3], (m[2] - m[1]) + m[0] + m[5]


_ORDER = (2, 4, 1, 3, 0, 6, 5)


def _kernel(q_hbm, k_hbm, v_hbm, sh_hbm, sk_hbm, sd_hbm, w1_hbm, w2_hbm, w3_hbm, w4_hbm, c_hbm, wm_hbm,
            o_hbm,
            q_v, k_v, v_v, sh_v, sk_v, sd_v, w1_v, w2_v, w3_v, w4_v, c_v, wm_v,
            fw_s, iv_s, o_v, u_s, kk_s, vv_s, wu_s, y_s, mod_s, par_s, h1_s, x_s, h_s, z_s, s3_s, s4_s, e4_s, g_s, zf_s, zr_s, la_s, lo_s, l2_s, s1_s, s2_s,
            sem, sem_o,
            *, S, D, FF, TILES, TB):
    NC = D // LANES
    NG = BLK // 8
    LB = PH * BLK
    NBL = S // LB
    R = BLK // PH
    HALO = 32
    FP = w4_v.shape[1]
    FH = FP // 2
    NH = FH // LANES

    small = [
        pltpu.make_async_copy(sh_hbm, sh_v, sem.at[0]),
        pltpu.make_async_copy(sd_hbm, sd_v, sem.at[0]),
        pltpu.make_async_copy(c_hbm, c_v, sem.at[0]),
    ]

    def conv_copies(c):
        col = pl.ds(c * LANES if isinstance(c, int) else pl.multiple_of(c * LANES, LANES), LANES)
        return [
            pltpu.make_async_copy(sk_hbm.at[col, :], sk_v.at[c], sem.at[9 + c if isinstance(c, int) and c < 2 else 1 + c]),
            pltpu.make_async_copy(k_hbm.at[:, col], k_v.at[c, pl.ds(16, S), :], sem.at[1 + c]),
            pltpu.make_async_copy(v_hbm.at[:, col], v_v.at[c, pl.ds(0, S), :], sem.at[1 + c]),
        ]

    def col_copies(src, dst, c0, s):
        rows = pl.ds(0, src.shape[0])
        return [pltpu.make_async_copy(src.at[:, pl.ds((c0 + c) * LANES, LANES)], dst.at[c0 + c, rows, :], sem.at[s])
                for c in range(NC)]

    WM = (0, 3 * D, 5 * D, 6 * D)
    wm_copies = [[pltpu.make_async_copy(wm_hbm.at[:, pl.ds(WM[j], WM[j + 1] - WM[j])],
                                        wm_v.at[:, pl.ds(WM[j], WM[j + 1] - WM[j])], sem.at[6 + j])]
                 for j in range(3)]
    w_copies = [col_copies(src, dst, 0, 12 + j)
                for j, (src, dst) in enumerate(((w1_hbm, w1_v), (w2_hbm, w2_v), (w3_hbm, w3_v), (w4_hbm, w4_v)))]

    B0 = [0]
    for n in TILES:
        B0.append(B0[-1] + n)
    NA = len(TILES)
    A0 = [0] + [r + HALO for r in B0[1:-1]] + [S]
    q_copies = [
        [pltpu.make_async_copy(q_hbm.at[pl.ds(A0[t], A0[t + 1] - A0[t])], q_v.at[pl.ds(A0[t], A0[t + 1] - A0[t])],
                               sem.at[16 + t])]
        for t in range(NA)
    ]

    def start_all(cps, priority=0):
        for cp in cps:
            cp.start(priority=priority)

    def wait_all(cps):
        for cp in cps:
            cp.wait()

    def packed(ref, c0=0):
        ru = ref.bitcast(U32)
        return _as_bf16(jnp.concatenate([ru[c0 + c] for c in range(NC)], axis=1))

    first, second = conv_copies(0), conv_copies(1)
    start_all(first[:1] + small + first[1:] + second)

    for c in range(NC):
        k_v[c, 0:16, :] = jnp.zeros((16, LANES), BF16)
        h1_s[c, 0:8, :] = jnp.zeros((8, LANES), F32)
        h1_s[c, S + 8:S + 16, :] = jnp.zeros((8, LANES), F32)
        w4_v[c, FF:FP, :] = jnp.zeros((FP - FF, LANES), BF16)

    prow = lax.broadcasted_iota(jnp.int32, (BLK, BLK), 0)
    pcol = lax.broadcasted_iota(jnp.int32, (BLK, BLK), 1)
    ang = (((4 * prow + 1) * pcol) & (4 * BLK - 1)).astype(F32) * (2.0 * math.pi / (4 * BLK))
    tw = (4 * prow + 1).astype(F32) * (2.0 * math.pi / (4 * LB))
    mr, mi = jnp.cos(ang), -jnp.sin(ang)
    zr_, zi_ = jnp.cos(tw), -jnp.sin(tw)
    eye = jnp.where(prow == pcol, 1.0 / LB, 0.0).astype(BF16)
    for i in range(PH):
        both = jnp.stack([mr.reshape(NG, 8, BLK), mi.reshape(NG, 8, BLK)], axis=1).reshape(2 * BLK, BLK)
        fw_s[i] = both.astype(BF16)
        for h in range(2):
            iv_s[i, h] = _dot_nt(eye, both[h * BLK:(h + 1) * BLK, :].astype(BF16)).astype(BF16)
        if i + 1 < PH:
            mr, mi = mr * zr_ - mi * zi_, mr * zi_ + mi * zr_
    perm = jnp.where(pcol == (prow % R) * PH + prow // R, 1.0, 0.0).astype(BF16)
    fw_u = fw_s.bitcast(U32)
    iv_u = iv_s.bitcast(U32)

    wait_all(small)
    shf = sh_v[...].astype(F32)
    sdf = sd_v[...].astype(F32).reshape(1, D)
    for c in range(NC):
        par_s[c, 0:4, :] = shf[:, c * LANES:(c + 1) * LANES]
        par_s[c, 4:5, :] = sdf[:, c * LANES:(c + 1) * LANES]
    cf = c_v[...].astype(F32)
    sc = (cf * jax.nn.sigmoid(cf)).astype(BF16)
    sc16 = jnp.broadcast_to(sc, (16, D))

    def mod_chunk(j):
        mod_s[j] = _dot(sc16, wm_v[:, j * D:(j + 1) * D])[0:8, :]

    k_u = k_v.bitcast(U32)
    v_u = v_v.bitcast(U32)
    wu_u = wu_s.bitcast(U32)
    z_u = z_s.bitcast(U32)
    vv_u = vv_s.bitcast(U32)
    lo_u = lo_s.bitcast(U32)
    l2_u = l2_s.bitcast(U32)

    never = zr_[0:8, :] > 2.0

    def after(token, x):
        if token.dtype != x.dtype:
            token = pltpu.bitcast(token, x.dtype)
        return jnp.where(jnp.broadcast_to(never, x.shape), token, x)

    def split(t):
        t4 = t.reshape(NG, 2, 8, LANES)
        return t4[:, 0], t4[:, 1]

    def perm_k(c, b, toks):
        kt = [_dot_nt(perm, sk_v[c, :, b * LB + t * BLK:b * LB + (t + 1) * BLK]) for t in range(PH)]
        for r in range(BLK // 16):
            toks.append(kt[0][16 * r:16 * r + 8, :])
        return [jnp.concatenate([kt[t][i * R:(i + 1) * R, :] for t in range(PH)], axis=0).astype(BF16)
                for i in range(PH)]

    def spectrum(wts, dst, c, b, toks, dc=None, pins=None):
        tr, ti = [], []
        for i in range(PH):
            lhs = fw_u[i]
            if pins is not None and i < len(pins):
                lhs = after(pins[i], lhs.reshape(NG, 8, LANES)).reshape(BLK, LANES)
            r_, i_ = split(_dot(_as_bf16(lhs), wts[i]))
            tr.append(r_)
            ti.append(i_)
        for g in range(NG):
            toks.append(ti[PH - 1][g])
        if dc is not None:
            tr[0] = tr[0] + dc
        sr, si = _dft4(tr, ti, -1)
        for qq in range(PH):
            dst[c, :, b, qq, 0] = sr[qq]
            dst[c, :, b, qq, 1] = si[qq]

    def gated(c, b):
        w = [par_s[c, t:t + 1, :] for t in range(4)]
        kc = {}
        for o in range(-2, 2):
            words = k_u[c, pl.ds(8 + b * (LB // 2) + o, BLK, stride=2), :]
            if o > -2:
                kc[2 * o] = _lo(words)
            kc[2 * o + 1] = _hi(words)
        vc = {}
        for o in range(2):
            words = v_u[c, pl.ds(b * (LB // 2) + o, BLK, stride=2), :]
            vc[2 * o] = _lo(words)
            vc[2 * o + 1] = _hi(words)
        for i in range(PH):
            ks = kc[i] * w[0]
            for t in range(1, 4):
                ks = ks + kc[i - t] * w[t]
            wu_s[b, i] = (ks * vc[i]).astype(BF16)
        return [wu_u[b, i] for i in range(PH)]

    def kv_pins(kvb):
        return [jnp.stack([kvb[2 * m + (r % 2)][8 * (r // 2):8 * (r // 2) + 8, :] for r in range(NG)])
                for m in range(2)]

    def mac(c, us, ks, toks):
        zp = None
        for o in range(NBL):
            zr, zi = [], []
            for qq in range(PH):
                accr = acci = None
                for b in range(o + 1):
                    a_, b_ = us[0, :, b, qq, 0], us[0, :, b, qq, 1]
                    c_, d_ = ks[0, :, o - b, qq, 0], ks[0, :, o - b, qq, 1]
                    if qq == 0 and b == o:
                        a_ = after(toks[o], a_)
                    tr_ = a_ * c_ - b_ * d_
                    ti_ = a_ * d_ + b_ * c_
                    accr = tr_ if accr is None else accr + tr_
                    acci = ti_ if acci is None else acci + ti_
                zr.append(accr)
                zi.append(acci)
            if zp is None:
                yr, yi = zr, zi
            else:
                yr = [zr[qq] - zp[1][qq] for qq in range(PH)]
                yi = [zi[qq] + zp[0][qq] for qq in range(PH)]
            zp = (zr, zi)
            vr, vi = _dft4(yr, yi, +1)
            for i in range(PH):
                vv_s[c, o, i] = jnp.stack([vr[i], vi[i]], axis=1).reshape(2 * BLK, LANES).astype(BF16)

    def inverse(c, toks, pins=None):
        HB = BLK // 2
        for o in range(NBL):
            for i in range(PH):
                yv = None
                for h in range(2):
                    lhs = iv_u[i, h]
                    if pins is not None and h == 0:
                        pin = pins[o][i % 2][8 * (i // 2):8 * (i // 2) + 8]
                        lhs = after(pin, lhs.reshape(8, 8, LANES)).reshape(HB, LANES)
                    t = _dot(_as_bf16(lhs), _as_bf16(vv_u[c, o, i, h * HB:(h + 1) * HB, :]))
                    yv = t if yv is None else yv + t
                if i % 2 == 0:
                    for r in range(BLK // 16):
                        toks.append(yv[16 * r:16 * r + 8, :])
                y_s[c, pl.ds(o * LB + i, BLK, stride=PH), :] = yv

    def mac_tokens(toks):
        n = len(toks) - 3
        cum = (44, 128, 244, 392)
        return [jnp.stack([toks[max(0, ((g * 392 + cum[o]) * n) // (392 * NG) - 1)] for g in range(NG)])
                for o in range(NBL)]

    def conv_round(c, fwd, mul, inv):
        toks = []
        kv = pins = None
        cur = 1 if mul else 0
        if fwd or mul:
            win = pl.ds(c - cur, 2 if fwd and mul else 1)
            us, ks = u_s.at[win], kk_s.at[win]
        if 'u' in fwd:
            kv = [gated(c, b) for b in range(NBL)]
            pins = [kv_pins(kv[b]) for b in range(NBL)]
        if inv:
            inverse(c - 2, toks, pins)
            if fwd:
                toks = []
        if 'k' in fwd:
            wts = [perm_k(c, b, toks) for b in range(NBL)]
        for b in range(NBL):
            if 'k' in fwd:
                spectrum(wts[b], ks, cur, b, toks, par_s[c, 4:5, :] if b == 0 else None)
            if 'u' in fwd:
                pin = pins[b + UL] if not inv and b + UL < NBL else None
                spectrum([_as_bf16(x) for x in kv[b]], us, cur, b, toks, None, pin)
        if mul:
            mac(c - 1, us, ks, mac_tokens(toks))

    def tokens_of(x):
        return [x[8 * r:8 * r + 8, c * LANES:(c + 1) * LANES] for c in range(NC) for r in range(x.shape[0] // 8)]

    def store_bf16(ref, r0, x):
        for c in range(NC):
            ref[c, r0:r0 + x.shape[0], :] = x[:, c * LANES:(c + 1) * LANES].astype(BF16)

    def load_bf16(ref_u, r0, n):
        return _as_bf16(jnp.concatenate([ref_u[c, pl.ds(r0 // 2, n // 2), :] for c in range(NC)], axis=1))

    def pick(toks, n, free):
        if toks is None:
            return [None] * n
        idx = [(r * (len(toks) + free)) // n - free for r in range(n)]
        return [toks[i] if i >= 0 else None for i in idx]

    def hold(x, tks):
        f = len([k for k in tks if k is None])
        n = len(tks)
        if f == n:
            return x
        first = after(jnp.stack(tks[f:]), x[8 * f:, 0:LANES].reshape(n - f, 8, LANES)).reshape(8 * (n - f), LANES)
        if f:
            first = jnp.concatenate([x[:8 * f, 0:LANES], first], axis=0)
        return jnp.concatenate([first, x[:, LANES:]], axis=1)

    def mods_a():
        ga = mod_s[2, 0:1, :]
        return ga * (1.0 + mod_s[1, 0:1, :]) * math.sqrt(D), ga * mod_s[0, 0:1, :]

    def mods_b():
        return (1.0 + mod_s[4, 0:1, :]) * (2.0 * math.sqrt(D)), 2.0 * mod_s[3, 0:1, :]

    def stage_p1(r0, r1, tks, ma):
        q = hold(q_v[r0:r1, :].astype(F32), tks)
        y = jnp.concatenate([y_s[c, r0:r1, :] for c in range(NC)], axis=1)
        x = q + (_ln(q, unit=False) * ma[0] + ma[1]) * y
        x_s[r0:r1, :] = x
        return _ln(x, unit=False)

    def halves(x):
        x4 = x.reshape(x.shape[0] // 32, 2, 16, LANES)
        return [x4[:, e].reshape(x.shape[0] // 2, LANES) for e in range(2)]

    def weave(top, bot):
        n = top.shape[0] // 16
        return jnp.stack([top.reshape(n, 16, LANES), bot.reshape(n, 16, LANES)], axis=1).reshape(32 * n, LANES)

    def row_ops(cols, tks=None):
        hv = [halves(x) for x in cols]
        if tks is not None:
            tk = jnp.stack(tks)

            def held(x):
                x4 = x.reshape(len(tks), 2, 8, LANES)
                return jnp.stack([after(tk, x4[:, 0]), x4[:, 1]], axis=1).reshape(x.shape)

            for k2 in range(2):
                hv[k2][0] = held(hv[k2][0])
                hv[2 + k2][1] = held(hv[2 + k2][1])
        per = [_lhs_ops(hv[k2][0], hv[2 + k2][0], hv[k2][1], hv[2 + k2][1]) + [hv[2 + k2][0], hv[k2][1]]
               for k2 in range(2)]
        return [[per[0][o], per[1][o]] for o in range(9)] + [hv[NC - 1]]

    def stage_p2(r0, r1, nx, mb, blockwise=False):
        h = nx * mb[0] + mb[1]
        h_s[r0:r1, :] = h
        zn = _ln(h, 4.0 * EPS)
        if not blockwise:
            store_bf16(z_s, r0, zn)
            return
        ops = row_ops([zn[:, c * LANES:(c + 1) * LANES] for c in range(NC)])
        for o in range(10):
            for e in range(2):
                lo_s[o, e, r0 // 2:r1 // 2, :] = ops[o][e].astype(BF16)

    def stage_p(t, toks, free):
        lo, hi = A0[t], A0[t + 1]
        stage_p2(lo, hi, stage_p1(lo, hi, pick(toks, (hi - lo) // 8, free), mods_a()), mods_b(), t in STR1)

    def square_ops(src, dst, toks):
        HK = 2 * LANES
        ng = HK // 16
        for n2 in range(2):
            tk = jnp.stack([toks[((n2 * ng + r) * len(toks)) // (2 * ng)] for r in range(ng)])

            def blk(c, k, hold_it):
                x = src[c, k * HK:(k + 1) * HK, :].astype(F32)
                if not hold_it:
                    return x
                x4 = x.reshape(ng, 2, 8, LANES)
                return jnp.stack([after(tk, x4[:, 0]), x4[:, 1]], axis=1).reshape(HK, LANES)

            for o, x in enumerate(_rhs_ops(blk(n2, 0, True), blk(2 + n2, 0, False), blk(n2, 1, False), blk(2 + n2, 1, True))):
                if o not in (1, 4):
                    dst[o, n2] = x.astype(BF16)

    def block_dots(lhs_of, w_ref, s_ref, parts, emit, WL, WH):
        w_u, s_u = w_ref.bitcast(U32), s_ref.bitcast(U32)
        toks = []

        def timed(x, weight):
            toks.extend(x[8 * r:8 * r + 8, 0:LANES] for r in range(x.shape[0] // 8) for _ in range(weight))
            return x

        def main(get):
            m = [None] * 7
            rem = [None, None]
            for o in ('t', 2, 4, 'b', 1, 3, 0, 6, 5):
                if o in ('t', 'b'):
                    e = 0 if o == 't' else 1
                    rhs = jnp.concatenate([w_u[c, 2 * LANES:D // 2, :] for c in range(NC - 1)], axis=1)
                    rem[e] = timed(_dot(get([(9, e)]), _as_bf16(rhs)), WL)
                    continue
                if o in (1, 4):
                    d = (1, 4).index(o)
                    rhs = jnp.concatenate([w_u[2 * d + n2, d * LANES:(d + 1) * LANES, :] for n2 in range(2)], axis=1)
                else:
                    rhs = jnp.concatenate([s_u[o, n2] for n2 in range(2)], axis=1)
                m[o] = timed(_dot(get([(o, 0), (o, 1)]), _as_bf16(rhs)), WH if o in (4, 3, 6, 5) else WL)
            c11, c12, c21, c22 = _combine(m)
            top = jnp.concatenate([c11, c12], axis=1) + rem[0]
            bot = jnp.concatenate([c21, c22], axis=1) + rem[1]
            return [weave(top[:, c * LANES:(c + 1) * LANES], bot[:, c * LANES:(c + 1) * LANES]) for c in range(NC - 1)]

        def last(get):
            w4c = _as_bf16(w_u[NC - 1])
            return weave(timed(_dot(get([(2, 0), (2, 1), (7, 0), (7, 1), (9, 0)]), w4c), WL),
                         timed(_dot(get([(8, 0), (8, 1), (3, 0), (3, 1), (9, 1)]), w4c), WL))

        marks = []
        for j, part in enumerate(parts):
            get = lhs_of(part, toks[marks[-1]:] if marks else None)
            marks.append(len(toks))
            if j % 2:
                tail = last(get)
                cols = main(get) + [tail]
            else:
                cols = main(get) + [last(get)]
            emit(part, cols)
        return toks

    def filler(t):
        if DUM:
            red = jnp.sum(y_s[t, 0:8 * DUM, :], axis=-1, keepdims=True).reshape(DUM, 8, 1)
            zf_s[1, (NC - 1) * (TQ + 8) + 8 * t:(NC - 1) * (TQ + 8) + 8 * t + 8, :] = jnp.broadcast_to(jnp.sum(red, axis=0), (8, LANES))

    def chunks(r0, r1, k, unit=16):
        n = (r1 - r0) // unit
        cuts = [r0 + unit * ((n * j) // k) for j in range(k + 1)]
        return list(zip(cuts[:-1], cuts[1:]))

    def stage_m1(t, k):
        def emit(part, cols):
            out = [_gelu2(x) for x in cols]
            for c in range(NC):
                h1_s[c, part[0] + 8:part[1] + 8, :] = out[c]
            return out

        if t in STR1:
            def lhs_of(part, _):
                return lambda keys: _as_bf16(jnp.concatenate(
                    [lo_u[o, e, part[0] // 4:part[1] // 4, :] for o, e in keys], axis=1))
            return block_dots(lhs_of, w1_v, s1_s, chunks(A0[t], A0[t + 1], k, 32), emit, WL, WH)
        toks = []
        for r0, r1 in chunks(A0[t], A0[t + 1], k):
            pre = _dot(load_bf16(z_u, r0, r1 - r0), packed(w1_v))
            out = emit((r0, r1), [pre[:, c * LANES:(c + 1) * LANES] for c in range(NC)])
            toks += [x for x in tokens_of(jnp.concatenate(out, axis=1)) for _ in range(W1N)]
        return toks

    grp = D // 4
    shifts = (-1, 1, -2, 2)

    def shifted(r0, r1):
        n = r1 - r0
        lane = lax.broadcasted_iota(jnp.int32, (n, LANES), 1)
        cols = []
        for c in range(NC):
            lo, hi = c * LANES, (c + 1) * LANES
            g_lo, g_hi = lo // grp, (hi - 1) // grp
            val = h1_s[c, pl.ds(r0 + 8 + shifts[g_lo], n), :]
            if g_hi != g_lo:
                other = h1_s[c, pl.ds(r0 + 8 + shifts[g_hi], n), :]
                val = jnp.where(lane < (g_hi * grp - lo), val, other)
            cols.append(val)
        return cols

    def stage_m2(t, k, before=None):
        def emit(part, cols):
            x1 = h_s[part[0]:part[1], :] + jnp.concatenate(cols, axis=1)
            h_s[part[0]:part[1], :] = x1
            return x1

        if t in STR2:
            def lhs_of(part, prev):
                prev = before if prev is None else prev
                prev = prev[len(prev) // 8:(len(prev) * 7) // 8]
                ops = row_ops(shifted(*part), pick(prev, (part[1] - part[0]) // 32, 0))
                for o in range(10):
                    for e in range(2):
                        l2_s[o, e, part[0] // 2:part[1] // 2, :] = ops[o][e].astype(BF16)
                return lambda keys: _as_bf16(jnp.concatenate(
                    [l2_u[o, e, part[0] // 4:part[1] // 4, :] for o, e in keys], axis=1))
            return block_dots(lhs_of, w2_v, s2_s, chunks(B0[t], B0[t + 1], k, 32), emit, WM2, WM2)
        toks = []
        for r0, r1 in chunks(B0[t], B0[t + 1], k):
            hs = _dot(jnp.concatenate(shifted(r0, r1), axis=1).astype(BF16), packed(w2_v))
            toks += [x for x in tokens_of(emit((r0, r1), [hs])) for _ in range(W2N)]
        return toks

    TQ = TB // 4
    NT = S // TB
    GB = 2 * NH + 1

    def blk_rows(b):
        return slice(b * (TQ + 8), b * (TQ + 8) + TQ)

    def store_z(r0, slot, toks, free):
        zn = _ln(hold(h_s[pl.ds(r0, TB), :], pick(toks, TB // 8, free)), 4.0 * EPS)
        for rq in range(4):
            for c in range(NC - 1):
                zf_s[slot, blk_rows(NC * rq + c), :] = zn[rq * TQ:(rq + 1) * TQ, c * LANES:(c + 1) * LANES]
        for c in range(NC):
            zr_s[c] = zn[:, c * LANES:(c + 1) * LANES].astype(BF16)

    def outer_lhs(i, blk):
        terms = ((0, 0, 1, 1, 1), (1, 0, 1, 1, 1), (0, 0), (1, 1), (0, 0, 1, 0, 1), (1, 0, -1, 0, 0), (0, 1, -1, 1, 1))[i]
        x = blk(terms[0], terms[1])
        if len(terms) > 2:
            y = blk(terms[3], terms[4])
            x = x + y if terms[2] > 0 else x - y
        return x

    def z_ops(slot_of, toks):
        ng = TQ // 16

        def held(x, k):
            tk = jnp.stack([toks[((k * ng + r) * len(toks)) // (7 * ng)] for r in range(ng)])
            x4 = x.reshape(ng, 2, 8, LANES)
            return jnp.stack([after(tk, x4[:, 0]), x4[:, 1]], axis=1).reshape(TQ, LANES)

        for k, i in enumerate(ZORD):
            slot = slot_of()
            so = [outer_lhs(i, lambda r1, k1: zf_s[slot, blk_rows(NC * (2 * r1 + r2) + 2 * k1 + k2), :])
                  for r2 in range(2) for k2 in range(2)]
            for j, x in enumerate(_lhs_ops(held(so[0], k), so[1], so[2], held(so[3], k))):
                la_s[i, j] = x.astype(BF16)

    NS = NH // 2

    RAW = (1, 4)

    def weight_ops(src, dst, ext, transposed, toks):
        ng = LANES // 16
        lead = 2 if ext is not None else 0
        total = (NS * 7 + lead) * ng

        def tile(c, n):
            return src[c, n * LANES:(n + 1) * LANES, :].astype(F32)

        def held(x, pos, step):
            tk = jnp.stack([toks[((pos + r * step) * len(toks)) // total] for r in range(ng)])
            x4 = x.reshape(ng, 2, 8, LANES)
            return jnp.stack([after(tk, x4[:, 0]), x4[:, 1]], axis=1).reshape(LANES, LANES)

        def outer(c2, n, pos=None):
            b11, b22 = tile(c2, n), tile(2 + c2, NH + n)
            if pos is not None:
                b11, b22 = held(b11, pos, 1), held(b22, pos, 1)
            e1, e2 = tile(c2, NH + n), tile(2 + c2, n)
            return _rhs_ops(b11, e1, e2, b22) if transposed else _rhs_ops(b11, e2, e1, b22)

        for c2 in range(2 if ext is not None else 0):
            for i, x in enumerate(outer(c2, NH - 1, c2 * ng)):
                if i not in RAW:
                    ext[i, c2] = x.astype(BF16)
        for st in range(NS):
            t00, t11 = outer(0, 2 * st), outer(1, 2 * st + 1)
            t01, t10 = outer(0, 2 * st + 1), outer(1, 2 * st)
            for k, i in enumerate((1, 5, 2, 4, 0, 3, 6)):
                pos = (lead + st * 7) * ng + k
                a, d = held(t00[i], pos, 7), held(t11[i], pos, 7)
                ops = _rhs_ops(a, t01[i], t10[i], d) if transposed else _rhs_ops(a, t10[i], t01[i], d)
                for j, x in enumerate(ops):
                    if i not in RAW or j not in RAW:
                        dst[i, j, st * LANES:(st + 1) * LANES, :] = x.astype(BF16)

    with jax.named_scope("r0a"):
        wait_all(first[:1])
        conv_round(0, 'k', False, False)
    with jax.named_scope("r0_wait"):
        wait_all(first[1:])
    with jax.named_scope("r0b"):
        start_all(conv_copies(2) + conv_copies(3) + conv_copies(4))
        conv_round(0, 'u', False, False)
    with jax.named_scope("r1a"):
        wait_all(second[:1])
        conv_round(1, 'k', True, False)
    with jax.named_scope("r1_wait"):
        wait_all(second[1:])
    with jax.named_scope("r1b"):
        start_all(wm_copies[0] + q_copies[0] + wm_copies[1] + w_copies[0])
        conv_round(1, 'u', False, False)

    def full_round(c, carry):
        wait_all(conv_copies(c))
        conv_round(c, 'ku', True, True)
        return carry

    with jax.named_scope("r234"):
        lax.fori_loop(2, NC, full_round, 0)
    with jax.named_scope("r5"):
        start_all(q_copies[1] + w_copies[1] + sum(q_copies[2:], []) + w_copies[2] + w_copies[3] + wm_copies[2], 1)
        conv_round(NC, '', True, True)
    with jax.named_scope("r6_wait"):
        wait_all(wm_copies[0] + q_copies[0])
    with jax.named_scope("r6"):
        for j in range(3):
            mod_chunk(j)
        conv_round(NC + 1, '', False, True)
        nx0 = stage_p1(0, A0[1], [None], mods_a())
    with jax.named_scope("p2_wait"):
        wait_all(wm_copies[1])
    with jax.named_scope("p2"):
        mod_chunk(4)
        mod_chunk(3)
        stage_p2(0, A0[1], nx0, mods_b())
    with jax.named_scope("w1_wait"):
        wait_all(w_copies[0])
    with jax.named_scope("m1_0"):
        toks = stage_m1(0, 4)
        if STR1:
            square_ops(w1_v, s1_s, toks[:len(toks) - 20 * W1N])
    with jax.named_scope("w2_wait"):
        wait_all(q_copies[1] + w_copies[1])
    with jax.named_scope("m2_0"):
        toks = stage_m2(0, 4)
        stage_p(1, toks[:len(toks) - TRIM * W2N], FREE * W2N)
        if STR2 and min(STR2) == 1:
            square_ops(w2_v, s2_s, toks[len(toks) // 2:len(toks) - 10 * W2N])
        filler(0)
    for t in range(1, NA):
        with jax.named_scope("a%d" % t):
            if t + 1 < NA:
                wait_all(q_copies[t + 1])
            else:
                wait_all(w_copies[2] + w_copies[3] + wm_copies[2])
            t1 = stage_m1(t, SPLIT)
            t2 = stage_m2(t, SPLIT, t1[len(t1) - len(t1) // SPLIT:])

            def weighted(trim):
                return t1 + t2[:len(t2) - trim * W2N]

            if t + 1 < NA:
                stage_p(t + 1, weighted(TRIM), FREE * W2N)
            if STR2 and t == W2P:
                square_ops(w2_v, s2_s, weighted(10))
            if t == NA - 1 - LAT:
                toks = weighted(TRIM // 2)
                store_z(0, 0, toks if LAT and not ZE else toks[:len(toks) // 2], FREE * W2N)
                if ZE:
                    toks = weighted(10)
                    z_ops(lambda: 0, toks[(len(toks) * 5) // 8:])
            if t == NA - 1:
                mod_chunk(NC)
                toks = weighted(20)
                toks = toks[:1] * PRE + toks
                cut = (len(toks) * 21) // 44
                weight_ops(w3_v, s3_s, None, True, toks[:cut])
                weight_ops(w4_v, s4_s, e4_s, False, toks[cut:])
                if not ZE:
                    z_ops(lambda: 0, toks if LAT else toks[(len(toks) * 5) // 8:])
            if t + 1 < NA or not LAT:
                filler(t)

    gb = 0.5 * mod_s[NC, 0:1, :]
    w3_u, w4_u, s3_u, s4_u, e4_u = (r.bitcast(U32) for r in (w3_v, w4_v, s3_s, s4_s, e4_s))
    HL = LANES // 2
    la_u = la_s.bitcast(U32)
    zr_u = zr_s.bitcast(U32)

    def out_copy(r0, n, c):
        rows = pl.ds(r0, n)
        return pltpu.make_async_copy(o_v.at[c, rows, :], o_hbm.at[rows, pl.ds(c * LANES, LANES)], sem_o.at[0])

    def one_level(w_u, e_u, i, c2):
        if i not in RAW:
            return e_u[i, c2]
        d = RAW.index(i)
        n = d * NH + NH - 1
        return w_u[2 * d + c2, n * HL:(n + 1) * HL, :]

    def two_level(w_u, s_u, i, j, st):
        if i not in RAW or j not in RAW:
            return s_u[i, j, st * HL:(st + 1) * HL, :]
        d, e = RAW.index(i), RAW.index(j)
        n = d * NH + 2 * st + e
        return w_u[2 * d + e, n * HL:(n + 1) * HL, :]

    def loop_b(t, carry):
        r0 = pl.multiple_of(t * TB, TB)
        ws = t & 1

        count = [0]

        def fresh():
            count[0] += 1
            return lax.rem(t + 2 * count[0], 2)

        zr = [_as_bf16(zr_u[NC - 1, rq * (TQ // 2):(rq + 1) * (TQ // 2), :]) for rq in range(4)]
        ltoks, ftoks = [], []

        def light(x):
            ltoks.extend(x[8 * r:8 * r + 8, 0:LANES] for r in range(x.shape[0] // 8))

        def rem3(rq, n):
            return _dot_nt(zr[rq], _as_bf16(w3_u[NC - 1, n * HL:(n + 1) * HL, :]))

        def put_g(rq, n, pre):
            g_s[ws, blk_rows(GB * rq + n), :] = _gelu2(pre)

        rem = {}
        for st in range(NS):
            rem[3, NH + 2 * st + 1] = rem3(3, NH + 2 * st + 1)
        n0 = NH - 1
        w_mid = _as_bf16(jnp.concatenate([w3_u[c, n0 * HL:(n0 + 1) * HL, :] for c in range(NC)], axis=1))
        lo = (2 * NH - 1) * HL
        w_end = _as_bf16(jnp.concatenate([w3_u[c, lo:FF // 2, :] for c in range(NC)], axis=1))
        for rq in range(4):
            zq = _as_bf16(jnp.concatenate([zr_u[c, rq * (TQ // 2):(rq + 1) * (TQ // 2), :] for c in range(NC)], axis=1))
            mid = _dot_nt(zq, w_mid)
            ftoks.extend(mid[8 * r:8 * r + 8, :] for r in range(TQ // 8))
            put_g(rq, n0, mid)
            gt = _gelu2(_dot_nt(w_end, zq))
            g_s[ws, blk_rows(GB * rq + 2 * NH - 1), :] = jnp.concatenate([gt, jnp.zeros((FP - FF, TQ), F32)], axis=0).T
        for st in range(NS):
            todo = [(2 * r1 + r2, h * NH + 2 * st + p) for r1, h in ((0, 1), (1, 0), (0, 0), (1, 1))
                    for r2 in range(2) for p in range(2)]
            todo = [x for x in todo if x not in rem]
            for key in todo[:8]:
                rem[key] = rem3(*key)
            if st >= LSETS:
                light(rem[todo[1]])
                light(rem[todo[5]])
            todo = todo[8:]
            pin = [None] * 7
            for i in _ORDER:
                m = [None] * 7
                for j in _ORDER:
                    m[j] = _dot_nt(_as_bf16(la_u[i, j]), _as_bf16(two_level(w3_u, s3_u, i, j, st)))
                if st >= LSETS and i in (2, 1, 0):
                    light(m[_ORDER[1]])
                    light(m[_ORDER[5]])
                key = todo.pop(0)
                rem[key] = rem3(*key)
                pin[i] = _combine(m)
            for inner in range(4):
                for blk, cval in enumerate(_combine([pin[i][inner] for i in range(7)])):
                    rq, n = 2 * (blk // 2) + inner // 2, (blk % 2) * NH + 2 * st + inner % 2
                    put_g(rq, n, cval + rem[rq, n])

        toks = []

        def timed(x):
            toks.extend(x[8 * r:8 * r + 8, 0:LANES] for r in range(x.shape[0] // 8))
            return x

        def finish(rq, c, h2):
            rows = pl.ds(pl.multiple_of(r0 + rq * TQ, TQ), TQ)
            cols = slice(c * LANES, (c + 1) * LANES)
            o_v[c, rows, :] = (x_s[rows, cols] + gb[:, cols] * (h_s[rows, cols] + h2)).astype(BF16)

        kord = [NH - 1, 2 * NH - 1] + [h * NH + n for st in range(NS) for h in (1, 0) for n in (2 * st + 1, 2 * st)]
        w4r = _as_bf16(jnp.concatenate([w4_u[NC - 1, n * HL:(n + 1) * HL, :] for n in kord], axis=0))

        def rem4(rq, slot):
            lhs = jnp.concatenate([g_s[slot, blk_rows(GB * rq + n), :] for n in kord], axis=1).astype(BF16)
            r = timed(_dot(lhs, w4r))
            finish(rq, NC - 1, r)

        rem4(0, fresh())
        rem4(1, fresh())
        pin = [None] * 7
        done = {_ORDER[1]: 1, _ORDER[3]: 2, _ORDER[5]: 0, _ORDER[6]: 3}
        for i in _ORDER:
            slot = fresh()
            rhs = _as_bf16(jnp.concatenate([one_level(w4_u, e4_u, i, c2) for c2 in range(2)], axis=1))
            ex = [_dot(outer_lhs(i, lambda r1, h: g_s[slot, blk_rows(GB * (2 * r1 + r2) + h * NH + NH - 1), :]).astype(BF16), rhs)
                  for r2 in range(2)]
            m = [None] * 7
            for j in _ORDER:
                slot = fresh()
                lhs = jnp.concatenate(
                    [outer_lhs(j, lambda r2, p: outer_lhs(
                        i, lambda r1, h: g_s[slot, blk_rows(GB * (2 * r1 + r2) + h * NH + 2 * st + p), :]))
                     for st in range(NS)], axis=1).astype(BF16)
                m[j] = timed(_dot(lhs, _as_bf16(jnp.concatenate([two_level(w4_u, s4_u, i, j, st) for st in range(NS)], axis=0))))
            pin[i] = [x + ex[inner // 2][:, (inner % 2) * LANES:(inner % 2 + 1) * LANES]
                      for inner, x in enumerate(_combine(m))]
            if i in done:
                blk = done[i]
                for inner in (1, 2, 0, 3):
                    p = [pin[k][inner] if pin[k] is not None else None for k in range(7)]
                    cval = (lambda: (p[3] - p[4]) + p[0] + p[6], lambda: p[2] + p[4], lambda: p[1] + p[3],
                            lambda: (p[2] - p[1]) + p[0] + p[5])[blk]()
                    finish(2 * (blk // 2) + inner // 2, 2 * (blk % 2) + inner % 2, cval)
                rb = pl.multiple_of(r0 + (blk // 2) * 2 * TQ, 2 * TQ)
                for e in range(2):
                    out_copy(rb, 2 * TQ, 2 * (blk % 2) + e).start()
                if blk == 0:
                    out_copy(r0, 3 * TQ, NC - 1).start()
            if i == _ORDER[REM2]:
                rem4(2, fresh())
        rem4(3, fresh())
        out_copy(pl.multiple_of(r0 + 3 * TQ, TQ), TQ, NC - 1).start()

        nxt = jnp.minimum(t + 1, NT - 1)
        store_z(pl.multiple_of(nxt * TB, TB), ws, ftoks[len(ftoks) - FT:] + ltoks[:LN1:LSTEP] + toks[:LB1], 0)
        z_ops(fresh, toks[ZB0:ZB1])
        if DUMB:
            filler(4)
        return carry

    with jax.named_scope("ph2b"):
        lax.fori_loop(0, NT, loop_b, 0)
    with jax.named_scope("tail"):
        pltpu.make_async_copy(o_v, o_v, sem_o.at[0]).wait()


@jax.jit
def pallas_adaLN_cond__ssm_conv_h3__mixer_s_mlp__prompt_kernel(
    A_q: jax.Array,
    A_k: jax.Array,
    A_v: jax.Array,
    A_shift_k: jax.Array,
    A_ssm_k: jax.Array,
    A_ssm_D: jax.Array,
    B_x: jax.Array,
    B_w1: jax.Array,
    B_w2: jax.Array,
    B_w3: jax.Array,
    B_w4: jax.Array,
    c: jax.Array,
    w_mod: jax.Array,
):
    B, S, D = A_q.shape
    assert B == 1
    FF = B_w3.shape[1]
    NC = D // LANES
    NG = BLK // 8
    NBL = S // (PH * BLK)
    FP = -(-FF // (2 * LANES)) * 2 * LANES
    TILES = (384, 384, 576, 704)
    assert sum(TILES) == S
    TB = 512

    args = (A_q.reshape(S, D), A_k.reshape(S, D), A_v.reshape(S, D), A_shift_k.T, A_ssm_k,
            A_ssm_D, B_w1, B_w2, B_w3.T, B_w4, c, w_mod)
    scratch = [
        pltpu.VMEM((S, D), BF16),
        pltpu.VMEM((NC, S + KP, LANES), BF16),
        pltpu.VMEM((NC, S + VP, LANES), BF16),
        pltpu.VMEM((4, D), BF16),
        pltpu.VMEM((NC, LANES, S), BF16),
        pltpu.VMEM((D,), BF16),
        pltpu.VMEM((NC, D, LANES), BF16),
        pltpu.VMEM((NC, D, LANES), BF16),
        pltpu.VMEM((NC, FF, LANES), BF16),
        pltpu.VMEM((NC, FP, LANES), BF16),
        pltpu.VMEM((1, D), BF16),
        pltpu.VMEM((D, 6 * D), BF16),
        pltpu.VMEM((PH, 2 * BLK, BLK), BF16),
        pltpu.VMEM((PH, 2, BLK, BLK), BF16),
        pltpu.VMEM((NC, S, LANES), BF16),
        pltpu.VMEM((NC, NG, NBL, PH, 2, 8, LANES), F32),
        pltpu.VMEM((NC, NG, NBL, PH, 2, 8, LANES), F32),
        pltpu.VMEM((NC, NBL, PH, 2 * BLK, LANES), BF16),
        pltpu.VMEM((NBL, PH, BLK, LANES), BF16),
        pltpu.VMEM((NC, S + YP, LANES), F32),
        pltpu.VMEM((6, 8, D), F32),
        pltpu.VMEM((NC, 8, LANES), F32),
        pltpu.VMEM((NC, S + 16, LANES), F32),
        pltpu.VMEM((S, D), F32),
        pltpu.VMEM((S, D), F32),
        pltpu.VMEM((NC, S, LANES), BF16),
        pltpu.VMEM((7, 7, FP // 512 * LANES, LANES), BF16),
        pltpu.VMEM((7, 7, FP // 512 * LANES, LANES), BF16),
        pltpu.VMEM((7, 2, LANES, LANES), BF16),
        pltpu.VMEM((2, GR, LANES), F32),
        pltpu.VMEM((2, ZR, LANES), F32),
        pltpu.VMEM((NC, TB, LANES), BF16),
        pltpu.VMEM((7, 7, TB // 4, LANES), BF16),
        pltpu.VMEM((10, 2, S // 2, LANES), BF16),
        pltpu.VMEM((10, 2, S // 2, LANES), BF16),
        pltpu.VMEM((7, 2, 2 * LANES, LANES), BF16),
        pltpu.VMEM((7, 2, 2 * LANES, LANES), BF16),
        pltpu.SemaphoreType.DMA((16 + len(TILES),)),
        pltpu.SemaphoreType.DMA((1,)),
    ]
    out = pl.pallas_call(
        functools.partial(_kernel, S=S, D=D, FF=FF, TILES=TILES, TB=TB),
        in_specs=[pl.BlockSpec(memory_space=pl.ANY)] * len(args),
        out_specs=pl.BlockSpec(memory_space=pl.ANY),
        out_shape=jax.ShapeDtypeStruct((S, D), BF16),
        scratch_shapes=scratch,
        compiler_params=pltpu.CompilerParams(
            vmem_limit_bytes=126 * 1024 * 1024,
            disable_bounds_checks=True,
            disable_semaphore_checks=True,
        ),
    )(*args)
    return out.reshape(B, S, D)
```

```python
import functools
import math

import jax
import jax.numpy as jnp
from jax import lax
import jax.experimental.pallas as pl
import jax.experimental.pallas.tpu as pltpu

F32 = jnp.float32
BF16 = jnp.bfloat16
U32 = jnp.uint32

LANES = 128
BLK = 128
PH = 4
EPS = 1e-05
TRIM = 60
SPLIT = 2
FREE = 30
DUM = 96
LN1 = 999
KP = 16
VP = 0
YP = 0
GR = 4080
ZR = 2720
FT = 0
DUMB = 1
STR1 = (3, )
STR2 = (2, 3, )
WL = 3
WH = 2
ZE = 1
PRE = 0
WM2 = 2
W2P = 1
UL = 2
ALN = 0
W1N = 2
W2N = 3
LAT = 1
LSETS = 0
LSTEP = 4
LB1 = 0
ZB0 = 0
ZB1 = 140
REM2 = 2
ZORD = (2, 3, 0, 1, 4, 5, 6)


def _as_bf16(x):
    return pltpu.bitcast(x, BF16)


def _lo(x):
    return pltpu.bitcast(x << 16, F32)


def _hi(x):
    return pltpu.bitcast(x & jnp.uint32(0xFFFF0000), F32)


def _dft4(re, im, sign):
    ar, ai = re[0] + re[2], im[0] + im[2]
    br, bi = re[0] - re[2], im[0] - im[2]
    cr, ci = re[1] + re[3], im[1] + im[3]
    dr, di = re[1] - re[3], im[1] - im[3]
    o0 = (ar + cr, ai + ci)
    o2 = (ar - cr, ai - ci)
    m = (br + di, bi - dr)
    p = (br - di, bi + dr)
    o1, o3 = (m, p) if sign < 0 else (p, m)
    return [o0[0], o1[0], o2[0], o3[0]], [o0[1], o1[1], o2[1], o3[1]]


def _ln(x, eps=EPS, unit=True):
    n = x.shape[-1]
    s1 = jnp.sum(x, axis=-1, keepdims=True)
    m = s1 * (1.0 / n)
    v = jnp.maximum(jnp.sum(x * x, axis=-1, keepdims=True) + (n * eps - s1 * m), n * eps)
    e = jnp.log(v) * (-0.5 / math.log(2.0))
    return (x - m) * jnp.exp2(e + 0.5 * math.log2(n) if unit else e)


def _gelu2(x):
    c0 = math.sqrt(2.0 / math.pi)
    return x + x * jnp.tanh(x * (c0 + (c0 * 0.044715) * (x * x)))


def _dot(a, b):
    return jnp.dot(a, b, preferred_element_type=F32)


def _dot_nt(a, b):
    return lax.dot_general(a, b, (((1,), (1,)), ((), ())), preferred_element_type=F32)


def _lhs_ops(a11, a12, a21, a22):
    return [a11 + a22, a21 + a22, a11, a22, a11 + a12, a21 - a11, a12 - a22]


def _rhs_ops(b11, b12, b21, b22):
    return [b11 + b22, b11, b12 - b22, b21 - b11, b22, b11 + b12, b21 + b22]


def _combine(m):
    return (m[3] - m[4]) + m[0] + m[6], m[2] + m[4], m[1] + m[3], (m[2] - m[1]) + m[0] + m[5]


_ORDER = (2, 4, 1, 3, 0, 6, 5)


def _kernel(q_hbm, k_hbm, v_hbm, sh_hbm, sk_hbm, sd_hbm, w1_hbm, w2_hbm, w3_hbm, w4_hbm, c_hbm, wm_hbm,
            o_hbm,
            q_v, k_v, v_v, sh_v, sk_v, sd_v, w1_v, w2_v, w3_v, w4_v, c_v, wm_v,
            fw_s, iv_s, o_v, u_s, kk_s, vv_s, wu_s, y_s, mod_s, par_s, h1_s, x_s, h_s, z_s, s3_s, s4_s, e4_s, g_s, zf_s, zr_s, la_s, lo_s, l2_s, s1_s, s2_s,
            sem, sem_o,
            *, S, D, FF, TILES, TB):
    NC = D // LANES
    NG = BLK // 8
    LB = PH * BLK
    NBL = S // LB
    R = BLK // PH
    HALO = 32
    FP = w4_v.shape[1]
    FH = FP // 2
    NH = FH // LANES

    small = [
        pltpu.make_async_copy(sh_hbm, sh_v, sem.at[0]),
        pltpu.make_async_copy(sd_hbm, sd_v, sem.at[0]),
        pltpu.make_async_copy(c_hbm, c_v, sem.at[0]),
    ]

    def conv_copies(c):
        col = pl.ds(c * LANES if isinstance(c, int) else pl.multiple_of(c * LANES, LANES), LANES)
        return [
            pltpu.make_async_copy(sk_hbm.at[col, :], sk_v.at[c], sem.at[9 + c if isinstance(c, int) and c < 2 else 1 + c]),
            pltpu.make_async_copy(k_hbm.at[:, col], k_v.at[c, pl.ds(16, S), :], sem.at[1 + c]),
            pltpu.make_async_copy(v_hbm.at[:, col], v_v.at[c, pl.ds(0, S), :], sem.at[1 + c]),
        ]

    def col_copies(src, dst, c0, s):
        rows = pl.ds(0, src.shape[0])
        return [pltpu.make_async_copy(src.at[:, pl.ds((c0 + c) * LANES, LANES)], dst.at[c0 + c, rows, :], sem.at[s])
                for c in range(NC)]

    WM = (0, 3 * D, 5 * D, 6 * D)
    wm_copies = [[pltpu.make_async_copy(wm_hbm.at[:, pl.ds(WM[j], WM[j + 1] - WM[j])],
                                        wm_v.at[:, pl.ds(WM[j], WM[j + 1] - WM[j])], sem.at[6 + j])]
                 for j in range(3)]
    w_copies = [col_copies(src, dst, 0, 12 + j)
                for j, (src, dst) in enumerate(((w1_hbm, w1_v), (w2_hbm, w2_v), (w3_hbm, w3_v), (w4_hbm, w4_v)))]

    B0 = [0]
    for n in TILES:
        B0.append(B0[-1] + n)
    NA = len(TILES)
    A0 = [0] + [r + HALO for r in B0[1:-1]] + [S]
    q_copies = [
        [pltpu.make_async_copy(q_hbm.at[pl.ds(A0[t], A0[t + 1] - A0[t])], q_v.at[pl.ds(A0[t], A0[t + 1] - A0[t])],
                               sem.at[16 + t])]
        for t in range(NA)
    ]

    def start_all(cps, priority=0):
        for cp in cps:
            cp.start(priority=priority)

    def wait_all(cps):
        for cp in cps:
            cp.wait()

    def packed(ref, c0=0):
        ru = ref.bitcast(U32)
        return _as_bf16(jnp.concatenate([ru[c0 + c] for c in range(NC)], axis=1))

    first, second = conv_copies(0), conv_copies(1)
    start_all(first[:1] + small + first[1:] + second)

    for c in range(NC):
        k_v[c, 0:16, :] = jnp.zeros((16, LANES), BF16)
        h1_s[c, 0:8, :] = jnp.zeros((8, LANES), F32)
        h1_s[c, S + 8:S + 16, :] = jnp.zeros((8, LANES), F32)
        w4_v[c, FF:FP, :] = jnp.zeros((FP - FF, LANES), BF16)

    prow = lax.broadcasted_iota(jnp.int32, (BLK, BLK), 0)
    pcol = lax.broadcasted_iota(jnp.int32, (BLK, BLK), 1)
    ang = (((4 * prow + 1) * pcol) & (4 * BLK - 1)).astype(F32) * (2.0 * math.pi / (4 * BLK))
    tw = (4 * prow + 1).astype(F32) * (2.0 * math.pi / (4 * LB))
    mr, mi = jnp.cos(ang), -jnp.sin(ang)
    zr_, zi_ = jnp.cos(tw), -jnp.sin(tw)
    eye = jnp.where(prow == pcol, 1.0 / LB, 0.0).astype(BF16)
    for i in range(PH):
        both = jnp.stack([mr.reshape(NG, 8, BLK), mi.reshape(NG, 8, BLK)], axis=1).reshape(2 * BLK, BLK)
        fw_s[i] = both.astype(BF16)
        for h in range(2):
            iv_s[i, h] = _dot_nt(eye, both[h * BLK:(h + 1) * BLK, :].astype(BF16)).astype(BF16)
        if i + 1 < PH:
            mr, mi = mr * zr_ - mi * zi_, mr * zi_ + mi * zr_
    perm = jnp.where(pcol == (prow % R) * PH + prow // R, 1.0, 0.0).astype(BF16)
    fw_u = fw_s.bitcast(U32)
    iv_u = iv_s.bitcast(U32)

    wait_all(small)
    shf = sh_v[...].astype(F32)
    sdf = sd_v[...].astype(F32).reshape(1, D)
    for c in range(NC):
        par_s[c, 0:4, :] = shf[:, c * LANES:(c + 1) * LANES]
        par_s[c, 4:5, :] = sdf[:, c * LANES:(c + 1) * LANES]
    cf = c_v[...].astype(F32)
    sc = (cf * jax.nn.sigmoid(cf)).astype(BF16)
    sc16 = jnp.broadcast_to(sc, (16, D))

    def mod_chunk(j):
        mod_s[j] = _dot(sc16, wm_v[:, j * D:(j + 1) * D])[0:8, :]

    k_u = k_v.bitcast(U32)
    v_u = v_v.bitcast(U32)
    wu_u = wu_s.bitcast(U32)
    z_u = z_s.bitcast(U32)
    vv_u = vv_s.bitcast(U32)
    lo_u = lo_s.bitcast(U32)
    l2_u = l2_s.bitcast(U32)

    never = zr_[0:8, :] > 2.0

    def after(token, x):
        if token.dtype != x.dtype:
            token = pltpu.bitcast(token, x.dtype)
        return jnp.where(jnp.broadcast_to(never, x.shape), token, x)

    def split(t):
        t4 = t.reshape(NG, 2, 8, LANES)
        return t4[:, 0], t4[:, 1]

    def perm_k(c, b, toks):
        kt = [_dot_nt(perm, sk_v[c, :, b * LB + t * BLK:b * LB + (t + 1) * BLK]) for t in range(PH)]
        for r in range(BLK // 16):
            toks.append(kt[0][16 * r:16 * r + 8, :])
        return [jnp.concatenate([kt[t][i * R:(i + 1) * R, :] for t in range(PH)], axis=0).astype(BF16)
                for i in range(PH)]

    def spectrum(wts, dst, c, b, toks, dc=None, pins=None):
        tr, ti = [], []
        for i in range(PH):
            lhs = fw_u[i]
            if pins is not None and i < len(pins):
                lhs = after(pins[i], lhs.reshape(NG, 8, LANES)).reshape(BLK, LANES)
            r_, i_ = split(_dot(_as_bf16(lhs), wts[i]))
            tr.append(r_)
            ti.append(i_)
        for g in range(NG):
            toks.append(ti[PH - 1][g])
        if dc is not None:
            tr[0] = tr[0] + dc
        sr, si = _dft4(tr, ti, -1)
        for qq in range(PH):
            dst[c, :, b, qq, 0] = sr[qq]
            dst[c, :, b, qq, 1] = si[qq]

    def gated(c, b):
        w = [par_s[c, t:t + 1, :] for t in range(4)]
        kc = {}
        for o in range(-2, 2):
            words = k_u[c, pl.ds(8 + b * (LB // 2) + o, BLK, stride=2), :]
            if o > -2:
                kc[2 * o] = _lo(words)
            kc[2 * o + 1] = _hi(words)
        vc = {}
        for o in range(2):
            words = v_u[c, pl.ds(b * (LB // 2) + o, BLK, stride=2), :]
            vc[2 * o] = _lo(words)
            vc[2 * o + 1] = _hi(words)
        for i in range(PH):
            ks = kc[i] * w[0]
            for t in range(1, 4):
                ks = ks + kc[i - t] * w[t]
            wu_s[b, i] = (ks * vc[i]).astype(BF16)
        return [wu_u[b, i] for i in range(PH)]

    def kv_pins(kvb):
        return [jnp.stack([kvb[2 * m + (r % 2)][8 * (r // 2):8 * (r // 2) + 8, :] for r in range(NG)])
                for m in range(2)]

    def mac(c, us, ks, toks):
        zp = None
        for o in range(NBL):
            zr, zi = [], []
            for qq in range(PH):
                accr = acci = None
                for b in range(o + 1):
                    a_, b_ = us[0, :, b, qq, 0], us[0, :, b, qq, 1]
                    c_, d_ = ks[0, :, o - b, qq, 0], ks[0, :, o - b, qq, 1]
                    if qq == 0 and b == o:
                        a_ = after(toks[o], a_)
                    tr_ = a_ * c_ - b_ * d_
                    ti_ = a_ * d_ + b_ * c_
                    accr = tr_ if accr is None else accr + tr_
                    acci = ti_ if acci is None else acci + ti_
                zr.append(accr)
                zi.append(acci)
            if zp is None:
                yr, yi = zr, zi
            else:
                yr = [zr[qq] - zp[1][qq] for qq in range(PH)]
                yi = [zi[qq] + zp[0][qq] for qq in range(PH)]
            zp = (zr, zi)
            vr, vi = _dft4(yr, yi, +1)
            for i in range(PH):
                vv_s[c, o, i] = jnp.stack([vr[i], vi[i]], axis=1).reshape(2 * BLK, LANES).astype(BF16)

    def inverse(c, toks, pins=None):
        HB = BLK // 2
        for o in range(NBL):
            for i in range(PH):
                yv = None
                for h in range(2):
                    lhs = iv_u[i, h]
                    if pins is not None and h == 0:
                        pin = pins[o][i % 2][8 * (i // 2):8 * (i // 2) + 8]
                        lhs = after(pin, lhs.reshape(8, 8, LANES)).reshape(HB, LANES)
                    t = _dot(_as_bf16(lhs), _as_bf16(vv_u[c, o, i, h * HB:(h + 1) * HB, :]))
                    yv = t if yv is None else yv + t
                if i % 2 == 0:
                    for r in range(BLK // 16):
                        toks.append(yv[16 * r:16 * r + 8, :])
                y_s[c, pl.ds(o * LB + i, BLK, stride=PH), :] = yv

    def mac_tokens(toks):
        n = len(toks) - 3
        cum = (44, 128, 244, 392)
        return [jnp.stack([toks[max(0, ((g * 392 + cum[o]) * n) // (392 * NG) - 1)] for g in range(NG)])
                for o in range(NBL)]

    def conv_round(c, fwd, mul, inv):
        toks = []
        kv = pins = None
        cur = 1 if mul else 0
        if fwd or mul:
            win = pl.ds(c - cur, 2 if fwd and mul else 1)
            us, ks = u_s.at[win], kk_s.at[win]
        if 'u' in fwd:
            kv = [gated(c, b) for b in range(NBL)]
            pins = [kv_pins(kv[b]) for b in range(NBL)]
        if inv:
            inverse(c - 2, toks, pins)
            if fwd:
                toks = []
        if 'k' in fwd:
            wts = [perm_k(c, b, toks) for b in range(NBL)]
        for b in range(NBL):
            if 'k' in fwd:
                spectrum(wts[b], ks, cur, b, toks, par_s[c, 4:5, :] if b == 0 else None)
            if 'u' in fwd:
                pin = pins[b + UL] if not inv and b + UL < NBL else None
                spectrum([_as_bf16(x) for x in kv[b]], us, cur, b, toks, None, pin)
        if mul:
            mac(c - 1, us, ks, mac_tokens(toks))

    def tokens_of(x):
        return [x[8 * r:8 * r + 8, c * LANES:(c + 1) * LANES] for c in range(NC) for r in range(x.shape[0] // 8)]

    def store_bf16(ref, r0, x):
        for c in range(NC):
            ref[c, r0:r0 + x.shape[0], :] = x[:, c * LANES:(c + 1) * LANES].astype(BF16)

    def load_bf16(ref_u, r0, n):
        return _as_bf16(jnp.concatenate([ref_u[c, pl.ds(r0 // 2, n // 2), :] for c in range(NC)], axis=1))

    def pick(toks, n, free):
        if toks is None:
            return [None] * n
        idx = [(r * (len(toks) + free)) // n - free for r in range(n)]
        return [toks[i] if i >= 0 else None for i in idx]

    def hold(x, tks):
        f = len([k for k in tks if k is None])
        n = len(tks)
        if f == n:
            return x
        first = after(jnp.stack(tks[f:]), x[8 * f:, 0:LANES].reshape(n - f, 8, LANES)).reshape(8 * (n - f), LANES)
        if f:
            first = jnp.concatenate([x[:8 * f, 0:LANES], first], axis=0)
        return jnp.concatenate([first, x[:, LANES:]], axis=1)

    def mods_a():
        ga = mod_s[2, 0:1, :]
        return ga * (1.0 + mod_s[1, 0:1, :]) * math.sqrt(D), ga * mod_s[0, 0:1, :]

    def mods_b():
        return (1.0 + mod_s[4, 0:1, :]) * (2.0 * math.sqrt(D)), 2.0 * mod_s[3, 0:1, :]

    def stage_p1(r0, r1, tks, ma):
        q = hold(q_v[r0:r1, :].astype(F32), tks)
        y = jnp.concatenate([y_s[c, r0:r1, :] for c in range(NC)], axis=1)
        x = q + (_ln(q, unit=False) * ma[0] + ma[1]) * y
        x_s[r0:r1, :] = x
        return _ln(x, unit=False)

    def halves(x):
        x4 = x.reshape(x.shape[0] // 32, 2, 16, LANES)
        return [x4[:, e].reshape(x.shape[0] // 2, LANES) for e in range(2)]

    def weave(top, bot):
        n = top.shape[0] // 16
        return jnp.stack([top.reshape(n, 16, LANES), bot.reshape(n, 16, LANES)], axis=1).reshape(32 * n, LANES)

    def row_ops(cols, tks=None):
        hv = [halves(x) for x in cols]
        if tks is not None:
            tk = jnp.stack(tks)

            def held(x):
                x4 = x.reshape(len(tks), 2, 8, LANES)
                return jnp.stack([after(tk, x4[:, 0]), x4[:, 1]], axis=1).reshape(x.shape)

            for k2 in range(2):
                hv[k2][0] = held(hv[k2][0])
                hv[2 + k2][1] = held(hv[2 + k2][1])
        per = [_lhs_ops(hv[k2][0], hv[2 + k2][0], hv[k2][1], hv[2 + k2][1]) + [hv[2 + k2][0], hv[k2][1]]
               for k2 in range(2)]
        return [[per[0][o], per[1][o]] for o in range(9)] + [hv[NC - 1]]

    def stage_p2(r0, r1, nx, mb, blockwise=False):
        h = nx * mb[0] + mb[1]
        h_s[r0:r1, :] = h
        zn = _ln(h, 4.0 * EPS)
        if not blockwise:
            store_bf16(z_s, r0, zn)
            return
        ops = row_ops([zn[:, c * LANES:(c + 1) * LANES] for c in range(NC)])
        for o in range(10):
            for e in range(2):
                lo_s[o, e, r0 // 2:r1 // 2, :] = ops[o][e].astype(BF16)

    def stage_p(t, toks, free):
        lo, hi = A0[t], A0[t + 1]
        stage_p2(lo, hi, stage_p1(lo, hi, pick(toks, (hi - lo) // 8, free), mods_a()), mods_b(), t in STR1)

    def square_ops(src, dst, toks):
        HK = 2 * LANES
        ng = HK // 16
        for n2 in range(2):
            tk = jnp.stack([toks[((n2 * ng + r) * len(toks)) // (2 * ng)] for r in range(ng)])

            def blk(c, k, hold_it):
                x = src[c, k * HK:(k + 1) * HK, :].astype(F32)
                if not hold_it:
                    return x
                x4 = x.reshape(ng, 2, 8, LANES)
                return jnp.stack([after(tk, x4[:, 0]), x4[:, 1]], axis=1).reshape(HK, LANES)

            for o, x in enumerate(_rhs_ops(blk(n2, 0, True), blk(2 + n2, 0, False), blk(n2, 1, False), blk(2 + n2, 1, True))):
                if o not in (1, 4):
                    dst[o, n2] = x.astype(BF16)

    def block_dots(lhs_of, w_ref, s_ref, parts, emit, WL, WH):
        w_u, s_u = w_ref.bitcast(U32), s_ref.bitcast(U32)
        toks = []

        def timed(x, weight):
            toks.extend(x[8 * r:8 * r + 8, 0:LANES] for r in range(x.shape[0] // 8) for _ in range(weight))
            return x

        def main(get):
            m = [None] * 7
            rem = [None, None]
            for o in ('t', 2, 4, 'b', 1, 3, 0, 6, 5):
                if o in ('t', 'b'):
                    e = 0 if o == 't' else 1
                    rhs = jnp.concatenate([w_u[c, 2 * LANES:D // 2, :] for c in range(NC - 1)], axis=1)
                    rem[e] = timed(_dot(get([(9, e)]), _as_bf16(rhs)), WL)
                    continue
                if o in (1, 4):
                    d = (1, 4).index(o)
                    rhs = jnp.concatenate([w_u[2 * d + n2, d * LANES:(d + 1) * LANES, :] for n2 in range(2)], axis=1)
                else:
                    rhs = jnp.concatenate([s_u[o, n2] for n2 in range(2)], axis=1)
                m[o] = timed(_dot(get([(o, 0), (o, 1)]), _as_bf16(rhs)), WH if o in (4, 3, 6, 5) else WL)
            c11, c12, c21, c22 = _combine(m)
            top = jnp.concatenate([c11, c12], axis=1) + rem[0]
            bot = jnp.concatenate([c21, c22], axis=1) + rem[1]
            return [weave(top[:, c * LANES:(c + 1) * LANES], bot[:, c * LANES:(c + 1) * LANES]) for c in range(NC - 1)]

        def last(get):
            w4c = _as_bf16(w_u[NC - 1])
            return weave(timed(_dot(get([(2, 0), (2, 1), (7, 0), (7, 1), (9, 0)]), w4c), WL),
                         timed(_dot(get([(8, 0), (8, 1), (3, 0), (3, 1), (9, 1)]), w4c), WL))

        marks = []
        for j, part in enumerate(parts):
            get = lhs_of(part, toks[marks[-1]:] if marks else None)
            marks.append(len(toks))
            if j % 2:
                tail = last(get)
                cols = main(get) + [tail]
            else:
                cols = main(get) + [last(get)]
            emit(part, cols)
        return toks

    def filler(t):
        if DUM:
            red = jnp.sum(y_s[t, 0:8 * DUM, :], axis=-1, keepdims=True).reshape(DUM, 8, 1)
            zf_s[1, (NC - 1) * (TQ + 8) + 8 * t:(NC - 1) * (TQ + 8) + 8 * t + 8, :] = jnp.broadcast_to(jnp.sum(red, axis=0), (8, LANES))

    def chunks(r0, r1, k, unit=16):
        n = (r1 - r0) // unit
        cuts = [r0 + unit * ((n * j) // k) for j in range(k + 1)]
        return list(zip(cuts[:-1], cuts[1:]))

    def stage_m1(t, k):
        def emit(part, cols):
            out = [_gelu2(x) for x in cols]
            for c in range(NC):
                h1_s[c, part[0] + 8:part[1] + 8, :] = out[c]
            return out

        if t in STR1:
            def lhs_of(part, _):
                return lambda keys: _as_bf16(jnp.concatenate(
                    [lo_u[o, e, part[0] // 4:part[1] // 4, :] for o, e in keys], axis=1))
            return block_dots(lhs_of, w1_v, s1_s, chunks(A0[t], A0[t + 1], k, 32), emit, WL, WH)
        toks = []
        for r0, r1 in chunks(A0[t], A0[t + 1], k):
            pre = _dot(load_bf16(z_u, r0, r1 - r0), packed(w1_v))
            out = emit((r0, r1), [pre[:, c * LANES:(c + 1) * LANES] for c in range(NC)])
            toks += [x for x in tokens_of(jnp.concatenate(out, axis=1)) for _ in range(W1N)]
        return toks

    grp = D // 4
    shifts = (-1, 1, -2, 2)

    def shifted(r0, r1):
        n = r1 - r0
        lane = lax.broadcasted_iota(jnp.int32, (n, LANES), 1)
        cols = []
        for c in range(NC):
            lo, hi = c * LANES, (c + 1) * LANES
            g_lo, g_hi = lo // grp, (hi - 1) // grp
            val = h1_s[c, pl.ds(r0 + 8 + shifts[g_lo], n), :]
            if g_hi != g_lo:
                other = h1_s[c, pl.ds(r0 + 8 + shifts[g_hi], n), :]
                val = jnp.where(lane < (g_hi * grp - lo), val, other)
            cols.append(val)
        return cols

    def stage_m2(t, k, before=None):
        def emit(part, cols):
            x1 = h_s[part[0]:part[1], :] + jnp.concatenate(cols, axis=1)
            h_s[part[0]:part[1], :] = x1
            return x1

        if t in STR2:
            def lhs_of(part, prev):
                prev = before if prev is None else prev
                prev = prev[len(prev) // 8:(len(prev) * 7) // 8]
                ops = row_ops(shifted(*part), pick(prev, (part[1] - part[0]) // 32, 0))
                for o in range(10):
                    for e in range(2):
                        l2_s[o, e, part[0] // 2:part[1] // 2, :] = ops[o][e].astype(BF16)
                return lambda keys: _as_bf16(jnp.concatenate(
                    [l2_u[o, e, part[0] // 4:part[1] // 4, :] for o, e in keys], axis=1))
            return block_dots(lhs_of, w2_v, s2_s, chunks(B0[t], B0[t + 1], k, 32), emit, WM2, WM2)
        toks = []
        for r0, r1 in chunks(B0[t], B0[t + 1], k):
            hs = _dot(jnp.concatenate(shifted(r0, r1), axis=1).astype(BF16), packed(w2_v))
            toks += [x for x in tokens_of(emit((r0, r1), [hs])) for _ in range(W2N)]
        return toks

    TQ = TB // 4
    NT = S // TB
    GB = 2 * NH + 1

    def blk_rows(b):
        return slice(b * (TQ + 8), b * (TQ + 8) + TQ)

    def store_z(r0, slot, toks, free):
        zn = _ln(hold(h_s[pl.ds(r0, TB), :], pick(toks, TB // 8, free)), 4.0 * EPS)
        for rq in range(4):
            for c in range(NC - 1):
                zf_s[slot, blk_rows(NC * rq + c), :] = zn[rq * TQ:(rq + 1) * TQ, c * LANES:(c + 1) * LANES]
        for c in range(NC):
            zr_s[c] = zn[:, c * LANES:(c + 1) * LANES].astype(BF16)

    def outer_lhs(i, blk):
        terms = ((0, 0, 1, 1, 1), (1, 0, 1, 1, 1), (0, 0), (1, 1), (0, 0, 1, 0, 1), (1, 0, -1, 0, 0), (0, 1, -1, 1, 1))[i]
        x = blk(terms[0], terms[1])
        if len(terms) > 2:
            y = blk(terms[3], terms[4])
            x = x + y if terms[2] > 0 else x - y
        return x

    def z_ops(slot_of, toks):
        ng = TQ // 16

        def held(x, k):
            tk = jnp.stack([toks[((k * ng + r) * len(toks)) // (7 * ng)] for r in range(ng)])
            x4 = x.reshape(ng, 2, 8, LANES)
            return jnp.stack([after(tk, x4[:, 0]), x4[:, 1]], axis=1).reshape(TQ, LANES)

        for k, i in enumerate(ZORD):
            slot = slot_of()
            so = [outer_lhs(i, lambda r1, k1: zf_s[slot, blk_rows(NC * (2 * r1 + r2) + 2 * k1 + k2), :])
                  for r2 in range(2) for k2 in range(2)]
            for j, x in enumerate(_lhs_ops(held(so[0], k), so[1], so[2], held(so[3], k))):
                la_s[i, j] = x.astype(BF16)

    NS = NH // 2

    RAW = (1, 4)

    def weight_ops(src, dst, ext, transposed, toks):
        ng = LANES // 16
        lead = 2 if ext is not None else 0
        total = (NS * 7 + lead) * ng

        def tile(c, n):
            return src[c, n * LANES:(n + 1) * LANES, :].astype(F32)

        def held(x, pos, step):
            tk = jnp.stack([toks[((pos + r * step) * len(toks)) // total] for r in range(ng)])
            x4 = x.reshape(ng, 2, 8, LANES)
            return jnp.stack([after(tk, x4[:, 0]), x4[:, 1]], axis=1).reshape(LANES, LANES)

        def outer(c2, n, pos=None):
            b11, b22 = tile(c2, n), tile(2 + c2, NH + n)
            if pos is not None:
                b11, b22 = held(b11, pos, 1), held(b22, pos, 1)
            e1, e2 = tile(c2, NH + n), tile(2 + c2, n)
            return _rhs_ops(b11, e1, e2, b22) if transposed else _rhs_ops(b11, e2, e1, b22)

        for c2 in range(2 if ext is not None else 0):
            for i, x in enumerate(outer(c2, NH - 1, c2 * ng)):
                if i not in RAW:
                    ext[i, c2] = x.astype(BF16)
        for st in range(NS):
            t00, t11 = outer(0, 2 * st), outer(1, 2 * st + 1)
            t01, t10 = outer(0, 2 * st + 1), outer(1, 2 * st)
            for k, i in enumerate((1, 5, 2, 4, 0, 3, 6)):
                pos = (lead + st * 7) * ng + k
                a, d = held(t00[i], pos, 7), held(t11[i], pos, 7)
                ops = _rhs_ops(a, t01[i], t10[i], d) if transposed else _rhs_ops(a, t10[i], t01[i], d)
                for j, x in enumerate(ops):
                    if i not in RAW or j not in RAW:
                        dst[i, j, st * LANES:(st + 1) * LANES, :] = x.astype(BF16)

    with jax.named_scope("r0a"):
        wait_all(first[:1])
        conv_round(0, 'k', False, False)
    with jax.named_scope("r0_wait"):
        wait_all(first[1:])
    with jax.named_scope("r0b"):
        start_all(conv_copies(2) + conv_copies(3) + conv_copies(4))
        conv_round(0, 'u', False, False)
    with jax.named_scope("r1a"):
        wait_all(second[:1])
        conv_round(1, 'k', True, False)
    with jax.named_scope("r1_wait"):
        wait_all(second[1:])
    with jax.named_scope("r1b"):
        start_all(wm_copies[0] + q_copies[0] + wm_copies[1] + w_copies[0])
        conv_round(1, 'u', False, False)

    def full_round(c, carry):
        wait_all(conv_copies(c))
        conv_round(c, 'ku', True, True)
        return carry

    with jax.named_scope("r234"):
        lax.fori_loop(2, NC, full_round, 0)
    with jax.named_scope("r5"):
        start_all(q_copies[1] + w_copies[1] + sum(q_copies[2:], []) + w_copies[2] + w_copies[3] + wm_copies[2], 1)
        conv_round(NC, '', True, True)
    with jax.named_scope("r6_wait"):
        wait_all(wm_copies[0] + q_copies[0])
    with jax.named_scope("r6"):
        for j in range(3):
            mod_chunk(j)
        conv_round(NC + 1, '', False, True)
        nx0 = stage_p1(0, A0[1], [None], mods_a())
    with jax.named_scope("p2_wait"):
        wait_all(wm_copies[1])
    with jax.named_scope("p2"):
        mod_chunk(4)
        mod_chunk(3)
        stage_p2(0, A0[1], nx0, mods_b())
    with jax.named_scope("w1_wait"):
        wait_all(w_copies[0])
    with jax.named_scope("m1_0"):
        toks = stage_m1(0, 4)
        if STR1:
            square_ops(w1_v, s1_s, toks[:len(toks) - 20 * W1N])
    with jax.named_scope("w2_wait"):
        wait_all(q_copies[1] + w_copies[1])
    with jax.named_scope("m2_0"):
        toks = stage_m2(0, 4)
        stage_p(1, toks[:len(toks) - TRIM * W2N], FREE * W2N)
        if STR2 and min(STR2) == 1:
            square_ops(w2_v, s2_s, toks[len(toks) // 2:len(toks) - 10 * W2N])
        filler(0)
    for t in range(1, NA):
        with jax.named_scope("a%d" % t):
            if t + 1 < NA:
                wait_all(q_copies[t + 1])
            else:
                wait_all(w_copies[2] + w_copies[3] + wm_copies[2])
            t1 = stage_m1(t, SPLIT)
            t2 = stage_m2(t, SPLIT, t1[len(t1) - len(t1) // SPLIT:])

            def weighted(trim):
                return t1 + t2[:len(t2) - trim * W2N]

            if t + 1 < NA:
                stage_p(t + 1, weighted(TRIM), FREE * W2N)
            if STR2 and t == W2P:
                square_ops(w2_v, s2_s, weighted(10))
            if t == NA - 1 - LAT:
                toks = weighted(TRIM // 2)
                store_z(0, 0, toks if LAT and not ZE else toks[:len(toks) // 2], FREE * W2N)
                if ZE:
                    toks = weighted(10)
                    z_ops(lambda: 0, toks[(len(toks) * 5) // 8:])
            if t == NA - 1:
                mod_chunk(NC)
                toks = weighted(20)
                toks = toks[:1] * PRE + toks
                cut = (len(toks) * 21) // 44
                weight_ops(w3_v, s3_s, None, True, toks[:cut])
                weight_ops(w4_v, s4_s, e4_s, False, toks[cut:])
                if not ZE:
                    z_ops(lambda: 0, toks if LAT else toks[(len(toks) * 5) // 8:])
            if t + 1 < NA or not LAT:
                filler(t)

    gb = 0.5 * mod_s[NC, 0:1, :]
    w3_u, w4_u, s3_u, s4_u, e4_u = (r.bitcast(U32) for r in (w3_v, w4_v, s3_s, s4_s, e4_s))
    HL = LANES // 2
    la_u = la_s.bitcast(U32)
    zr_u = zr_s.bitcast(U32)

    def out_copy(r0, n, c):
        rows = pl.ds(r0, n)
        return pltpu.make_async_copy(o_v.at[c, rows, :], o_hbm.at[rows, pl.ds(c * LANES, LANES)], sem_o.at[0])

    def one_level(w_u, e_u, i, c2):
        if i not in RAW:
            return e_u[i, c2]
        d = RAW.index(i)
        n = d * NH + NH - 1
        return w_u[2 * d + c2, n * HL:(n + 1) * HL, :]

    def two_level(w_u, s_u, i, j, st):
        if i not in RAW or j not in RAW:
            return s_u[i, j, st * HL:(st + 1) * HL, :]
        d, e = RAW.index(i), RAW.index(j)
        n = d * NH + 2 * st + e
        return w_u[2 * d + e, n * HL:(n + 1) * HL, :]

    def loop_b(t, carry):
        r0 = pl.multiple_of(t * TB, TB)
        ws = t & 1

        count = [0]

        def fresh():
            count[0] += 1
            return lax.rem(t + 2 * count[0], 2)

        zr = [_as_bf16(zr_u[NC - 1, rq * (TQ // 2):(rq + 1) * (TQ // 2), :]) for rq in range(4)]
        ltoks, ftoks = [], []

        def light(x):
            ltoks.extend(x[8 * r:8 * r + 8, 0:LANES] for r in range(x.shape[0] // 8))

        def rem3(rq, n):
            return _dot_nt(zr[rq], _as_bf16(w3_u[NC - 1, n * HL:(n + 1) * HL, :]))

        def put_g(rq, n, pre):
            g_s[rq // 2][ws, blk_rows(GB * (rq % 2) + n), :] = _gelu2(pre)

        rem = {}
        for st in range(NS - ALN):
            rem[3, NH + 2 * st + 1] = rem3(3, NH + 2 * st + 1)
        n0 = NH - 1
        w_mid = _as_bf16(jnp.concatenate([w3_u[c, n0 * HL:(n0 + 1) * HL, :] for c in range(NC)], axis=1))
        lo = (2 * NH - 1) * HL
        w_end = _as_bf16(jnp.concatenate([w3_u[c, lo:FF // 2, :] for c in range(NC)], axis=1))
        for rq in range(4):
            zq = _as_bf16(jnp.concatenate([zr_u[c, rq * (TQ // 2):(rq + 1) * (TQ // 2), :] for c in range(NC)], axis=1))
            mid = _dot_nt(zq, w_mid)
            ftoks.extend(mid[8 * r:8 * r + 8, :] for r in range(TQ // 8))
            put_g(rq, n0, mid)
            gt = _gelu2(_dot_nt(w_end, zq))
            g_s[rq // 2][ws, blk_rows(GB * (rq % 2) + 2 * NH - 1), :] = jnp.concatenate([gt, jnp.zeros((FP - FF, TQ), F32)], axis=0).T
        for st in range(NS):
            todo = [(2 * r1 + r2, h * NH + 2 * st + p) for r1, h in ((0, 1), (1, 0), (0, 0), (1, 1))
                    for r2 in range(2) for p in range(2)]
            todo = [x for x in todo if x not in rem]
            for key in todo[:8]:
                rem[key] = rem3(*key)
            if st >= LSETS:
                light(rem[todo[1]])
                light(rem[todo[5]])
            todo = todo[8:]
            pin = [None] * 7
            for i in _ORDER:
                m = [None] * 7
                for j in _ORDER:
                    m[j] = _dot_nt(_as_bf16(la_u[i, j]), _as_bf16(two_level(w3_u, s3_u, i, j, st)))
                if st >= LSETS and i in (2, 1, 0):
                    light(m[_ORDER[1]])
                    light(m[_ORDER[5]])
                key = todo.pop(0)
                rem[key] = rem3(*key)
                pin[i] = _combine(m)
            for key in todo:
                rem[key] = rem3(*key)
            for inner in range(4):
                for blk, cval in enumerate(_combine([pin[i][inner] for i in range(7)])):
                    rq, n = 2 * (blk // 2) + inner // 2, (blk % 2) * NH + 2 * st + inner % 2
                    put_g(rq, n, cval + rem[rq, n])

        toks = []

        def timed(x):
            toks.extend(x[8 * r:8 * r + 8, 0:LANES] for r in range(x.shape[0] // 8))
            return x

        def finish(rq, c, h2):
            rows = pl.ds(pl.multiple_of(r0 + rq * TQ, TQ), TQ)
            cols = slice(c * LANES, (c + 1) * LANES)
            o_v[c, rows, :] = (x_s[rows, cols] + gb[:, cols] * (h_s[rows, cols] + h2)).astype(BF16)

        kord = [NH - 1, 2 * NH - 1] + [h * NH + n for st in range(NS) for h in (1, 0) for n in (2 * st + 1, 2 * st)]
        w4r = _as_bf16(jnp.concatenate([w4_u[NC - 1, n * HL:(n + 1) * HL, :] for n in kord], axis=0))

        def rem4(rq, slot):
            lhs = jnp.concatenate([g_s[rq // 2][slot, blk_rows(GB * (rq % 2) + n), :] for n in kord], axis=1).astype(BF16)
            r = timed(_dot(lhs, w4r))
            finish(rq, NC - 1, r)

        rem4(0, fresh())
        rem4(1, fresh())
        pin = [None] * 7
        done = {_ORDER[1]: 1, _ORDER[3]: 2, _ORDER[5]: 0, _ORDER[6]: 3}
        for i in _ORDER:
            slot = fresh()
            rhs = _as_bf16(jnp.concatenate([one_level(w4_u, e4_u, i, c2) for c2 in range(2)], axis=1))
            ex = [_dot(outer_lhs(i, lambda r1, h: g_s[r1][slot, blk_rows(GB * r2 + h * NH + NH - 1), :]).astype(BF16), rhs)
                  for r2 in range(2)]
            m = [None] * 7
            for j in _ORDER:
                slot = fresh()
                lhs = jnp.concatenate(
                    [outer_lhs(j, lambda r2, p: outer_lhs(
                        i, lambda r1, h: g_s[r1][slot, blk_rows(GB * r2 + h * NH + 2 * st + p), :]))
                     for st in range(NS)], axis=1).astype(BF16)
                m[j] = timed(_dot(lhs, _as_bf16(jnp.concatenate([two_level(w4_u, s4_u, i, j, st) for st in range(NS)], axis=0))))
            pin[i] = [x + ex[inner // 2][:, (inner % 2) * LANES:(inner % 2 + 1) * LANES]
                      for inner, x in enumerate(_combine(m))]
            if i in done:
                blk = done[i]
                for inner in (1, 2, 0, 3):
                    p = [pin[k][inner] if pin[k] is not None else None for k in range(7)]
                    cval = (lambda: (p[3] - p[4]) + p[0] + p[6], lambda: p[2] + p[4], lambda: p[1] + p[3],
                            lambda: (p[2] - p[1]) + p[0] + p[5])[blk]()
                    finish(2 * (blk // 2) + inner // 2, 2 * (blk % 2) + inner % 2, cval)
                rb = pl.multiple_of(r0 + (blk // 2) * 2 * TQ, 2 * TQ)
                for e in range(2):
                    out_copy(rb, 2 * TQ, 2 * (blk % 2) + e).start()
                if blk == 0:
                    out_copy(r0, 3 * TQ, NC - 1).start()
            if i == _ORDER[REM2]:
                rem4(2, fresh())
        rem4(3, fresh())
        out_copy(pl.multiple_of(r0 + 3 * TQ, TQ), TQ, NC - 1).start()

        nxt = jnp.minimum(t + 1, NT - 1)
        store_z(pl.multiple_of(nxt * TB, TB), ws, ftoks[len(ftoks) - FT:] + ltoks[:LN1:LSTEP] + toks[:LB1], 0)
        z_ops(fresh, toks[ZB0:ZB1])
        if DUMB:
            filler(4)
        return carry

    with jax.named_scope("ph2b"):
        lax.fori_loop(0, NT, loop_b, 0)
    with jax.named_scope("tail"):
        pltpu.make_async_copy(o_v, o_v, sem_o.at[0]).wait()


@jax.jit
def pallas_adaLN_cond__ssm_conv_h3__mixer_s_mlp__prompt_kernel(
    A_q: jax.Array,
    A_k: jax.Array,
    A_v: jax.Array,
    A_shift_k: jax.Array,
    A_ssm_k: jax.Array,
    A_ssm_D: jax.Array,
    B_x: jax.Array,
    B_w1: jax.Array,
    B_w2: jax.Array,
    B_w3: jax.Array,
    B_w4: jax.Array,
    c: jax.Array,
    w_mod: jax.Array,
):
    B, S, D = A_q.shape
    assert B == 1
    FF = B_w3.shape[1]
    NC = D // LANES
    NG = BLK // 8
    NBL = S // (PH * BLK)
    FP = -(-FF // (2 * LANES)) * 2 * LANES
    TILES = (384, 384, 576, 704)
    assert sum(TILES) == S
    TB = 512

    args = (A_q.reshape(S, D), A_k.reshape(S, D), A_v.reshape(S, D), A_shift_k.T, A_ssm_k,
            A_ssm_D, B_w1, B_w2, B_w3.T, B_w4, c, w_mod)
    scratch = [
        pltpu.VMEM((S, D), BF16),
        pltpu.VMEM((NC, S + KP, LANES), BF16),
        pltpu.VMEM((NC, S + VP, LANES), BF16),
        pltpu.VMEM((4, D), BF16),
        pltpu.VMEM((NC, LANES, S), BF16),
        pltpu.VMEM((D,), BF16),
        pltpu.VMEM((NC, D, LANES), BF16),
        pltpu.VMEM((NC, D, LANES), BF16),
        pltpu.VMEM((NC, FF, LANES), BF16),
        pltpu.VMEM((NC, FP, LANES), BF16),
        pltpu.VMEM((1, D), BF16),
        pltpu.VMEM((D, 6 * D), BF16),
        pltpu.VMEM((PH, 2 * BLK, BLK), BF16),
        pltpu.VMEM((PH, 2, BLK, BLK), BF16),
        pltpu.VMEM((NC, S, LANES), BF16),
        pltpu.VMEM((NC, NG, NBL, PH, 2, 8, LANES), F32),
        pltpu.VMEM((NC, NG, NBL, PH, 2, 8, LANES), F32),
        pltpu.VMEM((NC, NBL, PH, 2 * BLK, LANES), BF16),
        pltpu.VMEM((NBL, PH, BLK, LANES), BF16),
        pltpu.VMEM((NC, S + YP, LANES), F32),
        pltpu.VMEM((6, 8, D), F32),
        pltpu.VMEM((NC, 8, LANES), F32),
        pltpu.VMEM((NC, S + 16, LANES), F32),
        pltpu.VMEM((S, D), F32),
        pltpu.VMEM((S, D), F32),
        pltpu.VMEM((NC, S, LANES), BF16),
        pltpu.VMEM((7, 7, FP // 512 * LANES, LANES), BF16),
        pltpu.VMEM((7, 7, FP // 512 * LANES, LANES), BF16),
        pltpu.VMEM((7, 2, LANES, LANES), BF16),
        [pltpu.VMEM((2, GR, LANES), F32)] * 2,
        pltpu.VMEM((2, ZR, LANES), F32),
        pltpu.VMEM((NC, TB, LANES), BF16),
        pltpu.VMEM((7, 7, TB // 4, LANES), BF16),
        pltpu.VMEM((10, 2, S // 2, LANES), BF16),
        pltpu.VMEM((10, 2, S // 2, LANES), BF16),
        pltpu.VMEM((7, 2, 2 * LANES, LANES), BF16),
        pltpu.VMEM((7, 2, 2 * LANES, LANES), BF16),
        pltpu.SemaphoreType.DMA((16 + len(TILES),)),
        pltpu.SemaphoreType.DMA((1,)),
    ]
    out = pl.pallas_call(
        functools.partial(_kernel, S=S, D=D, FF=FF, TILES=TILES, TB=TB),
        in_specs=[pl.BlockSpec(memory_space=pl.ANY)] * len(args),
        out_specs=pl.BlockSpec(memory_space=pl.ANY),
        out_shape=jax.ShapeDtypeStruct((S, D), BF16),
        scratch_shapes=scratch,
        compiler_params=pltpu.CompilerParams(
            vmem_limit_bytes=126 * 1024 * 1024,
            disable_bounds_checks=True,
            disable_semaphore_checks=True,
        ),
    )(*args)
    return out.reshape(B, S, D)
```

```python
import functools
import math

import jax
import jax.numpy as jnp
from jax import lax
import jax.experimental.pallas as pl
import jax.experimental.pallas.tpu as pltpu

F32 = jnp.float32
BF16 = jnp.bfloat16
U32 = jnp.uint32

LANES = 128
BLK = 128
PH = 4
EPS = 1e-05
TRIM = 60
SPLIT = 2
FREE = 30
DUM = 96
LN1 = 999
KP = 16
VP = 0
YP = 0
GR = 4080
ZR = 2720
FT = 0
DUMB = 1
STR1 = (3, )
STR2 = (2, 3, )
WL = 3
WH = 2
ZE = 1
PRE = 0
WM2 = 2
W2P = 1
UL = 2
ALN = 0
W1N = 2
W2N = 3
LAT = 1
LSETS = 1
LSTEP = 4
LB1 = 0
ZB0 = 0
ZB1 = 140
REM2 = 2
ZORD = (2, 3, 0, 1, 4, 5, 6)


def _as_bf16(x):
    return pltpu.bitcast(x, BF16)


def _lo(x):
    return pltpu.bitcast(x << 16, F32)


def _hi(x):
    return pltpu.bitcast(x & jnp.uint32(0xFFFF0000), F32)


def _dft4(re, im, sign):
    ar, ai = re[0] + re[2], im[0] + im[2]
    br, bi = re[0] - re[2], im[0] - im[2]
    cr, ci = re[1] + re[3], im[1] + im[3]
    dr, di = re[1] - re[3], im[1] - im[3]
    o0 = (ar + cr, ai + ci)
    o2 = (ar - cr, ai - ci)
    m = (br + di, bi - dr)
    p = (br - di, bi + dr)
    o1, o3 = (m, p) if sign < 0 else (p, m)
    return [o0[0], o1[0], o2[0], o3[0]], [o0[1], o1[1], o2[1], o3[1]]


def _ln(x, eps=EPS, unit=True):
    n = x.shape[-1]
    s1 = jnp.sum(x, axis=-1, keepdims=True)
    m = s1 * (1.0 / n)
    v = jnp.maximum(jnp.sum(x * x, axis=-1, keepdims=True) + (n * eps - s1 * m), n * eps)
    e = jnp.log(v) * (-0.5 / math.log(2.0))
    return (x - m) * jnp.exp2(e + 0.5 * math.log2(n) if unit else e)


def _gelu2(x):
    c0 = math.sqrt(2.0 / math.pi)
    return x + x * jnp.tanh(x * (c0 + (c0 * 0.044715) * (x * x)))


def _dot(a, b):
    return jnp.dot(a, b, preferred_element_type=F32)


def _dot_nt(a, b):
    return lax.dot_general(a, b, (((1,), (1,)), ((), ())), preferred_element_type=F32)


def _lhs_ops(a11, a12, a21, a22):
    return [a11 + a22, a21 + a22, a11, a22, a11 + a12, a21 - a11, a12 - a22]


def _rhs_ops(b11, b12, b21, b22):
    return [b11 + b22, b11, b12 - b22, b21 - b11, b22, b11 + b12, b21 + b22]


def _combine(m):
    return (m[3] - m[4]) + m[0] + m[6], m[2] + m[4], m[1] + m[3], (m[2] - m[1]) + m[0] + m[5]


_ORDER = (2, 4, 1, 3, 0, 6, 5)


def _kernel(q_hbm, k_hbm, v_hbm, sh_hbm, sk_hbm, sd_hbm, w1_hbm, w2_hbm, w3_hbm, w4_hbm, c_hbm, wm_hbm,
            o_hbm,
            q_v, k_v, v_v, sh_v, sk_v, sd_v, w1_v, w2_v, w3_v, w4_v, c_v, wm_v,
            fw_s, iv_s, o_v, u_s, kk_s, vv_s, wu_s, y_s, mod_s, par_s, h1_s, x_s, h_s, z_s, s3_s, s4_s, e4_s, g_s, zf_s, zr_s, la_s, lo_s, l2_s, s1_s, s2_s, sl_s,
            sem, sem_o,
            *, S, D, FF, TILES, TB):
    NC = D // LANES
    NG = BLK // 8
    LB = PH * BLK
    NBL = S // LB
    R = BLK // PH
    HALO = 32
    FP = w4_v.shape[1]
    FH = FP // 2
    NH = FH // LANES

    small = [
        pltpu.make_async_copy(sh_hbm, sh_v, sem.at[0]),
        pltpu.make_async_copy(sd_hbm, sd_v, sem.at[0]),
        pltpu.make_async_copy(c_hbm, c_v, sem.at[0]),
    ]

    def conv_copies(c):
        col = pl.ds(c * LANES if isinstance(c, int) else pl.multiple_of(c * LANES, LANES), LANES)
        return [
            pltpu.make_async_copy(sk_hbm.at[col, :], sk_v.at[c], sem.at[9 + c if isinstance(c, int) and c < 2 else 1 + c]),
            pltpu.make_async_copy(k_hbm.at[:, col], k_v.at[c, pl.ds(16, S), :], sem.at[1 + c]),
            pltpu.make_async_copy(v_hbm.at[:, col], v_v.at[c, pl.ds(0, S), :], sem.at[1 + c]),
        ]

    def col_copies(src, dst, c0, s):
        rows = pl.ds(0, src.shape[0])
        return [pltpu.make_async_copy(src.at[:, pl.ds((c0 + c) * LANES, LANES)], dst.at[c0 + c, rows, :], sem.at[s])
                for c in range(NC)]

    WM = (0, 3 * D, 5 * D, 6 * D)
    wm_copies = [[pltpu.make_async_copy(wm_hbm.at[:, pl.ds(WM[j], WM[j + 1] - WM[j])],
                                        wm_v.at[:, pl.ds(WM[j], WM[j + 1] - WM[j])], sem.at[6 + j])]
                 for j in range(3)]
    w_copies = [col_copies(src, dst, 0, 12 + j)
                for j, (src, dst) in enumerate(((w1_hbm, w1_v), (w2_hbm, w2_v), (w3_hbm, w3_v), (w4_hbm, w4_v)))]

    B0 = [0]
    for n in TILES:
        B0.append(B0[-1] + n)
    NA = len(TILES)
    A0 = [0] + [r + HALO for r in B0[1:-1]] + [S]
    q_copies = [
        [pltpu.make_async_copy(q_hbm.at[pl.ds(A0[t], A0[t + 1] - A0[t])], q_v.at[pl.ds(A0[t], A0[t + 1] - A0[t])],
                               sem.at[16 + t])]
        for t in range(NA)
    ]

    def start_all(cps, priority=0):
        for cp in cps:
            cp.start(priority=priority)

    def wait_all(cps):
        for cp in cps:
            cp.wait()

    def packed(ref, c0=0):
        ru = ref.bitcast(U32)
        return _as_bf16(jnp.concatenate([ru[c0 + c] for c in range(NC)], axis=1))

    first, second = conv_copies(0), conv_copies(1)
    start_all(first[:1] + small + first[1:] + second)

    for c in range(NC):
        k_v[c, 0:16, :] = jnp.zeros((16, LANES), BF16)
        h1_s[c, 0:8, :] = jnp.zeros((8, LANES), F32)
        h1_s[c, S + 8:S + 16, :] = jnp.zeros((8, LANES), F32)
        w4_v[c, FF:FP, :] = jnp.zeros((FP - FF, LANES), BF16)

    prow = lax.broadcasted_iota(jnp.int32, (BLK, BLK), 0)
    pcol = lax.broadcasted_iota(jnp.int32, (BLK, BLK), 1)
    ang = (((4 * prow + 1) * pcol) & (4 * BLK - 1)).astype(F32) * (2.0 * math.pi / (4 * BLK))
    tw = (4 * prow + 1).astype(F32) * (2.0 * math.pi / (4 * LB))
    mr, mi = jnp.cos(ang), -jnp.sin(ang)
    zr_, zi_ = jnp.cos(tw), -jnp.sin(tw)
    eye = jnp.where(prow == pcol, 1.0 / LB, 0.0).astype(BF16)
    for i in range(PH):
        both = jnp.stack([mr.reshape(NG, 8, BLK), mi.reshape(NG, 8, BLK)], axis=1).reshape(2 * BLK, BLK)
        fw_s[i] = both.astype(BF16)
        for h in range(2):
            iv_s[i, h] = _dot_nt(eye, both[h * BLK:(h + 1) * BLK, :].astype(BF16)).astype(BF16)
        if i + 1 < PH:
            mr, mi = mr * zr_ - mi * zi_, mr * zi_ + mi * zr_
    perm = jnp.where(pcol == (prow % R) * PH + prow // R, 1.0, 0.0).astype(BF16)
    fw_u = fw_s.bitcast(U32)
    iv_u = iv_s.bitcast(U32)

    wait_all(small)
    shf = sh_v[...].astype(F32)
    sdf = sd_v[...].astype(F32).reshape(1, D)
    for c in range(NC):
        par_s[c, 0:4, :] = shf[:, c * LANES:(c + 1) * LANES]
        par_s[c, 4:5, :] = sdf[:, c * LANES:(c + 1) * LANES]
    cf = c_v[...].astype(F32)
    sc = (cf * jax.nn.sigmoid(cf)).astype(BF16)
    sc16 = jnp.broadcast_to(sc, (16, D))

    def mod_chunk(j):
        mod_s[j] = _dot(sc16, wm_v[:, j * D:(j + 1) * D])[0:8, :]

    k_u = k_v.bitcast(U32)
    v_u = v_v.bitcast(U32)
    wu_u = wu_s.bitcast(U32)
    z_u = z_s.bitcast(U32)
    vv_u = vv_s.bitcast(U32)
    lo_u = lo_s.bitcast(U32)
    l2_u = l2_s.bitcast(U32)

    never = zr_[0:8, :] > 2.0

    def after(token, x):
        if token.dtype != x.dtype:
            token = pltpu.bitcast(token, x.dtype)
        return jnp.where(jnp.broadcast_to(never, x.shape), token, x)

    def split(t):
        t4 = t.reshape(NG, 2, 8, LANES)
        return t4[:, 0], t4[:, 1]

    def perm_k(c, b, toks):
        kt = [_dot_nt(perm, sk_v[c, :, b * LB + t * BLK:b * LB + (t + 1) * BLK]) for t in range(PH)]
        for r in range(BLK // 16):
            toks.append(kt[0][16 * r:16 * r + 8, :])
        return [jnp.concatenate([kt[t][i * R:(i + 1) * R, :] for t in range(PH)], axis=0).astype(BF16)
                for i in range(PH)]

    def spectrum(wts, dst, c, b, toks, dc=None, pins=None):
        tr, ti = [], []
        for i in range(PH):
            lhs = fw_u[i]
            if pins is not None and i < len(pins):
                lhs = after(pins[i], lhs.reshape(NG, 8, LANES)).reshape(BLK, LANES)
            r_, i_ = split(_dot(_as_bf16(lhs), wts[i]))
            tr.append(r_)
            ti.append(i_)
        for g in range(NG):
            toks.append(ti[PH - 1][g])
        if dc is not None:
            tr[0] = tr[0] + dc
        sr, si = _dft4(tr, ti, -1)
        for qq in range(PH):
            dst[c, :, b, qq, 0] = sr[qq]
            dst[c, :, b, qq, 1] = si[qq]

    def gated(c, b):
        w = [par_s[c, t:t + 1, :] for t in range(4)]
        kc = {}
        for o in range(-2, 2):
            words = k_u[c, pl.ds(8 + b * (LB // 2) + o, BLK, stride=2), :]
            if o > -2:
                kc[2 * o] = _lo(words)
            kc[2 * o + 1] = _hi(words)
        vc = {}
        for o in range(2):
            words = v_u[c, pl.ds(b * (LB // 2) + o, BLK, stride=2), :]
            vc[2 * o] = _lo(words)
            vc[2 * o + 1] = _hi(words)
        for i in range(PH):
            ks = kc[i] * w[0]
            for t in range(1, 4):
                ks = ks + kc[i - t] * w[t]
            wu_s[b, i] = (ks * vc[i]).astype(BF16)
        return [wu_u[b, i] for i in range(PH)]

    def kv_pins(kvb):
        return [jnp.stack([kvb[2 * m + (r % 2)][8 * (r // 2):8 * (r // 2) + 8, :] for r in range(NG)])
                for m in range(2)]

    def mac(c, us, ks, toks):
        zp = None
        for o in range(NBL):
            zr, zi = [], []
            for qq in range(PH):
                accr = acci = None
                for b in range(o + 1):
                    a_, b_ = us[0, :, b, qq, 0], us[0, :, b, qq, 1]
                    c_, d_ = ks[0, :, o - b, qq, 0], ks[0, :, o - b, qq, 1]
                    if qq == 0 and b == o:
                        a_ = after(toks[o], a_)
                    tr_ = a_ * c_ - b_ * d_
                    ti_ = a_ * d_ + b_ * c_
                    accr = tr_ if accr is None else accr + tr_
                    acci = ti_ if acci is None else acci + ti_
                zr.append(accr)
                zi.append(acci)
            if zp is None:
                yr, yi = zr, zi
            else:
                yr = [zr[qq] - zp[1][qq] for qq in range(PH)]
                yi = [zi[qq] + zp[0][qq] for qq in range(PH)]
            zp = (zr, zi)
            vr, vi = _dft4(yr, yi, +1)
            for i in range(PH):
                vv_s[c, o, i] = jnp.stack([vr[i], vi[i]], axis=1).reshape(2 * BLK, LANES).astype(BF16)

    def inverse(c, toks, pins=None):
        HB = BLK // 2
        for o in range(NBL):
            for i in range(PH):
                yv = None
                for h in range(2):
                    lhs = iv_u[i, h]
                    if pins is not None and h == 0:
                        pin = pins[o][i % 2][8 * (i // 2):8 * (i // 2) + 8]
                        lhs = after(pin, lhs.reshape(8, 8, LANES)).reshape(HB, LANES)
                    t = _dot(_as_bf16(lhs), _as_bf16(vv_u[c, o, i, h * HB:(h + 1) * HB, :]))
                    yv = t if yv is None else yv + t
                if i % 2 == 0:
                    for r in range(BLK // 16):
                        toks.append(yv[16 * r:16 * r + 8, :])
                y_s[c, pl.ds(o * LB + i, BLK, stride=PH), :] = yv

    def mac_tokens(toks):
        n = len(toks) - 3
        cum = (44, 128, 244, 392)
        return [jnp.stack([toks[max(0, ((g * 392 + cum[o]) * n) // (392 * NG) - 1)] for g in range(NG)])
                for o in range(NBL)]

    def conv_round(c, fwd, mul, inv):
        toks = []
        kv = pins = None
        cur = 1 if mul else 0
        if fwd or mul:
            win = pl.ds(c - cur, 2 if fwd and mul else 1)
            us, ks = u_s.at[win], kk_s.at[win]
        if 'u' in fwd:
            kv = [gated(c, b) for b in range(NBL)]
            pins = [kv_pins(kv[b]) for b in range(NBL)]
        if inv:
            inverse(c - 2, toks, pins)
            if fwd:
                toks = []
        if 'k' in fwd:
            wts = [perm_k(c, b, toks) for b in range(NBL)]
        for b in range(NBL):
            if 'k' in fwd:
                spectrum(wts[b], ks, cur, b, toks, par_s[c, 4:5, :] if b == 0 else None)
            if 'u' in fwd:
                pin = pins[b + UL] if not inv and b + UL < NBL else None
                spectrum([_as_bf16(x) for x in kv[b]], us, cur, b, toks, None, pin)
        if mul:
            mac(c - 1, us, ks, mac_tokens(toks))

    def tokens_of(x):
        return [x[8 * r:8 * r + 8, c * LANES:(c + 1) * LANES] for c in range(NC) for r in range(x.shape[0] // 8)]

    def store_bf16(ref, r0, x):
        for c in range(NC):
            ref[c, r0:r0 + x.shape[0], :] = x[:, c * LANES:(c + 1) * LANES].astype(BF16)

    def load_bf16(ref_u, r0, n):
        return _as_bf16(jnp.concatenate([ref_u[c, pl.ds(r0 // 2, n // 2), :] for c in range(NC)], axis=1))

    def pick(toks, n, free):
        if toks is None:
            return [None] * n
        idx = [(r * (len(toks) + free)) // n - free for r in range(n)]
        return [toks[i] if i >= 0 else None for i in idx]

    def hold(x, tks):
        f = len([k for k in tks if k is None])
        n = len(tks)
        if f == n:
            return x
        first = after(jnp.stack(tks[f:]), x[8 * f:, 0:LANES].reshape(n - f, 8, LANES)).reshape(8 * (n - f), LANES)
        if f:
            first = jnp.concatenate([x[:8 * f, 0:LANES], first], axis=0)
        return jnp.concatenate([first, x[:, LANES:]], axis=1)

    def mods_a():
        ga = mod_s[2, 0:1, :]
        return ga * (1.0 + mod_s[1, 0:1, :]) * math.sqrt(D), ga * mod_s[0, 0:1, :]

    def mods_b():
        return (1.0 + mod_s[4, 0:1, :]) * (2.0 * math.sqrt(D)), 2.0 * mod_s[3, 0:1, :]

    def stage_p1(r0, r1, tks, ma):
        q = hold(q_v[r0:r1, :].astype(F32), tks)
        y = jnp.concatenate([y_s[c, r0:r1, :] for c in range(NC)], axis=1)
        x = q + (_ln(q, unit=False) * ma[0] + ma[1]) * y
        x_s[r0:r1, :] = x
        return _ln(x, unit=False)

    def halves(x):
        x4 = x.reshape(x.shape[0] // 32, 2, 16, LANES)
        return [x4[:, e].reshape(x.shape[0] // 2, LANES) for e in range(2)]

    def weave(top, bot):
        n = top.shape[0] // 16
        return jnp.stack([top.reshape(n, 16, LANES), bot.reshape(n, 16, LANES)], axis=1).reshape(32 * n, LANES)

    def row_ops(cols, tks=None):
        hv = [halves(x) for x in cols]
        if tks is not None:
            tk = jnp.stack(tks)

            def held(x):
                x4 = x.reshape(len(tks), 2, 8, LANES)
                return jnp.stack([after(tk, x4[:, 0]), x4[:, 1]], axis=1).reshape(x.shape)

            for k2 in range(2):
                hv[k2][0] = held(hv[k2][0])
                hv[2 + k2][1] = held(hv[2 + k2][1])
        per = [_lhs_ops(hv[k2][0], hv[2 + k2][0], hv[k2][1], hv[2 + k2][1]) + [hv[2 + k2][0], hv[k2][1]]
               for k2 in range(2)]
        return [[per[0][o], per[1][o]] for o in range(9)] + [hv[NC - 1]]

    def stage_p2(r0, r1, nx, mb, blockwise=False):
        h = nx * mb[0] + mb[1]
        h_s[r0:r1, :] = h
        zn = _ln(h, 4.0 * EPS)
        if not blockwise:
            store_bf16(z_s, r0, zn)
            return
        ops = row_ops([zn[:, c * LANES:(c + 1) * LANES] for c in range(NC)])
        for o in range(10):
            for e in range(2):
                lo_s[o, e, r0 // 2:r1 // 2, :] = ops[o][e].astype(BF16)

    def stage_p(t, toks, free):
        lo, hi = A0[t], A0[t + 1]
        stage_p2(lo, hi, stage_p1(lo, hi, pick(toks, (hi - lo) // 8, free), mods_a()), mods_b(), t in STR1)

    def square_ops(src, dst, toks):
        HK = 2 * LANES
        ng = HK // 16
        for n2 in range(2):
            tk = jnp.stack([toks[((n2 * ng + r) * len(toks)) // (2 * ng)] for r in range(ng)])

            def blk(c, k, hold_it):
                x = src[c, k * HK:(k + 1) * HK, :].astype(F32)
                if not hold_it:
                    return x
                x4 = x.reshape(ng, 2, 8, LANES)
                return jnp.stack([after(tk, x4[:, 0]), x4[:, 1]], axis=1).reshape(HK, LANES)

            for o, x in enumerate(_rhs_ops(blk(n2, 0, True), blk(2 + n2, 0, False), blk(n2, 1, False), blk(2 + n2, 1, True))):
                if o not in (1, 4):
                    dst[o, n2] = x.astype(BF16)

    def block_dots(lhs_of, w_ref, s_ref, parts, emit, WL, WH):
        w_u, s_u = w_ref.bitcast(U32), s_ref.bitcast(U32)
        toks = []

        def timed(x, weight):
            toks.extend(x[8 * r:8 * r + 8, 0:LANES] for r in range(x.shape[0] // 8) for _ in range(weight))
            return x

        def main(get):
            m = [None] * 7
            rem = [None, None]
            for o in ('t', 2, 4, 'b', 1, 3, 0, 6, 5):
                if o in ('t', 'b'):
                    e = 0 if o == 't' else 1
                    rhs = jnp.concatenate([w_u[c, 2 * LANES:D // 2, :] for c in range(NC - 1)], axis=1)
                    rem[e] = timed(_dot(get([(9, e)]), _as_bf16(rhs)), WL)
                    continue
                if o in (1, 4):
                    d = (1, 4).index(o)
                    rhs = jnp.concatenate([w_u[2 * d + n2, d * LANES:(d + 1) * LANES, :] for n2 in range(2)], axis=1)
                else:
                    rhs = jnp.concatenate([s_u[o, n2] for n2 in range(2)], axis=1)
                m[o] = timed(_dot(get([(o, 0), (o, 1)]), _as_bf16(rhs)), WH if o in (4, 3, 6, 5) else WL)
            c11, c12, c21, c22 = _combine(m)
            top = jnp.concatenate([c11, c12], axis=1) + rem[0]
            bot = jnp.concatenate([c21, c22], axis=1) + rem[1]
            return [weave(top[:, c * LANES:(c + 1) * LANES], bot[:, c * LANES:(c + 1) * LANES]) for c in range(NC - 1)]

        def last(get):
            w4c = _as_bf16(w_u[NC - 1])
            return weave(timed(_dot(get([(2, 0), (2, 1), (7, 0), (7, 1), (9, 0)]), w4c), WL),
                         timed(_dot(get([(8, 0), (8, 1), (3, 0), (3, 1), (9, 1)]), w4c), WL))

        marks = []
        for j, part in enumerate(parts):
            get = lhs_of(part, toks[marks[-1]:] if marks else None)
            marks.append(len(toks))
            if j % 2:
                tail = last(get)
                cols = main(get) + [tail]
            else:
                cols = main(get) + [last(get)]
            emit(part, cols)
        return toks

    def filler(t):
        if DUM:
            red = jnp.sum(y_s[t, 0:8 * DUM, :], axis=-1, keepdims=True).reshape(DUM, 8, 1)
            zf_s[1, (NC - 1) * (TQ + 8) + 8 * t:(NC - 1) * (TQ + 8) + 8 * t + 8, :] = jnp.broadcast_to(jnp.sum(red, axis=0), (8, LANES))

    def chunks(r0, r1, k, unit=16):
        n = (r1 - r0) // unit
        cuts = [r0 + unit * ((n * j) // k) for j in range(k + 1)]
        return list(zip(cuts[:-1], cuts[1:]))

    def stage_m1(t, k):
        def emit(part, cols):
            out = [_gelu2(x) for x in cols]
            for c in range(NC):
                h1_s[c, part[0] + 8:part[1] + 8, :] = out[c]
            return out

        if t in STR1:
            def lhs_of(part, _):
                return lambda keys: _as_bf16(jnp.concatenate(
                    [lo_u[o, e, part[0] // 4:part[1] // 4, :] for o, e in keys], axis=1))
            return block_dots(lhs_of, w1_v, s1_s, chunks(A0[t], A0[t + 1], k, 32), emit, WL, WH)
        toks = []
        for r0, r1 in chunks(A0[t], A0[t + 1], k):
            pre = _dot(load_bf16(z_u, r0, r1 - r0), packed(w1_v))
            out = emit((r0, r1), [pre[:, c * LANES:(c + 1) * LANES] for c in range(NC)])
            toks += [x for x in tokens_of(jnp.concatenate(out, axis=1)) for _ in range(W1N)]
        return toks

    grp = D // 4
    shifts = (-1, 1, -2, 2)

    def shifted(r0, r1):
        n = r1 - r0
        lane = lax.broadcasted_iota(jnp.int32, (n, LANES), 1)
        cols = []
        for c in range(NC):
            lo, hi = c * LANES, (c + 1) * LANES
            g_lo, g_hi = lo // grp, (hi - 1) // grp
            val = h1_s[c, pl.ds(r0 + 8 + shifts[g_lo], n), :]
            if g_hi != g_lo:
                other = h1_s[c, pl.ds(r0 + 8 + shifts[g_hi], n), :]
                val = jnp.where(lane < (g_hi * grp - lo), val, other)
            cols.append(val)
        return cols

    def stage_m2(t, k, before=None):
        def emit(part, cols):
            x1 = h_s[part[0]:part[1], :] + jnp.concatenate(cols, axis=1)
            h_s[part[0]:part[1], :] = x1
            return x1

        if t in STR2:
            def lhs_of(part, prev):
                prev = before if prev is None else prev
                prev = prev[len(prev) // 8:(len(prev) * 7) // 8]
                ops = row_ops(shifted(*part), pick(prev, (part[1] - part[0]) // 32, 0))
                for o in range(10):
                    for e in range(2):
                        l2_s[o, e, part[0] // 2:part[1] // 2, :] = ops[o][e].astype(BF16)
                return lambda keys: _as_bf16(jnp.concatenate(
                    [l2_u[o, e, part[0] // 4:part[1] // 4, :] for o, e in keys], axis=1))
            return block_dots(lhs_of, w2_v, s2_s, chunks(B0[t], B0[t + 1], k, 32), emit, WM2, WM2)
        toks = []
        for r0, r1 in chunks(B0[t], B0[t + 1], k):
            hs = _dot(jnp.concatenate(shifted(r0, r1), axis=1).astype(BF16), packed(w2_v))
            toks += [x for x in tokens_of(emit((r0, r1), [hs])) for _ in range(W2N)]
        return toks

    TQ = TB // 4
    NT = S // TB
    GB = 2 * NH + 1

    def blk_rows(b):
        return slice(b * (TQ + 8), b * (TQ + 8) + TQ)

    def store_z(r0, slot, toks, free):
        zn = _ln(hold(h_s[pl.ds(r0, TB), :], pick(toks, TB // 8, free)), 4.0 * EPS)
        for rq in range(4):
            for c in range(NC - 1):
                zf_s[slot, blk_rows(NC * rq + c), :] = zn[rq * TQ:(rq + 1) * TQ, c * LANES:(c + 1) * LANES]
        zr_s[...] = zn[:, (NC - 1) * LANES:].astype(BF16)

    def outer_lhs(i, blk):
        terms = ((0, 0, 1, 1, 1), (1, 0, 1, 1, 1), (0, 0), (1, 1), (0, 0, 1, 0, 1), (1, 0, -1, 0, 0), (0, 1, -1, 1, 1))[i]
        x = blk(terms[0], terms[1])
        if len(terms) > 2:
            y = blk(terms[3], terms[4])
            x = x + y if terms[2] > 0 else x - y
        return x

    def z_ops(slot_of, toks):
        ng = TQ // 16

        def held(x, k):
            tk = jnp.stack([toks[((k * ng + r) * len(toks)) // (7 * ng)] for r in range(ng)])
            x4 = x.reshape(ng, 2, 8, LANES)
            return jnp.stack([after(tk, x4[:, 0]), x4[:, 1]], axis=1).reshape(TQ, LANES)

        for k, i in enumerate(ZORD):
            slot = slot_of()
            so = [outer_lhs(i, lambda r1, k1: zf_s[slot, blk_rows(NC * (2 * r1 + r2) + 2 * k1 + k2), :])
                  for r2 in range(2) for k2 in range(2)]
            for j, x in enumerate(_lhs_ops(held(so[0], k), so[1], so[2], held(so[3], k))):
                la_s[i, j] = x.astype(BF16)

    NS = NH // 2

    RAW = (1, 4)

    def weight_ops(src, dst, ext, transposed, toks):
        ng = LANES // 16
        lead = 2 if ext is not None else 0
        total = (NS * 7 + lead) * ng

        def tile(c, n):
            return src[c, n * LANES:(n + 1) * LANES, :].astype(F32)

        def held(x, pos, step):
            tk = jnp.stack([toks[((pos + r * step) * len(toks)) // total] for r in range(ng)])
            x4 = x.reshape(ng, 2, 8, LANES)
            return jnp.stack([after(tk, x4[:, 0]), x4[:, 1]], axis=1).reshape(LANES, LANES)

        def outer(c2, n, pos=None):
            b11, b22 = tile(c2, n), tile(2 + c2, NH + n)
            if pos is not None:
                b11, b22 = held(b11, pos, 1), held(b22, pos, 1)
            e1, e2 = tile(c2, NH + n), tile(2 + c2, n)
            return _rhs_ops(b11, e1, e2, b22) if transposed else _rhs_ops(b11, e2, e1, b22)

        for c2 in range(2 if ext is not None else 0):
            for i, x in enumerate(outer(c2, NH - 1, c2 * ng)):
                if i not in RAW:
                    ext[i, c2] = x.astype(BF16)
        for st in range(NS):
            t00, t11 = outer(0, 2 * st), outer(1, 2 * st + 1)
            t01, t10 = outer(0, 2 * st + 1), outer(1, 2 * st)
            for k, i in enumerate((1, 5, 2, 4, 0, 3, 6)):
                pos = (lead + st * 7) * ng + k
                a, d = held(t00[i], pos, 7), held(t11[i], pos, 7)
                ops = _rhs_ops(a, t01[i], t10[i], d) if transposed else _rhs_ops(a, t10[i], t01[i], d)
                for j, x in enumerate(ops):
                    if i not in RAW or j not in RAW:
                        dst[i, j, st * LANES:(st + 1) * LANES, :] = x.astype(BF16)

    LQ = (FF - 2 * NS * 2 * LANES) // 4
    LCUT = (NH - 1) * LANES

    def left_rows(ref, c, lo, hi, shift):
        parts = []
        if lo < LANES:
            parts.append(ref[c, (LCUT + lo) >> shift:(LCUT + min(hi, LANES)) >> shift, :])
        if hi > LANES:
            base = (2 * NH - 2) * LANES
            parts.append(ref[c, (base + max(lo, LANES)) >> shift:(base + hi) >> shift, :])
        return parts

    def left_ops(toks):
        ng = LQ // 16

        def blk(c, qd):
            return jnp.concatenate([x.astype(F32) for x in left_rows(w3_v, c, qd * LQ, (qd + 1) * LQ, 0)], axis=0)

        def outer(k2, p):
            return _rhs_ops(blk(k2, p), blk(k2, 2 + p), blk(2 + k2, p), blk(2 + k2, 2 + p))

        t00, t01, t10, t11 = outer(0, 0), outer(0, 1), outer(1, 0), outer(1, 1)
        for k, i in enumerate((1, 5, 2, 4, 0, 3, 6)):
            tk = jnp.stack([toks[((k + r * 7) * len(toks)) // (7 * ng)] for r in range(ng)])

            def held(x):
                x4 = x.reshape(ng, 2, 8, LANES)
                return jnp.stack([after(tk, x4[:, 0]), x4[:, 1]], axis=1).reshape(LQ, LANES)

            for j, x in enumerate(_rhs_ops(held(t00[i]), t01[i], t10[i], held(t11[i]))):
                sl_s[i, j] = x.astype(BF16)

    with jax.named_scope("r0a"):
        wait_all(first[:1])
        conv_round(0, 'k', False, False)
    with jax.named_scope("r0_wait"):
        wait_all(first[1:])
    with jax.named_scope("r0b"):
        start_all(conv_copies(2) + conv_copies(3) + conv_copies(4))
        conv_round(0, 'u', False, False)
    with jax.named_scope("r1a"):
        wait_all(second[:1])
        conv_round(1, 'k', True, False)
    with jax.named_scope("r1_wait"):
        wait_all(second[1:])
    with jax.named_scope("r1b"):
        start_all(wm_copies[0] + q_copies[0] + wm_copies[1] + w_copies[0])
        conv_round(1, 'u', False, False)

    def full_round(c, carry):
        wait_all(conv_copies(c))
        conv_round(c, 'ku', True, True)
        return carry

    with jax.named_scope("r234"):
        lax.fori_loop(2, NC, full_round, 0)
    with jax.named_scope("r5"):
        start_all(q_copies[1] + w_copies[1] + sum(q_copies[2:], []) + w_copies[2] + w_copies[3] + wm_copies[2], 1)
        conv_round(NC, '', True, True)
    with jax.named_scope("r6_wait"):
        wait_all(wm_copies[0] + q_copies[0])
    with jax.named_scope("r6"):
        for j in range(3):
            mod_chunk(j)
        conv_round(NC + 1, '', False, True)
        nx0 = stage_p1(0, A0[1], [None], mods_a())
    with jax.named_scope("p2_wait"):
        wait_all(wm_copies[1])
    with jax.named_scope("p2"):
        mod_chunk(4)
        mod_chunk(3)
        stage_p2(0, A0[1], nx0, mods_b())
    with jax.named_scope("w1_wait"):
        wait_all(w_copies[0])
    with jax.named_scope("m1_0"):
        toks = stage_m1(0, 4)
        if STR1:
            square_ops(w1_v, s1_s, toks[:len(toks) - 20 * W1N])
    with jax.named_scope("w2_wait"):
        wait_all(q_copies[1] + w_copies[1])
    with jax.named_scope("m2_0"):
        toks = stage_m2(0, 4)
        stage_p(1, toks[:len(toks) - TRIM * W2N], FREE * W2N)
        if STR2 and min(STR2) == 1:
            square_ops(w2_v, s2_s, toks[len(toks) // 2:len(toks) - 10 * W2N])
        filler(0)
    for t in range(1, NA):
        with jax.named_scope("a%d" % t):
            if t + 1 < NA:
                wait_all(q_copies[t + 1])
            else:
                wait_all(w_copies[2] + w_copies[3] + wm_copies[2])
            t1 = stage_m1(t, SPLIT)
            t2 = stage_m2(t, SPLIT, t1[len(t1) - len(t1) // SPLIT:])

            def weighted(trim):
                return t1 + t2[:len(t2) - trim * W2N]

            if t + 1 < NA:
                stage_p(t + 1, weighted(TRIM), FREE * W2N)
            if STR2 and t == W2P:
                square_ops(w2_v, s2_s, weighted(10))
            if t == NA - 1 - LAT:
                toks = weighted(TRIM // 2)
                store_z(0, 0, toks if LAT and not ZE else toks[:len(toks) // 2], FREE * W2N)
                if ZE:
                    toks = weighted(10)
                    z_ops(lambda: 0, toks[(len(toks) * 5) // 8:])
            if t == NA - 1:
                mod_chunk(NC)
                toks = weighted(20)
                toks = toks[:1] * PRE + toks
                cut0 = (len(toks) * 3) // 47
                cut = (len(toks) * 24) // 47
                left_ops(toks[:cut0])
                weight_ops(w3_v, s3_s, None, True, toks[cut0:cut])
                weight_ops(w4_v, s4_s, e4_s, False, toks[cut:])
                if not ZE:
                    z_ops(lambda: 0, toks if LAT else toks[(len(toks) * 5) // 8:])
            if t + 1 < NA or not LAT:
                filler(t)

    gb = 0.5 * mod_s[NC, 0:1, :]
    w3_u, w4_u, s3_u, s4_u, e4_u = (r.bitcast(U32) for r in (w3_v, w4_v, s3_s, s4_s, e4_s))
    HL = LANES // 2
    la_u = la_s.bitcast(U32)
    zr_u = zr_s.bitcast(U32)
    sl_u = sl_s.bitcast(U32)

    def out_copy(r0, n, c):
        rows = pl.ds(r0, n)
        return pltpu.make_async_copy(o_v.at[c, rows, :], o_hbm.at[rows, pl.ds(c * LANES, LANES)], sem_o.at[0])

    def one_level(w_u, e_u, i, c2):
        if i not in RAW:
            return e_u[i, c2]
        d = RAW.index(i)
        n = d * NH + NH - 1
        return w_u[2 * d + c2, n * HL:(n + 1) * HL, :]

    def two_level(w_u, s_u, i, j, st):
        if i not in RAW or j not in RAW:
            return s_u[i, j, st * HL:(st + 1) * HL, :]
        d, e = RAW.index(i), RAW.index(j)
        n = d * NH + 2 * st + e
        return w_u[2 * d + e, n * HL:(n + 1) * HL, :]

    def loop_b(t, carry):
        r0 = pl.multiple_of(t * TB, TB)
        ws = t & 1

        count = [0]

        def fresh():
            count[0] += 1
            return lax.rem(t + 2 * count[0], 2)

        zr = [_as_bf16(zr_u[rq * (TQ // 2):(rq + 1) * (TQ // 2), :]) for rq in range(4)]
        ltoks, ftoks = [], []

        def light(x):
            ltoks.extend(x[8 * r:8 * r + 8, 0:LANES] for r in range(x.shape[0] // 8))

        def rem3(rq, n):
            return _dot_nt(zr[rq], _as_bf16(w3_u[NC - 1, n * HL:(n + 1) * HL, :]))

        def put_g(rq, n, pre):
            g_s[rq // 2][ws, blk_rows(GB * (rq % 2) + n), :] = _gelu2(pre)

        rem = {}
        for st in range(NS):
            rem[3, NH + 2 * st + 1] = rem3(3, NH + 2 * st + 1)
        w_left = _as_bf16(jnp.concatenate(left_rows(w3_u, NC - 1, 0, 4 * LQ, 1), axis=0))
        rem_left = [_dot_nt(w_left, zr[rq]) for rq in range(4)]
        for st in range(NS):
            todo = [(2 * r1 + r2, h * NH + 2 * st + p) for r1, h in ((0, 1), (1, 0), (0, 0), (1, 1))
                    for r2 in range(2) for p in range(2)]
            todo = [x for x in todo if x not in rem]
            for key in todo[:8]:
                rem[key] = rem3(*key)
            if st >= LSETS:
                light(rem[todo[1]])
                light(rem[todo[5]])
            todo = todo[8:]
            pin = [None] * 7
            pil = [None] * 7
            for i in _ORDER:
                m = [None] * 7
                ml = [None] * 7
                for group in (_ORDER[:4], _ORDER[4:]):
                    for j in group:
                        m[j] = _dot_nt(_as_bf16(la_u[i, j]), _as_bf16(two_level(w3_u, s3_u, i, j, st)))
                    if len(group) == 3:
                        key = todo.pop(0)
                        rem[key] = rem3(*key)
                    if st == 0:
                        for j in group:
                            ml[j] = _dot_nt(_as_bf16(sl_u[i, j]), _as_bf16(la_u[i, j]))
                if st >= LSETS and i in (2, 1, 0):
                    light(m[_ORDER[1]])
                    light(m[_ORDER[5]])
                pin[i] = _combine(m)
                if st == 0:
                    pil[i] = _combine(ml)
            for inner in range(4):
                for blk, cval in enumerate(_combine([pin[i][inner] for i in range(7)])):
                    rq, n = 2 * (blk // 2) + inner // 2, (blk % 2) * NH + 2 * st + inner % 2
                    put_g(rq, n, cval + rem[rq, n])
            if st == 0:
                cl = [_combine([pil[i][inner] for i in range(7)]) for inner in range(4)]
                for rq in range(4):
                    r1, r2 = rq // 2, rq % 2
                    gt = _gelu2(jnp.concatenate([cl[2 * r2 + p][2 * r1 + h] for h in range(2) for p in range(2)], axis=0)
                                + rem_left[rq])
                    g_s[r1][ws, blk_rows(GB * r2 + NH - 1), :] = gt[0:LANES].T
                    g_s[r1][ws, blk_rows(GB * r2 + 2 * NH - 1), :] = jnp.concatenate(
                        [gt[LANES:], jnp.zeros((FP - FF, TQ), F32)], axis=0).T

        toks = []

        def timed(x):
            toks.extend(x[8 * r:8 * r + 8, 0:LANES] for r in range(x.shape[0] // 8))
            return x

        def finish(rq, c, h2):
            rows = pl.ds(pl.multiple_of(r0 + rq * TQ, TQ), TQ)
            cols = slice(c * LANES, (c + 1) * LANES)
            o_v[c, rows, :] = (x_s[rows, cols] + gb[:, cols] * (h_s[rows, cols] + h2)).astype(BF16)

        kord = [NH - 1, 2 * NH - 1] + [h * NH + n for st in range(NS) for h in (1, 0) for n in (2 * st + 1, 2 * st)]
        w4r = _as_bf16(jnp.concatenate([w4_u[NC - 1, n * HL:(n + 1) * HL, :] for n in kord], axis=0))

        def rem4(rq, slot):
            lhs = jnp.concatenate([g_s[rq // 2][slot, blk_rows(GB * (rq % 2) + n), :] for n in kord], axis=1).astype(BF16)
            r = timed(_dot(lhs, w4r))
            finish(rq, NC - 1, r)

        rem4(0, fresh())
        rem4(1, fresh())
        pin = [None] * 7
        done = {_ORDER[1]: 1, _ORDER[3]: 2, _ORDER[5]: 0, _ORDER[6]: 3}
        for i in _ORDER:
            slot = fresh()
            rhs = _as_bf16(jnp.concatenate([one_level(w4_u, e4_u, i, c2) for c2 in range(2)], axis=1))
            ex = [_dot(outer_lhs(i, lambda r1, h: g_s[r1][slot, blk_rows(GB * r2 + h * NH + NH - 1), :]).astype(BF16), rhs)
                  for r2 in range(2)]
            m = [None] * 7
            for j in _ORDER:
                slot = fresh()
                lhs = jnp.concatenate(
                    [outer_lhs(j, lambda r2, p: outer_lhs(
                        i, lambda r1, h: g_s[r1][slot, blk_rows(GB * r2 + h * NH + 2 * st + p), :]))
                     for st in range(NS)], axis=1).astype(BF16)
                m[j] = timed(_dot(lhs, _as_bf16(jnp.concatenate([two_level(w4_u, s4_u, i, j, st) for st in range(NS)], axis=0))))
            pin[i] = [x + ex[inner // 2][:, (inner % 2) * LANES:(inner % 2 + 1) * LANES]
                      for inner, x in enumerate(_combine(m))]
            if i in done:
                blk = done[i]
                for inner in (1, 2, 0, 3):
                    p = [pin[k][inner] if pin[k] is not None else None for k in range(7)]
                    cval = (lambda: (p[3] - p[4]) + p[0] + p[6], lambda: p[2] + p[4], lambda: p[1] + p[3],
                            lambda: (p[2] - p[1]) + p[0] + p[5])[blk]()
                    finish(2 * (blk // 2) + inner // 2, 2 * (blk % 2) + inner % 2, cval)
                rb = pl.multiple_of(r0 + (blk // 2) * 2 * TQ, 2 * TQ)
                for e in range(2):
                    out_copy(rb, 2 * TQ, 2 * (blk % 2) + e).start()
                if blk == 0:
                    out_copy(r0, 3 * TQ, NC - 1).start()
            if i == _ORDER[REM2]:
                rem4(2, fresh())
        rem4(3, fresh())
        out_copy(pl.multiple_of(r0 + 3 * TQ, TQ), TQ, NC - 1).start()

        nxt = jnp.minimum(t + 1, NT - 1)
        store_z(pl.multiple_of(nxt * TB, TB), ws, ftoks[len(ftoks) - FT:] + ltoks[:LN1:LSTEP] + toks[:LB1], 0)
        z_ops(fresh, toks[ZB0:ZB1])
        if DUMB:
            filler(4)
        return carry

    with jax.named_scope("ph2b"):
        lax.fori_loop(0, NT, loop_b, 0)
    with jax.named_scope("tail"):
        pltpu.make_async_copy(o_v, o_v, sem_o.at[0]).wait()


@jax.jit
def pallas_adaLN_cond__ssm_conv_h3__mixer_s_mlp__prompt_kernel(
    A_q: jax.Array,
    A_k: jax.Array,
    A_v: jax.Array,
    A_shift_k: jax.Array,
    A_ssm_k: jax.Array,
    A_ssm_D: jax.Array,
    B_x: jax.Array,
    B_w1: jax.Array,
    B_w2: jax.Array,
    B_w3: jax.Array,
    B_w4: jax.Array,
    c: jax.Array,
    w_mod: jax.Array,
):
    B, S, D = A_q.shape
    assert B == 1
    FF = B_w3.shape[1]
    NC = D // LANES
    NG = BLK // 8
    NBL = S // (PH * BLK)
    FP = -(-FF // (2 * LANES)) * 2 * LANES
    TILES = (384, 384, 576, 704)
    assert sum(TILES) == S
    TB = 512

    args = (A_q.reshape(S, D), A_k.reshape(S, D), A_v.reshape(S, D), A_shift_k.T, A_ssm_k,
            A_ssm_D, B_w1, B_w2, B_w3.T, B_w4, c, w_mod)
    scratch = [
        pltpu.VMEM((S, D), BF16),
        pltpu.VMEM((NC, S + KP, LANES), BF16),
        pltpu.VMEM((NC, S + VP, LANES), BF16),
        pltpu.VMEM((4, D), BF16),
        pltpu.VMEM((NC, LANES, S), BF16),
        pltpu.VMEM((D,), BF16),
        pltpu.VMEM((NC, D, LANES), BF16),
        pltpu.VMEM((NC, D, LANES), BF16),
        pltpu.VMEM((NC, FF, LANES), BF16),
        pltpu.VMEM((NC, FP, LANES), BF16),
        pltpu.VMEM((1, D), BF16),
        pltpu.VMEM((D, 6 * D), BF16),
        pltpu.VMEM((PH, 2 * BLK, BLK), BF16),
        pltpu.VMEM((PH, 2, BLK, BLK), BF16),
        pltpu.VMEM((NC, S, LANES), BF16),
        pltpu.VMEM((NC, NG, NBL, PH, 2, 8, LANES), F32),
        pltpu.VMEM((NC, NG, NBL, PH, 2, 8, LANES), F32),
        pltpu.VMEM((NC, NBL, PH, 2 * BLK, LANES), BF16),
        pltpu.VMEM((NBL, PH, BLK, LANES), BF16),
        pltpu.VMEM((NC, S + YP, LANES), F32),
        pltpu.VMEM((6, 8, D), F32),
        pltpu.VMEM((NC, 8, LANES), F32),
        pltpu.VMEM((NC, S + 16, LANES), F32),
        pltpu.VMEM((S, D), F32),
        pltpu.VMEM((S, D), F32),
        pltpu.VMEM((NC, S, LANES), BF16),
        pltpu.VMEM((7, 7, FP // 512 * LANES, LANES), BF16),
        pltpu.VMEM((7, 7, FP // 512 * LANES, LANES), BF16),
        pltpu.VMEM((7, 2, LANES, LANES), BF16),
        [pltpu.VMEM((2, GR, LANES), F32)] * 2,
        pltpu.VMEM((2, ZR, LANES), F32),
        pltpu.VMEM((TB, LANES), BF16),
        pltpu.VMEM((7, 7, TB // 4, LANES), BF16),
        pltpu.VMEM((10, 2, S // 2, LANES), BF16),
        pltpu.VMEM((10, 2, S // 2, LANES), BF16),
        pltpu.VMEM((7, 2, 2 * LANES, LANES), BF16),
        pltpu.VMEM((7, 2, 2 * LANES, LANES), BF16),
        pltpu.VMEM((7, 7, (FF - FP // 512 * 512) // 4, LANES), BF16),
        pltpu.SemaphoreType.DMA((16 + len(TILES),)),
        pltpu.SemaphoreType.DMA((1,)),
    ]
    out = pl.pallas_call(
        functools.partial(_kernel, S=S, D=D, FF=FF, TILES=TILES, TB=TB),
        in_specs=[pl.BlockSpec(memory_space=pl.ANY)] * len(args),
        out_specs=pl.BlockSpec(memory_space=pl.ANY),
        out_shape=jax.ShapeDtypeStruct((S, D), BF16),
        scratch_shapes=scratch,
        compiler_params=pltpu.CompilerParams(
            vmem_limit_bytes=126 * 1024 * 1024,
            disable_bounds_checks=True,
            disable_semaphore_checks=True,
        ),
    )(*args)
    return out.reshape(B, S, D)
```

```python
import functools
import math

import jax
import jax.numpy as jnp
from jax import lax
import jax.experimental.pallas as pl
import jax.experimental.pallas.tpu as pltpu

F32 = jnp.float32
BF16 = jnp.bfloat16
U32 = jnp.uint32

LANES = 128
BLK = 128
PH = 4
EPS = 1e-05
TRIM = 60
SPLIT = 2
FREE = 30
DUM = 96
LN1 = 999
KP = 16
VP = 0
YP = 0
GR = 1928
ZR = 2720
FT = 0
DUMB = 0
STR1 = (3, )
STR2 = (2, 3, )
WL = 3
WH = 2
ZE = 1
PRE = 0
WM2 = 2
W2P = 1
UL = 2
ALN = 0
LN0 = 32
SLAG = 1
NHEAD = 0
XTOK = 1
LASTO = 1
PINJ = ()
FLAG = 10
FSTEP = 1
WE = 2
XEND = 50
CUT = 50
VMOD = 1
W1N = 2
W2N = 3
LAT = 1
LSETS = 1
LSTEP = 1
LB1 = 0
ZB0 = 0
ZB1 = 700
REM2 = 2
ZORD = (2, 3, 0, 1, 4, 5, 6)


def _as_bf16(x):
    return pltpu.bitcast(x, BF16)


def _lo(x):
    return pltpu.bitcast(x << 16, F32)


def _hi(x):
    return pltpu.bitcast(x & jnp.uint32(0xFFFF0000), F32)


def _dft4(re, im, sign):
    ar, ai = re[0] + re[2], im[0] + im[2]
    br, bi = re[0] - re[2], im[0] - im[2]
    cr, ci = re[1] + re[3], im[1] + im[3]
    dr, di = re[1] - re[3], im[1] - im[3]
    o0 = (ar + cr, ai + ci)
    o2 = (ar - cr, ai - ci)
    m = (br + di, bi - dr)
    p = (br - di, bi + dr)
    o1, o3 = (m, p) if sign < 0 else (p, m)
    return [o0[0], o1[0], o2[0], o3[0]], [o0[1], o1[1], o2[1], o3[1]]


def _ln(x, eps=EPS, unit=True):
    n = x.shape[-1]
    s1 = jnp.sum(x, axis=-1, keepdims=True)
    m = s1 * (1.0 / n)
    v = jnp.maximum(jnp.sum(x * x, axis=-1, keepdims=True) + (n * eps - s1 * m), n * eps)
    e = jnp.log(v) * (-0.5 / math.log(2.0))
    return (x - m) * jnp.exp2(e + 0.5 * math.log2(n) if unit else e)


def _gelu2(x):
    c0 = math.sqrt(2.0 / math.pi)
    return x + x * jnp.tanh(x * (c0 + (c0 * 0.044715) * (x * x)))


def _dot(a, b):
    return jnp.dot(a, b, preferred_element_type=F32)


def _dot_nt(a, b):
    return lax.dot_general(a, b, (((1,), (1,)), ((), ())), preferred_element_type=F32)


def _lhs_ops(a11, a12, a21, a22):
    return [a11 + a22, a21 + a22, a11, a22, a11 + a12, a21 - a11, a12 - a22]


def _rhs_ops(b11, b12, b21, b22):
    return [b11 + b22, b11, b12 - b22, b21 - b11, b22, b11 + b12, b21 + b22]


def _combine(m):
    return (m[3] - m[4]) + m[0] + m[6], m[2] + m[4], m[1] + m[3], (m[2] - m[1]) + m[0] + m[5]


_ORDER = (2, 4, 1, 3, 0, 6, 5)


def _kernel(q_hbm, k_hbm, v_hbm, sh_hbm, sk_hbm, sd_hbm, w1_hbm, w2_hbm, w3_hbm, w4_hbm, c_hbm, wm_hbm,
            o_hbm,
            q_v, k_v, v_v, sh_v, sk_v, sd_v, w1_v, w2_v, w3_v, w4_v, c_v, wm_v,
            fw_s, iv_s, o_v, u_s, kk_s, vv_s, wu_s, y_s, mod_s, par_s, h1_s, x_s, h_s, z_s, s3_s, s4_s, e4_s, g_s, zf_s, zr_s, la_s, lo_s, l2_s, s1_s, s2_s, sl_s, sc_s, ec_s, rl_s, rh_s, wt_s, scol_s,
            sem, sem_o,
            *, S, D, FF, TILES, TB):
    NC = D // LANES
    NG = BLK // 8
    LB = PH * BLK
    NBL = S // LB
    R = BLK // PH
    HALO = 32
    FP = w4_v.shape[1]
    FH = FP // 2
    NH = FH // LANES

    small = [
        pltpu.make_async_copy(sh_hbm, sh_v, sem.at[0]),
        pltpu.make_async_copy(sd_hbm, sd_v, sem.at[0]),
        pltpu.make_async_copy(c_hbm, c_v, sem.at[0]),
    ]

    def conv_copies(c):
        col = pl.ds(c * LANES if isinstance(c, int) else pl.multiple_of(c * LANES, LANES), LANES)
        return [
            pltpu.make_async_copy(sk_hbm.at[col, :], sk_v.at[c], sem.at[9 + c if isinstance(c, int) and c < 2 else 1 + c]),
            pltpu.make_async_copy(k_hbm.at[:, col], k_v.at[c, pl.ds(16, S), :], sem.at[1 + c]),
            pltpu.make_async_copy(v_hbm.at[:, col], v_v.at[c, pl.ds(0, S), :], sem.at[1 + c]),
        ]

    def col_copies(src, dst, c0, s):
        rows = pl.ds(0, src.shape[0])
        return [pltpu.make_async_copy(src.at[:, pl.ds((c0 + c) * LANES, LANES)], dst.at[c0 + c, rows, :], sem.at[s])
                for c in range(NC)]

    WM = (0, 3 * D, 5 * D, 6 * D)
    wm_copies = [[pltpu.make_async_copy(wm_hbm.at[:, pl.ds(WM[j], WM[j + 1] - WM[j])],
                                        wm_v.at[:, pl.ds(WM[j], WM[j + 1] - WM[j])], sem.at[6 + j])]
                 for j in range(3)]
    w_copies = [col_copies(src, dst, 0, 12 + j)
                for j, (src, dst) in enumerate(((w1_hbm, w1_v), (w2_hbm, w2_v), (w3_hbm, w3_v), (w4_hbm, w4_v)))]

    B0 = [0]
    for n in TILES:
        B0.append(B0[-1] + n)
    NA = len(TILES)
    A0 = [0] + [r + HALO for r in B0[1:-1]] + [S]
    q_copies = [
        [pltpu.make_async_copy(q_hbm.at[pl.ds(A0[t], A0[t + 1] - A0[t])], q_v.at[pl.ds(A0[t], A0[t + 1] - A0[t])],
                               sem.at[16 + t])]
        for t in range(NA)
    ]

    def start_all(cps, priority=0):
        for cp in cps:
            cp.start(priority=priority)

    def wait_all(cps):
        for cp in cps:
            cp.wait()

    def packed(ref, c0=0):
        ru = ref.bitcast(U32)
        return _as_bf16(jnp.concatenate([ru[c0 + c] for c in range(NC)], axis=1))

    first, second = conv_copies(0), conv_copies(1)
    start_all(first[:1] + small + first[1:] + second)

    for c in range(NC):
        k_v[c, 0:16, :] = jnp.zeros((16, LANES), BF16)
        h1_s[c, 0:8, :] = jnp.zeros((8, LANES), F32)
        h1_s[c, S + 8:S + 16, :] = jnp.zeros((8, LANES), F32)
        w4_v[c, FF:FP, :] = jnp.zeros((FP - FF, LANES), BF16)

    prow = lax.broadcasted_iota(jnp.int32, (BLK, BLK), 0)
    pcol = lax.broadcasted_iota(jnp.int32, (BLK, BLK), 1)
    ang = (((4 * prow + 1) * pcol) & (4 * BLK - 1)).astype(F32) * (2.0 * math.pi / (4 * BLK))
    tw = (4 * prow + 1).astype(F32) * (2.0 * math.pi / (4 * LB))
    mr, mi = jnp.cos(ang), -jnp.sin(ang)
    zr_, zi_ = jnp.cos(tw), -jnp.sin(tw)
    eye = jnp.where(prow == pcol, 1.0 / LB, 0.0).astype(BF16)
    for i in range(PH):
        both = jnp.stack([mr.reshape(NG, 8, BLK), mi.reshape(NG, 8, BLK)], axis=1).reshape(2 * BLK, BLK)
        fw_s[i] = both.astype(BF16)
        for h in range(2):
            iv_s[i, h] = _dot_nt(eye, both[h * BLK:(h + 1) * BLK, :].astype(BF16)).astype(BF16)
        if i + 1 < PH:
            mr, mi = mr * zr_ - mi * zi_, mr * zi_ + mi * zr_
    perm = jnp.where(pcol == (prow % R) * PH + prow // R, 1.0, 0.0).astype(BF16)
    fw_u = fw_s.bitcast(U32)
    iv_u = iv_s.bitcast(U32)

    wait_all(small)
    shf = sh_v[...].astype(F32)
    sdf = sd_v[...].astype(F32).reshape(1, D)
    for c in range(NC):
        par_s[c, 0:4, :] = shf[:, c * LANES:(c + 1) * LANES]
        par_s[c, 4:5, :] = sdf[:, c * LANES:(c + 1) * LANES]
    cf = c_v[...].astype(F32)
    sc = (cf * jax.nn.sigmoid(cf)).astype(BF16)
    sc16 = jnp.broadcast_to(sc, (16, D))

    scol_s[...] = jnp.broadcast_to(sc.astype(F32), (LANES, D)).T

    def mod_chunk(j):
        mod_s[j] = _dot(sc16, wm_v[:, j * D:(j + 1) * D])[0:8, :]

    k_u = k_v.bitcast(U32)
    v_u = v_v.bitcast(U32)
    wu_u = wu_s.bitcast(U32)
    z_u = z_s.bitcast(U32)
    vv_u = vv_s.bitcast(U32)
    lo_u = lo_s.bitcast(U32)
    l2_u = l2_s.bitcast(U32)

    never = zr_[0:8, :] > 2.0

    def after(token, x):
        if token.dtype != x.dtype:
            token = pltpu.bitcast(token, x.dtype)
        return jnp.where(jnp.broadcast_to(never, x.shape), token, x)

    def split(t):
        t4 = t.reshape(NG, 2, 8, LANES)
        return t4[:, 0], t4[:, 1]

    def perm_k(c, b, toks):
        kt = [_dot_nt(perm, sk_v[c, :, b * LB + t * BLK:b * LB + (t + 1) * BLK]) for t in range(PH)]
        for r in range(BLK // 16):
            toks.append(kt[0][16 * r:16 * r + 8, :])
        return [jnp.concatenate([kt[t][i * R:(i + 1) * R, :] for t in range(PH)], axis=0).astype(BF16)
                for i in range(PH)]

    def spectrum(wts, dst, c, b, toks, dc=None, pins=None):
        tr, ti = [], []
        for i in range(PH):
            lhs = fw_u[i]
            if pins is not None and i < len(pins):
                lhs = after(pins[i], lhs.reshape(NG, 8, LANES)).reshape(BLK, LANES)
            r_, i_ = split(_dot(_as_bf16(lhs), wts[i]))
            tr.append(r_)
            ti.append(i_)
        for g in range(NG):
            toks.append(ti[PH - 1][g])
        if dc is not None:
            tr[0] = tr[0] + dc
        sr, si = _dft4(tr, ti, -1)
        for qq in range(PH):
            dst[c, :, b, qq, 0] = sr[qq]
            dst[c, :, b, qq, 1] = si[qq]

    def gated(c, b):
        w = [par_s[c, t:t + 1, :] for t in range(4)]
        kc = {}
        for o in range(-2, 2):
            words = k_u[c, pl.ds(8 + b * (LB // 2) + o, BLK, stride=2), :]
            if o > -2:
                kc[2 * o] = _lo(words)
            kc[2 * o + 1] = _hi(words)
        vc = {}
        for o in range(2):
            words = v_u[c, pl.ds(b * (LB // 2) + o, BLK, stride=2), :]
            vc[2 * o] = _lo(words)
            vc[2 * o + 1] = _hi(words)
        for i in range(PH):
            ks = kc[i] * w[0]
            for t in range(1, 4):
                ks = ks + kc[i - t] * w[t]
            wu_s[b, i] = (ks * vc[i]).astype(BF16)
        return [wu_u[b, i] for i in range(PH)]

    def kv_pins(kvb):
        return [jnp.stack([kvb[2 * m + (r % 2)][8 * (r // 2):8 * (r // 2) + 8, :] for r in range(NG)])
                for m in range(2)]

    def mac(c, us, ks, toks):
        zp = None
        for o in range(NBL):
            zr, zi = [], []
            for qq in range(PH):
                accr = acci = None
                for b in range(o + 1):
                    a_, b_ = us[0, :, b, qq, 0], us[0, :, b, qq, 1]
                    c_, d_ = ks[0, :, o - b, qq, 0], ks[0, :, o - b, qq, 1]
                    if qq == 0 and b == o:
                        a_ = after(toks[o], a_)
                    tr_ = a_ * c_ - b_ * d_
                    ti_ = a_ * d_ + b_ * c_
                    accr = tr_ if accr is None else accr + tr_
                    acci = ti_ if acci is None else acci + ti_
                zr.append(accr)
                zi.append(acci)
            if zp is None:
                yr, yi = zr, zi
            else:
                yr = [zr[qq] - zp[1][qq] for qq in range(PH)]
                yi = [zi[qq] + zp[0][qq] for qq in range(PH)]
            zp = (zr, zi)
            vr, vi = _dft4(yr, yi, +1)
            for i in range(PH):
                vv_s[c, o, i] = jnp.stack([vr[i], vi[i]], axis=1).reshape(2 * BLK, LANES).astype(BF16)

    def inverse(c, toks, pins=None):
        HB = BLK // 2
        for o in range(NBL):
            for i in range(PH):
                yv = None
                for h in range(2):
                    lhs = iv_u[i, h]
                    if pins is not None and h == 0:
                        pin = pins[o][i % 2][8 * (i // 2):8 * (i // 2) + 8]
                        lhs = after(pin, lhs.reshape(8, 8, LANES)).reshape(HB, LANES)
                    t = _dot(_as_bf16(lhs), _as_bf16(vv_u[c, o, i, h * HB:(h + 1) * HB, :]))
                    yv = t if yv is None else yv + t
                if i % 2 == 0:
                    for r in range(BLK // 16):
                        toks.append(yv[16 * r:16 * r + 8, :])
                y_s[c, pl.ds(o * LB + i, BLK, stride=PH), :] = yv

    def mac_tokens(toks):
        n = len(toks) - 3
        cum = (44, 128, 244, 392)
        return [jnp.stack([toks[max(0, ((g * 392 + cum[o]) * n) // (392 * NG) - 1)] for g in range(NG)])
                for o in range(NBL)]

    def conv_round(c, fwd, mul, inv):
        toks = []
        kv = pins = None
        cur = 1 if mul else 0
        if fwd or mul:
            win = pl.ds(c - cur, 2 if fwd and mul else 1)
            us, ks = u_s.at[win], kk_s.at[win]
        if 'u' in fwd:
            kv = [gated(c, b) for b in range(NBL)]
            pins = [kv_pins(kv[b]) for b in range(NBL)]
        if inv:
            inverse(c - 2, toks, pins)
            if fwd:
                toks = []
        if 'k' in fwd:
            wts = [perm_k(c, b, toks) for b in range(NBL)]
        for b in range(NBL):
            if 'k' in fwd:
                spectrum(wts[b], ks, cur, b, toks, par_s[c, 4:5, :] if b == 0 else None)
            if 'u' in fwd:
                pin = pins[b + UL] if not inv and b + UL < NBL else None
                spectrum([_as_bf16(x) for x in kv[b]], us, cur, b, toks, None, pin)
        if mul:
            mac(c - 1, us, ks, mac_tokens(toks))

    def tokens_of(x):
        return [x[8 * r:8 * r + 8, c * LANES:(c + 1) * LANES] for c in range(NC) for r in range(x.shape[0] // 8)]

    def store_bf16(ref, r0, x):
        for c in range(NC):
            ref[c, r0:r0 + x.shape[0], :] = x[:, c * LANES:(c + 1) * LANES].astype(BF16)

    def load_bf16(ref_u, r0, n):
        return _as_bf16(jnp.concatenate([ref_u[c, pl.ds(r0 // 2, n // 2), :] for c in range(NC)], axis=1))

    def pick(toks, n, free):
        if toks is None:
            return [None] * n
        idx = [(r * (len(toks) + free)) // n - free for r in range(n)]
        return [toks[i] if i >= 0 else None for i in idx]

    def hold(x, tks, head=False):
        if head:
            return jnp.concatenate([after(tks[0], x[0:8]), x[8:]], axis=0)
        f = len([k for k in tks if k is None])
        n = len(tks)
        if f == n:
            return x
        first = after(jnp.stack(tks[f:]), x[8 * f:, 0:LANES].reshape(n - f, 8, LANES)).reshape(8 * (n - f), LANES)
        if f:
            first = jnp.concatenate([x[:8 * f, 0:LANES], first], axis=0)
        return jnp.concatenate([first, x[:, LANES:]], axis=1)

    def mods_a():
        ga = mod_s[2, 0:1, :]
        return ga * (1.0 + mod_s[1, 0:1, :]) * math.sqrt(D), ga * mod_s[0, 0:1, :]

    def mods_b():
        return (1.0 + mod_s[4, 0:1, :]) * (2.0 * math.sqrt(D)), 2.0 * mod_s[3, 0:1, :]

    def stage_p1(r0, r1, tks, ma):
        q = hold(q_v[r0:r1, :].astype(F32), tks)
        y = jnp.concatenate([y_s[c, r0:r1, :] for c in range(NC)], axis=1)
        x = q + (_ln(q, unit=False) * ma[0] + ma[1]) * y
        x_s[r0:r1, :] = x
        return _ln(x, unit=False)

    def halves(x):
        x4 = x.reshape(x.shape[0] // 32, 2, 16, LANES)
        return [x4[:, e].reshape(x.shape[0] // 2, LANES) for e in range(2)]

    def weave(top, bot):
        n = top.shape[0] // 16
        return jnp.stack([top.reshape(n, 16, LANES), bot.reshape(n, 16, LANES)], axis=1).reshape(32 * n, LANES)

    def row_ops(cols, tks=None):
        hv = [halves(x) for x in cols]
        if tks is not None:
            tk = jnp.stack(tks)

            def held(x):
                x4 = x.reshape(len(tks), 2, 8, LANES)
                return jnp.stack([after(tk, x4[:, 0]), x4[:, 1]], axis=1).reshape(x.shape)

            for k2 in range(2):
                hv[k2][0] = held(hv[k2][0])
                hv[2 + k2][1] = held(hv[2 + k2][1])
        per = [_lhs_ops(hv[k2][0], hv[2 + k2][0], hv[k2][1], hv[2 + k2][1]) + [hv[2 + k2][0], hv[k2][1]]
               for k2 in range(2)]
        return [[per[0][o], per[1][o]] for o in range(9)] + [hv[NC - 1]]

    def stage_p2(r0, r1, nx, mb, blockwise=False):
        h = nx * mb[0] + mb[1]
        h_s[r0:r1, :] = h
        zn = _ln(h, 4.0 * EPS)
        if not blockwise:
            store_bf16(z_s, r0, zn)
            return
        ops = row_ops([zn[:, c * LANES:(c + 1) * LANES] for c in range(NC)])
        for o in range(10):
            for e in range(2):
                lo_s[o, e, r0 // 2:r1 // 2, :] = ops[o][e].astype(BF16)

    def stage_p(t, toks, free):
        lo, hi = A0[t], A0[t + 1]
        stage_p2(lo, hi, stage_p1(lo, hi, pick(toks, (hi - lo) // 8, free), mods_a()), mods_b(), t in STR1)

    def square_ops(src, dst, toks):
        HK = 2 * LANES
        ng = HK // 16
        for n2 in range(2):
            tk = jnp.stack([toks[((n2 * ng + r) * len(toks)) // (2 * ng)] for r in range(ng)])

            def blk(c, k, hold_it):
                x = src[c, k * HK:(k + 1) * HK, :].astype(F32)
                if not hold_it:
                    return x
                x4 = x.reshape(ng, 2, 8, LANES)
                return jnp.stack([after(tk, x4[:, 0]), x4[:, 1]], axis=1).reshape(HK, LANES)

            for o, x in enumerate(_rhs_ops(blk(n2, 0, True), blk(2 + n2, 0, False), blk(n2, 1, False), blk(2 + n2, 1, True))):
                if o not in (1, 4):
                    dst[o, n2] = x.astype(BF16)

    def block_dots(lhs_of, w_ref, s_ref, parts, emit, WL, WH):
        w_u, s_u = w_ref.bitcast(U32), s_ref.bitcast(U32)
        toks = []

        def timed(x, weight):
            toks.extend(x[8 * r:8 * r + 8, 0:LANES] for r in range(x.shape[0] // 8) for _ in range(weight))
            return x

        def main(get):
            m = [None] * 7
            rem = [None, None]
            for o in ('t', 2, 4, 'b', 1, 3, 0, 6, 5):
                if o in ('t', 'b'):
                    e = 0 if o == 't' else 1
                    rhs = jnp.concatenate([w_u[c, 2 * LANES:D // 2, :] for c in range(NC - 1)], axis=1)
                    rem[e] = timed(_dot(get([(9, e)]), _as_bf16(rhs)), WL)
                    continue
                if o in (1, 4):
                    d = (1, 4).index(o)
                    rhs = jnp.concatenate([w_u[2 * d + n2, d * LANES:(d + 1) * LANES, :] for n2 in range(2)], axis=1)
                else:
                    rhs = jnp.concatenate([s_u[o, n2] for n2 in range(2)], axis=1)
                m[o] = timed(_dot(get([(o, 0), (o, 1)]), _as_bf16(rhs)), WH if o in (4, 3, 6, 5) else WL)
            c11, c12, c21, c22 = _combine(m)
            top = jnp.concatenate([c11, c12], axis=1) + rem[0]
            bot = jnp.concatenate([c21, c22], axis=1) + rem[1]
            return [weave(top[:, c * LANES:(c + 1) * LANES], bot[:, c * LANES:(c + 1) * LANES]) for c in range(NC - 1)]

        def last(get):
            w4c = _as_bf16(w_u[NC - 1])
            return weave(timed(_dot(get([(2, 0), (2, 1), (7, 0), (7, 1), (9, 0)]), w4c), WL),
                         timed(_dot(get([(8, 0), (8, 1), (3, 0), (3, 1), (9, 1)]), w4c), WL))

        marks = []
        for j, part in enumerate(parts):
            get = lhs_of(part, toks[marks[-1]:] if marks else None)
            marks.append(len(toks))
            if j % 2:
                tail = last(get)
                cols = main(get) + [tail]
            else:
                cols = main(get) + [last(get)]
            emit(part, cols)
        return toks

    def filler(t):
        if DUM:
            red = jnp.sum(y_s[t, 0:8 * DUM, :], axis=-1, keepdims=True).reshape(DUM, 8, 1)
            zf_s[1, (NC - 1) * (TQ + 8) + 8 * t:(NC - 1) * (TQ + 8) + 8 * t + 8, :] = jnp.broadcast_to(jnp.sum(red, axis=0), (8, LANES))

    def chunks(r0, r1, k, unit=16):
        n = (r1 - r0) // unit
        cuts = [r0 + unit * ((n * j) // k) for j in range(k + 1)]
        return list(zip(cuts[:-1], cuts[1:]))

    def stage_m1(t, k):
        def emit(part, cols):
            out = [_gelu2(x) for x in cols]
            for c in range(NC):
                h1_s[c, part[0] + 8:part[1] + 8, :] = out[c]
            return out

        if t in STR1:
            def lhs_of(part, _):
                return lambda keys: _as_bf16(jnp.concatenate(
                    [lo_u[o, e, part[0] // 4:part[1] // 4, :] for o, e in keys], axis=1))
            return block_dots(lhs_of, w1_v, s1_s, chunks(A0[t], A0[t + 1], k, 32), emit, WL, WH)
        toks = []
        for r0, r1 in chunks(A0[t], A0[t + 1], k):
            pre = _dot(load_bf16(z_u, r0, r1 - r0), packed(w1_v))
            out = emit((r0, r1), [pre[:, c * LANES:(c + 1) * LANES] for c in range(NC)])
            toks += [x for x in tokens_of(jnp.concatenate(out, axis=1)) for _ in range(W1N)]
        return toks

    grp = D // 4
    shifts = (-1, 1, -2, 2)

    def shifted(r0, r1):
        n = r1 - r0
        lane = lax.broadcasted_iota(jnp.int32, (n, LANES), 1)
        cols = []
        for c in range(NC):
            lo, hi = c * LANES, (c + 1) * LANES
            g_lo, g_hi = lo // grp, (hi - 1) // grp
            val = h1_s[c, pl.ds(r0 + 8 + shifts[g_lo], n), :]
            if g_hi != g_lo:
                other = h1_s[c, pl.ds(r0 + 8 + shifts[g_hi], n), :]
                val = jnp.where(lane < (g_hi * grp - lo), val, other)
            cols.append(val)
        return cols

    def stage_m2(t, k, before=None):
        def emit(part, cols):
            x1 = h_s[part[0]:part[1], :] + jnp.concatenate(cols, axis=1)
            h_s[part[0]:part[1], :] = x1
            return x1

        if t in STR2:
            def lhs_of(part, prev):
                prev = before if prev is None else prev
                prev = prev[len(prev) // 8:(len(prev) * 7) // 8]
                ops = row_ops(shifted(*part), pick(prev, (part[1] - part[0]) // 32, 0))
                for o in range(10):
                    for e in range(2):
                        l2_s[o, e, part[0] // 2:part[1] // 2, :] = ops[o][e].astype(BF16)
                return lambda keys: _as_bf16(jnp.concatenate(
                    [l2_u[o, e, part[0] // 4:part[1] // 4, :] for o, e in keys], axis=1))
            return block_dots(lhs_of, w2_v, s2_s, chunks(B0[t], B0[t + 1], k, 32), emit, WM2, WM2)
        toks = []
        for r0, r1 in chunks(B0[t], B0[t + 1], k):
            hs = _dot(jnp.concatenate(shifted(r0, r1), axis=1).astype(BF16), packed(w2_v))
            toks += [x for x in tokens_of(emit((r0, r1), [hs])) for _ in range(W2N)]
        return toks

    TQ = TB // 4
    NT = S // TB
    GB = NH

    def blk_rows(b):
        return slice(b * (TQ + 8), b * (TQ + 8) + TQ)

    def store_z(r0, slot, toks, free):
        zn = _ln(hold(h_s[pl.ds(r0, TB), :], pick(toks, TB // 8, free)), 4.0 * EPS)
        for rq in range(4):
            for c in range(NC - 1):
                zf_s[slot, blk_rows(NC * rq + c), :] = zn[rq * TQ:(rq + 1) * TQ, c * LANES:(c + 1) * LANES]
        zr_s[...] = zn[:, (NC - 1) * LANES:].astype(BF16)

    def outer_lhs(i, blk):
        terms = ((0, 0, 1, 1, 1), (1, 0, 1, 1, 1), (0, 0), (1, 1), (0, 0, 1, 0, 1), (1, 0, -1, 0, 0), (0, 1, -1, 1, 1))[i]
        x = blk(terms[0], terms[1])
        if len(terms) > 2:
            y = blk(terms[3], terms[4])
            x = x + y if terms[2] > 0 else x - y
        return x

    def z_ops(slot_of, toks):
        ng = TQ // 16

        def held(x, k):
            tk = jnp.stack([toks[((k * ng + r) * len(toks)) // (7 * ng)] for r in range(ng)])
            x4 = x.reshape(ng, 2, 8, LANES)
            return jnp.stack([after(tk, x4[:, 0]), x4[:, 1]], axis=1).reshape(TQ, LANES)

        for k, i in enumerate(ZORD):
            slot = slot_of()
            so = [outer_lhs(i, lambda r1, k1: zf_s[slot, blk_rows(NC * (2 * r1 + r2) + 2 * k1 + k2), :])
                  for r2 in range(2) for k2 in range(2)]
            for j, x in enumerate(_lhs_ops(held(so[0], k), so[1], so[2], held(so[3], k))):
                la_s[i, j] = x.astype(BF16)

    NS = NH // 2

    RAW = (1, 4)

    def weight_ops(src, dst, ext, transposed, toks):
        ng = LANES // 16
        lead = 2 if ext is not None else 0
        total = (NS * 7 + lead) * ng

        def tile(c, n):
            return src[c, n * LANES:(n + 1) * LANES, :].astype(F32)

        def held(x, pos, step):
            tk = jnp.stack([toks[((pos + r * step) * len(toks)) // total] for r in range(ng)])
            x4 = x.reshape(ng, 2, 8, LANES)
            return jnp.stack([after(tk, x4[:, 0]), x4[:, 1]], axis=1).reshape(LANES, LANES)

        def outer(c2, n, pos=None):
            b11, b22 = tile(c2, n), tile(2 + c2, NH + n)
            if pos is not None:
                b11, b22 = held(b11, pos, 1), held(b22, pos, 1)
            e1, e2 = tile(c2, NH + n), tile(2 + c2, n)
            return _rhs_ops(b11, e1, e2, b22) if transposed else _rhs_ops(b11, e2, e1, b22)

        for c2 in range(2 if ext is not None else 0):
            for i, x in enumerate(outer(c2, NH - 1, c2 * ng)):
                if i not in RAW:
                    ext[i, c2] = x.astype(BF16)
        for st in range(NS):
            t00, t11 = outer(0, 2 * st), outer(1, 2 * st + 1)
            t01, t10 = outer(0, 2 * st + 1), outer(1, 2 * st)
            for k, i in enumerate((1, 5, 2, 4, 0, 3, 6)):
                pos = (lead + st * 7) * ng + k
                a, d = held(t00[i], pos, 7), held(t11[i], pos, 7)
                ops = _rhs_ops(a, t01[i], t10[i], d) if transposed else _rhs_ops(a, t10[i], t01[i], d)
                for j, x in enumerate(ops):
                    if i not in RAW or j not in RAW:
                        dst[i, j, st * LANES:(st + 1) * LANES, :] = x.astype(BF16)

    LQ = (FF - 2 * NS * 2 * LANES) // 4
    LCUT = (NH - 1) * LANES

    def left_rows(ref, c, lo, hi, shift):
        parts = []
        if lo < LANES:
            parts.append(ref[c, (LCUT + lo) >> shift:(LCUT + min(hi, LANES)) >> shift, :])
        if hi > LANES:
            base = (2 * NH - 2) * LANES
            parts.append(ref[c, (base + max(lo, LANES)) >> shift:(base + hi) >> shift, :])
        return parts

    def left_ops(toks):
        ng = LQ // 16

        def blk(c, qd):
            return jnp.concatenate([x.astype(F32) for x in left_rows(w3_v, c, qd * LQ, (qd + 1) * LQ, 0)], axis=0)

        def outer(k2, p):
            return _rhs_ops(blk(k2, p), blk(k2, 2 + p), blk(2 + k2, p), blk(2 + k2, 2 + p))

        t00, t01, t10, t11 = outer(0, 0), outer(0, 1), outer(1, 0), outer(1, 1)
        for k, i in enumerate((1, 5, 2, 4, 0, 3, 6)):
            tk = jnp.stack([toks[((k + r * 7) * len(toks)) // (7 * ng)] for r in range(ng)])

            def held(x):
                x4 = x.reshape(ng, 2, 8, LANES)
                return jnp.stack([after(tk, x4[:, 0]), x4[:, 1]], axis=1).reshape(LQ, LANES)

            for j, x in enumerate(_rhs_ops(held(t00[i]), t01[i], t10[i], held(t11[i]))):
                sl_s[i, j] = x.astype(BF16)

    WORD = [NH - 1, 2 * NH - 1] + [h * NH + 2 * st + p for st in range(NS) for h in range(2) for p in range(2)]
    CQ = LANES // 4

    def transpose_w4(toks):
        w_u = w4_v.bitcast(U32)
        order = [(c, n) for n in WORD for c in range(NC)]
        for k, (c, n) in enumerate(order):
            x = w_u[c, n * (LANES // 2):(n + 1) * (LANES // 2), :]
            if XTOK:
                x = hold(x, [toks[(k * len(toks)) // len(order)]], True)
            wt_s[c, n * LANES:(n + 1) * LANES, :] = _as_bf16(x).astype(F32).T.astype(BF16)

    def col_ops(late):
        nt = 2 * NH
        wt = [wt_s[NC - 1, n * LANES:(n + 1) * LANES, :].astype(F32) for n in range(nt)]
        HC = 2 * CQ
        for i, x in enumerate(_rhs_ops(wt[NH - 1][0:HC], wt[NH - 1][HC:], wt[nt - 1][0:HC], wt[nt - 1][HC:])):
            ec_s[i] = x.astype(BF16)
        for st in range(NS):
            def outer(p, e):
                blk = lambda h, d: wt[h * NH + 2 * st + p][(2 * d + e) * CQ:(2 * d + e + 1) * CQ]
                return _rhs_ops(blk(0, 0), blk(0, 1), blk(1, 0), blk(1, 1))

            t00, t01, t10, t11 = outer(0, 0), outer(0, 1), outer(1, 0), outer(1, 1)
            for k, i in enumerate((1, 5, 2, 4, 0, 3, 6)):
                tk = jnp.stack([late[((st * 7 + k) * len(late)) // (NS * 7)]] * (CQ // 16))

                def held(x):
                    x4 = x.reshape(CQ // 16, 2, 8, LANES)
                    return jnp.stack([after(tk, x4[:, 0]), x4[:, 1]], axis=1).reshape(CQ, LANES)

                for j, x in enumerate(_rhs_ops(held(t00[i]), t01[i], t10[i], held(t11[i]))):
                    sc_s[i, j, st] = x.astype(BF16)

    HL = LANES // 2
    w3_u = w3_v.bitcast(U32)
    zr_u = zr_s.bitcast(U32)
    HEAD = [(3, NH + 2 * st + 1) for st in range(NS)] + [(r2, NH + p) for r2 in range(2) for p in range(2)][:NHEAD]

    def z_last(rq):
        return _as_bf16(zr_u[rq * (TQ // 2):(rq + 1) * (TQ // 2), :])

    def rem3(rq, n):
        return _dot_nt(z_last(rq), _as_bf16(w3_u[NC - 1, n * HL:(n + 1) * HL, :]))

    def lead_in():
        w_left = _as_bf16(jnp.concatenate(left_rows(w3_u, NC - 1, 0, 4 * LQ, 1), axis=0))
        left = [_dot_nt(w_left, z_last(rq)) for rq in range(4)]
        for rq in range(4):
            rl_s[rq] = left[rq]
        for k, key in enumerate(HEAD):
            rh_s[k] = rem3(*key)
        return [left[0][8 * r:8 * r + 8, :] for r in range(LQ // 2)]

    with jax.named_scope("r0a"):
        wait_all(first[:1])
        conv_round(0, 'k', False, False)
    with jax.named_scope("r0_wait"):
        wait_all(first[1:])
    with jax.named_scope("r0b"):
        start_all(conv_copies(2) + conv_copies(3) + conv_copies(4))
        conv_round(0, 'u', False, False)
    with jax.named_scope("r1a"):
        wait_all(second[:1])
        conv_round(1, 'k', True, False)
    with jax.named_scope("r1_wait"):
        wait_all(second[1:])
    with jax.named_scope("r1b"):
        start_all(wm_copies[0] + q_copies[0] + wm_copies[1] + w_copies[0])
        conv_round(1, 'u', False, False)

    def full_round(c, carry):
        wait_all(conv_copies(c))
        conv_round(c, 'ku', True, True)
        return carry

    with jax.named_scope("r234"):
        lax.fori_loop(2, NC, full_round, 0)
    with jax.named_scope("r5"):
        start_all(q_copies[1] + w_copies[1] + sum(q_copies[2:], []) + w_copies[2] + w_copies[3] + wm_copies[2], 1)
        conv_round(NC, '', True, True)
    with jax.named_scope("r6_wait"):
        wait_all(wm_copies[0] + q_copies[0])
    with jax.named_scope("r6"):
        for j in range(3):
            mod_chunk(j)
        conv_round(NC + 1, '', False, True)
        nx0 = stage_p1(0, A0[1], [None], mods_a())
    with jax.named_scope("p2_wait"):
        wait_all(wm_copies[1])
    with jax.named_scope("p2"):
        mod_chunk(4)
        mod_chunk(3)
        stage_p2(0, A0[1], nx0, mods_b())
    with jax.named_scope("w1_wait"):
        wait_all(w_copies[0])
    with jax.named_scope("m1_0"):
        toks = stage_m1(0, 4)
        if STR1:
            square_ops(w1_v, s1_s, toks[:len(toks) - 20 * W1N])
    with jax.named_scope("w2_wait"):
        wait_all(q_copies[1] + w_copies[1])
    with jax.named_scope("m2_0"):
        toks = stage_m2(0, 4)
        stage_p(1, toks[:len(toks) - TRIM * W2N], FREE * W2N)
        if STR2 and min(STR2) == 1:
            square_ops(w2_v, s2_s, toks[len(toks) // 2:len(toks) - 10 * W2N])
        filler(0)
    for t in range(1, NA):
        with jax.named_scope("a%d" % t):
            if t + 1 < NA:
                wait_all(q_copies[t + 1])
            else:
                wait_all(w_copies[2] + w_copies[3] + wm_copies[2])
            t1 = stage_m1(t, SPLIT)
            t2 = stage_m2(t, SPLIT, t1[len(t1) - len(t1) // SPLIT:])

            def weighted(trim):
                return t1 + t2[:len(t2) - trim * W2N]

            if t + 1 < NA:
                stage_p(t + 1, weighted(TRIM), FREE * W2N)
            if STR2 and t == W2P:
                square_ops(w2_v, s2_s, weighted(10))
            if t == NA - 1 - LAT:
                toks = weighted(TRIM // 2)
                store_z(0, 0, toks if LAT and not ZE else toks[:len(toks) // 2], FREE * W2N)
                if ZE:
                    toks = weighted(10)
                    z_ops(lambda: 0, toks[(len(toks) * 5) // 8:])
            if t == NA - 1:
                if not VMOD:
                    mod_chunk(NC)
                toks = weighted(0) + [x for x in lead_in() for _ in range(WE)]
                cut0 = (len(toks) * CUT) // 800
                cut = (len(toks) * CUT) // 100
                left_ops(toks[:cut0])
                if VMOD:
                    ng = D // 8
                    col = after(jnp.stack(pick(toks[:(len(toks) * 9) // 10], ng, 0)), scol_s[...].reshape(ng, 8, LANES))
                    for c in range(NC):
                        wf = wm_v[:, (NC * NC + c) * LANES:(NC * NC + c + 1) * LANES].astype(F32).reshape(ng, 8, LANES)
                        acc = col[0] * wf[0]
                        for r in range(1, ng):
                            acc = acc + col[r] * wf[r]
                        mod_s[NC, :, c * LANES:(c + 1) * LANES] = jnp.broadcast_to(
                            jnp.sum(acc, axis=0, keepdims=True), (8, LANES))
                weight_ops(w3_v, s3_s, None, True, toks[cut0:cut])
                transpose_w4(toks[:(len(toks) * XEND) // 100])
                weight_ops(wt_s, s4_s, e4_s, False, toks[cut:])
                col_ops(toks[cut:])
                if not ZE:
                    z_ops(lambda: 0, toks if LAT else toks[(len(toks) * 5) // 8:])
            if t + 1 < NA or not LAT:
                filler(t)

    gb = 0.5 * mod_s[NC, 0:1, :]
    w3_u, w4_u, s3_u, s4_u, e4_u = (r.bitcast(U32) for r in (w3_v, wt_s, s3_s, s4_s, e4_s))
    HL = LANES // 2
    la_u = la_s.bitcast(U32)
    zr_u = zr_s.bitcast(U32)
    sl_u = sl_s.bitcast(U32)
    sc_u = sc_s.bitcast(U32)
    ec_u = ec_s.bitcast(U32)

    def out_copy(r0, n, c):
        rows = pl.ds(r0, n)
        return pltpu.make_async_copy(o_v.at[c, rows, :], o_hbm.at[rows, pl.ds(c * LANES, LANES)], sem_o.at[0])

    def one_level(w_u, e_u, i, c2):
        if i not in RAW:
            return e_u[i, c2]
        d = RAW.index(i)
        n = d * NH + NH - 1
        return w_u[2 * d + c2, n * HL:(n + 1) * HL, :]

    def two_level(w_u, s_u, i, j, st):
        if i not in RAW or j not in RAW:
            return s_u[i, j, st * HL:(st + 1) * HL, :]
        d, e = RAW.index(i), RAW.index(j)
        n = d * NH + 2 * st + e
        return w_u[2 * d + e, n * HL:(n + 1) * HL, :]

    def loop_b(t, carry):
        r0 = pl.multiple_of(t * TB, TB)
        ws = t & 1

        count = [0]

        def fresh():
            count[0] += 1
            return lax.rem(t + 2 * count[0], 2)

        ltoks, ftoks = [], []

        def light(x):
            ltoks.extend(x[8 * r:8 * r + 8, 0:LANES] for r in range(x.shape[0] // 8))

        def put_g(rq, n, pre):
            g_s[2 * (rq // 2) + n // NH][ws, blk_rows(GB * (rq % 2) + n % NH), :] = _gelu2(pre)

        rem = {}
        for k, key in enumerate(HEAD):
            rem[key] = rh_s[k]
        rem_left = [rl_s[rq] for rq in range(4)]
        for st in range(NS):
            early = LASTO and st == NS - 1
            todo = [(2 * r1 + r2, h * NH + 2 * st + p)
                    for r1, h in (((0, 0), (1, 0), (0, 1), (1, 1)) if early else ((0, 1), (1, 0), (0, 0), (1, 1)))
                    for r2 in range(2) for p in range(2)]
            todo = [x for x in todo if x not in rem]
            for key in todo[:-7]:
                rem[key] = rem3(*key)
            if st >= LSETS:
                light(rem[todo[1]])
                light(rem[todo[5]])
            todo = todo[-7:]
            pin = [None] * 7
            pil = [None] * 7
            for i in ((4, 3, 0, 6, 1, 2, 5) if early else _ORDER):
                m = [None] * 7
                ml = [None] * 7
                for group in (_ORDER[:4], _ORDER[4:]):
                    for j in group:
                        m[j] = _dot_nt(_as_bf16(la_u[i, j]), _as_bf16(two_level(w3_u, s3_u, i, j, st)))
                    if len(group) == 3:
                        key = todo.pop(0)
                        rem[key] = rem3(*key)
                    if st == 0:
                        for j in group:
                            ml[j] = _dot_nt(_as_bf16(sl_u[i, j]), _as_bf16(la_u[i, j]))
                if st >= LSETS and i in ((4, 3, 0) if early else (2, 1, 0)):
                    light(m[_ORDER[1]])
                    light(m[_ORDER[5]])
                pin[i] = _combine(m)
                if st == 0:
                    pil[i] = _combine(ml)
            for inner in range(4):
                for blk, cval in enumerate(_combine([pin[i][inner] for i in range(7)])):
                    rq, n = 2 * (blk // 2) + inner // 2, (blk % 2) * NH + 2 * st + inner % 2
                    put_g(rq, n, cval + rem[rq, n])
            if st == 0:
                cl = [_combine([pil[i][inner] for i in range(7)]) for inner in range(4)]
                for rq in range(4):
                    r1, r2 = rq // 2, rq % 2
                    gt = _gelu2(jnp.concatenate([cl[2 * r2 + p][2 * r1 + h] for h in range(2) for p in range(2)], axis=0)
                                + rem_left[rq])
                    g_s[2 * r1][ws, blk_rows(GB * r2 + NH - 1), :] = gt[0:LANES].T
                    g_s[2 * r1 + 1][ws, blk_rows(GB * r2 + NH - 1), :] = jnp.concatenate(
                        [gt[LANES:], jnp.zeros((FP - FF, TQ), F32)], axis=0).T

        nxt = jnp.minimum(t + 1, NT - 1)
        store_z(pl.multiple_of(nxt * TB, TB), ws, ltoks[LN0::LSTEP], 0)
        if DUMB:
            filler(4)

        toks = []

        def timed(x):
            toks.extend(x[8 * r:8 * r + 8, 0:LANES] for r in range(x.shape[0] // 8))
            return x

        def finish(rq, c, h2):
            rows = pl.ds(pl.multiple_of(r0 + rq * TQ, TQ), TQ)
            cols = slice(c * LANES, (c + 1) * LANES)
            o_v[c, rows, :] = (x_s[rows, cols] + gb[:, cols] * (h_s[rows, cols] + h2)).astype(BF16)

        def outer_sum(p, blk):
            return (lambda: (p[3] - p[4]) + p[0] + p[6], lambda: p[2] + p[4], lambda: p[1] + p[3],
                    lambda: (p[2] - p[1]) + p[0] + p[5])[blk]()

        QR = LANES + CQ
        pin = [[None] * 4 for _ in range(7)]
        tails = {}
        marks = {}
        done = {_ORDER[1]: 1, _ORDER[3]: 2, _ORDER[5]: 0, _ORDER[6]: 3}
        for i in _ORDER:
            slot = fresh()
            we = _as_bf16(jnp.concatenate(
                [x for c2 in range(2)
                 for x in (one_level(w4_u, e4_u, i, c2), ec_u[i, c2 * (CQ // 2):(c2 + 1) * (CQ // 2), :])], axis=0))
            ex = [_dot_nt(we, outer_lhs(i, lambda r1, h: g_s[2 * r1 + h][slot, blk_rows(GB * r2 + NH - 1), :]).astype(BF16))
                  for r2 in range(2)]
            m = [None] * 7
            for j in _ORDER:
                slot = fresh()
                act = jnp.concatenate(
                    [outer_lhs(j, lambda r2, p: outer_lhs(
                        i, lambda r1, h: g_s[2 * r1 + h][slot, blk_rows(GB * r2 + 2 * st + p), :]))
                     for st in range(NS)], axis=1).astype(BF16)
                wij = jnp.concatenate([jnp.concatenate([two_level(w4_u, s4_u, i, j, st), sc_u[i, j, st]], axis=0)
                                       for st in range(NS)], axis=1)
                m[j] = timed(_dot_nt(_as_bf16(wij), act))
            pin[i] = [x + ex[inner // 2][(inner % 2) * QR:(inner % 2 + 1) * QR]
                      for inner, x in enumerate(_combine(m))]
            marks[i] = len(toks)

        nv = TQ // 8
        for i in _ORDER:
            if i not in done:
                continue
            blk = done[i]
            r1 = blk // 2
            pos = [marks[i] + FLAG]

            def paced(x):
                tk = toks[pos[0]:pos[0] + nv * FSTEP:FSTEP]
                pos[0] += nv * FSTEP
                if len(tk) < nv or not FSTEP:
                    return x
                return after(jnp.stack(tk), x.reshape(nv, 8, LANES)).reshape(TQ, LANES)

            for inner in (1, 2, 0, 3):
                ht = outer_sum([pin[k][inner] for k in range(7)], blk)
                rq, c = 2 * r1 + inner // 2, 2 * (blk % 2) + inner % 2
                finish(rq, c, paced(ht[0:LANES].T))
                tails[rq, c] = ht[LANES:]
            rb = pl.multiple_of(r0 + r1 * 2 * TQ, 2 * TQ)
            for e in range(2):
                out_copy(rb, 2 * TQ, 2 * (blk % 2) + e).start()
            if blk in (0, 3):
                for rq in (2 * r1, 2 * r1 + 1):
                    finish(rq, NC - 1, paced(jnp.concatenate([tails[rq, c] for c in range(NC - 1)], axis=0).T))
                out_copy(rb, 2 * TQ, NC - 1).start()

        z_ops(fresh, toks[ZB0:ZB1])
        lead_in()
        return carry

    with jax.named_scope("ph2b"):
        lax.fori_loop(0, NT, loop_b, 0)
    with jax.named_scope("tail"):
        pltpu.make_async_copy(o_v, o_v, sem_o.at[0]).wait()


@jax.jit
def pallas_adaLN_cond__ssm_conv_h3__mixer_s_mlp__prompt_kernel(
    A_q: jax.Array,
    A_k: jax.Array,
    A_v: jax.Array,
    A_shift_k: jax.Array,
    A_ssm_k: jax.Array,
    A_ssm_D: jax.Array,
    B_x: jax.Array,
    B_w1: jax.Array,
    B_w2: jax.Array,
    B_w3: jax.Array,
    B_w4: jax.Array,
    c: jax.Array,
    w_mod: jax.Array,
):
    B, S, D = A_q.shape
    assert B == 1
    FF = B_w3.shape[1]
    NC = D // LANES
    NG = BLK // 8
    NBL = S // (PH * BLK)
    FP = -(-FF // (2 * LANES)) * 2 * LANES
    TILES = (384, 384, 576, 704)
    assert sum(TILES) == S
    TB = 512

    args = (A_q.reshape(S, D), A_k.reshape(S, D), A_v.reshape(S, D), A_shift_k.T, A_ssm_k,
            A_ssm_D, B_w1, B_w2, B_w3.T, B_w4, c, w_mod)
    scratch = [
        pltpu.VMEM((S, D), BF16),
        pltpu.VMEM((NC, S + KP, LANES), BF16),
        pltpu.VMEM((NC, S + VP, LANES), BF16),
        pltpu.VMEM((4, D), BF16),
        pltpu.VMEM((NC, LANES, S), BF16),
        pltpu.VMEM((D,), BF16),
        pltpu.VMEM((NC, D, LANES), BF16),
        pltpu.VMEM((NC, D, LANES), BF16),
        pltpu.VMEM((NC, FF, LANES), BF16),
        pltpu.VMEM((NC, FP, LANES), BF16),
        pltpu.VMEM((1, D), BF16),
        pltpu.VMEM((D, 6 * D), BF16),
        pltpu.VMEM((PH, 2 * BLK, BLK), BF16),
        pltpu.VMEM((PH, 2, BLK, BLK), BF16),
        pltpu.VMEM((NC, S, LANES), BF16),
        pltpu.VMEM((NC, NG, NBL, PH, 2, 8, LANES), F32),
        pltpu.VMEM((NC, NG, NBL, PH, 2, 8, LANES), F32),
        pltpu.VMEM((NC, NBL, PH, 2 * BLK, LANES), BF16),
        pltpu.VMEM((NBL, PH, BLK, LANES), BF16),
        pltpu.VMEM((NC, S + YP, LANES), F32),
        pltpu.VMEM((6, 8, D), F32),
        pltpu.VMEM((NC, 8, LANES), F32),
        pltpu.VMEM((NC, S + 16, LANES), F32),
        pltpu.VMEM((S, D), F32),
        pltpu.VMEM((S, D), F32),
        pltpu.VMEM((NC, S, LANES), BF16),
        pltpu.VMEM((7, 7, FP // 512 * LANES, LANES), BF16),
        pltpu.VMEM((7, 7, FP // 512 * LANES, LANES), BF16),
        pltpu.VMEM((7, 2, LANES, LANES), BF16),
        [pltpu.VMEM((2, GR, LANES), F32)] * 4,
        pltpu.VMEM((2, ZR, LANES), F32),
        pltpu.VMEM((TB, LANES), BF16),
        pltpu.VMEM((7, 7, TB // 4, LANES), BF16),
        pltpu.VMEM((10, 2, S // 2, LANES), BF16),
        pltpu.VMEM((10, 2, S // 2, LANES), BF16),
        pltpu.VMEM((7, 2, 2 * LANES, LANES), BF16),
        pltpu.VMEM((7, 2, 2 * LANES, LANES), BF16),
        pltpu.VMEM((7, 7, (FF - FP // 512 * 512) // 4, LANES), BF16),
        pltpu.VMEM((7, 7, FP // 512, LANES // 4, LANES), BF16),
        pltpu.VMEM((7, LANES // 2, LANES), BF16),
        pltpu.VMEM((4, FF - FP // 512 * 512, TB // 4), F32),
        pltpu.VMEM((8, TB // 4, LANES), F32),
        pltpu.VMEM((NC, FP, LANES), BF16),
        pltpu.VMEM((D, LANES), F32),
        pltpu.SemaphoreType.DMA((16 + len(TILES),)),
        pltpu.SemaphoreType.DMA((1,)),
    ]
    out = pl.pallas_call(
        functools.partial(_kernel, S=S, D=D, FF=FF, TILES=TILES, TB=TB),
        in_specs=[pl.BlockSpec(memory_space=pl.ANY)] * len(args),
        out_specs=pl.BlockSpec(memory_space=pl.ANY),
        out_shape=jax.ShapeDtypeStruct((S, D), BF16),
        scratch_shapes=scratch,
        compiler_params=pltpu.CompilerParams(
            vmem_limit_bytes=126 * 1024 * 1024,
            disable_bounds_checks=True,
            disable_semaphore_checks=True,
        ),
    )(*args)
    return out.reshape(B, S, D)
```

```python
import functools
import math

import jax
import jax.numpy as jnp
from jax import lax
import jax.experimental.pallas as pl
import jax.experimental.pallas.tpu as pltpu

F32 = jnp.float32
BF16 = jnp.bfloat16
U32 = jnp.uint32

LANES = 128
BLK = 128
PH = 4
EPS = 1e-05
TRIM = 60
SPLIT = 2
FREE = 30
DUM = 96
LN1 = 999
KP = 16
VP = 0
YP = 0
GR = 1928
ZR = 2720
FT = 0
DUMB = 0
STR1 = (3, )
STR2 = (2, 3, )
WL = 3
WH = 2
ZE = 1
PRE = 0
WM2 = 2
W2P = 1
UL = 2
ALN = 0
LN0 = 32
SLAG = 1
NHEAD = 0
XTOK = 1
LASTO = 1
PINJ = ()
FLAG = 10
FSTEP = 1
WE = 2
XEND = 50
CUT = 50
VMOD = 1
LT0 = 8
LT1 = 40
LTW = 3
LQ1 = 2
LQ2 = 3
ZC0 = 320
ZC1 = 450
ZD0 = 600
ZD1 = 730
W1N = 2
W2N = 3
LAT = 1
LSETS = 1
LSTEP = 1
LB1 = 0
ZB0 = 0
ZB1 = 160
REM2 = 2
ZORD = (2, 3, 0, 1, 4, 5, 6)


def _as_bf16(x):
    return pltpu.bitcast(x, BF16)


def _lo(x):
    return pltpu.bitcast(x << 16, F32)


def _hi(x):
    return pltpu.bitcast(x & jnp.uint32(0xFFFF0000), F32)


def _dft4(re, im, sign):
    ar, ai = re[0] + re[2], im[0] + im[2]
    br, bi = re[0] - re[2], im[0] - im[2]
    cr, ci = re[1] + re[3], im[1] + im[3]
    dr, di = re[1] - re[3], im[1] - im[3]
    o0 = (ar + cr, ai + ci)
    o2 = (ar - cr, ai - ci)
    m = (br + di, bi - dr)
    p = (br - di, bi + dr)
    o1, o3 = (m, p) if sign < 0 else (p, m)
    return [o0[0], o1[0], o2[0], o3[0]], [o0[1], o1[1], o2[1], o3[1]]


def _ln(x, eps=EPS, unit=True):
    n = x.shape[-1]
    s1 = jnp.sum(x, axis=-1, keepdims=True)
    m = s1 * (1.0 / n)
    v = jnp.maximum(jnp.sum(x * x, axis=-1, keepdims=True) + (n * eps - s1 * m), n * eps)
    e = jnp.log(v) * (-0.5 / math.log(2.0))
    return (x - m) * jnp.exp2(e + 0.5 * math.log2(n) if unit else e)


def _gelu2(x):
    c0 = math.sqrt(2.0 / math.pi)
    return x + x * jnp.tanh(x * (c0 + (c0 * 0.044715) * (x * x)))


def _dot(a, b):
    return jnp.dot(a, b, preferred_element_type=F32)


def _dot_nt(a, b):
    return lax.dot_general(a, b, (((1,), (1,)), ((), ())), preferred_element_type=F32)


def _lhs_ops(a11, a12, a21, a22):
    return [a11 + a22, a21 + a22, a11, a22, a11 + a12, a21 - a11, a12 - a22]


def _rhs_ops(b11, b12, b21, b22):
    return [b11 + b22, b11, b12 - b22, b21 - b11, b22, b11 + b12, b21 + b22]


def _combine(m):
    return (m[3] - m[4]) + m[0] + m[6], m[2] + m[4], m[1] + m[3], (m[2] - m[1]) + m[0] + m[5]


_ORDER = (2, 4, 1, 3, 0, 6, 5)


def _kernel(q_hbm, k_hbm, v_hbm, sh_hbm, sk_hbm, sd_hbm, w1_hbm, w2_hbm, w3_hbm, w4_hbm, c_hbm, wm_hbm,
            o_hbm,
            q_v, k_v, v_v, sh_v, sk_v, sd_v, w1_v, w2_v, w3_v, w4_v, c_v, wm_v,
            fw_s, iv_s, o_v, u_s, kk_s, vv_s, wu_s, y_s, mod_s, par_s, h1_s, x_s, h_s, z_s, s3_s, s4_s, e4_s, g_s, zf_s, zr_s, lo_s, l2_s, s1_s, s2_s, sl_s, sc_s, ec_s, rh_s, wt_s, scol_s,
            sem, sem_o,
            *, S, D, FF, TILES, TB):
    NC = D // LANES
    NG = BLK // 8
    LB = PH * BLK
    NBL = S // LB
    R = BLK // PH
    HALO = 32
    FP = wt_s.shape[1]
    FH = FP // 2
    NH = FH // LANES

    small = [
        pltpu.make_async_copy(sh_hbm, sh_v, sem.at[0]),
        pltpu.make_async_copy(sd_hbm, sd_v, sem.at[0]),
        pltpu.make_async_copy(c_hbm, c_v, sem.at[0]),
    ]

    def conv_copies(c):
        col = pl.ds(c * LANES if isinstance(c, int) else pl.multiple_of(c * LANES, LANES), LANES)
        return [
            pltpu.make_async_copy(sk_hbm.at[col, :], sk_v.at[c], sem.at[9 + c if isinstance(c, int) and c < 2 else 1 + c]),
            pltpu.make_async_copy(k_hbm.at[:, col], k_v.at[c, pl.ds(16, S), :], sem.at[1 + c]),
            pltpu.make_async_copy(v_hbm.at[:, col], v_v.at[c, pl.ds(0, S), :], sem.at[1 + c]),
        ]

    def col_copies(src, dst, c0, s):
        rows = pl.ds(0, src.shape[0])
        return [pltpu.make_async_copy(src.at[:, pl.ds((c0 + c) * LANES, LANES)], dst.at[c0 + c, rows, :], sem.at[s])
                for c in range(NC)]

    WM = (0, 3 * D, 5 * D, 6 * D)
    wm_copies = [[pltpu.make_async_copy(wm_hbm.at[:, pl.ds(WM[j], WM[j + 1] - WM[j])],
                                        wm_v.at[:, pl.ds(WM[j], WM[j + 1] - WM[j])], sem.at[6 + j])]
                 for j in range(3)]
    w_copies = [col_copies(src, dst, 0, 12 + j)
                for j, (src, dst) in enumerate(((w1_hbm, w1_v), (w2_hbm, w2_v), (w3_hbm, w3_v), (w4_hbm, w4_v)))]

    B0 = [0]
    for n in TILES:
        B0.append(B0[-1] + n)
    NA = len(TILES)
    A0 = [0] + [r + HALO for r in B0[1:-1]] + [S]
    q_copies = [
        [pltpu.make_async_copy(q_hbm.at[pl.ds(A0[t], A0[t + 1] - A0[t])], q_v.at[pl.ds(A0[t], A0[t + 1] - A0[t])],
                               sem.at[16 + t])]
        for t in range(NA)
    ]

    def start_all(cps, priority=0):
        for cp in cps:
            cp.start(priority=priority)

    def wait_all(cps):
        for cp in cps:
            cp.wait()

    def packed(ref, c0=0):
        ru = ref.bitcast(U32)
        return _as_bf16(jnp.concatenate([ru[c0 + c] for c in range(NC)], axis=1))

    first, second = conv_copies(0), conv_copies(1)
    start_all(first[:1] + small + first[1:] + second)

    for c in range(NC):
        k_v[c, 0:16, :] = jnp.zeros((16, LANES), BF16)
        h1_s[c, 0:8, :] = jnp.zeros((8, LANES), F32)
        h1_s[c, S + 8:S + 16, :] = jnp.zeros((8, LANES), F32)

    prow = lax.broadcasted_iota(jnp.int32, (BLK, BLK), 0)
    pcol = lax.broadcasted_iota(jnp.int32, (BLK, BLK), 1)
    ang = (((4 * prow + 1) * pcol) & (4 * BLK - 1)).astype(F32) * (2.0 * math.pi / (4 * BLK))
    tw = (4 * prow + 1).astype(F32) * (2.0 * math.pi / (4 * LB))
    mr, mi = jnp.cos(ang), -jnp.sin(ang)
    zr_, zi_ = jnp.cos(tw), -jnp.sin(tw)
    eye = jnp.where(prow == pcol, 1.0 / LB, 0.0).astype(BF16)
    for i in range(PH):
        both = jnp.stack([mr.reshape(NG, 8, BLK), mi.reshape(NG, 8, BLK)], axis=1).reshape(2 * BLK, BLK)
        fw_s[i] = both.astype(BF16)
        for h in range(2):
            iv_s[i, h] = _dot_nt(eye, both[h * BLK:(h + 1) * BLK, :].astype(BF16)).astype(BF16)
        if i + 1 < PH:
            mr, mi = mr * zr_ - mi * zi_, mr * zi_ + mi * zr_
    perm = jnp.where(pcol == (prow % R) * PH + prow // R, 1.0, 0.0).astype(BF16)
    fw_u = fw_s.bitcast(U32)
    iv_u = iv_s.bitcast(U32)

    wait_all(small)
    shf = sh_v[...].astype(F32)
    sdf = sd_v[...].astype(F32).reshape(1, D)
    for c in range(NC):
        par_s[c, 0:4, :] = shf[:, c * LANES:(c + 1) * LANES]
        par_s[c, 4:5, :] = sdf[:, c * LANES:(c + 1) * LANES]
    cf = c_v[...].astype(F32)
    sc = (cf * jax.nn.sigmoid(cf)).astype(BF16)
    sc16 = jnp.broadcast_to(sc, (16, D))

    scol_s[...] = jnp.broadcast_to(sc.astype(F32), (LANES, D)).T

    def mod_chunk(j):
        mod_s[j] = _dot(sc16, wm_v[:, j * D:(j + 1) * D])[0:8, :]

    k_u = k_v.bitcast(U32)
    v_u = v_v.bitcast(U32)
    wu_u = wu_s.bitcast(U32)
    z_u = z_s.bitcast(U32)
    vv_u = vv_s.bitcast(U32)
    lo_u = lo_s.bitcast(U32)
    l2_u = l2_s.bitcast(U32)

    never = zr_[0:8, :] > 2.0

    def after(token, x):
        if token.dtype != x.dtype:
            token = pltpu.bitcast(token, x.dtype)
        return jnp.where(jnp.broadcast_to(never, x.shape), token, x)

    def split(t):
        t4 = t.reshape(NG, 2, 8, LANES)
        return t4[:, 0], t4[:, 1]

    def perm_k(c, b, toks):
        kt = [_dot_nt(perm, sk_v[c, :, b * LB + t * BLK:b * LB + (t + 1) * BLK]) for t in range(PH)]
        for r in range(BLK // 16):
            toks.append(kt[0][16 * r:16 * r + 8, :])
        return [jnp.concatenate([kt[t][i * R:(i + 1) * R, :] for t in range(PH)], axis=0).astype(BF16)
                for i in range(PH)]

    def spectrum(wts, dst, c, b, toks, dc=None, pins=None):
        tr, ti = [], []
        for i in range(PH):
            lhs = fw_u[i]
            if pins is not None and i < len(pins):
                lhs = after(pins[i], lhs.reshape(NG, 8, LANES)).reshape(BLK, LANES)
            r_, i_ = split(_dot(_as_bf16(lhs), wts[i]))
            tr.append(r_)
            ti.append(i_)
        for g in range(NG):
            toks.append(ti[PH - 1][g])
        if dc is not None:
            tr[0] = tr[0] + dc
        sr, si = _dft4(tr, ti, -1)
        for qq in range(PH):
            dst[c, :, b, qq, 0] = sr[qq]
            dst[c, :, b, qq, 1] = si[qq]

    def gated(c, b):
        w = [par_s[c, t:t + 1, :] for t in range(4)]
        kc = {}
        for o in range(-2, 2):
            words = k_u[c, pl.ds(8 + b * (LB // 2) + o, BLK, stride=2), :]
            if o > -2:
                kc[2 * o] = _lo(words)
            kc[2 * o + 1] = _hi(words)
        vc = {}
        for o in range(2):
            words = v_u[c, pl.ds(b * (LB // 2) + o, BLK, stride=2), :]
            vc[2 * o] = _lo(words)
            vc[2 * o + 1] = _hi(words)
        for i in range(PH):
            ks = kc[i] * w[0]
            for t in range(1, 4):
                ks = ks + kc[i - t] * w[t]
            wu_s[b, i] = (ks * vc[i]).astype(BF16)
        return [wu_u[b, i] for i in range(PH)]

    def kv_pins(kvb):
        return [jnp.stack([kvb[2 * m + (r % 2)][8 * (r // 2):8 * (r // 2) + 8, :] for r in range(NG)])
                for m in range(2)]

    def mac(c, us, ks, toks):
        zp = None
        for o in range(NBL):
            zr, zi = [], []
            for qq in range(PH):
                accr = acci = None
                for b in range(o + 1):
                    a_, b_ = us[0, :, b, qq, 0], us[0, :, b, qq, 1]
                    c_, d_ = ks[0, :, o - b, qq, 0], ks[0, :, o - b, qq, 1]
                    if qq == 0 and b == o:
                        a_ = after(toks[o], a_)
                    tr_ = a_ * c_ - b_ * d_
                    ti_ = a_ * d_ + b_ * c_
                    accr = tr_ if accr is None else accr + tr_
                    acci = ti_ if acci is None else acci + ti_
                zr.append(accr)
                zi.append(acci)
            if zp is None:
                yr, yi = zr, zi
            else:
                yr = [zr[qq] - zp[1][qq] for qq in range(PH)]
                yi = [zi[qq] + zp[0][qq] for qq in range(PH)]
            zp = (zr, zi)
            vr, vi = _dft4(yr, yi, +1)
            for i in range(PH):
                vv_s[c, o, i] = jnp.stack([vr[i], vi[i]], axis=1).reshape(2 * BLK, LANES).astype(BF16)

    def inverse(c, toks, pins=None):
        HB = BLK // 2
        for o in range(NBL):
            for i in range(PH):
                yv = None
                for h in range(2):
                    lhs = iv_u[i, h]
                    if pins is not None and h == 0:
                        pin = pins[o][i % 2][8 * (i // 2):8 * (i // 2) + 8]
                        lhs = after(pin, lhs.reshape(8, 8, LANES)).reshape(HB, LANES)
                    t = _dot(_as_bf16(lhs), _as_bf16(vv_u[c, o, i, h * HB:(h + 1) * HB, :]))
                    yv = t if yv is None else yv + t
                if i % 2 == 0:
                    for r in range(BLK // 16):
                        toks.append(yv[16 * r:16 * r + 8, :])
                y_s[c, pl.ds(o * LB + i, BLK, stride=PH), :] = yv

    def mac_tokens(toks):
        n = len(toks) - 3
        cum = (44, 128, 244, 392)
        return [jnp.stack([toks[max(0, ((g * 392 + cum[o]) * n) // (392 * NG) - 1)] for g in range(NG)])
                for o in range(NBL)]

    def conv_round(c, fwd, mul, inv):
        toks = []
        kv = pins = None
        cur = 1 if mul else 0
        if fwd or mul:
            win = pl.ds(c - cur, 2 if fwd and mul else 1)
            us, ks = u_s.at[win], kk_s.at[win]
        if 'u' in fwd:
            kv = [gated(c, b) for b in range(NBL)]
            pins = [kv_pins(kv[b]) for b in range(NBL)]
        if inv:
            inverse(c - 2, toks, pins)
            if fwd:
                toks = []
        if 'k' in fwd:
            wts = [perm_k(c, b, toks) for b in range(NBL)]
        for b in range(NBL):
            if 'k' in fwd:
                spectrum(wts[b], ks, cur, b, toks, par_s[c, 4:5, :] if b == 0 else None)
            if 'u' in fwd:
                pin = pins[b + UL] if not inv and b + UL < NBL else None
                spectrum([_as_bf16(x) for x in kv[b]], us, cur, b, toks, None, pin)
        if mul:
            mac(c - 1, us, ks, mac_tokens(toks))

    def tokens_of(x):
        return [x[8 * r:8 * r + 8, c * LANES:(c + 1) * LANES] for c in range(NC) for r in range(x.shape[0] // 8)]

    def store_bf16(ref, r0, x):
        for c in range(NC):
            ref[c, r0:r0 + x.shape[0], :] = x[:, c * LANES:(c + 1) * LANES].astype(BF16)

    def load_bf16(ref_u, r0, n):
        return _as_bf16(jnp.concatenate([ref_u[c, pl.ds(r0 // 2, n // 2), :] for c in range(NC)], axis=1))

    def pick(toks, n, free):
        if toks is None:
            return [None] * n
        idx = [(r * (len(toks) + free)) // n - free for r in range(n)]
        return [toks[i] if i >= 0 else None for i in idx]

    def hold(x, tks, head=False):
        if head:
            return jnp.concatenate([after(tks[0], x[0:8]), x[8:]], axis=0)
        f = len([k for k in tks if k is None])
        n = len(tks)
        if f == n:
            return x
        first = after(jnp.stack(tks[f:]), x[8 * f:, 0:LANES].reshape(n - f, 8, LANES)).reshape(8 * (n - f), LANES)
        if f:
            first = jnp.concatenate([x[:8 * f, 0:LANES], first], axis=0)
        return jnp.concatenate([first, x[:, LANES:]], axis=1)

    def mods_a():
        ga = mod_s[2, 0:1, :]
        return ga * (1.0 + mod_s[1, 0:1, :]) * math.sqrt(D), ga * mod_s[0, 0:1, :]

    def mods_b():
        return (1.0 + mod_s[4, 0:1, :]) * (2.0 * math.sqrt(D)), 2.0 * mod_s[3, 0:1, :]

    def stage_p1(r0, r1, tks, ma):
        q = hold(q_v[r0:r1, :].astype(F32), tks)
        y = jnp.concatenate([y_s[c, r0:r1, :] for c in range(NC)], axis=1)
        x = q + (_ln(q, unit=False) * ma[0] + ma[1]) * y
        x_s[r0:r1, :] = x
        return _ln(x, unit=False)

    def halves(x):
        x4 = x.reshape(x.shape[0] // 32, 2, 16, LANES)
        return [x4[:, e].reshape(x.shape[0] // 2, LANES) for e in range(2)]

    def weave(top, bot):
        n = top.shape[0] // 16
        return jnp.stack([top.reshape(n, 16, LANES), bot.reshape(n, 16, LANES)], axis=1).reshape(32 * n, LANES)

    def row_ops(cols, tks=None):
        hv = [halves(x) for x in cols]
        if tks is not None:
            tk = jnp.stack(tks)

            def held(x):
                x4 = x.reshape(len(tks), 2, 8, LANES)
                return jnp.stack([after(tk, x4[:, 0]), x4[:, 1]], axis=1).reshape(x.shape)

            for k2 in range(2):
                hv[k2][0] = held(hv[k2][0])
                hv[2 + k2][1] = held(hv[2 + k2][1])
        per = [_lhs_ops(hv[k2][0], hv[2 + k2][0], hv[k2][1], hv[2 + k2][1]) + [hv[2 + k2][0], hv[k2][1]]
               for k2 in range(2)]
        return [[per[0][o], per[1][o]] for o in range(9)] + [hv[NC - 1]]

    def stage_p2(r0, r1, nx, mb, blockwise=False):
        h = nx * mb[0] + mb[1]
        h_s[r0:r1, :] = h
        zn = _ln(h, 4.0 * EPS)
        if not blockwise:
            store_bf16(z_s, r0, zn)
            return
        ops = row_ops([zn[:, c * LANES:(c + 1) * LANES] for c in range(NC)])
        for o in range(10):
            for e in range(2):
                lo_s[o, e, r0 // 2:r1 // 2, :] = ops[o][e].astype(BF16)

    def stage_p(t, toks, free):
        lo, hi = A0[t], A0[t + 1]
        stage_p2(lo, hi, stage_p1(lo, hi, pick(toks, (hi - lo) // 8, free), mods_a()), mods_b(), t in STR1)

    def square_ops(src, dst, toks):
        HK = 2 * LANES
        ng = HK // 16
        for n2 in range(2):
            tk = jnp.stack([toks[((n2 * ng + r) * len(toks)) // (2 * ng)] for r in range(ng)])

            def blk(c, k, hold_it):
                x = src[c, k * HK:(k + 1) * HK, :].astype(F32)
                if not hold_it:
                    return x
                x4 = x.reshape(ng, 2, 8, LANES)
                return jnp.stack([after(tk, x4[:, 0]), x4[:, 1]], axis=1).reshape(HK, LANES)

            for o, x in enumerate(_rhs_ops(blk(n2, 0, True), blk(2 + n2, 0, False), blk(n2, 1, False), blk(2 + n2, 1, True))):
                if o not in (1, 4):
                    dst[o, n2] = x.astype(BF16)

    def block_dots(lhs_of, w_ref, s_ref, parts, emit, WL, WH):
        w_u, s_u = w_ref.bitcast(U32), s_ref.bitcast(U32)
        toks = []

        def timed(x, weight):
            toks.extend(x[8 * r:8 * r + 8, 0:LANES] for r in range(x.shape[0] // 8) for _ in range(weight))
            return x

        def main(get):
            m = [None] * 7
            rem = [None, None]
            for o in ('t', 2, 4, 'b', 1, 3, 0, 6, 5):
                if o in ('t', 'b'):
                    e = 0 if o == 't' else 1
                    rhs = jnp.concatenate([w_u[c, 2 * LANES:D // 2, :] for c in range(NC - 1)], axis=1)
                    rem[e] = timed(_dot(get([(9, e)]), _as_bf16(rhs)), WL)
                    continue
                if o in (1, 4):
                    d = (1, 4).index(o)
                    rhs = jnp.concatenate([w_u[2 * d + n2, d * LANES:(d + 1) * LANES, :] for n2 in range(2)], axis=1)
                else:
                    rhs = jnp.concatenate([s_u[o, n2] for n2 in range(2)], axis=1)
                m[o] = timed(_dot(get([(o, 0), (o, 1)]), _as_bf16(rhs)), WH if o in (4, 3, 6, 5) else WL)
            c11, c12, c21, c22 = _combine(m)
            top = jnp.concatenate([c11, c12], axis=1) + rem[0]
            bot = jnp.concatenate([c21, c22], axis=1) + rem[1]
            return [weave(top[:, c * LANES:(c + 1) * LANES], bot[:, c * LANES:(c + 1) * LANES]) for c in range(NC - 1)]

        def last(get):
            w4c = _as_bf16(w_u[NC - 1])
            return weave(timed(_dot(get([(2, 0), (2, 1), (7, 0), (7, 1), (9, 0)]), w4c), WL),
                         timed(_dot(get([(8, 0), (8, 1), (3, 0), (3, 1), (9, 1)]), w4c), WL))

        marks = []
        for j, part in enumerate(parts):
            get = lhs_of(part, toks[marks[-1]:] if marks else None)
            marks.append(len(toks))
            if j % 2:
                tail = last(get)
                cols = main(get) + [tail]
            else:
                cols = main(get) + [last(get)]
            emit(part, cols)
        return toks

    def filler(t):
        if DUM:
            red = jnp.sum(y_s[t, 0:8 * DUM, :], axis=-1, keepdims=True).reshape(DUM, 8, 1)
            zf_s[1, (NC - 1) * (TQ + 8) + 8 * t:(NC - 1) * (TQ + 8) + 8 * t + 8, :] = jnp.broadcast_to(jnp.sum(red, axis=0), (8, LANES))

    def chunks(r0, r1, k, unit=16):
        n = (r1 - r0) // unit
        cuts = [r0 + unit * ((n * j) // k) for j in range(k + 1)]
        return list(zip(cuts[:-1], cuts[1:]))

    def stage_m1(t, k):
        def emit(part, cols):
            out = [_gelu2(x) for x in cols]
            for c in range(NC):
                h1_s[c, part[0] + 8:part[1] + 8, :] = out[c]
            return out

        if t in STR1:
            def lhs_of(part, _):
                return lambda keys: _as_bf16(jnp.concatenate(
                    [lo_u[o, e, part[0] // 4:part[1] // 4, :] for o, e in keys], axis=1))
            return block_dots(lhs_of, w1_v, s1_s, chunks(A0[t], A0[t + 1], k, 32), emit, WL, WH)
        toks = []
        for r0, r1 in chunks(A0[t], A0[t + 1], k):
            pre = _dot(load_bf16(z_u, r0, r1 - r0), packed(w1_v))
            out = emit((r0, r1), [pre[:, c * LANES:(c + 1) * LANES] for c in range(NC)])
            toks += [x for x in tokens_of(jnp.concatenate(out, axis=1)) for _ in range(W1N)]
        return toks

    grp = D // 4
    shifts = (-1, 1, -2, 2)

    def shifted(r0, r1):
        n = r1 - r0
        lane = lax.broadcasted_iota(jnp.int32, (n, LANES), 1)
        cols = []
        for c in range(NC):
            lo, hi = c * LANES, (c + 1) * LANES
            g_lo, g_hi = lo // grp, (hi - 1) // grp
            val = h1_s[c, pl.ds(r0 + 8 + shifts[g_lo], n), :]
            if g_hi != g_lo:
                other = h1_s[c, pl.ds(r0 + 8 + shifts[g_hi], n), :]
                val = jnp.where(lane < (g_hi * grp - lo), val, other)
            cols.append(val)
        return cols

    def stage_m2(t, k, before=None):
        def emit(part, cols):
            x1 = h_s[part[0]:part[1], :] + jnp.concatenate(cols, axis=1)
            h_s[part[0]:part[1], :] = x1
            return x1

        if t in STR2:
            def lhs_of(part, prev):
                prev = before if prev is None else prev
                prev = prev[len(prev) // 8:(len(prev) * 7) // 8]
                ops = row_ops(shifted(*part), pick(prev, (part[1] - part[0]) // 32, 0))
                for o in range(10):
                    for e in range(2):
                        l2_s[o, e, part[0] // 2:part[1] // 2, :] = ops[o][e].astype(BF16)
                return lambda keys: _as_bf16(jnp.concatenate(
                    [l2_u[o, e, part[0] // 4:part[1] // 4, :] for o, e in keys], axis=1))
            return block_dots(lhs_of, w2_v, s2_s, chunks(B0[t], B0[t + 1], k, 32), emit, WM2, WM2)
        toks = []
        for r0, r1 in chunks(B0[t], B0[t + 1], k):
            hs = _dot(jnp.concatenate(shifted(r0, r1), axis=1).astype(BF16), packed(w2_v))
            toks += [x for x in tokens_of(emit((r0, r1), [hs])) for _ in range(W2N)]
        return toks

    TQ = TB // 4
    NT = S // TB
    GB = NH

    def blk_rows(b):
        return slice(b * (TQ + 8), b * (TQ + 8) + TQ)

    def store_z(r0, slot, toks, free, q0=0, q1=4):
        n = (q1 - q0) * TQ
        rows = pl.ds(r0 + q0 * TQ if isinstance(r0, int) else pl.multiple_of(r0 + q0 * TQ, TQ), n)
        zn = _ln(hold(h_s[rows, :], pick(toks, n // 8, free)), 4.0 * EPS)
        for rq in range(q0, q1):
            for c in range(NC - 1):
                zf_s[slot, blk_rows(NC * rq + c), :] = zn[(rq - q0) * TQ:(rq - q0 + 1) * TQ, c * LANES:(c + 1) * LANES]
        zr_s[q0 * TQ:q1 * TQ, :] = zn[:, (NC - 1) * LANES:].astype(BF16)

    def outer_lhs(i, blk):
        terms = ((0, 0, 1, 1, 1), (1, 0, 1, 1, 1), (0, 0), (1, 1), (0, 0, 1, 0, 1), (1, 0, -1, 0, 0), (0, 1, -1, 1, 1))[i]
        x = blk(terms[0], terms[1])
        if len(terms) > 2:
            y = blk(terms[3], terms[4])
            x = x + y if terms[2] > 0 else x - y
        return x

    NS = NH // 2

    RAW = (1, 4)

    def weight_ops(src, dst, ext, transposed, toks):
        ng = LANES // 16
        lead = 2 if ext is not None else 0
        total = (NS * 7 + lead) * ng

        def tile(c, n):
            return src[c, n * LANES:(n + 1) * LANES, :].astype(F32)

        def held(x, pos, step):
            tk = jnp.stack([toks[((pos + r * step) * len(toks)) // total] for r in range(ng)])
            x4 = x.reshape(ng, 2, 8, LANES)
            return jnp.stack([after(tk, x4[:, 0]), x4[:, 1]], axis=1).reshape(LANES, LANES)

        def outer(c2, n, pos=None):
            b11, b22 = tile(c2, n), tile(2 + c2, NH + n)
            if pos is not None:
                b11, b22 = held(b11, pos, 1), held(b22, pos, 1)
            e1, e2 = tile(c2, NH + n), tile(2 + c2, n)
            return _rhs_ops(b11, e1, e2, b22) if transposed else _rhs_ops(b11, e2, e1, b22)

        for c2 in range(2 if ext is not None else 0):
            for i, x in enumerate(outer(c2, NH - 1, c2 * ng)):
                if i not in RAW:
                    ext[i, c2] = x.astype(BF16)
        for st in range(NS):
            t00, t11 = outer(0, 2 * st), outer(1, 2 * st + 1)
            t01, t10 = outer(0, 2 * st + 1), outer(1, 2 * st)
            for k, i in enumerate((1, 5, 2, 4, 0, 3, 6)):
                pos = (lead + st * 7) * ng + k
                a, d = held(t00[i], pos, 7), held(t11[i], pos, 7)
                ops = _rhs_ops(a, t01[i], t10[i], d) if transposed else _rhs_ops(a, t10[i], t01[i], d)
                for j, x in enumerate(ops):
                    if i not in RAW or j not in RAW:
                        dst[i, j, st * LANES:(st + 1) * LANES, :] = x.astype(BF16)

    LQ = (FF - 2 * NS * 2 * LANES) // 4
    LCUT = (NH - 1) * LANES

    def left_rows(ref, c, lo, hi, shift):
        parts = []
        if lo < LANES:
            parts.append(ref[c, (LCUT + lo) >> shift:(LCUT + min(hi, LANES)) >> shift, :])
        if hi > LANES:
            base = (2 * NH - 2) * LANES
            parts.append(ref[c, (base + max(lo, LANES)) >> shift:(base + hi) >> shift, :])
        return parts

    def left_ops(toks):
        ng = LQ // 16

        def blk(c, qd):
            return jnp.concatenate([x.astype(F32) for x in left_rows(w3_v, c, qd * LQ, (qd + 1) * LQ, 0)], axis=0)

        def outer(k2, p):
            return _rhs_ops(blk(k2, p), blk(k2, 2 + p), blk(2 + k2, p), blk(2 + k2, 2 + p))

        t00, t01, t10, t11 = outer(0, 0), outer(0, 1), outer(1, 0), outer(1, 1)
        for k, i in enumerate((1, 5, 2, 4, 0, 3, 6)):
            tk = jnp.stack([toks[((k + r * 7) * len(toks)) // (7 * ng)] for r in range(ng)])

            def held(x):
                x4 = x.reshape(ng, 2, 8, LANES)
                return jnp.stack([after(tk, x4[:, 0]), x4[:, 1]], axis=1).reshape(LQ, LANES)

            for j, x in enumerate(_rhs_ops(held(t00[i]), t01[i], t10[i], held(t11[i]))):
                sl_s[i, j] = x.astype(BF16)

    WORD = [NH - 1, 2 * NH - 1] + [h * NH + 2 * st + p for st in range(NS) for h in range(2) for p in range(2)]
    CQ = LANES // 4

    def transpose_w4(toks):
        w_u = w4_v.bitcast(U32)
        order = [(c, n) for n in WORD for c in range(NC)]
        for k, (c, n) in enumerate(order):
            if n % NH == NH - 1:
                x = jnp.concatenate(left_rows(w_u, c, (n // NH) * 2 * LQ, (n // NH + 1) * 2 * LQ, 1)
                                    + [jnp.zeros((LANES // 2 - LQ, LANES), U32)], axis=0)
            else:
                x = w_u[c, n * (LANES // 2):(n + 1) * (LANES // 2), :]
            if XTOK:
                x = hold(x, [toks[(k * len(toks)) // len(order)]], True)
            wt_s[c, n * LANES:(n + 1) * LANES, :] = _as_bf16(x).astype(F32).T.astype(BF16)

    def col_ops(late):
        nt = 2 * NH
        wt = [wt_s[NC - 1, n * LANES:(n + 1) * LANES, :].astype(F32) for n in range(nt)]
        HC = 2 * CQ
        for i, x in enumerate(_rhs_ops(wt[NH - 1][0:HC], wt[NH - 1][HC:], wt[nt - 1][0:HC], wt[nt - 1][HC:])):
            ec_s[i] = x.astype(BF16)
        for st in range(NS):
            def outer(p, e):
                blk = lambda h, d: wt[h * NH + 2 * st + p][(2 * d + e) * CQ:(2 * d + e + 1) * CQ]
                return _rhs_ops(blk(0, 0), blk(0, 1), blk(1, 0), blk(1, 1))

            t00, t01, t10, t11 = outer(0, 0), outer(0, 1), outer(1, 0), outer(1, 1)
            for k, i in enumerate((1, 5, 2, 4, 0, 3, 6)):
                tk = jnp.stack([late[((st * 7 + k) * len(late)) // (NS * 7)]] * (CQ // 16))

                def held(x):
                    x4 = x.reshape(CQ // 16, 2, 8, LANES)
                    return jnp.stack([after(tk, x4[:, 0]), x4[:, 1]], axis=1).reshape(CQ, LANES)

                for j, x in enumerate(_rhs_ops(held(t00[i]), t01[i], t10[i], held(t11[i]))):
                    sc_s[i, j, st] = x.astype(BF16)

    HL = LANES // 2
    w3_u = w3_v.bitcast(U32)
    zr_u = zr_s.bitcast(U32)
    FQ = FF // 4
    BLOCKS = [(2 * r1 + r2, 2 * h + p) for r1, h in ((0, 0), (1, 0), (0, 1), (1, 1)) for r2 in range(2) for p in range(2)]

    def rem3(rq, d, pieces=1):
        w = jnp.concatenate([w3_u[NC - 1, ((d // 2) * NH + 2 * st + d % 2) * HL:((d // 2) * NH + 2 * st + d % 2 + 1) * HL, :]
                             for st in range(NS)] + left_rows(w3_u, NC - 1, d * LQ, (d + 1) * LQ, 1), axis=0)
        z = _as_bf16(zr_u[rq * (TQ // 2):(rq + 1) * (TQ // 2), :])
        return jnp.concatenate([_dot_nt(_as_bf16(w[lo // 2:hi // 2]), z) for lo, hi in chunks(0, FQ, pieces)], axis=0)

    def lead_in():
        head = [rem3(*key) for key in BLOCKS[:4]]
        for k in range(4):
            rh_s[k] = head[k]
        return [head[0][8 * r:8 * r + 8, :] for r in range(FQ // 8)]

    with jax.named_scope("r0a"):
        wait_all(first[:1])
        conv_round(0, 'k', False, False)
    with jax.named_scope("r0_wait"):
        wait_all(first[1:])
    with jax.named_scope("r0b"):
        start_all(conv_copies(2) + conv_copies(3) + conv_copies(4))
        conv_round(0, 'u', False, False)
    with jax.named_scope("r1a"):
        wait_all(second[:1])
        conv_round(1, 'k', True, False)
    with jax.named_scope("r1_wait"):
        wait_all(second[1:])
    with jax.named_scope("r1b"):
        start_all(wm_copies[0] + q_copies[0] + wm_copies[1] + w_copies[0])
        conv_round(1, 'u', False, False)

    def full_round(c, carry):
        wait_all(conv_copies(c))
        conv_round(c, 'ku', True, True)
        return carry

    with jax.named_scope("r234"):
        lax.fori_loop(2, NC, full_round, 0)
    with jax.named_scope("r5"):
        start_all(q_copies[1] + w_copies[1] + sum(q_copies[2:], []) + w_copies[2] + w_copies[3] + wm_copies[2], 1)
        conv_round(NC, '', True, True)
    with jax.named_scope("r6_wait"):
        wait_all(wm_copies[0] + q_copies[0])
    with jax.named_scope("r6"):
        for j in range(3):
            mod_chunk(j)
        conv_round(NC + 1, '', False, True)
        nx0 = stage_p1(0, A0[1], [None], mods_a())
    with jax.named_scope("p2_wait"):
        wait_all(wm_copies[1])
    with jax.named_scope("p2"):
        mod_chunk(4)
        mod_chunk(3)
        stage_p2(0, A0[1], nx0, mods_b())
    with jax.named_scope("w1_wait"):
        wait_all(w_copies[0])
    with jax.named_scope("m1_0"):
        toks = stage_m1(0, 4)
        if STR1:
            square_ops(w1_v, s1_s, toks[:len(toks) - 20 * W1N])
    with jax.named_scope("w2_wait"):
        wait_all(q_copies[1] + w_copies[1])
    with jax.named_scope("m2_0"):
        toks = stage_m2(0, 4)
        stage_p(1, toks[:len(toks) - TRIM * W2N], FREE * W2N)
        if STR2 and min(STR2) == 1:
            square_ops(w2_v, s2_s, toks[len(toks) // 2:len(toks) - 10 * W2N])
        filler(0)
    for t in range(1, NA):
        with jax.named_scope("a%d" % t):
            if t + 1 < NA:
                wait_all(q_copies[t + 1])
            else:
                wait_all(w_copies[2] + w_copies[3] + wm_copies[2])
            t1 = stage_m1(t, SPLIT)
            t2 = stage_m2(t, SPLIT, t1[len(t1) - len(t1) // SPLIT:])

            def weighted(trim):
                return t1 + t2[:len(t2) - trim * W2N]

            if t + 1 < NA:
                stage_p(t + 1, weighted(TRIM), FREE * W2N)
            if STR2 and t == W2P:
                square_ops(w2_v, s2_s, weighted(10))
            if t == NA - 1 - LAT:
                toks = weighted(TRIM // 2)
                store_z(0, 0, toks, FREE * W2N)
            if t == NA - 1:
                if not VMOD:
                    mod_chunk(NC)
                toks = weighted(0) + [x for x in lead_in()[:40] for _ in range(WE)]
                cut0 = (len(toks) * CUT) // 800
                cut = (len(toks) * CUT) // 100
                left_ops(toks[:cut0])
                if VMOD:
                    ng = D // 8
                    col = after(jnp.stack(pick(toks[:(len(toks) * 9) // 10], ng, 0)), scol_s[...].reshape(ng, 8, LANES))
                    for c in range(NC):
                        wf = wm_v[:, (NC * NC + c) * LANES:(NC * NC + c + 1) * LANES].astype(F32).reshape(ng, 8, LANES)
                        acc = col[0] * wf[0]
                        for r in range(1, ng):
                            acc = acc + col[r] * wf[r]
                        mod_s[NC, :, c * LANES:(c + 1) * LANES] = jnp.broadcast_to(
                            jnp.sum(acc, axis=0, keepdims=True), (8, LANES))
                weight_ops(w3_v, s3_s, None, True, toks[cut0:cut])
                transpose_w4(toks[:(len(toks) * XEND) // 100])
                weight_ops(wt_s, s4_s, e4_s, False, toks[cut:])
                col_ops(toks[cut:])
            if t + 1 < NA or not LAT:
                filler(t)

    gb = 0.5 * mod_s[NC, 0:1, :]
    w3_u, w4_u, s3_u, s4_u, e4_u = (r.bitcast(U32) for r in (w3_v, wt_s, s3_s, s4_s, e4_s))
    HL = LANES // 2
    zr_u = zr_s.bitcast(U32)
    sl_u = sl_s.bitcast(U32)
    sc_u = sc_s.bitcast(U32)
    ec_u = ec_s.bitcast(U32)

    def out_copy(r0, n, c):
        rows = pl.ds(r0, n)
        return pltpu.make_async_copy(o_v.at[c, rows, :], o_hbm.at[rows, pl.ds(c * LANES, LANES)], sem_o.at[0])

    def one_level(w_u, e_u, i, c2):
        if i not in RAW:
            return e_u[i, c2]
        d = RAW.index(i)
        n = d * NH + NH - 1
        return w_u[2 * d + c2, n * HL:(n + 1) * HL, :]

    def two_level(w_u, s_u, i, j, st):
        if i not in RAW or j not in RAW:
            return s_u[i, j, st * HL:(st + 1) * HL, :]
        d, e = RAW.index(i), RAW.index(j)
        n = d * NH + 2 * st + e
        return w_u[2 * d + e, n * HL:(n + 1) * HL, :]

    def loop_b(t, carry):
        r0 = pl.multiple_of(t * TB, TB)
        ws = t & 1

        count = [0]

        def fresh():
            count[0] += 1
            return lax.rem(t + 2 * count[0], 2)

        rem = {key: rh_s[k] for k, key in enumerate(BLOCKS[:4])}
        for key in BLOCKS[4:8]:
            rem[key] = rem3(*key)
        rem[BLOCKS[8]] = rem3(*BLOCKS[8], pieces=4)
        todo = BLOCKS[9:]
        pin = [None] * 7
        for i in (4, 3, 0, 6, 1, 2, 5):
            m = [None] * 7
            for j in _ORDER:
                slot = fresh()
                act = outer_lhs(j, lambda r2, k2: outer_lhs(
                    i, lambda r1, k1: zf_s[slot, blk_rows(NC * (2 * r1 + r2) + 2 * k1 + k2), :])).astype(BF16)
                wij = jnp.concatenate([two_level(w3_u, s3_u, i, j, st) for st in range(NS)] + [sl_u[i, j]], axis=0)
                m[j] = _dot_nt(_as_bf16(wij), act)
            key = todo.pop(0)
            rem[key] = rem3(*key)
            pin[i] = _combine(m)
        for inner in range(4):
            r2, p = inner // 2, inner % 2
            for blk, cval in enumerate(_combine([pin[i][inner] for i in range(7)])):
                r1, h = blk // 2, blk % 2
                gt = _gelu2(cval + rem[2 * r1 + r2, 2 * h + p])
                for st in range(NS):
                    g_s[blk][ws, blk_rows(GB * r2 + 2 * st + p), :] = gt[st * LANES:(st + 1) * LANES]
                lo = blk_rows(GB * r2 + NH - 1).start + p * LQ
                g_s[blk][ws, lo:lo + LQ, :] = gt[NS * LANES:]

        toks = []

        def timed(x):
            toks.extend(x[8 * r:8 * r + 8, 0:LANES] for r in range(x.shape[0] // 8))
            return x

        def finish(rq, c, h2):
            rows = pl.ds(pl.multiple_of(r0 + rq * TQ, TQ), TQ)
            cols = slice(c * LANES, (c + 1) * LANES)
            o_v[c, rows, :] = (x_s[rows, cols] + gb[:, cols] * (h_s[rows, cols] + h2)).astype(BF16)

        def outer_sum(p, blk):
            return (lambda: (p[3] - p[4]) + p[0] + p[6], lambda: p[2] + p[4], lambda: p[1] + p[3],
                    lambda: (p[2] - p[1]) + p[0] + p[5])[blk]()

        QR = LANES + CQ
        pin = [[None] * 4 for _ in range(7)]
        tails = {}
        marks = {}
        done = {_ORDER[1]: 1, _ORDER[3]: 2, _ORDER[5]: 0, _ORDER[6]: 3}
        for i in _ORDER:
            slot = fresh()
            we = _as_bf16(jnp.concatenate(
                [x for c2 in range(2)
                 for x in (one_level(w4_u, e4_u, i, c2), ec_u[i, c2 * (CQ // 2):(c2 + 1) * (CQ // 2), :])], axis=0))
            ex = []
            for r2 in range(2):
                lo = blk_rows(GB * r2 + NH - 1).start
                act = outer_lhs(i, lambda r1, h: g_s[2 * r1 + h][slot, lo:lo + 2 * LQ, :])
                act = jnp.concatenate([act, jnp.zeros((LANES - 2 * LQ, TQ), F32)], axis=0).astype(BF16)
                ex.append(_dot(we, act))
            m = [None] * 7
            for j in _ORDER:
                slot = fresh()
                act = jnp.concatenate(
                    [outer_lhs(j, lambda r2, p: outer_lhs(
                        i, lambda r1, h: g_s[2 * r1 + h][slot, blk_rows(GB * r2 + 2 * st + p), :]))
                     for st in range(NS)], axis=0).astype(BF16)
                wij = jnp.concatenate([jnp.concatenate([two_level(w4_u, s4_u, i, j, st), sc_u[i, j, st]], axis=0)
                                       for st in range(NS)], axis=1)
                m[j] = timed(_dot(_as_bf16(wij), act))
            pin[i] = [x + ex[inner // 2][(inner % 2) * QR:(inner % 2 + 1) * QR]
                      for inner, x in enumerate(_combine(m))]
            marks[i] = len(toks)

        nxt = jnp.minimum(t + 1, NT - 1)
        wins = {1: (0, LQ1, ZB0, ZB1), 2: (LQ1, LQ2, ZC0, ZC1), 0: (LQ2, 4, ZD0, ZD1)}

        nv = TQ // 8
        for i in _ORDER:
            if i not in done:
                continue
            blk = done[i]
            r1 = blk // 2
            if blk == 3:
                toks += [x for x in lead_in()[LT0:LT1] for _ in range(LTW)]
            elif wins[blk][0] < wins[blk][1]:
                store_z(nxt * TB, 1 - ws, toks[wins[blk][2]:wins[blk][3]], 0, *wins[blk][:2])
            pos = [marks[i] + (FLAG if blk != 3 else 0)]

            def paced(x):
                tk = toks[pos[0]:pos[0] + nv * FSTEP:FSTEP]
                pos[0] += nv * FSTEP
                if len(tk) < nv or not FSTEP:
                    return x
                return after(jnp.stack(tk), x.reshape(nv, 8, LANES)).reshape(TQ, LANES)

            for inner in (1, 2, 0, 3):
                ht = outer_sum([pin[k][inner] for k in range(7)], blk)
                rq, c = 2 * r1 + inner // 2, 2 * (blk % 2) + inner % 2
                finish(rq, c, paced(ht[0:LANES].T))
                tails[rq, c] = ht[LANES:]
            rb = pl.multiple_of(r0 + r1 * 2 * TQ, 2 * TQ)
            for e in range(2):
                out_copy(rb, 2 * TQ, 2 * (blk % 2) + e).start()
            if blk in (0, 3):
                for rq in (2 * r1, 2 * r1 + 1):
                    finish(rq, NC - 1, paced(jnp.concatenate([tails[rq, c] for c in range(NC - 1)], axis=0).T))
                out_copy(rb, 2 * TQ, NC - 1).start()

        return carry

    with jax.named_scope("ph2b"):
        lax.fori_loop(0, NT, loop_b, 0)
    with jax.named_scope("tail"):
        pltpu.make_async_copy(o_v, o_v, sem_o.at[0]).wait()


@jax.jit
def pallas_adaLN_cond__ssm_conv_h3__mixer_s_mlp__prompt_kernel(
    A_q: jax.Array,
    A_k: jax.Array,
    A_v: jax.Array,
    A_shift_k: jax.Array,
    A_ssm_k: jax.Array,
    A_ssm_D: jax.Array,
    B_x: jax.Array,
    B_w1: jax.Array,
    B_w2: jax.Array,
    B_w3: jax.Array,
    B_w4: jax.Array,
    c: jax.Array,
    w_mod: jax.Array,
):
    B, S, D = A_q.shape
    assert B == 1
    FF = B_w3.shape[1]
    NC = D // LANES
    NG = BLK // 8
    NBL = S // (PH * BLK)
    FP = -(-FF // (2 * LANES)) * 2 * LANES
    TILES = (384, 384, 576, 704)
    assert sum(TILES) == S
    TB = 512

    args = (A_q.reshape(S, D), A_k.reshape(S, D), A_v.reshape(S, D), A_shift_k.T, A_ssm_k,
            A_ssm_D, B_w1, B_w2, B_w3.T, B_w4, c, w_mod)
    scratch = [
        pltpu.VMEM((S, D), BF16),
        pltpu.VMEM((NC, S + KP, LANES), BF16),
        pltpu.VMEM((NC, S + VP, LANES), BF16),
        pltpu.VMEM((4, D), BF16),
        pltpu.VMEM((NC, LANES, S), BF16),
        pltpu.VMEM((D,), BF16),
        pltpu.VMEM((NC, D, LANES), BF16),
        pltpu.VMEM((NC, D, LANES), BF16),
        pltpu.VMEM((NC, FF, LANES), BF16),
        pltpu.VMEM((NC, FF, LANES), BF16),
        pltpu.VMEM((1, D), BF16),
        pltpu.VMEM((D, 6 * D), BF16),
        pltpu.VMEM((PH, 2 * BLK, BLK), BF16),
        pltpu.VMEM((PH, 2, BLK, BLK), BF16),
        pltpu.VMEM((NC, S, LANES), BF16),
        pltpu.VMEM((NC, NG, NBL, PH, 2, 8, LANES), F32),
        pltpu.VMEM((NC, NG, NBL, PH, 2, 8, LANES), F32),
        pltpu.VMEM((NC, NBL, PH, 2 * BLK, LANES), BF16),
        pltpu.VMEM((NBL, PH, BLK, LANES), BF16),
        pltpu.VMEM((NC, S + YP, LANES), F32),
        pltpu.VMEM((6, 8, D), F32),
        pltpu.VMEM((NC, 8, LANES), F32),
        pltpu.VMEM((NC, S + 16, LANES), F32),
        pltpu.VMEM((S, D), F32),
        pltpu.VMEM((S, D), F32),
        pltpu.VMEM((NC, S, LANES), BF16),
        pltpu.VMEM((7, 7, FP // 512 * LANES, LANES), BF16),
        pltpu.VMEM((7, 7, FP // 512 * LANES, LANES), BF16),
        pltpu.VMEM((7, 2, LANES, LANES), BF16),
        [pltpu.VMEM((2, GR, LANES), F32)] * 4,
        pltpu.VMEM((2, ZR, LANES), F32),
        pltpu.VMEM((TB, LANES), BF16),
        pltpu.VMEM((10, 2, S // 2, LANES), BF16),
        pltpu.VMEM((10, 2, S // 2, LANES), BF16),
        pltpu.VMEM((7, 2, 2 * LANES, LANES), BF16),
        pltpu.VMEM((7, 2, 2 * LANES, LANES), BF16),
        pltpu.VMEM((7, 7, (FF - FP // 512 * 512) // 4, LANES), BF16),
        pltpu.VMEM((7, 7, FP // 512, LANES // 4, LANES), BF16),
        pltpu.VMEM((7, LANES // 2, LANES), BF16),
        pltpu.VMEM((4, FF // 4, TB // 4), F32),
        pltpu.VMEM((NC, FP, LANES), BF16),
        pltpu.VMEM((D, LANES), F32),
        pltpu.SemaphoreType.DMA((16 + len(TILES),)),
        pltpu.SemaphoreType.DMA((1,)),
    ]
    out = pl.pallas_call(
        functools.partial(_kernel, S=S, D=D, FF=FF, TILES=TILES, TB=TB),
        in_specs=[pl.BlockSpec(memory_space=pl.ANY)] * len(args),
        out_specs=pl.BlockSpec(memory_space=pl.ANY),
        out_shape=jax.ShapeDtypeStruct((S, D), BF16),
        scratch_shapes=scratch,
        compiler_params=pltpu.CompilerParams(
            vmem_limit_bytes=126 * 1024 * 1024,
            disable_bounds_checks=True,
            disable_semaphore_checks=True,
        ),
    )(*args)
    return out.reshape(B, S, D)
```

```python
import functools
import math

import jax
import jax.numpy as jnp
from jax import lax
import jax.experimental.pallas as pl
import jax.experimental.pallas.tpu as pltpu

F32 = jnp.float32
BF16 = jnp.bfloat16
U32 = jnp.uint32

LANES = 128
BLK = 128
PH = 4
EPS = 1e-05
TRIM = 60
SPLIT = 2
FREE = 30
DUM = 96
LN1 = 999
KP = 16
VP = 0
YP = 0
GR = 1928
ZR = 2720
FT = 0
DUMB = 0
STR1 = (3, )
STR2 = (2, 3, )
WL = 3
WH = 2
ZE = 1
PRE = 0
WM2 = 2
W2P = 1
UL = 2
ALN = 0
LN0 = 32
SLAG = 1
NHEAD = 0
XTOK = 1
LASTO = 1
PINJ = ()
FLAG = 10
FSTEP = 1
WE = 2
XEND = 45
CUT = 78
VMOD = 1
LT0 = 8
LT1 = 40
LTW = 3
LQ1 = 2
LQ2 = 3
ZC0 = 320
ZC1 = 450
ZD0 = 600
ZD1 = 730
NE = 4
PL = 2
INLOOP = (2, 4, 1, 3, 0, )
LA = 0
FILL3 = 1
ER = 2
EA = 1
EB = 2
W1N = 2
W2N = 3
LAT = 1
LSETS = 1
LSTEP = 1
LB1 = 0
ZB0 = 0
ZB1 = 160
REM2 = 2
ZORD = (2, 3, 0, 1, 4, 5, 6)


def _as_bf16(x):
    return pltpu.bitcast(x, BF16)


def _lo(x):
    return pltpu.bitcast(x << 16, F32)


def _hi(x):
    return pltpu.bitcast(x & jnp.uint32(0xFFFF0000), F32)


def _dft4(re, im, sign):
    ar, ai = re[0] + re[2], im[0] + im[2]
    br, bi = re[0] - re[2], im[0] - im[2]
    cr, ci = re[1] + re[3], im[1] + im[3]
    dr, di = re[1] - re[3], im[1] - im[3]
    o0 = (ar + cr, ai + ci)
    o2 = (ar - cr, ai - ci)
    m = (br + di, bi - dr)
    p = (br - di, bi + dr)
    o1, o3 = (m, p) if sign < 0 else (p, m)
    return [o0[0], o1[0], o2[0], o3[0]], [o0[1], o1[1], o2[1], o3[1]]


def _ln(x, eps=EPS, unit=True):
    n = x.shape[-1]
    s1 = jnp.sum(x, axis=-1, keepdims=True)
    m = s1 * (1.0 / n)
    v = jnp.maximum(jnp.sum(x * x, axis=-1, keepdims=True) + (n * eps - s1 * m), n * eps)
    e = jnp.log(v) * (-0.5 / math.log(2.0))
    return (x - m) * jnp.exp2(e + 0.5 * math.log2(n) if unit else e)


def _gelu2(x):
    c0 = math.sqrt(2.0 / math.pi)
    return x + x * jnp.tanh(x * (c0 + (c0 * 0.044715) * (x * x)))


def _dot(a, b):
    return jnp.dot(a, b, preferred_element_type=F32)


def _dot_nt(a, b):
    return lax.dot_general(a, b, (((1,), (1,)), ((), ())), preferred_element_type=F32)


def _lhs_ops(a11, a12, a21, a22):
    return [a11 + a22, a21 + a22, a11, a22, a11 + a12, a21 - a11, a12 - a22]


def _rhs_ops(b11, b12, b21, b22):
    return [b11 + b22, b11, b12 - b22, b21 - b11, b22, b11 + b12, b21 + b22]


def _combine(m):
    return (m[3] - m[4]) + m[0] + m[6], m[2] + m[4], m[1] + m[3], (m[2] - m[1]) + m[0] + m[5]


_ORDER = (2, 4, 1, 3, 0, 6, 5)


def _rhs_op(i, blk):
    terms = ((0, 0, 1, 1, 1), (0, 0), (0, 1, -1, 1, 1), (1, 0, -1, 0, 0), (1, 1), (0, 0, 1, 0, 1), (1, 0, 1, 1, 1))[i]
    x = blk(terms[0], terms[1])
    if len(terms) > 2:
        y = blk(terms[3], terms[4])
        x = x + y if terms[2] > 0 else x - y
    return x


def _kernel(q_hbm, k_hbm, v_hbm, sh_hbm, sk_hbm, sd_hbm, w1_hbm, w2_hbm, w3_hbm, w4_hbm, c_hbm, wm_hbm,
            o_hbm,
            q_v, k_v, v_v, sh_v, sk_v, sd_v, w1_v, w2_v, w3_v, w4_v, c_v, wm_v,
            fw_s, iv_s, o_v, u_s, kk_s, vv_s, wu_s, y_s, mod_s, par_s, h1_s, x_s, h_s, z_s, s3_s, s4_s, e4_s, g_s, zf_s, zr_s, lo_s, l2_s, s1_s, s2_s, sl_s, rh_s, wt_s, scol_s,
            sem, sem_o,
            *, S, D, FF, TILES, TB):
    NC = D // LANES
    NG = BLK // 8
    LB = PH * BLK
    NBL = S // LB
    R = BLK // PH
    HALO = 32
    FP = wt_s.shape[1]
    FH = FP // 2
    NH = FH // LANES

    small = [
        pltpu.make_async_copy(sh_hbm, sh_v, sem.at[0]),
        pltpu.make_async_copy(sd_hbm, sd_v, sem.at[0]),
        pltpu.make_async_copy(c_hbm, c_v, sem.at[0]),
    ]

    def conv_copies(c):
        col = pl.ds(c * LANES if isinstance(c, int) else pl.multiple_of(c * LANES, LANES), LANES)
        return [
            pltpu.make_async_copy(sk_hbm.at[col, :], sk_v.at[c], sem.at[9 + c if isinstance(c, int) and c < 2 else 1 + c]),
            pltpu.make_async_copy(k_hbm.at[:, col], k_v.at[c, pl.ds(16, S), :], sem.at[1 + c]),
            pltpu.make_async_copy(v_hbm.at[:, col], v_v.at[c, pl.ds(0, S), :], sem.at[1 + c]),
        ]

    def col_copies(src, dst, c0, s):
        rows = pl.ds(0, src.shape[0])
        return [pltpu.make_async_copy(src.at[:, pl.ds((c0 + c) * LANES, LANES)], dst.at[c0 + c, rows, :], sem.at[s])
                for c in range(NC)]

    WM = (0, 3 * D, 5 * D, 6 * D)
    wm_copies = [[pltpu.make_async_copy(wm_hbm.at[:, pl.ds(WM[j], WM[j + 1] - WM[j])],
                                        wm_v.at[:, pl.ds(WM[j], WM[j + 1] - WM[j])], sem.at[6 + j])]
                 for j in range(3)]
    w_copies = [col_copies(src, dst, 0, 12 + j)
                for j, (src, dst) in enumerate(((w1_hbm, w1_v), (w2_hbm, w2_v), (w3_hbm, w3_v), (w4_hbm, w4_v)))]

    B0 = [0]
    for n in TILES:
        B0.append(B0[-1] + n)
    NA = len(TILES)
    A0 = [0] + [r + HALO for r in B0[1:-1]] + [S]
    q_copies = [
        [pltpu.make_async_copy(q_hbm.at[pl.ds(A0[t], A0[t + 1] - A0[t])], q_v.at[pl.ds(A0[t], A0[t + 1] - A0[t])],
                               sem.at[16 + t])]
        for t in range(NA)
    ]

    def start_all(cps, priority=0):
        for cp in cps:
            cp.start(priority=priority)

    def wait_all(cps):
        for cp in cps:
            cp.wait()

    def packed(ref, c0=0):
        ru = ref.bitcast(U32)
        return _as_bf16(jnp.concatenate([ru[c0 + c] for c in range(NC)], axis=1))

    first, second = conv_copies(0), conv_copies(1)
    start_all(first[:1] + small + first[1:] + second)

    for c in range(NC):
        k_v[c, 0:16, :] = jnp.zeros((16, LANES), BF16)
        h1_s[c, 0:8, :] = jnp.zeros((8, LANES), F32)
        h1_s[c, S + 8:S + 16, :] = jnp.zeros((8, LANES), F32)

    prow = lax.broadcasted_iota(jnp.int32, (BLK, BLK), 0)
    pcol = lax.broadcasted_iota(jnp.int32, (BLK, BLK), 1)
    ang = (((4 * prow + 1) * pcol) & (4 * BLK - 1)).astype(F32) * (2.0 * math.pi / (4 * BLK))
    tw = (4 * prow + 1).astype(F32) * (2.0 * math.pi / (4 * LB))
    mr, mi = jnp.cos(ang), -jnp.sin(ang)
    zr_, zi_ = jnp.cos(tw), -jnp.sin(tw)
    eye = jnp.where(prow == pcol, 1.0 / LB, 0.0).astype(BF16)
    for i in range(PH):
        both = jnp.stack([mr.reshape(NG, 8, BLK), mi.reshape(NG, 8, BLK)], axis=1).reshape(2 * BLK, BLK)
        fw_s[i] = both.astype(BF16)
        for h in range(2):
            iv_s[i, h] = _dot_nt(eye, both[h * BLK:(h + 1) * BLK, :].astype(BF16)).astype(BF16)
        if i + 1 < PH:
            mr, mi = mr * zr_ - mi * zi_, mr * zi_ + mi * zr_
    perm = jnp.where(pcol == (prow % R) * PH + prow // R, 1.0, 0.0).astype(BF16)
    fw_u = fw_s.bitcast(U32)
    iv_u = iv_s.bitcast(U32)

    wait_all(small)
    shf = sh_v[...].astype(F32)
    sdf = sd_v[...].astype(F32).reshape(1, D)
    for c in range(NC):
        par_s[c, 0:4, :] = shf[:, c * LANES:(c + 1) * LANES]
        par_s[c, 4:5, :] = sdf[:, c * LANES:(c + 1) * LANES]
    cf = c_v[...].astype(F32)
    sc = (cf * jax.nn.sigmoid(cf)).astype(BF16)
    sc16 = jnp.broadcast_to(sc, (16, D))

    scol_s[...] = jnp.broadcast_to(sc.astype(F32), (LANES, D)).T

    def mod_chunk(j):
        mod_s[j] = _dot(sc16, wm_v[:, j * D:(j + 1) * D])[0:8, :]

    k_u = k_v.bitcast(U32)
    v_u = v_v.bitcast(U32)
    wu_u = wu_s.bitcast(U32)
    z_u = z_s.bitcast(U32)
    vv_u = vv_s.bitcast(U32)
    lo_u = lo_s.bitcast(U32)
    l2_u = l2_s.bitcast(U32)

    never = zr_[0:8, :] > 2.0

    def after(token, x):
        if token.dtype != x.dtype:
            token = pltpu.bitcast(token, x.dtype)
        return jnp.where(jnp.broadcast_to(never, x.shape), token, x)

    def split(t):
        t4 = t.reshape(NG, 2, 8, LANES)
        return t4[:, 0], t4[:, 1]

    def perm_k(c, b, toks):
        kt = [_dot_nt(perm, sk_v[c, :, b * LB + t * BLK:b * LB + (t + 1) * BLK]) for t in range(PH)]
        for r in range(BLK // 16):
            toks.append(kt[0][16 * r:16 * r + 8, :])
        return [jnp.concatenate([kt[t][i * R:(i + 1) * R, :] for t in range(PH)], axis=0).astype(BF16)
                for i in range(PH)]

    def spectrum(wts, dst, c, b, toks, dc=None, pins=None):
        tr, ti = [], []
        for i in range(PH):
            lhs = fw_u[i]
            if pins is not None and i < len(pins):
                lhs = after(pins[i], lhs.reshape(NG, 8, LANES)).reshape(BLK, LANES)
            r_, i_ = split(_dot(_as_bf16(lhs), wts[i]))
            tr.append(r_)
            ti.append(i_)
        for g in range(NG):
            toks.append(ti[PH - 1][g])
        if dc is not None:
            tr[0] = tr[0] + dc
        sr, si = _dft4(tr, ti, -1)
        for qq in range(PH):
            dst[c, :, b, qq, 0] = sr[qq]
            dst[c, :, b, qq, 1] = si[qq]

    def gated(c, b):
        w = [par_s[c, t:t + 1, :] for t in range(4)]
        kc = {}
        for o in range(-2, 2):
            words = k_u[c, pl.ds(8 + b * (LB // 2) + o, BLK, stride=2), :]
            if o > -2:
                kc[2 * o] = _lo(words)
            kc[2 * o + 1] = _hi(words)
        vc = {}
        for o in range(2):
            words = v_u[c, pl.ds(b * (LB // 2) + o, BLK, stride=2), :]
            vc[2 * o] = _lo(words)
            vc[2 * o + 1] = _hi(words)
        for i in range(PH):
            ks = kc[i] * w[0]
            for t in range(1, 4):
                ks = ks + kc[i - t] * w[t]
            wu_s[b, i] = (ks * vc[i]).astype(BF16)
        return [wu_u[b, i] for i in range(PH)]

    def kv_pins(kvb):
        return [jnp.stack([kvb[2 * m + (r % 2)][8 * (r // 2):8 * (r // 2) + 8, :] for r in range(NG)])
                for m in range(2)]

    def mac(c, us, ks, toks):
        zp = None
        for o in range(NBL):
            zr, zi = [], []
            for qq in range(PH):
                accr = acci = None
                for b in range(o + 1):
                    a_, b_ = us[0, :, b, qq, 0], us[0, :, b, qq, 1]
                    c_, d_ = ks[0, :, o - b, qq, 0], ks[0, :, o - b, qq, 1]
                    if qq == 0 and b == o:
                        a_ = after(toks[o], a_)
                    tr_ = a_ * c_ - b_ * d_
                    ti_ = a_ * d_ + b_ * c_
                    accr = tr_ if accr is None else accr + tr_
                    acci = ti_ if acci is None else acci + ti_
                zr.append(accr)
                zi.append(acci)
            if zp is None:
                yr, yi = zr, zi
            else:
                yr = [zr[qq] - zp[1][qq] for qq in range(PH)]
                yi = [zi[qq] + zp[0][qq] for qq in range(PH)]
            zp = (zr, zi)
            vr, vi = _dft4(yr, yi, +1)
            for i in range(PH):
                vv_s[c, o, i] = jnp.stack([vr[i], vi[i]], axis=1).reshape(2 * BLK, LANES).astype(BF16)

    def inverse(c, toks, pins=None):
        HB = BLK // 2
        for o in range(NBL):
            for i in range(PH):
                yv = None
                for h in range(2):
                    lhs = iv_u[i, h]
                    if pins is not None and h == 0:
                        pin = pins[o][i % 2][8 * (i // 2):8 * (i // 2) + 8]
                        lhs = after(pin, lhs.reshape(8, 8, LANES)).reshape(HB, LANES)
                    t = _dot(_as_bf16(lhs), _as_bf16(vv_u[c, o, i, h * HB:(h + 1) * HB, :]))
                    yv = t if yv is None else yv + t
                if i % 2 == 0:
                    for r in range(BLK // 16):
                        toks.append(yv[16 * r:16 * r + 8, :])
                y_s[c, pl.ds(o * LB + i, BLK, stride=PH), :] = yv

    def mac_tokens(toks):
        n = len(toks) - 3
        cum = (44, 128, 244, 392)
        return [jnp.stack([toks[max(0, ((g * 392 + cum[o]) * n) // (392 * NG) - 1)] for g in range(NG)])
                for o in range(NBL)]

    def conv_round(c, fwd, mul, inv):
        toks = []
        kv = pins = None
        cur = 1 if mul else 0
        if fwd or mul:
            win = pl.ds(c - cur, 2 if fwd and mul else 1)
            us, ks = u_s.at[win], kk_s.at[win]
        if 'u' in fwd:
            kv = [gated(c, b) for b in range(NBL)]
            pins = [kv_pins(kv[b]) for b in range(NBL)]
        if inv:
            inverse(c - 2, toks, pins)
            if fwd:
                toks = []
        if 'k' in fwd:
            wts = [perm_k(c, b, toks) for b in range(NBL)]
        for b in range(NBL):
            if 'k' in fwd:
                spectrum(wts[b], ks, cur, b, toks, par_s[c, 4:5, :] if b == 0 else None)
            if 'u' in fwd:
                pin = pins[b + UL] if not inv and b + UL < NBL else None
                spectrum([_as_bf16(x) for x in kv[b]], us, cur, b, toks, None, pin)
        if mul:
            mac(c - 1, us, ks, mac_tokens(toks))

    def tokens_of(x):
        return [x[8 * r:8 * r + 8, c * LANES:(c + 1) * LANES] for c in range(NC) for r in range(x.shape[0] // 8)]

    def store_bf16(ref, r0, x):
        for c in range(NC):
            ref[c, r0:r0 + x.shape[0], :] = x[:, c * LANES:(c + 1) * LANES].astype(BF16)

    def load_bf16(ref_u, r0, n):
        return _as_bf16(jnp.concatenate([ref_u[c, pl.ds(r0 // 2, n // 2), :] for c in range(NC)], axis=1))

    def pick(toks, n, free):
        if toks is None:
            return [None] * n
        idx = [(r * (len(toks) + free)) // n - free for r in range(n)]
        return [toks[i] if i >= 0 else None for i in idx]

    def hold(x, tks, head=False):
        if head:
            return jnp.concatenate([after(tks[0], x[0:8]), x[8:]], axis=0)
        f = len([k for k in tks if k is None])
        n = len(tks)
        if f == n:
            return x
        first = after(jnp.stack(tks[f:]), x[8 * f:, 0:LANES].reshape(n - f, 8, LANES)).reshape(8 * (n - f), LANES)
        if f:
            first = jnp.concatenate([x[:8 * f, 0:LANES], first], axis=0)
        return jnp.concatenate([first, x[:, LANES:]], axis=1)

    def mods_a():
        ga = mod_s[2, 0:1, :]
        return ga * (1.0 + mod_s[1, 0:1, :]) * math.sqrt(D), ga * mod_s[0, 0:1, :]

    def mods_b():
        return (1.0 + mod_s[4, 0:1, :]) * (2.0 * math.sqrt(D)), 2.0 * mod_s[3, 0:1, :]

    def stage_p1(r0, r1, tks, ma):
        q = hold(q_v[r0:r1, :].astype(F32), tks)
        y = jnp.concatenate([y_s[c, r0:r1, :] for c in range(NC)], axis=1)
        x = q + (_ln(q, unit=False) * ma[0] + ma[1]) * y
        x_s[r0:r1, :] = x
        return _ln(x, unit=False)

    def halves(x):
        x4 = x.reshape(x.shape[0] // 32, 2, 16, LANES)
        return [x4[:, e].reshape(x.shape[0] // 2, LANES) for e in range(2)]

    def weave(top, bot):
        n = top.shape[0] // 16
        return jnp.stack([top.reshape(n, 16, LANES), bot.reshape(n, 16, LANES)], axis=1).reshape(32 * n, LANES)

    def row_ops(cols, tks=None):
        hv = [halves(x) for x in cols]
        if tks is not None:
            tk = jnp.stack(tks)

            def held(x):
                x4 = x.reshape(len(tks), 2, 8, LANES)
                return jnp.stack([after(tk, x4[:, 0]), x4[:, 1]], axis=1).reshape(x.shape)

            for k2 in range(2):
                hv[k2][0] = held(hv[k2][0])
                hv[2 + k2][1] = held(hv[2 + k2][1])
        per = [_lhs_ops(hv[k2][0], hv[2 + k2][0], hv[k2][1], hv[2 + k2][1]) + [hv[2 + k2][0], hv[k2][1]]
               for k2 in range(2)]
        return [[per[0][o], per[1][o]] for o in range(9)] + [hv[NC - 1]]

    def stage_p2(r0, r1, nx, mb, blockwise=False):
        h = nx * mb[0] + mb[1]
        h_s[r0:r1, :] = h
        zn = _ln(h, 4.0 * EPS)
        if not blockwise:
            store_bf16(z_s, r0, zn)
            return
        ops = row_ops([zn[:, c * LANES:(c + 1) * LANES] for c in range(NC)])
        for o in range(10):
            for e in range(2):
                lo_s[o, e, r0 // 2:r1 // 2, :] = ops[o][e].astype(BF16)

    def stage_p(t, toks, free):
        lo, hi = A0[t], A0[t + 1]
        stage_p2(lo, hi, stage_p1(lo, hi, pick(toks, (hi - lo) // 8, free), mods_a()), mods_b(), t in STR1)

    def square_ops(src, dst, toks):
        HK = 2 * LANES
        ng = HK // 16
        for n2 in range(2):
            tk = jnp.stack([toks[((n2 * ng + r) * len(toks)) // (2 * ng)] for r in range(ng)])

            def blk(c, k, hold_it):
                x = src[c, k * HK:(k + 1) * HK, :].astype(F32)
                if not hold_it:
                    return x
                x4 = x.reshape(ng, 2, 8, LANES)
                return jnp.stack([after(tk, x4[:, 0]), x4[:, 1]], axis=1).reshape(HK, LANES)

            for o, x in enumerate(_rhs_ops(blk(n2, 0, True), blk(2 + n2, 0, False), blk(n2, 1, False), blk(2 + n2, 1, True))):
                if o not in (1, 4):
                    dst[o, n2] = x.astype(BF16)

    def block_dots(lhs_of, w_ref, s_ref, parts, emit, WL, WH):
        w_u, s_u = w_ref.bitcast(U32), s_ref.bitcast(U32)
        toks = []

        def timed(x, weight):
            toks.extend(x[8 * r:8 * r + 8, 0:LANES] for r in range(x.shape[0] // 8) for _ in range(weight))
            return x

        def main(get):
            m = [None] * 7
            rem = [None, None]
            for o in ('t', 2, 4, 'b', 1, 3, 0, 6, 5):
                if o in ('t', 'b'):
                    e = 0 if o == 't' else 1
                    rhs = jnp.concatenate([w_u[c, 2 * LANES:D // 2, :] for c in range(NC - 1)], axis=1)
                    rem[e] = timed(_dot(get([(9, e)]), _as_bf16(rhs)), WL)
                    continue
                if o in (1, 4):
                    d = (1, 4).index(o)
                    rhs = jnp.concatenate([w_u[2 * d + n2, d * LANES:(d + 1) * LANES, :] for n2 in range(2)], axis=1)
                else:
                    rhs = jnp.concatenate([s_u[o, n2] for n2 in range(2)], axis=1)
                m[o] = timed(_dot(get([(o, 0), (o, 1)]), _as_bf16(rhs)), WH if o in (4, 3, 6, 5) else WL)
            c11, c12, c21, c22 = _combine(m)
            top = jnp.concatenate([c11, c12], axis=1) + rem[0]
            bot = jnp.concatenate([c21, c22], axis=1) + rem[1]
            return [weave(top[:, c * LANES:(c + 1) * LANES], bot[:, c * LANES:(c + 1) * LANES]) for c in range(NC - 1)]

        def last(get):
            w4c = _as_bf16(w_u[NC - 1])
            return weave(timed(_dot(get([(2, 0), (2, 1), (7, 0), (7, 1), (9, 0)]), w4c), WL),
                         timed(_dot(get([(8, 0), (8, 1), (3, 0), (3, 1), (9, 1)]), w4c), WL))

        marks = []
        for j, part in enumerate(parts):
            get = lhs_of(part, toks[marks[-1]:] if marks else None)
            marks.append(len(toks))
            if j % 2:
                tail = last(get)
                cols = main(get) + [tail]
            else:
                cols = main(get) + [last(get)]
            emit(part, cols)
        return toks

    def filler(t):
        if DUM:
            red = jnp.sum(y_s[t, 0:8 * DUM, :], axis=-1, keepdims=True).reshape(DUM, 8, 1)
            zf_s[1, (NC - 1) * (TQ + 8) + 8 * t:(NC - 1) * (TQ + 8) + 8 * t + 8, :] = jnp.broadcast_to(jnp.sum(red, axis=0), (8, LANES))

    def chunks(r0, r1, k, unit=16):
        n = (r1 - r0) // unit
        cuts = [r0 + unit * ((n * j) // k) for j in range(k + 1)]
        return list(zip(cuts[:-1], cuts[1:]))

    def stage_m1(t, k):
        def emit(part, cols):
            out = [_gelu2(x) for x in cols]
            for c in range(NC):
                h1_s[c, part[0] + 8:part[1] + 8, :] = out[c]
            return out

        if t in STR1:
            def lhs_of(part, _):
                return lambda keys: _as_bf16(jnp.concatenate(
                    [lo_u[o, e, part[0] // 4:part[1] // 4, :] for o, e in keys], axis=1))
            return block_dots(lhs_of, w1_v, s1_s, chunks(A0[t], A0[t + 1], k, 32), emit, WL, WH)
        toks = []
        for r0, r1 in chunks(A0[t], A0[t + 1], k):
            pre = _dot(load_bf16(z_u, r0, r1 - r0), packed(w1_v))
            out = emit((r0, r1), [pre[:, c * LANES:(c + 1) * LANES] for c in range(NC)])
            toks += [x for x in tokens_of(jnp.concatenate(out, axis=1)) for _ in range(W1N)]
        return toks

    grp = D // 4
    shifts = (-1, 1, -2, 2)

    def shifted(r0, r1):
        n = r1 - r0
        lane = lax.broadcasted_iota(jnp.int32, (n, LANES), 1)
        cols = []
        for c in range(NC):
            lo, hi = c * LANES, (c + 1) * LANES
            g_lo, g_hi = lo // grp, (hi - 1) // grp
            val = h1_s[c, pl.ds(r0 + 8 + shifts[g_lo], n), :]
            if g_hi != g_lo:
                other = h1_s[c, pl.ds(r0 + 8 + shifts[g_hi], n), :]
                val = jnp.where(lane < (g_hi * grp - lo), val, other)
            cols.append(val)
        return cols

    def stage_m2(t, k, before=None):
        def emit(part, cols):
            x1 = h_s[part[0]:part[1], :] + jnp.concatenate(cols, axis=1)
            h_s[part[0]:part[1], :] = x1
            return x1

        if t in STR2:
            def lhs_of(part, prev):
                prev = before if prev is None else prev
                prev = prev[len(prev) // 8:(len(prev) * 7) // 8]
                ops = row_ops(shifted(*part), pick(prev, (part[1] - part[0]) // 32, 0))
                for o in range(10):
                    for e in range(2):
                        l2_s[o, e, part[0] // 2:part[1] // 2, :] = ops[o][e].astype(BF16)
                return lambda keys: _as_bf16(jnp.concatenate(
                    [l2_u[o, e, part[0] // 4:part[1] // 4, :] for o, e in keys], axis=1))
            return block_dots(lhs_of, w2_v, s2_s, chunks(B0[t], B0[t + 1], k, 32), emit, WM2, WM2)
        toks = []
        for r0, r1 in chunks(B0[t], B0[t + 1], k):
            hs = _dot(jnp.concatenate(shifted(r0, r1), axis=1).astype(BF16), packed(w2_v))
            toks += [x for x in tokens_of(emit((r0, r1), [hs])) for _ in range(W2N)]
        return toks

    TQ = TB // 4
    NT = S // TB
    GB = NH

    def blk_rows(b):
        return slice(b * (TQ + 8), b * (TQ + 8) + TQ)

    def store_z(r0, slot, toks, free, q0=0, q1=4):
        n = (q1 - q0) * TQ
        rows = pl.ds(r0 + q0 * TQ if isinstance(r0, int) else pl.multiple_of(r0 + q0 * TQ, TQ), n)
        zn = _ln(hold(h_s[rows, :], pick(toks, n // 8, free)), 4.0 * EPS)
        for rq in range(q0, q1):
            for c in range(NC - 1):
                zf_s[slot, blk_rows(NC * rq + c), :] = zn[(rq - q0) * TQ:(rq - q0 + 1) * TQ, c * LANES:(c + 1) * LANES]
        zr_s[q0 * TQ:q1 * TQ, :] = zn[:, (NC - 1) * LANES:].astype(BF16)

    def outer_lhs(i, blk):
        terms = ((0, 0, 1, 1, 1), (1, 0, 1, 1, 1), (0, 0), (1, 1), (0, 0, 1, 0, 1), (1, 0, -1, 0, 0), (0, 1, -1, 1, 1))[i]
        x = blk(terms[0], terms[1])
        if len(terms) > 2:
            y = blk(terms[3], terms[4])
            x = x + y if terms[2] > 0 else x - y
        return x

    NS = NH // 2

    RAW = (1, 4)

    def weight_ops(src, dst, ext, transposed, toks):
        ng = LANES // 16
        lead = 2 if ext is not None else 0
        total = (NS * 7 + lead) * ng

        def tile(c, n):
            return src[c, n * LANES:(n + 1) * LANES, :].astype(F32)

        def held(x, pos, step):
            tk = jnp.stack([toks[((pos + r * step) * len(toks)) // total] for r in range(ng)])
            x4 = x.reshape(ng, 2, 8, LANES)
            return jnp.stack([after(tk, x4[:, 0]), x4[:, 1]], axis=1).reshape(LANES, LANES)

        def outer(c2, n, pos=None):
            b11, b22 = tile(c2, n), tile(2 + c2, NH + n)
            if pos is not None:
                b11, b22 = held(b11, pos, 1), held(b22, pos, 1)
            e1, e2 = tile(c2, NH + n), tile(2 + c2, n)
            return _rhs_ops(b11, e1, e2, b22) if transposed else _rhs_ops(b11, e2, e1, b22)

        for c2 in range(2 if ext is not None else 0):
            for i, x in enumerate(outer(c2, NH - 1, c2 * ng)):
                if i not in RAW:
                    ext[i, c2] = x.astype(BF16)
        for st in range(NS):
            t00, t11 = outer(0, 2 * st), outer(1, 2 * st + 1)
            t01, t10 = outer(0, 2 * st + 1), outer(1, 2 * st)
            for k, i in enumerate((1, 5, 2, 4, 0, 3, 6)):
                pos = (lead + st * 7) * ng + k
                a, d = held(t00[i], pos, 7), held(t11[i], pos, 7)
                ops = _rhs_ops(a, t01[i], t10[i], d) if transposed else _rhs_ops(a, t10[i], t01[i], d)
                for j, x in enumerate(ops):
                    if i not in RAW or j not in RAW:
                        dst[i, j, st * LANES:(st + 1) * LANES, :] = x.astype(BF16)

    LQ = (FF - 2 * NS * 2 * LANES) // 4
    LCUT = (NH - 1) * LANES

    def left_rows(ref, c, lo, hi, shift):
        parts = []
        if lo < LANES:
            parts.append(ref[c, (LCUT + lo) >> shift:(LCUT + min(hi, LANES)) >> shift, :])
        if hi > LANES:
            base = (2 * NH - 2) * LANES
            parts.append(ref[c, (base + max(lo, LANES)) >> shift:(base + hi) >> shift, :])
        return parts

    def left_ops(toks):
        ng = LQ // 16

        def blk(c, qd):
            return jnp.concatenate([x.astype(F32) for x in left_rows(w3_v, c, qd * LQ, (qd + 1) * LQ, 0)], axis=0)

        def outer(k2, p):
            return _rhs_ops(blk(k2, p), blk(k2, 2 + p), blk(2 + k2, p), blk(2 + k2, 2 + p))

        t00, t01, t10, t11 = outer(0, 0), outer(0, 1), outer(1, 0), outer(1, 1)
        for k, i in enumerate((1, 5, 2, 4, 0, 3, 6)):
            tk = jnp.stack([toks[((k + r * 7) * len(toks)) // (7 * ng)] for r in range(ng)])

            def held(x):
                x4 = x.reshape(ng, 2, 8, LANES)
                return jnp.stack([after(tk, x4[:, 0]), x4[:, 1]], axis=1).reshape(LQ, LANES)

            for j, x in enumerate(_rhs_ops(held(t00[i]), t01[i], t10[i], held(t11[i]))):
                sl_s[i, j] = x.astype(BF16)

    WORD = [NH - 1, 2 * NH - 1] + [h * NH + 2 * st + p for st in range(NS) for h in range(2) for p in range(2)]
    CQ = LANES // 4

    def transpose_w4(toks):
        w_u = w4_v.bitcast(U32)
        order = [(c, n) for n in WORD for c in range(NC)]
        for k, (c, n) in enumerate(order):
            if n % NH == NH - 1:
                x = jnp.concatenate(left_rows(w_u, c, (n // NH) * 2 * LQ, (n // NH + 1) * 2 * LQ, 1)
                                    + [jnp.zeros((LANES // 2 - LQ, LANES), U32)], axis=0)
            else:
                x = w_u[c, n * (LANES // 2):(n + 1) * (LANES // 2), :]
            if XTOK:
                x = hold(x, [toks[(k * len(toks)) // len(order)]], True)
            wt_s[c, n * LANES:(n + 1) * LANES, :] = _as_bf16(x).astype(F32).T.astype(BF16)

    def w4_ops(i, zero, toks):
        QR = LANES + CQ
        ng = QR // 16
        total = (NS * 7 + 2) * ng

        def quarter(n, d):
            return jnp.concatenate(
                [wt_s[d, n * LANES:(n + 1) * LANES, :].astype(F32),
                 wt_s[NC - 1, n * LANES + d * CQ:n * LANES + (d + 1) * CQ, :].astype(F32)], axis=0)

        def held(x, pos, step):
            tk = jnp.stack([toks[((pos + r * step) * len(toks)) // total] for r in range(ng)])
            x4 = x.reshape(ng, 2, 8, LANES)
            return jnp.stack([after(tk, x4[:, 0]), x4[:, 1]], axis=1).reshape(QR, LANES)

        if i not in RAW:
            for e in range(2):
                x = _rhs_op(i, lambda h, d: quarter(h * NH + NH - 1, 2 * d + e))
                e4_s[i + zero, e] = held(x, e * ng, 1).astype(BF16)
        for st in range(NS):
            t = [[_rhs_op(i, lambda h, d: quarter(h * NH + 2 * st + p, 2 * d + e)) for e in range(2)] for p in range(2)]
            pos = (2 + st * 7) * ng
            for j, x in enumerate(_rhs_ops(held(t[0][0], pos, 7), t[0][1], t[1][0], held(t[1][1], pos, 7))):
                if i not in RAW or j not in RAW:
                    s4_s[i + zero, j, st] = x.astype(BF16)

    HL = LANES // 2
    w3_u = w3_v.bitcast(U32)
    zr_u = zr_s.bitcast(U32)
    FQ = FF // 4
    BLOCKS = [(2 * r1 + r2, 2 * h + p) for r1, h in ((0, 0), (1, 0), (0, 1), (1, 1)) for r2 in range(2) for p in range(2)]

    def rem3(rq, d, pieces=1):
        w = jnp.concatenate([w3_u[NC - 1, ((d // 2) * NH + 2 * st + d % 2) * HL:((d // 2) * NH + 2 * st + d % 2 + 1) * HL, :]
                             for st in range(NS)] + left_rows(w3_u, NC - 1, d * LQ, (d + 1) * LQ, 1), axis=0)
        z = _as_bf16(zr_u[rq * (TQ // 2):(rq + 1) * (TQ // 2), :])
        return jnp.concatenate([_dot_nt(_as_bf16(w[lo // 2:hi // 2]), z) for lo, hi in chunks(0, FQ, pieces)], axis=0)

    def lead_in():
        head = [rem3(*key) for key in BLOCKS[:4]]
        for k in range(4):
            rh_s[k] = head[k]
        return [head[0][8 * r:8 * r + 8, :] for r in range(FQ // 8)]

    with jax.named_scope("r0a"):
        wait_all(first[:1])
        conv_round(0, 'k', False, False)
    with jax.named_scope("r0_wait"):
        wait_all(first[1:])
    with jax.named_scope("r0b"):
        start_all(conv_copies(2) + conv_copies(3) + conv_copies(4))
        conv_round(0, 'u', False, False)
    with jax.named_scope("r1a"):
        wait_all(second[:1])
        conv_round(1, 'k', True, False)
    with jax.named_scope("r1_wait"):
        wait_all(second[1:])
    with jax.named_scope("r1b"):
        start_all(wm_copies[0] + q_copies[0] + wm_copies[1] + w_copies[0])
        conv_round(1, 'u', False, False)

    def full_round(c, carry):
        wait_all(conv_copies(c))
        conv_round(c, 'ku', True, True)
        return carry

    with jax.named_scope("r234"):
        lax.fori_loop(2, NC, full_round, 0)
    with jax.named_scope("r5"):
        start_all(q_copies[1] + w_copies[1] + sum(q_copies[2:], []) + w_copies[2] + w_copies[3] + wm_copies[2], 1)
        conv_round(NC, '', True, True)
    with jax.named_scope("r6_wait"):
        wait_all(wm_copies[0] + q_copies[0])
    with jax.named_scope("r6"):
        for j in range(3):
            mod_chunk(j)
        conv_round(NC + 1, '', False, True)
        nx0 = stage_p1(0, A0[1], [None], mods_a())
    with jax.named_scope("p2_wait"):
        wait_all(wm_copies[1])
    with jax.named_scope("p2"):
        mod_chunk(4)
        mod_chunk(3)
        stage_p2(0, A0[1], nx0, mods_b())
    with jax.named_scope("w1_wait"):
        wait_all(w_copies[0])
    with jax.named_scope("m1_0"):
        toks = stage_m1(0, 4)
        if STR1:
            square_ops(w1_v, s1_s, toks[:len(toks) - 20 * W1N])
    with jax.named_scope("w2_wait"):
        wait_all(q_copies[1] + w_copies[1])
    with jax.named_scope("m2_0"):
        toks = stage_m2(0, 4)
        stage_p(1, toks[:len(toks) - TRIM * W2N], FREE * W2N)
        if STR2 and min(STR2) == 1:
            square_ops(w2_v, s2_s, toks[len(toks) // 2:len(toks) - 10 * W2N])
        filler(0)
    for t in range(1, NA):
        with jax.named_scope("a%d" % t):
            if t + 1 < NA:
                wait_all(q_copies[t + 1])
            else:
                wait_all(w_copies[2] + w_copies[3] + wm_copies[2])
            t1 = stage_m1(t, SPLIT)
            t2 = stage_m2(t, SPLIT, t1[len(t1) - len(t1) // SPLIT:])

            def weighted(trim):
                return t1 + t2[:len(t2) - trim * W2N]

            if t + 1 < NA:
                stage_p(t + 1, weighted(TRIM), FREE * W2N)
            if STR2 and t == W2P:
                square_ops(w2_v, s2_s, weighted(10))
            if t == NA - 2 and LA:
                store_z(0, 0, weighted(TRIM // 2), FREE * W2N, 0, LA)
            if t == NA - 1:
                toks = weighted(0)
                transpose_w4(toks[:(len(toks) * XEND) // 100])
                if LA < 4:
                    store_z(0, 0, toks[(len(toks) * (XEND + 5)) // 100:(len(toks) * 88) // 100], 0, LA, 4)
            if t == NA - 1:
                if not VMOD:
                    mod_chunk(NC)
                toks = weighted(0) + [x for x in lead_in()[:40] for _ in range(WE)]
                cut = (len(toks) * CUT) // 100
                cut0 = cut // 9
                left_ops(toks[:cut0])
                if VMOD:
                    ng = D // 8
                    col = after(jnp.stack(pick(toks[:(len(toks) * 9) // 10], ng, 0)), scol_s[...].reshape(ng, 8, LANES))
                    for c in range(NC):
                        wf = wm_v[:, (NC * NC + c) * LANES:(NC * NC + c + 1) * LANES].astype(F32).reshape(ng, 8, LANES)
                        acc = col[0] * wf[0]
                        for r in range(1, ng):
                            acc = acc + col[r] * wf[r]
                        mod_s[NC, :, c * LANES:(c + 1) * LANES] = jnp.broadcast_to(
                            jnp.sum(acc, axis=0, keepdims=True), (8, LANES))
                weight_ops(w3_v, s3_s, None, True, toks[cut0:cut])
                rest = [i for i in range(7) if i not in INLOOP]
                for k, i in enumerate(rest):
                    w4_ops(i, 0, toks[cut + k::len(rest)])

            if t + 1 < NA or (LA < 4 and FILL3):
                filler(t)

    gb = 0.5 * mod_s[NC, 0:1, :]
    w3_u, w4_u, s3_u, s4_u, e4_u = (r.bitcast(U32) for r in (w3_v, wt_s, s3_s, s4_s, e4_s))
    HL = LANES // 2
    zr_u = zr_s.bitcast(U32)
    sl_u = sl_s.bitcast(U32)

    def out_copy(r0, n, c):
        rows = pl.ds(r0, n)
        return pltpu.make_async_copy(o_v.at[c, rows, :], o_hbm.at[rows, pl.ds(c * LANES, LANES)], sem_o.at[0])

    def raw4(n, d):
        lo = n * HL + d * (CQ // 2)
        return jnp.concatenate([w4_u[d, n * HL:(n + 1) * HL, :], w4_u[NC - 1, lo:lo + CQ // 2, :]], axis=0)

    def one_level4(i, e, zero):
        if i not in RAW:
            return e4_u[i, e]
        d = RAW.index(i)
        return raw4(d * NH + NH - 1, 2 * d + e)

    def two_level4(i, j, st, zero):
        if i not in RAW or j not in RAW:
            return s4_u[i, j, st]
        d, e = RAW.index(i), RAW.index(j)
        return raw4(d * NH + 2 * st + e, 2 * d + e)

    def two_level(w_u, s_u, i, j, st):
        if i not in RAW or j not in RAW:
            return s_u[i, j, st * HL:(st + 1) * HL, :]
        d, e = RAW.index(i), RAW.index(j)
        n = d * NH + 2 * st + e
        return w_u[2 * d + e, n * HL:(n + 1) * HL, :]

    def loop_b(t, carry):
        r0 = pl.multiple_of(t * TB, TB)
        ws = t & 1

        count = [0]

        def fresh():
            count[0] += 1
            return lax.rem(t + 2 * count[0], 2)

        rem = {key: rh_s[k] for k, key in enumerate(BLOCKS[:4])}
        for key in BLOCKS[4:8]:
            rem[key] = rem3(*key)
        early = [rem[BLOCKS[4]][8 * r:8 * r + 8, :] for r in range(FQ // 8) for _ in range(ER)]
        rem[BLOCKS[8]] = rem3(*BLOCKS[8], pieces=4)
        todo = BLOCKS[9:]
        pin = [None] * 7
        for i in (4, 3, 0, 6, 1, 2, 5):
            m = [None] * 7
            for j in _ORDER:
                slot = fresh()
                act = outer_lhs(j, lambda r2, k2: outer_lhs(
                    i, lambda r1, k1: zf_s[slot, blk_rows(NC * (2 * r1 + r2) + 2 * k1 + k2), :])).astype(BF16)
                wij = jnp.concatenate([two_level(w3_u, s3_u, i, j, st) for st in range(NS)] + [sl_u[i, j]], axis=0)
                m[j] = _dot_nt(_as_bf16(wij), act)
            key = todo.pop(0)
            rem[key] = rem3(*key)
            pin[i] = _combine(m)
            if i in (4, 3, 0):
                early += [m[j][8 * r:8 * r + 8, :] for j, w in ((_ORDER[0], EA), (_ORDER[4], EB))
                          for r in range(FQ // 8) for _ in range(w)]
        zero = fresh() - ws
        fine = [x for x in early for _ in range(len(INLOOP))]
        hop = len(fine) // (len(INLOOP) * 33)
        for k, i in enumerate(INLOOP):
            w4_ops(i, zero, fine[k * hop:len(fine) - (len(INLOOP) - k) * hop])
        for inner in range(4):
            r2, p = inner // 2, inner % 2
            for blk, cval in enumerate(_combine([pin[i][inner] for i in range(7)])):
                r1, h = blk // 2, blk % 2
                gt = _gelu2(cval + rem[2 * r1 + r2, 2 * h + p])
                for st in range(NS):
                    g_s[blk][ws, blk_rows(GB * r2 + 2 * st + p), :] = gt[st * LANES:(st + 1) * LANES]
                lo = blk_rows(GB * r2 + NH - 1).start + p * LQ
                g_s[blk][ws, lo:lo + LQ, :] = gt[NS * LANES:]

        toks = []

        def timed(x):
            toks.extend(x[8 * r:8 * r + 8, 0:LANES] for r in range(x.shape[0] // 8))
            return x

        def finish(rq, c, h2):
            rows = pl.ds(pl.multiple_of(r0 + rq * TQ, TQ), TQ)
            cols = slice(c * LANES, (c + 1) * LANES)
            o_v[c, rows, :] = (x_s[rows, cols] + gb[:, cols] * (h_s[rows, cols] + h2)).astype(BF16)

        def outer_sum(p, blk):
            return (lambda: (p[3] - p[4]) + p[0] + p[6], lambda: p[2] + p[4], lambda: p[1] + p[3],
                    lambda: (p[2] - p[1]) + p[0] + p[5])[blk]()

        QR = LANES + CQ
        pin = [[None] * 4 for _ in range(7)]
        tails = {}
        marks = {}
        done = {_ORDER[1]: 1, _ORDER[3]: 2, _ORDER[5]: 0, _ORDER[6]: 3}
        for i in _ORDER:
            slot = fresh()
            we = _as_bf16(jnp.concatenate([one_level4(i, e, zero) for e in range(2)], axis=0))
            ex = []
            for r2 in range(2):
                lo = blk_rows(GB * r2 + NH - 1).start
                act = outer_lhs(i, lambda r1, h: g_s[2 * r1 + h][slot, lo:lo + 2 * LQ, :])
                act = jnp.concatenate([act, jnp.zeros((LANES - 2 * LQ, TQ), F32)], axis=0).astype(BF16)
                ex.append(_dot(we, act))
            m = [None] * 7
            for j in _ORDER:
                slot = fresh()
                act = jnp.concatenate(
                    [outer_lhs(j, lambda r2, p: outer_lhs(
                        i, lambda r1, h: g_s[2 * r1 + h][slot, blk_rows(GB * r2 + 2 * st + p), :]))
                     for st in range(NS)], axis=0).astype(BF16)
                wij = jnp.concatenate([two_level4(i, j, st, zero) for st in range(NS)], axis=1)
                m[j] = timed(_dot(_as_bf16(wij), act))
            pin[i] = [x + ex[inner // 2][(inner % 2) * QR:(inner % 2 + 1) * QR]
                      for inner, x in enumerate(_combine(m))]
            marks[i] = len(toks)

        nxt = jnp.minimum(t + 1, NT - 1)
        wins = {1: (0, LQ1, ZB0, ZB1), 2: (LQ1, LQ2, ZC0, ZC1), 0: (LQ2, 4, ZD0, ZD1)}

        nv = TQ // 8
        for i in _ORDER:
            if i not in done:
                continue
            blk = done[i]
            r1 = blk // 2
            if blk == 3:
                toks += [x for x in lead_in()[LT0:LT1] for _ in range(LTW)]
            elif wins[blk][0] < wins[blk][1]:
                store_z(nxt * TB, 1 - ws, toks[wins[blk][2]:wins[blk][3]], 0, *wins[blk][:2])
            pos = [marks[i] + (FLAG if blk != 3 else 0)]

            def paced(x):
                tk = toks[pos[0]:pos[0] + nv * FSTEP:FSTEP]
                pos[0] += nv * FSTEP
                if len(tk) < nv or not FSTEP:
                    return x
                return after(jnp.stack(tk), x.reshape(nv, 8, LANES)).reshape(TQ, LANES)

            for inner in (1, 2, 0, 3):
                ht = outer_sum([pin[k][inner] for k in range(7)], blk)
                rq, c = 2 * r1 + inner // 2, 2 * (blk % 2) + inner % 2
                finish(rq, c, paced(ht[0:LANES].T))
                tails[rq, c] = ht[LANES:]
            rb = pl.multiple_of(r0 + r1 * 2 * TQ, 2 * TQ)
            for e in range(2):
                out_copy(rb, 2 * TQ, 2 * (blk % 2) + e).start()
            if blk in (0, 3):
                for rq in (2 * r1, 2 * r1 + 1):
                    finish(rq, NC - 1, paced(jnp.concatenate([tails[rq, c] for c in range(NC - 1)], axis=0).T))
                out_copy(rb, 2 * TQ, NC - 1).start()

        return carry

    with jax.named_scope("ph2b"):
        lax.fori_loop(0, NT, loop_b, 0)
    with jax.named_scope("tail"):
        pltpu.make_async_copy(o_v, o_v, sem_o.at[0]).wait()


@jax.jit
def pallas_adaLN_cond__ssm_conv_h3__mixer_s_mlp__prompt_kernel(
    A_q: jax.Array,
    A_k: jax.Array,
    A_v: jax.Array,
    A_shift_k: jax.Array,
    A_ssm_k: jax.Array,
    A_ssm_D: jax.Array,
    B_x: jax.Array,
    B_w1: jax.Array,
    B_w2: jax.Array,
    B_w3: jax.Array,
    B_w4: jax.Array,
    c: jax.Array,
    w_mod: jax.Array,
):
    B, S, D = A_q.shape
    assert B == 1
    FF = B_w3.shape[1]
    NC = D // LANES
    NG = BLK // 8
    NBL = S // (PH * BLK)
    FP = -(-FF // (2 * LANES)) * 2 * LANES
    TILES = (384, 384, 576, 704)
    assert sum(TILES) == S
    TB = 512

    args = (A_q.reshape(S, D), A_k.reshape(S, D), A_v.reshape(S, D), A_shift_k.T, A_ssm_k,
            A_ssm_D, B_w1, B_w2, B_w3.T, B_w4, c, w_mod)
    scratch = [
        pltpu.VMEM((S, D), BF16),
        pltpu.VMEM((NC, S + KP, LANES), BF16),
        pltpu.VMEM((NC, S + VP, LANES), BF16),
        pltpu.VMEM((4, D), BF16),
        pltpu.VMEM((NC, LANES, S), BF16),
        pltpu.VMEM((D,), BF16),
        pltpu.VMEM((NC, D, LANES), BF16),
        pltpu.VMEM((NC, D, LANES), BF16),
        pltpu.VMEM((NC, FF, LANES), BF16),
        pltpu.VMEM((NC, FF, LANES), BF16),
        pltpu.VMEM((1, D), BF16),
        pltpu.VMEM((D, 6 * D), BF16),
        pltpu.VMEM((PH, 2 * BLK, BLK), BF16),
        pltpu.VMEM((PH, 2, BLK, BLK), BF16),
        pltpu.VMEM((NC, S, LANES), BF16),
        pltpu.VMEM((NC, NG, NBL, PH, 2, 8, LANES), F32),
        pltpu.VMEM((NC, NG, NBL, PH, 2, 8, LANES), F32),
        pltpu.VMEM((NC, NBL, PH, 2 * BLK, LANES), BF16),
        pltpu.VMEM((NBL, PH, BLK, LANES), BF16),
        pltpu.VMEM((NC, S + YP, LANES), F32),
        pltpu.VMEM((6, 8, D), F32),
        pltpu.VMEM((NC, 8, LANES), F32),
        pltpu.VMEM((NC, S + 16, LANES), F32),
        pltpu.VMEM((S, D), F32),
        pltpu.VMEM((S, D), F32),
        pltpu.VMEM((NC, S, LANES), BF16),
        pltpu.VMEM((7, 7, FP // 512 * LANES, LANES), BF16),
        pltpu.VMEM((7, 7, FP // 512, D // 4, LANES), BF16),
        pltpu.VMEM((7, 2, D // 4, LANES), BF16),
        [pltpu.VMEM((2, GR, LANES), F32)] * 4,
        pltpu.VMEM((2, ZR, LANES), F32),
        pltpu.VMEM((TB, LANES), BF16),
        pltpu.VMEM((10, 2, S // 2, LANES), BF16),
        pltpu.VMEM((10, 2, S // 2, LANES), BF16),
        pltpu.VMEM((7, 2, 2 * LANES, LANES), BF16),
        pltpu.VMEM((7, 2, 2 * LANES, LANES), BF16),
        pltpu.VMEM((7, 7, (FF - FP // 512 * 512) // 4, LANES), BF16),
        pltpu.VMEM((4, FF // 4, TB // 4), F32),
        pltpu.VMEM((NC, FP, LANES), BF16),
        pltpu.VMEM((D, LANES), F32),
        pltpu.SemaphoreType.DMA((16 + len(TILES),)),
        pltpu.SemaphoreType.DMA((1,)),
    ]
    out = pl.pallas_call(
        functools.partial(_kernel, S=S, D=D, FF=FF, TILES=TILES, TB=TB),
        in_specs=[pl.BlockSpec(memory_space=pl.ANY)] * len(args),
        out_specs=pl.BlockSpec(memory_space=pl.ANY),
        out_shape=jax.ShapeDtypeStruct((S, D), BF16),
        scratch_shapes=scratch,
        compiler_params=pltpu.CompilerParams(
            vmem_limit_bytes=126 * 1024 * 1024,
            disable_bounds_checks=True,
            disable_semaphore_checks=True,
        ),
    )(*args)
    return out.reshape(B, S, D)
```

```python
import functools
import math

import jax
import jax.numpy as jnp
from jax import lax
import jax.experimental.pallas as pl
import jax.experimental.pallas.tpu as pltpu

F32 = jnp.float32
BF16 = jnp.bfloat16
U32 = jnp.uint32

LANES = 128
BLK = 128
PH = 4
EPS = 1e-05
TB = 512
TQ = TB // 4
HALO = 32
TILES = (384, 384, 576, 704)
BLOCKWISE1 = (3,)
BLOCKWISE2 = (2, 3)
IN_LOOP = (2, 4, 1, 3, 0)
GPAD = 8
GROWS = 1768
XEND = 45
CUT = 78

_ORDER = (2, 4, 1, 3, 0, 6, 5)
_RAW = (1, 4)
_LHS = (((0, 0), 1, (1, 1)), ((1, 0), 1, (1, 1)), ((0, 0),), ((1, 1),),
        ((0, 0), 1, (0, 1)), ((1, 0), -1, (0, 0)), ((0, 1), -1, (1, 1)))
_RHS = (((0, 0), 1, (1, 1)), ((0, 0),), ((0, 1), -1, (1, 1)), ((1, 0), -1, (0, 0)),
        ((1, 1),), ((0, 0), 1, (0, 1)), ((1, 0), 1, (1, 1)))


def _operand(terms, blk):
    x = blk(*terms[0])
    if len(terms) > 1:
        y = blk(*terms[2])
        x = x + y if terms[1] > 0 else x - y
    return x


def _all_operands(table, b00, b01, b10, b11):
    blocks = ((b00, b01), (b10, b11))
    return [_operand(terms, lambda i, j: blocks[i][j]) for terms in table]


def _block(m, which):
    if which == 0:
        return (m[3] - m[4]) + m[0] + m[6]
    if which == 1:
        return m[2] + m[4]
    if which == 2:
        return m[1] + m[3]
    return (m[2] - m[1]) + m[0] + m[5]


def _combine(m):
    return [_block(m, which) for which in range(4)]


def _as_bf16(x):
    return pltpu.bitcast(x, BF16)


def _lo(x):
    return pltpu.bitcast(x << 16, F32)


def _hi(x):
    return pltpu.bitcast(x & jnp.uint32(0xFFFF0000), F32)


def _dft4(re, im, sign):
    ar, ai = re[0] + re[2], im[0] + im[2]
    br, bi = re[0] - re[2], im[0] - im[2]
    cr, ci = re[1] + re[3], im[1] + im[3]
    dr, di = re[1] - re[3], im[1] - im[3]
    o0 = (ar + cr, ai + ci)
    o2 = (ar - cr, ai - ci)
    m = (br + di, bi - dr)
    p = (br - di, bi + dr)
    o1, o3 = (m, p) if sign < 0 else (p, m)
    return [o0[0], o1[0], o2[0], o3[0]], [o0[1], o1[1], o2[1], o3[1]]


def _ln(x, eps=EPS, unit=True):
    n = x.shape[-1]
    s1 = jnp.sum(x, axis=-1, keepdims=True)
    m = s1 * (1.0 / n)
    v = jnp.maximum(jnp.sum(x * x, axis=-1, keepdims=True) + (n * eps - s1 * m), n * eps)
    e = jnp.log(v) * (-0.5 / math.log(2.0))
    return (x - m) * jnp.exp2(e + 0.5 * math.log2(n) if unit else e)


def _gelu2(x):
    c0 = math.sqrt(2.0 / math.pi)
    return x + x * jnp.tanh(x * (c0 + (c0 * 0.044715) * (x * x)))


def _dot(a, b):
    return jnp.dot(a, b, preferred_element_type=F32)


def _dot_nt(a, b):
    return lax.dot_general(a, b, (((1,), (1,)), ((), ())), preferred_element_type=F32)


def _rows8(x, repeat=1):
    return [x[8 * r:8 * r + 8, 0:LANES] for r in range(x.shape[0] // 8) for _ in range(repeat)]


def _chunks(r0, r1, k, unit=16):
    n = (r1 - r0) // unit
    cuts = [r0 + unit * ((n * j) // k) for j in range(k + 1)]
    return list(zip(cuts[:-1], cuts[1:]))


def _pick(toks, n, free=0):
    idx = [(r * (len(toks) + free)) // n - free for r in range(n)]
    return [toks[i] if i >= 0 else None for i in idx]


def _kernel(q_hbm, k_hbm, v_hbm, sh_hbm, sk_hbm, sd_hbm, w1_hbm, w2_hbm, w3_hbm, w4_hbm, c_hbm, wm_hbm,
            o_hbm,
            q_v, k_v, v_v, sh_v, sk_v, sd_v, w1_v, w2_v, w3_v, w4_v, c_v, wm_v,
            fw_s, iv_s, o_v, u_s, kk_s, vv_s, wu_s, y_s, mod_s, par_s, h1_s, x_s, h_s, z_s,
            s3_s, s4_s, e4_s, g_s, zf_s, zr_s, l1_s, l2_s, s1_s, s2_s, rh_s, wt_s, scol_s,
            sem, sem_o,
            *, S, D, FF):
    NC = D // LANES
    NG = BLK // 8
    LB = PH * BLK
    NBL = S // LB
    R = BLK // PH
    HL = LANES // 2

    small = [
        pltpu.make_async_copy(sh_hbm, sh_v, sem.at[0]),
        pltpu.make_async_copy(sd_hbm, sd_v, sem.at[0]),
        pltpu.make_async_copy(c_hbm, c_v, sem.at[0]),
    ]

    def conv_copies(c):
        static = isinstance(c, int)
        col = pl.ds(c * LANES if static else pl.multiple_of(c * LANES, LANES), LANES)
        return [
            pltpu.make_async_copy(sk_hbm.at[col, :], sk_v.at[c], sem.at[9 + c if static and c < 2 else 1 + c]),
            pltpu.make_async_copy(k_hbm.at[:, col], k_v.at[c, pl.ds(16, S), :], sem.at[1 + c]),
            pltpu.make_async_copy(v_hbm.at[:, col], v_v.at[c], sem.at[1 + c]),
        ]

    WM = (0, 3 * D, 5 * D, 6 * D)
    wm_copies = [[pltpu.make_async_copy(wm_hbm.at[:, pl.ds(WM[j], WM[j + 1] - WM[j])],
                                        wm_v.at[:, pl.ds(WM[j], WM[j + 1] - WM[j])], sem.at[6 + j])]
                 for j in range(3)]
    w_copies = [[pltpu.make_async_copy(src.at[:, pl.ds(c * LANES, LANES)], dst.at[c], sem.at[12 + j])
                 for c in range(NC)]
                for j, (src, dst) in enumerate(((w1_hbm, w1_v), (w2_hbm, w2_v), (w3_hbm, w3_v), (w4_hbm, w4_v)))]

    B0 = [0]
    for n in TILES:
        B0.append(B0[-1] + n)
    NA = len(TILES)
    A0 = [0] + [r + HALO for r in B0[1:-1]] + [S]
    q_copies = [
        [pltpu.make_async_copy(q_hbm.at[pl.ds(A0[t], A0[t + 1] - A0[t])], q_v.at[pl.ds(A0[t], A0[t + 1] - A0[t])],
                               sem.at[16 + t])]
        for t in range(NA)
    ]

    def start_all(cps, priority=0):
        for cp in cps:
            cp.start(priority=priority)

    def wait_all(cps):
        for cp in cps:
            cp.wait()

    first, second = conv_copies(0), conv_copies(1)
    start_all(first[:1] + small + first[1:] + second)

    for c in range(NC):
        k_v[c, 0:16, :] = jnp.zeros((16, LANES), BF16)
        h1_s[c, 0:8, :] = jnp.zeros((8, LANES), F32)
        h1_s[c, S + 8:S + 16, :] = jnp.zeros((8, LANES), F32)

    prow = lax.broadcasted_iota(jnp.int32, (BLK, BLK), 0)
    pcol = lax.broadcasted_iota(jnp.int32, (BLK, BLK), 1)
    ang = (((4 * prow + 1) * pcol) & (4 * BLK - 1)).astype(F32) * (2.0 * math.pi / (4 * BLK))
    tw = (4 * prow + 1).astype(F32) * (2.0 * math.pi / (4 * LB))
    mr, mi = jnp.cos(ang), -jnp.sin(ang)
    twr, twi = jnp.cos(tw), -jnp.sin(tw)
    eye = jnp.where(prow == pcol, 1.0 / LB, 0.0).astype(BF16)
    for i in range(PH):
        both = jnp.stack([mr.reshape(NG, 8, BLK), mi.reshape(NG, 8, BLK)], axis=1).reshape(2 * BLK, BLK)
        fw_s[i] = both.astype(BF16)
        for h in range(2):
            iv_s[i, h] = _dot_nt(eye, both[h * BLK:(h + 1) * BLK, :].astype(BF16)).astype(BF16)
        if i + 1 < PH:
            mr, mi = mr * twr - mi * twi, mr * twi + mi * twr
    perm = jnp.where(pcol == (prow % R) * PH + prow // R, 1.0, 0.0).astype(BF16)

    wait_all(small)
    shf = sh_v[...].astype(F32)
    sdf = sd_v[...].astype(F32).reshape(1, D)
    for c in range(NC):
        par_s[c, 0:4, :] = shf[:, c * LANES:(c + 1) * LANES]
        par_s[c, 4:5, :] = sdf[:, c * LANES:(c + 1) * LANES]
    cf = c_v[...].astype(F32)
    sc = (cf * jax.nn.sigmoid(cf)).astype(BF16)
    sc16 = jnp.broadcast_to(sc, (16, D))
    scol_s[...] = jnp.broadcast_to(sc.astype(F32), (LANES, D)).T

    def mod_chunk(j):
        mod_s[j] = _dot(sc16, wm_v[:, j * D:(j + 1) * D])[0:8, :]

    (fw_u, iv_u, k_u, v_u, wu_u, vv_u, z_u, l1_u, l2_u, w1_u, w2_u, s1_u, s2_u, w3_u, w4_u, wt_u, s3_u, s4_u,
     e4_u, zr_u) = (r.bitcast(U32) for r in (fw_s, iv_s, k_v, v_v, wu_s, vv_s, z_s, l1_s, l2_s, w1_v, w2_v,
                                             s1_s, s2_s, w3_v, w4_v, wt_s, s3_s, s4_s, e4_s, zr_s))

    never = twr[0:8, :] > 2.0

    def after(token, x):
        if token.dtype != x.dtype:
            token = pltpu.bitcast(token, x.dtype)
        return jnp.where(jnp.broadcast_to(never, x.shape), token, x)

    def hold(x, tks):
        f = len([k for k in tks if k is None])
        n = len(tks)
        head = after(jnp.stack(tks[f:]), x[8 * f:, 0:LANES].reshape(n - f, 8, LANES)).reshape(8 * (n - f), LANES)
        if f:
            head = jnp.concatenate([x[:8 * f, 0:LANES], head], axis=0)
        return head if x.shape[1] == LANES else jnp.concatenate([head, x[:, LANES:]], axis=1)

    def hold16(x, tks):
        x4 = x.reshape(len(tks), 2, 8, LANES)
        return jnp.stack([after(jnp.stack(tks), x4[:, 0]), x4[:, 1]], axis=1).reshape(x.shape)

    def perm_k(c, b, toks):
        kt = [_dot_nt(perm, sk_v[c, :, b * LB + t * BLK:b * LB + (t + 1) * BLK]) for t in range(PH)]
        toks += _rows8(kt[0])[::2]
        return [jnp.concatenate([kt[t][i * R:(i + 1) * R, :] for t in range(PH)], axis=0).astype(BF16)
                for i in range(PH)]

    def spectrum(comps, dst, slot, b, toks, dc=None, pins=None):
        tr, ti = [], []
        for i in range(PH):
            lhs = fw_u[i]
            if pins is not None and i < len(pins):
                lhs = after(pins[i], lhs.reshape(NG, 8, LANES)).reshape(BLK, LANES)
            t4 = _dot(_as_bf16(lhs), comps[i]).reshape(NG, 2, 8, LANES)
            tr.append(t4[:, 0])
            ti.append(t4[:, 1])
        toks += [ti[PH - 1][g] for g in range(NG)]
        if dc is not None:
            tr[0] = tr[0] + dc
        sr, si = _dft4(tr, ti, -1)
        for qq in range(PH):
            dst[slot, :, b, qq, 0] = sr[qq]
            dst[slot, :, b, qq, 1] = si[qq]

    def gated(c, b):
        w = [par_s[c, t:t + 1, :] for t in range(4)]
        kc = {}
        for o in range(-2, 2):
            words = k_u[c, pl.ds(8 + b * (LB // 2) + o, BLK, stride=2), :]
            if o > -2:
                kc[2 * o] = _lo(words)
            kc[2 * o + 1] = _hi(words)
        vc = {}
        for o in range(2):
            words = v_u[c, pl.ds(b * (LB // 2) + o, BLK, stride=2), :]
            vc[2 * o] = _lo(words)
            vc[2 * o + 1] = _hi(words)
        for i in range(PH):
            ks = kc[i] * w[0]
            for t in range(1, 4):
                ks = ks + kc[i - t] * w[t]
            wu_s[b, i] = (ks * vc[i]).astype(BF16)
        return [wu_u[b, i] for i in range(PH)]

    def kv_pins(kvb):
        return [jnp.stack([kvb[2 * m + (r % 2)][8 * (r // 2):8 * (r // 2) + 8, :] for r in range(NG)])
                for m in range(2)]

    def products(c, us, ks, toks):
        n = len(toks) - 3
        cum = (44, 128, 244, 392)
        zp = None
        for o in range(NBL):
            tk = jnp.stack([toks[max(0, ((g * cum[-1] + cum[o]) * n) // (cum[-1] * NG) - 1)] for g in range(NG)])
            zr, zi = [], []
            for qq in range(PH):
                accr = acci = None
                for b in range(o + 1):
                    a_, b_ = us[0, :, b, qq, 0], us[0, :, b, qq, 1]
                    c_, d_ = ks[0, :, o - b, qq, 0], ks[0, :, o - b, qq, 1]
                    if qq == 0 and b == o:
                        a_ = after(tk, a_)
                    tr_ = a_ * c_ - b_ * d_
                    ti_ = a_ * d_ + b_ * c_
                    accr = tr_ if accr is None else accr + tr_
                    acci = ti_ if acci is None else acci + ti_
                zr.append(accr)
                zi.append(acci)
            if zp is None:
                yr, yi = zr, zi
            else:
                yr = [zr[qq] - zp[1][qq] for qq in range(PH)]
                yi = [zi[qq] + zp[0][qq] for qq in range(PH)]
            zp = (zr, zi)
            vr, vi = _dft4(yr, yi, +1)
            for i in range(PH):
                vv_s[c, o, i] = jnp.stack([vr[i], vi[i]], axis=1).reshape(2 * BLK, LANES).astype(BF16)

    def inverse(c, toks, pins):
        for o in range(NBL):
            for i in range(PH):
                yv = None
                for h in range(2):
                    lhs = iv_u[i, h]
                    if pins is not None and h == 0:
                        pin = pins[o][i % 2][8 * (i // 2):8 * (i // 2) + 8]
                        lhs = after(pin, lhs.reshape(8, 8, LANES)).reshape(HL, LANES)
                    t = _dot(_as_bf16(lhs), _as_bf16(vv_u[c, o, i, h * HL:(h + 1) * HL, :]))
                    yv = t if yv is None else yv + t
                if i % 2 == 0:
                    toks += _rows8(yv)[::2]
                y_s[c, pl.ds(o * LB + i, BLK, stride=PH), :] = yv

    def conv_round(c, fwd, mul, inv):
        toks = []
        kv = pins = None
        cur = 1 if mul else 0
        if fwd or mul:
            win = pl.ds(c - cur, 2 if fwd and mul else 1)
            us, ks = u_s.at[win], kk_s.at[win]
        if 'u' in fwd:
            kv = [gated(c, b) for b in range(NBL)]
            pins = [kv_pins(kv[b]) for b in range(NBL)]
        if inv:
            inverse(c - 2, toks, pins)
            if fwd:
                toks = []
        if 'k' in fwd:
            comps = [perm_k(c, b, toks) for b in range(NBL)]
        for b in range(NBL):
            if 'k' in fwd:
                spectrum(comps[b], ks, cur, b, toks, par_s[c, 4:5, :] if b == 0 else None)
            if 'u' in fwd:
                pin = pins[b + 2] if not inv and b + 2 < NBL else None
                spectrum([_as_bf16(x) for x in kv[b]], us, cur, b, toks, None, pin)
        if mul:
            products(c - 1, us, ks, toks)

    def lane_tiles(x):
        return [x[:, c * LANES:(c + 1) * LANES] for c in range(NC)]

    def stage_p1(r0, r1, tks=None):
        ga = mod_s[2, 0:1, :]
        a_mul, a_add = ga * (1.0 + mod_s[1, 0:1, :]) * math.sqrt(D), ga * mod_s[0, 0:1, :]
        q = q_v[r0:r1, :].astype(F32)
        if tks is not None:
            q = hold(q, tks)
        y = jnp.concatenate([y_s[c, r0:r1, :] for c in range(NC)], axis=1)
        x = q + (_ln(q, unit=False) * a_mul + a_add) * y
        x_s[r0:r1, :] = x
        return _ln(x, unit=False)

    def store_row_ops(dst, base, r0, r1, cols, tks=None):
        hv = []
        for x in cols:
            x4 = x.reshape(x.shape[0] // 32, 2, 16, LANES)
            hv.append([x4[:, e].reshape(x.shape[0] // 2, LANES) for e in range(2)])
        for k2 in range(2):
            a00, a01, a10, a11 = hv[k2][0], hv[2 + k2][0], hv[k2][1], hv[2 + k2][1]
            if tks is not None:
                a00, a11 = hold16(a00, tks), hold16(a11, tks)
            for o, x in enumerate(_all_operands(_LHS, a00, a01, a10, a11) + [a01, a10, hv[NC - 1][k2]]):
                dst[o, k2, (r0 - base) // 2:(r1 - base) // 2, :] = x.astype(BF16)

    L1B = A0[BLOCKWISE1[0]]
    L2B = B0[BLOCKWISE2[0]]

    def stage_p2(r0, r1, nx, blockwise=False):
        h = nx * ((1.0 + mod_s[4, 0:1, :]) * (2.0 * math.sqrt(D))) + 2.0 * mod_s[3, 0:1, :]
        h_s[r0:r1, :] = h
        zn = lane_tiles(_ln(h, 4.0 * EPS))
        if blockwise:
            store_row_ops(l1_s, L1B, r0, r1, zn)
        else:
            for c in range(NC):
                z_s[c, r0:r1, :] = zn[c].astype(BF16)

    def stage_p(t, toks):
        lo, hi = A0[t], A0[t + 1]
        stage_p2(lo, hi, stage_p1(lo, hi, _pick(toks, (hi - lo) // 8, 90)), t in BLOCKWISE1)

    def filler(t):
        red = jnp.sum(y_s[t, 0:768, :], axis=-1, keepdims=True).reshape(96, 8, 1)
        spare = (NC - 1) * (TQ + 8) + 8 * t
        zf_s[1, spare:spare + 8, :] = jnp.broadcast_to(jnp.sum(red, axis=0), (8, LANES))

    def square_ops(src, dst, toks):
        HK = 2 * LANES
        tks = _pick(toks, 2 * HK // 16)
        for n2 in range(2):
            tk = tks[n2 * (HK // 16):(n2 + 1) * (HK // 16)]
            blk = lambda k, n: src[2 * n + n2, k * HK:(k + 1) * HK, :].astype(F32)
            for o, x in enumerate(_all_operands(_RHS, hold16(blk(0, 0), tk), blk(0, 1), blk(1, 0), hold16(blk(1, 1), tk))):
                if o not in _RAW:
                    dst[o, n2] = x.astype(BF16)

    def block_dots(ops_u, base, prepare, w_u, s_u, parts, emit, light, heavy):
        toks = []

        def timed(x, weight):
            toks.extend(_rows8(x, weight))
            return x

        def weave(top, bot):
            n = top.shape[0] // 16
            return jnp.stack([top.reshape(n, 16, LANES), bot.reshape(n, 16, LANES)], axis=1).reshape(32 * n, LANES)

        def main(get):
            m = [None] * 7
            rem = [None, None]
            for o in ('t', 2, 4, 'b', 1, 3, 0, 6, 5):
                if o in ('t', 'b'):
                    e = 0 if o == 't' else 1
                    rhs = jnp.concatenate([w_u[c, 2 * LANES:D // 2, :] for c in range(NC - 1)], axis=1)
                    rem[e] = timed(_dot(get([(9, e)]), _as_bf16(rhs)), light)
                    continue
                if o in _RAW:
                    d = _RAW.index(o)
                    rhs = jnp.concatenate([w_u[2 * d + n2, d * LANES:(d + 1) * LANES, :] for n2 in range(2)], axis=1)
                else:
                    rhs = jnp.concatenate([s_u[o, n2] for n2 in range(2)], axis=1)
                m[o] = timed(_dot(get([(o, 0), (o, 1)]), _as_bf16(rhs)), heavy if o in (4, 3, 6, 5) else light)
            c00, c01, c10, c11 = _combine(m)
            top = jnp.concatenate([c00, c01], axis=1) + rem[0]
            bot = jnp.concatenate([c10, c11], axis=1) + rem[1]
            return [weave(top[:, c * LANES:(c + 1) * LANES], bot[:, c * LANES:(c + 1) * LANES]) for c in range(NC - 1)]

        def last(get):
            w = _as_bf16(w_u[NC - 1])
            return weave(timed(_dot(get([(2, 0), (2, 1), (7, 0), (7, 1), (9, 0)]), w), light),
                         timed(_dot(get([(8, 0), (8, 1), (3, 0), (3, 1), (9, 1)]), w), light))

        mark = None
        for j, (r0, r1) in enumerate(parts):
            prepare(r0, r1, None if mark is None else toks[mark:])
            mark = len(toks)
            get = lambda keys: _as_bf16(jnp.concatenate(
                [ops_u[o, e, (r0 - base) // 4:(r1 - base) // 4, :] for o, e in keys], axis=1))
            if j % 2:
                tail = last(get)
                emit(r0, r1, main(get) + [tail])
            else:
                emit(r0, r1, main(get) + [last(get)])
        return toks

    def stage_m1(t, k):
        def emit(r0, r1, cols):
            out = [_gelu2(x) for x in cols]
            for c in range(NC):
                h1_s[c, r0 + 8:r1 + 8, :] = out[c]
            return out

        if t in BLOCKWISE1:
            return block_dots(l1_u, L1B, lambda *_: None, w1_u, s1_u, _chunks(A0[t], A0[t + 1], k, 32), emit, 3, 2)
        toks = []
        for r0, r1 in _chunks(A0[t], A0[t + 1], k):
            lhs = jnp.concatenate([z_u[c, r0 // 2:r1 // 2, :] for c in range(NC)], axis=1)
            w = jnp.concatenate([w1_u[c] for c in range(NC)], axis=1)
            for x in emit(r0, r1, lane_tiles(_dot(_as_bf16(lhs), _as_bf16(w)))):
                toks += _rows8(x, 2)
        return toks

    def shifted(r0, r1):
        n, grp, shifts = r1 - r0, D // 4, (-1, 1, -2, 2)
        lane = lax.broadcasted_iota(jnp.int32, (n, LANES), 1)
        cols = []
        for c in range(NC):
            lo, hi = c * LANES, (c + 1) * LANES
            g_lo, g_hi = lo // grp, (hi - 1) // grp
            val = h1_s[c, pl.ds(r0 + 8 + shifts[g_lo], n), :]
            if g_hi != g_lo:
                other = h1_s[c, pl.ds(r0 + 8 + shifts[g_hi], n), :]
                val = jnp.where(lane < (g_hi * grp - lo), val, other)
            cols.append(val)
        return cols

    def stage_m2(t, k, before=None):
        def emit(r0, r1, cols):
            x1 = h_s[r0:r1, :] + jnp.concatenate(cols, axis=1)
            h_s[r0:r1, :] = x1
            return x1

        if t in BLOCKWISE2:
            def prepare(r0, r1, prev):
                prev = before if prev is None else prev
                prev = prev[len(prev) // 8:(len(prev) * 7) // 8]
                store_row_ops(l2_s, L2B, r0, r1, shifted(r0, r1), _pick(prev, (r1 - r0) // 32))
            return block_dots(l2_u, L2B, prepare, w2_u, s2_u, _chunks(B0[t], B0[t + 1], k, 32), emit, 2, 2)
        toks = []
        for r0, r1 in _chunks(B0[t], B0[t + 1], k):
            w = jnp.concatenate([w2_u[c] for c in range(NC)], axis=1)
            hs = _dot(jnp.concatenate(shifted(r0, r1), axis=1).astype(BF16), _as_bf16(w))
            for x in lane_tiles(emit(r0, r1, [hs])):
                toks += _rows8(x, 3)
        return toks

    NT = S // TB
    FQ = FF // 4
    NS = FQ // LANES
    LQ = FQ - NS * LANES
    CQ = LANES // 4
    QR = LANES + CQ
    BLOCKS = [(2 * r1 + r2, 2 * h + p)
              for r1, h in ((0, 0), (1, 0), (0, 1), (1, 1)) for r2 in range(2) for p in range(2)]

    def z_rows(rq, c):
        lo = (NC * rq + c) * (TQ + 8)
        return slice(lo, lo + TQ)

    def store_z(r0, slot, toks, q0=0, q1=4):
        n = (q1 - q0) * TQ
        rows = pl.ds(r0 + q0 * TQ if isinstance(r0, int) else pl.multiple_of(r0 + q0 * TQ, TQ), n)
        zn = lane_tiles(_ln(hold(h_s[rows, :], _pick(toks, n // 8)), 4.0 * EPS))
        for rq in range(q0, q1):
            for c in range(NC - 1):
                zf_s[slot, z_rows(rq, c), :] = zn[c][(rq - q0) * TQ:(rq - q0 + 1) * TQ]
        zr_s[q0 * TQ:q1 * TQ, :] = zn[NC - 1].astype(BF16)

    def w3_ops(toks):
        ng = FQ // 16
        blk = lambda c, d: w3_v[c, d * FQ:(d + 1) * FQ, :].astype(F32)
        outer = [[_all_operands(_RHS, blk(k2, p), blk(k2, 2 + p), blk(2 + k2, p), blk(2 + k2, 2 + p))
                  for p in range(2)] for k2 in range(2)]
        for k, i in enumerate((1, 5, 2, 4, 0, 3, 6)):
            tk = [toks[((k + r * 7) * len(toks)) // (7 * ng)] for r in range(ng)]
            for j, x in enumerate(_all_operands(_RHS, hold16(outer[0][0][i], tk), outer[0][1][i], outer[1][0][i],
                                                hold16(outer[1][1][i], tk))):
                if i not in _RAW or j not in _RAW:
                    s3_s[i, j] = x.astype(BF16)

    def transpose_w4(toks):
        order = [(c, n) for n in (4 * NS, 4 * NS + 1) + tuple(range(4 * NS)) for c in range(NC)]
        for k, (c, n) in enumerate(order):
            if n >= 4 * NS:
                ends = [(2 * (n - 4 * NS) + p + 1) * FQ // 2 for p in range(2)]
                x = jnp.concatenate([w4_u[c, e - LQ // 2:e, :] for e in ends]
                                    + [jnp.zeros((HL - LQ, LANES), U32)], axis=0)
            else:
                lo = (n % 4) * FQ // 2 + (n // 4) * HL
                x = w4_u[c, lo:lo + HL, :]
            x = jnp.concatenate([after(toks[(k * len(toks)) // len(order)], x[0:8]), x[8:]], axis=0)
            wt_s[c, n] = _as_bf16(x).astype(F32).T.astype(BF16)

    def w4_ops(i, zero, toks):
        ng = QR // 16
        total = (NS * 7 + 2) * ng
        tk = lambda pos, step: [toks[((pos + r * step) * len(toks)) // total] for r in range(ng)]
        quarter = lambda n, d: jnp.concatenate(
            [wt_s[d, n].astype(F32), wt_s[NC - 1, n, d * CQ:(d + 1) * CQ, :].astype(F32)], axis=0)
        if i not in _RAW:
            for e in range(2):
                x = _operand(_RHS[i], lambda h, d: quarter(4 * NS + h, 2 * d + e))
                e4_s[i + zero, e] = hold16(x, tk(e * ng, 1)).astype(BF16)
        for st in range(NS):
            t = [[_operand(_RHS[i], lambda h, d: quarter(4 * st + 2 * h + p, 2 * d + e)) for e in range(2)]
                 for p in range(2)]
            tks = tk((2 + st * 7) * ng, 7)
            for j, x in enumerate(_all_operands(_RHS, hold16(t[0][0], tks), t[0][1], t[1][0], hold16(t[1][1], tks))):
                if i not in _RAW or j not in _RAW:
                    s4_s[i + zero, j, st] = x.astype(BF16)

    def gate_row(toks):
        ng = D // 8
        col = after(jnp.stack(_pick(toks, ng)), scol_s[...].reshape(ng, 8, LANES))
        for c in range(NC):
            wf = wm_v[:, (NC * NC + c) * LANES:(NC * NC + c + 1) * LANES].astype(F32).reshape(ng, 8, LANES)
            acc = col[0] * wf[0]
            for r in range(1, ng):
                acc = acc + col[r] * wf[r]
            mod_s[NC, :, c * LANES:(c + 1) * LANES] = jnp.broadcast_to(jnp.sum(acc, axis=0, keepdims=True), (8, LANES))

    def rem3(rq, d, pieces=1):
        z = _as_bf16(zr_u[rq * (TQ // 2):(rq + 1) * (TQ // 2), :])
        return jnp.concatenate([_dot_nt(_as_bf16(w3_u[NC - 1, lo // 2:hi // 2, :]), z)
                                for lo, hi in _chunks(d * FQ, (d + 1) * FQ, pieces)], axis=0)

    def lead_in():
        head = [rem3(*key) for key in BLOCKS[:4]]
        for k in range(4):
            rh_s[k] = head[k]
        return _rows8(head[0])

    with jax.named_scope("r0a"):
        wait_all(first[:1])
        conv_round(0, 'k', False, False)
    with jax.named_scope("r0_wait"):
        wait_all(first[1:])
    with jax.named_scope("r0b"):
        start_all(conv_copies(2) + conv_copies(3) + conv_copies(4))
        conv_round(0, 'u', False, False)
    with jax.named_scope("r1a"):
        wait_all(second[:1])
        conv_round(1, 'k', True, False)
    with jax.named_scope("r1_wait"):
        wait_all(second[1:])
    with jax.named_scope("r1b"):
        start_all(wm_copies[0] + q_copies[0] + wm_copies[1] + w_copies[0])
        conv_round(1, 'u', False, False)

    def full_round(c, carry):
        wait_all(conv_copies(c))
        conv_round(c, 'ku', True, True)
        return carry

    with jax.named_scope("r234"):
        lax.fori_loop(2, NC, full_round, 0)
    with jax.named_scope("r5"):
        start_all(q_copies[1] + w_copies[1] + sum(q_copies[2:], []) + w_copies[2] + w_copies[3] + wm_copies[2], 1)
        conv_round(NC, '', True, True)
    with jax.named_scope("r6_wait"):
        wait_all(wm_copies[0] + q_copies[0])
    with jax.named_scope("r6"):
        for j in range(3):
            mod_chunk(j)
        conv_round(NC + 1, '', False, True)
        nx0 = stage_p1(0, A0[1])
    with jax.named_scope("p2_wait"):
        wait_all(wm_copies[1])
    with jax.named_scope("p2"):
        mod_chunk(4)
        mod_chunk(3)
        stage_p2(0, A0[1], nx0)
    with jax.named_scope("w1_wait"):
        wait_all(w_copies[0])
    with jax.named_scope("m1_0"):
        square_ops(w1_v, s1_s, stage_m1(0, 4)[:-40])
    with jax.named_scope("w2_wait"):
        wait_all(q_copies[1] + w_copies[1])
    with jax.named_scope("m2_0"):
        stage_p(1, stage_m2(0, 4)[:-180])
        filler(0)
    for t in range(1, NA):
        with jax.named_scope("a%d" % t):
            wait_all(q_copies[t + 1] if t + 1 < NA else w_copies[2] + w_copies[3] + wm_copies[2])
            toks = stage_m1(t, 2)
            toks = toks + stage_m2(t, 2, toks[len(toks) - len(toks) // 2:])
            if t + 1 < NA:
                stage_p(t + 1, toks[:-180])
            if t == 1:
                square_ops(w2_v, s2_s, toks[:-30])
            if t == NA - 1:
                transpose_w4(toks[:(len(toks) * XEND) // 100])
                store_z(0, 0, toks[(len(toks) * (XEND + 5)) // 100:(len(toks) * 88) // 100])
                toks = toks + [x for x in lead_in()[:40] for _ in range(2)]
                cut = (len(toks) * CUT) // 100
                gate_row(toks[:(len(toks) * 9) // 10])
                w3_ops(toks[:cut])
                rest = [i for i in range(7) if i not in IN_LOOP]
                for k, i in enumerate(rest):
                    w4_ops(i, 0, toks[cut + k::len(rest)])
            filler(t)

    def out_copy(r0, n, c):
        rows = pl.ds(r0, n)
        return pltpu.make_async_copy(o_v.at[c, rows, :], o_hbm.at[rows, pl.ds(c * LANES, LANES)], sem_o.at[0])

    def raw4(n, d):
        return jnp.concatenate([wt_u[d, n], wt_u[NC - 1, n, d * (CQ // 2):(d + 1) * (CQ // 2), :]], axis=0)

    def mlp_tile(t, carry):
        r0 = pl.multiple_of(t * TB, TB)
        ws = t & 1
        count = [0]

        def fresh():
            count[0] += 1
            return lax.rem(t + 2 * count[0], 2)

        def g_rows(r2, p, lo, hi):
            base = (2 * r2 + p) * (FQ + GPAD)
            return slice(base + lo, base + hi)

        rem = {key: rh_s[k] for k, key in enumerate(BLOCKS[:4])}
        for key in BLOCKS[4:8]:
            rem[key] = rem3(*key)
        early = _rows8(rem[BLOCKS[4]], 2)
        rem[BLOCKS[8]] = rem3(*BLOCKS[8], pieces=4)
        todo = BLOCKS[9:]
        part = [None] * 7
        for i in (4, 3, 0, 6, 1, 2, 5):
            m = [None] * 7
            for j in _ORDER:
                slot = fresh()
                act = _operand(_LHS[j], lambda r2, k2: _operand(
                    _LHS[i], lambda r1, k1: zf_s[slot, z_rows(2 * r1 + r2, 2 * k1 + k2), :])).astype(BF16)
                if i in _RAW and j in _RAW:
                    d = 2 * _RAW.index(i) + _RAW.index(j)
                    wij = w3_u[d, d * (FQ // 2):(d + 1) * (FQ // 2), :]
                else:
                    wij = s3_u[i, j]
                m[j] = _dot_nt(_as_bf16(wij), act)
            key = todo.pop(0)
            rem[key] = rem3(*key)
            part[i] = _combine(m)
            if i in (4, 3, 0):
                early += _rows8(m[_ORDER[0]]) + _rows8(m[_ORDER[4]], 2)
        zero = fresh() - ws
        fine = [x for x in early for _ in IN_LOOP]
        hop = len(fine) // (len(IN_LOOP) * 33)
        for k, i in enumerate(IN_LOOP):
            w4_ops(i, zero, fine[k * hop:len(fine) - (len(IN_LOOP) - k) * hop])
        for inner in range(4):
            r2, p = inner // 2, inner % 2
            for blk, pre in enumerate(_combine([part[i][inner] for i in range(7)])):
                g_s[blk][ws, g_rows(r2, p, 0, FQ), :] = _gelu2(pre + rem[2 * (blk // 2) + r2, 2 * (blk % 2) + p])

        toks = []
        marks = {}
        part = [[None] * 4 for _ in range(7)]
        for i in _ORDER:
            slot = fresh()
            we = jnp.concatenate([raw4(4 * NS + _RAW.index(i), 2 * _RAW.index(i) + e) if i in _RAW else e4_u[i, e]
                                  for e in range(2)], axis=0)
            ex = []
            for r2 in range(2):
                act = [_operand(_LHS[i], lambda r1, h: g_s[2 * r1 + h][slot, g_rows(r2, p, NS * LANES, FQ), :])
                       for p in range(2)]
                act = jnp.concatenate(act + [jnp.zeros((LANES - 2 * LQ, TQ), F32)], axis=0).astype(BF16)
                ex.append(_dot(_as_bf16(we), act))
            m = [None] * 7
            for j in _ORDER:
                slot = fresh()
                act = _operand(_LHS[j], lambda r2, p: _operand(
                    _LHS[i], lambda r1, h: g_s[2 * r1 + h][slot, g_rows(r2, p, 0, NS * LANES), :])).astype(BF16)
                if i in _RAW and j in _RAW:
                    d = 2 * _RAW.index(i) + _RAW.index(j)
                    wij = [raw4(4 * st + d, d) for st in range(NS)]
                else:
                    wij = [s4_u[i, j, st] for st in range(NS)]
                m[j] = _dot(_as_bf16(jnp.concatenate(wij, axis=1)), act)
                toks += _rows8(m[j])
            part[i] = [x + ex[inner // 2][(inner % 2) * QR:(inner % 2 + 1) * QR]
                       for inner, x in enumerate(_combine(m))]
            marks[i] = len(toks)

        gb = 0.5 * mod_s[NC, 0:1, :]
        nxt = jnp.minimum(t + 1, NT - 1) * TB
        tails = {}
        for i, blk, norm in ((_ORDER[1], 1, (0, 2, 0, 160)), (_ORDER[3], 2, (2, 3, 320, 450)),
                             (_ORDER[5], 0, (3, 4, 600, 730)), (_ORDER[6], 3, None)):
            r1 = blk // 2
            if norm is None:
                toks += [x for x in lead_in()[8:40] for _ in range(3)]
            else:
                store_z(nxt, 1 - ws, toks[norm[2]:norm[3]], norm[0], norm[1])
            pos = [marks[i] + (10 if norm else -32)]

            def finish(rq, c, h2t):
                h2 = hold(h2t.T, toks[pos[0]:pos[0] + TQ // 8])
                pos[0] += TQ // 8
                rows = pl.ds(pl.multiple_of(r0 + rq * TQ, TQ), TQ)
                cols = slice(c * LANES, (c + 1) * LANES)
                o_v[c, rows, :] = (x_s[rows, cols] + gb[:, cols] * (h_s[rows, cols] + h2)).astype(BF16)
                if blk == 3:
                    out_copy(rows.start, TQ, c).start()

            for inner in (1, 2, 0, 3):
                ht = _block([part[k][inner] for k in range(7)], blk)
                rq, c = 2 * r1 + inner // 2, 2 * (blk % 2) + inner % 2
                finish(rq, c, ht[0:LANES])
                tails[rq, c] = ht[LANES:]
            rb = pl.multiple_of(r0 + r1 * 2 * TQ, 2 * TQ)
            if blk != 3:
                for e in range(2):
                    out_copy(rb, 2 * TQ, 2 * (blk % 2) + e).start()
            if blk in (0, 3):
                for rq in (2 * r1, 2 * r1 + 1):
                    finish(rq, NC - 1, jnp.concatenate([tails[rq, c] for c in range(NC - 1)], axis=0))
                if blk == 0:
                    out_copy(rb, 2 * TQ, NC - 1).start()
        return carry

    with jax.named_scope("ph2b"):
        lax.fori_loop(0, NT, mlp_tile, 0)
    with jax.named_scope("tail"):
        pltpu.make_async_copy(o_v, o_v, sem_o.at[0]).wait()


@jax.jit
def pallas_adaLN_cond__ssm_conv_h3__mixer_s_mlp__prompt_kernel(
    A_q: jax.Array,
    A_k: jax.Array,
    A_v: jax.Array,
    A_shift_k: jax.Array,
    A_ssm_k: jax.Array,
    A_ssm_D: jax.Array,
    B_x: jax.Array,
    B_w1: jax.Array,
    B_w2: jax.Array,
    B_w3: jax.Array,
    B_w4: jax.Array,
    c: jax.Array,
    w_mod: jax.Array,
):
    B, S, D = A_q.shape
    FF = B_w3.shape[1]
    assert (B, S, D, FF, A_shift_k.shape[1]) == (1, sum(TILES), 5 * LANES, 1728, 4)
    NC = D // LANES
    NG = BLK // 8
    NBL = S // (PH * BLK)
    NS = FF // 4 // LANES
    n1 = S - sum(TILES[:BLOCKWISE1[0]]) - HALO
    n2 = S - sum(TILES[:BLOCKWISE2[0]])

    args = (A_q.reshape(S, D), A_k.reshape(S, D), A_v.reshape(S, D), A_shift_k.T, A_ssm_k,
            A_ssm_D, B_w1, B_w2, B_w3.T, B_w4, c, w_mod)
    scratch = [
        pltpu.VMEM((S, D), BF16),
        pltpu.VMEM((NC, S + 16, LANES), BF16),
        pltpu.VMEM((NC, S, LANES), BF16),
        pltpu.VMEM((4, D), BF16),
        pltpu.VMEM((NC, LANES, S), BF16),
        pltpu.VMEM((D,), BF16),
        pltpu.VMEM((NC, D, LANES), BF16),
        pltpu.VMEM((NC, D, LANES), BF16),
        pltpu.VMEM((NC, FF, LANES), BF16),
        pltpu.VMEM((NC, FF, LANES), BF16),
        pltpu.VMEM((1, D), BF16),
        pltpu.VMEM((D, 6 * D), BF16),
        pltpu.VMEM((PH, 2 * BLK, BLK), BF16),
        pltpu.VMEM((PH, 2, BLK, BLK), BF16),
        pltpu.VMEM((NC, S, LANES), BF16),
        pltpu.VMEM((NC, NG, NBL, PH, 2, 8, LANES), F32),
        pltpu.VMEM((NC, NG, NBL, PH, 2, 8, LANES), F32),
        pltpu.VMEM((NC, NBL, PH, 2 * BLK, LANES), BF16),
        pltpu.VMEM((NBL, PH, BLK, LANES), BF16),
        pltpu.VMEM((NC, S, LANES), F32),
        pltpu.VMEM((6, 8, D), F32),
        pltpu.VMEM((NC, 8, LANES), F32),
        pltpu.VMEM((NC, S + 16, LANES), F32),
        pltpu.VMEM((S, D), F32),
        pltpu.VMEM((S, D), F32),
        pltpu.VMEM((NC, S, LANES), BF16),
        pltpu.VMEM((7, 7, FF // 4, LANES), BF16),
        pltpu.VMEM((7, 7, NS, D // 4, LANES), BF16),
        pltpu.VMEM((7, 2, D // 4, LANES), BF16),
        [pltpu.VMEM((2, GROWS, TQ), F32)] * 4,
        pltpu.VMEM((2, 4 * NC * (TQ + 8), LANES), F32),
        pltpu.VMEM((TB, LANES), BF16),
        pltpu.VMEM((10, 2, n1 // 2, LANES), BF16),
        pltpu.VMEM((10, 2, n2 // 2, LANES), BF16),
        pltpu.VMEM((7, 2, 2 * LANES, LANES), BF16),
        pltpu.VMEM((7, 2, 2 * LANES, LANES), BF16),
        pltpu.VMEM((4, FF // 4, TQ), F32),
        pltpu.VMEM((NC, 4 * NS + 2, LANES, LANES), BF16),
        pltpu.VMEM((D, LANES), F32),
        pltpu.SemaphoreType.DMA((16 + len(TILES),)),
        pltpu.SemaphoreType.DMA((1,)),
    ]
    out = pl.pallas_call(
        functools.partial(_kernel, S=S, D=D, FF=FF),
        in_specs=[pl.BlockSpec(memory_space=pl.ANY)] * len(args),
        out_specs=pl.BlockSpec(memory_space=pl.ANY),
        out_shape=jax.ShapeDtypeStruct((S, D), BF16),
        scratch_shapes=scratch,
        compiler_params=pltpu.CompilerParams(
            vmem_limit_bytes=120 * 1024 * 1024,
            disable_bounds_checks=True,
            disable_semaphore_checks=True,
        ),
    )(*args)
    return out.reshape(B, S, D)
```

```python
import functools
import math

import jax
import jax.numpy as jnp
from jax import lax
import jax.experimental.pallas as pl
import jax.experimental.pallas.tpu as pltpu

F32 = jnp.float32
BF16 = jnp.bfloat16
U32 = jnp.uint32

LANES = 128
BLK = 128
PH = 4
EPS = 1e-05
TB = 512
TQ = TB // 4
HALO = 32
TILES = (384, 384, 576, 704)
BLOCKWISE1 = (3,)
BLOCKWISE2 = (2, 3)
IN_LOOP = (2, 4, 1, 3, 0)
O4 = (2, 4, 1, 3, 0, 6, 5)
NW = (1, 3, 0, 150, 320, 460, 600, 730)
PLAN = ((4, 1, (0, NW[0], NW[2], NW[3])), (3, 2, (NW[0], NW[1], NW[4], NW[5])), (6, 0, (NW[1], 4, NW[6], NW[7])), (5, 3, None))
FL = (10, 10, 25, -32)
EW = (2, 1, 2)
TRS = (135, 165, 180)
FRS = (45, 90, 90)
WS = (2, 3, 3, 2, 2, 2, 2, 4)
LW = (50, 88)
FI = (48, 96, 96, 96)
SP0 = 4
GPAD = 8
GROWS = 1768
XEND = 45
CUT = 82

_ORDER = (2, 4, 1, 3, 0, 6, 5)
_RAW = (1, 4)
_LHS = (((0, 0), 1, (1, 1)), ((1, 0), 1, (1, 1)), ((0, 0),), ((1, 1),),
        ((0, 0), 1, (0, 1)), ((1, 0), -1, (0, 0)), ((0, 1), -1, (1, 1)))
_RHS = (((0, 0), 1, (1, 1)), ((0, 0),), ((0, 1), -1, (1, 1)), ((1, 0), -1, (0, 0)),
        ((1, 1),), ((0, 0), 1, (0, 1)), ((1, 0), 1, (1, 1)))


def _operand(terms, blk):
    x = blk(*terms[0])
    if len(terms) > 1:
        y = blk(*terms[2])
        x = x + y if terms[1] > 0 else x - y
    return x


def _all_operands(table, b00, b01, b10, b11):
    blocks = ((b00, b01), (b10, b11))
    return [_operand(terms, lambda i, j: blocks[i][j]) for terms in table]


def _block(m, which):
    if which == 0:
        return (m[3] - m[4]) + m[0] + m[6]
    if which == 1:
        return m[2] + m[4]
    if which == 2:
        return m[1] + m[3]
    return (m[2] - m[1]) + m[0] + m[5]


def _combine(m):
    return [_block(m, which) for which in range(4)]


def _as_bf16(x):
    return pltpu.bitcast(x, BF16)


def _lo(x):
    return pltpu.bitcast(x << 16, F32)


def _hi(x):
    return pltpu.bitcast(x & jnp.uint32(0xFFFF0000), F32)


def _dft4(re, im, sign):
    ar, ai = re[0] + re[2], im[0] + im[2]
    br, bi = re[0] - re[2], im[0] - im[2]
    cr, ci = re[1] + re[3], im[1] + im[3]
    dr, di = re[1] - re[3], im[1] - im[3]
    o0 = (ar + cr, ai + ci)
    o2 = (ar - cr, ai - ci)
    m = (br + di, bi - dr)
    p = (br - di, bi + dr)
    o1, o3 = (m, p) if sign < 0 else (p, m)
    return [o0[0], o1[0], o2[0], o3[0]], [o0[1], o1[1], o2[1], o3[1]]


def _ln(x, eps=EPS, unit=True):
    n = x.shape[-1]
    s1 = jnp.sum(x, axis=-1, keepdims=True)
    m = s1 * (1.0 / n)
    v = jnp.maximum(jnp.sum(x * x, axis=-1, keepdims=True) + (n * eps - s1 * m), n * eps)
    e = jnp.log(v) * (-0.5 / math.log(2.0))
    return (x - m) * jnp.exp2(e + 0.5 * math.log2(n) if unit else e)


def _gelu2(x):
    c0 = math.sqrt(2.0 / math.pi)
    return x + x * jnp.tanh(x * (c0 + (c0 * 0.044715) * (x * x)))


def _dot(a, b):
    return jnp.dot(a, b, preferred_element_type=F32)


def _dot_nt(a, b):
    return lax.dot_general(a, b, (((1,), (1,)), ((), ())), preferred_element_type=F32)


def _rows8(x, repeat=1):
    return [x[8 * r:8 * r + 8, 0:LANES] for r in range(x.shape[0] // 8) for _ in range(repeat)]


def _chunks(r0, r1, k, unit=16):
    n = (r1 - r0) // unit
    cuts = [r0 + unit * ((n * j) // k) for j in range(k + 1)]
    return list(zip(cuts[:-1], cuts[1:]))


def _pick(toks, n, free=0):
    idx = [(r * (len(toks) + free)) // n - free for r in range(n)]
    return [toks[i] if i >= 0 else None for i in idx]


def _kernel(q_hbm, k_hbm, v_hbm, sh_hbm, sk_hbm, sd_hbm, w1_hbm, w2_hbm, w3_hbm, w4_hbm, c_hbm, wm_hbm,
            o_hbm,
            q_v, k_v, v_v, sh_v, sk_v, sd_v, w1_v, w2_v, w3_v, w4_v, c_v, wm_v,
            fw_s, iv_s, o_v, u_s, kk_s, vv_s, wu_s, y_s, mod_s, par_s, h1_s, x_s, h_s, z_s,
            s3_s, s4_s, e4_s, g_s, zf_s, zr_s, l1_s, l2_s, s1_s, s2_s, rh_s, wt_s, scol_s,
            sem, sem_o,
            *, S, D, FF):
    NC = D // LANES
    NG = BLK // 8
    LB = PH * BLK
    NBL = S // LB
    R = BLK // PH
    HL = LANES // 2

    small = [
        pltpu.make_async_copy(sh_hbm, sh_v, sem.at[0]),
        pltpu.make_async_copy(sd_hbm, sd_v, sem.at[0]),
        pltpu.make_async_copy(c_hbm, c_v, sem.at[0]),
    ]

    def conv_copies(c):
        static = isinstance(c, int)
        col = pl.ds(c * LANES if static else pl.multiple_of(c * LANES, LANES), LANES)
        return [
            pltpu.make_async_copy(sk_hbm.at[col, :], sk_v.at[c], sem.at[9 + c if static and c < 2 else 1 + c]),
            pltpu.make_async_copy(k_hbm.at[:, col], k_v.at[c, pl.ds(16, S), :], sem.at[1 + c]),
            pltpu.make_async_copy(v_hbm.at[:, col], v_v.at[c], sem.at[1 + c]),
        ]

    WM = (0, 3 * D, 5 * D, 6 * D)
    wm_copies = [[pltpu.make_async_copy(wm_hbm.at[:, pl.ds(WM[j], WM[j + 1] - WM[j])],
                                        wm_v.at[:, pl.ds(WM[j], WM[j + 1] - WM[j])], sem.at[6 + j])]
                 for j in range(3)]
    w_copies = [[pltpu.make_async_copy(src.at[:, pl.ds(c * LANES, LANES)], dst.at[c], sem.at[12 + j])
                 for c in range(NC)]
                for j, (src, dst) in enumerate(((w1_hbm, w1_v), (w2_hbm, w2_v), (w3_hbm, w3_v), (w4_hbm, w4_v)))]

    B0 = [0]
    for n in TILES:
        B0.append(B0[-1] + n)
    NA = len(TILES)
    A0 = [0] + [r + HALO for r in B0[1:-1]] + [S]
    q_copies = [
        [pltpu.make_async_copy(q_hbm.at[pl.ds(A0[t], A0[t + 1] - A0[t])], q_v.at[pl.ds(A0[t], A0[t + 1] - A0[t])],
                               sem.at[16 + t])]
        for t in range(NA)
    ]

    def start_all(cps, priority=0):
        for cp in cps:
            cp.start(priority=priority)

    def wait_all(cps):
        for cp in cps:
            cp.wait()

    first, second = conv_copies(0), conv_copies(1)
    start_all(first[:1] + small + first[1:] + second)

    for c in range(NC):
        k_v[c, 0:16, :] = jnp.zeros((16, LANES), BF16)
        h1_s[c, 0:8, :] = jnp.zeros((8, LANES), F32)
        h1_s[c, S + 8:S + 16, :] = jnp.zeros((8, LANES), F32)

    prow = lax.broadcasted_iota(jnp.int32, (BLK, BLK), 0)
    pcol = lax.broadcasted_iota(jnp.int32, (BLK, BLK), 1)
    ang = (((4 * prow + 1) * pcol) & (4 * BLK - 1)).astype(F32) * (2.0 * math.pi / (4 * BLK))
    tw = (4 * prow + 1).astype(F32) * (2.0 * math.pi / (4 * LB))
    mr, mi = jnp.cos(ang), -jnp.sin(ang)
    twr, twi = jnp.cos(tw), -jnp.sin(tw)
    eye = jnp.where(prow == pcol, 1.0 / LB, 0.0).astype(BF16)
    for i in range(PH):
        both = jnp.stack([mr.reshape(NG, 8, BLK), mi.reshape(NG, 8, BLK)], axis=1).reshape(2 * BLK, BLK)
        fw_s[i] = both.astype(BF16)
        for h in range(2):
            iv_s[i, h] = _dot_nt(eye, both[h * BLK:(h + 1) * BLK, :].astype(BF16)).astype(BF16)
        if i + 1 < PH:
            mr, mi = mr * twr - mi * twi, mr * twi + mi * twr
    perm = jnp.where(pcol == (prow % R) * PH + prow // R, 1.0, 0.0).astype(BF16)

    wait_all(small)
    shf = sh_v[...].astype(F32)
    sdf = sd_v[...].astype(F32).reshape(1, D)
    for c in range(NC):
        par_s[c, 0:4, :] = shf[:, c * LANES:(c + 1) * LANES]
        par_s[c, 4:5, :] = sdf[:, c * LANES:(c + 1) * LANES]
    cf = c_v[...].astype(F32)
    sc = (cf * jax.nn.sigmoid(cf)).astype(BF16)
    sc16 = jnp.broadcast_to(sc, (16, D))
    scol_s[...] = jnp.broadcast_to(sc.astype(F32), (LANES, D)).T

    def mod_chunk(j):
        mod_s[j] = _dot(sc16, wm_v[:, j * D:(j + 1) * D])[0:8, :]

    (fw_u, iv_u, k_u, v_u, wu_u, vv_u, z_u, l1_u, l2_u, w1_u, w2_u, s1_u, s2_u, w3_u, w4_u, wt_u, s3_u, s4_u,
     e4_u, zr_u) = (r.bitcast(U32) for r in (fw_s, iv_s, k_v, v_v, wu_s, vv_s, z_s, l1_s, l2_s, w1_v, w2_v,
                                             s1_s, s2_s, w3_v, w4_v, wt_s, s3_s, s4_s, e4_s, zr_s))

    never = twr[0:8, :] > 2.0

    def after(token, x):
        if token.dtype != x.dtype:
            token = pltpu.bitcast(token, x.dtype)
        return jnp.where(jnp.broadcast_to(never, x.shape), token, x)

    def hold(x, tks):
        f = len([k for k in tks if k is None])
        n = len(tks)
        head = after(jnp.stack(tks[f:]), x[8 * f:, 0:LANES].reshape(n - f, 8, LANES)).reshape(8 * (n - f), LANES)
        if f:
            head = jnp.concatenate([x[:8 * f, 0:LANES], head], axis=0)
        return head if x.shape[1] == LANES else jnp.concatenate([head, x[:, LANES:]], axis=1)

    def hold16(x, tks):
        x4 = x.reshape(len(tks), 2, 8, LANES)
        return jnp.stack([after(jnp.stack(tks), x4[:, 0]), x4[:, 1]], axis=1).reshape(x.shape)

    def perm_k(c, b, toks):
        kt = [_dot_nt(perm, sk_v[c, :, b * LB + t * BLK:b * LB + (t + 1) * BLK]) for t in range(PH)]
        toks += _rows8(kt[0])[::2]
        return [jnp.concatenate([kt[t][i * R:(i + 1) * R, :] for t in range(PH)], axis=0).astype(BF16)
                for i in range(PH)]

    def spectrum(comps, dst, slot, b, toks, dc=None, pins=None):
        tr, ti = [], []
        for i in range(PH):
            lhs = fw_u[i]
            if pins is not None and i < len(pins):
                lhs = after(pins[i], lhs.reshape(NG, 8, LANES)).reshape(BLK, LANES)
            t4 = _dot(_as_bf16(lhs), comps[i]).reshape(NG, 2, 8, LANES)
            tr.append(t4[:, 0])
            ti.append(t4[:, 1])
        toks += [ti[PH - 1][g] for g in range(NG)]
        if dc is not None:
            tr[0] = tr[0] + dc
        sr, si = _dft4(tr, ti, -1)
        for qq in range(PH):
            dst[slot, :, b, qq, 0] = sr[qq]
            dst[slot, :, b, qq, 1] = si[qq]

    def gated(c, b):
        w = [par_s[c, t:t + 1, :] for t in range(4)]
        kc = {}
        for o in range(-2, 2):
            words = k_u[c, pl.ds(8 + b * (LB // 2) + o, BLK, stride=2), :]
            if o > -2:
                kc[2 * o] = _lo(words)
            kc[2 * o + 1] = _hi(words)
        vc = {}
        for o in range(2):
            words = v_u[c, pl.ds(b * (LB // 2) + o, BLK, stride=2), :]
            vc[2 * o] = _lo(words)
            vc[2 * o + 1] = _hi(words)
        for i in range(PH):
            ks = kc[i] * w[0]
            for t in range(1, 4):
                ks = ks + kc[i - t] * w[t]
            wu_s[b, i] = (ks * vc[i]).astype(BF16)
        return [wu_u[b, i] for i in range(PH)]

    def kv_pins(kvb):
        return [jnp.stack([kvb[2 * m + (r % 2)][8 * (r // 2):8 * (r // 2) + 8, :] for r in range(NG)])
                for m in range(2)]

    def products(c, us, ks, toks):
        n = len(toks) - 3
        cum = (44, 128, 244, 392)
        zp = None
        for o in range(NBL):
            tk = jnp.stack([toks[max(0, ((g * cum[-1] + cum[o]) * n) // (cum[-1] * NG) - 1)] for g in range(NG)])
            zr, zi = [], []
            for qq in range(PH):
                accr = acci = None
                for b in range(o + 1):
                    a_, b_ = us[0, :, b, qq, 0], us[0, :, b, qq, 1]
                    c_, d_ = ks[0, :, o - b, qq, 0], ks[0, :, o - b, qq, 1]
                    if qq == 0 and b == o:
                        a_ = after(tk, a_)
                    tr_ = a_ * c_ - b_ * d_
                    ti_ = a_ * d_ + b_ * c_
                    accr = tr_ if accr is None else accr + tr_
                    acci = ti_ if acci is None else acci + ti_
                zr.append(accr)
                zi.append(acci)
            if zp is None:
                yr, yi = zr, zi
            else:
                yr = [zr[qq] - zp[1][qq] for qq in range(PH)]
                yi = [zi[qq] + zp[0][qq] for qq in range(PH)]
            zp = (zr, zi)
            vr, vi = _dft4(yr, yi, +1)
            for i in range(PH):
                vv_s[c, o, i] = jnp.stack([vr[i], vi[i]], axis=1).reshape(2 * BLK, LANES).astype(BF16)

    def inverse(c, toks, pins):
        for o in range(NBL):
            for i in range(PH):
                yv = None
                for h in range(2):
                    lhs = iv_u[i, h]
                    if pins is not None and h == 0:
                        pin = pins[o][i % 2][8 * (i // 2):8 * (i // 2) + 8]
                        lhs = after(pin, lhs.reshape(8, 8, LANES)).reshape(HL, LANES)
                    t = _dot(_as_bf16(lhs), _as_bf16(vv_u[c, o, i, h * HL:(h + 1) * HL, :]))
                    yv = t if yv is None else yv + t
                if i % 2 == 0:
                    toks += _rows8(yv)[::2]
                y_s[c, pl.ds(o * LB + i, BLK, stride=PH), :] = yv

    def conv_round(c, fwd, mul, inv):
        toks = []
        kv = pins = None
        cur = 1 if mul else 0
        if fwd or mul:
            win = pl.ds(c - cur, 2 if fwd and mul else 1)
            us, ks = u_s.at[win], kk_s.at[win]
        if 'u' in fwd:
            kv = [gated(c, b) for b in range(NBL)]
            pins = [kv_pins(kv[b]) for b in range(NBL)]
        if inv:
            inverse(c - 2, toks, pins)
            if fwd:
                toks = []
        if 'k' in fwd:
            comps = [perm_k(c, b, toks) for b in range(NBL)]
        for b in range(NBL):
            if 'k' in fwd:
                spectrum(comps[b], ks, cur, b, toks, par_s[c, 4:5, :] if b == 0 else None)
            if 'u' in fwd:
                pin = pins[b + 2] if not inv and b + 2 < NBL else None
                spectrum([_as_bf16(x) for x in kv[b]], us, cur, b, toks, None, pin)
        if mul:
            products(c - 1, us, ks, toks)

    def lane_tiles(x):
        return [x[:, c * LANES:(c + 1) * LANES] for c in range(NC)]

    def stage_p1(r0, r1, tks=None):
        ga = mod_s[2, 0:1, :]
        a_mul, a_add = ga * (1.0 + mod_s[1, 0:1, :]) * math.sqrt(D), ga * mod_s[0, 0:1, :]
        q = q_v[r0:r1, :].astype(F32)
        if tks is not None:
            q = hold(q, tks)
        y = jnp.concatenate([y_s[c, r0:r1, :] for c in range(NC)], axis=1)
        x = q + (_ln(q, unit=False) * a_mul + a_add) * y
        x_s[r0:r1, :] = x
        return _ln(x, unit=False)

    def store_row_ops(dst, base, r0, r1, cols, tks=None):
        hv = []
        for x in cols:
            x4 = x.reshape(x.shape[0] // 32, 2, 16, LANES)
            hv.append([x4[:, e].reshape(x.shape[0] // 2, LANES) for e in range(2)])
        for k2 in range(2):
            a00, a01, a10, a11 = hv[k2][0], hv[2 + k2][0], hv[k2][1], hv[2 + k2][1]
            if tks is not None:
                a00, a11 = hold16(a00, tks), hold16(a11, tks)
            for o, x in enumerate(_all_operands(_LHS, a00, a01, a10, a11) + [a01, a10, hv[NC - 1][k2]]):
                dst[o, k2, (r0 - base) // 2:(r1 - base) // 2, :] = x.astype(BF16)

    L1B = A0[BLOCKWISE1[0]]
    L2B = B0[BLOCKWISE2[0]]

    def stage_p2(r0, r1, nx, blockwise=False):
        h = nx * ((1.0 + mod_s[4, 0:1, :]) * (2.0 * math.sqrt(D))) + 2.0 * mod_s[3, 0:1, :]
        h_s[r0:r1, :] = h
        zn = lane_tiles(_ln(h, 4.0 * EPS))
        if blockwise:
            store_row_ops(l1_s, L1B, r0, r1, zn)
        else:
            for c in range(NC):
                z_s[c, r0:r1, :] = zn[c].astype(BF16)

    def stage_p(t, toks):
        lo, hi = A0[t], A0[t + 1]
        stage_p2(lo, hi, stage_p1(lo, hi, _pick(toks[:-TRS[t - 1]], (hi - lo) // 8, FRS[t - 1])), t in BLOCKWISE1)

    def filler(t):
        red = jnp.sum(y_s[t, 0:8 * FI[t], :], axis=-1, keepdims=True).reshape(FI[t], 8, 1)
        spare = (NC - 1) * (TQ + 8) + 8 * t
        zf_s[1, spare:spare + 8, :] = jnp.broadcast_to(jnp.sum(red, axis=0), (8, LANES))

    def square_ops(src, dst, toks):
        HK = 2 * LANES
        tks = _pick(toks, 2 * HK // 16)
        for n2 in range(2):
            tk = tks[n2 * (HK // 16):(n2 + 1) * (HK // 16)]
            blk = lambda k, n: src[2 * n + n2, k * HK:(k + 1) * HK, :].astype(F32)
            for o, x in enumerate(_all_operands(_RHS, hold16(blk(0, 0), tk), blk(0, 1), blk(1, 0), hold16(blk(1, 1), tk))):
                if o not in _RAW:
                    dst[o, n2] = x.astype(BF16)

    def block_dots(ops_u, base, prepare, w_u, s_u, parts, emit, light, heavy):
        toks = []

        def timed(x, weight):
            toks.extend(_rows8(x, weight))
            return x

        def weave(top, bot):
            n = top.shape[0] // 16
            return jnp.stack([top.reshape(n, 16, LANES), bot.reshape(n, 16, LANES)], axis=1).reshape(32 * n, LANES)

        def main(get):
            m = [None] * 7
            rem = [None, None]
            for o in ('t', 2, 4, 'b', 1, 3, 0, 6, 5):
                if o in ('t', 'b'):
                    e = 0 if o == 't' else 1
                    rhs = jnp.concatenate([w_u[c, 2 * LANES:D // 2, :] for c in range(NC - 1)], axis=1)
                    rem[e] = timed(_dot(get([(9, e)]), _as_bf16(rhs)), light)
                    continue
                if o in _RAW:
                    d = _RAW.index(o)
                    rhs = jnp.concatenate([w_u[2 * d + n2, d * LANES:(d + 1) * LANES, :] for n2 in range(2)], axis=1)
                else:
                    rhs = jnp.concatenate([s_u[o, n2] for n2 in range(2)], axis=1)
                m[o] = timed(_dot(get([(o, 0), (o, 1)]), _as_bf16(rhs)), heavy if o in (4, 3, 6, 5) else light)
            c00, c01, c10, c11 = _combine(m)
            top = jnp.concatenate([c00, c01], axis=1) + rem[0]
            bot = jnp.concatenate([c10, c11], axis=1) + rem[1]
            return [weave(top[:, c * LANES:(c + 1) * LANES], bot[:, c * LANES:(c + 1) * LANES]) for c in range(NC - 1)]

        def last(get):
            w = _as_bf16(w_u[NC - 1])
            return weave(timed(_dot(get([(2, 0), (2, 1), (7, 0), (7, 1), (9, 0)]), w), light),
                         timed(_dot(get([(8, 0), (8, 1), (3, 0), (3, 1), (9, 1)]), w), light))

        mark = None
        for j, (r0, r1) in enumerate(parts):
            prepare(r0, r1, None if mark is None else toks[mark:])
            mark = len(toks)
            get = lambda keys: _as_bf16(jnp.concatenate(
                [ops_u[o, e, (r0 - base) // 4:(r1 - base) // 4, :] for o, e in keys], axis=1))
            if j % 2:
                tail = last(get)
                emit(r0, r1, main(get) + [tail])
            else:
                emit(r0, r1, main(get) + [last(get)])
        return toks

    def stage_m1(t, k):
        def emit(r0, r1, cols):
            out = [_gelu2(x) for x in cols]
            for c in range(NC):
                h1_s[c, r0 + 8:r1 + 8, :] = out[c]
            return out

        if t in BLOCKWISE1:
            return block_dots(l1_u, L1B, lambda *_: None, w1_u, s1_u, _chunks(A0[t], A0[t + 1], k, 32), emit, WS[2], WS[3])
        toks = []
        for r0, r1 in _chunks(A0[t], A0[t + 1], k):
            lhs = jnp.concatenate([z_u[c, r0 // 2:r1 // 2, :] for c in range(NC)], axis=1)
            w = jnp.concatenate([w1_u[c] for c in range(NC)], axis=1)
            for x in emit(r0, r1, lane_tiles(_dot(_as_bf16(lhs), _as_bf16(w)))):
                toks += _rows8(x, WS[0] if t != 2 else WS[6])
        return toks

    def shifted(r0, r1):
        n, grp, shifts = r1 - r0, D // 4, (-1, 1, -2, 2)
        lane = lax.broadcasted_iota(jnp.int32, (n, LANES), 1)
        cols = []
        for c in range(NC):
            lo, hi = c * LANES, (c + 1) * LANES
            g_lo, g_hi = lo // grp, (hi - 1) // grp
            val = h1_s[c, pl.ds(r0 + 8 + shifts[g_lo], n), :]
            if g_hi != g_lo:
                other = h1_s[c, pl.ds(r0 + 8 + shifts[g_hi], n), :]
                val = jnp.where(lane < (g_hi * grp - lo), val, other)
            cols.append(val)
        return cols

    def stage_m2(t, k, before=None):
        def emit(r0, r1, cols):
            x1 = h_s[r0:r1, :] + jnp.concatenate(cols, axis=1)
            h_s[r0:r1, :] = x1
            return x1

        if t in BLOCKWISE2:
            def prepare(r0, r1, prev):
                prev = before if prev is None else prev
                prev = prev[len(prev) // 8:(len(prev) * 7) // 8]
                store_row_ops(l2_s, L2B, r0, r1, shifted(r0, r1), _pick(prev, (r1 - r0) // 32))
            return block_dots(l2_u, L2B, prepare, w2_u, s2_u, _chunks(B0[t], B0[t + 1], k, 32), emit, WS[4 if t == 2 else 5], WS[4 if t == 2 else 5])
        toks = []
        for r0, r1 in _chunks(B0[t], B0[t + 1], k):
            w = jnp.concatenate([w2_u[c] for c in range(NC)], axis=1)
            hs = _dot(jnp.concatenate(shifted(r0, r1), axis=1).astype(BF16), _as_bf16(w))
            for x in lane_tiles(emit(r0, r1, [hs])):
                toks += _rows8(x, WS[1])
        return toks

    NT = S // TB
    FQ = FF // 4
    NS = FQ // LANES
    LQ = FQ - NS * LANES
    CQ = LANES // 4
    QR = LANES + CQ
    BLOCKS = [(2 * r1 + r2, 2 * h + p)
              for r1, h in ((0, 0), (1, 0), (0, 1), (1, 1)) for r2 in range(2) for p in range(2)]

    def z_rows(rq, c):
        lo = (NC * rq + c) * (TQ + 8)
        return slice(lo, lo + TQ)

    def store_z(r0, slot, toks, q0=0, q1=4):
        n = (q1 - q0) * TQ
        rows = pl.ds(r0 + q0 * TQ if isinstance(r0, int) else pl.multiple_of(r0 + q0 * TQ, TQ), n)
        zn = lane_tiles(_ln(hold(h_s[rows, :], _pick(toks, n // 8)), 4.0 * EPS))
        for rq in range(q0, q1):
            for c in range(NC - 1):
                zf_s[slot, z_rows(rq, c), :] = zn[c][(rq - q0) * TQ:(rq - q0 + 1) * TQ]
        zr_s[q0 * TQ:q1 * TQ, :] = zn[NC - 1].astype(BF16)

    def w3_ops(toks):
        ng = FQ // 16
        blk = lambda c, d: w3_v[c, d * FQ:(d + 1) * FQ, :].astype(F32)
        outer = [[_all_operands(_RHS, blk(k2, p), blk(k2, 2 + p), blk(2 + k2, p), blk(2 + k2, 2 + p))
                  for p in range(2)] for k2 in range(2)]
        for k, i in enumerate((1, 5, 2, 4, 0, 3, 6)):
            tk = [toks[((k + r * 7) * len(toks)) // (7 * ng)] for r in range(ng)]
            for j, x in enumerate(_all_operands(_RHS, hold16(outer[0][0][i], tk), outer[0][1][i], outer[1][0][i],
                                                hold16(outer[1][1][i], tk))):
                if i not in _RAW or j not in _RAW:
                    s3_s[i, j] = x.astype(BF16)

    def transpose_w4(toks):
        order = [(c, n) for n in (4 * NS, 4 * NS + 1) + tuple(range(4 * NS)) for c in range(NC)]
        for k, (c, n) in enumerate(order):
            if n >= 4 * NS:
                ends = [(2 * (n - 4 * NS) + p + 1) * FQ // 2 for p in range(2)]
                x = jnp.concatenate([w4_u[c, e - LQ // 2:e, :] for e in ends]
                                    + [jnp.zeros((HL - LQ, LANES), U32)], axis=0)
            else:
                lo = (n % 4) * FQ // 2 + (n // 4) * HL
                x = w4_u[c, lo:lo + HL, :]
            x = jnp.concatenate([after(toks[(k * len(toks)) // len(order)], x[0:8]), x[8:]], axis=0)
            wt_s[c, n] = _as_bf16(x).astype(F32).T.astype(BF16)

    def w4_ops(i, zero, toks):
        ng = QR // 16
        total = (NS * 7 + 2) * ng
        tk = lambda pos, step: [toks[((pos + r * step) * len(toks)) // total] for r in range(ng)]
        quarter = lambda n, d: jnp.concatenate(
            [wt_s[d, n].astype(F32), wt_s[NC - 1, n, d * CQ:(d + 1) * CQ, :].astype(F32)], axis=0)
        if i not in _RAW:
            for e in range(2):
                x = _operand(_RHS[i], lambda h, d: quarter(4 * NS + h, 2 * d + e))
                e4_s[i + zero, e] = hold16(x, tk(e * ng, 1)).astype(BF16)
        for st in range(NS):
            t = [[_operand(_RHS[i], lambda h, d: quarter(4 * st + 2 * h + p, 2 * d + e)) for e in range(2)]
                 for p in range(2)]
            tks = tk((2 + st * 7) * ng, 7)
            for j, x in enumerate(_all_operands(_RHS, hold16(t[0][0], tks), t[0][1], t[1][0], hold16(t[1][1], tks))):
                if i not in _RAW or j not in _RAW:
                    s4_s[i + zero, j, st] = x.astype(BF16)

    def gate_row(toks):
        ng = D // 8
        col = after(jnp.stack(_pick(toks, ng)), scol_s[...].reshape(ng, 8, LANES))
        for c in range(NC):
            wf = wm_v[:, (NC * NC + c) * LANES:(NC * NC + c + 1) * LANES].astype(F32).reshape(ng, 8, LANES)
            acc = col[0] * wf[0]
            for r in range(1, ng):
                acc = acc + col[r] * wf[r]
            mod_s[NC, :, c * LANES:(c + 1) * LANES] = jnp.broadcast_to(jnp.sum(acc, axis=0, keepdims=True), (8, LANES))

    def rem3(rq, d, pieces=1):
        z = _as_bf16(zr_u[rq * (TQ // 2):(rq + 1) * (TQ // 2), :])
        return jnp.concatenate([_dot_nt(_as_bf16(w3_u[NC - 1, lo // 2:hi // 2, :]), z)
                                for lo, hi in _chunks(d * FQ, (d + 1) * FQ, pieces)], axis=0)

    def lead_in():
        head = [rem3(*key) for key in BLOCKS[:4]]
        for k in range(4):
            rh_s[k] = head[k]
        return _rows8(head[0])

    with jax.named_scope("r0a"):
        wait_all(first[:1])
        conv_round(0, 'k', False, False)
    with jax.named_scope("r0_wait"):
        wait_all(first[1:])
    with jax.named_scope("r0b"):
        start_all(conv_copies(2) + conv_copies(3) + conv_copies(4))
        conv_round(0, 'u', False, False)
    with jax.named_scope("r1a"):
        wait_all(second[:1])
        conv_round(1, 'k', True, False)
    with jax.named_scope("r1_wait"):
        wait_all(second[1:])
    with jax.named_scope("r1b"):
        start_all(wm_copies[0] + q_copies[0] + wm_copies[1] + w_copies[0])
        conv_round(1, 'u', False, False)

    def full_round(c, carry):
        wait_all(conv_copies(c))
        conv_round(c, 'ku', True, True)
        return carry

    with jax.named_scope("r234"):
        lax.fori_loop(2, NC, full_round, 0)
    with jax.named_scope("r5"):
        start_all(q_copies[1] + w_copies[1] + sum(q_copies[2:], []) + w_copies[2] + w_copies[3] + wm_copies[2], 1)
        conv_round(NC, '', True, True)
    with jax.named_scope("r6_wait"):
        wait_all(wm_copies[0] + q_copies[0])
    with jax.named_scope("r6"):
        for j in range(3):
            mod_chunk(j)
        conv_round(NC + 1, '', False, True)
        nx0 = stage_p1(0, A0[1])
    with jax.named_scope("p2_wait"):
        wait_all(wm_copies[1])
    with jax.named_scope("p2"):
        mod_chunk(4)
        mod_chunk(3)
        stage_p2(0, A0[1], nx0)
    with jax.named_scope("w1_wait"):
        wait_all(w_copies[0])
    with jax.named_scope("m1_0"):
        square_ops(w1_v, s1_s, stage_m1(0, 4)[:-40])
    with jax.named_scope("w2_wait"):
        wait_all(q_copies[1] + w_copies[1])
    with jax.named_scope("m2_0"):
        stage_p(1, stage_m2(0, SP0))
        filler(0)
    for t in range(1, NA):
        with jax.named_scope("a%d" % t):
            wait_all(q_copies[t + 1] if t + 1 < NA else w_copies[2] + w_copies[3] + wm_copies[2])
            toks = stage_m1(t, 2)
            toks = toks + stage_m2(t, 2, toks[len(toks) - len(toks) // 2:])
            if t + 1 < NA:
                stage_p(t + 1, toks)
            if t == 1:
                square_ops(w2_v, s2_s, toks[:-30])
            if t == NA - 1:
                transpose_w4(toks[:(len(toks) * XEND) // 100])
                store_z(0, 0, toks[(len(toks) * LW[0]) // 100:(len(toks) * LW[1]) // 100])
                toks = toks + [x for x in lead_in()[:40] for _ in range(WS[7])]
                cut = (len(toks) * CUT) // 100
                gate_row(toks[:(len(toks) * 9) // 10])
                w3_ops(toks[:cut])
                rest = [i for i in range(7) if i not in IN_LOOP]
                for k, i in enumerate(rest):
                    w4_ops(i, 0, toks[cut + k::len(rest)])
            filler(t)

    def out_copy(r0, n, c):
        rows = pl.ds(r0, n)
        return pltpu.make_async_copy(o_v.at[c, rows, :], o_hbm.at[rows, pl.ds(c * LANES, LANES)], sem_o.at[0])

    def raw4(n, d):
        return jnp.concatenate([wt_u[d, n], wt_u[NC - 1, n, d * (CQ // 2):(d + 1) * (CQ // 2), :]], axis=0)

    def mlp_tile(t, carry):
        r0 = pl.multiple_of(t * TB, TB)
        ws = t & 1
        count = [0]

        def fresh():
            count[0] += 1
            return lax.rem(t + 2 * count[0], 2)

        def g_rows(r2, p, lo, hi):
            base = (2 * r2 + p) * (FQ + GPAD)
            return slice(base + lo, base + hi)

        rem = {key: rh_s[k] for k, key in enumerate(BLOCKS[:4])}
        for key in BLOCKS[4:8]:
            rem[key] = rem3(*key)
        early = _rows8(rem[BLOCKS[4]], EW[0])
        rem[BLOCKS[8]] = rem3(*BLOCKS[8], pieces=4)
        todo = BLOCKS[9:]
        part = [None] * 7
        for i in (4, 3, 0, 6, 1, 2, 5):
            m = [None] * 7
            for j in _ORDER:
                slot = fresh()
                act = _operand(_LHS[j], lambda r2, k2: _operand(
                    _LHS[i], lambda r1, k1: zf_s[slot, z_rows(2 * r1 + r2, 2 * k1 + k2), :])).astype(BF16)
                if i in _RAW and j in _RAW:
                    d = 2 * _RAW.index(i) + _RAW.index(j)
                    wij = w3_u[d, d * (FQ // 2):(d + 1) * (FQ // 2), :]
                else:
                    wij = s3_u[i, j]
                m[j] = _dot_nt(_as_bf16(wij), act)
            key = todo.pop(0)
            rem[key] = rem3(*key)
            part[i] = _combine(m)
            if i in (4, 3, 0):
                early += _rows8(m[_ORDER[0]], EW[1]) + _rows8(m[_ORDER[4]], EW[2])
        zero = fresh() - ws
        fine = [x for x in early for _ in IN_LOOP]
        hop = len(fine) // (len(IN_LOOP) * 33)
        for k, i in enumerate(IN_LOOP):
            w4_ops(i, zero, fine[k * hop:len(fine) - (len(IN_LOOP) - k) * hop])
        for inner in range(4):
            r2, p = inner // 2, inner % 2
            for blk, pre in enumerate(_combine([part[i][inner] for i in range(7)])):
                g_s[blk][ws, g_rows(r2, p, 0, FQ), :] = _gelu2(pre + rem[2 * (blk // 2) + r2, 2 * (blk % 2) + p])

        toks = []
        marks = {}
        part = [[None] * 4 for _ in range(7)]
        for i in O4:
            slot = fresh()
            we = jnp.concatenate([raw4(4 * NS + _RAW.index(i), 2 * _RAW.index(i) + e) if i in _RAW else e4_u[i, e]
                                  for e in range(2)], axis=0)
            ex = []
            for r2 in range(2):
                act = [_operand(_LHS[i], lambda r1, h: g_s[2 * r1 + h][slot, g_rows(r2, p, NS * LANES, FQ), :])
                       for p in range(2)]
                act = jnp.concatenate(act + [jnp.zeros((LANES - 2 * LQ, TQ), F32)], axis=0).astype(BF16)
                ex.append(_dot(_as_bf16(we), act))
            m = [None] * 7
            for j in _ORDER:
                slot = fresh()
                act = _operand(_LHS[j], lambda r2, p: _operand(
                    _LHS[i], lambda r1, h: g_s[2 * r1 + h][slot, g_rows(r2, p, 0, NS * LANES), :])).astype(BF16)
                if i in _RAW and j in _RAW:
                    d = 2 * _RAW.index(i) + _RAW.index(j)
                    wij = [raw4(4 * st + d, d) for st in range(NS)]
                else:
                    wij = [s4_u[i, j, st] for st in range(NS)]
                m[j] = _dot(_as_bf16(jnp.concatenate(wij, axis=1)), act)
                toks += _rows8(m[j])
            part[i] = [x + ex[inner // 2][(inner % 2) * QR:(inner % 2 + 1) * QR]
                       for inner, x in enumerate(_combine(m))]
            marks[i] = len(toks)

        gb = 0.5 * mod_s[NC, 0:1, :]
        nxt = jnp.minimum(t + 1, NT - 1) * TB
        tails = {}
        for i, blk, norm in PLAN:
            r1 = blk // 2
            if norm is None:
                toks += [x for x in lead_in()[8:40] for _ in range(3)]
            elif norm[0] < norm[1]:
                store_z(nxt, 1 - ws, toks[norm[2]:norm[3]], norm[0], norm[1])
            pos = [marks[i] + FL[(1, 2, 0, 3).index(blk)]]

            def finish(rq, c, h2t):
                h2 = hold(h2t.T, toks[pos[0]:pos[0] + TQ // 8])
                pos[0] += TQ // 8
                rows = pl.ds(pl.multiple_of(r0 + rq * TQ, TQ), TQ)
                cols = slice(c * LANES, (c + 1) * LANES)
                o_v[c, rows, :] = (x_s[rows, cols] + gb[:, cols] * (h_s[rows, cols] + h2)).astype(BF16)
                if blk == 3:
                    out_copy(rows.start, TQ, c).start()

            for inner in (1, 2, 0, 3):
                ht = _block([part[k][inner] for k in range(7)], blk)
                rq, c = 2 * r1 + inner // 2, 2 * (blk % 2) + inner % 2
                finish(rq, c, ht[0:LANES])
                tails[rq, c] = ht[LANES:]
            rb = pl.multiple_of(r0 + r1 * 2 * TQ, 2 * TQ)
            if blk != 3:
                for e in range(2):
                    out_copy(rb, 2 * TQ, 2 * (blk % 2) + e).start()
            if blk in (0, 3):
                for rq in (2 * r1, 2 * r1 + 1):
                    finish(rq, NC - 1, jnp.concatenate([tails[rq, c] for c in range(NC - 1)], axis=0))
                if blk == 0:
                    out_copy(rb, 2 * TQ, NC - 1).start()
        return carry

    with jax.named_scope("ph2b"):
        lax.fori_loop(0, NT, mlp_tile, 0)
    with jax.named_scope("tail"):
        pltpu.make_async_copy(o_v, o_v, sem_o.at[0]).wait()


@jax.jit
def pallas_adaLN_cond__ssm_conv_h3__mixer_s_mlp__prompt_kernel(
    A_q: jax.Array,
    A_k: jax.Array,
    A_v: jax.Array,
    A_shift_k: jax.Array,
    A_ssm_k: jax.Array,
    A_ssm_D: jax.Array,
    B_x: jax.Array,
    B_w1: jax.Array,
    B_w2: jax.Array,
    B_w3: jax.Array,
    B_w4: jax.Array,
    c: jax.Array,
    w_mod: jax.Array,
):
    B, S, D = A_q.shape
    FF = B_w3.shape[1]
    assert (B, S, D, FF, A_shift_k.shape[1]) == (1, sum(TILES), 5 * LANES, 1728, 4)
    NC = D // LANES
    NG = BLK // 8
    NBL = S // (PH * BLK)
    NS = FF // 4 // LANES
    n1 = S - sum(TILES[:BLOCKWISE1[0]]) - HALO
    n2 = S - sum(TILES[:BLOCKWISE2[0]])

    args = (A_q.reshape(S, D), A_k.reshape(S, D), A_v.reshape(S, D), A_shift_k.T, A_ssm_k,
            A_ssm_D, B_w1, B_w2, B_w3.T, B_w4, c, w_mod)
    scratch = [
        pltpu.VMEM((S, D), BF16),
        pltpu.VMEM((NC, S + 16, LANES), BF16),
        pltpu.VMEM((NC, S, LANES), BF16),
        pltpu.VMEM((4, D), BF16),
        pltpu.VMEM((NC, LANES, S), BF16),
        pltpu.VMEM((D,), BF16),
        pltpu.VMEM((NC, D, LANES), BF16),
        pltpu.VMEM((NC, D, LANES), BF16),
        pltpu.VMEM((NC, FF, LANES), BF16),
        pltpu.VMEM((NC, FF, LANES), BF16),
        pltpu.VMEM((1, D), BF16),
        pltpu.VMEM((D, 6 * D), BF16),
        pltpu.VMEM((PH, 2 * BLK, BLK), BF16),
        pltpu.VMEM((PH, 2, BLK, BLK), BF16),
        pltpu.VMEM((NC, S, LANES), BF16),
        pltpu.VMEM((NC, NG, NBL, PH, 2, 8, LANES), F32),
        pltpu.VMEM((NC, NG, NBL, PH, 2, 8, LANES), F32),
        pltpu.VMEM((NC, NBL, PH, 2 * BLK, LANES), BF16),
        pltpu.VMEM((NBL, PH, BLK, LANES), BF16),
        pltpu.VMEM((NC, S, LANES), F32),
        pltpu.VMEM((6, 8, D), F32),
        pltpu.VMEM((NC, 8, LANES), F32),
        pltpu.VMEM((NC, S + 16, LANES), F32),
        pltpu.VMEM((S, D), F32),
        pltpu.VMEM((S, D), F32),
        pltpu.VMEM((NC, S, LANES), BF16),
        pltpu.VMEM((7, 7, FF // 4, LANES), BF16),
        pltpu.VMEM((7, 7, NS, D // 4, LANES), BF16),
        pltpu.VMEM((7, 2, D // 4, LANES), BF16),
        [pltpu.VMEM((2, GROWS, TQ), F32)] * 4,
        pltpu.VMEM((2, 4 * NC * (TQ + 8), LANES), F32),
        pltpu.VMEM((TB, LANES), BF16),
        pltpu.VMEM((10, 2, n1 // 2, LANES), BF16),
        pltpu.VMEM((10, 2, n2 // 2, LANES), BF16),
        pltpu.VMEM((7, 2, 2 * LANES, LANES), BF16),
        pltpu.VMEM((7, 2, 2 * LANES, LANES), BF16),
        pltpu.VMEM((4, FF // 4, TQ), F32),
        pltpu.VMEM((NC, 4 * NS + 2, LANES, LANES), BF16),
        pltpu.VMEM((D, LANES), F32),
        pltpu.SemaphoreType.DMA((16 + len(TILES),)),
        pltpu.SemaphoreType.DMA((1,)),
    ]
    out = pl.pallas_call(
        functools.partial(_kernel, S=S, D=D, FF=FF),
        in_specs=[pl.BlockSpec(memory_space=pl.ANY)] * len(args),
        out_specs=pl.BlockSpec(memory_space=pl.ANY),
        out_shape=jax.ShapeDtypeStruct((S, D), BF16),
        scratch_shapes=scratch,
        compiler_params=pltpu.CompilerParams(
            vmem_limit_bytes=120 * 1024 * 1024,
            disable_bounds_checks=True,
            disable_semaphore_checks=True,
        ),
    )(*args)
    return out.reshape(B, S, D)
```

```python
import functools
import math

import jax
import jax.numpy as jnp
from jax import lax
import jax.experimental.pallas as pl
import jax.experimental.pallas.tpu as pltpu

F32 = jnp.float32
BF16 = jnp.bfloat16
U32 = jnp.uint32

LANES = 128
BLK = 128
PH = 4
EPS = 1e-05
TB = 512
TQ = TB // 4
HALO = 32
TILES = (384, 384, 576, 704)
BLOCKWISE1 = (3,)
BLOCKWISE2 = (2, 3)
IN_LOOP = (2, 4, 1, 3, 0)
O4 = (2, 4, 1, 3, 0, 6, 5)
NW = (1, 3, 0, 150, 320, 460, 600, 730)
PLAN = ((4, 1, (0, NW[0], NW[2], NW[3])), (3, 2, (NW[0], NW[1], NW[4], NW[5])), (6, 0, (NW[1], 4, NW[6], NW[7])), (5, 3, None))
FL = (10, 10, 25, -32)
EW = (2, 1, 2)
TRS = (135, 165, 180)
FRS = (45, 90, 90)
WS = (2, 3, 3, 2, 2, 2, 2, 4)
LW = (66, 92)
FI = (48, 96, 96, 96)
SP0 = 4
NB1 = 1
ESH = 0
ULAG = 9
R6 = 2
R6N = 36
R6F = 18
MF = (6, 0, 5, 4)
MT = (3, 0, 3, 3)
IG = 2
IJ = 6
IP = 2
P2N = 28
P2F = 6
GPAD = 8
GROWS = 1768
XEND = 55
CUT = 82

_ORDER = (2, 4, 1, 3, 0, 6, 5)
_RAW = (1, 4)
_LHS = (((0, 0), 1, (1, 1)), ((1, 0), 1, (1, 1)), ((0, 0),), ((1, 1),),
        ((0, 0), 1, (0, 1)), ((1, 0), -1, (0, 0)), ((0, 1), -1, (1, 1)))
_RHS = (((0, 0), 1, (1, 1)), ((0, 0),), ((0, 1), -1, (1, 1)), ((1, 0), -1, (0, 0)),
        ((1, 1),), ((0, 0), 1, (0, 1)), ((1, 0), 1, (1, 1)))


def _operand(terms, blk):
    x = blk(*terms[0])
    if len(terms) > 1:
        y = blk(*terms[2])
        x = x + y if terms[1] > 0 else x - y
    return x


def _all_operands(table, b00, b01, b10, b11):
    blocks = ((b00, b01), (b10, b11))
    return [_operand(terms, lambda i, j: blocks[i][j]) for terms in table]


def _block(m, which):
    if which == 0:
        return (m[3] - m[4]) + m[0] + m[6]
    if which == 1:
        return m[2] + m[4]
    if which == 2:
        return m[1] + m[3]
    return (m[2] - m[1]) + m[0] + m[5]


def _combine(m):
    return [_block(m, which) for which in range(4)]


def _as_bf16(x):
    return pltpu.bitcast(x, BF16)


def _lo(x):
    return pltpu.bitcast(x << 16, F32)


def _hi(x):
    return pltpu.bitcast(x & jnp.uint32(0xFFFF0000), F32)


def _dft4(re, im, sign):
    ar, ai = re[0] + re[2], im[0] + im[2]
    br, bi = re[0] - re[2], im[0] - im[2]
    cr, ci = re[1] + re[3], im[1] + im[3]
    dr, di = re[1] - re[3], im[1] - im[3]
    o0 = (ar + cr, ai + ci)
    o2 = (ar - cr, ai - ci)
    m = (br + di, bi - dr)
    p = (br - di, bi + dr)
    o1, o3 = (m, p) if sign < 0 else (p, m)
    return [o0[0], o1[0], o2[0], o3[0]], [o0[1], o1[1], o2[1], o3[1]]


def _ln(x, eps=EPS, unit=True):
    n = x.shape[-1]
    s1 = jnp.sum(x, axis=-1, keepdims=True)
    m = s1 * (1.0 / n)
    v = jnp.maximum(jnp.sum(x * x, axis=-1, keepdims=True) + (n * eps - s1 * m), n * eps)
    e = jnp.log(v) * (-0.5 / math.log(2.0))
    return (x - m) * jnp.exp2(e + 0.5 * math.log2(n) if unit else e)


def _gelu2(x):
    c0 = math.sqrt(2.0 / math.pi)
    return x + x * jnp.tanh(x * (c0 + (c0 * 0.044715) * (x * x)))


def _dot(a, b):
    return jnp.dot(a, b, preferred_element_type=F32)


def _dot_nt(a, b):
    return lax.dot_general(a, b, (((1,), (1,)), ((), ())), preferred_element_type=F32)


def _rows8(x, repeat=1):
    return [x[8 * r:8 * r + 8, 0:LANES] for r in range(x.shape[0] // 8) for _ in range(repeat)]


def _chunks(r0, r1, k, unit=16):
    n = (r1 - r0) // unit
    cuts = [r0 + unit * ((n * j) // k) for j in range(k + 1)]
    return list(zip(cuts[:-1], cuts[1:]))


def _pick(toks, n, free=0):
    idx = [(r * (len(toks) + free)) // n - free for r in range(n)]
    return [toks[i] if i >= 0 else None for i in idx]


def _kernel(q_hbm, k_hbm, v_hbm, sh_hbm, sk_hbm, sd_hbm, w1_hbm, w2_hbm, w3_hbm, w4_hbm, c_hbm, wm_hbm,
            o_hbm,
            q_v, k_v, v_v, sh_v, sk_v, sd_v, w1_v, w2_v, w3_v, w4_v, c_v, wm_v,
            fw_s, iv_s, o_v, u_s, kk_s, vv_s, wu_s, y_s, mod_s, par_s, h1_s, x_s, h_s, z_s,
            s3_s, s4_s, e4_s, g_s, zf_s, zr_s, l1_s, l2_s, s1_s, s2_s, rh_s, wt_s, scol_s,
            sem, sem_o,
            *, S, D, FF):
    NC = D // LANES
    NG = BLK // 8
    LB = PH * BLK
    NBL = S // LB
    R = BLK // PH
    HL = LANES // 2

    small = [
        pltpu.make_async_copy(sh_hbm, sh_v, sem.at[0]),
        pltpu.make_async_copy(sd_hbm, sd_v, sem.at[0]),
        pltpu.make_async_copy(c_hbm, c_v, sem.at[0]),
    ]

    def sk_copy(c):
        rows = pl.ds(c * LANES if isinstance(c, int) else pl.multiple_of(c * LANES, LANES), LANES)
        return [pltpu.make_async_copy(sk_hbm.at[rows, :], sk_v.at[c], sem.at[1 + c])]

    def kv_copies(tiles, blocks, s):
        return [pltpu.make_async_copy(src.at[pl.ds(b * LB, LB), pl.ds(c * LANES, LANES)],
                                      dst.at[c, pl.ds(off + b * LB, LB), :], sem.at[s])
                for b in blocks for src, dst, off in ((k_hbm, k_v, 16), (v_hbm, v_v, 0)) for c in tiles]

    PAIR, TRIPLE = (0, 1), (2, 3, 4)
    kv_groups = [kv_copies(PAIR, range(0, NB1), 9), kv_copies(PAIR, range(NB1, NBL), 10),
                 kv_copies(TRIPLE, range(0, 2), 11), kv_copies(TRIPLE, range(2, NBL), 20)]

    WM = (0, 3 * D, 5 * D, 6 * D)
    wm_copies = [[pltpu.make_async_copy(wm_hbm.at[:, pl.ds(WM[j], WM[j + 1] - WM[j])],
                                        wm_v.at[:, pl.ds(WM[j], WM[j + 1] - WM[j])], sem.at[6 + j])]
                 for j in range(3)]
    w_copies = [[pltpu.make_async_copy(src.at[:, pl.ds(c * LANES, LANES)], dst.at[c], sem.at[12 + j])
                 for c in range(NC)]
                for j, (src, dst) in enumerate(((w1_hbm, w1_v), (w2_hbm, w2_v), (w3_hbm, w3_v), (w4_hbm, w4_v)))]

    B0 = [0]
    for n in TILES:
        B0.append(B0[-1] + n)
    NA = len(TILES)
    A0 = [0] + [r + HALO for r in B0[1:-1]] + [S]
    q_copies = [
        [pltpu.make_async_copy(q_hbm.at[pl.ds(A0[t], A0[t + 1] - A0[t])], q_v.at[pl.ds(A0[t], A0[t + 1] - A0[t])],
                               sem.at[16 + t])]
        for t in range(NA)
    ]

    def start_all(cps, priority=0):
        for cp in cps:
            cp.start(priority=priority)

    def wait_all(cps):
        for cp in cps:
            cp.wait()

    for c in range(NC):
        k_v[c, 0:16, :] = jnp.zeros((16, LANES), BF16)
    start_all(sk_copy(0) + small + sk_copy(1) + kv_groups[0] + kv_groups[1] + sk_copy(2))

    for c in range(NC):
        h1_s[c, 0:8, :] = jnp.zeros((8, LANES), F32)
        h1_s[c, S + 8:S + 16, :] = jnp.zeros((8, LANES), F32)

    prow = lax.broadcasted_iota(jnp.int32, (BLK, BLK), 0)
    pcol = lax.broadcasted_iota(jnp.int32, (BLK, BLK), 1)
    ang = (((4 * prow + 1) * pcol) & (4 * BLK - 1)).astype(F32) * (2.0 * math.pi / (4 * BLK))
    tw = (4 * prow + 1).astype(F32) * (2.0 * math.pi / (4 * LB))
    mr, mi = jnp.cos(ang), -jnp.sin(ang)
    twr, twi = jnp.cos(tw), -jnp.sin(tw)
    eye = jnp.where(prow == pcol, 1.0 / LB, 0.0).astype(BF16)
    for i in range(PH):
        both = jnp.stack([mr.reshape(NG, 8, BLK), mi.reshape(NG, 8, BLK)], axis=1).reshape(2 * BLK, BLK)
        fw_s[i] = both.astype(BF16)
        for h in range(2):
            iv_s[i, h] = _dot_nt(eye, both[h * BLK:(h + 1) * BLK, :].astype(BF16)).astype(BF16)
        if i + 1 < PH:
            mr, mi = mr * twr - mi * twi, mr * twi + mi * twr
    perm = jnp.where(pcol == (prow % R) * PH + prow // R, 1.0, 0.0).astype(BF16)

    wait_all(small)
    shf = sh_v[...].astype(F32)
    sdf = sd_v[...].astype(F32).reshape(1, D)
    for c in range(NC):
        par_s[c, 0:4, :] = shf[:, c * LANES:(c + 1) * LANES]
        par_s[c, 4:5, :] = sdf[:, c * LANES:(c + 1) * LANES]
    cf = c_v[...].astype(F32)
    sc = (cf * jax.nn.sigmoid(cf)).astype(BF16)
    sc16 = jnp.broadcast_to(sc, (16, D))

    def mod_chunk(j):
        mod_s[j] = _dot(sc16, wm_v[:, j * D:(j + 1) * D])[0:8, :]

    (fw_u, iv_u, k_u, v_u, wu_u, vv_u, z_u, l1_u, l2_u, w1_u, w2_u, s1_u, s2_u, w3_u, w4_u, wt_u, s3_u, s4_u,
     e4_u, zr_u) = (r.bitcast(U32) for r in (fw_s, iv_s, k_v, v_v, wu_s, vv_s, z_s, l1_s, l2_s, w1_v, w2_v,
                                             s1_s, s2_s, w3_v, w4_v, wt_s, s3_s, s4_s, e4_s, zr_s))

    never = twr[0:8, :] > 2.0

    def after(token, x):
        if token.dtype != x.dtype:
            token = pltpu.bitcast(token, x.dtype)
        return jnp.where(jnp.broadcast_to(never, x.shape), token, x)

    def hold(x, tks):
        f = len([k for k in tks if k is None])
        n = len(tks)
        head = after(jnp.stack(tks[f:]), x[8 * f:, 0:LANES].reshape(n - f, 8, LANES)).reshape(8 * (n - f), LANES)
        if f:
            head = jnp.concatenate([x[:8 * f, 0:LANES], head], axis=0)
        return head if x.shape[1] == LANES else jnp.concatenate([head, x[:, LANES:]], axis=1)

    def hold16(x, tks):
        x4 = x.reshape(len(tks), 2, 8, LANES)
        return jnp.stack([after(jnp.stack(tks), x4[:, 0]), x4[:, 1]], axis=1).reshape(x.shape)

    def perm_k(c, b, toks):
        kt = [_dot_nt(perm, sk_v[c, :, b * LB + t * BLK:b * LB + (t + 1) * BLK]) for t in range(PH)]
        toks += _rows8(kt[0])[::2]
        return [jnp.concatenate([kt[t][i * R:(i + 1) * R, :] for t in range(PH)], axis=0).astype(BF16)
                for i in range(PH)]

    def spectrum(comps, dst, slot, b, toks, dc=None, pins=None):
        tr, ti = [], []
        for i in range(PH):
            lhs = fw_u[i]
            if pins is not None and i < len(pins):
                lhs = after(pins[i], lhs.reshape(NG, 8, LANES)).reshape(BLK, LANES)
            t4 = _dot(_as_bf16(lhs), comps[i]).reshape(NG, 2, 8, LANES)
            tr.append(t4[:, 0])
            ti.append(t4[:, 1])
        toks += [ti[PH - 1][g] for g in range(NG)]
        if dc is not None:
            tr[0] = tr[0] + dc
        sr, si = _dft4(tr, ti, -1)
        for qq in range(PH):
            dst[slot, :, b, qq, 0] = sr[qq]
            dst[slot, :, b, qq, 1] = si[qq]

    def gated(c, b, n):
        w = [par_s[c, t:t + 1, :] for t in range(4)]
        kc = {}
        for o in range(-2, 2):
            words = k_u[c, pl.ds(8 + b * (LB // 2) + o, BLK, stride=2), :]
            if o > -2:
                kc[2 * o] = _lo(words)
            kc[2 * o + 1] = _hi(words)
        vc = {}
        for o in range(2):
            words = v_u[c, pl.ds(b * (LB // 2) + o, BLK, stride=2), :]
            vc[2 * o] = _lo(words)
            vc[2 * o + 1] = _hi(words)
        for i in range(PH):
            ks = kc[i] * w[0]
            for t in range(1, 4):
                ks = ks + kc[i - t] * w[t]
            wu_s[n, i] = (ks * vc[i]).astype(BF16)
        return [wu_u[n, i] for i in range(PH)]

    def kv_pins(kvb):
        return [jnp.stack([kvb[2 * m + (r % 2)][8 * (r // 2):8 * (r // 2) + 8, :] for r in range(NG)])
                for m in range(2)]

    def products(c, ks, kc, toks, free, trim):
        n = len(toks) - trim + free
        cum = (44, 128, 244, 392)
        zp = None
        for o in range(NBL):
            idx = [((g * cum[-1] + cum[o]) * n) // (cum[-1] * NG) - 1 - free for g in range(NG)]
            tk = [toks[max(i, 0)] if i >= 0 or not free else None for i in idx]
            zr, zi = [], []
            for qq in range(PH):
                accr = acci = None
                for b in range(o + 1):
                    a_, b_ = u_s[c, :, b, qq, 0], u_s[c, :, b, qq, 1]
                    c_, d_ = ks[kc, :, o - b, qq, 0], ks[kc, :, o - b, qq, 1]
                    if qq == 0 and b == o:
                        a_ = hold(a_.reshape(BLK, LANES), tk).reshape(NG, 8, LANES)
                    tr_ = a_ * c_ - b_ * d_
                    ti_ = a_ * d_ + b_ * c_
                    accr = tr_ if accr is None else accr + tr_
                    acci = ti_ if acci is None else acci + ti_
                zr.append(accr)
                zi.append(acci)
            if zp is None:
                yr, yi = zr, zi
            else:
                yr = [zr[qq] - zp[1][qq] for qq in range(PH)]
                yi = [zi[qq] + zp[0][qq] for qq in range(PH)]
            zp = (zr, zi)
            vr, vi = _dft4(yr, yi, +1)
            for i in range(PH):
                vv_s[c, o, i] = jnp.stack([vr[i], vi[i]], axis=1).reshape(2 * BLK, LANES).astype(BF16)

    def inverse(c, o, toks, pins):
        for i in range(PH):
            yv = None
            for h in range(2):
                lhs = iv_u[i, h]
                if pins is not None and h == 0:
                    pin = pins[i % 2][8 * (i // 2):8 * (i // 2) + 8]
                    lhs = after(pin, lhs.reshape(8, 8, LANES)).reshape(HL, LANES)
                t = _dot(_as_bf16(lhs), _as_bf16(vv_u[c, o, i, h * HL:(h + 1) * HL, :]))
                yv = t if yv is None else yv + t
            if i % 2 == 0:
                toks += _rows8(yv)[::2]
            y_s[c, pl.ds(o * LB + i, BLK, stride=PH), :] = yv

    def conv_step(filt=None, units=(), mul=None, inv=(), shift=0, lag=2, free=0, trim=3):
        toks = []
        kv = [gated(c, b, n) for n, (c, b) in enumerate(units)]
        lead = len(inv) + (NBL if filt is not None else 0)
        pin_at = {}
        for n in range(len(units)):
            at = n + min(shift, lead - lag)
            if at >= 0:
                pin_at[at] = kv_pins(kv[n])
        if filt is not None and mul is not None and not isinstance(filt, int):
            ks = kk_s.at[pl.ds(mul, 2)]
            k_rd, k_wr = (ks, 0), (ks, 1)
        else:
            k_rd, k_wr = (kk_s, mul), (kk_s, filt)
        pos = 0
        for c, o in inv:
            inverse(c, o, toks, pin_at.get(pos))
            pos += 1
        if filt is not None:
            comps = [perm_k(filt, b, toks) for b in range(NBL)]
            for b in range(NBL):
                spectrum(comps[b], *k_wr, b, toks, par_s[filt, 4:5, :] if b == 0 else None, pin_at.get(pos))
                pos += 1
        for n, (c, b) in enumerate(units):
            spectrum([_as_bf16(x) for x in kv[n]], u_s, c, b, toks, None, pin_at.get(pos))
            pos += 1
        if mul is not None:
            products(mul, *k_rd, toks, free, trim)
        return toks

    def lane_tiles(x):
        return [x[:, c * LANES:(c + 1) * LANES] for c in range(NC)]

    def stage_p1(r0, r1, tks=None, ytks=None):
        ga = mod_s[2, 0:1, :]
        a_mul, a_add = ga * (1.0 + mod_s[1, 0:1, :]) * math.sqrt(D), ga * mod_s[0, 0:1, :]
        q = q_v[r0:r1, :].astype(F32)
        if tks is not None:
            q = hold(q, tks)
        y = jnp.concatenate([y_s[c, r0:r1, :] for c in range(NC)], axis=1)
        if ytks is not None:
            y = hold(y, ytks)
        x = q + (_ln(q, unit=False) * a_mul + a_add) * y
        x_s[r0:r1, :] = x
        return _ln(x, unit=False)

    def store_row_ops(dst, base, r0, r1, cols, tks=None):
        hv = []
        for x in cols:
            x4 = x.reshape(x.shape[0] // 32, 2, 16, LANES)
            hv.append([x4[:, e].reshape(x.shape[0] // 2, LANES) for e in range(2)])
        for k2 in range(2):
            a00, a01, a10, a11 = hv[k2][0], hv[2 + k2][0], hv[k2][1], hv[2 + k2][1]
            if tks is not None:
                a00, a11 = hold16(a00, tks), hold16(a11, tks)
            for o, x in enumerate(_all_operands(_LHS, a00, a01, a10, a11) + [a01, a10, hv[NC - 1][k2]]):
                dst[o, k2, (r0 - base) // 2:(r1 - base) // 2, :] = x.astype(BF16)

    L1B = A0[BLOCKWISE1[0]]
    L2B = B0[BLOCKWISE2[0]]

    def stage_p2(r0, r1, nx, blockwise=False):
        h = nx * ((1.0 + mod_s[4, 0:1, :]) * (2.0 * math.sqrt(D))) + 2.0 * mod_s[3, 0:1, :]
        h_s[r0:r1, :] = h
        zn = lane_tiles(_ln(h, 4.0 * EPS))
        if blockwise:
            store_row_ops(l1_s, L1B, r0, r1, zn)
        else:
            for c in range(NC):
                z_s[c, r0:r1, :] = zn[c].astype(BF16)

    def stage_p(t, toks):
        lo, hi = A0[t], A0[t + 1]
        stage_p2(lo, hi, stage_p1(lo, hi, _pick(toks[:-TRS[t - 1]], (hi - lo) // 8, FRS[t - 1])), t in BLOCKWISE1)

    def filler(t):
        red = jnp.sum(y_s[t, 0:8 * FI[t], :], axis=-1, keepdims=True).reshape(FI[t], 8, 1)
        spare = (NC - 1) * (TQ + 8) + 8 * t
        zf_s[1, spare:spare + 8, :] = jnp.broadcast_to(jnp.sum(red, axis=0), (8, LANES))

    def square_ops(src, dst, toks):
        HK = 2 * LANES
        tks = _pick(toks, 2 * HK // 16)
        for n2 in range(2):
            tk = tks[n2 * (HK // 16):(n2 + 1) * (HK // 16)]
            blk = lambda k, n: src[2 * n + n2, k * HK:(k + 1) * HK, :].astype(F32)
            for o, x in enumerate(_all_operands(_RHS, hold16(blk(0, 0), tk), blk(0, 1), blk(1, 0), hold16(blk(1, 1), tk))):
                if o not in _RAW:
                    dst[o, n2] = x.astype(BF16)

    def block_dots(ops_u, base, prepare, w_u, s_u, parts, emit, light, heavy):
        toks = []

        def timed(x, weight):
            toks.extend(_rows8(x, weight))
            return x

        def weave(top, bot):
            n = top.shape[0] // 16
            return jnp.stack([top.reshape(n, 16, LANES), bot.reshape(n, 16, LANES)], axis=1).reshape(32 * n, LANES)

        def main(get):
            m = [None] * 7
            rem = [None, None]
            for o in ('t', 2, 4, 'b', 1, 3, 0, 6, 5):
                if o in ('t', 'b'):
                    e = 0 if o == 't' else 1
                    rhs = jnp.concatenate([w_u[c, 2 * LANES:D // 2, :] for c in range(NC - 1)], axis=1)
                    rem[e] = timed(_dot(get([(9, e)]), _as_bf16(rhs)), light)
                    continue
                if o in _RAW:
                    d = _RAW.index(o)
                    rhs = jnp.concatenate([w_u[2 * d + n2, d * LANES:(d + 1) * LANES, :] for n2 in range(2)], axis=1)
                else:
                    rhs = jnp.concatenate([s_u[o, n2] for n2 in range(2)], axis=1)
                m[o] = timed(_dot(get([(o, 0), (o, 1)]), _as_bf16(rhs)), heavy if o in (4, 3, 6, 5) else light)
            c00, c01, c10, c11 = _combine(m)
            top = jnp.concatenate([c00, c01], axis=1) + rem[0]
            bot = jnp.concatenate([c10, c11], axis=1) + rem[1]
            return [weave(top[:, c * LANES:(c + 1) * LANES], bot[:, c * LANES:(c + 1) * LANES]) for c in range(NC - 1)]

        def last(get):
            w = _as_bf16(w_u[NC - 1])
            return weave(timed(_dot(get([(2, 0), (2, 1), (7, 0), (7, 1), (9, 0)]), w), light),
                         timed(_dot(get([(8, 0), (8, 1), (3, 0), (3, 1), (9, 1)]), w), light))

        mark = None
        for j, (r0, r1) in enumerate(parts):
            prepare(r0, r1, None if mark is None else toks[mark:])
            mark = len(toks)
            get = lambda keys: _as_bf16(jnp.concatenate(
                [ops_u[o, e, (r0 - base) // 4:(r1 - base) // 4, :] for o, e in keys], axis=1))
            if j % 2:
                tail = last(get)
                emit(r0, r1, main(get) + [tail])
            else:
                emit(r0, r1, main(get) + [last(get)])
        return toks

    def stage_m1(t, k):
        def emit(r0, r1, cols):
            out = [_gelu2(x) for x in cols]
            for c in range(NC):
                h1_s[c, r0 + 8:r1 + 8, :] = out[c]
            return out

        if t in BLOCKWISE1:
            return block_dots(l1_u, L1B, lambda *_: None, w1_u, s1_u, _chunks(A0[t], A0[t + 1], k, 32), emit, WS[2], WS[3])
        toks = []
        for r0, r1 in _chunks(A0[t], A0[t + 1], k):
            lhs = jnp.concatenate([z_u[c, r0 // 2:r1 // 2, :] for c in range(NC)], axis=1)
            w = jnp.concatenate([w1_u[c] for c in range(NC)], axis=1)
            for x in emit(r0, r1, lane_tiles(_dot(_as_bf16(lhs), _as_bf16(w)))):
                toks += _rows8(x, WS[0] if t != 2 else WS[6])
        return toks

    def shifted(r0, r1):
        n, grp, shifts = r1 - r0, D // 4, (-1, 1, -2, 2)
        lane = lax.broadcasted_iota(jnp.int32, (n, LANES), 1)
        cols = []
        for c in range(NC):
            lo, hi = c * LANES, (c + 1) * LANES
            g_lo, g_hi = lo // grp, (hi - 1) // grp
            val = h1_s[c, pl.ds(r0 + 8 + shifts[g_lo], n), :]
            if g_hi != g_lo:
                other = h1_s[c, pl.ds(r0 + 8 + shifts[g_hi], n), :]
                val = jnp.where(lane < (g_hi * grp - lo), val, other)
            cols.append(val)
        return cols

    def stage_m2(t, k, before=None):
        def emit(r0, r1, cols):
            x1 = h_s[r0:r1, :] + jnp.concatenate(cols, axis=1)
            h_s[r0:r1, :] = x1
            return x1

        if t in BLOCKWISE2:
            def prepare(r0, r1, prev):
                prev = before if prev is None else prev
                prev = prev[len(prev) // 8:(len(prev) * 7) // 8]
                store_row_ops(l2_s, L2B, r0, r1, shifted(r0, r1), _pick(prev, (r1 - r0) // 32))
            return block_dots(l2_u, L2B, prepare, w2_u, s2_u, _chunks(B0[t], B0[t + 1], k, 32), emit, WS[4 if t == 2 else 5], WS[4 if t == 2 else 5])
        toks = []
        for r0, r1 in _chunks(B0[t], B0[t + 1], k):
            w = jnp.concatenate([w2_u[c] for c in range(NC)], axis=1)
            hs = _dot(jnp.concatenate(shifted(r0, r1), axis=1).astype(BF16), _as_bf16(w))
            for x in lane_tiles(emit(r0, r1, [hs])):
                toks += _rows8(x, WS[1])
        return toks

    NT = S // TB
    FQ = FF // 4
    NS = FQ // LANES
    LQ = FQ - NS * LANES
    CQ = LANES // 4
    QR = LANES + CQ
    BLOCKS = [(2 * r1 + r2, 2 * h + p)
              for r1, h in ((0, 0), (1, 0), (0, 1), (1, 1)) for r2 in range(2) for p in range(2)]

    def z_rows(rq, c):
        lo = (NC * rq + c) * (TQ + 8)
        return slice(lo, lo + TQ)

    def store_z(r0, slot, toks, q0=0, q1=4):
        n = (q1 - q0) * TQ
        rows = pl.ds(r0 + q0 * TQ if isinstance(r0, int) else pl.multiple_of(r0 + q0 * TQ, TQ), n)
        zn = lane_tiles(_ln(hold(h_s[rows, :], _pick(toks, n // 8)), 4.0 * EPS))
        for rq in range(q0, q1):
            for c in range(NC - 1):
                zf_s[slot, z_rows(rq, c), :] = zn[c][(rq - q0) * TQ:(rq - q0 + 1) * TQ]
        zr_s[q0 * TQ:q1 * TQ, :] = zn[NC - 1].astype(BF16)

    def w3_ops(toks):
        ng = FQ // 16
        blk = lambda c, d: w3_v[c, d * FQ:(d + 1) * FQ, :].astype(F32)
        outer = [[_all_operands(_RHS, blk(k2, p), blk(k2, 2 + p), blk(2 + k2, p), blk(2 + k2, 2 + p))
                  for p in range(2)] for k2 in range(2)]
        for k, i in enumerate((1, 5, 2, 4, 0, 3, 6)):
            tk = [toks[((k + r * 7) * len(toks)) // (7 * ng)] for r in range(ng)]
            for j, x in enumerate(_all_operands(_RHS, hold16(outer[0][0][i], tk), outer[0][1][i], outer[1][0][i],
                                                hold16(outer[1][1][i], tk))):
                if i not in _RAW or j not in _RAW:
                    s3_s[i, j] = x.astype(BF16)

    def transpose_w4(toks):
        order = [(c, n) for n in (4 * NS, 4 * NS + 1) + tuple(range(4 * NS)) for c in range(NC)]
        for k, (c, n) in enumerate(order):
            if n >= 4 * NS:
                ends = [(2 * (n - 4 * NS) + p + 1) * FQ // 2 for p in range(2)]
                x = jnp.concatenate([w4_u[c, e - LQ // 2:e, :] for e in ends]
                                    + [jnp.zeros((HL - LQ, LANES), U32)], axis=0)
            else:
                lo = (n % 4) * FQ // 2 + (n // 4) * HL
                x = w4_u[c, lo:lo + HL, :]
            x = jnp.concatenate([after(toks[(k * len(toks)) // len(order)], x[0:8]), x[8:]], axis=0)
            wt_s[c, n] = _as_bf16(x).astype(F32).T.astype(BF16)

    def w4_ops(i, zero, toks):
        ng = QR // 16
        total = (NS * 7 + 2) * ng
        tk = lambda pos, step: [toks[((pos + r * step) * len(toks)) // total] for r in range(ng)]
        quarter = lambda n, d: jnp.concatenate(
            [wt_s[d, n].astype(F32), wt_s[NC - 1, n, d * CQ:(d + 1) * CQ, :].astype(F32)], axis=0)
        if i not in _RAW:
            for e in range(2):
                x = _operand(_RHS[i], lambda h, d: quarter(4 * NS + h, 2 * d + e))
                e4_s[i + zero, e] = hold16(x, tk(e * ng, 1)).astype(BF16)
        for st in range(NS):
            t = [[_operand(_RHS[i], lambda h, d: quarter(4 * st + 2 * h + p, 2 * d + e)) for e in range(2)]
                 for p in range(2)]
            tks = tk((2 + st * 7) * ng, 7)
            for j, x in enumerate(_all_operands(_RHS, hold16(t[0][0], tks), t[0][1], t[1][0], hold16(t[1][1], tks))):
                if i not in _RAW or j not in _RAW:
                    s4_s[i + zero, j, st] = x.astype(BF16)

    def gate_row(toks):
        ng = D // 8
        col = after(jnp.stack(_pick(toks, ng)), scol_s[...].reshape(ng, 8, LANES))
        for c in range(NC):
            wf = wm_v[:, (NC * NC + c) * LANES:(NC * NC + c + 1) * LANES].astype(F32).reshape(ng, 8, LANES)
            acc = col[0] * wf[0]
            for r in range(1, ng):
                acc = acc + col[r] * wf[r]
            mod_s[NC, :, c * LANES:(c + 1) * LANES] = jnp.broadcast_to(jnp.sum(acc, axis=0, keepdims=True), (8, LANES))

    def rem3(rq, d, pieces=1):
        z = _as_bf16(zr_u[rq * (TQ // 2):(rq + 1) * (TQ // 2), :])
        return jnp.concatenate([_dot_nt(_as_bf16(w3_u[NC - 1, lo // 2:hi // 2, :]), z)
                                for lo, hi in _chunks(d * FQ, (d + 1) * FQ, pieces)], axis=0)

    def lead_in():
        head = [rem3(*key) for key in BLOCKS[:4]]
        for k in range(4):
            rh_s[k] = head[k]
        return _rows8(head[0])

    def units(tiles, blocks):
        return [(c, b) for b in blocks for c in tiles]

    with jax.named_scope("A"):
        wait_all(sk_copy(0))
        conv_step(filt=0)
    with jax.named_scope("B_wait"):
        wait_all(sk_copy(1) + kv_groups[0])
    with jax.named_scope("B"):
        start_all(kv_groups[2] + kv_groups[3] + sk_copy(3) + sk_copy(4))
        conv_step(filt=1, units=units(PAIR, range(0, NB1)))
        scol_s[...] = jnp.broadcast_to(sc.astype(F32), (LANES, D)).T
    with jax.named_scope("C_wait"):
        wait_all(kv_groups[1])
    with jax.named_scope("C"):
        conv_step(units=units(PAIR, range(NB1, NBL)), lag=ULAG)
    with jax.named_scope("D_wait"):
        wait_all(sk_copy(2))
    with jax.named_scope("D"):
        start_all(wm_copies[0] + q_copies[0] + wm_copies[1] + w_copies[0])
        conv_step(filt=2, mul=0, free=MF[0], trim=MT[0])
    with jax.named_scope("E_wait"):
        wait_all(kv_groups[2])
    with jax.named_scope("E"):
        conv_step(units=units(TRIPLE, range(0, 2)), mul=1, inv=units((0,), range(NBL)), shift=ESH, free=MF[1], trim=MT[1])
    with jax.named_scope("F_wait"):
        wait_all(kv_groups[3])
    with jax.named_scope("F"):
        conv_step(units=units(TRIPLE, range(2, NBL)), lag=ULAG)

    def full_step(j, carry):
        wait_all(sk_copy(j + 2))
        conv_step(filt=j + 2, mul=j + 1, inv=units((j,), range(IG)), free=MF[2], trim=MT[2])
        return carry

    with jax.named_scope("GH"):
        lax.fori_loop(1, NC - 2, full_step, 0)
    late = units((NC - 2,), range(NBL)) + units(range(1, NC - 2), range(IG, NBL))
    late = late[:IJ] + units((NC - 1,), range(NBL)) + late[IJ:]
    with jax.named_scope("J"):
        start_all(q_copies[1] + w_copies[1] + sum(q_copies[2:], []) + w_copies[2] + w_copies[3] + wm_copies[2], 1)
        conv_step(mul=NC - 1, inv=late[:IJ], free=MF[3], trim=MT[3])
    with jax.named_scope("r6_wait"):
        wait_all(wm_copies[0] + q_copies[0])
    with jax.named_scope("r6"):
        for j in range(3):
            mod_chunk(j)
        conv_step(inv=late[IJ:IJ + 1])
        toks = conv_step(inv=late[IJ + 1:len(late) - IP])
        nx0 = stage_p1(0, A0[1], None, _pick(toks[:R6N], A0[1] // 8, R6F) if toks else None)
    with jax.named_scope("p2_wait"):
        wait_all(wm_copies[1])
    with jax.named_scope("p2"):
        mod_chunk(4)
        mod_chunk(3)
        toks = conv_step(inv=late[len(late) - IP:])
        if toks:
            nx0 = hold(nx0, _pick(toks[:P2N], A0[1] // 8, P2F))
        stage_p2(0, A0[1], nx0)
    with jax.named_scope("w1_wait"):
        wait_all(w_copies[0])
    with jax.named_scope("m1_0"):
        square_ops(w1_v, s1_s, stage_m1(0, 4)[:-40])
    with jax.named_scope("w2_wait"):
        wait_all(q_copies[1] + w_copies[1])
    with jax.named_scope("m2_0"):
        stage_p(1, stage_m2(0, SP0))
        filler(0)
    for t in range(1, NA):
        with jax.named_scope("a%d" % t):
            wait_all(q_copies[t + 1] if t + 1 < NA else w_copies[2] + w_copies[3] + wm_copies[2])
            toks = stage_m1(t, 2)
            toks = toks + stage_m2(t, 2, toks[len(toks) - len(toks) // 2:])
            if t + 1 < NA:
                stage_p(t + 1, toks)
            if t == 1:
                square_ops(w2_v, s2_s, toks[:-30])
            if t == NA - 1:
                transpose_w4(toks[:(len(toks) * XEND) // 100])
                store_z(0, 0, toks[(len(toks) * LW[0]) // 100:(len(toks) * LW[1]) // 100])
                toks = toks + [x for x in lead_in()[:40] for _ in range(WS[7])]
                cut = (len(toks) * CUT) // 100
                gate_row(toks[:(len(toks) * 9) // 10])
                w3_ops(toks[:cut])
                rest = [i for i in range(7) if i not in IN_LOOP]
                for k, i in enumerate(rest):
                    w4_ops(i, 0, toks[cut + k::len(rest)])
            filler(t)

    def out_copy(r0, n, c):
        rows = pl.ds(r0, n)
        return pltpu.make_async_copy(o_v.at[c, rows, :], o_hbm.at[rows, pl.ds(c * LANES, LANES)], sem_o.at[0])

    def raw4(n, d):
        return jnp.concatenate([wt_u[d, n], wt_u[NC - 1, n, d * (CQ // 2):(d + 1) * (CQ // 2), :]], axis=0)

    def mlp_tile(t, carry):
        r0 = pl.multiple_of(t * TB, TB)
        ws = t & 1
        count = [0]

        def fresh():
            count[0] += 1
            return lax.rem(t + 2 * count[0], 2)

        def g_rows(r2, p, lo, hi):
            base = (2 * r2 + p) * (FQ + GPAD)
            return slice(base + lo, base + hi)

        rem = {key: rh_s[k] for k, key in enumerate(BLOCKS[:4])}
        for key in BLOCKS[4:8]:
            rem[key] = rem3(*key)
        early = _rows8(rem[BLOCKS[4]], EW[0])
        rem[BLOCKS[8]] = rem3(*BLOCKS[8], pieces=4)
        todo = BLOCKS[9:]
        part = [None] * 7
        for i in (4, 3, 0, 6, 1, 2, 5):
            m = [None] * 7
            for j in _ORDER:
                slot = fresh()
                act = _operand(_LHS[j], lambda r2, k2: _operand(
                    _LHS[i], lambda r1, k1: zf_s[slot, z_rows(2 * r1 + r2, 2 * k1 + k2), :])).astype(BF16)
                if i in _RAW and j in _RAW:
                    d = 2 * _RAW.index(i) + _RAW.index(j)
                    wij = w3_u[d, d * (FQ // 2):(d + 1) * (FQ // 2), :]
                else:
                    wij = s3_u[i, j]
                m[j] = _dot_nt(_as_bf16(wij), act)
            key = todo.pop(0)
            rem[key] = rem3(*key)
            part[i] = _combine(m)
            if i in (4, 3, 0):
                early += _rows8(m[_ORDER[0]], EW[1]) + _rows8(m[_ORDER[4]], EW[2])
        zero = fresh() - ws
        fine = [x for x in early for _ in IN_LOOP]
        hop = len(fine) // (len(IN_LOOP) * 33)
        for k, i in enumerate(IN_LOOP):
            w4_ops(i, zero, fine[k * hop:len(fine) - (len(IN_LOOP) - k) * hop])
        for inner in range(4):
            r2, p = inner // 2, inner % 2
            for blk, pre in enumerate(_combine([part[i][inner] for i in range(7)])):
                g_s[blk][ws, g_rows(r2, p, 0, FQ), :] = _gelu2(pre + rem[2 * (blk // 2) + r2, 2 * (blk % 2) + p])

        toks = []
        marks = {}
        part = [[None] * 4 for _ in range(7)]
        for i in O4:
            slot = fresh()
            we = jnp.concatenate([raw4(4 * NS + _RAW.index(i), 2 * _RAW.index(i) + e) if i in _RAW else e4_u[i, e]
                                  for e in range(2)], axis=0)
            ex = []
            for r2 in range(2):
                act = [_operand(_LHS[i], lambda r1, h: g_s[2 * r1 + h][slot, g_rows(r2, p, NS * LANES, FQ), :])
                       for p in range(2)]
                act = jnp.concatenate(act + [jnp.zeros((LANES - 2 * LQ, TQ), F32)], axis=0).astype(BF16)
                ex.append(_dot(_as_bf16(we), act))
            m = [None] * 7
            for j in _ORDER:
                slot = fresh()
                act = _operand(_LHS[j], lambda r2, p: _operand(
                    _LHS[i], lambda r1, h: g_s[2 * r1 + h][slot, g_rows(r2, p, 0, NS * LANES), :])).astype(BF16)
                if i in _RAW and j in _RAW:
                    d = 2 * _RAW.index(i) + _RAW.index(j)
                    wij = [raw4(4 * st + d, d) for st in range(NS)]
                else:
                    wij = [s4_u[i, j, st] for st in range(NS)]
                m[j] = _dot(_as_bf16(jnp.concatenate(wij, axis=1)), act)
                toks += _rows8(m[j])
            part[i] = [x + ex[inner // 2][(inner % 2) * QR:(inner % 2 + 1) * QR]
                       for inner, x in enumerate(_combine(m))]
            marks[i] = len(toks)

        gb = 0.5 * mod_s[NC, 0:1, :]
        nxt = jnp.minimum(t + 1, NT - 1) * TB
        tails = {}
        for i, blk, norm in PLAN:
            r1 = blk // 2
            if norm is None:
                toks += [x for x in lead_in()[8:40] for _ in range(3)]
            elif norm[0] < norm[1]:
                store_z(nxt, 1 - ws, toks[norm[2]:norm[3]], norm[0], norm[1])
            pos = [marks[i] + FL[(1, 2, 0, 3).index(blk)]]

            def finish(rq, c, h2t):
                h2 = hold(h2t.T, toks[pos[0]:pos[0] + TQ // 8])
                pos[0] += TQ // 8
                rows = pl.ds(pl.multiple_of(r0 + rq * TQ, TQ), TQ)
                cols = slice(c * LANES, (c + 1) * LANES)
                o_v[c, rows, :] = (x_s[rows, cols] + gb[:, cols] * (h_s[rows, cols] + h2)).astype(BF16)
                if blk == 3:
                    out_copy(rows.start, TQ, c).start()

            for inner in (1, 2, 0, 3):
                ht = _block([part[k][inner] for k in range(7)], blk)
                rq, c = 2 * r1 + inner // 2, 2 * (blk % 2) + inner % 2
                finish(rq, c, ht[0:LANES])
                tails[rq, c] = ht[LANES:]
            rb = pl.multiple_of(r0 + r1 * 2 * TQ, 2 * TQ)
            if blk != 3:
                for e in range(2):
                    out_copy(rb, 2 * TQ, 2 * (blk % 2) + e).start()
            if blk in (0, 3):
                for rq in (2 * r1, 2 * r1 + 1):
                    finish(rq, NC - 1, jnp.concatenate([tails[rq, c] for c in range(NC - 1)], axis=0))
                if blk == 0:
                    out_copy(rb, 2 * TQ, NC - 1).start()
        return carry

    with jax.named_scope("ph2b"):
        lax.fori_loop(0, NT, mlp_tile, 0)
    with jax.named_scope("tail"):
        pltpu.make_async_copy(o_v, o_v, sem_o.at[0]).wait()


@jax.jit
def pallas_adaLN_cond__ssm_conv_h3__mixer_s_mlp__prompt_kernel(
    A_q: jax.Array,
    A_k: jax.Array,
    A_v: jax.Array,
    A_shift_k: jax.Array,
    A_ssm_k: jax.Array,
    A_ssm_D: jax.Array,
    B_x: jax.Array,
    B_w1: jax.Array,
    B_w2: jax.Array,
    B_w3: jax.Array,
    B_w4: jax.Array,
    c: jax.Array,
    w_mod: jax.Array,
):
    B, S, D = A_q.shape
    FF = B_w3.shape[1]
    assert (B, S, D, FF, A_shift_k.shape[1]) == (1, sum(TILES), 5 * LANES, 1728, 4)
    NC = D // LANES
    NG = BLK // 8
    NBL = S // (PH * BLK)
    NS = FF // 4 // LANES
    n1 = S - sum(TILES[:BLOCKWISE1[0]]) - HALO
    n2 = S - sum(TILES[:BLOCKWISE2[0]])

    args = (A_q.reshape(S, D), A_k.reshape(S, D), A_v.reshape(S, D), A_shift_k.T, A_ssm_k,
            A_ssm_D, B_w1, B_w2, B_w3.T, B_w4, c, w_mod)
    scratch = [
        pltpu.VMEM((S, D), BF16),
        pltpu.VMEM((NC, S + 16, LANES), BF16),
        pltpu.VMEM((NC, S, LANES), BF16),
        pltpu.VMEM((4, D), BF16),
        pltpu.VMEM((NC, LANES, S), BF16),
        pltpu.VMEM((D,), BF16),
        pltpu.VMEM((NC, D, LANES), BF16),
        pltpu.VMEM((NC, D, LANES), BF16),
        pltpu.VMEM((NC, FF, LANES), BF16),
        pltpu.VMEM((NC, FF, LANES), BF16),
        pltpu.VMEM((1, D), BF16),
        pltpu.VMEM((D, 6 * D), BF16),
        pltpu.VMEM((PH, 2 * BLK, BLK), BF16),
        pltpu.VMEM((PH, 2, BLK, BLK), BF16),
        pltpu.VMEM((NC, S, LANES), BF16),
        pltpu.VMEM((NC, NG, NBL, PH, 2, 8, LANES), F32),
        pltpu.VMEM((NC, NG, NBL, PH, 2, 8, LANES), F32),
        pltpu.VMEM((NC, NBL, PH, 2 * BLK, LANES), BF16),
        pltpu.VMEM((6, PH, BLK, LANES), BF16),
        pltpu.VMEM((NC, S, LANES), F32),
        pltpu.VMEM((6, 8, D), F32),
        pltpu.VMEM((NC, 8, LANES), F32),
        pltpu.VMEM((NC, S + 16, LANES), F32),
        pltpu.VMEM((S, D), F32),
        pltpu.VMEM((S, D), F32),
        pltpu.VMEM((NC, S, LANES), BF16),
        pltpu.VMEM((7, 7, FF // 4, LANES), BF16),
        pltpu.VMEM((7, 7, NS, D // 4, LANES), BF16),
        pltpu.VMEM((7, 2, D // 4, LANES), BF16),
        [pltpu.VMEM((2, GROWS, TQ), F32)] * 4,
        pltpu.VMEM((2, 4 * NC * (TQ + 8), LANES), F32),
        pltpu.VMEM((TB, LANES), BF16),
        pltpu.VMEM((10, 2, n1 // 2, LANES), BF16),
        pltpu.VMEM((10, 2, n2 // 2, LANES), BF16),
        pltpu.VMEM((7, 2, 2 * LANES, LANES), BF16),
        pltpu.VMEM((7, 2, 2 * LANES, LANES), BF16),
        pltpu.VMEM((4, FF // 4, TQ), F32),
        pltpu.VMEM((NC, 4 * NS + 2, LANES, LANES), BF16),
        pltpu.VMEM((D, LANES), F32),
        pltpu.SemaphoreType.DMA((21,)),
        pltpu.SemaphoreType.DMA((1,)),
    ]
    out = pl.pallas_call(
        functools.partial(_kernel, S=S, D=D, FF=FF),
        in_specs=[pl.BlockSpec(memory_space=pl.ANY)] * len(args),
        out_specs=pl.BlockSpec(memory_space=pl.ANY),
        out_shape=jax.ShapeDtypeStruct((S, D), BF16),
        scratch_shapes=scratch,
        compiler_params=pltpu.CompilerParams(
            vmem_limit_bytes=120 * 1024 * 1024,
            disable_bounds_checks=True,
            disable_semaphore_checks=True,
        ),
    )(*args)
    return out.reshape(B, S, D)
```

```python
import functools
import math

import jax
import jax.numpy as jnp
from jax import lax
import jax.experimental.pallas as pl
import jax.experimental.pallas.tpu as pltpu

F32 = jnp.float32
BF16 = jnp.bfloat16
U32 = jnp.uint32

LANES = 128
BLK = 128
PH = 4
EPS = 1e-05
TB = 512
TQ = TB // 4
HALO = 32
TILES = (384, 384, 576, 704)
BLOCKWISE1 = (3,)
BLOCKWISE2 = (2, 3)
IN_LOOP = (2, 4, 1, 3, 0)
O4 = (2, 4, 1, 3, 0, 6, 5)
NW = (1, 3, 0, 150, 320, 460, 600, 730)
PLAN = ((4, 1, (0, NW[0], NW[2], NW[3])), (3, 2, (NW[0], NW[1], NW[4], NW[5])), (6, 0, (NW[1], 4, NW[6], NW[7])), (5, 3, None))
FL = (10, 10, 25, -32)
EW = (2, 1, 2)
TRS = (135, 165, 180)
FRS = (45, 90, 90)
WS = (2, 3, 3, 2, 2, 2, 2, 4)
LW = (66, 92)
FI = (48, 96, 96, 96)
SP0 = 4
NB1 = 1
ESH = 0
ULAG = 9
R6 = 2
R6N = 36
R6F = 18
MF = (6, 0, 5, 4)
MT = (3, 0, 3, 3)
IG = 2
IJ = 6
IP = 2
P2N = 28
P2F = 6
ROT = 3
KR = 256
GPAD = 8
GROWS = 1768
XEND = 55
CUT = 82

_ORDER = (2, 4, 1, 3, 0, 6, 5)
_RAW = (1, 4)
_LHS = (((0, 0), 1, (1, 1)), ((1, 0), 1, (1, 1)), ((0, 0),), ((1, 1),),
        ((0, 0), 1, (0, 1)), ((1, 0), -1, (0, 0)), ((0, 1), -1, (1, 1)))
_RHS = (((0, 0), 1, (1, 1)), ((0, 0),), ((0, 1), -1, (1, 1)), ((1, 0), -1, (0, 0)),
        ((1, 1),), ((0, 0), 1, (0, 1)), ((1, 0), 1, (1, 1)))


def _operand(terms, blk):
    x = blk(*terms[0])
    if len(terms) > 1:
        y = blk(*terms[2])
        x = x + y if terms[1] > 0 else x - y
    return x


def _all_operands(table, b00, b01, b10, b11):
    blocks = ((b00, b01), (b10, b11))
    return [_operand(terms, lambda i, j: blocks[i][j]) for terms in table]


def _block(m, which):
    if which == 0:
        return (m[3] - m[4]) + m[0] + m[6]
    if which == 1:
        return m[2] + m[4]
    if which == 2:
        return m[1] + m[3]
    return (m[2] - m[1]) + m[0] + m[5]


def _combine(m):
    return [_block(m, which) for which in range(4)]


def _as_bf16(x):
    return pltpu.bitcast(x, BF16)


def _lo(x):
    return pltpu.bitcast(x << 16, F32)


def _hi(x):
    return pltpu.bitcast(x & jnp.uint32(0xFFFF0000), F32)


def _dft4(re, im, sign):
    ar, ai = re[0] + re[2], im[0] + im[2]
    br, bi = re[0] - re[2], im[0] - im[2]
    cr, ci = re[1] + re[3], im[1] + im[3]
    dr, di = re[1] - re[3], im[1] - im[3]
    o0 = (ar + cr, ai + ci)
    o2 = (ar - cr, ai - ci)
    m = (br + di, bi - dr)
    p = (br - di, bi + dr)
    o1, o3 = (m, p) if sign < 0 else (p, m)
    return [o0[0], o1[0], o2[0], o3[0]], [o0[1], o1[1], o2[1], o3[1]]


def _ln(x, eps=EPS, unit=True):
    n = x.shape[-1]
    s1 = jnp.sum(x, axis=-1, keepdims=True)
    m = s1 * (1.0 / n)
    v = jnp.maximum(jnp.sum(x * x, axis=-1, keepdims=True) + (n * eps - s1 * m), n * eps)
    e = jnp.log(v) * (-0.5 / math.log(2.0))
    return (x - m) * jnp.exp2(e + 0.5 * math.log2(n) if unit else e)


def _gelu2(x):
    c0 = math.sqrt(2.0 / math.pi)
    return x + x * jnp.tanh(x * (c0 + (c0 * 0.044715) * (x * x)))


def _dot(a, b):
    return jnp.dot(a, b, preferred_element_type=F32)


def _dot_nt(a, b):
    return lax.dot_general(a, b, (((1,), (1,)), ((), ())), preferred_element_type=F32)


def _rows8(x, repeat=1):
    return [x[8 * r:8 * r + 8, 0:LANES] for r in range(x.shape[0] // 8) for _ in range(repeat)]


def _chunks(r0, r1, k, unit=16):
    n = (r1 - r0) // unit
    cuts = [r0 + unit * ((n * j) // k) for j in range(k + 1)]
    return list(zip(cuts[:-1], cuts[1:]))


def _pick(toks, n, free=0):
    idx = [(r * (len(toks) + free)) // n - free for r in range(n)]
    return [toks[i] if i >= 0 else None for i in idx]


def _kernel(q_hbm, k_hbm, v_hbm, sh_hbm, sk_hbm, sd_hbm, w1_hbm, w2_hbm, w3_hbm, w4_hbm, c_hbm, wm_hbm,
            o_hbm,
            q_v, k_v, v_v, sh_v, sk_v, sd_v, w1_v, w2_v, w3_v, w4_v, c_v, wm_v,
            fw_s, iv_s, o_v, u_s, kk_s, vv_s, wu_s, y_s, mod_s, par_s, h1_s, x_s, h_s, z_s,
            s3_s, s4_s, e4_s, g_s, zf_s, zr_s, l1_s, l2_s, s1_s, s2_s, rh_s, wt_s, scol_s,
            sem, sem_o,
            *, S, D, FF):
    NC = D // LANES
    NG = BLK // 8
    LB = PH * BLK
    NBL = S // LB
    R = BLK // PH
    HL = LANES // 2

    small = [
        pltpu.make_async_copy(sh_hbm, sh_v, sem.at[0]),
        pltpu.make_async_copy(sd_hbm, sd_v, sem.at[0]),
        pltpu.make_async_copy(c_hbm, c_v, sem.at[0]),
    ]

    def sk_copy(c):
        ch = (c + ROT) % NC * LANES
        rows = pl.ds(ch if isinstance(c, int) else pl.multiple_of(ch, LANES), LANES)
        return [pltpu.make_async_copy(sk_hbm.at[rows, :], sk_v.at[c], sem.at[1 + c])]

    def kv_copies(tiles, blocks, s):
        return [pltpu.make_async_copy(src.at[pl.ds(r, KR), pl.ds((c + ROT) % NC * LANES, LANES)],
                                      dst.at[c, pl.ds(off + r, KR), :], sem.at[s])
                for r in range(blocks[0] * LB, (blocks[-1] + 1) * LB, KR)
                for src, dst, off in ((k_hbm, k_v, 16), (v_hbm, v_v, 0)) for c in tiles]

    PAIR, TRIPLE = (0, 1), (2, 3, 4)
    kv_groups = [kv_copies(PAIR, range(0, NB1), 9), kv_copies(PAIR, range(NB1, NBL), 10),
                 kv_copies(TRIPLE, range(0, 2), 11), kv_copies(TRIPLE, range(2, NBL), 20)]

    WM = (0, 3 * D, 5 * D, 6 * D)
    wm_copies = [[pltpu.make_async_copy(wm_hbm.at[:, pl.ds(WM[j], WM[j + 1] - WM[j])],
                                        wm_v.at[:, pl.ds(WM[j], WM[j + 1] - WM[j])], sem.at[6 + j])]
                 for j in range(3)]
    w_copies = [[pltpu.make_async_copy(src.at[:, pl.ds(c * LANES, LANES)], dst.at[c], sem.at[12 + j])
                 for c in range(NC)]
                for j, (src, dst) in enumerate(((w1_hbm, w1_v), (w2_hbm, w2_v), (w3_hbm, w3_v), (w4_hbm, w4_v)))]

    B0 = [0]
    for n in TILES:
        B0.append(B0[-1] + n)
    NA = len(TILES)
    A0 = [0] + [r + HALO for r in B0[1:-1]] + [S]
    q_copies = [
        [pltpu.make_async_copy(q_hbm.at[pl.ds(A0[t], A0[t + 1] - A0[t])], q_v.at[pl.ds(A0[t], A0[t + 1] - A0[t])],
                               sem.at[16 + t])]
        for t in range(NA)
    ]

    def start_all(cps, priority=0):
        for cp in cps:
            cp.start(priority=priority)

    def wait_all(cps):
        for cp in cps:
            cp.wait()

    for c in range(NC):
        k_v[c, 0:16, :] = jnp.zeros((16, LANES), BF16)
    start_all(sk_copy(0) + small + sk_copy(1) + kv_groups[0] + kv_groups[1] + sk_copy(2))

    for c in range(NC):
        h1_s[c, 0:8, :] = jnp.zeros((8, LANES), F32)
        h1_s[c, S + 8:S + 16, :] = jnp.zeros((8, LANES), F32)

    prow = lax.broadcasted_iota(jnp.int32, (BLK, BLK), 0)
    pcol = lax.broadcasted_iota(jnp.int32, (BLK, BLK), 1)
    ang = (((4 * prow + 1) * pcol) & (4 * BLK - 1)).astype(F32) * (2.0 * math.pi / (4 * BLK))
    tw = (4 * prow + 1).astype(F32) * (2.0 * math.pi / (4 * LB))
    mr, mi = jnp.cos(ang), -jnp.sin(ang)
    twr, twi = jnp.cos(tw), -jnp.sin(tw)
    eye = jnp.where(prow == pcol, 1.0 / LB, 0.0).astype(BF16)
    for i in range(PH):
        both = jnp.stack([mr.reshape(NG, 8, BLK), mi.reshape(NG, 8, BLK)], axis=1).reshape(2 * BLK, BLK)
        fw_s[i] = both.astype(BF16)
        for h in range(2):
            iv_s[i, h] = _dot_nt(eye, both[h * BLK:(h + 1) * BLK, :].astype(BF16)).astype(BF16)
        if i + 1 < PH:
            mr, mi = mr * twr - mi * twi, mr * twi + mi * twr
    perm = jnp.where(pcol == (prow % R) * PH + prow // R, 1.0, 0.0).astype(BF16)

    wait_all(small)
    shf = sh_v[...].astype(F32)
    sdf = sd_v[...].astype(F32).reshape(1, D)
    for c in range(NC):
        par_s[(c - ROT) % NC, 0:4, :] = shf[:, c * LANES:(c + 1) * LANES]
        par_s[(c - ROT) % NC, 4:5, :] = sdf[:, c * LANES:(c + 1) * LANES]
    cf = c_v[...].astype(F32)
    sc = (cf * jax.nn.sigmoid(cf)).astype(BF16)
    sc16 = jnp.broadcast_to(sc, (16, D))

    def mod_chunk(j):
        mod_s[j] = _dot(sc16, wm_v[:, j * D:(j + 1) * D])[0:8, :]

    (fw_u, iv_u, k_u, v_u, wu_u, vv_u, z_u, l1_u, l2_u, w1_u, w2_u, s1_u, s2_u, w3_u, w4_u, wt_u, s3_u, s4_u,
     e4_u, zr_u) = (r.bitcast(U32) for r in (fw_s, iv_s, k_v, v_v, wu_s, vv_s, z_s, l1_s, l2_s, w1_v, w2_v,
                                             s1_s, s2_s, w3_v, w4_v, wt_s, s3_s, s4_s, e4_s, zr_s))

    never = twr[0:8, :] > 2.0

    def after(token, x):
        if token.dtype != x.dtype:
            token = pltpu.bitcast(token, x.dtype)
        return jnp.where(jnp.broadcast_to(never, x.shape), token, x)

    def hold(x, tks):
        f = len([k for k in tks if k is None])
        n = len(tks)
        head = after(jnp.stack(tks[f:]), x[8 * f:, 0:LANES].reshape(n - f, 8, LANES)).reshape(8 * (n - f), LANES)
        if f:
            head = jnp.concatenate([x[:8 * f, 0:LANES], head], axis=0)
        return head if x.shape[1] == LANES else jnp.concatenate([head, x[:, LANES:]], axis=1)

    def hold16(x, tks):
        x4 = x.reshape(len(tks), 2, 8, LANES)
        return jnp.stack([after(jnp.stack(tks), x4[:, 0]), x4[:, 1]], axis=1).reshape(x.shape)

    def perm_k(c, b, toks):
        kt = [_dot_nt(perm, sk_v[c, :, b * LB + t * BLK:b * LB + (t + 1) * BLK]) for t in range(PH)]
        toks += _rows8(kt[0])[::2]
        return [jnp.concatenate([kt[t][i * R:(i + 1) * R, :] for t in range(PH)], axis=0).astype(BF16)
                for i in range(PH)]

    def spectrum(comps, dst, slot, b, toks, dc=None, pins=None):
        tr, ti = [], []
        for i in range(PH):
            lhs = fw_u[i]
            if pins is not None and i < len(pins):
                lhs = after(pins[i], lhs.reshape(NG, 8, LANES)).reshape(BLK, LANES)
            t4 = _dot(_as_bf16(lhs), comps[i]).reshape(NG, 2, 8, LANES)
            tr.append(t4[:, 0])
            ti.append(t4[:, 1])
        toks += [ti[PH - 1][g] for g in range(NG)]
        if dc is not None:
            tr[0] = tr[0] + dc
        sr, si = _dft4(tr, ti, -1)
        for qq in range(PH):
            dst[slot, :, b, qq, 0] = sr[qq]
            dst[slot, :, b, qq, 1] = si[qq]

    def gated(c, b, n):
        w = [par_s[c, t:t + 1, :] for t in range(4)]
        kc = {}
        for o in range(-2, 2):
            words = k_u[c, pl.ds(8 + b * (LB // 2) + o, BLK, stride=2), :]
            if o > -2:
                kc[2 * o] = _lo(words)
            kc[2 * o + 1] = _hi(words)
        vc = {}
        for o in range(2):
            words = v_u[c, pl.ds(b * (LB // 2) + o, BLK, stride=2), :]
            vc[2 * o] = _lo(words)
            vc[2 * o + 1] = _hi(words)
        for i in range(PH):
            ks = kc[i] * w[0]
            for t in range(1, 4):
                ks = ks + kc[i - t] * w[t]
            wu_s[n, i] = (ks * vc[i]).astype(BF16)
        return [wu_u[n, i] for i in range(PH)]

    def kv_pins(kvb):
        return [jnp.stack([kvb[2 * m + (r % 2)][8 * (r // 2):8 * (r // 2) + 8, :] for r in range(NG)])
                for m in range(2)]

    def products(c, ks, kc, toks, free, trim):
        n = len(toks) - trim + free
        cum = (44, 128, 244, 392)
        zp = None
        for o in range(NBL):
            idx = [((g * cum[-1] + cum[o]) * n) // (cum[-1] * NG) - 1 - free for g in range(NG)]
            tk = [toks[max(i, 0)] if i >= 0 or not free else None for i in idx]
            zr, zi = [], []
            for qq in range(PH):
                accr = acci = None
                for b in range(o + 1):
                    a_, b_ = u_s[c, :, b, qq, 0], u_s[c, :, b, qq, 1]
                    c_, d_ = ks[kc, :, o - b, qq, 0], ks[kc, :, o - b, qq, 1]
                    if qq == 0 and b == o:
                        a_ = hold(a_.reshape(BLK, LANES), tk).reshape(NG, 8, LANES)
                    tr_ = a_ * c_ - b_ * d_
                    ti_ = a_ * d_ + b_ * c_
                    accr = tr_ if accr is None else accr + tr_
                    acci = ti_ if acci is None else acci + ti_
                zr.append(accr)
                zi.append(acci)
            if zp is None:
                yr, yi = zr, zi
            else:
                yr = [zr[qq] - zp[1][qq] for qq in range(PH)]
                yi = [zi[qq] + zp[0][qq] for qq in range(PH)]
            zp = (zr, zi)
            vr, vi = _dft4(yr, yi, +1)
            for i in range(PH):
                vv_s[c, o, i] = jnp.stack([vr[i], vi[i]], axis=1).reshape(2 * BLK, LANES).astype(BF16)

    def inverse(c, o, toks, pins):
        for i in range(PH):
            yv = None
            for h in range(2):
                lhs = iv_u[i, h]
                if pins is not None and h == 0:
                    pin = pins[i % 2][8 * (i // 2):8 * (i // 2) + 8]
                    lhs = after(pin, lhs.reshape(8, 8, LANES)).reshape(HL, LANES)
                t = _dot(_as_bf16(lhs), _as_bf16(vv_u[c, o, i, h * HL:(h + 1) * HL, :]))
                yv = t if yv is None else yv + t
            if i % 2 == 0:
                toks += _rows8(yv)[::2]
            y_s[c, pl.ds(o * LB + i, BLK, stride=PH), :] = yv

    def conv_step(filt=None, units=(), mul=None, inv=(), shift=0, lag=2, free=0, trim=3):
        toks = []
        kv = [gated(c, b, n) for n, (c, b) in enumerate(units)]
        lead = len(inv) + (NBL if filt is not None else 0)
        pin_at = {}
        for n in range(len(units)):
            at = n + min(shift, lead - lag)
            if at >= 0:
                pin_at[at] = kv_pins(kv[n])
        if filt is not None and mul is not None and not isinstance(filt, int):
            ks = kk_s.at[pl.ds(mul, 2)]
            k_rd, k_wr = (ks, 0), (ks, 1)
        else:
            k_rd, k_wr = (kk_s, mul), (kk_s, filt)
        pos = 0
        for c, o in inv:
            inverse(c, o, toks, pin_at.get(pos))
            pos += 1
        if filt is not None:
            comps = [perm_k(filt, b, toks) for b in range(NBL)]
            for b in range(NBL):
                spectrum(comps[b], *k_wr, b, toks, par_s[filt, 4:5, :] if b == 0 else None, pin_at.get(pos))
                pos += 1
        for n, (c, b) in enumerate(units):
            spectrum([_as_bf16(x) for x in kv[n]], u_s, c, b, toks, None, pin_at.get(pos))
            pos += 1
        if mul is not None:
            products(mul, *k_rd, toks, free, trim)
        return toks

    def lane_tiles(x):
        return [x[:, c * LANES:(c + 1) * LANES] for c in range(NC)]

    def stage_p1(r0, r1, tks=None, ytks=None):
        ga = mod_s[2, 0:1, :]
        a_mul, a_add = ga * (1.0 + mod_s[1, 0:1, :]) * math.sqrt(D), ga * mod_s[0, 0:1, :]
        q = q_v[r0:r1, :].astype(F32)
        if tks is not None:
            q = hold(q, tks)
        y = jnp.concatenate([y_s[(c - ROT) % NC, r0:r1, :] for c in range(NC)], axis=1)
        if ytks is not None:
            y = hold(y, ytks)
        x = q + (_ln(q, unit=False) * a_mul + a_add) * y
        x_s[r0:r1, :] = x
        return _ln(x, unit=False)

    def store_row_ops(dst, base, r0, r1, cols, tks=None):
        hv = []
        for x in cols:
            x4 = x.reshape(x.shape[0] // 32, 2, 16, LANES)
            hv.append([x4[:, e].reshape(x.shape[0] // 2, LANES) for e in range(2)])
        for k2 in range(2):
            a00, a01, a10, a11 = hv[k2][0], hv[2 + k2][0], hv[k2][1], hv[2 + k2][1]
            if tks is not None:
                a00, a11 = hold16(a00, tks), hold16(a11, tks)
            for o, x in enumerate(_all_operands(_LHS, a00, a01, a10, a11) + [a01, a10, hv[NC - 1][k2]]):
                dst[o, k2, (r0 - base) // 2:(r1 - base) // 2, :] = x.astype(BF16)

    L1B = A0[BLOCKWISE1[0]]
    L2B = B0[BLOCKWISE2[0]]

    def stage_p2(r0, r1, nx, blockwise=False):
        h = nx * ((1.0 + mod_s[4, 0:1, :]) * (2.0 * math.sqrt(D))) + 2.0 * mod_s[3, 0:1, :]
        h_s[r0:r1, :] = h
        zn = lane_tiles(_ln(h, 4.0 * EPS))
        if blockwise:
            store_row_ops(l1_s, L1B, r0, r1, zn)
        else:
            for c in range(NC):
                z_s[c, r0:r1, :] = zn[c].astype(BF16)

    def stage_p(t, toks):
        lo, hi = A0[t], A0[t + 1]
        stage_p2(lo, hi, stage_p1(lo, hi, _pick(toks[:-TRS[t - 1]], (hi - lo) // 8, FRS[t - 1])), t in BLOCKWISE1)

    def filler(t):
        red = jnp.sum(y_s[t, 0:8 * FI[t], :], axis=-1, keepdims=True).reshape(FI[t], 8, 1)
        spare = (NC - 1) * (TQ + 8) + 8 * t
        zf_s[1, spare:spare + 8, :] = jnp.broadcast_to(jnp.sum(red, axis=0), (8, LANES))

    def square_ops(src, dst, toks):
        HK = 2 * LANES
        tks = _pick(toks, 2 * HK // 16)
        for n2 in range(2):
            tk = tks[n2 * (HK // 16):(n2 + 1) * (HK // 16)]
            blk = lambda k, n: src[2 * n + n2, k * HK:(k + 1) * HK, :].astype(F32)
            for o, x in enumerate(_all_operands(_RHS, hold16(blk(0, 0), tk), blk(0, 1), blk(1, 0), hold16(blk(1, 1), tk))):
                if o not in _RAW:
                    dst[o, n2] = x.astype(BF16)

    def block_dots(ops_u, base, prepare, w_u, s_u, parts, emit, light, heavy):
        toks = []

        def timed(x, weight):
            toks.extend(_rows8(x, weight))
            return x

        def weave(top, bot):
            n = top.shape[0] // 16
            return jnp.stack([top.reshape(n, 16, LANES), bot.reshape(n, 16, LANES)], axis=1).reshape(32 * n, LANES)

        def main(get):
            m = [None] * 7
            rem = [None, None]
            for o in ('t', 2, 4, 'b', 1, 3, 0, 6, 5):
                if o in ('t', 'b'):
                    e = 0 if o == 't' else 1
                    rhs = jnp.concatenate([w_u[c, 2 * LANES:D // 2, :] for c in range(NC - 1)], axis=1)
                    rem[e] = timed(_dot(get([(9, e)]), _as_bf16(rhs)), light)
                    continue
                if o in _RAW:
                    d = _RAW.index(o)
                    rhs = jnp.concatenate([w_u[2 * d + n2, d * LANES:(d + 1) * LANES, :] for n2 in range(2)], axis=1)
                else:
                    rhs = jnp.concatenate([s_u[o, n2] for n2 in range(2)], axis=1)
                m[o] = timed(_dot(get([(o, 0), (o, 1)]), _as_bf16(rhs)), heavy if o in (4, 3, 6, 5) else light)
            c00, c01, c10, c11 = _combine(m)
            top = jnp.concatenate([c00, c01], axis=1) + rem[0]
            bot = jnp.concatenate([c10, c11], axis=1) + rem[1]
            return [weave(top[:, c * LANES:(c + 1) * LANES], bot[:, c * LANES:(c + 1) * LANES]) for c in range(NC - 1)]

        def last(get):
            w = _as_bf16(w_u[NC - 1])
            return weave(timed(_dot(get([(2, 0), (2, 1), (7, 0), (7, 1), (9, 0)]), w), light),
                         timed(_dot(get([(8, 0), (8, 1), (3, 0), (3, 1), (9, 1)]), w), light))

        mark = None
        for j, (r0, r1) in enumerate(parts):
            prepare(r0, r1, None if mark is None else toks[mark:])
            mark = len(toks)
            get = lambda keys: _as_bf16(jnp.concatenate(
                [ops_u[o, e, (r0 - base) // 4:(r1 - base) // 4, :] for o, e in keys], axis=1))
            if j % 2:
                tail = last(get)
                emit(r0, r1, main(get) + [tail])
            else:
                emit(r0, r1, main(get) + [last(get)])
        return toks

    def stage_m1(t, k):
        def emit(r0, r1, cols):
            out = [_gelu2(x) for x in cols]
            for c in range(NC):
                h1_s[c, r0 + 8:r1 + 8, :] = out[c]
            return out

        if t in BLOCKWISE1:
            return block_dots(l1_u, L1B, lambda *_: None, w1_u, s1_u, _chunks(A0[t], A0[t + 1], k, 32), emit, WS[2], WS[3])
        toks = []
        for r0, r1 in _chunks(A0[t], A0[t + 1], k):
            lhs = jnp.concatenate([z_u[c, r0 // 2:r1 // 2, :] for c in range(NC)], axis=1)
            w = jnp.concatenate([w1_u[c] for c in range(NC)], axis=1)
            for x in emit(r0, r1, lane_tiles(_dot(_as_bf16(lhs), _as_bf16(w)))):
                toks += _rows8(x, WS[0] if t != 2 else WS[6])
        return toks

    def shifted(r0, r1):
        n, grp, shifts = r1 - r0, D // 4, (-1, 1, -2, 2)
        lane = lax.broadcasted_iota(jnp.int32, (n, LANES), 1)
        cols = []
        for c in range(NC):
            lo, hi = c * LANES, (c + 1) * LANES
            g_lo, g_hi = lo // grp, (hi - 1) // grp
            val = h1_s[c, pl.ds(r0 + 8 + shifts[g_lo], n), :]
            if g_hi != g_lo:
                other = h1_s[c, pl.ds(r0 + 8 + shifts[g_hi], n), :]
                val = jnp.where(lane < (g_hi * grp - lo), val, other)
            cols.append(val)
        return cols

    def stage_m2(t, k, before=None):
        def emit(r0, r1, cols):
            x1 = h_s[r0:r1, :] + jnp.concatenate(cols, axis=1)
            h_s[r0:r1, :] = x1
            return x1

        if t in BLOCKWISE2:
            def prepare(r0, r1, prev):
                prev = before if prev is None else prev
                prev = prev[len(prev) // 8:(len(prev) * 7) // 8]
                store_row_ops(l2_s, L2B, r0, r1, shifted(r0, r1), _pick(prev, (r1 - r0) // 32))
            return block_dots(l2_u, L2B, prepare, w2_u, s2_u, _chunks(B0[t], B0[t + 1], k, 32), emit, WS[4 if t == 2 else 5], WS[4 if t == 2 else 5])
        toks = []
        for r0, r1 in _chunks(B0[t], B0[t + 1], k):
            w = jnp.concatenate([w2_u[c] for c in range(NC)], axis=1)
            hs = _dot(jnp.concatenate(shifted(r0, r1), axis=1).astype(BF16), _as_bf16(w))
            for x in lane_tiles(emit(r0, r1, [hs])):
                toks += _rows8(x, WS[1])
        return toks

    NT = S // TB
    FQ = FF // 4
    NS = FQ // LANES
    LQ = FQ - NS * LANES
    CQ = LANES // 4
    QR = LANES + CQ
    BLOCKS = [(2 * r1 + r2, 2 * h + p)
              for r1, h in ((0, 0), (1, 0), (0, 1), (1, 1)) for r2 in range(2) for p in range(2)]

    def z_rows(rq, c):
        lo = (NC * rq + c) * (TQ + 8)
        return slice(lo, lo + TQ)

    def store_z(r0, slot, toks, q0=0, q1=4):
        n = (q1 - q0) * TQ
        rows = pl.ds(r0 + q0 * TQ if isinstance(r0, int) else pl.multiple_of(r0 + q0 * TQ, TQ), n)
        zn = lane_tiles(_ln(hold(h_s[rows, :], _pick(toks, n // 8)), 4.0 * EPS))
        for rq in range(q0, q1):
            for c in range(NC - 1):
                zf_s[slot, z_rows(rq, c), :] = zn[c][(rq - q0) * TQ:(rq - q0 + 1) * TQ]
        zr_s[q0 * TQ:q1 * TQ, :] = zn[NC - 1].astype(BF16)

    def w3_ops(toks):
        ng = FQ // 16
        blk = lambda c, d: w3_v[c, d * FQ:(d + 1) * FQ, :].astype(F32)
        outer = [[_all_operands(_RHS, blk(k2, p), blk(k2, 2 + p), blk(2 + k2, p), blk(2 + k2, 2 + p))
                  for p in range(2)] for k2 in range(2)]
        for k, i in enumerate((1, 5, 2, 4, 0, 3, 6)):
            tk = [toks[((k + r * 7) * len(toks)) // (7 * ng)] for r in range(ng)]
            for j, x in enumerate(_all_operands(_RHS, hold16(outer[0][0][i], tk), outer[0][1][i], outer[1][0][i],
                                                hold16(outer[1][1][i], tk))):
                if i not in _RAW or j not in _RAW:
                    s3_s[i, j] = x.astype(BF16)

    def transpose_w4(toks):
        order = [(c, n) for n in (4 * NS, 4 * NS + 1) + tuple(range(4 * NS)) for c in range(NC)]
        for k, (c, n) in enumerate(order):
            if n >= 4 * NS:
                ends = [(2 * (n - 4 * NS) + p + 1) * FQ // 2 for p in range(2)]
                x = jnp.concatenate([w4_u[c, e - LQ // 2:e, :] for e in ends]
                                    + [jnp.zeros((HL - LQ, LANES), U32)], axis=0)
            else:
                lo = (n % 4) * FQ // 2 + (n // 4) * HL
                x = w4_u[c, lo:lo + HL, :]
            x = jnp.concatenate([after(toks[(k * len(toks)) // len(order)], x[0:8]), x[8:]], axis=0)
            wt_s[c, n] = _as_bf16(x).astype(F32).T.astype(BF16)

    def w4_ops(i, zero, toks):
        ng = QR // 16
        total = (NS * 7 + 2) * ng
        tk = lambda pos, step: [toks[((pos + r * step) * len(toks)) // total] for r in range(ng)]
        quarter = lambda n, d: jnp.concatenate(
            [wt_s[d, n].astype(F32), wt_s[NC - 1, n, d * CQ:(d + 1) * CQ, :].astype(F32)], axis=0)
        if i not in _RAW:
            for e in range(2):
                x = _operand(_RHS[i], lambda h, d: quarter(4 * NS + h, 2 * d + e))
                e4_s[i + zero, e] = hold16(x, tk(e * ng, 1)).astype(BF16)
        for st in range(NS):
            t = [[_operand(_RHS[i], lambda h, d: quarter(4 * st + 2 * h + p, 2 * d + e)) for e in range(2)]
                 for p in range(2)]
            tks = tk((2 + st * 7) * ng, 7)
            for j, x in enumerate(_all_operands(_RHS, hold16(t[0][0], tks), t[0][1], t[1][0], hold16(t[1][1], tks))):
                if i not in _RAW or j not in _RAW:
                    s4_s[i + zero, j, st] = x.astype(BF16)

    def gate_row(toks):
        ng = D // 8
        col = after(jnp.stack(_pick(toks, ng)), scol_s[...].reshape(ng, 8, LANES))
        for c in range(NC):
            wf = wm_v[:, (NC * NC + c) * LANES:(NC * NC + c + 1) * LANES].astype(F32).reshape(ng, 8, LANES)
            acc = col[0] * wf[0]
            for r in range(1, ng):
                acc = acc + col[r] * wf[r]
            mod_s[NC, :, c * LANES:(c + 1) * LANES] = jnp.broadcast_to(jnp.sum(acc, axis=0, keepdims=True), (8, LANES))

    def rem3(rq, d, pieces=1):
        z = _as_bf16(zr_u[rq * (TQ // 2):(rq + 1) * (TQ // 2), :])
        return jnp.concatenate([_dot_nt(_as_bf16(w3_u[NC - 1, lo // 2:hi // 2, :]), z)
                                for lo, hi in _chunks(d * FQ, (d + 1) * FQ, pieces)], axis=0)

    def lead_in():
        head = [rem3(*key) for key in BLOCKS[:4]]
        for k in range(4):
            rh_s[k] = head[k]
        return _rows8(head[0])

    def units(tiles, blocks):
        return [(c, b) for b in blocks for c in tiles]

    with jax.named_scope("A"):
        wait_all(sk_copy(0))
        conv_step(filt=0)
    with jax.named_scope("B_wait"):
        wait_all(sk_copy(1) + kv_groups[0])
    with jax.named_scope("B"):
        start_all(kv_groups[2] + kv_groups[3] + sk_copy(3) + sk_copy(4))
        conv_step(filt=1, units=units(PAIR, range(0, NB1)))
        scol_s[...] = jnp.broadcast_to(sc.astype(F32), (LANES, D)).T
    with jax.named_scope("C_wait"):
        wait_all(kv_groups[1])
    with jax.named_scope("C"):
        conv_step(units=units(PAIR, range(NB1, NBL)), lag=ULAG)
    with jax.named_scope("D_wait"):
        wait_all(sk_copy(2))
    with jax.named_scope("D"):
        start_all(wm_copies[0] + q_copies[0] + wm_copies[1] + w_copies[0])
        conv_step(filt=2, mul=0, free=MF[0], trim=MT[0])
    with jax.named_scope("E_wait"):
        wait_all(kv_groups[2])
    with jax.named_scope("E"):
        conv_step(units=units(TRIPLE, range(0, 2)), mul=1, inv=units((0,), range(NBL)), shift=ESH, free=MF[1], trim=MT[1])
    with jax.named_scope("F_wait"):
        wait_all(kv_groups[3])
    with jax.named_scope("F"):
        conv_step(units=units(TRIPLE, range(2, NBL)), lag=ULAG)

    def full_step(j, carry):
        wait_all(sk_copy(j + 2))
        conv_step(filt=j + 2, mul=j + 1, inv=units((j,), range(IG)), free=MF[2], trim=MT[2])
        return carry

    with jax.named_scope("GH"):
        lax.fori_loop(1, NC - 2, full_step, 0)
    late = units((NC - 2,), range(NBL)) + units(range(1, NC - 2), range(IG, NBL))
    late = late[:IJ] + units((NC - 1,), range(NBL)) + late[IJ:]
    with jax.named_scope("J"):
        start_all(q_copies[1] + w_copies[1] + sum(q_copies[2:], []) + w_copies[2] + w_copies[3] + wm_copies[2], 1)
        conv_step(mul=NC - 1, inv=late[:IJ], free=MF[3], trim=MT[3])
    with jax.named_scope("r6_wait"):
        wait_all(wm_copies[0] + q_copies[0])
    with jax.named_scope("r6"):
        for j in range(3):
            mod_chunk(j)
        conv_step(inv=late[IJ:IJ + 1])
        toks = conv_step(inv=late[IJ + 1:len(late) - IP])
        nx0 = stage_p1(0, A0[1], None, _pick(toks[:R6N], A0[1] // 8, R6F) if toks else None)
    with jax.named_scope("p2_wait"):
        wait_all(wm_copies[1])
    with jax.named_scope("p2"):
        mod_chunk(4)
        mod_chunk(3)
        toks = conv_step(inv=late[len(late) - IP:])
        if toks:
            nx0 = hold(nx0, _pick(toks[:P2N], A0[1] // 8, P2F))
        stage_p2(0, A0[1], nx0)
    with jax.named_scope("w1_wait"):
        wait_all(w_copies[0])
    with jax.named_scope("m1_0"):
        square_ops(w1_v, s1_s, stage_m1(0, 4)[:-40])
    with jax.named_scope("w2_wait"):
        wait_all(q_copies[1] + w_copies[1])
    with jax.named_scope("m2_0"):
        stage_p(1, stage_m2(0, SP0))
        filler(0)
    for t in range(1, NA):
        with jax.named_scope("a%d" % t):
            wait_all(q_copies[t + 1] if t + 1 < NA else w_copies[2] + w_copies[3] + wm_copies[2])
            toks = stage_m1(t, 2)
            toks = toks + stage_m2(t, 2, toks[len(toks) - len(toks) // 2:])
            if t + 1 < NA:
                stage_p(t + 1, toks)
            if t == 1:
                square_ops(w2_v, s2_s, toks[:-30])
            if t == NA - 1:
                transpose_w4(toks[:(len(toks) * XEND) // 100])
                store_z(0, 0, toks[(len(toks) * LW[0]) // 100:(len(toks) * LW[1]) // 100])
                toks = toks + [x for x in lead_in()[:40] for _ in range(WS[7])]
                cut = (len(toks) * CUT) // 100
                gate_row(toks[:(len(toks) * 9) // 10])
                w3_ops(toks[:cut])
                rest = [i for i in range(7) if i not in IN_LOOP]
                for k, i in enumerate(rest):
                    w4_ops(i, 0, toks[cut + k::len(rest)])
            filler(t)

    def out_copy(r0, n, c):
        rows = pl.ds(r0, n)
        return pltpu.make_async_copy(o_v.at[c, rows, :], o_hbm.at[rows, pl.ds(c * LANES, LANES)], sem_o.at[0])

    def raw4(n, d):
        return jnp.concatenate([wt_u[d, n], wt_u[NC - 1, n, d * (CQ // 2):(d + 1) * (CQ // 2), :]], axis=0)

    def mlp_tile(t, carry):
        r0 = pl.multiple_of(t * TB, TB)
        ws = t & 1
        count = [0]

        def fresh():
            count[0] += 1
            return lax.rem(t + 2 * count[0], 2)

        def g_rows(r2, p, lo, hi):
            base = (2 * r2 + p) * (FQ + GPAD)
            return slice(base + lo, base + hi)

        rem = {key: rh_s[k] for k, key in enumerate(BLOCKS[:4])}
        for key in BLOCKS[4:8]:
            rem[key] = rem3(*key)
        early = _rows8(rem[BLOCKS[4]], EW[0])
        rem[BLOCKS[8]] = rem3(*BLOCKS[8], pieces=4)
        todo = BLOCKS[9:]
        part = [None] * 7
        for i in (4, 3, 0, 6, 1, 2, 5):
            m = [None] * 7
            for j in _ORDER:
                slot = fresh()
                act = _operand(_LHS[j], lambda r2, k2: _operand(
                    _LHS[i], lambda r1, k1: zf_s[slot, z_rows(2 * r1 + r2, 2 * k1 + k2), :])).astype(BF16)
                if i in _RAW and j in _RAW:
                    d = 2 * _RAW.index(i) + _RAW.index(j)
                    wij = w3_u[d, d * (FQ // 2):(d + 1) * (FQ // 2), :]
                else:
                    wij = s3_u[i, j]
                m[j] = _dot_nt(_as_bf16(wij), act)
            key = todo.pop(0)
            rem[key] = rem3(*key)
            part[i] = _combine(m)
            if i in (4, 3, 0):
                early += _rows8(m[_ORDER[0]], EW[1]) + _rows8(m[_ORDER[4]], EW[2])
        zero = fresh() - ws
        fine = [x for x in early for _ in IN_LOOP]
        hop = len(fine) // (len(IN_LOOP) * 33)
        for k, i in enumerate(IN_LOOP):
            w4_ops(i, zero, fine[k * hop:len(fine) - (len(IN_LOOP) - k) * hop])
        for inner in range(4):
            r2, p = inner // 2, inner % 2
            for blk, pre in enumerate(_combine([part[i][inner] for i in range(7)])):
                g_s[blk][ws, g_rows(r2, p, 0, FQ), :] = _gelu2(pre + rem[2 * (blk // 2) + r2, 2 * (blk % 2) + p])

        toks = []
        marks = {}
        part = [[None] * 4 for _ in range(7)]
        for i in O4:
            slot = fresh()
            we = jnp.concatenate([raw4(4 * NS + _RAW.index(i), 2 * _RAW.index(i) + e) if i in _RAW else e4_u[i, e]
                                  for e in range(2)], axis=0)
            ex = []
            for r2 in range(2):
                act = [_operand(_LHS[i], lambda r1, h: g_s[2 * r1 + h][slot, g_rows(r2, p, NS * LANES, FQ), :])
                       for p in range(2)]
                act = jnp.concatenate(act + [jnp.zeros((LANES - 2 * LQ, TQ), F32)], axis=0).astype(BF16)
                ex.append(_dot(_as_bf16(we), act))
            m = [None] * 7
            for j in _ORDER:
                slot = fresh()
                act = _operand(_LHS[j], lambda r2, p: _operand(
                    _LHS[i], lambda r1, h: g_s[2 * r1 + h][slot, g_rows(r2, p, 0, NS * LANES), :])).astype(BF16)
                if i in _RAW and j in _RAW:
                    d = 2 * _RAW.index(i) + _RAW.index(j)
                    wij = [raw4(4 * st + d, d) for st in range(NS)]
                else:
                    wij = [s4_u[i, j, st] for st in range(NS)]
                m[j] = _dot(_as_bf16(jnp.concatenate(wij, axis=1)), act)
                toks += _rows8(m[j])
            part[i] = [x + ex[inner // 2][(inner % 2) * QR:(inner % 2 + 1) * QR]
                       for inner, x in enumerate(_combine(m))]
            marks[i] = len(toks)

        gb = 0.5 * mod_s[NC, 0:1, :]
        nxt = jnp.minimum(t + 1, NT - 1) * TB
        tails = {}
        for i, blk, norm in PLAN:
            r1 = blk // 2
            if norm is None:
                toks += [x for x in lead_in()[8:40] for _ in range(3)]
            elif norm[0] < norm[1]:
                store_z(nxt, 1 - ws, toks[norm[2]:norm[3]], norm[0], norm[1])
            pos = [marks[i] + FL[(1, 2, 0, 3).index(blk)]]

            def finish(rq, c, h2t):
                h2 = hold(h2t.T, toks[pos[0]:pos[0] + TQ // 8])
                pos[0] += TQ // 8
                rows = pl.ds(pl.multiple_of(r0 + rq * TQ, TQ), TQ)
                cols = slice(c * LANES, (c + 1) * LANES)
                o_v[c, rows, :] = (x_s[rows, cols] + gb[:, cols] * (h_s[rows, cols] + h2)).astype(BF16)
                if blk == 3:
                    out_copy(rows.start, TQ, c).start()

            for inner in (1, 2, 0, 3):
                ht = _block([part[k][inner] for k in range(7)], blk)
                rq, c = 2 * r1 + inner // 2, 2 * (blk % 2) + inner % 2
                finish(rq, c, ht[0:LANES])
                tails[rq, c] = ht[LANES:]
            rb = pl.multiple_of(r0 + r1 * 2 * TQ, 2 * TQ)
            if blk != 3:
                for e in range(2):
                    out_copy(rb, 2 * TQ, 2 * (blk % 2) + e).start()
            if blk in (0, 3):
                for rq in (2 * r1, 2 * r1 + 1):
                    finish(rq, NC - 1, jnp.concatenate([tails[rq, c] for c in range(NC - 1)], axis=0))
                if blk == 0:
                    out_copy(rb, 2 * TQ, NC - 1).start()
        return carry

    with jax.named_scope("ph2b"):
        lax.fori_loop(0, NT, mlp_tile, 0)
    with jax.named_scope("tail"):
        pltpu.make_async_copy(o_v, o_v, sem_o.at[0]).wait()


@jax.jit
def pallas_adaLN_cond__ssm_conv_h3__mixer_s_mlp__prompt_kernel(
    A_q: jax.Array,
    A_k: jax.Array,
    A_v: jax.Array,
    A_shift_k: jax.Array,
    A_ssm_k: jax.Array,
    A_ssm_D: jax.Array,
    B_x: jax.Array,
    B_w1: jax.Array,
    B_w2: jax.Array,
    B_w3: jax.Array,
    B_w4: jax.Array,
    c: jax.Array,
    w_mod: jax.Array,
):
    B, S, D = A_q.shape
    FF = B_w3.shape[1]
    assert (B, S, D, FF, A_shift_k.shape[1]) == (1, sum(TILES), 5 * LANES, 1728, 4)
    NC = D // LANES
    NG = BLK // 8
    NBL = S // (PH * BLK)
    NS = FF // 4 // LANES
    n1 = S - sum(TILES[:BLOCKWISE1[0]]) - HALO
    n2 = S - sum(TILES[:BLOCKWISE2[0]])

    args = (A_q.reshape(S, D), A_k.reshape(S, D), A_v.reshape(S, D), A_shift_k.T, A_ssm_k,
            A_ssm_D, B_w1, B_w2, B_w3.T, B_w4, c, w_mod)
    scratch = [
        pltpu.VMEM((S, D), BF16),
        pltpu.VMEM((NC, S + 16, LANES), BF16),
        pltpu.VMEM((NC, S, LANES), BF16),
        pltpu.VMEM((4, D), BF16),
        pltpu.VMEM((NC, LANES, S), BF16),
        pltpu.VMEM((D,), BF16),
        pltpu.VMEM((NC, D, LANES), BF16),
        pltpu.VMEM((NC, D, LANES), BF16),
        pltpu.VMEM((NC, FF, LANES), BF16),
        pltpu.VMEM((NC, FF, LANES), BF16),
        pltpu.VMEM((1, D), BF16),
        pltpu.VMEM((D, 6 * D), BF16),
        pltpu.VMEM((PH, 2 * BLK, BLK), BF16),
        pltpu.VMEM((PH, 2, BLK, BLK), BF16),
        pltpu.VMEM((NC, S, LANES), BF16),
        pltpu.VMEM((NC, NG, NBL, PH, 2, 8, LANES), F32),
        pltpu.VMEM((NC, NG, NBL, PH, 2, 8, LANES), F32),
        pltpu.VMEM((NC, NBL, PH, 2 * BLK, LANES), BF16),
        pltpu.VMEM((6, PH, BLK, LANES), BF16),
        pltpu.VMEM((NC, S, LANES), F32),
        pltpu.VMEM((6, 8, D), F32),
        pltpu.VMEM((NC, 8, LANES), F32),
        pltpu.VMEM((NC, S + 16, LANES), F32),
        pltpu.VMEM((S, D), F32),
        pltpu.VMEM((S, D), F32),
        pltpu.VMEM((NC, S, LANES), BF16),
        pltpu.VMEM((7, 7, FF // 4, LANES), BF16),
        pltpu.VMEM((7, 7, NS, D // 4, LANES), BF16),
        pltpu.VMEM((7, 2, D // 4, LANES), BF16),
        [pltpu.VMEM((2, GROWS, TQ), F32)] * 4,
        pltpu.VMEM((2, 4 * NC * (TQ + 8), LANES), F32),
        pltpu.VMEM((TB, LANES), BF16),
        pltpu.VMEM((10, 2, n1 // 2, LANES), BF16),
        pltpu.VMEM((10, 2, n2 // 2, LANES), BF16),
        pltpu.VMEM((7, 2, 2 * LANES, LANES), BF16),
        pltpu.VMEM((7, 2, 2 * LANES, LANES), BF16),
        pltpu.VMEM((4, FF // 4, TQ), F32),
        pltpu.VMEM((NC, 4 * NS + 2, LANES, LANES), BF16),
        pltpu.VMEM((D, LANES), F32),
        pltpu.SemaphoreType.DMA((21,)),
        pltpu.SemaphoreType.DMA((1,)),
    ]
    out = pl.pallas_call(
        functools.partial(_kernel, S=S, D=D, FF=FF),
        in_specs=[pl.BlockSpec(memory_space=pl.ANY)] * len(args),
        out_specs=pl.BlockSpec(memory_space=pl.ANY),
        out_shape=jax.ShapeDtypeStruct((S, D), BF16),
        scratch_shapes=scratch,
        compiler_params=pltpu.CompilerParams(
            vmem_limit_bytes=120 * 1024 * 1024,
            disable_bounds_checks=True,
            disable_semaphore_checks=True,
        ),
    )(*args)
    return out.reshape(B, S, D)
```

```python
import functools
import math

import jax
import jax.numpy as jnp
from jax import lax
import jax.experimental.pallas as pl
import jax.experimental.pallas.tpu as pltpu

F32 = jnp.float32
BF16 = jnp.bfloat16
U32 = jnp.uint32

LANES = 128
BLK = 128
PH = 4
EPS = 1e-05
TB = 512
TQ = TB // 4
HALO = 32
TILES = (384, 384, 576, 704)
BLOCKWISE1 = (3,)
BLOCKWISE2 = (2, 3)
IN_LOOP = (2, 4, 1, 3, 0)
ROT = 3
KR = 256
NB1 = 1
IG = 2
IJ = 6
IP = 2
GPAD = 8
GROWS = 1768

MF = (6, 0, 5, 4)
MT = (3, 0, 3, 3)
R6 = (36, 18, 28, 6)
TRS = (145, 175, 180)
FRS = (50, 90, 90)
WS = (2, 3, 3, 2, 2, 4)
FI = (48, 88, 96, 96)
LAST = (55, 66, 92, 82)
EW = (2, 1, 2)
NW = (1, 3, 0, 150, 320, 460, 600, 730)
FL = (10, 10, 25, -32)

_ORDER = (2, 4, 1, 3, 0, 6, 5)
_RAW = (1, 4)
_LHS = (((0, 0), 1, (1, 1)), ((1, 0), 1, (1, 1)), ((0, 0),), ((1, 1),),
        ((0, 0), 1, (0, 1)), ((1, 0), -1, (0, 0)), ((0, 1), -1, (1, 1)))
_RHS = (((0, 0), 1, (1, 1)), ((0, 0),), ((0, 1), -1, (1, 1)), ((1, 0), -1, (0, 0)),
        ((1, 1),), ((0, 0), 1, (0, 1)), ((1, 0), 1, (1, 1)))


def _operand(terms, blk):
    x = blk(*terms[0])
    if len(terms) > 1:
        y = blk(*terms[2])
        x = x + y if terms[1] > 0 else x - y
    return x


def _all_operands(table, b00, b01, b10, b11):
    blocks = ((b00, b01), (b10, b11))
    return [_operand(terms, lambda i, j: blocks[i][j]) for terms in table]


def _block(m, which):
    if which == 0:
        return (m[3] - m[4]) + m[0] + m[6]
    if which == 1:
        return m[2] + m[4]
    if which == 2:
        return m[1] + m[3]
    return (m[2] - m[1]) + m[0] + m[5]


def _combine(m):
    return [_block(m, which) for which in range(4)]


def _as_bf16(x):
    return pltpu.bitcast(x, BF16)


def _lo(x):
    return pltpu.bitcast(x << 16, F32)


def _hi(x):
    return pltpu.bitcast(x & jnp.uint32(0xFFFF0000), F32)


def _dft4(re, im, sign):
    ar, ai = re[0] + re[2], im[0] + im[2]
    br, bi = re[0] - re[2], im[0] - im[2]
    cr, ci = re[1] + re[3], im[1] + im[3]
    dr, di = re[1] - re[3], im[1] - im[3]
    o0 = (ar + cr, ai + ci)
    o2 = (ar - cr, ai - ci)
    m = (br + di, bi - dr)
    p = (br - di, bi + dr)
    o1, o3 = (m, p) if sign < 0 else (p, m)
    return [o0[0], o1[0], o2[0], o3[0]], [o0[1], o1[1], o2[1], o3[1]]


def _ln(x, eps=EPS, unit=True):
    n = x.shape[-1]
    s1 = jnp.sum(x, axis=-1, keepdims=True)
    m = s1 * (1.0 / n)
    v = jnp.maximum(jnp.sum(x * x, axis=-1, keepdims=True) + (n * eps - s1 * m), n * eps)
    e = jnp.log(v) * (-0.5 / math.log(2.0))
    return (x - m) * jnp.exp2(e + 0.5 * math.log2(n) if unit else e)


def _gelu2(x):
    c0 = math.sqrt(2.0 / math.pi)
    return x + x * jnp.tanh(x * (c0 + (c0 * 0.044715) * (x * x)))


def _dot(a, b):
    return jnp.dot(a, b, preferred_element_type=F32)


def _dot_nt(a, b):
    return lax.dot_general(a, b, (((1,), (1,)), ((), ())), preferred_element_type=F32)


def _rows8(x, repeat=1):
    return [x[8 * r:8 * r + 8, 0:LANES] for r in range(x.shape[0] // 8) for _ in range(repeat)]


def _chunks(r0, r1, k, unit=16):
    n = (r1 - r0) // unit
    cuts = [r0 + unit * ((n * j) // k) for j in range(k + 1)]
    return list(zip(cuts[:-1], cuts[1:]))


def _pick(toks, n, free=0):
    idx = [(r * (len(toks) + free)) // n - free for r in range(n)]
    return [toks[i] if i >= 0 else None for i in idx]


def _kernel(q_hbm, k_hbm, v_hbm, sh_hbm, sk_hbm, sd_hbm, w1_hbm, w2_hbm, w3_hbm, w4_hbm, c_hbm, wm_hbm,
            o_hbm,
            q_v, k_v, v_v, sh_v, sk_v, sd_v, w1_v, w2_v, w3_v, w4_v, c_v, wm_v,
            fw_s, iv_s, o_v, u_s, kk_s, vv_s, wu_s, y_s, mod_s, par_s, h1_s, x_s, h_s, z_s,
            s3_s, s4_s, e4_s, g_s, zf_s, zr_s, l1_s, l2_s, s1_s, s2_s, rh_s, wt_s, scol_s,
            sem, sem_o,
            *, S, D, FF):
    NC = D // LANES
    NG = BLK // 8
    LB = PH * BLK
    NBL = S // LB
    R = BLK // PH
    HL = LANES // 2

    small = [
        pltpu.make_async_copy(sh_hbm, sh_v, sem.at[0]),
        pltpu.make_async_copy(sd_hbm, sd_v, sem.at[0]),
        pltpu.make_async_copy(c_hbm, c_v, sem.at[0]),
    ]

    def sk_copy(c):
        ch = (c + ROT) % NC * LANES
        rows = pl.ds(ch if isinstance(c, int) else pl.multiple_of(ch, LANES), LANES)
        return [pltpu.make_async_copy(sk_hbm.at[rows, :], sk_v.at[c], sem.at[1 + c])]

    def kv_copies(tiles, blocks, s):
        return [pltpu.make_async_copy(src.at[pl.ds(r, KR), pl.ds((c + ROT) % NC * LANES, LANES)],
                                      dst.at[c, pl.ds(off + r, KR), :], sem.at[s])
                for r in range(blocks[0] * LB, (blocks[-1] + 1) * LB, KR)
                for src, dst, off in ((k_hbm, k_v, 16), (v_hbm, v_v, 0)) for c in tiles]

    PAIR, TRIPLE = (0, 1), (2, 3, 4)
    kv_groups = [kv_copies(PAIR, range(0, NB1), 9), kv_copies(PAIR, range(NB1, NBL), 10),
                 kv_copies(TRIPLE, range(0, 2), 11), kv_copies(TRIPLE, range(2, NBL), 20)]

    WM = (0, 3 * D, 5 * D, 6 * D)
    wm_copies = [[pltpu.make_async_copy(wm_hbm.at[:, pl.ds(WM[j], WM[j + 1] - WM[j])],
                                        wm_v.at[:, pl.ds(WM[j], WM[j + 1] - WM[j])], sem.at[6 + j])]
                 for j in range(3)]
    w_copies = [[pltpu.make_async_copy(src.at[:, pl.ds(c * LANES, LANES)], dst.at[c], sem.at[12 + j])
                 for c in range(NC)]
                for j, (src, dst) in enumerate(((w1_hbm, w1_v), (w2_hbm, w2_v), (w3_hbm, w3_v), (w4_hbm, w4_v)))]

    B0 = [0]
    for n in TILES:
        B0.append(B0[-1] + n)
    NA = len(TILES)
    A0 = [0] + [r + HALO for r in B0[1:-1]] + [S]
    q_copies = [
        [pltpu.make_async_copy(q_hbm.at[pl.ds(A0[t], A0[t + 1] - A0[t])], q_v.at[pl.ds(A0[t], A0[t + 1] - A0[t])],
                               sem.at[16 + t])]
        for t in range(NA)
    ]

    def start_all(cps, priority=0):
        for cp in cps:
            cp.start(priority=priority)

    def wait_all(cps):
        for cp in cps:
            cp.wait()

    for c in range(NC):
        k_v[c, 0:16, :] = jnp.zeros((16, LANES), BF16)
    start_all(sk_copy(0) + small + sk_copy(1) + kv_groups[0] + kv_groups[1] + sk_copy(2))

    for c in range(NC):
        h1_s[c, 0:8, :] = jnp.zeros((8, LANES), F32)
        h1_s[c, S + 8:S + 16, :] = jnp.zeros((8, LANES), F32)

    prow = lax.broadcasted_iota(jnp.int32, (BLK, BLK), 0)
    pcol = lax.broadcasted_iota(jnp.int32, (BLK, BLK), 1)
    ang = (((4 * prow + 1) * pcol) & (4 * BLK - 1)).astype(F32) * (2.0 * math.pi / (4 * BLK))
    tw = (4 * prow + 1).astype(F32) * (2.0 * math.pi / (4 * LB))
    mr, mi = jnp.cos(ang), -jnp.sin(ang)
    twr, twi = jnp.cos(tw), -jnp.sin(tw)
    eye = jnp.where(prow == pcol, 1.0 / LB, 0.0).astype(BF16)
    for i in range(PH):
        both = jnp.stack([mr.reshape(NG, 8, BLK), mi.reshape(NG, 8, BLK)], axis=1).reshape(2 * BLK, BLK)
        fw_s[i] = both.astype(BF16)
        for h in range(2):
            iv_s[i, h] = _dot_nt(eye, both[h * BLK:(h + 1) * BLK, :].astype(BF16)).astype(BF16)
        if i + 1 < PH:
            mr, mi = mr * twr - mi * twi, mr * twi + mi * twr
    perm = jnp.where(pcol == (prow % R) * PH + prow // R, 1.0, 0.0).astype(BF16)

    wait_all(small)
    shf = sh_v[...].astype(F32)
    sdf = sd_v[...].astype(F32).reshape(1, D)
    for c in range(NC):
        par_s[(c - ROT) % NC, 0:4, :] = shf[:, c * LANES:(c + 1) * LANES]
        par_s[(c - ROT) % NC, 4:5, :] = sdf[:, c * LANES:(c + 1) * LANES]
    cf = c_v[...].astype(F32)
    sc = (cf * jax.nn.sigmoid(cf)).astype(BF16)
    sc16 = jnp.broadcast_to(sc, (16, D))

    def mod_chunk(j):
        mod_s[j] = _dot(sc16, wm_v[:, j * D:(j + 1) * D])[0:8, :]

    (fw_u, iv_u, k_u, v_u, wu_u, vv_u, z_u, l1_u, l2_u, w1_u, w2_u, s1_u, s2_u, w3_u, w4_u, wt_u, s3_u, s4_u,
     e4_u, zr_u) = (r.bitcast(U32) for r in (fw_s, iv_s, k_v, v_v, wu_s, vv_s, z_s, l1_s, l2_s, w1_v, w2_v,
                                             s1_s, s2_s, w3_v, w4_v, wt_s, s3_s, s4_s, e4_s, zr_s))

    never = twr[0:8, :] > 2.0

    def after(token, x):
        if token.dtype != x.dtype:
            token = pltpu.bitcast(token, x.dtype)
        return jnp.where(jnp.broadcast_to(never, x.shape), token, x)

    def hold(x, tks):
        f = len([k for k in tks if k is None])
        n = len(tks)
        head = after(jnp.stack(tks[f:]), x[8 * f:, 0:LANES].reshape(n - f, 8, LANES)).reshape(8 * (n - f), LANES)
        if f:
            head = jnp.concatenate([x[:8 * f, 0:LANES], head], axis=0)
        return head if x.shape[1] == LANES else jnp.concatenate([head, x[:, LANES:]], axis=1)

    def hold16(x, tks):
        x4 = x.reshape(len(tks), 2, 8, LANES)
        return jnp.stack([after(jnp.stack(tks), x4[:, 0]), x4[:, 1]], axis=1).reshape(x.shape)

    def perm_k(c, b, toks):
        kt = [_dot_nt(perm, sk_v[c, :, b * LB + t * BLK:b * LB + (t + 1) * BLK]) for t in range(PH)]
        toks += _rows8(kt[0])[::2]
        return [jnp.concatenate([kt[t][i * R:(i + 1) * R, :] for t in range(PH)], axis=0).astype(BF16)
                for i in range(PH)]

    def spectrum(comps, dst, slot, b, toks, dc=None, pins=None):
        tr, ti = [], []
        for i in range(PH):
            lhs = fw_u[i]
            if pins is not None and i < len(pins):
                lhs = after(pins[i], lhs.reshape(NG, 8, LANES)).reshape(BLK, LANES)
            t4 = _dot(_as_bf16(lhs), comps[i]).reshape(NG, 2, 8, LANES)
            tr.append(t4[:, 0])
            ti.append(t4[:, 1])
        toks += [ti[PH - 1][g] for g in range(NG)]
        if dc is not None:
            tr[0] = tr[0] + dc
        sr, si = _dft4(tr, ti, -1)
        for qq in range(PH):
            dst[slot, :, b, qq, 0] = sr[qq]
            dst[slot, :, b, qq, 1] = si[qq]

    def gated(c, b, n):
        w = [par_s[c, t:t + 1, :] for t in range(4)]
        kc = {}
        for o in range(-2, 2):
            words = k_u[c, pl.ds(8 + b * (LB // 2) + o, BLK, stride=2), :]
            if o > -2:
                kc[2 * o] = _lo(words)
            kc[2 * o + 1] = _hi(words)
        vc = {}
        for o in range(2):
            words = v_u[c, pl.ds(b * (LB // 2) + o, BLK, stride=2), :]
            vc[2 * o] = _lo(words)
            vc[2 * o + 1] = _hi(words)
        for i in range(PH):
            ks = kc[i] * w[0]
            for t in range(1, 4):
                ks = ks + kc[i - t] * w[t]
            wu_s[n, i] = (ks * vc[i]).astype(BF16)
        return [wu_u[n, i] for i in range(PH)]

    def kv_pins(kvb):
        return [jnp.stack([kvb[2 * m + (r % 2)][8 * (r // 2):8 * (r // 2) + 8, :] for r in range(NG)])
                for m in range(2)]

    def products(c, ks, kc, toks, free, trim):
        n = len(toks) - trim + free
        cum = (44, 128, 244, 392)
        zp = None
        for o in range(NBL):
            idx = [((g * cum[-1] + cum[o]) * n) // (cum[-1] * NG) - 1 - free for g in range(NG)]
            tk = [toks[max(i, 0)] if i >= 0 or not free else None for i in idx]
            zr, zi = [], []
            for qq in range(PH):
                accr = acci = None
                for b in range(o + 1):
                    a_, b_ = u_s[c, :, b, qq, 0], u_s[c, :, b, qq, 1]
                    c_, d_ = ks[kc, :, o - b, qq, 0], ks[kc, :, o - b, qq, 1]
                    if qq == 0 and b == o:
                        a_ = hold(a_.reshape(BLK, LANES), tk).reshape(NG, 8, LANES)
                    tr_ = a_ * c_ - b_ * d_
                    ti_ = a_ * d_ + b_ * c_
                    accr = tr_ if accr is None else accr + tr_
                    acci = ti_ if acci is None else acci + ti_
                zr.append(accr)
                zi.append(acci)
            if zp is None:
                yr, yi = zr, zi
            else:
                yr = [zr[qq] - zp[1][qq] for qq in range(PH)]
                yi = [zi[qq] + zp[0][qq] for qq in range(PH)]
            zp = (zr, zi)
            vr, vi = _dft4(yr, yi, +1)
            for i in range(PH):
                vv_s[c, o, i] = jnp.stack([vr[i], vi[i]], axis=1).reshape(2 * BLK, LANES).astype(BF16)

    def inverse(c, o, toks, pins):
        for i in range(PH):
            yv = None
            for h in range(2):
                lhs = iv_u[i, h]
                if pins is not None and h == 0:
                    pin = pins[i % 2][8 * (i // 2):8 * (i // 2) + 8]
                    lhs = after(pin, lhs.reshape(8, 8, LANES)).reshape(HL, LANES)
                t = _dot(_as_bf16(lhs), _as_bf16(vv_u[c, o, i, h * HL:(h + 1) * HL, :]))
                yv = t if yv is None else yv + t
            if i % 2 == 0:
                toks += _rows8(yv)[::2]
            y_s[c, pl.ds(o * LB + i, BLK, stride=PH), :] = yv

    def conv_step(filt=None, units=(), mul=None, inv=(), free=0, trim=3):
        toks = []
        kv = [gated(c, b, n) for n, (c, b) in enumerate(units)]
        pin_at = {n: kv_pins(kv[n]) for n in range(len(units))} if inv or filt is not None else {}
        if filt is not None and mul is not None and not isinstance(filt, int):
            ks = kk_s.at[pl.ds(mul, 2)]
            k_rd, k_wr = (ks, 0), (ks, 1)
        else:
            k_rd, k_wr = (kk_s, mul), (kk_s, filt)
        pos = 0
        for c, o in inv:
            inverse(c, o, toks, pin_at.get(pos))
            pos += 1
        if filt is not None:
            comps = [perm_k(filt, b, toks) for b in range(NBL)]
            for b in range(NBL):
                spectrum(comps[b], *k_wr, b, toks, par_s[filt, 4:5, :] if b == 0 else None, pin_at.get(pos))
                pos += 1
        for n, (c, b) in enumerate(units):
            spectrum([_as_bf16(x) for x in kv[n]], u_s, c, b, toks, None, pin_at.get(pos))
            pos += 1
        if mul is not None:
            products(mul, *k_rd, toks, free, trim)
        return toks

    def lane_tiles(x):
        return [x[:, c * LANES:(c + 1) * LANES] for c in range(NC)]

    def stage_p1(r0, r1, tks=None, ytks=None):
        ga = mod_s[2, 0:1, :]
        a_mul, a_add = ga * (1.0 + mod_s[1, 0:1, :]) * math.sqrt(D), ga * mod_s[0, 0:1, :]
        q = q_v[r0:r1, :].astype(F32)
        if tks is not None:
            q = hold(q, tks)
        y = jnp.concatenate([y_s[(c - ROT) % NC, r0:r1, :] for c in range(NC)], axis=1)
        if ytks is not None:
            y = hold(y, ytks)
        x = q + (_ln(q, unit=False) * a_mul + a_add) * y
        x_s[r0:r1, :] = x
        return _ln(x, unit=False)

    def store_row_ops(dst, base, r0, r1, cols, tks=None):
        hv = []
        for x in cols:
            x4 = x.reshape(x.shape[0] // 32, 2, 16, LANES)
            hv.append([x4[:, e].reshape(x.shape[0] // 2, LANES) for e in range(2)])
        for k2 in range(2):
            a00, a01, a10, a11 = hv[k2][0], hv[2 + k2][0], hv[k2][1], hv[2 + k2][1]
            if tks is not None:
                a00, a11 = hold16(a00, tks), hold16(a11, tks)
            for o, x in enumerate(_all_operands(_LHS, a00, a01, a10, a11) + [a01, a10, hv[NC - 1][k2]]):
                dst[o, k2, (r0 - base) // 2:(r1 - base) // 2, :] = x.astype(BF16)

    L1B = A0[BLOCKWISE1[0]]
    L2B = B0[BLOCKWISE2[0]]

    def stage_p2(r0, r1, nx, blockwise=False):
        h = nx * ((1.0 + mod_s[4, 0:1, :]) * (2.0 * math.sqrt(D))) + 2.0 * mod_s[3, 0:1, :]
        h_s[r0:r1, :] = h
        zn = lane_tiles(_ln(h, 4.0 * EPS))
        if blockwise:
            store_row_ops(l1_s, L1B, r0, r1, zn)
        else:
            for c in range(NC):
                z_s[c, r0:r1, :] = zn[c].astype(BF16)

    def stage_p(t, toks):
        lo, hi = A0[t], A0[t + 1]
        stage_p2(lo, hi, stage_p1(lo, hi, _pick(toks[:-TRS[t - 1]], (hi - lo) // 8, FRS[t - 1])), t in BLOCKWISE1)

    def filler(t):
        red = jnp.sum(y_s[t, 0:8 * FI[t], :], axis=-1, keepdims=True).reshape(FI[t], 8, 1)
        spare = (NC - 1) * (TQ + 8) + 8 * t
        zf_s[1, spare:spare + 8, :] = jnp.broadcast_to(jnp.sum(red, axis=0), (8, LANES))

    def square_ops(src, dst, toks):
        HK = 2 * LANES
        tks = _pick(toks, 2 * HK // 16)
        for n2 in range(2):
            tk = tks[n2 * (HK // 16):(n2 + 1) * (HK // 16)]
            blk = lambda k, n: src[2 * n + n2, k * HK:(k + 1) * HK, :].astype(F32)
            for o, x in enumerate(_all_operands(_RHS, hold16(blk(0, 0), tk), blk(0, 1), blk(1, 0), hold16(blk(1, 1), tk))):
                if o not in _RAW:
                    dst[o, n2] = x.astype(BF16)

    def block_dots(ops_u, base, prepare, w_u, s_u, parts, emit, light, heavy):
        toks = []

        def timed(x, weight):
            toks.extend(_rows8(x, weight))
            return x

        def weave(top, bot):
            n = top.shape[0] // 16
            return jnp.stack([top.reshape(n, 16, LANES), bot.reshape(n, 16, LANES)], axis=1).reshape(32 * n, LANES)

        def main(get):
            m = [None] * 7
            rem = [None, None]
            for o in ('t', 2, 4, 'b', 1, 3, 0, 6, 5):
                if o in ('t', 'b'):
                    e = 0 if o == 't' else 1
                    rhs = jnp.concatenate([w_u[c, 2 * LANES:D // 2, :] for c in range(NC - 1)], axis=1)
                    rem[e] = timed(_dot(get([(9, e)]), _as_bf16(rhs)), light)
                    continue
                if o in _RAW:
                    d = _RAW.index(o)
                    rhs = jnp.concatenate([w_u[2 * d + n2, d * LANES:(d + 1) * LANES, :] for n2 in range(2)], axis=1)
                else:
                    rhs = jnp.concatenate([s_u[o, n2] for n2 in range(2)], axis=1)
                m[o] = timed(_dot(get([(o, 0), (o, 1)]), _as_bf16(rhs)), heavy if o in (4, 3, 6, 5) else light)
            c00, c01, c10, c11 = _combine(m)
            top = jnp.concatenate([c00, c01], axis=1) + rem[0]
            bot = jnp.concatenate([c10, c11], axis=1) + rem[1]
            return [weave(top[:, c * LANES:(c + 1) * LANES], bot[:, c * LANES:(c + 1) * LANES]) for c in range(NC - 1)]

        def last(get):
            w = _as_bf16(w_u[NC - 1])
            return weave(timed(_dot(get([(2, 0), (2, 1), (7, 0), (7, 1), (9, 0)]), w), light),
                         timed(_dot(get([(8, 0), (8, 1), (3, 0), (3, 1), (9, 1)]), w), light))

        mark = None
        for j, (r0, r1) in enumerate(parts):
            prepare(r0, r1, None if mark is None else toks[mark:])
            mark = len(toks)
            get = lambda keys: _as_bf16(jnp.concatenate(
                [ops_u[o, e, (r0 - base) // 4:(r1 - base) // 4, :] for o, e in keys], axis=1))
            if j % 2:
                tail = last(get)
                emit(r0, r1, main(get) + [tail])
            else:
                emit(r0, r1, main(get) + [last(get)])
        return toks

    def stage_m1(t, k):
        def emit(r0, r1, cols):
            out = [_gelu2(x) for x in cols]
            for c in range(NC):
                h1_s[c, r0 + 8:r1 + 8, :] = out[c]
            return out

        if t in BLOCKWISE1:
            return block_dots(l1_u, L1B, lambda *_: None, w1_u, s1_u, _chunks(A0[t], A0[t + 1], k, 32), emit, WS[2], WS[3])
        toks = []
        for r0, r1 in _chunks(A0[t], A0[t + 1], k):
            lhs = jnp.concatenate([z_u[c, r0 // 2:r1 // 2, :] for c in range(NC)], axis=1)
            w = jnp.concatenate([w1_u[c] for c in range(NC)], axis=1)
            for x in emit(r0, r1, lane_tiles(_dot(_as_bf16(lhs), _as_bf16(w)))):
                toks += _rows8(x, WS[0])
        return toks

    def shifted(r0, r1):
        n, grp, shifts = r1 - r0, D // 4, (-1, 1, -2, 2)
        lane = lax.broadcasted_iota(jnp.int32, (n, LANES), 1)
        cols = []
        for c in range(NC):
            lo, hi = c * LANES, (c + 1) * LANES
            g_lo, g_hi = lo // grp, (hi - 1) // grp
            val = h1_s[c, pl.ds(r0 + 8 + shifts[g_lo], n), :]
            if g_hi != g_lo:
                other = h1_s[c, pl.ds(r0 + 8 + shifts[g_hi], n), :]
                val = jnp.where(lane < (g_hi * grp - lo), val, other)
            cols.append(val)
        return cols

    def stage_m2(t, k, before=None):
        def emit(r0, r1, cols):
            x1 = h_s[r0:r1, :] + jnp.concatenate(cols, axis=1)
            h_s[r0:r1, :] = x1
            return x1

        if t in BLOCKWISE2:
            def prepare(r0, r1, prev):
                prev = before if prev is None else prev
                prev = prev[len(prev) // 8:(len(prev) * 7) // 8]
                store_row_ops(l2_s, L2B, r0, r1, shifted(r0, r1), _pick(prev, (r1 - r0) // 32))
            return block_dots(l2_u, L2B, prepare, w2_u, s2_u, _chunks(B0[t], B0[t + 1], k, 32), emit, WS[4], WS[4])
        toks = []
        for r0, r1 in _chunks(B0[t], B0[t + 1], k):
            w = jnp.concatenate([w2_u[c] for c in range(NC)], axis=1)
            hs = _dot(jnp.concatenate(shifted(r0, r1), axis=1).astype(BF16), _as_bf16(w))
            for x in lane_tiles(emit(r0, r1, [hs])):
                toks += _rows8(x, WS[1])
        return toks

    NT = S // TB
    FQ = FF // 4
    NS = FQ // LANES
    LQ = FQ - NS * LANES
    CQ = LANES // 4
    QR = LANES + CQ
    BLOCKS = [(2 * r1 + r2, 2 * h + p)
              for r1, h in ((0, 0), (1, 0), (0, 1), (1, 1)) for r2 in range(2) for p in range(2)]

    def z_rows(rq, c):
        lo = (NC * rq + c) * (TQ + 8)
        return slice(lo, lo + TQ)

    def store_z(r0, slot, toks, q0=0, q1=4):
        n = (q1 - q0) * TQ
        rows = pl.ds(r0 + q0 * TQ if isinstance(r0, int) else pl.multiple_of(r0 + q0 * TQ, TQ), n)
        zn = lane_tiles(_ln(hold(h_s[rows, :], _pick(toks, n // 8)), 4.0 * EPS))
        for rq in range(q0, q1):
            for c in range(NC - 1):
                zf_s[slot, z_rows(rq, c), :] = zn[c][(rq - q0) * TQ:(rq - q0 + 1) * TQ]
        zr_s[q0 * TQ:q1 * TQ, :] = zn[NC - 1].astype(BF16)

    def w3_ops(toks):
        ng = FQ // 16
        blk = lambda c, d: w3_v[c, d * FQ:(d + 1) * FQ, :].astype(F32)
        outer = [[_all_operands(_RHS, blk(k2, p), blk(k2, 2 + p), blk(2 + k2, p), blk(2 + k2, 2 + p))
                  for p in range(2)] for k2 in range(2)]
        for k, i in enumerate((1, 5, 2, 4, 0, 3, 6)):
            tk = [toks[((k + r * 7) * len(toks)) // (7 * ng)] for r in range(ng)]
            for j, x in enumerate(_all_operands(_RHS, hold16(outer[0][0][i], tk), outer[0][1][i], outer[1][0][i],
                                                hold16(outer[1][1][i], tk))):
                if i not in _RAW or j not in _RAW:
                    s3_s[i, j] = x.astype(BF16)

    def transpose_w4(toks):
        order = [(c, n) for n in (4 * NS, 4 * NS + 1) + tuple(range(4 * NS)) for c in range(NC)]
        for k, (c, n) in enumerate(order):
            if n >= 4 * NS:
                ends = [(2 * (n - 4 * NS) + p + 1) * FQ // 2 for p in range(2)]
                x = jnp.concatenate([w4_u[c, e - LQ // 2:e, :] for e in ends]
                                    + [jnp.zeros((HL - LQ, LANES), U32)], axis=0)
            else:
                lo = (n % 4) * FQ // 2 + (n // 4) * HL
                x = w4_u[c, lo:lo + HL, :]
            x = jnp.concatenate([after(toks[(k * len(toks)) // len(order)], x[0:8]), x[8:]], axis=0)
            wt_s[c, n] = _as_bf16(x).astype(F32).T.astype(BF16)

    def w4_ops(i, zero, toks):
        ng = QR // 16
        total = (NS * 7 + 2) * ng
        tk = lambda pos, step: [toks[((pos + r * step) * len(toks)) // total] for r in range(ng)]
        quarter = lambda n, d: jnp.concatenate(
            [wt_s[d, n].astype(F32), wt_s[NC - 1, n, d * CQ:(d + 1) * CQ, :].astype(F32)], axis=0)
        if i not in _RAW:
            for e in range(2):
                x = _operand(_RHS[i], lambda h, d: quarter(4 * NS + h, 2 * d + e))
                e4_s[i + zero, e] = hold16(x, tk(e * ng, 1)).astype(BF16)
        for st in range(NS):
            t = [[_operand(_RHS[i], lambda h, d: quarter(4 * st + 2 * h + p, 2 * d + e)) for e in range(2)]
                 for p in range(2)]
            tks = tk((2 + st * 7) * ng, 7)
            for j, x in enumerate(_all_operands(_RHS, hold16(t[0][0], tks), t[0][1], t[1][0], hold16(t[1][1], tks))):
                if i not in _RAW or j not in _RAW:
                    s4_s[i + zero, j, st] = x.astype(BF16)

    def gate_row(toks):
        ng = D // 8
        col = after(jnp.stack(_pick(toks, ng)), scol_s[...].reshape(ng, 8, LANES))
        for c in range(NC):
            wf = wm_v[:, (NC * NC + c) * LANES:(NC * NC + c + 1) * LANES].astype(F32).reshape(ng, 8, LANES)
            acc = col[0] * wf[0]
            for r in range(1, ng):
                acc = acc + col[r] * wf[r]
            mod_s[NC, :, c * LANES:(c + 1) * LANES] = jnp.broadcast_to(jnp.sum(acc, axis=0, keepdims=True), (8, LANES))

    def rem3(rq, d, pieces=1):
        z = _as_bf16(zr_u[rq * (TQ // 2):(rq + 1) * (TQ // 2), :])
        return jnp.concatenate([_dot_nt(_as_bf16(w3_u[NC - 1, lo // 2:hi // 2, :]), z)
                                for lo, hi in _chunks(d * FQ, (d + 1) * FQ, pieces)], axis=0)

    def lead_in():
        head = [rem3(*key) for key in BLOCKS[:4]]
        for k in range(4):
            rh_s[k] = head[k]
        return _rows8(head[0])

    def units(tiles, blocks):
        return [(c, b) for b in blocks for c in tiles]

    with jax.named_scope("A"):
        wait_all(sk_copy(0))
        conv_step(filt=0)
    with jax.named_scope("B_wait"):
        wait_all(sk_copy(1) + kv_groups[0])
    with jax.named_scope("B"):
        start_all(kv_groups[2] + kv_groups[3] + sk_copy(3) + sk_copy(4))
        conv_step(filt=1, units=units(PAIR, range(0, NB1)))
        scol_s[...] = jnp.broadcast_to(sc.astype(F32), (LANES, D)).T
    with jax.named_scope("C_wait"):
        wait_all(kv_groups[1])
    with jax.named_scope("C"):
        conv_step(units=units(PAIR, range(NB1, NBL)))
    with jax.named_scope("D_wait"):
        wait_all(sk_copy(2))
    with jax.named_scope("D"):
        start_all(wm_copies[0] + q_copies[0] + wm_copies[1] + w_copies[0])
        conv_step(filt=2, mul=0, free=MF[0], trim=MT[0])
    with jax.named_scope("E_wait"):
        wait_all(kv_groups[2])
    with jax.named_scope("E"):
        conv_step(units=units(TRIPLE, range(0, 2)), mul=1, inv=units((0,), range(NBL)), free=MF[1], trim=MT[1])
    with jax.named_scope("F_wait"):
        wait_all(kv_groups[3])
    with jax.named_scope("F"):
        conv_step(units=units(TRIPLE, range(2, NBL)))

    def full_step(j, carry):
        wait_all(sk_copy(j + 2))
        conv_step(filt=j + 2, mul=j + 1, inv=units((j,), range(IG)), free=MF[2], trim=MT[2])
        return carry

    with jax.named_scope("GH"):
        lax.fori_loop(1, NC - 2, full_step, 0)
    late = units((NC - 2,), range(NBL)) + units(range(1, NC - 2), range(IG, NBL))
    late = late[:IJ] + units((NC - 1,), range(NBL)) + late[IJ:]
    with jax.named_scope("J"):
        start_all(q_copies[1] + w_copies[1] + sum(q_copies[2:], []) + w_copies[2] + w_copies[3] + wm_copies[2], 1)
        conv_step(mul=NC - 1, inv=late[:IJ], free=MF[3], trim=MT[3])
    with jax.named_scope("r6_wait"):
        wait_all(wm_copies[0] + q_copies[0])
    with jax.named_scope("r6"):
        for j in range(3):
            mod_chunk(j)
        conv_step(inv=late[IJ:IJ + 1])
        toks = conv_step(inv=late[IJ + 1:len(late) - IP])
        nx0 = stage_p1(0, A0[1], None, _pick(toks[:R6[0]], A0[1] // 8, R6[1]) if toks else None)
    with jax.named_scope("p2_wait"):
        wait_all(wm_copies[1])
    with jax.named_scope("p2"):
        mod_chunk(4)
        mod_chunk(3)
        toks = conv_step(inv=late[len(late) - IP:])
        if toks:
            nx0 = hold(nx0, _pick(toks[:R6[2]], A0[1] // 8, R6[3]))
        stage_p2(0, A0[1], nx0)
    with jax.named_scope("w1_wait"):
        wait_all(w_copies[0])
    with jax.named_scope("m1_0"):
        square_ops(w1_v, s1_s, stage_m1(0, 4)[:-40])
    with jax.named_scope("w2_wait"):
        wait_all(q_copies[1] + w_copies[1])
    with jax.named_scope("m2_0"):
        stage_p(1, stage_m2(0, 4))
        filler(0)
    for t in range(1, NA):
        with jax.named_scope("a%d" % t):
            wait_all(q_copies[t + 1] if t + 1 < NA else w_copies[2] + w_copies[3] + wm_copies[2])
            toks = stage_m1(t, 2)
            toks = toks + stage_m2(t, 2, toks[len(toks) - len(toks) // 2:])
            if t + 1 < NA:
                stage_p(t + 1, toks)
            if t == 1:
                square_ops(w2_v, s2_s, toks[:-30])
            if t == NA - 1:
                transpose_w4(toks[:(len(toks) * LAST[0]) // 100])
                store_z(0, 0, toks[(len(toks) * LAST[1]) // 100:(len(toks) * LAST[2]) // 100])
                toks = toks + [x for x in lead_in()[:40] for _ in range(WS[5])]
                cut = (len(toks) * LAST[3]) // 100
                gate_row(toks[:(len(toks) * 9) // 10])
                w3_ops(toks[:cut])
                rest = [i for i in range(7) if i not in IN_LOOP]
                for k, i in enumerate(rest):
                    w4_ops(i, 0, toks[cut + k::len(rest)])
            filler(t)

    def out_copy(r0, n, c):
        rows = pl.ds(r0, n)
        return pltpu.make_async_copy(o_v.at[c, rows, :], o_hbm.at[rows, pl.ds(c * LANES, LANES)], sem_o.at[0])

    def raw4(n, d):
        return jnp.concatenate([wt_u[d, n], wt_u[NC - 1, n, d * (CQ // 2):(d + 1) * (CQ // 2), :]], axis=0)

    def mlp_tile(t, carry):
        r0 = pl.multiple_of(t * TB, TB)
        ws = t & 1
        count = [0]

        def fresh():
            count[0] += 1
            return lax.rem(t + 2 * count[0], 2)

        def g_rows(r2, p, lo, hi):
            base = (2 * r2 + p) * (FQ + GPAD)
            return slice(base + lo, base + hi)

        rem = {key: rh_s[k] for k, key in enumerate(BLOCKS[:4])}
        for key in BLOCKS[4:8]:
            rem[key] = rem3(*key)
        early = _rows8(rem[BLOCKS[4]], EW[0])
        rem[BLOCKS[8]] = rem3(*BLOCKS[8], pieces=4)
        todo = BLOCKS[9:]
        part = [None] * 7
        for i in (4, 3, 0, 6, 1, 2, 5):
            m = [None] * 7
            for j in _ORDER:
                slot = fresh()
                act = _operand(_LHS[j], lambda r2, k2: _operand(
                    _LHS[i], lambda r1, k1: zf_s[slot, z_rows(2 * r1 + r2, 2 * k1 + k2), :])).astype(BF16)
                if i in _RAW and j in _RAW:
                    d = 2 * _RAW.index(i) + _RAW.index(j)
                    wij = w3_u[d, d * (FQ // 2):(d + 1) * (FQ // 2), :]
                else:
                    wij = s3_u[i, j]
                m[j] = _dot_nt(_as_bf16(wij), act)
            key = todo.pop(0)
            rem[key] = rem3(*key)
            part[i] = _combine(m)
            if i in (4, 3, 0):
                early += _rows8(m[_ORDER[0]], EW[1]) + _rows8(m[_ORDER[4]], EW[2])
        zero = fresh() - ws
        fine = [x for x in early for _ in IN_LOOP]
        hop = len(fine) // (len(IN_LOOP) * 33)
        for k, i in enumerate(IN_LOOP):
            w4_ops(i, zero, fine[k * hop:len(fine) - (len(IN_LOOP) - k) * hop])
        for inner in range(4):
            r2, p = inner // 2, inner % 2
            for blk, pre in enumerate(_combine([part[i][inner] for i in range(7)])):
                g_s[blk][ws, g_rows(r2, p, 0, FQ), :] = _gelu2(pre + rem[2 * (blk // 2) + r2, 2 * (blk % 2) + p])

        toks = []
        marks = {}
        part = [[None] * 4 for _ in range(7)]
        for i in _ORDER:
            slot = fresh()
            we = jnp.concatenate([raw4(4 * NS + _RAW.index(i), 2 * _RAW.index(i) + e) if i in _RAW else e4_u[i, e]
                                  for e in range(2)], axis=0)
            ex = []
            for r2 in range(2):
                act = [_operand(_LHS[i], lambda r1, h: g_s[2 * r1 + h][slot, g_rows(r2, p, NS * LANES, FQ), :])
                       for p in range(2)]
                act = jnp.concatenate(act + [jnp.zeros((LANES - 2 * LQ, TQ), F32)], axis=0).astype(BF16)
                ex.append(_dot(_as_bf16(we), act))
            m = [None] * 7
            for j in _ORDER:
                slot = fresh()
                act = _operand(_LHS[j], lambda r2, p: _operand(
                    _LHS[i], lambda r1, h: g_s[2 * r1 + h][slot, g_rows(r2, p, 0, NS * LANES), :])).astype(BF16)
                if i in _RAW and j in _RAW:
                    d = 2 * _RAW.index(i) + _RAW.index(j)
                    wij = [raw4(4 * st + d, d) for st in range(NS)]
                else:
                    wij = [s4_u[i, j, st] for st in range(NS)]
                m[j] = _dot(_as_bf16(jnp.concatenate(wij, axis=1)), act)
                toks += _rows8(m[j])
            part[i] = [x + ex[inner // 2][(inner % 2) * QR:(inner % 2 + 1) * QR]
                       for inner, x in enumerate(_combine(m))]
            marks[i] = len(toks)

        gb = 0.5 * mod_s[NC, 0:1, :]
        nxt = jnp.minimum(t + 1, NT - 1) * TB
        tails = {}
        for i, blk, norm in ((4, 1, (0, NW[0]) + NW[2:4]), (3, 2, NW[0:2] + NW[4:6]), (6, 0, (NW[1], 4) + NW[6:8]),
                             (5, 3, None)):
            r1 = blk // 2
            if norm is None:
                toks += [x for x in lead_in()[8:40] for _ in range(3)]
            else:
                store_z(nxt, 1 - ws, toks[norm[2]:norm[3]], norm[0], norm[1])
            pos = [marks[i] + FL[(1, 2, 0, 3).index(blk)]]

            def finish(rq, c, h2t):
                h2 = hold(h2t.T, toks[pos[0]:pos[0] + TQ // 8])
                pos[0] += TQ // 8
                rows = pl.ds(pl.multiple_of(r0 + rq * TQ, TQ), TQ)
                cols = slice(c * LANES, (c + 1) * LANES)
                o_v[c, rows, :] = (x_s[rows, cols] + gb[:, cols] * (h_s[rows, cols] + h2)).astype(BF16)
                if blk == 3:
                    out_copy(rows.start, TQ, c).start()

            for inner in (1, 2, 0, 3):
                ht = _block([part[k][inner] for k in range(7)], blk)
                rq, c = 2 * r1 + inner // 2, 2 * (blk % 2) + inner % 2
                finish(rq, c, ht[0:LANES])
                tails[rq, c] = ht[LANES:]
            rb = pl.multiple_of(r0 + r1 * 2 * TQ, 2 * TQ)
            if blk != 3:
                for e in range(2):
                    out_copy(rb, 2 * TQ, 2 * (blk % 2) + e).start()
            if blk in (0, 3):
                for rq in (2 * r1, 2 * r1 + 1):
                    finish(rq, NC - 1, jnp.concatenate([tails[rq, c] for c in range(NC - 1)], axis=0))
                if blk == 0:
                    out_copy(rb, 2 * TQ, NC - 1).start()
        return carry

    with jax.named_scope("ph2b"):
        lax.fori_loop(0, NT, mlp_tile, 0)
    with jax.named_scope("tail"):
        pltpu.make_async_copy(o_v, o_v, sem_o.at[0]).wait()


@jax.jit
def pallas_adaLN_cond__ssm_conv_h3__mixer_s_mlp__prompt_kernel(
    A_q: jax.Array,
    A_k: jax.Array,
    A_v: jax.Array,
    A_shift_k: jax.Array,
    A_ssm_k: jax.Array,
    A_ssm_D: jax.Array,
    B_x: jax.Array,
    B_w1: jax.Array,
    B_w2: jax.Array,
    B_w3: jax.Array,
    B_w4: jax.Array,
    c: jax.Array,
    w_mod: jax.Array,
):
    B, S, D = A_q.shape
    FF = B_w3.shape[1]
    assert (B, S, D, FF, A_shift_k.shape[1]) == (1, sum(TILES), 5 * LANES, 1728, 4)
    NC = D // LANES
    NG = BLK // 8
    NBL = S // (PH * BLK)
    NS = FF // 4 // LANES
    n1 = S - sum(TILES[:BLOCKWISE1[0]]) - HALO
    n2 = S - sum(TILES[:BLOCKWISE2[0]])

    args = (A_q.reshape(S, D), A_k.reshape(S, D), A_v.reshape(S, D), A_shift_k.T, A_ssm_k,
            A_ssm_D, B_w1, B_w2, B_w3.T, B_w4, c, w_mod)
    scratch = [
        pltpu.VMEM((S, D), BF16),
        pltpu.VMEM((NC, S + 16, LANES), BF16),
        pltpu.VMEM((NC, S, LANES), BF16),
        pltpu.VMEM((4, D), BF16),
        pltpu.VMEM((NC, LANES, S), BF16),
        pltpu.VMEM((D,), BF16),
        pltpu.VMEM((NC, D, LANES), BF16),
        pltpu.VMEM((NC, D, LANES), BF16),
        pltpu.VMEM((NC, FF, LANES), BF16),
        pltpu.VMEM((NC, FF, LANES), BF16),
        pltpu.VMEM((1, D), BF16),
        pltpu.VMEM((D, 6 * D), BF16),
        pltpu.VMEM((PH, 2 * BLK, BLK), BF16),
        pltpu.VMEM((PH, 2, BLK, BLK), BF16),
        pltpu.VMEM((NC, S, LANES), BF16),
        pltpu.VMEM((NC, NG, NBL, PH, 2, 8, LANES), F32),
        pltpu.VMEM((NC, NG, NBL, PH, 2, 8, LANES), F32),
        pltpu.VMEM((NC, NBL, PH, 2 * BLK, LANES), BF16),
        pltpu.VMEM((6, PH, BLK, LANES), BF16),
        pltpu.VMEM((NC, S, LANES), F32),
        pltpu.VMEM((6, 8, D), F32),
        pltpu.VMEM((NC, 8, LANES), F32),
        pltpu.VMEM((NC, S + 16, LANES), F32),
        pltpu.VMEM((S, D), F32),
        pltpu.VMEM((S, D), F32),
        pltpu.VMEM((NC, S, LANES), BF16),
        pltpu.VMEM((7, 7, FF // 4, LANES), BF16),
        pltpu.VMEM((7, 7, NS, D // 4, LANES), BF16),
        pltpu.VMEM((7, 2, D // 4, LANES), BF16),
        [pltpu.VMEM((2, GROWS, TQ), F32)] * 4,
        pltpu.VMEM((2, 4 * NC * (TQ + 8), LANES), F32),
        pltpu.VMEM((TB, LANES), BF16),
        pltpu.VMEM((10, 2, n1 // 2, LANES), BF16),
        pltpu.VMEM((10, 2, n2 // 2, LANES), BF16),
        pltpu.VMEM((7, 2, 2 * LANES, LANES), BF16),
        pltpu.VMEM((7, 2, 2 * LANES, LANES), BF16),
        pltpu.VMEM((4, FF // 4, TQ), F32),
        pltpu.VMEM((NC, 4 * NS + 2, LANES, LANES), BF16),
        pltpu.VMEM((D, LANES), F32),
        pltpu.SemaphoreType.DMA((21,)),
        pltpu.SemaphoreType.DMA((1,)),
    ]
    out = pl.pallas_call(
        functools.partial(_kernel, S=S, D=D, FF=FF),
        in_specs=[pl.BlockSpec(memory_space=pl.ANY)] * len(args),
        out_specs=pl.BlockSpec(memory_space=pl.ANY),
        out_shape=jax.ShapeDtypeStruct((S, D), BF16),
        scratch_shapes=scratch,
        compiler_params=pltpu.CompilerParams(
            vmem_limit_bytes=120 * 1024 * 1024,
            disable_bounds_checks=True,
            disable_semaphore_checks=True,
        ),
    )(*args)
    return out.reshape(B, S, D)
```

```python
import functools
import math

import jax
import jax.numpy as jnp
from jax import lax
import jax.experimental.pallas as pl
import jax.experimental.pallas.tpu as pltpu

F32 = jnp.float32
BF16 = jnp.bfloat16
U32 = jnp.uint32

LANES = 128
BLK = 128
PH = 4
EPS = 1e-05
TB = 512
TQ = TB // 4
HALO = 32
TILES = (384, 384, 576, 704)
BLOCKWISE1 = (3,)
BLOCKWISE2 = (2, 3)
IN_LOOP = (4, 2, 0, 1, 3)
ROT = 3
KR = 256
NB1 = 1
IG = 2
IJ = 6
IP = 2
GPAD = 8
GROWS = 1768

MF = (6, 0, 5, 4)
MT = (3, 0, 3, 3)
R6 = (36, 18, 28, 6)
TRS = (145, 175, 180)
FRS = (50, 90, 90)
WS = (2, 3, 3, 2, 2, 4)
FI = (48, 88, 96, 96)
LAST = (55, 66, 92, 82)
EW = (2, 1, 2)
NW = (1, 3, 0, 150, 320, 460, 600, 730)
FL = (10, 10, 25, -32)
O3 = (4, 3, 0, 6, 2, 1, 5)
J3 = (1, 2, 3, 4, 5, 6, 0)
J4 = (4, 2, 3, 1, 0, 6, 5)
ET = (0, 4)
EC = 10

_ORDER = (2, 4, 1, 3, 0, 6, 5)
_RAW = (1, 4)
_LHS = (((0, 0), 1, (1, 1)), ((1, 0), 1, (1, 1)), ((0, 0),), ((1, 1),),
        ((0, 0), 1, (0, 1)), ((1, 0), -1, (0, 0)), ((0, 1), -1, (1, 1)))
_RHS = (((0, 0), 1, (1, 1)), ((0, 0),), ((0, 1), -1, (1, 1)), ((1, 0), -1, (0, 0)),
        ((1, 1),), ((0, 0), 1, (0, 1)), ((1, 0), 1, (1, 1)))


def _operand(terms, blk):
    x = blk(*terms[0])
    if len(terms) > 1:
        y = blk(*terms[2])
        x = x + y if terms[1] > 0 else x - y
    return x


def _all_operands(table, b00, b01, b10, b11):
    blocks = ((b00, b01), (b10, b11))
    return [_operand(terms, lambda i, j: blocks[i][j]) for terms in table]


def _block(m, which):
    if which == 0:
        return (m[3] - m[4]) + m[0] + m[6]
    if which == 1:
        return m[2] + m[4]
    if which == 2:
        return m[1] + m[3]
    return (m[2] - m[1]) + m[0] + m[5]


def _combine(m):
    return [_block(m, which) for which in range(4)]


def _as_bf16(x):
    return pltpu.bitcast(x, BF16)


def _lo(x):
    return pltpu.bitcast(x << 16, F32)


def _hi(x):
    return pltpu.bitcast(x & jnp.uint32(0xFFFF0000), F32)


def _dft4(re, im, sign):
    ar, ai = re[0] + re[2], im[0] + im[2]
    br, bi = re[0] - re[2], im[0] - im[2]
    cr, ci = re[1] + re[3], im[1] + im[3]
    dr, di = re[1] - re[3], im[1] - im[3]
    o0 = (ar + cr, ai + ci)
    o2 = (ar - cr, ai - ci)
    m = (br + di, bi - dr)
    p = (br - di, bi + dr)
    o1, o3 = (m, p) if sign < 0 else (p, m)
    return [o0[0], o1[0], o2[0], o3[0]], [o0[1], o1[1], o2[1], o3[1]]


def _ln(x, eps=EPS, unit=True):
    n = x.shape[-1]
    s1 = jnp.sum(x, axis=-1, keepdims=True)
    m = s1 * (1.0 / n)
    v = jnp.maximum(jnp.sum(x * x, axis=-1, keepdims=True) + (n * eps - s1 * m), n * eps)
    e = jnp.log(v) * (-0.5 / math.log(2.0))
    return (x - m) * jnp.exp2(e + 0.5 * math.log2(n) if unit else e)


def _gelu2(x):
    c0 = math.sqrt(2.0 / math.pi)
    return x + x * jnp.tanh(x * (c0 + (c0 * 0.044715) * (x * x)))


def _dot(a, b):
    return jnp.dot(a, b, preferred_element_type=F32)


def _dot_nt(a, b):
    return lax.dot_general(a, b, (((1,), (1,)), ((), ())), preferred_element_type=F32)


def _rows8(x, repeat=1):
    return [x[8 * r:8 * r + 8, 0:LANES] for r in range(x.shape[0] // 8) for _ in range(repeat)]


def _chunks(r0, r1, k, unit=16):
    n = (r1 - r0) // unit
    cuts = [r0 + unit * ((n * j) // k) for j in range(k + 1)]
    return list(zip(cuts[:-1], cuts[1:]))


def _pick(toks, n, free=0):
    idx = [(r * (len(toks) + free)) // n - free for r in range(n)]
    return [toks[i] if i >= 0 else None for i in idx]


def _kernel(q_hbm, k_hbm, v_hbm, sh_hbm, sk_hbm, sd_hbm, w1_hbm, w2_hbm, w3_hbm, w4_hbm, c_hbm, wm_hbm,
            o_hbm,
            q_v, k_v, v_v, sh_v, sk_v, sd_v, w1_v, w2_v, w3_v, w4_v, c_v, wm_v,
            fw_s, iv_s, o_v, u_s, kk_s, vv_s, wu_s, y_s, mod_s, par_s, h1_s, x_s, h_s, z_s,
            s3_s, s4_s, e4_s, g_s, zf_s, zr_s, l1_s, l2_s, s1_s, s2_s, rh_s, wt_s, scol_s,
            sem, sem_o,
            *, S, D, FF):
    NC = D // LANES
    NG = BLK // 8
    LB = PH * BLK
    NBL = S // LB
    R = BLK // PH
    HL = LANES // 2

    small = [
        pltpu.make_async_copy(sh_hbm, sh_v, sem.at[0]),
        pltpu.make_async_copy(sd_hbm, sd_v, sem.at[0]),
        pltpu.make_async_copy(c_hbm, c_v, sem.at[0]),
    ]

    def sk_copy(c):
        ch = (c + ROT) % NC * LANES
        rows = pl.ds(ch if isinstance(c, int) else pl.multiple_of(ch, LANES), LANES)
        return [pltpu.make_async_copy(sk_hbm.at[rows, :], sk_v.at[c], sem.at[1 + c])]

    def kv_copies(tiles, blocks, s):
        return [pltpu.make_async_copy(src.at[pl.ds(r, KR), pl.ds((c + ROT) % NC * LANES, LANES)],
                                      dst.at[c, pl.ds(off + r, KR), :], sem.at[s])
                for r in range(blocks[0] * LB, (blocks[-1] + 1) * LB, KR)
                for src, dst, off in ((k_hbm, k_v, 16), (v_hbm, v_v, 0)) for c in tiles]

    PAIR, TRIPLE = (0, 1), (2, 3, 4)
    kv_groups = [kv_copies(PAIR, range(0, NB1), 9), kv_copies(PAIR, range(NB1, NBL), 10),
                 kv_copies(TRIPLE, range(0, 2), 11), kv_copies(TRIPLE, range(2, NBL), 20)]

    WM = (0, 3 * D, 5 * D, 6 * D)
    wm_copies = [[pltpu.make_async_copy(wm_hbm.at[:, pl.ds(WM[j], WM[j + 1] - WM[j])],
                                        wm_v.at[:, pl.ds(WM[j], WM[j + 1] - WM[j])], sem.at[6 + j])]
                 for j in range(3)]
    w_copies = [[pltpu.make_async_copy(src.at[:, pl.ds(c * LANES, LANES)], dst.at[c], sem.at[12 + j])
                 for c in range(NC)]
                for j, (src, dst) in enumerate(((w1_hbm, w1_v), (w2_hbm, w2_v), (w3_hbm, w3_v), (w4_hbm, w4_v)))]

    B0 = [0]
    for n in TILES:
        B0.append(B0[-1] + n)
    NA = len(TILES)
    A0 = [0] + [r + HALO for r in B0[1:-1]] + [S]
    q_copies = [
        [pltpu.make_async_copy(q_hbm.at[pl.ds(A0[t], A0[t + 1] - A0[t])], q_v.at[pl.ds(A0[t], A0[t + 1] - A0[t])],
                               sem.at[16 + t])]
        for t in range(NA)
    ]

    def start_all(cps, priority=0):
        for cp in cps:
            cp.start(priority=priority)

    def wait_all(cps):
        for cp in cps:
            cp.wait()

    for c in range(NC):
        k_v[c, 0:16, :] = jnp.zeros((16, LANES), BF16)
    start_all(sk_copy(0) + small + sk_copy(1) + kv_groups[0] + kv_groups[1] + sk_copy(2))

    for c in range(NC):
        h1_s[c, 0:8, :] = jnp.zeros((8, LANES), F32)
        h1_s[c, S + 8:S + 16, :] = jnp.zeros((8, LANES), F32)

    prow = lax.broadcasted_iota(jnp.int32, (BLK, BLK), 0)
    pcol = lax.broadcasted_iota(jnp.int32, (BLK, BLK), 1)
    ang = (((4 * prow + 1) * pcol) & (4 * BLK - 1)).astype(F32) * (2.0 * math.pi / (4 * BLK))
    tw = (4 * prow + 1).astype(F32) * (2.0 * math.pi / (4 * LB))
    mr, mi = jnp.cos(ang), -jnp.sin(ang)
    twr, twi = jnp.cos(tw), -jnp.sin(tw)
    eye = jnp.where(prow == pcol, 1.0 / LB, 0.0).astype(BF16)
    for i in range(PH):
        both = jnp.stack([mr.reshape(NG, 8, BLK), mi.reshape(NG, 8, BLK)], axis=1).reshape(2 * BLK, BLK)
        fw_s[i] = both.astype(BF16)
        for h in range(2):
            iv_s[i, h] = _dot_nt(eye, both[h * BLK:(h + 1) * BLK, :].astype(BF16)).astype(BF16)
        if i + 1 < PH:
            mr, mi = mr * twr - mi * twi, mr * twi + mi * twr
    perm = jnp.where(pcol == (prow % R) * PH + prow // R, 1.0, 0.0).astype(BF16)

    wait_all(small)
    shf = sh_v[...].astype(F32)
    sdf = sd_v[...].astype(F32).reshape(1, D)
    for c in range(NC):
        par_s[(c - ROT) % NC, 0:4, :] = shf[:, c * LANES:(c + 1) * LANES]
        par_s[(c - ROT) % NC, 4:5, :] = sdf[:, c * LANES:(c + 1) * LANES]
    cf = c_v[...].astype(F32)
    sc = (cf * jax.nn.sigmoid(cf)).astype(BF16)
    sc16 = jnp.broadcast_to(sc, (16, D))

    def mod_chunk(j):
        mod_s[j] = _dot(sc16, wm_v[:, j * D:(j + 1) * D])[0:8, :]

    (fw_u, iv_u, k_u, v_u, wu_u, vv_u, z_u, l1_u, l2_u, w1_u, w2_u, s1_u, s2_u, w3_u, w4_u, wt_u, s3_u, s4_u,
     e4_u, zr_u) = (r.bitcast(U32) for r in (fw_s, iv_s, k_v, v_v, wu_s, vv_s, z_s, l1_s, l2_s, w1_v, w2_v,
                                             s1_s, s2_s, w3_v, w4_v, wt_s, s3_s, s4_s, e4_s, zr_s))

    never = twr[0:8, :] > 2.0

    def after(token, x):
        if token.dtype != x.dtype:
            token = pltpu.bitcast(token, x.dtype)
        return jnp.where(jnp.broadcast_to(never, x.shape), token, x)

    def hold(x, tks):
        f = len([k for k in tks if k is None])
        n = len(tks)
        head = after(jnp.stack(tks[f:]), x[8 * f:, 0:LANES].reshape(n - f, 8, LANES)).reshape(8 * (n - f), LANES)
        if f:
            head = jnp.concatenate([x[:8 * f, 0:LANES], head], axis=0)
        return head if x.shape[1] == LANES else jnp.concatenate([head, x[:, LANES:]], axis=1)

    def hold16(x, tks):
        x4 = x.reshape(len(tks), 2, 8, LANES)
        return jnp.stack([after(jnp.stack(tks), x4[:, 0]), x4[:, 1]], axis=1).reshape(x.shape)

    def perm_k(c, b, toks):
        kt = [_dot_nt(perm, sk_v[c, :, b * LB + t * BLK:b * LB + (t + 1) * BLK]) for t in range(PH)]
        toks += _rows8(kt[0])[::2]
        return [jnp.concatenate([kt[t][i * R:(i + 1) * R, :] for t in range(PH)], axis=0).astype(BF16)
                for i in range(PH)]

    def spectrum(comps, dst, slot, b, toks, dc=None, pins=None):
        tr, ti = [], []
        for i in range(PH):
            lhs = fw_u[i]
            if pins is not None and i < len(pins):
                lhs = after(pins[i], lhs.reshape(NG, 8, LANES)).reshape(BLK, LANES)
            t4 = _dot(_as_bf16(lhs), comps[i]).reshape(NG, 2, 8, LANES)
            tr.append(t4[:, 0])
            ti.append(t4[:, 1])
        toks += [ti[PH - 1][g] for g in range(NG)]
        if dc is not None:
            tr[0] = tr[0] + dc
        sr, si = _dft4(tr, ti, -1)
        for qq in range(PH):
            dst[slot, :, b, qq, 0] = sr[qq]
            dst[slot, :, b, qq, 1] = si[qq]

    def gated(c, b, n):
        w = [par_s[c, t:t + 1, :] for t in range(4)]
        kc = {}
        for o in range(-2, 2):
            words = k_u[c, pl.ds(8 + b * (LB // 2) + o, BLK, stride=2), :]
            if o > -2:
                kc[2 * o] = _lo(words)
            kc[2 * o + 1] = _hi(words)
        vc = {}
        for o in range(2):
            words = v_u[c, pl.ds(b * (LB // 2) + o, BLK, stride=2), :]
            vc[2 * o] = _lo(words)
            vc[2 * o + 1] = _hi(words)
        for i in range(PH):
            ks = kc[i] * w[0]
            for t in range(1, 4):
                ks = ks + kc[i - t] * w[t]
            wu_s[n, i] = (ks * vc[i]).astype(BF16)
        return [wu_u[n, i] for i in range(PH)]

    def kv_pins(kvb):
        return [jnp.stack([kvb[2 * m + (r % 2)][8 * (r // 2):8 * (r // 2) + 8, :] for r in range(NG)])
                for m in range(2)]

    def products(c, ks, kc, toks, free, trim):
        n = len(toks) - trim + free
        cum = (44, 128, 244, 392)
        zp = None
        for o in range(NBL):
            idx = [((g * cum[-1] + cum[o]) * n) // (cum[-1] * NG) - 1 - free for g in range(NG)]
            tk = [toks[max(i, 0)] if i >= 0 or not free else None for i in idx]
            zr, zi = [], []
            for qq in range(PH):
                accr = acci = None
                for b in range(o + 1):
                    a_, b_ = u_s[c, :, b, qq, 0], u_s[c, :, b, qq, 1]
                    c_, d_ = ks[kc, :, o - b, qq, 0], ks[kc, :, o - b, qq, 1]
                    if qq == 0 and b == o:
                        a_ = hold(a_.reshape(BLK, LANES), tk).reshape(NG, 8, LANES)
                    tr_ = a_ * c_ - b_ * d_
                    ti_ = a_ * d_ + b_ * c_
                    accr = tr_ if accr is None else accr + tr_
                    acci = ti_ if acci is None else acci + ti_
                zr.append(accr)
                zi.append(acci)
            if zp is None:
                yr, yi = zr, zi
            else:
                yr = [zr[qq] - zp[1][qq] for qq in range(PH)]
                yi = [zi[qq] + zp[0][qq] for qq in range(PH)]
            zp = (zr, zi)
            vr, vi = _dft4(yr, yi, +1)
            for i in range(PH):
                vv_s[c, o, i] = jnp.stack([vr[i], vi[i]], axis=1).reshape(2 * BLK, LANES).astype(BF16)

    def inverse(c, o, toks, pins):
        for i in range(PH):
            yv = None
            for h in range(2):
                lhs = iv_u[i, h]
                if pins is not None and h == 0:
                    pin = pins[i % 2][8 * (i // 2):8 * (i // 2) + 8]
                    lhs = after(pin, lhs.reshape(8, 8, LANES)).reshape(HL, LANES)
                t = _dot(_as_bf16(lhs), _as_bf16(vv_u[c, o, i, h * HL:(h + 1) * HL, :]))
                yv = t if yv is None else yv + t
            if i % 2 == 0:
                toks += _rows8(yv)[::2]
            y_s[c, pl.ds(o * LB + i, BLK, stride=PH), :] = yv

    def conv_step(filt=None, units=(), mul=None, inv=(), free=0, trim=3):
        toks = []
        kv = [gated(c, b, n) for n, (c, b) in enumerate(units)]
        pin_at = {n: kv_pins(kv[n]) for n in range(len(units))} if inv or filt is not None else {}
        if filt is not None and mul is not None and not isinstance(filt, int):
            ks = kk_s.at[pl.ds(mul, 2)]
            k_rd, k_wr = (ks, 0), (ks, 1)
        else:
            k_rd, k_wr = (kk_s, mul), (kk_s, filt)
        pos = 0
        for c, o in inv:
            inverse(c, o, toks, pin_at.get(pos))
            pos += 1
        if filt is not None:
            comps = [perm_k(filt, b, toks) for b in range(NBL)]
            for b in range(NBL):
                spectrum(comps[b], *k_wr, b, toks, par_s[filt, 4:5, :] if b == 0 else None, pin_at.get(pos))
                pos += 1
        for n, (c, b) in enumerate(units):
            spectrum([_as_bf16(x) for x in kv[n]], u_s, c, b, toks, None, pin_at.get(pos))
            pos += 1
        if mul is not None:
            products(mul, *k_rd, toks, free, trim)
        return toks

    def lane_tiles(x):
        return [x[:, c * LANES:(c + 1) * LANES] for c in range(NC)]

    def stage_p1(r0, r1, tks=None, ytks=None):
        ga = mod_s[2, 0:1, :]
        a_mul, a_add = ga * (1.0 + mod_s[1, 0:1, :]) * math.sqrt(D), ga * mod_s[0, 0:1, :]
        q = q_v[r0:r1, :].astype(F32)
        if tks is not None:
            q = hold(q, tks)
        y = jnp.concatenate([y_s[(c - ROT) % NC, r0:r1, :] for c in range(NC)], axis=1)
        if ytks is not None:
            y = hold(y, ytks)
        x = q + (_ln(q, unit=False) * a_mul + a_add) * y
        x_s[r0:r1, :] = x
        return _ln(x, unit=False)

    def store_row_ops(dst, base, r0, r1, cols, tks=None):
        hv = []
        for x in cols:
            x4 = x.reshape(x.shape[0] // 32, 2, 16, LANES)
            hv.append([x4[:, e].reshape(x.shape[0] // 2, LANES) for e in range(2)])
        for k2 in range(2):
            a00, a01, a10, a11 = hv[k2][0], hv[2 + k2][0], hv[k2][1], hv[2 + k2][1]
            if tks is not None:
                a00, a11 = hold16(a00, tks), hold16(a11, tks)
            for o, x in enumerate(_all_operands(_LHS, a00, a01, a10, a11) + [a01, a10, hv[NC - 1][k2]]):
                dst[o, k2, (r0 - base) // 2:(r1 - base) // 2, :] = x.astype(BF16)

    L1B = A0[BLOCKWISE1[0]]
    L2B = B0[BLOCKWISE2[0]]

    def stage_p2(r0, r1, nx, blockwise=False):
        h = nx * ((1.0 + mod_s[4, 0:1, :]) * (2.0 * math.sqrt(D))) + 2.0 * mod_s[3, 0:1, :]
        h_s[r0:r1, :] = h
        zn = lane_tiles(_ln(h, 4.0 * EPS))
        if blockwise:
            store_row_ops(l1_s, L1B, r0, r1, zn)
        else:
            for c in range(NC):
                z_s[c, r0:r1, :] = zn[c].astype(BF16)

    def stage_p(t, toks):
        lo, hi = A0[t], A0[t + 1]
        stage_p2(lo, hi, stage_p1(lo, hi, _pick(toks[:-TRS[t - 1]], (hi - lo) // 8, FRS[t - 1])), t in BLOCKWISE1)

    def filler(t):
        red = jnp.sum(y_s[t, 0:8 * FI[t], :], axis=-1, keepdims=True).reshape(FI[t], 8, 1)
        spare = (NC - 1) * (TQ + 8) + 8 * t
        zf_s[1, spare:spare + 8, :] = jnp.broadcast_to(jnp.sum(red, axis=0), (8, LANES))

    def square_ops(src, dst, toks):
        HK = 2 * LANES
        tks = _pick(toks, 2 * HK // 16)
        for n2 in range(2):
            tk = tks[n2 * (HK // 16):(n2 + 1) * (HK // 16)]
            blk = lambda k, n: src[2 * n + n2, k * HK:(k + 1) * HK, :].astype(F32)
            for o, x in enumerate(_all_operands(_RHS, hold16(blk(0, 0), tk), blk(0, 1), blk(1, 0), hold16(blk(1, 1), tk))):
                if o not in _RAW:
                    dst[o, n2] = x.astype(BF16)

    def block_dots(ops_u, base, prepare, w_u, s_u, parts, emit, light, heavy):
        toks = []

        def timed(x, weight):
            toks.extend(_rows8(x, weight))
            return x

        def weave(top, bot):
            n = top.shape[0] // 16
            return jnp.stack([top.reshape(n, 16, LANES), bot.reshape(n, 16, LANES)], axis=1).reshape(32 * n, LANES)

        def main(get):
            m = [None] * 7
            rem = [None, None]
            for o in ('t', 2, 4, 'b', 1, 3, 0, 6, 5):
                if o in ('t', 'b'):
                    e = 0 if o == 't' else 1
                    rhs = jnp.concatenate([w_u[c, 2 * LANES:D // 2, :] for c in range(NC - 1)], axis=1)
                    rem[e] = timed(_dot(get([(9, e)]), _as_bf16(rhs)), light)
                    continue
                if o in _RAW:
                    d = _RAW.index(o)
                    rhs = jnp.concatenate([w_u[2 * d + n2, d * LANES:(d + 1) * LANES, :] for n2 in range(2)], axis=1)
                else:
                    rhs = jnp.concatenate([s_u[o, n2] for n2 in range(2)], axis=1)
                m[o] = timed(_dot(get([(o, 0), (o, 1)]), _as_bf16(rhs)), heavy if o in (4, 3, 6, 5) else light)
            c00, c01, c10, c11 = _combine(m)
            top = jnp.concatenate([c00, c01], axis=1) + rem[0]
            bot = jnp.concatenate([c10, c11], axis=1) + rem[1]
            return [weave(top[:, c * LANES:(c + 1) * LANES], bot[:, c * LANES:(c + 1) * LANES]) for c in range(NC - 1)]

        def last(get):
            w = _as_bf16(w_u[NC - 1])
            return weave(timed(_dot(get([(2, 0), (2, 1), (7, 0), (7, 1), (9, 0)]), w), light),
                         timed(_dot(get([(8, 0), (8, 1), (3, 0), (3, 1), (9, 1)]), w), light))

        mark = None
        for j, (r0, r1) in enumerate(parts):
            prepare(r0, r1, None if mark is None else toks[mark:])
            mark = len(toks)
            get = lambda keys: _as_bf16(jnp.concatenate(
                [ops_u[o, e, (r0 - base) // 4:(r1 - base) // 4, :] for o, e in keys], axis=1))
            if j % 2:
                tail = last(get)
                emit(r0, r1, main(get) + [tail])
            else:
                emit(r0, r1, main(get) + [last(get)])
        return toks

    def stage_m1(t, k):
        def emit(r0, r1, cols):
            out = [_gelu2(x) for x in cols]
            for c in range(NC):
                h1_s[c, r0 + 8:r1 + 8, :] = out[c]
            return out

        if t in BLOCKWISE1:
            return block_dots(l1_u, L1B, lambda *_: None, w1_u, s1_u, _chunks(A0[t], A0[t + 1], k, 32), emit, WS[2], WS[3])
        toks = []
        for r0, r1 in _chunks(A0[t], A0[t + 1], k):
            lhs = jnp.concatenate([z_u[c, r0 // 2:r1 // 2, :] for c in range(NC)], axis=1)
            w = jnp.concatenate([w1_u[c] for c in range(NC)], axis=1)
            for x in emit(r0, r1, lane_tiles(_dot(_as_bf16(lhs), _as_bf16(w)))):
                toks += _rows8(x, WS[0])
        return toks

    def shifted(r0, r1):
        n, grp, shifts = r1 - r0, D // 4, (-1, 1, -2, 2)
        lane = lax.broadcasted_iota(jnp.int32, (n, LANES), 1)
        cols = []
        for c in range(NC):
            lo, hi = c * LANES, (c + 1) * LANES
            g_lo, g_hi = lo // grp, (hi - 1) // grp
            val = h1_s[c, pl.ds(r0 + 8 + shifts[g_lo], n), :]
            if g_hi != g_lo:
                other = h1_s[c, pl.ds(r0 + 8 + shifts[g_hi], n), :]
                val = jnp.where(lane < (g_hi * grp - lo), val, other)
            cols.append(val)
        return cols

    def stage_m2(t, k, before=None):
        def emit(r0, r1, cols):
            x1 = h_s[r0:r1, :] + jnp.concatenate(cols, axis=1)
            h_s[r0:r1, :] = x1
            return x1

        if t in BLOCKWISE2:
            def prepare(r0, r1, prev):
                prev = before if prev is None else prev
                prev = prev[len(prev) // 8:(len(prev) * 7) // 8]
                store_row_ops(l2_s, L2B, r0, r1, shifted(r0, r1), _pick(prev, (r1 - r0) // 32))
            return block_dots(l2_u, L2B, prepare, w2_u, s2_u, _chunks(B0[t], B0[t + 1], k, 32), emit, WS[4], WS[4])
        toks = []
        for r0, r1 in _chunks(B0[t], B0[t + 1], k):
            w = jnp.concatenate([w2_u[c] for c in range(NC)], axis=1)
            hs = _dot(jnp.concatenate(shifted(r0, r1), axis=1).astype(BF16), _as_bf16(w))
            for x in lane_tiles(emit(r0, r1, [hs])):
                toks += _rows8(x, WS[1])
        return toks

    NT = S // TB
    FQ = FF // 4
    NS = FQ // LANES
    LQ = FQ - NS * LANES
    CQ = LANES // 4
    QR = LANES + CQ
    BLOCKS = [(2 * r1 + r2, 2 * h + p)
              for r1, h in ((0, 0), (1, 0), (0, 1), (1, 1)) for r2 in range(2) for p in range(2)]

    def z_rows(rq, c):
        lo = (NC * rq + c) * (TQ + 8)
        return slice(lo, lo + TQ)

    def store_z(r0, slot, toks, q0=0, q1=4):
        n = (q1 - q0) * TQ
        rows = pl.ds(r0 + q0 * TQ if isinstance(r0, int) else pl.multiple_of(r0 + q0 * TQ, TQ), n)
        zn = lane_tiles(_ln(hold(h_s[rows, :], _pick(toks, n // 8)), 4.0 * EPS))
        for rq in range(q0, q1):
            for c in range(NC - 1):
                zf_s[slot, z_rows(rq, c), :] = zn[c][(rq - q0) * TQ:(rq - q0 + 1) * TQ]
        zr_s[q0 * TQ:q1 * TQ, :] = zn[NC - 1].astype(BF16)

    def w3_ops(toks):
        ng = FQ // 16
        blk = lambda c, d: w3_v[c, d * FQ:(d + 1) * FQ, :].astype(F32)
        outer = [[_all_operands(_RHS, blk(k2, p), blk(k2, 2 + p), blk(2 + k2, p), blk(2 + k2, 2 + p))
                  for p in range(2)] for k2 in range(2)]
        for k, i in enumerate((1, 5, 2, 4, 0, 3, 6)):
            tk = [toks[((k + r * 7) * len(toks)) // (7 * ng)] for r in range(ng)]
            for j, x in enumerate(_all_operands(_RHS, hold16(outer[0][0][i], tk), outer[0][1][i], outer[1][0][i],
                                                hold16(outer[1][1][i], tk))):
                if i not in _RAW or j not in _RAW:
                    s3_s[i, j] = x.astype(BF16)

    def transpose_w4(toks):
        order = [(c, n) for n in (4 * NS, 4 * NS + 1) + tuple(range(4 * NS)) for c in range(NC)]
        for k, (c, n) in enumerate(order):
            if n >= 4 * NS:
                ends = [(2 * (n - 4 * NS) + p + 1) * FQ // 2 for p in range(2)]
                x = jnp.concatenate([w4_u[c, e - LQ // 2:e, :] for e in ends]
                                    + [jnp.zeros((HL - LQ, LANES), U32)], axis=0)
            else:
                lo = (n % 4) * FQ // 2 + (n // 4) * HL
                x = w4_u[c, lo:lo + HL, :]
            x = jnp.concatenate([after(toks[(k * len(toks)) // len(order)], x[0:8]), x[8:]], axis=0)
            wt_s[c, n] = _as_bf16(x).astype(F32).T.astype(BF16)

    def w4_ops(i, zero, toks):
        ng = QR // 16
        total = (NS * 7 + 2) * ng
        tk = lambda pos, step: [toks[((pos + r * step) * len(toks)) // total] for r in range(ng)]
        quarter = lambda n, d: jnp.concatenate(
            [wt_s[d, n].astype(F32), wt_s[NC - 1, n, d * CQ:(d + 1) * CQ, :].astype(F32)], axis=0)
        if i not in _RAW:
            for e in range(2):
                x = _operand(_RHS[i], lambda h, d: quarter(4 * NS + h, 2 * d + e))
                e4_s[i + zero, e] = hold16(x, tk(e * ng, 1)).astype(BF16)
        for st in range(NS):
            t = [[_operand(_RHS[i], lambda h, d: quarter(4 * st + 2 * h + p, 2 * d + e)) for e in range(2)]
                 for p in range(2)]
            tks = tk((2 + st * 7) * ng, 7)
            for j, x in enumerate(_all_operands(_RHS, hold16(t[0][0], tks), t[0][1], t[1][0], hold16(t[1][1], tks))):
                if i not in _RAW or j not in _RAW:
                    s4_s[i + zero, j, st] = x.astype(BF16)

    def gate_row(toks):
        ng = D // 8
        col = after(jnp.stack(_pick(toks, ng)), scol_s[...].reshape(ng, 8, LANES))
        for c in range(NC):
            wf = wm_v[:, (NC * NC + c) * LANES:(NC * NC + c + 1) * LANES].astype(F32).reshape(ng, 8, LANES)
            acc = col[0] * wf[0]
            for r in range(1, ng):
                acc = acc + col[r] * wf[r]
            mod_s[NC, :, c * LANES:(c + 1) * LANES] = jnp.broadcast_to(jnp.sum(acc, axis=0, keepdims=True), (8, LANES))

    def rem3(rq, d, pieces=1):
        z = _as_bf16(zr_u[rq * (TQ // 2):(rq + 1) * (TQ // 2), :])
        return jnp.concatenate([_dot_nt(_as_bf16(w3_u[NC - 1, lo // 2:hi // 2, :]), z)
                                for lo, hi in _chunks(d * FQ, (d + 1) * FQ, pieces)], axis=0)

    def lead_in():
        head = [rem3(*key) for key in BLOCKS[:4]]
        for k in range(4):
            rh_s[k] = head[k]
        return _rows8(head[0])

    def units(tiles, blocks):
        return [(c, b) for b in blocks for c in tiles]

    with jax.named_scope("A"):
        wait_all(sk_copy(0))
        conv_step(filt=0)
    with jax.named_scope("B_wait"):
        wait_all(sk_copy(1) + kv_groups[0])
    with jax.named_scope("B"):
        start_all(kv_groups[2] + kv_groups[3] + sk_copy(3) + sk_copy(4))
        conv_step(filt=1, units=units(PAIR, range(0, NB1)))
        scol_s[...] = jnp.broadcast_to(sc.astype(F32), (LANES, D)).T
    with jax.named_scope("C_wait"):
        wait_all(kv_groups[1])
    with jax.named_scope("C"):
        conv_step(units=units(PAIR, range(NB1, NBL)))
    with jax.named_scope("D_wait"):
        wait_all(sk_copy(2))
    with jax.named_scope("D"):
        start_all(wm_copies[0] + q_copies[0] + wm_copies[1] + w_copies[0])
        conv_step(filt=2, mul=0, free=MF[0], trim=MT[0])
    with jax.named_scope("E_wait"):
        wait_all(kv_groups[2])
    with jax.named_scope("E"):
        conv_step(units=units(TRIPLE, range(0, 2)), mul=1, inv=units((0,), range(NBL)), free=MF[1], trim=MT[1])
    with jax.named_scope("F_wait"):
        wait_all(kv_groups[3])
    with jax.named_scope("F"):
        conv_step(units=units(TRIPLE, range(2, NBL)))

    def full_step(j, carry):
        wait_all(sk_copy(j + 2))
        conv_step(filt=j + 2, mul=j + 1, inv=units((j,), range(IG)), free=MF[2], trim=MT[2])
        return carry

    with jax.named_scope("GH"):
        lax.fori_loop(1, NC - 2, full_step, 0)
    late = units((NC - 2,), range(NBL)) + units(range(1, NC - 2), range(IG, NBL))
    late = late[:IJ] + units((NC - 1,), range(NBL)) + late[IJ:]
    with jax.named_scope("J"):
        start_all(q_copies[1] + w_copies[1] + sum(q_copies[2:], []) + w_copies[2] + w_copies[3] + wm_copies[2], 1)
        conv_step(mul=NC - 1, inv=late[:IJ], free=MF[3], trim=MT[3])
    with jax.named_scope("r6_wait"):
        wait_all(wm_copies[0] + q_copies[0])
    with jax.named_scope("r6"):
        for j in range(3):
            mod_chunk(j)
        conv_step(inv=late[IJ:IJ + 1])
        toks = conv_step(inv=late[IJ + 1:len(late) - IP])
        nx0 = stage_p1(0, A0[1], None, _pick(toks[:R6[0]], A0[1] // 8, R6[1]) if toks else None)
    with jax.named_scope("p2_wait"):
        wait_all(wm_copies[1])
    with jax.named_scope("p2"):
        mod_chunk(4)
        mod_chunk(3)
        toks = conv_step(inv=late[len(late) - IP:])
        if toks:
            nx0 = hold(nx0, _pick(toks[:R6[2]], A0[1] // 8, R6[3]))
        stage_p2(0, A0[1], nx0)
    with jax.named_scope("w1_wait"):
        wait_all(w_copies[0])
    with jax.named_scope("m1_0"):
        square_ops(w1_v, s1_s, stage_m1(0, 4)[:-40])
    with jax.named_scope("w2_wait"):
        wait_all(q_copies[1] + w_copies[1])
    with jax.named_scope("m2_0"):
        stage_p(1, stage_m2(0, 4))
        filler(0)
    for t in range(1, NA):
        with jax.named_scope("a%d" % t):
            wait_all(q_copies[t + 1] if t + 1 < NA else w_copies[2] + w_copies[3] + wm_copies[2])
            toks = stage_m1(t, 2)
            toks = toks + stage_m2(t, 2, toks[len(toks) - len(toks) // 2:])
            if t + 1 < NA:
                stage_p(t + 1, toks)
            if t == 1:
                square_ops(w2_v, s2_s, toks[:-30])
            if t == NA - 1:
                transpose_w4(toks[:(len(toks) * LAST[0]) // 100])
                store_z(0, 0, toks[(len(toks) * LAST[1]) // 100:(len(toks) * LAST[2]) // 100])
                toks = toks + [x for x in lead_in()[:40] for _ in range(WS[5])]
                cut = (len(toks) * LAST[3]) // 100
                gate_row(toks[:(len(toks) * 9) // 10])
                w3_ops(toks[:cut])
                rest = [i for i in range(7) if i not in IN_LOOP]
                for k, i in enumerate(rest):
                    w4_ops(i, 0, toks[cut + k::len(rest)])
            filler(t)

    def out_copy(r0, n, c):
        rows = pl.ds(r0, n)
        return pltpu.make_async_copy(o_v.at[c, rows, :], o_hbm.at[rows, pl.ds(c * LANES, LANES)], sem_o.at[0])

    def raw4(n, d):
        return jnp.concatenate([wt_u[d, n], wt_u[NC - 1, n, d * (CQ // 2):(d + 1) * (CQ // 2), :]], axis=0)

    def mlp_tile(t, carry):
        r0 = pl.multiple_of(t * TB, TB)
        ws = t & 1
        count = [0]

        def fresh():
            count[0] += 1
            return lax.rem(t + 2 * count[0], 2)

        def g_rows(r2, p, lo, hi):
            base = (2 * r2 + p) * (FQ + GPAD)
            return slice(base + lo, base + hi)

        rem = {key: rh_s[k] for k, key in enumerate(BLOCKS[:4])}
        for key in BLOCKS[4:8]:
            rem[key] = rem3(*key)
        early = _rows8(rem[BLOCKS[4]], EW[0])
        rem[BLOCKS[8]] = rem3(*BLOCKS[8], pieces=4)
        todo = BLOCKS[9:]
        part = [None] * 7
        for i in O3:
            m = [None] * 7
            for j in J3:
                slot = fresh()
                act = _operand(_LHS[j], lambda r2, k2: _operand(
                    _LHS[i], lambda r1, k1: zf_s[slot, z_rows(2 * r1 + r2, 2 * k1 + k2), :])).astype(BF16)
                if i in _RAW and j in _RAW:
                    d = 2 * _RAW.index(i) + _RAW.index(j)
                    wij = w3_u[d, d * (FQ // 2):(d + 1) * (FQ // 2), :]
                else:
                    wij = s3_u[i, j]
                m[j] = _dot_nt(_as_bf16(wij), act)
            key = todo.pop(0)
            rem[key] = rem3(*key)
            part[i] = _combine(m)
            if i in (4, 3, 0):
                early += _rows8(m[J3[ET[0]]], EW[1]) + _rows8(rem[key] if ET[1] == 7 else m[J3[ET[1]]], EW[2])
        zero = fresh() - ws
        fine = [x for x in early for _ in IN_LOOP]
        fine = fine[:len(fine) - EC * len(IN_LOOP)]
        hop = len(fine) // (len(IN_LOOP) * 33)
        for k, i in enumerate(IN_LOOP):
            w4_ops(i, zero, fine[k * hop:len(fine) - (len(IN_LOOP) - k) * hop])
        for inner in range(4):
            r2, p = inner // 2, inner % 2
            for blk, pre in enumerate(_combine([part[i][inner] for i in range(7)])):
                g_s[blk][ws, g_rows(r2, p, 0, FQ), :] = _gelu2(pre + rem[2 * (blk // 2) + r2, 2 * (blk % 2) + p])

        toks = []
        marks = {}
        part = [[None] * 4 for _ in range(7)]
        for i in _ORDER:
            slot = fresh()
            we = jnp.concatenate([raw4(4 * NS + _RAW.index(i), 2 * _RAW.index(i) + e) if i in _RAW else e4_u[i, e]
                                  for e in range(2)], axis=0)
            ex = []
            for r2 in range(2):
                act = [_operand(_LHS[i], lambda r1, h: g_s[2 * r1 + h][slot, g_rows(r2, p, NS * LANES, FQ), :])
                       for p in range(2)]
                act = jnp.concatenate(act + [jnp.zeros((LANES - 2 * LQ, TQ), F32)], axis=0).astype(BF16)
                ex.append(_dot(_as_bf16(we), act))
            m = [None] * 7
            for j in J4:
                slot = fresh()
                act = _operand(_LHS[j], lambda r2, p: _operand(
                    _LHS[i], lambda r1, h: g_s[2 * r1 + h][slot, g_rows(r2, p, 0, NS * LANES), :])).astype(BF16)
                if i in _RAW and j in _RAW:
                    d = 2 * _RAW.index(i) + _RAW.index(j)
                    wij = [raw4(4 * st + d, d) for st in range(NS)]
                else:
                    wij = [s4_u[i, j, st] for st in range(NS)]
                m[j] = _dot(_as_bf16(jnp.concatenate(wij, axis=1)), act)
                toks += _rows8(m[j])
            part[i] = [x + ex[inner // 2][(inner % 2) * QR:(inner % 2 + 1) * QR]
                       for inner, x in enumerate(_combine(m))]
            marks[i] = len(toks)

        gb = 0.5 * mod_s[NC, 0:1, :]
        nxt = jnp.minimum(t + 1, NT - 1) * TB
        tails = {}
        for i, blk, norm in ((4, 1, (0, NW[0]) + NW[2:4]), (3, 2, NW[0:2] + NW[4:6]), (6, 0, (NW[1], 4) + NW[6:8]),
                             (5, 3, None)):
            r1 = blk // 2
            if norm is None:
                toks += [x for x in lead_in()[8:40] for _ in range(3)]
            else:
                store_z(nxt, 1 - ws, toks[norm[2]:norm[3]], norm[0], norm[1])
            pos = [marks[i] + FL[(1, 2, 0, 3).index(blk)]]

            def finish(rq, c, h2t):
                h2 = hold(h2t.T, toks[pos[0]:pos[0] + TQ // 8])
                pos[0] += TQ // 8
                rows = pl.ds(pl.multiple_of(r0 + rq * TQ, TQ), TQ)
                cols = slice(c * LANES, (c + 1) * LANES)
                o_v[c, rows, :] = (x_s[rows, cols] + gb[:, cols] * (h_s[rows, cols] + h2)).astype(BF16)
                if blk == 3:
                    out_copy(rows.start, TQ, c).start()

            for inner in (1, 2, 0, 3):
                ht = _block([part[k][inner] for k in range(7)], blk)
                rq, c = 2 * r1 + inner // 2, 2 * (blk % 2) + inner % 2
                finish(rq, c, ht[0:LANES])
                tails[rq, c] = ht[LANES:]
            rb = pl.multiple_of(r0 + r1 * 2 * TQ, 2 * TQ)
            if blk != 3:
                for e in range(2):
                    out_copy(rb, 2 * TQ, 2 * (blk % 2) + e).start()
            if blk in (0, 3):
                for rq in (2 * r1, 2 * r1 + 1):
                    finish(rq, NC - 1, jnp.concatenate([tails[rq, c] for c in range(NC - 1)], axis=0))
                if blk == 0:
                    out_copy(rb, 2 * TQ, NC - 1).start()
        return carry

    with jax.named_scope("ph2b"):
        lax.fori_loop(0, NT, mlp_tile, 0)
    with jax.named_scope("tail"):
        pltpu.make_async_copy(o_v, o_v, sem_o.at[0]).wait()


@jax.jit
def pallas_adaLN_cond__ssm_conv_h3__mixer_s_mlp__prompt_kernel(
    A_q: jax.Array,
    A_k: jax.Array,
    A_v: jax.Array,
    A_shift_k: jax.Array,
    A_ssm_k: jax.Array,
    A_ssm_D: jax.Array,
    B_x: jax.Array,
    B_w1: jax.Array,
    B_w2: jax.Array,
    B_w3: jax.Array,
    B_w4: jax.Array,
    c: jax.Array,
    w_mod: jax.Array,
):
    B, S, D = A_q.shape
    FF = B_w3.shape[1]
    assert (B, S, D, FF, A_shift_k.shape[1]) == (1, sum(TILES), 5 * LANES, 1728, 4)
    NC = D // LANES
    NG = BLK // 8
    NBL = S // (PH * BLK)
    NS = FF // 4 // LANES
    n1 = S - sum(TILES[:BLOCKWISE1[0]]) - HALO
    n2 = S - sum(TILES[:BLOCKWISE2[0]])

    args = (A_q.reshape(S, D), A_k.reshape(S, D), A_v.reshape(S, D), A_shift_k.T, A_ssm_k,
            A_ssm_D, B_w1, B_w2, B_w3.T, B_w4, c, w_mod)
    scratch = [
        pltpu.VMEM((S, D), BF16),
        pltpu.VMEM((NC, S + 16, LANES), BF16),
        pltpu.VMEM((NC, S, LANES), BF16),
        pltpu.VMEM((4, D), BF16),
        pltpu.VMEM((NC, LANES, S), BF16),
        pltpu.VMEM((D,), BF16),
        pltpu.VMEM((NC, D, LANES), BF16),
        pltpu.VMEM((NC, D, LANES), BF16),
        pltpu.VMEM((NC, FF, LANES), BF16),
        pltpu.VMEM((NC, FF, LANES), BF16),
        pltpu.VMEM((1, D), BF16),
        pltpu.VMEM((D, 6 * D), BF16),
        pltpu.VMEM((PH, 2 * BLK, BLK), BF16),
        pltpu.VMEM((PH, 2, BLK, BLK), BF16),
        pltpu.VMEM((NC, S, LANES), BF16),
        pltpu.VMEM((NC, NG, NBL, PH, 2, 8, LANES), F32),
        pltpu.VMEM((NC, NG, NBL, PH, 2, 8, LANES), F32),
        pltpu.VMEM((NC, NBL, PH, 2 * BLK, LANES), BF16),
        pltpu.VMEM((6, PH, BLK, LANES), BF16),
        pltpu.VMEM((NC, S, LANES), F32),
        pltpu.VMEM((6, 8, D), F32),
        pltpu.VMEM((NC, 8, LANES), F32),
        pltpu.VMEM((NC, S + 16, LANES), F32),
        pltpu.VMEM((S, D), F32),
        pltpu.VMEM((S, D), F32),
        pltpu.VMEM((NC, S, LANES), BF16),
        pltpu.VMEM((7, 7, FF // 4, LANES), BF16),
        pltpu.VMEM((7, 7, NS, D // 4, LANES), BF16),
        pltpu.VMEM((7, 2, D // 4, LANES), BF16),
        [pltpu.VMEM((2, GROWS, TQ), F32)] * 4,
        pltpu.VMEM((2, 4 * NC * (TQ + 8), LANES), F32),
        pltpu.VMEM((TB, LANES), BF16),
        pltpu.VMEM((10, 2, n1 // 2, LANES), BF16),
        pltpu.VMEM((10, 2, n2 // 2, LANES), BF16),
        pltpu.VMEM((7, 2, 2 * LANES, LANES), BF16),
        pltpu.VMEM((7, 2, 2 * LANES, LANES), BF16),
        pltpu.VMEM((4, FF // 4, TQ), F32),
        pltpu.VMEM((NC, 4 * NS + 2, LANES, LANES), BF16),
        pltpu.VMEM((D, LANES), F32),
        pltpu.SemaphoreType.DMA((21,)),
        pltpu.SemaphoreType.DMA((1,)),
    ]
    out = pl.pallas_call(
        functools.partial(_kernel, S=S, D=D, FF=FF),
        in_specs=[pl.BlockSpec(memory_space=pl.ANY)] * len(args),
        out_specs=pl.BlockSpec(memory_space=pl.ANY),
        out_shape=jax.ShapeDtypeStruct((S, D), BF16),
        scratch_shapes=scratch,
        compiler_params=pltpu.CompilerParams(
            vmem_limit_bytes=120 * 1024 * 1024,
            disable_bounds_checks=True,
            disable_semaphore_checks=True,
        ),
    )(*args)
    return out.reshape(B, S, D)
```

```python
import functools
import math

import jax
import jax.numpy as jnp
from jax import lax
import jax.experimental.pallas as pl
import jax.experimental.pallas.tpu as pltpu

F32 = jnp.float32
BF16 = jnp.bfloat16
U32 = jnp.uint32

LANES = 128
BLK = 128
PH = 4
EPS = 1e-05
TB = 512
TQ = TB // 4
HALO = 32
TILES = (384, 384, 576, 704)
BLOCKWISE1 = (3,)
BLOCKWISE2 = (2, 3)
IN_LOOP = (4, 2, 0, 1, 3)
ROT = 3
KR = 256
NB1 = 1
IG = 2
IJ = 6
IP = 2
GPAD = 8
GROWS = 1768

MF = (6, 0, 5, 4)
MT = (3, 0, 3, 3)
R6 = (36, 18, 28, 6)
TRS = (145, 175, 180)
FRS = (50, 90, 90)
WS = (2, 3, 3, 2, 2, 4)
FI = (48, 88, 96, 96)
LAST = (55, 66, 92, 82)
EW = (2, 1, 2)
NW = (1, 3, 0, 150, 320, 460, 600, 730)
FL = (10, 10, 25, -32)
O3 = (4, 3, 0, 6, 2, 1, 5)
J3 = (1, 2, 3, 4, 5, 6, 0)
J4 = (4, 2, 3, 1, 0, 6, 5)
ET = (0, 4)
EC = 10
YP = 128
LT = (8, 3)

_ORDER = (2, 4, 1, 3, 0, 6, 5)
_RAW = (1, 4)
_LHS = (((0, 0), 1, (1, 1)), ((1, 0), 1, (1, 1)), ((0, 0),), ((1, 1),),
        ((0, 0), 1, (0, 1)), ((1, 0), -1, (0, 0)), ((0, 1), -1, (1, 1)))
_RHS = (((0, 0), 1, (1, 1)), ((0, 0),), ((0, 1), -1, (1, 1)), ((1, 0), -1, (0, 0)),
        ((1, 1),), ((0, 0), 1, (0, 1)), ((1, 0), 1, (1, 1)))


def _operand(terms, blk):
    x = blk(*terms[0])
    if len(terms) > 1:
        y = blk(*terms[2])
        x = x + y if terms[1] > 0 else x - y
    return x


def _all_operands(table, b00, b01, b10, b11):
    blocks = ((b00, b01), (b10, b11))
    return [_operand(terms, lambda i, j: blocks[i][j]) for terms in table]


def _block(m, which):
    if which == 0:
        return (m[3] - m[4]) + m[0] + m[6]
    if which == 1:
        return m[2] + m[4]
    if which == 2:
        return m[1] + m[3]
    return (m[2] - m[1]) + m[0] + m[5]


def _combine(m):
    return [_block(m, which) for which in range(4)]


def _as_bf16(x):
    return pltpu.bitcast(x, BF16)


def _lo(x):
    return pltpu.bitcast(x << 16, F32)


def _hi(x):
    return pltpu.bitcast(x & jnp.uint32(0xFFFF0000), F32)


def _dft4(re, im, sign):
    ar, ai = re[0] + re[2], im[0] + im[2]
    br, bi = re[0] - re[2], im[0] - im[2]
    cr, ci = re[1] + re[3], im[1] + im[3]
    dr, di = re[1] - re[3], im[1] - im[3]
    o0 = (ar + cr, ai + ci)
    o2 = (ar - cr, ai - ci)
    m = (br + di, bi - dr)
    p = (br - di, bi + dr)
    o1, o3 = (m, p) if sign < 0 else (p, m)
    return [o0[0], o1[0], o2[0], o3[0]], [o0[1], o1[1], o2[1], o3[1]]


def _ln(x, eps=EPS, unit=True):
    n = x.shape[-1]
    s1 = jnp.sum(x, axis=-1, keepdims=True)
    m = s1 * (1.0 / n)
    v = jnp.maximum(jnp.sum(x * x, axis=-1, keepdims=True) + (n * eps - s1 * m), n * eps)
    e = jnp.log(v) * (-0.5 / math.log(2.0))
    return (x - m) * jnp.exp2(e + 0.5 * math.log2(n) if unit else e)


def _gelu2(x):
    c0 = math.sqrt(2.0 / math.pi)
    return x + x * jnp.tanh(x * (c0 + (c0 * 0.044715) * (x * x)))


def _dot(a, b):
    return jnp.dot(a, b, preferred_element_type=F32)


def _dot_nt(a, b):
    return lax.dot_general(a, b, (((1,), (1,)), ((), ())), preferred_element_type=F32)


def _rows8(x, repeat=1):
    return [x[8 * r:8 * r + 8, 0:LANES] for r in range(x.shape[0] // 8) for _ in range(repeat)]


def _chunks(r0, r1, k, unit=16):
    n = (r1 - r0) // unit
    cuts = [r0 + unit * ((n * j) // k) for j in range(k + 1)]
    return list(zip(cuts[:-1], cuts[1:]))


def _pick(toks, n, free=0):
    idx = [(r * (len(toks) + free)) // n - free for r in range(n)]
    return [toks[i] if i >= 0 else None for i in idx]


def _kernel(q_hbm, k_hbm, v_hbm, sh_hbm, sk_hbm, sd_hbm, w1_hbm, w2_hbm, w3_hbm, w4_hbm, c_hbm, wm_hbm,
            o_hbm,
            q_v, k_v, v_v, sh_v, sk_v, sd_v, w1_v, w2_v, w3_v, w4_v, c_v, wm_v,
            fw_s, iv_s, o_v, u_s, kk_s, vv_s, wu_s, y_s, mod_s, par_s, h1_s, x_s, h_s, z_s,
            s3_s, s4_s, e4_s, g_s, zf_s, zr_s, l1_s, l2_s, s1_s, s2_s, rh_s, wt_s, scol_s,
            sem, sem_o,
            *, S, D, FF):
    NC = D // LANES
    NG = BLK // 8
    LB = PH * BLK
    NBL = S // LB
    R = BLK // PH
    HL = LANES // 2

    small = [
        pltpu.make_async_copy(sh_hbm, sh_v, sem.at[0]),
        pltpu.make_async_copy(sd_hbm, sd_v, sem.at[0]),
        pltpu.make_async_copy(c_hbm, c_v, sem.at[0]),
    ]

    def sk_copy(c):
        ch = (c + ROT) % NC * LANES
        rows = pl.ds(ch if isinstance(c, int) else pl.multiple_of(ch, LANES), LANES)
        return [pltpu.make_async_copy(sk_hbm.at[rows, :], sk_v.at[c], sem.at[1 + c])]

    def kv_copies(tiles, lo, hi, s):
        return [pltpu.make_async_copy(src.at[pl.ds(r0, r1 - r0), pl.ds((c + ROT) % NC * LANES, LANES)],
                                      dst.at[c, pl.ds(off + r0, r1 - r0), :], sem.at[s])
                for r0, r1 in _chunks(lo, hi, (hi - lo + 16) // KR)
                for src, dst, off in ((k_hbm, k_v, 16), (v_hbm, v_v, 0)) for c in tiles]

    PAIR, TRIPLE = (0, 1), (2, 3, 4)
    kv_groups = [kv_copies(PAIR, 0, NB1 * LB + 16, 9), kv_copies(PAIR, NB1 * LB + 16, S, 10),
                 kv_copies(TRIPLE, 0, 2 * LB + 16, 11), kv_copies(TRIPLE, 2 * LB + 16, S, 20)]

    WM = (0, 3 * D, 5 * D, 6 * D)
    wm_copies = [[pltpu.make_async_copy(wm_hbm.at[:, pl.ds(WM[j], WM[j + 1] - WM[j])],
                                        wm_v.at[:, pl.ds(WM[j], WM[j + 1] - WM[j])], sem.at[6 + j])]
                 for j in range(3)]
    w_copies = [[pltpu.make_async_copy(src.at[:, pl.ds(c * LANES, LANES)], dst.at[c], sem.at[12 + j])
                 for c in range(NC)]
                for j, (src, dst) in enumerate(((w1_hbm, w1_v), (w2_hbm, w2_v), (w3_hbm, w3_v), (w4_hbm, w4_v)))]

    B0 = [0]
    for n in TILES:
        B0.append(B0[-1] + n)
    NA = len(TILES)
    A0 = [0] + [r + HALO for r in B0[1:-1]] + [S]
    q_copies = [
        [pltpu.make_async_copy(q_hbm.at[pl.ds(A0[t], A0[t + 1] - A0[t])], q_v.at[pl.ds(A0[t], A0[t + 1] - A0[t])],
                               sem.at[16 + t])]
        for t in range(NA)
    ]

    def start_all(cps, priority=0):
        for cp in cps:
            cp.start(priority=priority)

    def wait_all(cps):
        for cp in cps:
            cp.wait()

    for c in range(NC):
        k_v[c, 0:16, :] = jnp.zeros((16, LANES), BF16)
    start_all(sk_copy(0) + small + sk_copy(1) + kv_groups[0] + kv_groups[1] + sk_copy(2))

    for c in range(NC):
        h1_s[c, 0:8, :] = jnp.zeros((8, LANES), F32)
        h1_s[c, S + 8:S + 16, :] = jnp.zeros((8, LANES), F32)

    prow = lax.broadcasted_iota(jnp.int32, (BLK, BLK), 0)
    pcol = lax.broadcasted_iota(jnp.int32, (BLK, BLK), 1)
    ang = (((4 * prow + 1) * pcol) & (4 * BLK - 1)).astype(F32) * (2.0 * math.pi / (4 * BLK))
    tw = (4 * prow + 1).astype(F32) * (2.0 * math.pi / (4 * LB))
    mr, mi = jnp.cos(ang), -jnp.sin(ang)
    twr, twi = jnp.cos(tw), -jnp.sin(tw)
    eye = jnp.where(prow == pcol, 1.0 / LB, 0.0).astype(BF16)
    for i in range(PH):
        both = jnp.stack([mr.reshape(NG, 8, BLK), mi.reshape(NG, 8, BLK)], axis=1).reshape(2 * BLK, BLK)
        fw_s[i] = both.astype(BF16)
        for h in range(2):
            iv_s[i, h] = _dot_nt(eye, both[h * BLK:(h + 1) * BLK, :].astype(BF16)).astype(BF16)
        if i + 1 < PH:
            mr, mi = mr * twr - mi * twi, mr * twi + mi * twr
    perm = jnp.where(pcol == (prow % R) * PH + prow // R, 1.0, 0.0).astype(BF16)

    wait_all(small)
    shf = sh_v[...].astype(F32)
    sdf = sd_v[...].astype(F32).reshape(1, D)
    for c in range(NC):
        par_s[(c - ROT) % NC, 0:4, :] = shf[:, c * LANES:(c + 1) * LANES]
        par_s[(c - ROT) % NC, 4:5, :] = sdf[:, c * LANES:(c + 1) * LANES]
    cf = c_v[...].astype(F32)
    sc = (cf * jax.nn.sigmoid(cf)).astype(BF16)
    sc16 = jnp.broadcast_to(sc, (16, D))

    def mod_chunk(j):
        mod_s[j] = _dot(sc16, wm_v[:, j * D:(j + 1) * D])[0:8, :]

    (fw_u, iv_u, k_u, v_u, wu_u, vv_u, z_u, l1_u, l2_u, w1_u, w2_u, s1_u, s2_u, w3_u, w4_u, wt_u, s3_u, s4_u,
     e4_u, zr_u) = (r.bitcast(U32) for r in (fw_s, iv_s, k_v, v_v, wu_s, vv_s, z_s, l1_s, l2_s, w1_v, w2_v,
                                             s1_s, s2_s, w3_v, w4_v, wt_s, s3_s, s4_s, e4_s, zr_s))

    never = twr[0:8, :] > 2.0

    def after(token, x):
        if token.dtype != x.dtype:
            token = pltpu.bitcast(token, x.dtype)
        return jnp.where(jnp.broadcast_to(never, x.shape), token, x)

    def hold(x, tks):
        f = len([k for k in tks if k is None])
        n = len(tks)
        head = after(jnp.stack(tks[f:]), x[8 * f:, 0:LANES].reshape(n - f, 8, LANES)).reshape(8 * (n - f), LANES)
        if f:
            head = jnp.concatenate([x[:8 * f, 0:LANES], head], axis=0)
        return head if x.shape[1] == LANES else jnp.concatenate([head, x[:, LANES:]], axis=1)

    def hold16(x, tks):
        x4 = x.reshape(len(tks), 2, 8, LANES)
        return jnp.stack([after(jnp.stack(tks), x4[:, 0]), x4[:, 1]], axis=1).reshape(x.shape)

    def perm_k(c, b, toks):
        kt = [_dot_nt(perm, sk_v[c, :, b * LB + t * BLK:b * LB + (t + 1) * BLK]) for t in range(PH)]
        toks += _rows8(kt[0])[::2]
        return [jnp.concatenate([kt[t][i * R:(i + 1) * R, :] for t in range(PH)], axis=0).astype(BF16)
                for i in range(PH)]

    def spectrum(comps, dst, slot, b, toks, dc=None, pins=None):
        tr, ti = [], []
        for i in range(PH):
            lhs = fw_u[i]
            if pins is not None and i < len(pins):
                lhs = after(pins[i], lhs.reshape(NG, 8, LANES)).reshape(BLK, LANES)
            t4 = _dot(_as_bf16(lhs), comps[i]).reshape(NG, 2, 8, LANES)
            tr.append(t4[:, 0])
            ti.append(t4[:, 1])
        toks += [ti[PH - 1][g] for g in range(NG)]
        if dc is not None:
            tr[0] = tr[0] + dc
        sr, si = _dft4(tr, ti, -1)
        for qq in range(PH):
            dst[slot, :, b, qq, 0] = sr[qq]
            dst[slot, :, b, qq, 1] = si[qq]

    def gated(c, b, n):
        w = [par_s[c, t:t + 1, :] for t in range(4)]
        kc = {}
        for o in range(-2, 2):
            words = k_u[c, pl.ds(8 + b * (LB // 2) + o, BLK, stride=2), :]
            if o > -2:
                kc[2 * o] = _lo(words)
            kc[2 * o + 1] = _hi(words)
        vc = {}
        for o in range(2):
            words = v_u[c, pl.ds(b * (LB // 2) + o, BLK, stride=2), :]
            vc[2 * o] = _lo(words)
            vc[2 * o + 1] = _hi(words)
        for i in range(PH):
            ks = kc[i] * w[0]
            for t in range(1, 4):
                ks = ks + kc[i - t] * w[t]
            wu_s[n, i] = (ks * vc[i]).astype(BF16)
        return [wu_u[n, i] for i in range(PH)]

    def kv_pins(kvb):
        return [jnp.stack([kvb[2 * m + (r % 2)][8 * (r // 2):8 * (r // 2) + 8, :] for r in range(NG)])
                for m in range(2)]

    def products(c, ks, kc, toks, free, trim):
        n = len(toks) - trim + free
        cum = (44, 128, 244, 392)
        zp = None
        for o in range(NBL):
            idx = [((g * cum[-1] + cum[o]) * n) // (cum[-1] * NG) - 1 - free for g in range(NG)]
            tk = [toks[max(i, 0)] if i >= 0 or not free else None for i in idx]
            zr, zi = [], []
            for qq in range(PH):
                accr = acci = None
                for b in range(o + 1):
                    a_, b_ = u_s[c, :, b, qq, 0], u_s[c, :, b, qq, 1]
                    c_, d_ = ks[kc, :, o - b, qq, 0], ks[kc, :, o - b, qq, 1]
                    if qq == 0 and b == o:
                        a_ = hold(a_.reshape(BLK, LANES), tk).reshape(NG, 8, LANES)
                    tr_ = a_ * c_ - b_ * d_
                    ti_ = a_ * d_ + b_ * c_
                    accr = tr_ if accr is None else accr + tr_
                    acci = ti_ if acci is None else acci + ti_
                zr.append(accr)
                zi.append(acci)
            if zp is None:
                yr, yi = zr, zi
            else:
                yr = [zr[qq] - zp[1][qq] for qq in range(PH)]
                yi = [zi[qq] + zp[0][qq] for qq in range(PH)]
            zp = (zr, zi)
            vr, vi = _dft4(yr, yi, +1)
            for i in range(PH):
                vv_s[c, o, i] = jnp.stack([vr[i], vi[i]], axis=1).reshape(2 * BLK, LANES).astype(BF16)

    def inverse(c, o, toks, pins):
        for i in range(PH):
            yv = None
            for h in range(2):
                lhs = iv_u[i, h]
                if pins is not None and h == 0:
                    pin = pins[i % 2][8 * (i // 2):8 * (i // 2) + 8]
                    lhs = after(pin, lhs.reshape(8, 8, LANES)).reshape(HL, LANES)
                t = _dot(_as_bf16(lhs), _as_bf16(vv_u[c, o, i, h * HL:(h + 1) * HL, :]))
                yv = t if yv is None else yv + t
            if i % 2 == 0:
                toks += _rows8(yv)[::2]
            y_s[c, pl.ds(o * LB + i, BLK, stride=PH), :] = yv

    def conv_step(filt=None, units=(), mul=None, inv=(), free=0, trim=3):
        toks = []
        kv = [gated(c, b, n) for n, (c, b) in enumerate(units)]
        pin_at = {n: kv_pins(kv[n]) for n in range(len(units))} if inv or filt is not None else {}
        if filt is not None and mul is not None and not isinstance(filt, int):
            ks = kk_s.at[pl.ds(mul, 2)]
            k_rd, k_wr = (ks, 0), (ks, 1)
        else:
            k_rd, k_wr = (kk_s, mul), (kk_s, filt)
        pos = 0
        for c, o in inv:
            inverse(c, o, toks, pin_at.get(pos))
            pos += 1
        if filt is not None:
            comps = [perm_k(filt, b, toks) for b in range(NBL)]
            for b in range(NBL):
                spectrum(comps[b], *k_wr, b, toks, par_s[filt, 4:5, :] if b == 0 else None, pin_at.get(pos))
                pos += 1
        for n, (c, b) in enumerate(units):
            spectrum([_as_bf16(x) for x in kv[n]], u_s, c, b, toks, None, pin_at.get(pos))
            pos += 1
        if mul is not None:
            products(mul, *k_rd, toks, free, trim)
        return toks

    def lane_tiles(x):
        return [x[:, c * LANES:(c + 1) * LANES] for c in range(NC)]

    def stage_p1(r0, r1, tks=None, ytks=None):
        ga = mod_s[2, 0:1, :]
        a_mul, a_add = ga * (1.0 + mod_s[1, 0:1, :]) * math.sqrt(D), ga * mod_s[0, 0:1, :]
        q = q_v[r0:r1, :].astype(F32)
        if tks is not None:
            q = hold(q, tks)
        y = jnp.concatenate([y_s[(c - ROT) % NC, r0:r1, :] for c in range(NC)], axis=1)
        if ytks is not None:
            y = hold(y, ytks)
        x = q + (_ln(q, unit=False) * a_mul + a_add) * y
        x_s[r0:r1, :] = x
        return _ln(x, unit=False)

    def store_row_ops(dst, base, r0, r1, cols, tks=None):
        hv = []
        for x in cols:
            x4 = x.reshape(x.shape[0] // 32, 2, 16, LANES)
            hv.append([x4[:, e].reshape(x.shape[0] // 2, LANES) for e in range(2)])
        for k2 in range(2):
            a00, a01, a10, a11 = hv[k2][0], hv[2 + k2][0], hv[k2][1], hv[2 + k2][1]
            if tks is not None:
                a00, a11 = hold16(a00, tks), hold16(a11, tks)
            for o, x in enumerate(_all_operands(_LHS, a00, a01, a10, a11) + [a01, a10, hv[NC - 1][k2]]):
                dst[o, k2, (r0 - base) // 2:(r1 - base) // 2, :] = x.astype(BF16)

    L1B = A0[BLOCKWISE1[0]]
    L2B = B0[BLOCKWISE2[0]]

    def stage_p2(r0, r1, nx, blockwise=False):
        h = nx * ((1.0 + mod_s[4, 0:1, :]) * (2.0 * math.sqrt(D))) + 2.0 * mod_s[3, 0:1, :]
        h_s[r0:r1, :] = h
        zn = lane_tiles(_ln(h, 4.0 * EPS))
        if blockwise:
            store_row_ops(l1_s, L1B, r0, r1, zn)
        else:
            for c in range(NC):
                z_s[c, r0:r1, :] = zn[c].astype(BF16)

    def stage_p(t, toks):
        lo, hi = A0[t], A0[t + 1]
        stage_p2(lo, hi, stage_p1(lo, hi, _pick(toks[:-TRS[t - 1]], (hi - lo) // 8, FRS[t - 1])), t in BLOCKWISE1)

    def filler(t):
        red = jnp.sum(y_s[t, 0:8 * FI[t], :], axis=-1, keepdims=True).reshape(FI[t], 8, 1)
        spare = (NC - 1) * (TQ + 8) + 8 * t
        zf_s[1, spare:spare + 8, :] = jnp.broadcast_to(jnp.sum(red, axis=0), (8, LANES))

    def square_ops(src, dst, toks):
        HK = 2 * LANES
        tks = _pick(toks, 2 * HK // 16)
        for n2 in range(2):
            tk = tks[n2 * (HK // 16):(n2 + 1) * (HK // 16)]
            blk = lambda k, n: src[2 * n + n2, k * HK:(k + 1) * HK, :].astype(F32)
            for o, x in enumerate(_all_operands(_RHS, hold16(blk(0, 0), tk), blk(0, 1), blk(1, 0), hold16(blk(1, 1), tk))):
                if o not in _RAW:
                    dst[o, n2] = x.astype(BF16)

    def block_dots(ops_u, base, prepare, w_u, s_u, parts, emit, light, heavy):
        toks = []

        def timed(x, weight):
            toks.extend(_rows8(x, weight))
            return x

        def weave(top, bot):
            n = top.shape[0] // 16
            return jnp.stack([top.reshape(n, 16, LANES), bot.reshape(n, 16, LANES)], axis=1).reshape(32 * n, LANES)

        def main(get):
            m = [None] * 7
            rem = [None, None]
            for o in ('t', 2, 4, 'b', 1, 3, 0, 6, 5):
                if o in ('t', 'b'):
                    e = 0 if o == 't' else 1
                    rhs = jnp.concatenate([w_u[c, 2 * LANES:D // 2, :] for c in range(NC - 1)], axis=1)
                    rem[e] = timed(_dot(get([(9, e)]), _as_bf16(rhs)), light)
                    continue
                if o in _RAW:
                    d = _RAW.index(o)
                    rhs = jnp.concatenate([w_u[2 * d + n2, d * LANES:(d + 1) * LANES, :] for n2 in range(2)], axis=1)
                else:
                    rhs = jnp.concatenate([s_u[o, n2] for n2 in range(2)], axis=1)
                m[o] = timed(_dot(get([(o, 0), (o, 1)]), _as_bf16(rhs)), heavy if o in (4, 3, 6, 5) else light)
            c00, c01, c10, c11 = _combine(m)
            top = jnp.concatenate([c00, c01], axis=1) + rem[0]
            bot = jnp.concatenate([c10, c11], axis=1) + rem[1]
            return [weave(top[:, c * LANES:(c + 1) * LANES], bot[:, c * LANES:(c + 1) * LANES]) for c in range(NC - 1)]

        def last(get):
            w = _as_bf16(w_u[NC - 1])
            return weave(timed(_dot(get([(2, 0), (2, 1), (7, 0), (7, 1), (9, 0)]), w), light),
                         timed(_dot(get([(8, 0), (8, 1), (3, 0), (3, 1), (9, 1)]), w), light))

        mark = None
        for j, (r0, r1) in enumerate(parts):
            prepare(r0, r1, None if mark is None else toks[mark:])
            mark = len(toks)
            get = lambda keys: _as_bf16(jnp.concatenate(
                [ops_u[o, e, (r0 - base) // 4:(r1 - base) // 4, :] for o, e in keys], axis=1))
            if j % 2:
                tail = last(get)
                emit(r0, r1, main(get) + [tail])
            else:
                emit(r0, r1, main(get) + [last(get)])
        return toks

    def stage_m1(t, k):
        def emit(r0, r1, cols):
            out = [_gelu2(x) for x in cols]
            for c in range(NC):
                h1_s[c, r0 + 8:r1 + 8, :] = out[c]
            return out

        if t in BLOCKWISE1:
            return block_dots(l1_u, L1B, lambda *_: None, w1_u, s1_u, _chunks(A0[t], A0[t + 1], k, 32), emit, WS[2], WS[3])
        toks = []
        for r0, r1 in _chunks(A0[t], A0[t + 1], k):
            lhs = jnp.concatenate([z_u[c, r0 // 2:r1 // 2, :] for c in range(NC)], axis=1)
            w = jnp.concatenate([w1_u[c] for c in range(NC)], axis=1)
            for x in emit(r0, r1, lane_tiles(_dot(_as_bf16(lhs), _as_bf16(w)))):
                toks += _rows8(x, WS[0])
        return toks

    def shifted(r0, r1):
        n, grp, shifts = r1 - r0, D // 4, (-1, 1, -2, 2)
        lane = lax.broadcasted_iota(jnp.int32, (n, LANES), 1)
        cols = []
        for c in range(NC):
            lo, hi = c * LANES, (c + 1) * LANES
            g_lo, g_hi = lo // grp, (hi - 1) // grp
            val = h1_s[c, pl.ds(r0 + 8 + shifts[g_lo], n), :]
            if g_hi != g_lo:
                other = h1_s[c, pl.ds(r0 + 8 + shifts[g_hi], n), :]
                val = jnp.where(lane < (g_hi * grp - lo), val, other)
            cols.append(val)
        return cols

    def stage_m2(t, k, before=None):
        def emit(r0, r1, cols):
            x1 = h_s[r0:r1, :] + jnp.concatenate(cols, axis=1)
            h_s[r0:r1, :] = x1
            return x1

        if t in BLOCKWISE2:
            def prepare(r0, r1, prev):
                prev = before if prev is None else prev
                prev = prev[len(prev) // 8:(len(prev) * 7) // 8]
                store_row_ops(l2_s, L2B, r0, r1, shifted(r0, r1), _pick(prev, (r1 - r0) // 32))
            return block_dots(l2_u, L2B, prepare, w2_u, s2_u, _chunks(B0[t], B0[t + 1], k, 32), emit, WS[4], WS[4])
        toks = []
        for r0, r1 in _chunks(B0[t], B0[t + 1], k):
            w = jnp.concatenate([w2_u[c] for c in range(NC)], axis=1)
            hs = _dot(jnp.concatenate(shifted(r0, r1), axis=1).astype(BF16), _as_bf16(w))
            for x in lane_tiles(emit(r0, r1, [hs])):
                toks += _rows8(x, WS[1])
        return toks

    NT = S // TB
    FQ = FF // 4
    NS = FQ // LANES
    LQ = FQ - NS * LANES
    CQ = LANES // 4
    QR = LANES + CQ
    BLOCKS = [(2 * r1 + r2, 2 * h + p)
              for r1, h in ((0, 0), (1, 0), (0, 1), (1, 1)) for r2 in range(2) for p in range(2)]

    def z_rows(rq, c):
        lo = (NC * rq + c) * (TQ + 8)
        return slice(lo, lo + TQ)

    def store_z(r0, slot, toks, q0=0, q1=4):
        n = (q1 - q0) * TQ
        rows = pl.ds(r0 + q0 * TQ if isinstance(r0, int) else pl.multiple_of(r0 + q0 * TQ, TQ), n)
        zn = lane_tiles(_ln(hold(h_s[rows, :], _pick(toks, n // 8)), 4.0 * EPS))
        for rq in range(q0, q1):
            for c in range(NC - 1):
                zf_s[slot, z_rows(rq, c), :] = zn[c][(rq - q0) * TQ:(rq - q0 + 1) * TQ]
        zr_s[q0 * TQ:q1 * TQ, :] = zn[NC - 1].astype(BF16)

    def w3_ops(toks):
        ng = FQ // 16
        blk = lambda c, d: w3_v[c, d * FQ:(d + 1) * FQ, :].astype(F32)
        outer = [[_all_operands(_RHS, blk(k2, p), blk(k2, 2 + p), blk(2 + k2, p), blk(2 + k2, 2 + p))
                  for p in range(2)] for k2 in range(2)]
        for k, i in enumerate((1, 5, 2, 4, 0, 3, 6)):
            tk = [toks[((k + r * 7) * len(toks)) // (7 * ng)] for r in range(ng)]
            for j, x in enumerate(_all_operands(_RHS, hold16(outer[0][0][i], tk), outer[0][1][i], outer[1][0][i],
                                                hold16(outer[1][1][i], tk))):
                if i not in _RAW or j not in _RAW:
                    s3_s[i, j] = x.astype(BF16)

    def transpose_w4(toks):
        order = [(c, n) for n in (4 * NS, 4 * NS + 1) + tuple(range(4 * NS)) for c in range(NC)]
        for k, (c, n) in enumerate(order):
            if n >= 4 * NS:
                ends = [(2 * (n - 4 * NS) + p + 1) * FQ // 2 for p in range(2)]
                x = jnp.concatenate([w4_u[c, e - LQ // 2:e, :] for e in ends]
                                    + [jnp.zeros((HL - LQ, LANES), U32)], axis=0)
            else:
                lo = (n % 4) * FQ // 2 + (n // 4) * HL
                x = w4_u[c, lo:lo + HL, :]
            x = jnp.concatenate([after(toks[(k * len(toks)) // len(order)], x[0:8]), x[8:]], axis=0)
            wt_s[c, n] = _as_bf16(x).astype(F32).T.astype(BF16)

    def w4_ops(i, zero, toks):
        ng = QR // 16
        total = (NS * 7 + 2) * ng
        tk = lambda pos, step: [toks[((pos + r * step) * len(toks)) // total] for r in range(ng)]
        quarter = lambda n, d: jnp.concatenate(
            [wt_s[d, n].astype(F32), wt_s[NC - 1, n, d * CQ:(d + 1) * CQ, :].astype(F32)], axis=0)
        if i not in _RAW:
            for e in range(2):
                x = _operand(_RHS[i], lambda h, d: quarter(4 * NS + h, 2 * d + e))
                e4_s[i + zero, e] = hold16(x, tk(e * ng, 1)).astype(BF16)
        for st in range(NS):
            t = [[_operand(_RHS[i], lambda h, d: quarter(4 * st + 2 * h + p, 2 * d + e)) for e in range(2)]
                 for p in range(2)]
            tks = tk((2 + st * 7) * ng, 7)
            for j, x in enumerate(_all_operands(_RHS, hold16(t[0][0], tks), t[0][1], t[1][0], hold16(t[1][1], tks))):
                if i not in _RAW or j not in _RAW:
                    s4_s[i + zero, j, st] = x.astype(BF16)

    def gate_row(toks):
        ng = D // 8
        col = after(jnp.stack(_pick(toks, ng)), scol_s[...].reshape(ng, 8, LANES))
        for c in range(NC):
            wf = wm_v[:, (NC * NC + c) * LANES:(NC * NC + c + 1) * LANES].astype(F32).reshape(ng, 8, LANES)
            acc = col[0] * wf[0]
            for r in range(1, ng):
                acc = acc + col[r] * wf[r]
            mod_s[NC, :, c * LANES:(c + 1) * LANES] = jnp.broadcast_to(jnp.sum(acc, axis=0, keepdims=True), (8, LANES))

    def rem3(rq, d, pieces=1):
        z = _as_bf16(zr_u[rq * (TQ // 2):(rq + 1) * (TQ // 2), :])
        return jnp.concatenate([_dot_nt(_as_bf16(w3_u[NC - 1, lo // 2:hi // 2, :]), z)
                                for lo, hi in _chunks(d * FQ, (d + 1) * FQ, pieces)], axis=0)

    def lead_in():
        head = [rem3(*key) for key in BLOCKS[:4]]
        for k in range(4):
            rh_s[k] = head[k]
        return _rows8(head[0])

    def units(tiles, blocks):
        return [(c, b) for b in blocks for c in tiles]

    with jax.named_scope("A"):
        wait_all(sk_copy(0))
        conv_step(filt=0)
    with jax.named_scope("B_wait"):
        wait_all(sk_copy(1) + kv_groups[0])
    with jax.named_scope("B"):
        start_all(kv_groups[2] + kv_groups[3] + sk_copy(3) + sk_copy(4))
        conv_step(filt=1, units=units(PAIR, range(0, NB1)))
        scol_s[...] = jnp.broadcast_to(sc.astype(F32), (LANES, D)).T
    with jax.named_scope("C_wait"):
        wait_all(kv_groups[1])
    with jax.named_scope("C"):
        conv_step(units=units(PAIR, range(NB1, NBL)))
    with jax.named_scope("D_wait"):
        wait_all(sk_copy(2))
    with jax.named_scope("D"):
        start_all(wm_copies[0] + q_copies[0] + wm_copies[1] + w_copies[0])
        conv_step(filt=2, mul=0, free=MF[0], trim=MT[0])
    with jax.named_scope("E_wait"):
        wait_all(kv_groups[2])
    with jax.named_scope("E"):
        conv_step(units=units(TRIPLE, range(0, 2)), mul=1, inv=units((0,), range(NBL)), free=MF[1], trim=MT[1])
    with jax.named_scope("F_wait"):
        wait_all(kv_groups[3])
    with jax.named_scope("F"):
        conv_step(units=units(TRIPLE, range(2, NBL)))

    def full_step(j, carry):
        wait_all(sk_copy(j + 2))
        conv_step(filt=j + 2, mul=j + 1, inv=units((j,), range(IG)), free=MF[2], trim=MT[2])
        return carry

    with jax.named_scope("GH"):
        lax.fori_loop(1, NC - 2, full_step, 0)
    late = units((NC - 2,), range(NBL)) + units(range(1, NC - 2), range(IG, NBL))
    late = late[:IJ] + units((NC - 1,), range(NBL)) + late[IJ:]
    with jax.named_scope("J"):
        start_all(q_copies[1] + w_copies[1] + sum(q_copies[2:], []) + w_copies[2] + w_copies[3] + wm_copies[2], 1)
        conv_step(mul=NC - 1, inv=late[:IJ], free=MF[3], trim=MT[3])
    with jax.named_scope("r6_wait"):
        wait_all(wm_copies[0] + q_copies[0])
    with jax.named_scope("r6"):
        for j in range(3):
            mod_chunk(j)
        conv_step(inv=late[IJ:IJ + 1])
        toks = conv_step(inv=late[IJ + 1:len(late) - IP])
        nx0 = stage_p1(0, A0[1], None, _pick(toks[:R6[0]], A0[1] // 8, R6[1]) if toks else None)
    with jax.named_scope("p2_wait"):
        wait_all(wm_copies[1])
    with jax.named_scope("p2"):
        mod_chunk(4)
        mod_chunk(3)
        toks = conv_step(inv=late[len(late) - IP:])
        if toks:
            nx0 = hold(nx0, _pick(toks[:R6[2]], A0[1] // 8, R6[3]))
        stage_p2(0, A0[1], nx0)
    with jax.named_scope("w1_wait"):
        wait_all(w_copies[0])
    with jax.named_scope("m1_0"):
        square_ops(w1_v, s1_s, stage_m1(0, 4)[:-40])
    with jax.named_scope("w2_wait"):
        wait_all(q_copies[1] + w_copies[1])
    with jax.named_scope("m2_0"):
        stage_p(1, stage_m2(0, 4))
        filler(0)
    for t in range(1, NA):
        with jax.named_scope("a%d" % t):
            wait_all(q_copies[t + 1] if t + 1 < NA else w_copies[2] + w_copies[3] + wm_copies[2])
            toks = stage_m1(t, 2)
            toks = toks + stage_m2(t, 2, toks[len(toks) - len(toks) // 2:])
            if t + 1 < NA:
                stage_p(t + 1, toks)
            if t == 1:
                square_ops(w2_v, s2_s, toks[:-30])
            if t == NA - 1:
                transpose_w4(toks[:(len(toks) * LAST[0]) // 100])
                store_z(0, 0, toks[(len(toks) * LAST[1]) // 100:(len(toks) * LAST[2]) // 100])
                toks = toks + [x for x in lead_in()[:40] for _ in range(WS[5])]
                cut = (len(toks) * LAST[3]) // 100
                gate_row(toks[:(len(toks) * 9) // 10])
                w3_ops(toks[:cut])
                rest = [i for i in range(7) if i not in IN_LOOP]
                for k, i in enumerate(rest):
                    w4_ops(i, 0, toks[cut + k::len(rest)])
            filler(t)

    def out_copy(r0, n, c):
        rows = pl.ds(r0, n)
        return pltpu.make_async_copy(o_v.at[c, rows, :], o_hbm.at[rows, pl.ds(c * LANES, LANES)], sem_o.at[0])

    def raw4(n, d):
        return jnp.concatenate([wt_u[d, n], wt_u[NC - 1, n, d * (CQ // 2):(d + 1) * (CQ // 2), :]], axis=0)

    def mlp_tile(t, carry):
        r0 = pl.multiple_of(t * TB, TB)
        ws = t & 1
        count = [0]

        def fresh():
            count[0] += 1
            return lax.rem(t + 2 * count[0], 2)

        def g_rows(r2, p, lo, hi):
            base = (2 * r2 + p) * (FQ + GPAD)
            return slice(base + lo, base + hi)

        rem = {key: rh_s[k] for k, key in enumerate(BLOCKS[:4])}
        for key in BLOCKS[4:8]:
            rem[key] = rem3(*key)
        early = _rows8(rem[BLOCKS[4]], EW[0])
        rem[BLOCKS[8]] = rem3(*BLOCKS[8], pieces=4)
        todo = BLOCKS[9:]
        part = [None] * 7
        for i in O3:
            m = [None] * 7
            for j in J3:
                slot = fresh()
                act = _operand(_LHS[j], lambda r2, k2: _operand(
                    _LHS[i], lambda r1, k1: zf_s[slot, z_rows(2 * r1 + r2, 2 * k1 + k2), :])).astype(BF16)
                if i in _RAW and j in _RAW:
                    d = 2 * _RAW.index(i) + _RAW.index(j)
                    wij = w3_u[d, d * (FQ // 2):(d + 1) * (FQ // 2), :]
                else:
                    wij = s3_u[i, j]
                m[j] = _dot_nt(_as_bf16(wij), act)
            key = todo.pop(0)
            rem[key] = rem3(*key)
            part[i] = _combine(m)
            if i in (4, 3, 0):
                early += _rows8(m[J3[ET[0]]], EW[1]) + _rows8(rem[key] if ET[1] == 7 else m[J3[ET[1]]], EW[2])
        zero = fresh() - ws
        fine = [x for x in early for _ in IN_LOOP]
        fine = fine[:len(fine) - EC * len(IN_LOOP)]
        hop = len(fine) // (len(IN_LOOP) * 33)
        for k, i in enumerate(IN_LOOP):
            w4_ops(i, zero, fine[k * hop:len(fine) - (len(IN_LOOP) - k) * hop])
        for inner in range(4):
            r2, p = inner // 2, inner % 2
            for blk, pre in enumerate(_combine([part[i][inner] for i in range(7)])):
                g_s[blk][ws, g_rows(r2, p, 0, FQ), :] = _gelu2(pre + rem[2 * (blk // 2) + r2, 2 * (blk % 2) + p])

        toks = []
        marks = {}
        part = [[None] * 4 for _ in range(7)]
        for i in _ORDER:
            slot = fresh()
            we = jnp.concatenate([raw4(4 * NS + _RAW.index(i), 2 * _RAW.index(i) + e) if i in _RAW else e4_u[i, e]
                                  for e in range(2)], axis=0)
            ex = []
            for r2 in range(2):
                act = [_operand(_LHS[i], lambda r1, h: g_s[2 * r1 + h][slot, g_rows(r2, p, NS * LANES, FQ), :])
                       for p in range(2)]
                act = jnp.concatenate(act + [jnp.zeros((LANES - 2 * LQ, TQ), F32)], axis=0).astype(BF16)
                ex.append(_dot(_as_bf16(we), act))
            m = [None] * 7
            for j in J4:
                slot = fresh()
                act = _operand(_LHS[j], lambda r2, p: _operand(
                    _LHS[i], lambda r1, h: g_s[2 * r1 + h][slot, g_rows(r2, p, 0, NS * LANES), :])).astype(BF16)
                if i in _RAW and j in _RAW:
                    d = 2 * _RAW.index(i) + _RAW.index(j)
                    wij = [raw4(4 * st + d, d) for st in range(NS)]
                else:
                    wij = [s4_u[i, j, st] for st in range(NS)]
                m[j] = _dot(_as_bf16(jnp.concatenate(wij, axis=1)), act)
                toks += _rows8(m[j])
            part[i] = [x + ex[inner // 2][(inner % 2) * QR:(inner % 2 + 1) * QR]
                       for inner, x in enumerate(_combine(m))]
            marks[i] = len(toks)

        gb = 0.5 * mod_s[NC, 0:1, :]
        nxt = jnp.minimum(t + 1, NT - 1) * TB
        tails = {}
        for i, blk, norm in ((4, 1, (0, NW[0]) + NW[2:4]), (3, 2, NW[0:2] + NW[4:6]), (6, 0, (NW[1], 4) + NW[6:8]),
                             (5, 3, None)):
            r1 = blk // 2
            if norm is None:
                toks += [x for x in lead_in()[LT[0]:] for _ in range(LT[1])]
            else:
                store_z(nxt, 1 - ws, toks[norm[2]:norm[3]], norm[0], norm[1])
            pos = [marks[i] + FL[(1, 2, 0, 3).index(blk)]]

            def finish(rq, c, h2t):
                h2 = hold(h2t.T, toks[pos[0]:pos[0] + TQ // 8])
                pos[0] += TQ // 8
                rows = pl.ds(pl.multiple_of(r0 + rq * TQ, TQ), TQ)
                cols = slice(c * LANES, (c + 1) * LANES)
                o_v[c, rows, :] = (x_s[rows, cols] + gb[:, cols] * (h_s[rows, cols] + h2)).astype(BF16)
                if blk == 3:
                    out_copy(rows.start, TQ, c).start()

            for inner in (1, 2, 0, 3):
                ht = _block([part[k][inner] for k in range(7)], blk)
                rq, c = 2 * r1 + inner // 2, 2 * (blk % 2) + inner % 2
                finish(rq, c, ht[0:LANES])
                tails[rq, c] = ht[LANES:]
            rb = pl.multiple_of(r0 + r1 * 2 * TQ, 2 * TQ)
            if blk != 3:
                for e in range(2):
                    out_copy(rb, 2 * TQ, 2 * (blk % 2) + e).start()
            if blk in (0, 3):
                for rq in (2 * r1, 2 * r1 + 1):
                    finish(rq, NC - 1, jnp.concatenate([tails[rq, c] for c in range(NC - 1)], axis=0))
                if blk == 0:
                    out_copy(rb, 2 * TQ, NC - 1).start()
        return carry

    with jax.named_scope("ph2b"):
        lax.fori_loop(0, NT, mlp_tile, 0)
    with jax.named_scope("tail"):
        pltpu.make_async_copy(o_v, o_v, sem_o.at[0]).wait()


@jax.jit
def pallas_adaLN_cond__ssm_conv_h3__mixer_s_mlp__prompt_kernel(
    A_q: jax.Array,
    A_k: jax.Array,
    A_v: jax.Array,
    A_shift_k: jax.Array,
    A_ssm_k: jax.Array,
    A_ssm_D: jax.Array,
    B_x: jax.Array,
    B_w1: jax.Array,
    B_w2: jax.Array,
    B_w3: jax.Array,
    B_w4: jax.Array,
    c: jax.Array,
    w_mod: jax.Array,
):
    B, S, D = A_q.shape
    FF = B_w3.shape[1]
    assert (B, S, D, FF, A_shift_k.shape[1]) == (1, sum(TILES), 5 * LANES, 1728, 4)
    NC = D // LANES
    NG = BLK // 8
    NBL = S // (PH * BLK)
    NS = FF // 4 // LANES
    n1 = S - sum(TILES[:BLOCKWISE1[0]]) - HALO
    n2 = S - sum(TILES[:BLOCKWISE2[0]])

    args = (A_q.reshape(S, D), A_k.reshape(S, D), A_v.reshape(S, D), A_shift_k.T, A_ssm_k,
            A_ssm_D, B_w1, B_w2, B_w3.T, B_w4, c, w_mod)
    scratch = [
        pltpu.VMEM((S, D), BF16),
        pltpu.VMEM((NC, S + 16 + 2 * YP, LANES), BF16),
        pltpu.VMEM((NC, S + 2 * YP, LANES), BF16),
        pltpu.VMEM((4, D), BF16),
        pltpu.VMEM((NC, LANES, S), BF16),
        pltpu.VMEM((D,), BF16),
        pltpu.VMEM((NC, D, LANES), BF16),
        pltpu.VMEM((NC, D, LANES), BF16),
        pltpu.VMEM((NC, FF, LANES), BF16),
        pltpu.VMEM((NC, FF, LANES), BF16),
        pltpu.VMEM((1, D), BF16),
        pltpu.VMEM((D, 6 * D), BF16),
        pltpu.VMEM((PH, 2 * BLK, BLK), BF16),
        pltpu.VMEM((PH, 2, BLK, BLK), BF16),
        pltpu.VMEM((NC, S, LANES), BF16),
        pltpu.VMEM((NC, NG, NBL, PH, 2, 8, LANES), F32),
        pltpu.VMEM((NC, NG, NBL, PH, 2, 8, LANES), F32),
        pltpu.VMEM((NC, NBL, PH, 2 * BLK, LANES), BF16),
        pltpu.VMEM((6, PH, BLK, LANES), BF16),
        pltpu.VMEM((NC, S + YP, LANES), F32),
        pltpu.VMEM((6, 8, D), F32),
        pltpu.VMEM((NC, 8, LANES), F32),
        pltpu.VMEM((NC, S + 16, LANES), F32),
        pltpu.VMEM((S, D), F32),
        pltpu.VMEM((S, D), F32),
        pltpu.VMEM((NC, S, LANES), BF16),
        pltpu.VMEM((7, 7, FF // 4, LANES), BF16),
        pltpu.VMEM((7, 7, NS, D // 4, LANES), BF16),
        pltpu.VMEM((7, 2, D // 4, LANES), BF16),
        [pltpu.VMEM((2, GROWS, TQ), F32)] * 4,
        pltpu.VMEM((2, 4 * NC * (TQ + 8), LANES), F32),
        pltpu.VMEM((TB, LANES), BF16),
        pltpu.VMEM((10, 2, n1 // 2, LANES), BF16),
        pltpu.VMEM((10, 2, n2 // 2, LANES), BF16),
        pltpu.VMEM((7, 2, 2 * LANES, LANES), BF16),
        pltpu.VMEM((7, 2, 2 * LANES, LANES), BF16),
        pltpu.VMEM((4, FF // 4, TQ), F32),
        pltpu.VMEM((NC, 4 * NS + 2, LANES, LANES), BF16),
        pltpu.VMEM((D, LANES), F32),
        pltpu.SemaphoreType.DMA((21,)),
        pltpu.SemaphoreType.DMA((1,)),
    ]
    out = pl.pallas_call(
        functools.partial(_kernel, S=S, D=D, FF=FF),
        in_specs=[pl.BlockSpec(memory_space=pl.ANY)] * len(args),
        out_specs=pl.BlockSpec(memory_space=pl.ANY),
        out_shape=jax.ShapeDtypeStruct((S, D), BF16),
        scratch_shapes=scratch,
        compiler_params=pltpu.CompilerParams(
            vmem_limit_bytes=120 * 1024 * 1024,
            disable_bounds_checks=True,
            disable_semaphore_checks=True,
        ),
    )(*args)
    return out.reshape(B, S, D)
```

```python
import functools
import math

import jax
import jax.numpy as jnp
from jax import lax
import jax.experimental.pallas as pl
import jax.experimental.pallas.tpu as pltpu

F32 = jnp.float32
BF16 = jnp.bfloat16
U32 = jnp.uint32

LANES = 128
BLK = 128
PH = 4
EPS = 1e-05
TB = 512
TQ = TB // 4
HALO = 32
TILES = (384, 384, 576, 704)
BLOCKWISE1 = (3,)
BLOCKWISE2 = (2, 3)
IN_LOOP = (4, 2, 0, 1, 3)
ROT = 3
KR = 256
NB1 = 1
IG = 2
IJ = 6
IP = 2
GPAD = 8
GROWS = 1768

MF = (6, 0, 5, 4)
MT = (3, 0, 3, 3)
R6 = (36, 18, 28, 6)
TRS = (145, 175, 180)
FRS = (50, 90, 90)
WS = (2, 3, 3, 2, 2, 4)
FI = (48, 88, 96, 96)
LAST = (55, 66, 92, 82)
EW = (2, 1, 2)
NW = (1, 3, 0, 150, 320, 460, 600, 730)
FL = (10, 10, 25, -32)
O3 = (4, 3, 0, 6, 2, 1, 5)
J3 = (1, 2, 3, 4, 5, 6, 0)
J4 = (4, 2, 3, 1, 0, 6, 5)
ET = (0, 4)
EC = 10
YP = 128
LT = (8, 3)

_ORDER = (2, 4, 1, 3, 0, 6, 5)
_RAW = (1, 4)
_LHS = (((0, 0), 1, (1, 1)), ((1, 0), 1, (1, 1)), ((0, 0),), ((1, 1),),
        ((0, 0), 1, (0, 1)), ((1, 0), -1, (0, 0)), ((0, 1), -1, (1, 1)))
_RHS = (((0, 0), 1, (1, 1)), ((0, 0),), ((0, 1), -1, (1, 1)), ((1, 0), -1, (0, 0)),
        ((1, 1),), ((0, 0), 1, (0, 1)), ((1, 0), 1, (1, 1)))


def _operand(terms, blk):
    x = blk(*terms[0])
    if len(terms) > 1:
        y = blk(*terms[2])
        x = x + y if terms[1] > 0 else x - y
    return x


def _all_operands(table, b00, b01, b10, b11):
    blocks = ((b00, b01), (b10, b11))
    return [_operand(terms, lambda i, j: blocks[i][j]) for terms in table]


def _block(m, which):
    if which == 0:
        return (m[3] - m[4]) + m[0] + m[6]
    if which == 1:
        return m[2] + m[4]
    if which == 2:
        return m[1] + m[3]
    return (m[2] - m[1]) + m[0] + m[5]


def _combine(m):
    return [_block(m, which) for which in range(4)]


def _as_bf16(x):
    return pltpu.bitcast(x, BF16)


def _lo(x):
    return pltpu.bitcast(x << 16, F32)


def _hi(x):
    return pltpu.bitcast(x & jnp.uint32(0xFFFF0000), F32)


def _dft4(re, im, sign):
    ar, ai = re[0] + re[2], im[0] + im[2]
    br, bi = re[0] - re[2], im[0] - im[2]
    cr, ci = re[1] + re[3], im[1] + im[3]
    dr, di = re[1] - re[3], im[1] - im[3]
    o0 = (ar + cr, ai + ci)
    o2 = (ar - cr, ai - ci)
    m = (br + di, bi - dr)
    p = (br - di, bi + dr)
    o1, o3 = (m, p) if sign < 0 else (p, m)
    return [o0[0], o1[0], o2[0], o3[0]], [o0[1], o1[1], o2[1], o3[1]]


def _ln(x, eps=EPS, unit=True):
    n = x.shape[-1]
    s1 = jnp.sum(x, axis=-1, keepdims=True)
    m = s1 * (1.0 / n)
    v = jnp.maximum(jnp.sum(x * x, axis=-1, keepdims=True) + (n * eps - s1 * m), n * eps)
    e = jnp.log(v) * (-0.5 / math.log(2.0))
    return (x - m) * jnp.exp2(e + 0.5 * math.log2(n) if unit else e)


def _gelu2(x):
    c0 = math.sqrt(2.0 / math.pi)
    return x + x * jnp.tanh(x * (c0 + (c0 * 0.044715) * (x * x)))


def _dot(a, b):
    return jnp.dot(a, b, preferred_element_type=F32)


def _dot_nt(a, b):
    return lax.dot_general(a, b, (((1,), (1,)), ((), ())), preferred_element_type=F32)


def _rows8(x, repeat=1):
    return [(x, r) for r in range(x.shape[0] // 8) for _ in range(repeat)]


def _stack(tks):
    return jnp.concatenate([x[8 * r:8 * r + 8, 0:LANES] for x, r in tks], axis=0).reshape(len(tks), 8, LANES)


def _chunks(r0, r1, k, unit=16):
    n = (r1 - r0) // unit
    cuts = [r0 + unit * ((n * j) // k) for j in range(k + 1)]
    return list(zip(cuts[:-1], cuts[1:]))


def _pick(toks, n, free=0):
    idx = [(r * (len(toks) + free)) // n - free for r in range(n)]
    return [toks[i] if i >= 0 else None for i in idx]


def _kernel(q_hbm, k_hbm, v_hbm, sh_hbm, sk_hbm, sd_hbm, w1_hbm, w2_hbm, w3_hbm, w4_hbm, c_hbm, wm_hbm,
            o_hbm,
            q_v, k_v, v_v, sh_v, sk_v, sd_v, w1_v, w2_v, w3_v, w4_v, c_v, wm_v,
            fw_s, iv_s, o_v, u_s, kk_s, vv_s, wu_s, y_s, mod_s, par_s, h1_s, x_s, h_s, z_s,
            s3_s, s4_s, e4_s, g_s, zf_s, zr_s, l1_s, l2_s, s1_s, s2_s, rh_s, wt_s, scol_s,
            sem, sem_o,
            *, S, D, FF):
    NC = D // LANES
    NG = BLK // 8
    LB = PH * BLK
    NBL = S // LB
    R = BLK // PH
    HL = LANES // 2

    small = [
        pltpu.make_async_copy(sh_hbm, sh_v, sem.at[0]),
        pltpu.make_async_copy(sd_hbm, sd_v, sem.at[0]),
        pltpu.make_async_copy(c_hbm, c_v, sem.at[0]),
    ]

    def sk_copy(c):
        ch = (c + ROT) % NC * LANES
        rows = pl.ds(ch if isinstance(c, int) else pl.multiple_of(ch, LANES), LANES)
        return [pltpu.make_async_copy(sk_hbm.at[rows, :], sk_v.at[c], sem.at[1 + c])]

    def kv_copies(tiles, lo, hi, s):
        return [pltpu.make_async_copy(src.at[pl.ds(r0, r1 - r0), pl.ds((c + ROT) % NC * LANES, LANES)],
                                      dst.at[c, pl.ds(off + r0, r1 - r0), :], sem.at[s])
                for r0, r1 in _chunks(lo, hi, (hi - lo + 16) // KR)
                for src, dst, off in ((k_hbm, k_v, 16), (v_hbm, v_v, 0)) for c in tiles]

    PAIR, TRIPLE = (0, 1), (2, 3, 4)
    kv_groups = [kv_copies(PAIR, 0, NB1 * LB + 16, 9), kv_copies(PAIR, NB1 * LB + 16, S, 10),
                 kv_copies(TRIPLE, 0, 2 * LB + 16, 11), kv_copies(TRIPLE, 2 * LB + 16, S, 20)]

    WM = (0, 3 * D, 5 * D, 6 * D)
    wm_copies = [[pltpu.make_async_copy(wm_hbm.at[:, pl.ds(WM[j], WM[j + 1] - WM[j])],
                                        wm_v.at[:, pl.ds(WM[j], WM[j + 1] - WM[j])], sem.at[6 + j])]
                 for j in range(3)]
    w_copies = [[pltpu.make_async_copy(src.at[:, pl.ds(c * LANES, LANES)], dst.at[c], sem.at[12 + j])
                 for c in range(NC)]
                for j, (src, dst) in enumerate(((w1_hbm, w1_v), (w2_hbm, w2_v), (w3_hbm, w3_v), (w4_hbm, w4_v)))]

    B0 = [0]
    for n in TILES:
        B0.append(B0[-1] + n)
    NA = len(TILES)
    A0 = [0] + [r + HALO for r in B0[1:-1]] + [S]
    q_copies = [
        [pltpu.make_async_copy(q_hbm.at[pl.ds(A0[t], A0[t + 1] - A0[t])], q_v.at[pl.ds(A0[t], A0[t + 1] - A0[t])],
                               sem.at[16 + t])]
        for t in range(NA)
    ]

    def start_all(cps, priority=0):
        for cp in cps:
            cp.start(priority=priority)

    def wait_all(cps):
        for cp in cps:
            cp.wait()

    for c in range(NC):
        k_v[c, 0:16, :] = jnp.zeros((16, LANES), BF16)
    start_all(sk_copy(0) + small + sk_copy(1) + kv_groups[0] + kv_groups[1] + sk_copy(2))

    for c in range(NC):
        h1_s[c, 0:8, :] = jnp.zeros((8, LANES), F32)
        h1_s[c, S + 8:S + 16, :] = jnp.zeros((8, LANES), F32)

    prow = lax.broadcasted_iota(jnp.int32, (BLK, BLK), 0)
    pcol = lax.broadcasted_iota(jnp.int32, (BLK, BLK), 1)
    ang = (((4 * prow + 1) * pcol) & (4 * BLK - 1)).astype(F32) * (2.0 * math.pi / (4 * BLK))
    tw = (4 * prow + 1).astype(F32) * (2.0 * math.pi / (4 * LB))
    mr, mi = jnp.cos(ang), -jnp.sin(ang)
    twr, twi = jnp.cos(tw), -jnp.sin(tw)
    eye = jnp.where(prow == pcol, 1.0 / LB, 0.0).astype(BF16)
    for i in range(PH):
        both = jnp.concatenate([mr.reshape(NG, 8, BLK), mi.reshape(NG, 8, BLK)], axis=1).reshape(2 * BLK, BLK)
        fw_s[i] = both.astype(BF16)
        for h in range(2):
            iv_s[i, h] = _dot_nt(eye, both[h * BLK:(h + 1) * BLK, :].astype(BF16)).astype(BF16)
        if i + 1 < PH:
            mr, mi = mr * twr - mi * twi, mr * twi + mi * twr
    perm = jnp.where(pcol == (prow % R) * PH + prow // R, 1.0, 0.0).astype(BF16)

    wait_all(small)
    shf = sh_v[...].astype(F32)
    sdf = sd_v[...].astype(F32).reshape(1, D)
    for c in range(NC):
        par_s[(c - ROT) % NC, 0:4, :] = shf[:, c * LANES:(c + 1) * LANES]
        par_s[(c - ROT) % NC, 4:5, :] = sdf[:, c * LANES:(c + 1) * LANES]
    cf = c_v[...].astype(F32)
    sc = (cf * jax.nn.sigmoid(cf)).astype(BF16)
    sc16 = jnp.broadcast_to(sc, (16, D))

    def mod_chunk(j):
        mod_s[j] = _dot(sc16, wm_v[:, j * D:(j + 1) * D])[0:8, :]

    (fw_u, iv_u, k_u, v_u, wu_u, vv_u, z_u, l1_u, l2_u, w1_u, w2_u, s1_u, s2_u, w3_u, w4_u, wt_u, s3_u, s4_u,
     e4_u, zr_u) = (r.bitcast(U32) for r in (fw_s, iv_s, k_v, v_v, wu_s, vv_s, z_s, l1_s, l2_s, w1_v, w2_v,
                                             s1_s, s2_s, w3_v, w4_v, wt_s, s3_s, s4_s, e4_s, zr_s))

    never = twr[0:8, :] > 2.0

    def after(token, x):
        if token.dtype != x.dtype:
            token = pltpu.bitcast(token, x.dtype)
        return jnp.where(jnp.broadcast_to(never, x.shape), token, x)

    def hold(x, tks):
        f = len([k for k in tks if k is None])
        n = len(tks)
        head = after(_stack(tks[f:]), x[8 * f:, 0:LANES].reshape(n - f, 8, LANES)).reshape(8 * (n - f), LANES)
        if f:
            head = jnp.concatenate([x[:8 * f, 0:LANES], head], axis=0)
        return head if x.shape[1] == LANES else jnp.concatenate([head, x[:, LANES:]], axis=1)

    def hold16(x, tks):
        x3 = x.reshape(len(tks), 16, LANES)
        return jnp.concatenate([after(_stack(tks), x3[:, 0:8]), x3[:, 8:16]], axis=1).reshape(x.shape)

    def perm_k(c, b, toks):
        kt = [_dot_nt(perm, sk_v[c, :, b * LB + t * BLK:b * LB + (t + 1) * BLK]) for t in range(PH)]
        toks += _rows8(kt[0])[::2]
        return [jnp.concatenate([kt[t][i * R:(i + 1) * R, :] for t in range(PH)], axis=0).astype(BF16)
                for i in range(PH)]

    def spectrum(comps, dst, slot, b, toks, dc=None, pins=None):
        tr, ti = [], []
        for i in range(PH):
            lhs = fw_u[i]
            if pins is not None and i < len(pins):
                lhs = after(pins[i], lhs.reshape(NG, 8, LANES)).reshape(BLK, LANES)
            res = _dot(_as_bf16(lhs), comps[i])
            t3 = res.reshape(NG, 16, LANES)
            tr.append(t3[:, 0:8])
            ti.append(t3[:, 8:16])
        toks += _rows8(res)[1::2]
        if dc is not None:
            tr[0] = tr[0] + dc
        sr, si = _dft4(tr, ti, -1)
        for qq in range(PH):
            dst[slot, :, b, qq, 0] = sr[qq]
            dst[slot, :, b, qq, 1] = si[qq]

    def gated(c, b, n):
        w = [par_s[c, t:t + 1, :] for t in range(4)]
        kc = {}
        for o in range(-2, 2):
            words = k_u[c, pl.ds(8 + b * (LB // 2) + o, BLK, stride=2), :]
            if o > -2:
                kc[2 * o] = _lo(words)
            kc[2 * o + 1] = _hi(words)
        vc = {}
        for o in range(2):
            words = v_u[c, pl.ds(b * (LB // 2) + o, BLK, stride=2), :]
            vc[2 * o] = _lo(words)
            vc[2 * o + 1] = _hi(words)
        for i in range(PH):
            ks = kc[i] * w[0]
            for t in range(1, 4):
                ks = ks + kc[i - t] * w[t]
            wu_s[n, i] = (ks * vc[i]).astype(BF16)
        return [wu_u[n, i] for i in range(PH)]

    def kv_pins(kvb):
        return [_stack([(kvb[2 * m + (r % 2)], r // 2) for r in range(NG)]) for m in range(2)]

    def products(c, ks, kc, toks, free, trim):
        n = len(toks) - trim + free
        cum = (44, 128, 244, 392)
        zp = None
        for o in range(NBL):
            idx = [((g * cum[-1] + cum[o]) * n) // (cum[-1] * NG) - 1 - free for g in range(NG)]
            tk = [toks[max(i, 0)] if i >= 0 or not free else None for i in idx]
            zr, zi = [], []
            for qq in range(PH):
                accr = acci = None
                for b in range(o + 1):
                    a_, b_ = u_s[c, :, b, qq, 0], u_s[c, :, b, qq, 1]
                    c_, d_ = ks[kc, :, o - b, qq, 0], ks[kc, :, o - b, qq, 1]
                    if qq == 0 and b == o:
                        a_ = hold(a_.reshape(BLK, LANES), tk).reshape(NG, 8, LANES)
                    tr_ = a_ * c_ - b_ * d_
                    ti_ = a_ * d_ + b_ * c_
                    accr = tr_ if accr is None else accr + tr_
                    acci = ti_ if acci is None else acci + ti_
                zr.append(accr)
                zi.append(acci)
            if zp is None:
                yr, yi = zr, zi
            else:
                yr = [zr[qq] - zp[1][qq] for qq in range(PH)]
                yi = [zi[qq] + zp[0][qq] for qq in range(PH)]
            zp = (zr, zi)
            vr, vi = _dft4(yr, yi, +1)
            for i in range(PH):
                vv_s[c, o, i] = jnp.concatenate([vr[i], vi[i]], axis=1).reshape(2 * BLK, LANES).astype(BF16)

    def inverse(c, o, toks, pins):
        for i in range(PH):
            yv = None
            for h in range(2):
                lhs = iv_u[i, h]
                if pins is not None and h == 0:
                    pin = pins[i % 2][8 * (i // 2):8 * (i // 2) + 8]
                    lhs = after(pin, lhs.reshape(8, 8, LANES)).reshape(HL, LANES)
                t = _dot(_as_bf16(lhs), _as_bf16(vv_u[c, o, i, h * HL:(h + 1) * HL, :]))
                yv = t if yv is None else yv + t
            if i % 2 == 0:
                toks += _rows8(yv)[::2]
            y_s[c, pl.ds(o * LB + i, BLK, stride=PH), :] = yv

    def conv_step(filt=None, units=(), mul=None, inv=(), free=0, trim=3):
        toks = []
        kv = [gated(c, b, n) for n, (c, b) in enumerate(units)]
        pin_at = {n: kv_pins(kv[n]) for n in range(len(units))} if inv or filt is not None else {}
        if filt is not None and mul is not None and not isinstance(filt, int):
            ks = kk_s.at[pl.ds(mul, 2)]
            k_rd, k_wr = (ks, 0), (ks, 1)
        else:
            k_rd, k_wr = (kk_s, mul), (kk_s, filt)
        pos = 0
        for c, o in inv:
            inverse(c, o, toks, pin_at.get(pos))
            pos += 1
        if filt is not None:
            comps = [perm_k(filt, b, toks) for b in range(NBL)]
            for b in range(NBL):
                spectrum(comps[b], *k_wr, b, toks, par_s[filt, 4:5, :] if b == 0 else None, pin_at.get(pos))
                pos += 1
        for n, (c, b) in enumerate(units):
            spectrum([_as_bf16(x) for x in kv[n]], u_s, c, b, toks, None, pin_at.get(pos))
            pos += 1
        if mul is not None:
            products(mul, *k_rd, toks, free, trim)
        return toks

    def lane_tiles(x):
        return [x[:, c * LANES:(c + 1) * LANES] for c in range(NC)]

    def stage_p1(r0, r1, tks=None, ytks=None):
        ga = mod_s[2, 0:1, :]
        a_mul, a_add = ga * (1.0 + mod_s[1, 0:1, :]) * math.sqrt(D), ga * mod_s[0, 0:1, :]
        q = q_v[r0:r1, :].astype(F32)
        if tks is not None:
            q = hold(q, tks)
        y = jnp.concatenate([y_s[(c - ROT) % NC, r0:r1, :] for c in range(NC)], axis=1)
        if ytks is not None:
            y = hold(y, ytks)
        x = q + (_ln(q, unit=False) * a_mul + a_add) * y
        x_s[r0:r1, :] = x
        return _ln(x, unit=False)

    def store_row_ops(dst, base, r0, r1, cols, tks=None):
        hv = []
        for x in cols:
            x3 = x.reshape(x.shape[0] // 32, 32, LANES)
            hv.append([x3[:, 16 * e:16 * e + 16].reshape(x.shape[0] // 2, LANES) for e in range(2)])
        for k2 in range(2):
            a00, a01, a10, a11 = hv[k2][0], hv[2 + k2][0], hv[k2][1], hv[2 + k2][1]
            if tks is not None:
                a00, a11 = hold16(a00, tks), hold16(a11, tks)
            for o, x in enumerate(_all_operands(_LHS, a00, a01, a10, a11) + [a01, a10, hv[NC - 1][k2]]):
                dst[o, k2, (r0 - base) // 2:(r1 - base) // 2, :] = x.astype(BF16)

    L1B = A0[BLOCKWISE1[0]]
    L2B = B0[BLOCKWISE2[0]]

    def stage_p2(r0, r1, nx, blockwise=False):
        h = nx * ((1.0 + mod_s[4, 0:1, :]) * (2.0 * math.sqrt(D))) + 2.0 * mod_s[3, 0:1, :]
        h_s[r0:r1, :] = h
        zn = lane_tiles(_ln(h, 4.0 * EPS))
        if blockwise:
            store_row_ops(l1_s, L1B, r0, r1, zn)
        else:
            for c in range(NC):
                z_s[c, r0:r1, :] = zn[c].astype(BF16)

    def stage_p(t, toks):
        lo, hi = A0[t], A0[t + 1]
        stage_p2(lo, hi, stage_p1(lo, hi, _pick(toks[:-TRS[t - 1]], (hi - lo) // 8, FRS[t - 1])), t in BLOCKWISE1)

    def filler(t):
        red = jnp.sum(y_s[t, 0:8 * FI[t], :], axis=-1, keepdims=True).reshape(FI[t], 8, 1)
        spare = (NC - 1) * (TQ + 8) + 8 * t
        zf_s[1, spare:spare + 8, :] = jnp.broadcast_to(jnp.sum(red, axis=0), (8, LANES))

    def square_ops(src, dst, toks):
        HK = 2 * LANES
        tks = _pick(toks, 2 * HK // 16)
        for n2 in range(2):
            tk = tks[n2 * (HK // 16):(n2 + 1) * (HK // 16)]
            blk = lambda k, n: src[2 * n + n2, k * HK:(k + 1) * HK, :].astype(F32)
            for o, x in enumerate(_all_operands(_RHS, hold16(blk(0, 0), tk), blk(0, 1), blk(1, 0), hold16(blk(1, 1), tk))):
                if o not in _RAW:
                    dst[o, n2] = x.astype(BF16)

    def block_dots(ops_u, base, prepare, w_u, s_u, parts, emit, light, heavy):
        toks = []

        def timed(x, weight):
            toks.extend(_rows8(x, weight))
            return x

        def weave(top, bot):
            n = top.shape[0] // 16
            return jnp.concatenate([top.reshape(n, 16, LANES), bot.reshape(n, 16, LANES)], axis=1).reshape(32 * n, LANES)

        def main(get):
            m = [None] * 7
            rem = [None, None]
            for o in ('t', 2, 4, 'b', 1, 3, 0, 6, 5):
                if o in ('t', 'b'):
                    e = 0 if o == 't' else 1
                    rhs = jnp.concatenate([w_u[c, 2 * LANES:D // 2, :] for c in range(NC - 1)], axis=1)
                    rem[e] = timed(_dot(get([(9, e)]), _as_bf16(rhs)), light)
                    continue
                if o in _RAW:
                    d = _RAW.index(o)
                    rhs = jnp.concatenate([w_u[2 * d + n2, d * LANES:(d + 1) * LANES, :] for n2 in range(2)], axis=1)
                else:
                    rhs = jnp.concatenate([s_u[o, n2] for n2 in range(2)], axis=1)
                m[o] = timed(_dot(get([(o, 0), (o, 1)]), _as_bf16(rhs)), heavy if o in (4, 3, 6, 5) else light)
            c00, c01, c10, c11 = _combine(m)
            top = jnp.concatenate([c00, c01], axis=1) + rem[0]
            bot = jnp.concatenate([c10, c11], axis=1) + rem[1]
            return [weave(top[:, c * LANES:(c + 1) * LANES], bot[:, c * LANES:(c + 1) * LANES]) for c in range(NC - 1)]

        def last(get):
            w = _as_bf16(w_u[NC - 1])
            return weave(timed(_dot(get([(2, 0), (2, 1), (7, 0), (7, 1), (9, 0)]), w), light),
                         timed(_dot(get([(8, 0), (8, 1), (3, 0), (3, 1), (9, 1)]), w), light))

        mark = None
        for j, (r0, r1) in enumerate(parts):
            prepare(r0, r1, None if mark is None else toks[mark:])
            mark = len(toks)
            get = lambda keys: _as_bf16(jnp.concatenate(
                [ops_u[o, e, (r0 - base) // 4:(r1 - base) // 4, :] for o, e in keys], axis=1))
            if j % 2:
                tail = last(get)
                emit(r0, r1, main(get) + [tail])
            else:
                emit(r0, r1, main(get) + [last(get)])
        return toks

    def stage_m1(t, k):
        def emit(r0, r1, cols):
            out = [_gelu2(x) for x in cols]
            for c in range(NC):
                h1_s[c, r0 + 8:r1 + 8, :] = out[c]
            return out

        if t in BLOCKWISE1:
            return block_dots(l1_u, L1B, lambda *_: None, w1_u, s1_u, _chunks(A0[t], A0[t + 1], k, 32), emit, WS[2], WS[3])
        toks = []
        for r0, r1 in _chunks(A0[t], A0[t + 1], k):
            lhs = jnp.concatenate([z_u[c, r0 // 2:r1 // 2, :] for c in range(NC)], axis=1)
            w = jnp.concatenate([w1_u[c] for c in range(NC)], axis=1)
            for x in emit(r0, r1, lane_tiles(_dot(_as_bf16(lhs), _as_bf16(w)))):
                toks += _rows8(x, WS[0])
        return toks

    def shifted(r0, r1):
        n, grp, shifts = r1 - r0, D // 4, (-1, 1, -2, 2)
        lane = lax.broadcasted_iota(jnp.int32, (n, LANES), 1)
        cols = []
        for c in range(NC):
            lo, hi = c * LANES, (c + 1) * LANES
            g_lo, g_hi = lo // grp, (hi - 1) // grp
            val = h1_s[c, pl.ds(r0 + 8 + shifts[g_lo], n), :]
            if g_hi != g_lo:
                other = h1_s[c, pl.ds(r0 + 8 + shifts[g_hi], n), :]
                val = jnp.where(lane < (g_hi * grp - lo), val, other)
            cols.append(val)
        return cols

    def stage_m2(t, k, before=None):
        def emit(r0, r1, cols):
            x1 = h_s[r0:r1, :] + jnp.concatenate(cols, axis=1)
            h_s[r0:r1, :] = x1
            return x1

        if t in BLOCKWISE2:
            def prepare(r0, r1, prev):
                prev = before if prev is None else prev
                prev = prev[len(prev) // 8:(len(prev) * 7) // 8]
                store_row_ops(l2_s, L2B, r0, r1, shifted(r0, r1), _pick(prev, (r1 - r0) // 32))
            return block_dots(l2_u, L2B, prepare, w2_u, s2_u, _chunks(B0[t], B0[t + 1], k, 32), emit, WS[4], WS[4])
        toks = []
        for r0, r1 in _chunks(B0[t], B0[t + 1], k):
            w = jnp.concatenate([w2_u[c] for c in range(NC)], axis=1)
            hs = _dot(jnp.concatenate(shifted(r0, r1), axis=1).astype(BF16), _as_bf16(w))
            for x in lane_tiles(emit(r0, r1, [hs])):
                toks += _rows8(x, WS[1])
        return toks

    NT = S // TB
    FQ = FF // 4
    NS = FQ // LANES
    LQ = FQ - NS * LANES
    CQ = LANES // 4
    QR = LANES + CQ
    BLOCKS = [(2 * r1 + r2, 2 * h + p)
              for r1, h in ((0, 0), (1, 0), (0, 1), (1, 1)) for r2 in range(2) for p in range(2)]

    def z_rows(rq, c):
        lo = (NC * rq + c) * (TQ + 8)
        return slice(lo, lo + TQ)

    def store_z(r0, slot, toks, q0=0, q1=4):
        n = (q1 - q0) * TQ
        rows = pl.ds(r0 + q0 * TQ if isinstance(r0, int) else pl.multiple_of(r0 + q0 * TQ, TQ), n)
        zn = lane_tiles(_ln(hold(h_s[rows, :], _pick(toks, n // 8)), 4.0 * EPS))
        for rq in range(q0, q1):
            for c in range(NC - 1):
                zf_s[slot, z_rows(rq, c), :] = zn[c][(rq - q0) * TQ:(rq - q0 + 1) * TQ]
        zr_s[q0 * TQ:q1 * TQ, :] = zn[NC - 1].astype(BF16)

    def w3_ops(toks):
        ng = FQ // 16
        blk = lambda c, d: w3_v[c, d * FQ:(d + 1) * FQ, :].astype(F32)
        outer = [[_all_operands(_RHS, blk(k2, p), blk(k2, 2 + p), blk(2 + k2, p), blk(2 + k2, 2 + p))
                  for p in range(2)] for k2 in range(2)]
        for k, i in enumerate((1, 5, 2, 4, 0, 3, 6)):
            tk = [toks[((k + r * 7) * len(toks)) // (7 * ng)] for r in range(ng)]
            for j, x in enumerate(_all_operands(_RHS, hold16(outer[0][0][i], tk), outer[0][1][i], outer[1][0][i],
                                                hold16(outer[1][1][i], tk))):
                if i not in _RAW or j not in _RAW:
                    s3_s[i, j] = x.astype(BF16)

    def transpose_w4(toks):
        order = [(c, n) for n in (4 * NS, 4 * NS + 1) + tuple(range(4 * NS)) for c in range(NC)]
        for k, (c, n) in enumerate(order):
            if n >= 4 * NS:
                ends = [(2 * (n - 4 * NS) + p + 1) * FQ // 2 for p in range(2)]
                x = jnp.concatenate([w4_u[c, e - LQ // 2:e, :] for e in ends]
                                    + [jnp.zeros((HL - LQ, LANES), U32)], axis=0)
            else:
                lo = (n % 4) * FQ // 2 + (n // 4) * HL
                x = w4_u[c, lo:lo + HL, :]
            x = jnp.concatenate([hold(x[0:8], [toks[(k * len(toks)) // len(order)]]), x[8:]], axis=0)
            wt_s[c, n] = _as_bf16(x).astype(F32).T.astype(BF16)

    def w4_ops(i, zero, toks):
        ng = QR // 16
        total = (NS * 7 + 2) * ng
        tk = lambda pos, step: [toks[((pos + r * step) * len(toks)) // total] for r in range(ng)]
        quarter = lambda n, d: jnp.concatenate(
            [wt_s[d, n].astype(F32), wt_s[NC - 1, n, d * CQ:(d + 1) * CQ, :].astype(F32)], axis=0)
        if i not in _RAW:
            for e in range(2):
                x = _operand(_RHS[i], lambda h, d: quarter(4 * NS + h, 2 * d + e))
                e4_s[i + zero, e] = hold16(x, tk(e * ng, 1)).astype(BF16)
        for st in range(NS):
            t = [[_operand(_RHS[i], lambda h, d: quarter(4 * st + 2 * h + p, 2 * d + e)) for e in range(2)]
                 for p in range(2)]
            tks = tk((2 + st * 7) * ng, 7)
            for j, x in enumerate(_all_operands(_RHS, hold16(t[0][0], tks), t[0][1], t[1][0], hold16(t[1][1], tks))):
                if i not in _RAW or j not in _RAW:
                    s4_s[i + zero, j, st] = x.astype(BF16)

    def gate_row(toks):
        ng = D // 8
        col = hold(scol_s[...], _pick(toks, ng))
        for c in range(NC):
            prod = col * wm_v[:, (NC * NC + c) * LANES:(NC * NC + c + 1) * LANES].astype(F32)
            acc = prod[0:8]
            for r in range(1, ng):
                acc = acc + prod[8 * r:8 * r + 8]
            mod_s[NC, :, c * LANES:(c + 1) * LANES] = jnp.broadcast_to(jnp.sum(acc, axis=0, keepdims=True), (8, LANES))

    def rem3(rq, d, pieces=1):
        z = _as_bf16(zr_u[rq * (TQ // 2):(rq + 1) * (TQ // 2), :])
        return jnp.concatenate([_dot_nt(_as_bf16(w3_u[NC - 1, lo // 2:hi // 2, :]), z)
                                for lo, hi in _chunks(d * FQ, (d + 1) * FQ, pieces)], axis=0)

    def lead_in():
        head = [rem3(*key) for key in BLOCKS[:4]]
        for k in range(4):
            rh_s[k] = head[k]
        return _rows8(head[0])

    def units(tiles, blocks):
        return [(c, b) for b in blocks for c in tiles]

    with jax.named_scope("A"):
        wait_all(sk_copy(0))
        conv_step(filt=0)
    with jax.named_scope("B_wait"):
        wait_all(sk_copy(1) + kv_groups[0])
    with jax.named_scope("B"):
        start_all(kv_groups[2] + kv_groups[3] + sk_copy(3) + sk_copy(4))
        conv_step(filt=1, units=units(PAIR, range(0, NB1)))
        scol_s[...] = jnp.broadcast_to(sc.astype(F32), (LANES, D)).T
    with jax.named_scope("C_wait"):
        wait_all(kv_groups[1])
    with jax.named_scope("C"):
        conv_step(units=units(PAIR, range(NB1, NBL)))
    with jax.named_scope("D_wait"):
        wait_all(sk_copy(2))
    with jax.named_scope("D"):
        start_all(wm_copies[0] + q_copies[0] + wm_copies[1] + w_copies[0])
        conv_step(filt=2, mul=0, free=MF[0], trim=MT[0])
    with jax.named_scope("E_wait"):
        wait_all(kv_groups[2])
    with jax.named_scope("E"):
        conv_step(units=units(TRIPLE, range(0, 2)), mul=1, inv=units((0,), range(NBL)), free=MF[1], trim=MT[1])
    with jax.named_scope("F_wait"):
        wait_all(kv_groups[3])
    with jax.named_scope("F"):
        conv_step(units=units(TRIPLE, range(2, NBL)))

    def full_step(j, carry):
        wait_all(sk_copy(j + 2))
        conv_step(filt=j + 2, mul=j + 1, inv=units((j,), range(IG)), free=MF[2], trim=MT[2])
        return carry

    with jax.named_scope("GH"):
        lax.fori_loop(1, NC - 2, full_step, 0)
    late = units((NC - 2,), range(NBL)) + units(range(1, NC - 2), range(IG, NBL))
    late = late[:IJ] + units((NC - 1,), range(NBL)) + late[IJ:]
    with jax.named_scope("J"):
        start_all(q_copies[1] + w_copies[1] + sum(q_copies[2:], []) + w_copies[2] + w_copies[3] + wm_copies[2], 1)
        conv_step(mul=NC - 1, inv=late[:IJ], free=MF[3], trim=MT[3])
    with jax.named_scope("r6_wait"):
        wait_all(wm_copies[0] + q_copies[0])
    with jax.named_scope("r6"):
        for j in range(3):
            mod_chunk(j)
        conv_step(inv=late[IJ:IJ + 1])
        toks = conv_step(inv=late[IJ + 1:len(late) - IP])
        nx0 = stage_p1(0, A0[1], None, _pick(toks[:R6[0]], A0[1] // 8, R6[1]) if toks else None)
    with jax.named_scope("p2_wait"):
        wait_all(wm_copies[1])
    with jax.named_scope("p2"):
        mod_chunk(4)
        mod_chunk(3)
        toks = conv_step(inv=late[len(late) - IP:])
        if toks:
            nx0 = hold(nx0, _pick(toks[:R6[2]], A0[1] // 8, R6[3]))
        stage_p2(0, A0[1], nx0)
    with jax.named_scope("w1_wait"):
        wait_all(w_copies[0])
    with jax.named_scope("m1_0"):
        square_ops(w1_v, s1_s, stage_m1(0, 4)[:-40])
    with jax.named_scope("w2_wait"):
        wait_all(q_copies[1] + w_copies[1])
    with jax.named_scope("m2_0"):
        stage_p(1, stage_m2(0, 4))
        filler(0)
    for t in range(1, NA):
        with jax.named_scope("a%d" % t):
            wait_all(q_copies[t + 1] if t + 1 < NA else w_copies[2] + w_copies[3] + wm_copies[2])
            toks = stage_m1(t, 2)
            toks = toks + stage_m2(t, 2, toks[len(toks) - len(toks) // 2:])
            if t + 1 < NA:
                stage_p(t + 1, toks)
            if t == 1:
                square_ops(w2_v, s2_s, toks[:-30])
            if t == NA - 1:
                transpose_w4(toks[:(len(toks) * LAST[0]) // 100])
                store_z(0, 0, toks[(len(toks) * LAST[1]) // 100:(len(toks) * LAST[2]) // 100])
                toks = toks + [x for x in lead_in()[:40] for _ in range(WS[5])]
                cut = (len(toks) * LAST[3]) // 100
                gate_row(toks[:(len(toks) * 9) // 10])
                w3_ops(toks[:cut])
                rest = [i for i in range(7) if i not in IN_LOOP]
                for k, i in enumerate(rest):
                    w4_ops(i, 0, toks[cut + k::len(rest)])
            filler(t)

    def out_copy(r0, n, c):
        rows = pl.ds(r0, n)
        return pltpu.make_async_copy(o_v.at[c, rows, :], o_hbm.at[rows, pl.ds(c * LANES, LANES)], sem_o.at[0])

    def raw4(n, d):
        return jnp.concatenate([wt_u[d, n], wt_u[NC - 1, n, d * (CQ // 2):(d + 1) * (CQ // 2), :]], axis=0)

    def mlp_tile(t, carry):
        r0 = pl.multiple_of(t * TB, TB)
        ws = t & 1
        count = [0]

        def fresh():
            count[0] += 1
            return lax.rem(t + 2 * count[0], 2)

        def g_rows(r2, p, lo, hi):
            base = (2 * r2 + p) * (FQ + GPAD)
            return slice(base + lo, base + hi)

        rem = {key: rh_s[k] for k, key in enumerate(BLOCKS[:4])}
        for key in BLOCKS[4:8]:
            rem[key] = rem3(*key)
        early = _rows8(rem[BLOCKS[4]], EW[0])
        rem[BLOCKS[8]] = rem3(*BLOCKS[8], pieces=4)
        todo = BLOCKS[9:]
        part = [None] * 7
        for i in O3:
            m = [None] * 7
            for j in J3:
                slot = fresh()
                act = _operand(_LHS[j], lambda r2, k2: _operand(
                    _LHS[i], lambda r1, k1: zf_s[slot, z_rows(2 * r1 + r2, 2 * k1 + k2), :])).astype(BF16)
                if i in _RAW and j in _RAW:
                    d = 2 * _RAW.index(i) + _RAW.index(j)
                    wij = w3_u[d, d * (FQ // 2):(d + 1) * (FQ // 2), :]
                else:
                    wij = s3_u[i, j]
                m[j] = _dot_nt(_as_bf16(wij), act)
            key = todo.pop(0)
            rem[key] = rem3(*key)
            part[i] = _combine(m)
            if i in (4, 3, 0):
                early += _rows8(m[J3[ET[0]]], EW[1]) + _rows8(rem[key] if ET[1] == 7 else m[J3[ET[1]]], EW[2])
        zero = fresh() - ws
        fine = [x for x in early for _ in IN_LOOP]
        fine = fine[:len(fine) - EC * len(IN_LOOP)]
        hop = len(fine) // (len(IN_LOOP) * 33)
        for k, i in enumerate(IN_LOOP):
            w4_ops(i, zero, fine[k * hop:len(fine) - (len(IN_LOOP) - k) * hop])
        for inner in range(4):
            r2, p = inner // 2, inner % 2
            for blk, pre in enumerate(_combine([part[i][inner] for i in range(7)])):
                g_s[blk][ws, g_rows(r2, p, 0, FQ), :] = _gelu2(pre + rem[2 * (blk // 2) + r2, 2 * (blk % 2) + p])

        toks = []
        marks = {}
        part = [[None] * 4 for _ in range(7)]
        for i in _ORDER:
            slot = fresh()
            we = jnp.concatenate([raw4(4 * NS + _RAW.index(i), 2 * _RAW.index(i) + e) if i in _RAW else e4_u[i, e]
                                  for e in range(2)], axis=0)
            ex = []
            for r2 in range(2):
                act = [_operand(_LHS[i], lambda r1, h: g_s[2 * r1 + h][slot, g_rows(r2, p, NS * LANES, FQ), :])
                       for p in range(2)]
                act = jnp.concatenate(act + [jnp.zeros((LANES - 2 * LQ, TQ), F32)], axis=0).astype(BF16)
                ex.append(_dot(_as_bf16(we), act))
            m = [None] * 7
            for j in J4:
                slot = fresh()
                act = _operand(_LHS[j], lambda r2, p: _operand(
                    _LHS[i], lambda r1, h: g_s[2 * r1 + h][slot, g_rows(r2, p, 0, NS * LANES), :])).astype(BF16)
                if i in _RAW and j in _RAW:
                    d = 2 * _RAW.index(i) + _RAW.index(j)
                    wij = [raw4(4 * st + d, d) for st in range(NS)]
                else:
                    wij = [s4_u[i, j, st] for st in range(NS)]
                m[j] = _dot(_as_bf16(jnp.concatenate(wij, axis=1)), act)
                toks += _rows8(m[j])
            part[i] = [x + ex[inner // 2][(inner % 2) * QR:(inner % 2 + 1) * QR]
                       for inner, x in enumerate(_combine(m))]
            marks[i] = len(toks)

        gb = 0.5 * mod_s[NC, 0:1, :]
        nxt = jnp.minimum(t + 1, NT - 1) * TB
        tails = {}
        for i, blk, norm in ((4, 1, (0, NW[0]) + NW[2:4]), (3, 2, NW[0:2] + NW[4:6]), (6, 0, (NW[1], 4) + NW[6:8]),
                             (5, 3, None)):
            r1 = blk // 2
            if norm is None:
                toks += [x for x in lead_in()[LT[0]:] for _ in range(LT[1])]
            else:
                store_z(nxt, 1 - ws, toks[norm[2]:norm[3]], norm[0], norm[1])
            pos = [marks[i] + FL[(1, 2, 0, 3).index(blk)]]

            def finish(rq, c, h2t):
                h2 = hold(h2t.T, toks[pos[0]:pos[0] + TQ // 8])
                pos[0] += TQ // 8
                rows = pl.ds(pl.multiple_of(r0 + rq * TQ, TQ), TQ)
                cols = slice(c * LANES, (c + 1) * LANES)
                o_v[c, rows, :] = (x_s[rows, cols] + gb[:, cols] * (h_s[rows, cols] + h2)).astype(BF16)
                if blk == 3:
                    out_copy(rows.start, TQ, c).start()

            for inner in (1, 2, 0, 3):
                ht = _block([part[k][inner] for k in range(7)], blk)
                rq, c = 2 * r1 + inner // 2, 2 * (blk % 2) + inner % 2
                finish(rq, c, ht[0:LANES])
                tails[rq, c] = ht[LANES:]
            rb = pl.multiple_of(r0 + r1 * 2 * TQ, 2 * TQ)
            if blk != 3:
                for e in range(2):
                    out_copy(rb, 2 * TQ, 2 * (blk % 2) + e).start()
            if blk in (0, 3):
                for rq in (2 * r1, 2 * r1 + 1):
                    finish(rq, NC - 1, jnp.concatenate([tails[rq, c] for c in range(NC - 1)], axis=0))
                if blk == 0:
                    out_copy(rb, 2 * TQ, NC - 1).start()
        return carry

    with jax.named_scope("ph2b"):
        lax.fori_loop(0, NT, mlp_tile, 0)
    with jax.named_scope("tail"):
        pltpu.make_async_copy(o_v, o_v, sem_o.at[0]).wait()


@jax.jit
def pallas_adaLN_cond__ssm_conv_h3__mixer_s_mlp__prompt_kernel(
    A_q: jax.Array,
    A_k: jax.Array,
    A_v: jax.Array,
    A_shift_k: jax.Array,
    A_ssm_k: jax.Array,
    A_ssm_D: jax.Array,
    B_x: jax.Array,
    B_w1: jax.Array,
    B_w2: jax.Array,
    B_w3: jax.Array,
    B_w4: jax.Array,
    c: jax.Array,
    w_mod: jax.Array,
):
    B, S, D = A_q.shape
    FF = B_w3.shape[1]
    assert (B, S, D, FF, A_shift_k.shape[1]) == (1, sum(TILES), 5 * LANES, 1728, 4)
    NC = D // LANES
    NG = BLK // 8
    NBL = S // (PH * BLK)
    NS = FF // 4 // LANES
    n1 = S - sum(TILES[:BLOCKWISE1[0]]) - HALO
    n2 = S - sum(TILES[:BLOCKWISE2[0]])

    args = (A_q.reshape(S, D), A_k.reshape(S, D), A_v.reshape(S, D), A_shift_k.T, A_ssm_k,
            A_ssm_D, B_w1, B_w2, B_w3.T, B_w4, c, w_mod)
    scratch = [
        pltpu.VMEM((S, D), BF16),
        pltpu.VMEM((NC, S + 16 + 2 * YP, LANES), BF16),
        pltpu.VMEM((NC, S + 2 * YP, LANES), BF16),
        pltpu.VMEM((4, D), BF16),
        pltpu.VMEM((NC, LANES, S), BF16),
        pltpu.VMEM((D,), BF16),
        pltpu.VMEM((NC, D, LANES), BF16),
        pltpu.VMEM((NC, D, LANES), BF16),
        pltpu.VMEM((NC, FF, LANES), BF16),
        pltpu.VMEM((NC, FF, LANES), BF16),
        pltpu.VMEM((1, D), BF16),
        pltpu.VMEM((D, 6 * D), BF16),
        pltpu.VMEM((PH, 2 * BLK, BLK), BF16),
        pltpu.VMEM((PH, 2, BLK, BLK), BF16),
        pltpu.VMEM((NC, S, LANES), BF16),
        pltpu.VMEM((NC, NG, NBL, PH, 2, 8, LANES), F32),
        pltpu.VMEM((NC, NG, NBL, PH, 2, 8, LANES), F32),
        pltpu.VMEM((NC, NBL, PH, 2 * BLK, LANES), BF16),
        pltpu.VMEM((6, PH, BLK, LANES), BF16),
        pltpu.VMEM((NC, S + YP, LANES), F32),
        pltpu.VMEM((6, 8, D), F32),
        pltpu.VMEM((NC, 8, LANES), F32),
        pltpu.VMEM((NC, S + 16, LANES), F32),
        pltpu.VMEM((S, D), F32),
        pltpu.VMEM((S, D), F32),
        pltpu.VMEM((NC, S, LANES), BF16),
        pltpu.VMEM((7, 7, FF // 4, LANES), BF16),
        pltpu.VMEM((7, 7, NS, D // 4, LANES), BF16),
        pltpu.VMEM((7, 2, D // 4, LANES), BF16),
        [pltpu.VMEM((2, GROWS, TQ), F32)] * 4,
        pltpu.VMEM((2, 4 * NC * (TQ + 8), LANES), F32),
        pltpu.VMEM((TB, LANES), BF16),
        pltpu.VMEM((10, 2, n1 // 2, LANES), BF16),
        pltpu.VMEM((10, 2, n2 // 2, LANES), BF16),
        pltpu.VMEM((7, 2, 2 * LANES, LANES), BF16),
        pltpu.VMEM((7, 2, 2 * LANES, LANES), BF16),
        pltpu.VMEM((4, FF // 4, TQ), F32),
        pltpu.VMEM((NC, 4 * NS + 2, LANES, LANES), BF16),
        pltpu.VMEM((D, LANES), F32),
        pltpu.SemaphoreType.DMA((21,)),
        pltpu.SemaphoreType.DMA((1,)),
    ]
    out = pl.pallas_call(
        functools.partial(_kernel, S=S, D=D, FF=FF),
        in_specs=[pl.BlockSpec(memory_space=pl.ANY)] * len(args),
        out_specs=pl.BlockSpec(memory_space=pl.ANY),
        out_shape=jax.ShapeDtypeStruct((S, D), BF16),
        scratch_shapes=scratch,
        compiler_params=pltpu.CompilerParams(
            vmem_limit_bytes=120 * 1024 * 1024,
            disable_bounds_checks=True,
            disable_semaphore_checks=True,
        ),
    )(*args)
    return out.reshape(B, S, D)
```

```python
import functools
import math

import jax
import jax.numpy as jnp
from jax import lax
import jax.experimental.pallas as pl
import jax.experimental.pallas.tpu as pltpu

F32 = jnp.float32
BF16 = jnp.bfloat16
U32 = jnp.uint32

LANES = 128
BLK = 128
PH = 4
EPS = 1e-05
TB = 512
TQ = TB // 4
HALO = 32
TILES = (384, 384, 576, 704)
BLOCKWISE1 = (3,)
BLOCKWISE2 = (2, 3)
IN_LOOP = (4, 2, 0, 1, 3)
ROT = 3
KR = 256
NB1 = 1
IG = 2
IJ = 6
IP = 2
GPAD = 8
GROWS = 1768

MF = (6, 0, 5, 4)
MT = (3, 0, 3, 3)
R6 = (36, 18, 28, 6)
TRS = (145, 175, 180)
FRS = (50, 90, 90)
WS = (2, 3, 3, 2, 2, 4)
FI = (48, 88, 96, 96)
LAST = (55, 66, 92, 82)
EW = (2, 1, 2)
NW = (1, 3, 0, 150, 320, 460, 600, 730)
FL = (10, 10, 25, -32)
O3 = (4, 3, 0, 6, 2, 1, 5)
J3 = (1, 2, 3, 4, 5, 6, 0)
J4 = (4, 2, 3, 1, 0, 6, 5)
ET = (0, 4)
EC = 10
YP = 128
LT = (8, 3)

_ORDER = (2, 4, 1, 3, 0, 6, 5)
_RAW = (1, 4)
_LHS = (((0, 0), 1, (1, 1)), ((1, 0), 1, (1, 1)), ((0, 0),), ((1, 1),),
        ((0, 0), 1, (0, 1)), ((1, 0), -1, (0, 0)), ((0, 1), -1, (1, 1)))
_RHS = (((0, 0), 1, (1, 1)), ((0, 0),), ((0, 1), -1, (1, 1)), ((1, 0), -1, (0, 0)),
        ((1, 1),), ((0, 0), 1, (0, 1)), ((1, 0), 1, (1, 1)))


def _operand(terms, blk):
    x = blk(*terms[0])
    if len(terms) > 1:
        y = blk(*terms[2])
        x = x + y if terms[1] > 0 else x - y
    return x


def _all_operands(table, b00, b01, b10, b11):
    blocks = ((b00, b01), (b10, b11))
    return [_operand(terms, lambda i, j: blocks[i][j]) for terms in table]


def _block(m, which):
    if which == 0:
        return (m[3] - m[4]) + m[0] + m[6]
    if which == 1:
        return m[2] + m[4]
    if which == 2:
        return m[1] + m[3]
    return (m[2] - m[1]) + m[0] + m[5]


def _combine(m):
    return [_block(m, which) for which in range(4)]


def _as_bf16(x):
    return pltpu.bitcast(x, BF16)


def _lo(x):
    return pltpu.bitcast(x << 16, F32)


def _hi(x):
    return pltpu.bitcast(x & jnp.uint32(0xFFFF0000), F32)


def _dft4(re, im, sign):
    ar, ai = re[0] + re[2], im[0] + im[2]
    br, bi = re[0] - re[2], im[0] - im[2]
    cr, ci = re[1] + re[3], im[1] + im[3]
    dr, di = re[1] - re[3], im[1] - im[3]
    o0 = (ar + cr, ai + ci)
    o2 = (ar - cr, ai - ci)
    m = (br + di, bi - dr)
    p = (br - di, bi + dr)
    o1, o3 = (m, p) if sign < 0 else (p, m)
    return [o0[0], o1[0], o2[0], o3[0]], [o0[1], o1[1], o2[1], o3[1]]


def _ln(x, eps=EPS, unit=True):
    n = x.shape[-1]
    s1 = jnp.sum(x, axis=-1, keepdims=True)
    m = s1 * (1.0 / n)
    v = jnp.maximum(jnp.sum(x * x, axis=-1, keepdims=True) + (n * eps - s1 * m), n * eps)
    e = jnp.log(v) * (-0.5 / math.log(2.0))
    return (x - m) * jnp.exp2(e + 0.5 * math.log2(n) if unit else e)


def _gelu2(x):
    c0 = math.sqrt(2.0 / math.pi)
    return x + x * jnp.tanh(x * (c0 + (c0 * 0.044715) * (x * x)))


def _dot(a, b):
    return jnp.dot(a, b, preferred_element_type=F32)


def _dot_nt(a, b):
    return lax.dot_general(a, b, (((1,), (1,)), ((), ())), preferred_element_type=F32)


def _rows8(x, repeat=1):
    return [(x, r) for r in range(x.shape[0] // 8) for _ in range(repeat)]


def _stack(tks):
    return jnp.concatenate([x[8 * r:8 * r + 8, 0:LANES] for x, r in tks], axis=0).reshape(len(tks), 8, LANES)


def _chunks(r0, r1, k, unit=16):
    n = (r1 - r0) // unit
    cuts = [r0 + unit * ((n * j) // k) for j in range(k + 1)]
    return list(zip(cuts[:-1], cuts[1:]))


def _pick(toks, n, free=0):
    idx = [(r * (len(toks) + free)) // n - free for r in range(n)]
    return [toks[i] if i >= 0 else None for i in idx]


def _kernel(q_hbm, k_hbm, v_hbm, sh_hbm, sk_hbm, sd_hbm, w1_hbm, w2_hbm, w3_hbm, w4_hbm, c_hbm, wm_hbm,
            o_hbm,
            q_v, k_v, v_v, sh_v, sk_v, sd_v, w1_v, w2_v, w3_v, w4_v, c_v, wm_v,
            fw_s, iv_s, o_v, u_s, kk_s, vv_s, wu_s, y_s, mod_s, par_s, h1_s, x_s, h_s, z_s,
            s3_s, s4_s, e4_s, g_s, zf_s, zr_s, l1_s, l2_s, s1_s, s2_s, rh_s, wt_s, scol_s, l0_s,
            sem, sem_o,
            *, S, D, FF):
    NC = D // LANES
    NG = BLK // 8
    LB = PH * BLK
    NBL = S // LB
    R = BLK // PH
    HL = LANES // 2

    small = [
        pltpu.make_async_copy(sh_hbm, sh_v, sem.at[0]),
        pltpu.make_async_copy(sd_hbm, sd_v, sem.at[0]),
        pltpu.make_async_copy(c_hbm, c_v, sem.at[0]),
    ]

    def sk_copy(c):
        ch = (c + ROT) % NC * LANES
        rows = pl.ds(ch if isinstance(c, int) else pl.multiple_of(ch, LANES), LANES)
        return [pltpu.make_async_copy(sk_hbm.at[rows, :], sk_v.at[c], sem.at[1 + c])]

    def kv_copies(tiles, lo, hi, s):
        return [pltpu.make_async_copy(src.at[pl.ds(r0, r1 - r0), pl.ds((c + ROT) % NC * LANES, LANES)],
                                      dst.at[c, pl.ds(off + r0, r1 - r0), :], sem.at[s])
                for r0, r1 in _chunks(lo, hi, (hi - lo + 16) // KR)
                for src, dst, off in ((k_hbm, k_v, 16), (v_hbm, v_v, 0)) for c in tiles]

    PAIR, TRIPLE = (0, 1), (2, 3, 4)
    kv_groups = [kv_copies(PAIR, 0, NB1 * LB + 16, 9), kv_copies(PAIR, NB1 * LB + 16, S, 10),
                 kv_copies(TRIPLE, 0, 2 * LB + 16, 11), kv_copies(TRIPLE, 2 * LB + 16, S, 20)]

    WM = (0, 3 * D, 5 * D, 6 * D)
    wm_copies = [[pltpu.make_async_copy(wm_hbm.at[:, pl.ds(WM[j], WM[j + 1] - WM[j])],
                                        wm_v.at[:, pl.ds(WM[j], WM[j + 1] - WM[j])], sem.at[6 + j])]
                 for j in range(3)]
    w_copies = [[pltpu.make_async_copy(src.at[:, pl.ds(c * LANES, LANES)], dst.at[c], sem.at[12 + j])
                 for c in range(NC)]
                for j, (src, dst) in enumerate(((w1_hbm, w1_v), (w2_hbm, w2_v), (w3_hbm, w3_v), (w4_hbm, w4_v)))]

    B0 = [0]
    for n in TILES:
        B0.append(B0[-1] + n)
    NA = len(TILES)
    A0 = [0] + [r + HALO for r in B0[1:-1]] + [S]
    q_copies = [
        [pltpu.make_async_copy(q_hbm.at[pl.ds(A0[t], A0[t + 1] - A0[t])], q_v.at[pl.ds(A0[t], A0[t + 1] - A0[t])],
                               sem.at[16 + t])]
        for t in range(NA)
    ]

    def start_all(cps, priority=0):
        for cp in cps:
            cp.start(priority=priority)

    def wait_all(cps):
        for cp in cps:
            cp.wait()

    for c in range(NC):
        k_v[c, 0:16, :] = jnp.zeros((16, LANES), BF16)
    start_all(sk_copy(0) + small + sk_copy(1) + kv_groups[0] + kv_groups[1] + sk_copy(2))

    for c in range(NC):
        h1_s[c, 0:8, :] = jnp.zeros((8, LANES), F32)
        h1_s[c, S + 8:S + 16, :] = jnp.zeros((8, LANES), F32)

    prow = lax.broadcasted_iota(jnp.int32, (BLK, BLK), 0)
    pcol = lax.broadcasted_iota(jnp.int32, (BLK, BLK), 1)
    ang = (((4 * prow + 1) * pcol) & (4 * BLK - 1)).astype(F32) * (2.0 * math.pi / (4 * BLK))
    tw = (4 * prow + 1).astype(F32) * (2.0 * math.pi / (4 * LB))
    mr, mi = jnp.cos(ang), -jnp.sin(ang)
    twr, twi = jnp.cos(tw), -jnp.sin(tw)
    eye = jnp.where(prow == pcol, 1.0 / LB, 0.0).astype(BF16)
    for i in range(PH):
        both = jnp.concatenate([mr.reshape(NG, 8, BLK), mi.reshape(NG, 8, BLK)], axis=1).reshape(2 * BLK, BLK)
        fw_s[i] = both.astype(BF16)
        for h in range(2):
            iv_s[i, h] = _dot_nt(eye, both[h * BLK:(h + 1) * BLK, :].astype(BF16)).astype(BF16)
        if i + 1 < PH:
            mr, mi = mr * twr - mi * twi, mr * twi + mi * twr
    perm = jnp.where(pcol == (prow % R) * PH + prow // R, 1.0, 0.0).astype(BF16)

    wait_all(small)
    shf = sh_v[...].astype(F32)
    sdf = sd_v[...].astype(F32).reshape(1, D)
    for c in range(NC):
        par_s[(c - ROT) % NC, 0:4, :] = shf[:, c * LANES:(c + 1) * LANES]
        par_s[(c - ROT) % NC, 4:5, :] = sdf[:, c * LANES:(c + 1) * LANES]
    cf = c_v[...].astype(F32)
    sc = (cf * jax.nn.sigmoid(cf)).astype(BF16)
    sc16 = jnp.broadcast_to(sc, (16, D))

    def mod_chunk(j):
        mod_s[j] = _dot(sc16, wm_v[:, j * D:(j + 1) * D])[0:8, :]

    (fw_u, iv_u, k_u, v_u, wu_u, vv_u, z_u, l1_u, l2_u, w1_u, w2_u, s1_u, s2_u, w3_u, w4_u, wt_u, s3_u, s4_u,
     e4_u, zr_u) = (r.bitcast(U32) for r in (fw_s, iv_s, k_v, v_v, wu_s, vv_s, z_s, l1_s, l2_s, w1_v, w2_v,
                                             s1_s, s2_s, w3_v, w4_v, wt_s, s3_s, s4_s, e4_s, zr_s))

    never = twr[0:8, :] > 2.0

    def after(token, x):
        if token.dtype != x.dtype:
            token = pltpu.bitcast(token, x.dtype)
        return jnp.where(jnp.broadcast_to(never, x.shape), token, x)

    def hold(x, tks):
        f = len([k for k in tks if k is None])
        n = len(tks)
        head = after(_stack(tks[f:]), x[8 * f:, 0:LANES].reshape(n - f, 8, LANES)).reshape(8 * (n - f), LANES)
        if f:
            head = jnp.concatenate([x[:8 * f, 0:LANES], head], axis=0)
        return head if x.shape[1] == LANES else jnp.concatenate([head, x[:, LANES:]], axis=1)

    def hold16(x, tks):
        x3 = x.reshape(len(tks), 16, LANES)
        return jnp.concatenate([after(_stack(tks), x3[:, 0:8]), x3[:, 8:16]], axis=1).reshape(x.shape)

    def perm_k(c, b, toks):
        kt = [_dot_nt(perm, sk_v[c, :, b * LB + t * BLK:b * LB + (t + 1) * BLK]) for t in range(PH)]
        toks += _rows8(kt[0])[::2]
        return [jnp.concatenate([kt[t][i * R:(i + 1) * R, :] for t in range(PH)], axis=0).astype(BF16)
                for i in range(PH)]

    def spectrum(comps, dst, slot, b, toks, dc=None, pins=None):
        tr, ti = [], []
        for i in range(PH):
            lhs = fw_u[i]
            if pins is not None and i < len(pins):
                lhs = after(pins[i], lhs.reshape(NG, 8, LANES)).reshape(BLK, LANES)
            res = _dot(_as_bf16(lhs), comps[i])
            t3 = res.reshape(NG, 16, LANES)
            tr.append(t3[:, 0:8])
            ti.append(t3[:, 8:16])
        toks += _rows8(res)[1::2]
        if dc is not None:
            tr[0] = tr[0] + dc
        sr, si = _dft4(tr, ti, -1)
        for qq in range(PH):
            dst[slot, :, b, qq, 0] = sr[qq]
            dst[slot, :, b, qq, 1] = si[qq]

    def gated(c, b, n):
        w = [par_s[c, t:t + 1, :] for t in range(4)]
        kc = {}
        for o in range(-2, 2):
            words = k_u[c, pl.ds(8 + b * (LB // 2) + o, BLK, stride=2), :]
            if o > -2:
                kc[2 * o] = _lo(words)
            kc[2 * o + 1] = _hi(words)
        vc = {}
        for o in range(2):
            words = v_u[c, pl.ds(b * (LB // 2) + o, BLK, stride=2), :]
            vc[2 * o] = _lo(words)
            vc[2 * o + 1] = _hi(words)
        for i in range(PH):
            ks = kc[i] * w[0]
            for t in range(1, 4):
                ks = ks + kc[i - t] * w[t]
            wu_s[n, i] = (ks * vc[i]).astype(BF16)
        return [wu_u[n, i] for i in range(PH)]

    def kv_pins(kvb):
        return [_stack([(kvb[2 * m + (r % 2)], r // 2) for r in range(NG)]) for m in range(2)]

    def products(c, ks, kc, toks, free, trim):
        n = len(toks) - trim + free
        cum = (44, 128, 244, 392)
        zp = None
        for o in range(NBL):
            idx = [((g * cum[-1] + cum[o]) * n) // (cum[-1] * NG) - 1 - free for g in range(NG)]
            tk = [toks[max(i, 0)] if i >= 0 or not free else None for i in idx]
            zr, zi = [], []
            for qq in range(PH):
                accr = acci = None
                for b in range(o + 1):
                    a_, b_ = u_s[c, :, b, qq, 0], u_s[c, :, b, qq, 1]
                    c_, d_ = ks[kc, :, o - b, qq, 0], ks[kc, :, o - b, qq, 1]
                    if qq == 0 and b == o:
                        a_ = hold(a_.reshape(BLK, LANES), tk).reshape(NG, 8, LANES)
                    tr_ = a_ * c_ - b_ * d_
                    ti_ = a_ * d_ + b_ * c_
                    accr = tr_ if accr is None else accr + tr_
                    acci = ti_ if acci is None else acci + ti_
                zr.append(accr)
                zi.append(acci)
            if zp is None:
                yr, yi = zr, zi
            else:
                yr = [zr[qq] - zp[1][qq] for qq in range(PH)]
                yi = [zi[qq] + zp[0][qq] for qq in range(PH)]
            zp = (zr, zi)
            vr, vi = _dft4(yr, yi, +1)
            for i in range(PH):
                vv_s[c, o, i] = jnp.concatenate([vr[i], vi[i]], axis=1).reshape(2 * BLK, LANES).astype(BF16)

    def inverse(c, o, toks, pins):
        for i in range(PH):
            yv = None
            for h in range(2):
                lhs = iv_u[i, h]
                if pins is not None and h == 0:
                    pin = pins[i % 2][8 * (i // 2):8 * (i // 2) + 8]
                    lhs = after(pin, lhs.reshape(8, 8, LANES)).reshape(HL, LANES)
                t = _dot(_as_bf16(lhs), _as_bf16(vv_u[c, o, i, h * HL:(h + 1) * HL, :]))
                yv = t if yv is None else yv + t
            if i % 2 == 0:
                toks += _rows8(yv)[::2]
            y_s[c, pl.ds(o * LB + i, BLK, stride=PH), :] = yv

    def conv_step(filt=None, units=(), mul=None, inv=(), free=0, trim=3):
        toks = []
        kv = [gated(c, b, n) for n, (c, b) in enumerate(units)]
        pin_at = {n: kv_pins(kv[n]) for n in range(len(units))} if inv or filt is not None else {}
        if filt is not None and mul is not None and not isinstance(filt, int):
            ks = kk_s.at[pl.ds(mul, 2)]
            k_rd, k_wr = (ks, 0), (ks, 1)
        else:
            k_rd, k_wr = (kk_s, mul), (kk_s, filt)
        pos = 0
        for c, o in inv:
            inverse(c, o, toks, pin_at.get(pos))
            pos += 1
        if filt is not None:
            comps = [perm_k(filt, b, toks) for b in range(NBL)]
            for b in range(NBL):
                spectrum(comps[b], *k_wr, b, toks, par_s[filt, 4:5, :] if b == 0 else None, pin_at.get(pos))
                pos += 1
        for n, (c, b) in enumerate(units):
            spectrum([_as_bf16(x) for x in kv[n]], u_s, c, b, toks, None, pin_at.get(pos))
            pos += 1
        if mul is not None:
            products(mul, *k_rd, toks, free, trim)
        return toks

    def lane_tiles(x):
        return [x[:, c * LANES:(c + 1) * LANES] for c in range(NC)]

    def stage_p1(r0, r1, tks=None, ytks=None):
        ga = mod_s[2, 0:1, :]
        a_mul, a_add = ga * (1.0 + mod_s[1, 0:1, :]) * math.sqrt(D), ga * mod_s[0, 0:1, :]
        q = q_v[r0:r1, :].astype(F32)
        if tks is not None:
            q = hold(q, tks)
        y = jnp.concatenate([y_s[(c - ROT) % NC, r0:r1, :] for c in range(NC)], axis=1)
        if ytks is not None:
            y = hold(y, ytks)
        x = q + (_ln(q, unit=False) * a_mul + a_add) * y
        x_s[r0:r1, :] = x
        return _ln(x, unit=False)

    def store_row_ops(dst, base, r0, r1, cols, tks=None, only=range(10)):
        hv = []
        for x in cols:
            x3 = x.reshape(x.shape[0] // 32, 32, LANES)
            hv.append([x3[:, 16 * e:16 * e + 16].reshape(x.shape[0] // 2, LANES) for e in range(2)])
        for k2 in range(2):
            a00, a01, a10, a11 = hv[k2][0], hv[2 + k2][0], hv[k2][1], hv[2 + k2][1]
            if tks is not None:
                a00, a11 = hold16(a00, tks), hold16(a11, tks)
            for o, x in enumerate(_all_operands(_LHS, a00, a01, a10, a11) + [a01, a10, hv[NC - 1][k2]]):
                if o in only:
                    dst[o, k2, (r0 - base) // 2:(r1 - base) // 2, :] = x.astype(BF16)

    L1B = A0[BLOCKWISE1[0]]
    L2B = B0[BLOCKWISE2[0]]

    def stage_p2(r0, r1, nx, blockwise=False):
        h = nx * ((1.0 + mod_s[4, 0:1, :]) * (2.0 * math.sqrt(D))) + 2.0 * mod_s[3, 0:1, :]
        h_s[r0:r1, :] = h
        zn = lane_tiles(_ln(h, 4.0 * EPS))
        if blockwise:
            store_row_ops(l1_s, L1B, r0, r1, zn)
        else:
            for c in range(NC):
                z_s[c, r0:r1, :] = zn[c].astype(BF16)

    def stage_p(t, toks):
        lo, hi = A0[t], A0[t + 1]
        stage_p2(lo, hi, stage_p1(lo, hi, _pick(toks[:-TRS[t - 1]], (hi - lo) // 8, FRS[t - 1])), t in BLOCKWISE1)

    def filler(t):
        red = jnp.sum(y_s[t, 0:8 * FI[t], :], axis=-1, keepdims=True).reshape(FI[t], 8, 1)
        spare = (NC - 1) * (TQ + 8) + 8 * t
        zf_s[1, spare:spare + 8, :] = jnp.broadcast_to(jnp.sum(red, axis=0), (8, LANES))

    def square_ops(src, dst, toks):
        HK = 2 * LANES
        for n2 in range(2):
            blk = lambda k, n: src[2 * n + n2, k * HK:(k + 1) * HK, :].astype(F32)
            tk = _pick(toks, 2 * HK // 16)[n2 * (HK // 16):(n2 + 1) * (HK // 16)]
            b00, b11 = hold16(blk(0, 0), tk), hold16(blk(1, 1), tk)
            for o, x in enumerate(_all_operands(_RHS, b00, blk(0, 1), blk(1, 0), b11)):
                if o not in _RAW:
                    dst[o, n2] = x.astype(BF16)

    def block_dots(ops_u, base, prepare, w_u, s_u, parts, emit, light, heavy, first=False):
        toks = []

        def timed(x, weight):
            toks.extend(_rows8(x, weight))
            return x

        def weave(top, bot):
            n = top.shape[0] // 16
            return jnp.concatenate([top.reshape(n, 16, LANES), bot.reshape(n, 16, LANES)], axis=1).reshape(32 * n, LANES)

        def main(get):
            m = [None] * 7
            rem = [None, None]
            for o in (('t', 'b', 4, 1, 2, 3, 0, 6, 5) if first else ('t', 2, 4, 'b', 1, 3, 0, 6, 5)):
                if o in ('t', 'b'):
                    e = 0 if o == 't' else 1
                    rhs = jnp.concatenate([w_u[c, 2 * LANES:D // 2, :] for c in range(NC - 1)], axis=1)
                    rem[e] = timed(_dot(get([(9, e)]), _as_bf16(rhs)), light)
                    continue
                if o in _RAW:
                    d = _RAW.index(o)
                    rhs = jnp.concatenate([w_u[2 * d + n2, d * LANES:(d + 1) * LANES, :] for n2 in range(2)], axis=1)
                else:
                    rhs = jnp.concatenate([s_u[o, n2] for n2 in range(2)], axis=1)
                m[o] = timed(_dot(get([(o, 0), (o, 1)]), rhs if rhs.dtype == BF16 else _as_bf16(rhs)), heavy if o in (4, 3, 6, 5) else light)
            c00, c01, c10, c11 = _combine(m)
            top = jnp.concatenate([c00, c01], axis=1) + rem[0]
            bot = jnp.concatenate([c10, c11], axis=1) + rem[1]
            return [weave(top[:, c * LANES:(c + 1) * LANES], bot[:, c * LANES:(c + 1) * LANES]) for c in range(NC - 1)]

        def last(get):
            w = _as_bf16(w_u[NC - 1])
            return weave(timed(_dot(get([(2, 0), (2, 1), (7, 0), (7, 1), (9, 0)]), w), light),
                         timed(_dot(get([(8, 0), (8, 1), (3, 0), (3, 1), (9, 1)]), w), light))

        if first:
            raw = {2: (0, 0), 7: (2, 0), 8: (0, 1), 3: (2, 1)}
            gets = []
            for r0, r1 in parts:
                def get(keys, r0=r0, r1=r1):
                    out = []
                    for o, e in keys:
                        if o in raw or o == 9:
                            c, half = (NC - 1, e) if o == 9 else (raw[o][0] + e, raw[o][1])
                            w3d = z_u[c, r0 // 2:r1 // 2, :].reshape((r1 - r0) // 32, 16, LANES)
                            out.append(w3d[:, 8 * half:8 * half + 8].reshape((r1 - r0) // 4, LANES))
                        else:
                            out.append(l0_s[o, e, r0 // 2:r1 // 2, :])
                    out = jnp.concatenate(out, axis=1)
                    return out if out.dtype == BF16 else _as_bf16(out)
                gets.append(get)
            tails = [last(get) for get in gets]
            prepare(toks)
            for (r0, r1), get, tail in zip(parts, gets, tails):
                emit(r0, r1, main(get) + [tail])
            return toks
        mark = None
        for j, (r0, r1) in enumerate(parts):
            prepare(r0, r1, None if mark is None else toks[mark:])
            mark = len(toks)
            get = lambda keys: _as_bf16(jnp.concatenate(
                [ops_u[o, e, (r0 - base) // 4:(r1 - base) // 4, :] for o, e in keys], axis=1))
            if j % 2:
                tail = last(get)
                emit(r0, r1, main(get) + [tail])
            else:
                emit(r0, r1, main(get) + [last(get)])
        return toks

    def stage_m1(t, k):
        def emit(r0, r1, cols):
            out = [_gelu2(x) for x in cols]
            for c in range(NC):
                h1_s[c, r0 + 8:r1 + 8, :] = out[c]
            return out

        if t == 0:
            def prepare(toks):
                square_ops(w1_v, s1_s, toks)
                store_row_ops(l0_s, 0, 0, A0[1], [z_s[c, 0:A0[1], :].astype(F32) for c in range(NC)],
                              _pick(toks, A0[1] // 32), (0, 1, 4, 5, 6))
            return block_dots(None, 0, prepare, w1_u, s1_s, _chunks(0, A0[1], k, 32), emit, 1, 1, True)
        if t in BLOCKWISE1:
            return block_dots(l1_u, L1B, lambda *_: None, w1_u, s1_u, _chunks(A0[t], A0[t + 1], k, 32), emit, WS[2], WS[3])
        toks = []
        for r0, r1 in _chunks(A0[t], A0[t + 1], k):
            lhs = jnp.concatenate([z_u[c, r0 // 2:r1 // 2, :] for c in range(NC)], axis=1)
            w = jnp.concatenate([w1_u[c] for c in range(NC)], axis=1)
            for x in emit(r0, r1, lane_tiles(_dot(_as_bf16(lhs), _as_bf16(w)))):
                toks += _rows8(x, WS[0])
        return toks

    def shifted(r0, r1):
        n, grp, shifts = r1 - r0, D // 4, (-1, 1, -2, 2)
        lane = lax.broadcasted_iota(jnp.int32, (n, LANES), 1)
        cols = []
        for c in range(NC):
            lo, hi = c * LANES, (c + 1) * LANES
            g_lo, g_hi = lo // grp, (hi - 1) // grp
            val = h1_s[c, pl.ds(r0 + 8 + shifts[g_lo], n), :]
            if g_hi != g_lo:
                other = h1_s[c, pl.ds(r0 + 8 + shifts[g_hi], n), :]
                val = jnp.where(lane < (g_hi * grp - lo), val, other)
            cols.append(val)
        return cols

    def stage_m2(t, k, before=None):
        def emit(r0, r1, cols):
            x1 = h_s[r0:r1, :] + jnp.concatenate(cols, axis=1)
            h_s[r0:r1, :] = x1
            return x1

        if t in BLOCKWISE2:
            def prepare(r0, r1, prev):
                prev = before if prev is None else prev
                prev = prev[len(prev) // 8:(len(prev) * 7) // 8]
                store_row_ops(l2_s, L2B, r0, r1, shifted(r0, r1), _pick(prev, (r1 - r0) // 32))
            return block_dots(l2_u, L2B, prepare, w2_u, s2_u, _chunks(B0[t], B0[t + 1], k, 32), emit, WS[4], WS[4])
        toks = []
        for r0, r1 in _chunks(B0[t], B0[t + 1], k):
            w = jnp.concatenate([w2_u[c] for c in range(NC)], axis=1)
            hs = _dot(jnp.concatenate(shifted(r0, r1), axis=1).astype(BF16), _as_bf16(w))
            for x in lane_tiles(emit(r0, r1, [hs])):
                toks += _rows8(x, WS[1])
        return toks

    NT = S // TB
    FQ = FF // 4
    NS = FQ // LANES
    LQ = FQ - NS * LANES
    CQ = LANES // 4
    QR = LANES + CQ
    BLOCKS = [(2 * r1 + r2, 2 * h + p)
              for r1, h in ((0, 0), (1, 0), (0, 1), (1, 1)) for r2 in range(2) for p in range(2)]

    def z_rows(rq, c):
        lo = (NC * rq + c) * (TQ + 8)
        return slice(lo, lo + TQ)

    def store_z(r0, slot, toks, q0=0, q1=4):
        n = (q1 - q0) * TQ
        rows = pl.ds(r0 + q0 * TQ if isinstance(r0, int) else pl.multiple_of(r0 + q0 * TQ, TQ), n)
        zn = lane_tiles(_ln(hold(h_s[rows, :], _pick(toks, n // 8)), 4.0 * EPS))
        for rq in range(q0, q1):
            for c in range(NC - 1):
                zf_s[slot, z_rows(rq, c), :] = zn[c][(rq - q0) * TQ:(rq - q0 + 1) * TQ]
        zr_s[q0 * TQ:q1 * TQ, :] = zn[NC - 1].astype(BF16)

    def w3_ops(toks):
        ng = FQ // 16
        blk = lambda c, d: w3_v[c, d * FQ:(d + 1) * FQ, :].astype(F32)
        outer = [[_all_operands(_RHS, blk(k2, p), blk(k2, 2 + p), blk(2 + k2, p), blk(2 + k2, 2 + p))
                  for p in range(2)] for k2 in range(2)]
        for k, i in enumerate((1, 5, 2, 4, 0, 3, 6)):
            tk = [toks[((k + r * 7) * len(toks)) // (7 * ng)] for r in range(ng)]
            for j, x in enumerate(_all_operands(_RHS, hold16(outer[0][0][i], tk), outer[0][1][i], outer[1][0][i],
                                                hold16(outer[1][1][i], tk))):
                if i not in _RAW or j not in _RAW:
                    s3_s[i, j] = x.astype(BF16)

    def transpose_w4(toks):
        order = [(c, n) for n in (4 * NS, 4 * NS + 1) + tuple(range(4 * NS)) for c in range(NC)]
        for k, (c, n) in enumerate(order):
            if n >= 4 * NS:
                ends = [(2 * (n - 4 * NS) + p + 1) * FQ // 2 for p in range(2)]
                x = jnp.concatenate([w4_u[c, e - LQ // 2:e, :] for e in ends]
                                    + [jnp.zeros((HL - LQ, LANES), U32)], axis=0)
            else:
                lo = (n % 4) * FQ // 2 + (n // 4) * HL
                x = w4_u[c, lo:lo + HL, :]
            x = jnp.concatenate([hold(x[0:8], [toks[(k * len(toks)) // len(order)]]), x[8:]], axis=0)
            wt_s[c, n] = _as_bf16(x).astype(F32).T.astype(BF16)

    def w4_ops(i, zero, toks):
        ng = QR // 16
        total = (NS * 7 + 2) * ng
        tk = lambda pos, step: [toks[((pos + r * step) * len(toks)) // total] for r in range(ng)]
        quarter = lambda n, d: jnp.concatenate(
            [wt_s[d, n].astype(F32), wt_s[NC - 1, n, d * CQ:(d + 1) * CQ, :].astype(F32)], axis=0)
        if i not in _RAW:
            for e in range(2):
                x = _operand(_RHS[i], lambda h, d: quarter(4 * NS + h, 2 * d + e))
                e4_s[i + zero, e] = hold16(x, tk(e * ng, 1)).astype(BF16)
        for st in range(NS):
            t = [[_operand(_RHS[i], lambda h, d: quarter(4 * st + 2 * h + p, 2 * d + e)) for e in range(2)]
                 for p in range(2)]
            tks = tk((2 + st * 7) * ng, 7)
            for j, x in enumerate(_all_operands(_RHS, hold16(t[0][0], tks), t[0][1], t[1][0], hold16(t[1][1], tks))):
                if i not in _RAW or j not in _RAW:
                    s4_s[i + zero, j, st] = x.astype(BF16)

    def gate_row(toks):
        ng = D // 8
        col = hold(scol_s[...], _pick(toks, ng))
        for c in range(NC):
            prod = col * wm_v[:, (NC * NC + c) * LANES:(NC * NC + c + 1) * LANES].astype(F32)
            acc = prod[0:8]
            for r in range(1, ng):
                acc = acc + prod[8 * r:8 * r + 8]
            mod_s[NC, :, c * LANES:(c + 1) * LANES] = jnp.broadcast_to(jnp.sum(acc, axis=0, keepdims=True), (8, LANES))

    def rem3(rq, d, pieces=1):
        z = _as_bf16(zr_u[rq * (TQ // 2):(rq + 1) * (TQ // 2), :])
        return jnp.concatenate([_dot_nt(_as_bf16(w3_u[NC - 1, lo // 2:hi // 2, :]), z)
                                for lo, hi in _chunks(d * FQ, (d + 1) * FQ, pieces)], axis=0)

    def lead_in():
        head = [rem3(*key) for key in BLOCKS[:4]]
        for k in range(4):
            rh_s[k] = head[k]
        return _rows8(head[0])

    def units(tiles, blocks):
        return [(c, b) for b in blocks for c in tiles]

    with jax.named_scope("A"):
        wait_all(sk_copy(0))
        conv_step(filt=0)
    with jax.named_scope("B_wait"):
        wait_all(sk_copy(1) + kv_groups[0])
    with jax.named_scope("B"):
        start_all(kv_groups[2] + kv_groups[3] + sk_copy(3) + sk_copy(4))
        conv_step(filt=1, units=units(PAIR, range(0, NB1)))
        scol_s[...] = jnp.broadcast_to(sc.astype(F32), (LANES, D)).T
    with jax.named_scope("C_wait"):
        wait_all(kv_groups[1])
    with jax.named_scope("C"):
        conv_step(units=units(PAIR, range(NB1, NBL)))
    with jax.named_scope("D_wait"):
        wait_all(sk_copy(2))
    with jax.named_scope("D"):
        start_all(wm_copies[0] + q_copies[0] + wm_copies[1] + w_copies[0])
        conv_step(filt=2, mul=0, free=MF[0], trim=MT[0])
    with jax.named_scope("E_wait"):
        wait_all(kv_groups[2])
    with jax.named_scope("E"):
        conv_step(units=units(TRIPLE, range(0, 2)), mul=1, inv=units((0,), range(NBL)), free=MF[1], trim=MT[1])
    with jax.named_scope("F_wait"):
        wait_all(kv_groups[3])
    with jax.named_scope("F"):
        conv_step(units=units(TRIPLE, range(2, NBL)))

    def full_step(j, carry):
        wait_all(sk_copy(j + 2))
        conv_step(filt=j + 2, mul=j + 1, inv=units((j,), range(IG)), free=MF[2], trim=MT[2])
        return carry

    with jax.named_scope("GH"):
        lax.fori_loop(1, NC - 2, full_step, 0)
    late = units((NC - 2,), range(NBL)) + units(range(1, NC - 2), range(IG, NBL))
    late = late[:IJ] + units((NC - 1,), range(NBL)) + late[IJ:]
    with jax.named_scope("J"):
        start_all(q_copies[1] + w_copies[1])
        start_all(sum(q_copies[2:], []) + w_copies[2] + w_copies[3] + wm_copies[2], 1)
        conv_step(mul=NC - 1, inv=late[:IJ], free=MF[3], trim=MT[3])
    with jax.named_scope("r6_wait"):
        wait_all(wm_copies[0] + q_copies[0])
    with jax.named_scope("r6"):
        for j in range(3):
            mod_chunk(j)
        conv_step(inv=late[IJ:IJ + 1])
        toks = conv_step(inv=late[IJ + 1:len(late) - IP])
        nx0 = stage_p1(0, A0[1], None, _pick(toks[:R6[0]], A0[1] // 8, R6[1]) if toks else None)
    with jax.named_scope("p2_wait"):
        wait_all(wm_copies[1])
    with jax.named_scope("p2"):
        mod_chunk(4)
        mod_chunk(3)
        toks = conv_step(inv=late[len(late) - IP:])
        if toks:
            nx0 = hold(nx0, _pick(toks[:R6[2]], A0[1] // 8, R6[3]))
        stage_p2(0, A0[1], nx0)
    with jax.named_scope("w1_wait"):
        wait_all(w_copies[0])
    with jax.named_scope("m1_0"):
        stage_m1(0, 2)
    with jax.named_scope("w2_wait"):
        wait_all(q_copies[1] + w_copies[1])
    with jax.named_scope("m2_0"):
        stage_p(1, stage_m2(0, 4))
        filler(0)
    for t in range(1, NA):
        with jax.named_scope("a%d" % t):
            wait_all(q_copies[t + 1] if t + 1 < NA else w_copies[2] + w_copies[3] + wm_copies[2])
            toks = stage_m1(t, 2)
            toks = toks + stage_m2(t, 2, toks[len(toks) - len(toks) // 2:])
            if t + 1 < NA:
                stage_p(t + 1, toks)
            if t == 1:
                square_ops(w2_v, s2_s, toks[:-30])
            if t == NA - 1:
                transpose_w4(toks[:(len(toks) * LAST[0]) // 100])
                store_z(0, 0, toks[(len(toks) * LAST[1]) // 100:(len(toks) * LAST[2]) // 100])
                toks = toks + [x for x in lead_in()[:40] for _ in range(WS[5])]
                cut = (len(toks) * LAST[3]) // 100
                gate_row(toks[:(len(toks) * 9) // 10])
                w3_ops(toks[:cut])
                rest = [i for i in range(7) if i not in IN_LOOP]
                for k, i in enumerate(rest):
                    w4_ops(i, 0, toks[cut + k::len(rest)])
            filler(t)

    def out_copy(r0, n, c):
        rows = pl.ds(r0, n)
        return pltpu.make_async_copy(o_v.at[c, rows, :], o_hbm.at[rows, pl.ds(c * LANES, LANES)], sem_o.at[0])

    def raw4(n, d):
        return jnp.concatenate([wt_u[d, n], wt_u[NC - 1, n, d * (CQ // 2):(d + 1) * (CQ // 2), :]], axis=0)

    def mlp_tile(t, carry):
        r0 = pl.multiple_of(t * TB, TB)
        ws = t & 1
        count = [0]

        def fresh():
            count[0] += 1
            return lax.rem(t + 2 * count[0], 2)

        def g_rows(r2, p, lo, hi):
            base = (2 * r2 + p) * (FQ + GPAD)
            return slice(base + lo, base + hi)

        rem = {key: rh_s[k] for k, key in enumerate(BLOCKS[:4])}
        for key in BLOCKS[4:8]:
            rem[key] = rem3(*key)
        early = _rows8(rem[BLOCKS[4]], EW[0])
        rem[BLOCKS[8]] = rem3(*BLOCKS[8], pieces=4)
        todo = BLOCKS[9:]
        part = [None] * 7
        for i in O3:
            m = [None] * 7
            for j in J3:
                slot = fresh()
                act = _operand(_LHS[j], lambda r2, k2: _operand(
                    _LHS[i], lambda r1, k1: zf_s[slot, z_rows(2 * r1 + r2, 2 * k1 + k2), :])).astype(BF16)
                if i in _RAW and j in _RAW:
                    d = 2 * _RAW.index(i) + _RAW.index(j)
                    wij = w3_u[d, d * (FQ // 2):(d + 1) * (FQ // 2), :]
                else:
                    wij = s3_u[i, j]
                m[j] = _dot_nt(_as_bf16(wij), act)
            key = todo.pop(0)
            rem[key] = rem3(*key)
            part[i] = _combine(m)
            if i in (4, 3, 0):
                early += _rows8(m[J3[ET[0]]], EW[1]) + _rows8(rem[key] if ET[1] == 7 else m[J3[ET[1]]], EW[2])
        zero = fresh() - ws
        fine = [x for x in early for _ in IN_LOOP]
        fine = fine[:len(fine) - EC * len(IN_LOOP)]
        hop = len(fine) // (len(IN_LOOP) * 33)
        for k, i in enumerate(IN_LOOP):
            w4_ops(i, zero, fine[k * hop:len(fine) - (len(IN_LOOP) - k) * hop])
        for inner in range(4):
            r2, p = inner // 2, inner % 2
            for blk, pre in enumerate(_combine([part[i][inner] for i in range(7)])):
                g_s[blk][ws, g_rows(r2, p, 0, FQ), :] = _gelu2(pre + rem[2 * (blk // 2) + r2, 2 * (blk % 2) + p])

        toks = []
        marks = {}
        part = [[None] * 4 for _ in range(7)]
        for i in _ORDER:
            slot = fresh()
            we = jnp.concatenate([raw4(4 * NS + _RAW.index(i), 2 * _RAW.index(i) + e) if i in _RAW else e4_u[i, e]
                                  for e in range(2)], axis=0)
            ex = []
            for r2 in range(2):
                act = [_operand(_LHS[i], lambda r1, h: g_s[2 * r1 + h][slot, g_rows(r2, p, NS * LANES, FQ), :])
                       for p in range(2)]
                act = jnp.concatenate(act + [jnp.zeros((LANES - 2 * LQ, TQ), F32)], axis=0).astype(BF16)
                ex.append(_dot(_as_bf16(we), act))
            m = [None] * 7
            for j in J4:
                slot = fresh()
                act = _operand(_LHS[j], lambda r2, p: _operand(
                    _LHS[i], lambda r1, h: g_s[2 * r1 + h][slot, g_rows(r2, p, 0, NS * LANES), :])).astype(BF16)
                if i in _RAW and j in _RAW:
                    d = 2 * _RAW.index(i) + _RAW.index(j)
                    wij = [raw4(4 * st + d, d) for st in range(NS)]
                else:
                    wij = [s4_u[i, j, st] for st in range(NS)]
                m[j] = _dot(_as_bf16(jnp.concatenate(wij, axis=1)), act)
                toks += _rows8(m[j])
            part[i] = [x + ex[inner // 2][(inner % 2) * QR:(inner % 2 + 1) * QR]
                       for inner, x in enumerate(_combine(m))]
            marks[i] = len(toks)

        gb = 0.5 * mod_s[NC, 0:1, :]
        nxt = jnp.minimum(t + 1, NT - 1) * TB
        tails = {}
        for i, blk, norm in ((4, 1, (0, NW[0]) + NW[2:4]), (3, 2, NW[0:2] + NW[4:6]), (6, 0, (NW[1], 4) + NW[6:8]),
                             (5, 3, None)):
            r1 = blk // 2
            if norm is None:
                toks += [x for x in lead_in()[LT[0]:] for _ in range(LT[1])]
            else:
                store_z(nxt, 1 - ws, toks[norm[2]:norm[3]], norm[0], norm[1])
            pos = [marks[i] + FL[(1, 2, 0, 3).index(blk)]]

            def finish(rq, c, h2t):
                h2 = hold(h2t.T, toks[pos[0]:pos[0] + TQ // 8])
                pos[0] += TQ // 8
                rows = pl.ds(pl.multiple_of(r0 + rq * TQ, TQ), TQ)
                cols = slice(c * LANES, (c + 1) * LANES)
                o_v[c, rows, :] = (x_s[rows, cols] + gb[:, cols] * (h_s[rows, cols] + h2)).astype(BF16)
                if blk == 3:
                    out_copy(rows.start, TQ, c).start()

            for inner in (1, 2, 0, 3):
                ht = _block([part[k][inner] for k in range(7)], blk)
                rq, c = 2 * r1 + inner // 2, 2 * (blk % 2) + inner % 2
                finish(rq, c, ht[0:LANES])
                tails[rq, c] = ht[LANES:]
            rb = pl.multiple_of(r0 + r1 * 2 * TQ, 2 * TQ)
            if blk != 3:
                for e in range(2):
                    out_copy(rb, 2 * TQ, 2 * (blk % 2) + e).start()
            if blk in (0, 3):
                for rq in (2 * r1, 2 * r1 + 1):
                    finish(rq, NC - 1, jnp.concatenate([tails[rq, c] for c in range(NC - 1)], axis=0))
                if blk == 0:
                    out_copy(rb, 2 * TQ, NC - 1).start()
        return carry

    with jax.named_scope("ph2b"):
        lax.fori_loop(0, NT, mlp_tile, 0)
    with jax.named_scope("tail"):
        pltpu.make_async_copy(o_v, o_v, sem_o.at[0]).wait()


@jax.jit
def pallas_adaLN_cond__ssm_conv_h3__mixer_s_mlp__prompt_kernel(
    A_q: jax.Array,
    A_k: jax.Array,
    A_v: jax.Array,
    A_shift_k: jax.Array,
    A_ssm_k: jax.Array,
    A_ssm_D: jax.Array,
    B_x: jax.Array,
    B_w1: jax.Array,
    B_w2: jax.Array,
    B_w3: jax.Array,
    B_w4: jax.Array,
    c: jax.Array,
    w_mod: jax.Array,
):
    B, S, D = A_q.shape
    FF = B_w3.shape[1]
    assert (B, S, D, FF, A_shift_k.shape[1]) == (1, sum(TILES), 5 * LANES, 1728, 4)
    NC = D // LANES
    NG = BLK // 8
    NBL = S // (PH * BLK)
    NS = FF // 4 // LANES
    n1 = S - sum(TILES[:BLOCKWISE1[0]]) - HALO
    n2 = S - sum(TILES[:BLOCKWISE2[0]])

    args = (A_q.reshape(S, D), A_k.reshape(S, D), A_v.reshape(S, D), A_shift_k.T, A_ssm_k,
            A_ssm_D, B_w1, B_w2, B_w3.T, B_w4, c, w_mod)
    scratch = [
        pltpu.VMEM((S, D), BF16),
        pltpu.VMEM((NC, S + 16 + 2 * YP, LANES), BF16),
        pltpu.VMEM((NC, S + 2 * YP, LANES), BF16),
        pltpu.VMEM((4, D), BF16),
        pltpu.VMEM((NC, LANES, S), BF16),
        pltpu.VMEM((D,), BF16),
        pltpu.VMEM((NC, D, LANES), BF16),
        pltpu.VMEM((NC, D, LANES), BF16),
        pltpu.VMEM((NC, FF, LANES), BF16),
        pltpu.VMEM((NC, FF, LANES), BF16),
        pltpu.VMEM((1, D), BF16),
        pltpu.VMEM((D, 6 * D), BF16),
        pltpu.VMEM((PH, 2 * BLK, BLK), BF16),
        pltpu.VMEM((PH, 2, BLK, BLK), BF16),
        pltpu.VMEM((NC, S, LANES), BF16),
        pltpu.VMEM((NC, NG, NBL, PH, 2, 8, LANES), F32),
        pltpu.VMEM((NC, NG, NBL, PH, 2, 8, LANES), F32),
        pltpu.VMEM((NC, NBL, PH, 2 * BLK, LANES), BF16),
        pltpu.VMEM((6, PH, BLK, LANES), BF16),
        pltpu.VMEM((NC, S + YP, LANES), F32),
        pltpu.VMEM((6, 8, D), F32),
        pltpu.VMEM((NC, 8, LANES), F32),
        pltpu.VMEM((NC, S + 16, LANES), F32),
        pltpu.VMEM((S, D), F32),
        pltpu.VMEM((S, D), F32),
        pltpu.VMEM((NC, S, LANES), BF16),
        pltpu.VMEM((7, 7, FF // 4, LANES), BF16),
        pltpu.VMEM((7, 7, NS, D // 4, LANES), BF16),
        pltpu.VMEM((7, 2, D // 4, LANES), BF16),
        [pltpu.VMEM((2, GROWS, TQ), F32)] * 4,
        pltpu.VMEM((2, 4 * NC * (TQ + 8), LANES), F32),
        pltpu.VMEM((TB, LANES), BF16),
        pltpu.VMEM((10, 2, n1 // 2, LANES), BF16),
        pltpu.VMEM((10, 2, n2 // 2, LANES), BF16),
        pltpu.VMEM((7, 2, 2 * LANES, LANES), BF16),
        pltpu.VMEM((7, 2, 2 * LANES, LANES), BF16),
        pltpu.VMEM((4, FF // 4, TQ), F32),
        pltpu.VMEM((NC, 4 * NS + 2, LANES, LANES), BF16),
        pltpu.VMEM((D, LANES), F32),
        pltpu.VMEM((8, 2, 2 * LANES, LANES), BF16),
        pltpu.SemaphoreType.DMA((21,)),
        pltpu.SemaphoreType.DMA((1,)),
    ]
    out = pl.pallas_call(
        functools.partial(_kernel, S=S, D=D, FF=FF),
        in_specs=[pl.BlockSpec(memory_space=pl.ANY)] * len(args),
        out_specs=pl.BlockSpec(memory_space=pl.ANY),
        out_shape=jax.ShapeDtypeStruct((S, D), BF16),
        scratch_shapes=scratch,
        compiler_params=pltpu.CompilerParams(
            vmem_limit_bytes=120 * 1024 * 1024,
            disable_bounds_checks=True,
            disable_semaphore_checks=True,
        ),
    )(*args)
    return out.reshape(B, S, D)
```
